```python
import jax
import jax.numpy as jnp

def _softmax(x, axis=-1):
    return jax.nn.softmax(x, axis=axis)
def _gelu(x):
    return jax.nn.gelu(x, approximate=True)
def _silu(x):
    return jax.nn.silu(x)
def _sigmoid(x):
    return jax.nn.sigmoid(x)
def _layernorm(x, axis=-1, eps=1e-5):
    m = jnp.mean(x, axis=axis, keepdims=True)
    v = jnp.var(x, axis=axis, keepdims=True)
    return (x - m) / jnp.sqrt(v + eps)
def _scatter_add(tgt, idx, src, axis=0):
    return tgt.at[idx].add(src)
def _segment_sum(src, seg, n):
    return jax.ops.segment_sum(src, seg, n)
class _Rng:
    def __init__(self, key):
        self._k = key
    def _next(self):
        self._k, sub = jax.random.split(self._k)
        return sub
    def normal(self, shape):
        return jax.random.normal(self._next(), shape, dtype=jnp.bfloat16)
    def randint(self, lo, hi, shape):
        return jax.random.randint(self._next(), shape, lo, hi, dtype=jnp.int32)
    def uniform(self, shape, lo=0.0, hi=1.0):
        return jax.random.uniform(self._next(), shape, jnp.bfloat16, lo, hi)
    def permutation(self, n):
        return jax.random.permutation(self._next(), n)


kernel_name = 'gated_mix__compressed_kv_cla__sliding_local_dilated__prompt'

def setup_inputs():
    _rng = _Rng(jax.random.key(int.from_bytes(__import__("os").urandom(4), "little")))
    _w = (lambda a: (lambda t: t.astype(jnp.bfloat16) if jnp.issubdtype(t.dtype, jnp.floating) else t)(jnp.asarray(a)))
    def _A_setup():
        B, H, Sq, Sk, D, M = 1, 32, 2048, 2048, 128, 1024
        Dc = 4 * D
        return {
            "x": _w((lambda *s: _rng.normal(s) * 0.05)(B, Sq, M)),
            "c_kv": _w((lambda *s: _rng.normal(s) * 0.05)(B, Sk, Dc)),
            "w_q": _w((lambda *s: _rng.normal(s) * 0.05)(M, H, D) * (M ** -0.5)),
            "w_uk": _w((lambda *s: _rng.normal(s) * 0.05)(Dc, H, D) * (Dc ** -0.5)),
            "w_uv": _w((lambda *s: _rng.normal(s) * 0.05)(Dc, H, D) * (Dc ** -0.5)),
            "w_o": _w((lambda *s: _rng.normal(s) * 0.05)(H, D, M) * ((H * D) ** -0.5)),
        }
    _A_in = _A_setup()

    def _B_setup():
        B, S, D = 1, 2048, 1024
        return {
            "x": _w((lambda *s: _rng.normal(s) * 0.05)(B, S, D)),
            "wqkv": _w((lambda *s: _rng.normal(s) * 0.05)(D, 3 * D)),
            "wo": _w((lambda *s: _rng.normal(s) * 0.05)(D, D)),
        }
    _B_in = _B_setup()

    return {
        "A_x": _A_in["x"],
        "A_c_kv": _A_in["c_kv"],
        "A_w_q": _A_in["w_q"],
        "A_w_uk": _A_in["w_uk"],
        "A_w_uv": _A_in["w_uv"],
        "A_w_o": _A_in["w_o"],
        "B_x": _B_in["x"],
        "B_wqkv": _B_in["wqkv"],
        "B_wo": _B_in["wo"],
        "gate_w": _w((lambda *s: _rng.normal(s) * 0.05)(1024)),
    }

def reference(A_x, A_c_kv, A_w_q, A_w_uk, A_w_uv, A_w_o, B_x, B_wqkv, B_wo, gate_w):
    def _A_ref(x, c_kv, w_q, w_uk, w_uv, w_o):
        B, Sq, M = x.shape[0], x.shape[1], x.shape[2]
        Sk = c_kv.shape[1]
        H, D = w_q.shape[1], w_q.shape[2]
        q = jnp.einsum("bqm,mhd->bhqd", x, w_q)
        k = jnp.einsum("bkc,chd->bhkd", c_kv, w_uk)
        v = jnp.einsum("bkc,chd->bhkd", c_kv, w_uv)
        scores = jnp.einsum("bhqd,bhkd->bhqk", q, k) * (D ** -0.5)
        off = Sk - Sq
        qi = jnp.arange(Sq)[:, None]
        kj = jnp.arange(Sk)[None, :]
        cmask = kj <= (qi + off)
        scores = jnp.where(cmask[None, None], scores, -1e9)
        p = _softmax(scores, axis=-1)
        ctx = jnp.einsum("bhqk,bhkd->bhqd", p, v)
        return jnp.einsum("bhqd,hdm->bqm", ctx, w_o)

    def _B_ref(x, wqkv, wo):
        B, S, D = x.shape
        H = 32; Dh = D // H
        W, dil = 8, 2
        qkv = (lambda x, *d: x.transpose(*d))((x @ wqkv).reshape(B, S, 3, H, Dh), 2, 0, 3, 1, 4)
        q, k, v = qkv[0], qkv[1], qkv[2]
        scale = Dh ** -0.5
        pos = jnp.arange(S)
        off = jnp.arange(W) * dil
        idx = pos[:, None] - off[None, :]
        mask = idx >= 0
        idx_c = jnp.where(mask, idx, 0).reshape(-1)
        kg = k[:, :, idx_c, :].reshape(B, H, S, W, Dh)
        vg = v[:, :, idx_c, :].reshape(B, H, S, W, Dh)
        logits = jnp.einsum("bhsd,bhswd->bhsw", q, kg) * scale
        logits = jnp.where(mask[None, None, :, :], logits, -1e9)
        attn = _softmax(logits, axis=-1)
        o = jnp.einsum("bhsw,bhswd->bhsd", attn, vg)
        return (lambda x, *d: x.transpose(*d))(o, 0, 2, 1, 3).reshape(B, S, D) @ wo

    x = A_x
    g = _sigmoid((x * gate_w).sum(-1, keepdims=True))
    a = _A_ref(x, A_c_kv, A_w_q, A_w_uk, A_w_uv, A_w_o)
    b = _B_ref(x, B_wqkv, B_wo)
    return g * a + (1 - g) * b
```

```python
import functools
import math

import jax
import jax.numpy as jnp
import jax.experimental.pallas as pl
import jax.experimental.pallas.tpu as pltpu

F32 = jnp.float32
BF16 = jnp.bfloat16
U32 = jnp.uint32

S = 2048
M = 1024
HA = 32
DA = 128
DC = 512
HB = 32
DB = 32
WIN = 8
DIL = 2
PAD = 16
LOG2E = math.log2(math.e)
NEG = -1e9

TQ = 128
NQ = S // TQ
NP = HA // 2
TO = 256
NT = (((1,), (1,)), ((), ()))

_STAGES = ((2, 4), (1, 3), (0, 2), (0, 6), (0, 1), (0, 5), (0, 0))


def _pi(d):
    b = [(d >> i) & 1 for i in range(5)]
    return (b[4] << 4) | (b[3] << 3) | (b[0] << 2) | (b[2] << 1) | b[1]


def _permute8(cols):
    cols = list(cols)
    lane = jax.lax.broadcasted_iota(jnp.int32, cols[0].shape, 1)
    for va, lb in _STAGES:
        lo = (lane & (1 << lb)) == 0
        sh = 1 << lb
        idx = [i for i in range(8) if not (i >> va) & 1]
        if lb == 6:
            rr = [pltpu.roll(jnp.where(lo, cols[i | (1 << va)], cols[i]), 64, 1) for i in idx]
            for i, r in zip(idx, rr):
                a, b = cols[i], cols[i | (1 << va)]
                cols[i] = jnp.where(lo, a, r)
                cols[i | (1 << va)] = jnp.where(lo, r, b)
        else:
            rb = [pltpu.roll(cols[i | (1 << va)], sh, 1) for i in idx]
            ra = [pltpu.roll(cols[i], 128 - sh, 1) for i in idx]
            for i, xa, xb in zip(idx, ra, rb):
                a, b = cols[i], cols[i | (1 << va)]
                cols[i] = jnp.where(lo, a, xb)
                cols[i | (1 << va)] = jnp.where(lo, xa, b)
    return cols


def _unpack_pair(e):
    lo = pltpu.bitcast(e << 16, F32).astype(BF16)
    hi = pltpu.bitcast(e & jnp.uint32(0xFFFF0000), F32).astype(BF16)
    return lo, hi


def _fold(xs, op):
    acc = xs[0]
    for x in xs[1:]:
        acc = op(acc, x)
    return acc


def _lane_chunks(x):
    return [x[:, j * 128:(j + 1) * 128] for j in range(x.shape[1] // 128)]


def _kernel(x_hbm, c_hbm, wq_hbm, wuk_hbm, wuv_hbm, wo_hbm, wqkv_hbm, wob_hbm, gw_ref,
            out_hbm,
            xs, cs, wp, wraw, wperm, qb, kb, vb, ctx, wo_s, wob_raw, wob_p, out_s,
            sem_x, sem_w, sem_c, sem_p, sem_o, sem_out):
    xs_u = xs.bitcast(U32)
    cs_u = cs.bitcast(U32)
    wq_u = wq_hbm.bitcast(U32)
    wuk_u = wuk_hbm.bitcast(U32)
    wuv_u = wuv_hbm.bitcast(U32)
    wob_u = wob_hbm.bitcast(U32)

    def cp_x(j):
        return pltpu.make_async_copy(x_hbm.at[:, pl.ds(j * 128, 128)], xs.at[j], sem_x.at[j])

    def cp_w(j):
        return pltpu.make_async_copy(wqkv_hbm.at[pl.ds(j * 128, 128), :],
                                     wraw.at[pl.ds(j * 128, 128), :], sem_w.at[j])

    def cp_c(j):
        return pltpu.make_async_copy(c_hbm.at[:, pl.ds(j * 128, 128)], cs.at[j], sem_c.at[0])

    def cp_p(p):
        return (
            pltpu.make_async_copy(wuk_u.at[:, p, :], wp.at[p, pl.ds(0, DC), :], sem_p.at[p]),
            pltpu.make_async_copy(wuv_u.at[:, p, :], wp.at[p, pl.ds(DC, DC), :], sem_p.at[p]),
            pltpu.make_async_copy(wq_u.at[:, p, :], wp.at[p, pl.ds(2 * DC, M), :], sem_p.at[p]),
        )

    def cp_wo():
        return pltpu.make_async_copy(wo_hbm, wo_s, sem_o.at[0])

    def cp_wob(dp):
        return pltpu.make_async_copy(wob_u.at[:, dp, :], wob_raw.at[dp], sem_o.at[1])

    def cp_out(i):
        r0 = pl.multiple_of(i * TO, TO)
        return pltpu.make_async_copy(out_s.at[pl.ds(r0, TO), :], out_hbm.at[pl.ds(r0, TO), :],
                                     sem_out.at[i])

    def x_rows(r0, n, j):
        return pltpu.bitcast(xs_u[j, pl.ds(r0 // 2, n // 2), :], BF16)

    cp_w(0).start()
    cp_x(0).start()
    for j in range(1, 8):
        cp_w(j).start()
        cp_x(j).start()
    for j in range(4):
        cp_c(j).start()
    for p in range(NP):
        for d in cp_p(p):
            d.start()
    for dp in range(16):
        cp_wob(dp).start()
    cp_wo().start()

    for cc in range(8):
        kb[cc, pl.ds(0, PAD), :] = jnp.zeros((PAD, 128), F32)
        vb[cc, pl.ds(0, PAD), :] = jnp.zeros((PAD, 128), F32)

    def permute_chunk(src, dst, sec):
        r0 = pl.multiple_of(src * 128, 128)
        w = pltpu.bitcast(wraw[pl.ds(r0, 128), pl.ds(sec * M, M)], U32)
        cols = _permute8(_lane_chunks(w))
        for cc in range(8):
            wperm[dst, sec * 8 + cc] = cols[cc]

    cp_w(0).wait()
    for sec in range(3):
        permute_chunk(0, 0, sec)

    def p1_body(kt, carry):
        nxt = jnp.minimum(kt + 1, 7)
        cur = kt & 1

        @pl.when(kt < 7)
        def _():
            cp_w(kt + 1).wait()

        cp_x(kt).wait()
        first = kt == 0
        xk = pltpu.bitcast(xs_u[kt], BF16)
        for sec, (dst, off) in enumerate(((qb, 0), (kb, PAD), (vb, PAD))):
            for half in range(2):
                w = pltpu.bitcast(
                    jnp.concatenate([wperm[cur, sec * 8 + half * 4 + cc] for cc in range(4)], axis=1),
                    BF16)
                for rb in range(4):
                    r = jnp.dot(xk[rb * 512:(rb + 1) * 512], w, preferred_element_type=F32)
                    for cc in range(4):
                        sl = (half * 4 + cc, pl.ds(off + rb * 512, 512), slice(None))
                        old = jnp.where(first, 0.0, dst[sl])
                        dst[sl] = old + r[:, cc * 128:(cc + 1) * 128]
            permute_chunk(nxt, 1 - cur, sec)
        return carry

    jax.lax.fori_loop(0, 8, p1_body, 0)

    for j in range(4):
        cp_c(j).wait()
    for dp in range(16):
        cp_wob(dp).wait()

    row = jax.lax.broadcasted_iota(jnp.int32, (TQ, TQ), 0)
    col = jax.lax.broadcasted_iota(jnp.int32, (TQ, TQ), 1)

    def p2_body(p, carry):
        for d in cp_p(p):
            d.wait()
        causal = col <= row
        wk = jnp.concatenate(_unpack_pair(wp[p, pl.ds(0, DC), :]), axis=1)
        wv = jnp.concatenate(_unpack_pair(wp[p, pl.ds(DC, DC), :]), axis=1)
        wq = jnp.concatenate(_unpack_pair(wp[p, pl.ds(2 * DC, M), :]), axis=1)

        lo, hi = _unpack_pair(wob_raw[p])
        b2 = (p >> 1) & 1
        b1 = p & 1
        base = ((p >> 2) << 3) + (b2 << 1) + b1
        wob_p[base] = pltpu.bitcast(lo, U32)
        wob_p[base + 4] = pltpu.bitcast(hi, U32)

        ks, vs, qs = [], [], []

        def proj(i):
            cb = pltpu.bitcast(
                jnp.concatenate([cs_u[j, pl.ds(i * TQ // 2, TQ // 2), :] for j in range(4)], axis=1),
                BF16)
            xb = pltpu.bitcast(
                jnp.concatenate([xs_u[j, pl.ds(i * TQ // 2, TQ // 2), :] for j in range(8)], axis=1),
                BF16)
            ks.append(jnp.dot(cb, wk, preferred_element_type=F32).astype(BF16))
            q = jnp.dot(xb, wq, preferred_element_type=F32) * (DA ** -0.5 * LOG2E)
            qs.append(q.astype(BF16))
            vs.append(jnp.dot(cb, wv, preferred_element_type=F32).astype(BF16))

        def qk(h, i):
            hs = slice(h * DA, (h + 1) * DA)
            kk = jnp.concatenate([ks[j][:, hs] for j in range(i + 1)], axis=0)
            s = jax.lax.dot_general(qs[i][:, hs], kk, NT, preferred_element_type=F32)
            ch = _lane_chunks(s)
            ch[i] = jnp.where(causal, ch[i], NEG)
            return ch

        def softmax_pv(h, i, ch):
            hs = slice(h * DA, (h + 1) * DA)
            m = jnp.max(_fold(ch, jnp.maximum), axis=1, keepdims=True)
            ps = [jnp.exp2(c - m) for c in ch]
            l = jnp.sum(_fold(ps, jnp.add), axis=1, keepdims=True)
            pb = jnp.concatenate([x.astype(BF16) for x in ps], axis=1)
            vv = jnp.concatenate([vs[j][:, hs] for j in range(i + 1)], axis=0)
            o = jnp.dot(pb, vv, preferred_element_type=F32)
            r = pl.reciprocal(l, approx=True)
            r = r * (2.0 - l * r)
            ctx[2 * p + h, pl.ds(i * TQ // 2, TQ // 2), :] = pltpu.bitcast((o * r).astype(BF16), U32)

        proj(0)
        for i in range(NQ):
            s0 = qk(0, i)
            s1 = qk(1, i)
            if i + 1 < NQ:
                proj(i + 1)
            softmax_pv(0, i, s0)
            softmax_pv(1, i, s1)
        return carry

    jax.lax.fori_loop(0, NP, p2_body, 0)

    cp_wo().wait()
    gw = gw_ref[...].astype(F32)
    RB = 32
    rowi = jax.lax.broadcasted_iota(jnp.int32, (RB, 128), 0)

    def p3_body(i, carry):
        r0 = pl.multiple_of(i * TO, TO)
        h0 = pl.multiple_of(i * (TO // 2), TO // 2)
        ca = pltpu.bitcast(
            jnp.concatenate([ctx[h, pl.ds(h0, TO // 2), :] for h in range(HA)], axis=1), BF16)
        a = jnp.dot(ca, wo_s[...], preferred_element_type=F32)

        gs = _fold([pltpu.bitcast(xs_u[j, pl.ds(h0, TO // 2), :], BF16).astype(F32) * gw[j:j + 1]
                    for j in range(8)], jnp.add)
        g = jax.nn.sigmoid(jnp.sum(gs, axis=1, keepdims=True))

        obs = []
        for rb in range(TO // RB):
            q = [qb[cc, pl.ds(r0 + rb * RB, RB), :] for cc in range(8)]
            lg = [_fold([q[cc] * kb[cc, pl.ds(r0 + (PAD + rb * RB - DIL * w), RB), :]
                         for cc in range(8)], jnp.add) for w in range(WIN)]
            lg = [t + pltpu.roll(t, 64, 1) for t in lg]
            lg = [t + pltpu.roll(t, 32, 1) for t in lg]
            lg = [t * (DB ** -0.5 * LOG2E) for t in lg]
            if rb == 0:
                lg = [lg[0]] + [jnp.where(rowi + r0 >= DIL * w, lg[w], NEG) for w in range(1, WIN)]
            m = _fold(lg, jnp.maximum)
            ps = [jnp.exp2(t - m) for t in lg]
            l = _fold(ps, jnp.add)
            r = pl.reciprocal(l, approx=True)
            r = r * (2.0 - l * r)
            ps = [t * r for t in ps]
            o = [_fold([ps[w] * vb[cc, pl.ds(r0 + (PAD + rb * RB - DIL * w), RB), :]
                        for w in range(WIN)], jnp.add).astype(BF16) for cc in range(8)]
            obs.append(jnp.concatenate(o, axis=1))
        ob = jnp.concatenate(obs, axis=0)
        wb = pltpu.bitcast(jnp.concatenate([wob_p[d] for d in range(DB)], axis=0), BF16)
        b = jnp.dot(ob, wb, preferred_element_type=F32)
        out_s[pl.ds(r0, TO), :] = (g * a + (1.0 - g) * b).astype(BF16)
        cp_out(i).start()
        return carry

    jax.lax.fori_loop(0, S // TO, p3_body, 0)
    for i in range(S // TO):
        cp_out(i).wait()


@jax.jit
def pallas_gated_mix__compressed_kv_cla__sliding_local_dilated__prompt_kernel(
    A_x: jax.Array,
    A_c_kv: jax.Array,
    A_w_q: jax.Array,
    A_w_uk: jax.Array,
    A_w_uv: jax.Array,
    A_w_o: jax.Array,
    B_x: jax.Array,
    B_wqkv: jax.Array,
    B_wo: jax.Array,
    gate_w: jax.Array,
):
    del B_x
    any_spec = pl.BlockSpec(memory_space=pl.ANY)
    out = pl.pallas_call(
        _kernel,
        in_specs=[any_spec] * 8 + [pl.BlockSpec(memory_space=pltpu.VMEM)],
        out_specs=any_spec,
        out_shape=jax.ShapeDtypeStruct((S, M), BF16),
        scratch_shapes=[
            pltpu.VMEM((8, S, 128), BF16),
            pltpu.VMEM((4, S, 128), BF16),
            pltpu.VMEM((NP, 2 * DC + M, 128), U32),
            pltpu.VMEM((M, 3 * M), BF16),
            pltpu.VMEM((2, 24, 64, 128), U32),
            pltpu.VMEM((8, S, 128), F32),
            pltpu.VMEM((8, S + PAD, 128), F32),
            pltpu.VMEM((8, S + PAD, 128), F32),
            pltpu.VMEM((HA, S // 2, 128), U32),
            pltpu.VMEM((HA * DA, M), BF16),
            pltpu.VMEM((16, HB, M), U32),
            pltpu.VMEM((DB, HB // 2, M), U32),
            pltpu.VMEM((S, M), BF16),
            pltpu.SemaphoreType.DMA((8,)),
            pltpu.SemaphoreType.DMA((8,)),
            pltpu.SemaphoreType.DMA((1,)),
            pltpu.SemaphoreType.DMA((NP,)),
            pltpu.SemaphoreType.DMA((2,)),
            pltpu.SemaphoreType.DMA((S // TO,)),
        ],
        compiler_params=pltpu.CompilerParams(vmem_limit_bytes=120 * 1024 * 1024),
    )(
        A_x.reshape(S, M),
        A_c_kv.reshape(S, DC),
        A_w_q,
        A_w_uk,
        A_w_uv,
        A_w_o.reshape(HA * DA, M),
        B_wqkv,
        B_wo.reshape(HB, DB, M),
        gate_w.reshape(8, 128),
    )
    return out.reshape(1, S, M)
```

```python
import functools
import math

import jax
import jax.numpy as jnp
import jax.experimental.pallas as pl
import jax.experimental.pallas.tpu as pltpu

F32 = jnp.float32
BF16 = jnp.bfloat16
U32 = jnp.uint32

S = 2048
M = 1024
HA = 32
DA = 128
DC = 512
HB = 32
DB = 32
WIN = 8
DIL = 2
PAD = 16
LOG2E = math.log2(math.e)
NEG = -1e9

TQ = 128
NQ = S // TQ
NP = HA // 2
TO = 128
NT = (((1,), (1,)), ((), ()))

_STAGES = ((2, 4), (1, 3), (0, 2), (0, 6), (0, 1), (0, 5), (0, 0))


def _pi(d):
    b = [(d >> i) & 1 for i in range(5)]
    return (b[4] << 4) | (b[3] << 3) | (b[0] << 2) | (b[2] << 1) | b[1]


def _permute8(cols):
    cols = list(cols)
    lane = jax.lax.broadcasted_iota(jnp.int32, cols[0].shape, 1)
    for va, lb in _STAGES:
        lo = (lane & (1 << lb)) == 0
        sh = 1 << lb
        idx = [i for i in range(8) if not (i >> va) & 1]
        if lb == 6:
            rr = [pltpu.roll(jnp.where(lo, cols[i | (1 << va)], cols[i]), 64, 1) for i in idx]
            for i, r in zip(idx, rr):
                a, b = cols[i], cols[i | (1 << va)]
                cols[i] = jnp.where(lo, a, r)
                cols[i | (1 << va)] = jnp.where(lo, r, b)
        else:
            rb = [pltpu.roll(cols[i | (1 << va)], sh, 1) for i in idx]
            ra = [pltpu.roll(cols[i], 128 - sh, 1) for i in idx]
            for i, xa, xb in zip(idx, ra, rb):
                a, b = cols[i], cols[i | (1 << va)]
                cols[i] = jnp.where(lo, a, xb)
                cols[i | (1 << va)] = jnp.where(lo, xa, b)
    return cols


def _unpack_pair(e):
    lo = pltpu.bitcast(e << 16, F32).astype(BF16)
    hi = pltpu.bitcast(e & jnp.uint32(0xFFFF0000), F32).astype(BF16)
    return lo, hi


def _fold(xs, op):
    acc = xs[0]
    for x in xs[1:]:
        acc = op(acc, x)
    return acc


def _lane_chunks(x):
    return [x[:, j * 128:(j + 1) * 128] for j in range(x.shape[1] // 128)]


def _kernel(x_hbm, c_hbm, wq_hbm, wuk_hbm, wuv_hbm, wo_hbm, wqkv_hbm, wob_hbm, gw_ref,
            out_hbm,
            xs, cs, wp, wraw, wperm, qb, kb, vb, ctx, wo_s, wob_raw, wob_p, out_s,
            sem_x, sem_w, sem_c, sem_p, sem_o, sem_out):
    xs_u = xs.bitcast(U32)
    cs_u = cs.bitcast(U32)
    wq_u = wq_hbm.bitcast(U32)
    wuk_u = wuk_hbm.bitcast(U32)
    wuv_u = wuv_hbm.bitcast(U32)
    wob_u = wob_hbm.bitcast(U32)

    def cp_x(j):
        return pltpu.make_async_copy(x_hbm.at[:, pl.ds(pl.multiple_of(j * 128, 128), 128)], xs.at[j], sem_x.at[j])

    def cp_w(j):
        r0 = pl.multiple_of(j * 128, 128)
        return pltpu.make_async_copy(wqkv_hbm.at[pl.ds(r0, 128), :],
                                     wraw.at[pl.ds(r0, 128), :], sem_w.at[j])

    def cp_c(j):
        return pltpu.make_async_copy(c_hbm.at[:, pl.ds(pl.multiple_of(j * 128, 128), 128)], cs.at[j], sem_c.at[0])

    def cp_p(p):
        return (
            pltpu.make_async_copy(wuk_u.at[:, p, :], wp.at[p, pl.ds(0, DC), :], sem_p.at[p]),
            pltpu.make_async_copy(wuv_u.at[:, p, :], wp.at[p, pl.ds(DC, DC), :], sem_p.at[p]),
            pltpu.make_async_copy(wq_u.at[:, p, :], wp.at[p, pl.ds(2 * DC, M), :], sem_p.at[p]),
        )

    def cp_wo():
        return pltpu.make_async_copy(wo_hbm, wo_s, sem_o.at[0])

    def cp_wob(dp):
        return pltpu.make_async_copy(wob_u.at[:, dp, :], wob_raw.at[dp], sem_o.at[1])

    def cp_out(i):
        r0 = pl.multiple_of(i * TO, TO)
        return pltpu.make_async_copy(out_s.at[pl.ds(r0, TO), :], out_hbm.at[pl.ds(r0, TO), :],
                                     sem_out.at[i])

    def x_rows(r0, n, j):
        return pltpu.bitcast(xs_u[j, pl.ds(r0 // 2, n // 2), :], BF16)

    cp_w(0).start()
    cp_x(0).start()
    cp_w(1).start()
    cp_x(1).start()

    for cc in range(8):
        kb[cc, pl.ds(0, PAD), :] = jnp.zeros((PAD, 128), F32)
        vb[cc, pl.ds(0, PAD), :] = jnp.zeros((PAD, 128), F32)

    def permute_chunk(src, dst, sec):
        r0 = pl.multiple_of(src * 128, 128)
        w = pltpu.bitcast(wraw[pl.ds(r0, 128), pl.ds(sec * M, M)], U32)
        cols = _permute8(_lane_chunks(w))
        for cc in range(8):
            wperm[dst, sec * 8 + cc] = cols[cc]

    cp_w(0).wait()
    for sec in range(3):
        permute_chunk(0, 0, sec)

    def p1_body(kt, carry):
        nxt = jnp.minimum(kt + 1, 7)
        cur = kt & 1

        @pl.when(kt < 7)
        def _():
            cp_w(kt + 1).wait()

        cp_x(kt).wait()

        @pl.when(kt < 6)
        def _():
            cp_w(kt + 2).start()
            cp_x(kt + 2).start()

        @pl.when(kt < 4)
        def _():
            cp_c(kt).start()

        for e in range(2):
            for d in cp_p(2 * kt + e):
                d.start()
            cp_wob(2 * kt + e).start()

        first = kt == 0
        xk = pltpu.bitcast(xs_u[kt], BF16)
        for sec, (dst, off) in enumerate(((qb, 0), (kb, PAD), (vb, PAD))):
            for half in range(2):
                w = pltpu.bitcast(
                    jnp.concatenate([wperm[cur, sec * 8 + half * 4 + cc] for cc in range(4)], axis=1),
                    BF16)
                for rb in range(4):
                    r = jnp.dot(xk[rb * 512:(rb + 1) * 512], w, preferred_element_type=F32)
                    for cc in range(4):
                        sl = (half * 4 + cc, pl.ds(off + rb * 512, 512), slice(None))
                        old = jnp.where(first, 0.0, dst[sl])
                        dst[sl] = old + r[:, cc * 128:(cc + 1) * 128]
            permute_chunk(nxt, 1 - cur, sec)
        return carry

    jax.lax.fori_loop(0, 8, p1_body, 0)

    for j in range(4):
        cp_c(j).wait()
    for dp in range(16):
        cp_wob(dp).wait()

    row = jax.lax.broadcasted_iota(jnp.int32, (TQ, TQ), 0)
    col = jax.lax.broadcasted_iota(jnp.int32, (TQ, TQ), 1)

    def p2_body(p, carry):
        for d in cp_p(p):
            d.wait()

        @pl.when(p == 0)
        def _():
            cp_wo().start()

        causal = col <= row
        wk = jnp.concatenate(_unpack_pair(wp[p, pl.ds(0, DC), :]), axis=1)
        wv = jnp.concatenate(_unpack_pair(wp[p, pl.ds(DC, DC), :]), axis=1)
        wq = jnp.concatenate(_unpack_pair(wp[p, pl.ds(2 * DC, M), :]), axis=1)

        lo, hi = _unpack_pair(wob_raw[p])
        b2 = (p >> 1) & 1
        b1 = p & 1
        base = ((p >> 2) << 3) + (b2 << 1) + b1
        wob_p[base] = pltpu.bitcast(lo, U32)
        wob_p[base + 4] = pltpu.bitcast(hi, U32)

        ks, vs, qs = [], [], []

        def proj(i):
            cb = pltpu.bitcast(
                jnp.concatenate([cs_u[j, pl.ds(i * TQ // 2, TQ // 2), :] for j in range(4)], axis=1),
                BF16)
            xb = pltpu.bitcast(
                jnp.concatenate([xs_u[j, pl.ds(i * TQ // 2, TQ // 2), :] for j in range(8)], axis=1),
                BF16)
            ks.append(jnp.dot(cb, wk, preferred_element_type=F32).astype(BF16))
            q = jnp.dot(xb, wq, preferred_element_type=F32) * (DA ** -0.5 * LOG2E)
            qs.append(q.astype(BF16))
            vs.append(jnp.dot(cb, wv, preferred_element_type=F32).astype(BF16))

        def qk(h, i):
            hs = slice(h * DA, (h + 1) * DA)
            kk = jnp.concatenate([ks[j][:, hs] for j in range(i + 1)], axis=0)
            s = jax.lax.dot_general(qs[i][:, hs], kk, NT, preferred_element_type=F32)
            ch = _lane_chunks(s)
            ch[i] = jnp.where(causal, ch[i], NEG)
            return ch

        def softmax_pv(h, i, ch):
            hs = slice(h * DA, (h + 1) * DA)
            m = jnp.max(_fold(ch, jnp.maximum), axis=1, keepdims=True)
            ps = [jnp.exp2(c - m) for c in ch]
            l = jnp.sum(_fold(ps, jnp.add), axis=1, keepdims=True)
            pb = jnp.concatenate([x.astype(BF16) for x in ps], axis=1)
            vv = jnp.concatenate([vs[j][:, hs] for j in range(i + 1)], axis=0)
            o = jnp.dot(pb, vv, preferred_element_type=F32)
            r = pl.reciprocal(l, approx=True)
            r = r * (2.0 - l * r)
            ctx[2 * p + h, pl.ds(i * TQ // 2, TQ // 2), :] = pltpu.bitcast((o * r).astype(BF16), U32)

        proj(0)
        for i in range(NQ):
            s0 = qk(0, i)
            s1 = qk(1, i)
            if i + 1 < NQ:
                proj(i + 1)
            softmax_pv(0, i, s0)
            softmax_pv(1, i, s1)
        return carry

    jax.lax.fori_loop(0, NP, p2_body, 0)

    cp_wo().wait()
    gw = gw_ref[...].astype(F32)
    RB = 32
    rowi = jax.lax.broadcasted_iota(jnp.int32, (RB, 128), 0)

    def p3_body(i, carry):
        r0 = pl.multiple_of(i * TO, TO)
        h0 = pl.multiple_of(i * (TO // 2), TO // 2)
        ca = pltpu.bitcast(
            jnp.concatenate([ctx[h, pl.ds(h0, TO // 2), :] for h in range(HA)], axis=1), BF16)
        a = jnp.dot(ca, wo_s[...], preferred_element_type=F32)

        gs = _fold([pltpu.bitcast(xs_u[j, pl.ds(h0, TO // 2), :], BF16).astype(F32) * gw[j:j + 1]
                    for j in range(8)], jnp.add)
        g = jax.nn.sigmoid(jnp.sum(gs, axis=1, keepdims=True))

        obs = []
        for rb in range(TO // RB):
            q = [qb[cc, pl.ds(r0 + rb * RB, RB), :] for cc in range(8)]
            lg = [_fold([q[cc] * kb[cc, pl.ds(r0 + (PAD + rb * RB - DIL * w), RB), :]
                         for cc in range(8)], jnp.add) for w in range(WIN)]
            lg = [t + pltpu.roll(t, 64, 1) for t in lg]
            lg = [t + pltpu.roll(t, 32, 1) for t in lg]
            lg = [t * (DB ** -0.5 * LOG2E) for t in lg]
            if rb == 0:
                lg = [lg[0]] + [jnp.where(rowi + r0 >= DIL * w, lg[w], NEG) for w in range(1, WIN)]
            m = _fold(lg, jnp.maximum)
            ps = [jnp.exp2(t - m) for t in lg]
            l = _fold(ps, jnp.add)
            r = pl.reciprocal(l, approx=True)
            r = r * (2.0 - l * r)
            ps = [t * r for t in ps]
            o = [_fold([ps[w] * vb[cc, pl.ds(r0 + (PAD + rb * RB - DIL * w), RB), :]
                        for w in range(WIN)], jnp.add).astype(BF16) for cc in range(8)]
            obs.append(jnp.concatenate(o, axis=1))
        ob = jnp.concatenate(obs, axis=0)
        wb = pltpu.bitcast(jnp.concatenate([wob_p[d] for d in range(DB)], axis=0), BF16)
        b = jnp.dot(ob, wb, preferred_element_type=F32)
        out_s[pl.ds(r0, TO), :] = (g * a + (1.0 - g) * b).astype(BF16)
        cp_out(i).start()
        return carry

    jax.lax.fori_loop(0, S // TO, p3_body, 0)
    for i in range(S // TO):
        cp_out(i).wait()


@jax.jit
def pallas_gated_mix__compressed_kv_cla__sliding_local_dilated__prompt_kernel(
    A_x: jax.Array,
    A_c_kv: jax.Array,
    A_w_q: jax.Array,
    A_w_uk: jax.Array,
    A_w_uv: jax.Array,
    A_w_o: jax.Array,
    B_x: jax.Array,
    B_wqkv: jax.Array,
    B_wo: jax.Array,
    gate_w: jax.Array,
):
    del B_x
    any_spec = pl.BlockSpec(memory_space=pl.ANY)
    out = pl.pallas_call(
        _kernel,
        in_specs=[any_spec] * 8 + [pl.BlockSpec(memory_space=pltpu.VMEM)],
        out_specs=any_spec,
        out_shape=jax.ShapeDtypeStruct((S, M), BF16),
        scratch_shapes=[
            pltpu.VMEM((8, S, 128), BF16),
            pltpu.VMEM((4, S, 128), BF16),
            pltpu.VMEM((NP, 2 * DC + M, 128), U32),
            pltpu.VMEM((M, 3 * M), BF16),
            pltpu.VMEM((2, 24, 64, 128), U32),
            pltpu.VMEM((8, S, 128), F32),
            pltpu.VMEM((8, S + PAD, 128), F32),
            pltpu.VMEM((8, S + PAD, 128), F32),
            pltpu.VMEM((HA, S // 2, 128), U32),
            pltpu.VMEM((HA * DA, M), BF16),
            pltpu.VMEM((16, HB, M), U32),
            pltpu.VMEM((DB, HB // 2, M), U32),
            pltpu.VMEM((S, M), BF16),
            pltpu.SemaphoreType.DMA((8,)),
            pltpu.SemaphoreType.DMA((8,)),
            pltpu.SemaphoreType.DMA((1,)),
            pltpu.SemaphoreType.DMA((NP,)),
            pltpu.SemaphoreType.DMA((2,)),
            pltpu.SemaphoreType.DMA((S // TO,)),
        ],
        compiler_params=pltpu.CompilerParams(vmem_limit_bytes=120 * 1024 * 1024),
    )(
        A_x.reshape(S, M),
        A_c_kv.reshape(S, DC),
        A_w_q,
        A_w_uk,
        A_w_uv,
        A_w_o.reshape(HA * DA, M),
        B_wqkv,
        B_wo.reshape(HB, DB, M),
        gate_w.reshape(8, 128),
    )
    return out.reshape(1, S, M)
```

```python
import functools
import math

import jax
import jax.numpy as jnp
import jax.experimental.pallas as pl
import jax.experimental.pallas.tpu as pltpu

F32 = jnp.float32
BF16 = jnp.bfloat16
U32 = jnp.uint32

S = 2048
M = 1024
HA = 32
DA = 128
DC = 512
HB = 32
DB = 32
WIN = 8
DIL = 2
PAD = 16
LOG2E = math.log2(math.e)
NEG = -1e9

TQ = 128
NQ = S // TQ
NP = HA // 2
DEP = 2
LDEP = 1
NLAST = 1
TO = 128
NT = (((1,), (1,)), ((), ()))

_STAGES = ((2, 4), (1, 3), (0, 2), (0, 6), (0, 1), (0, 5), (0, 0))


def _pi(d):
    b = [(d >> i) & 1 for i in range(5)]
    return (b[4] << 4) | (b[3] << 3) | (b[0] << 2) | (b[2] << 1) | b[1]


def _permute8(cols):
    cols = list(cols)
    lane = jax.lax.broadcasted_iota(jnp.int32, cols[0].shape, 1)
    for va, lb in _STAGES:
        lo = (lane & (1 << lb)) == 0
        sh = 1 << lb
        idx = [i for i in range(8) if not (i >> va) & 1]
        if lb == 6:
            rr = [pltpu.roll(jnp.where(lo, cols[i | (1 << va)], cols[i]), 64, 1) for i in idx]
            for i, r in zip(idx, rr):
                a, b = cols[i], cols[i | (1 << va)]
                cols[i] = jnp.where(lo, a, r)
                cols[i | (1 << va)] = jnp.where(lo, r, b)
        else:
            rb = [pltpu.roll(cols[i | (1 << va)], sh, 1) for i in idx]
            ra = [pltpu.roll(cols[i], 128 - sh, 1) for i in idx]
            for i, xa, xb in zip(idx, ra, rb):
                a, b = cols[i], cols[i | (1 << va)]
                cols[i] = jnp.where(lo, a, xb)
                cols[i | (1 << va)] = jnp.where(lo, xa, b)
    return cols


def _pack(x):
    return pltpu.bitcast(x.astype(BF16), U32)


def _bf(x):
    return pltpu.bitcast(x, BF16)


def _unpack_pair(e):
    lo = _pack(pltpu.bitcast(e << 16, F32))
    hi = _pack(pltpu.bitcast(e & jnp.uint32(0xFFFF0000), F32))
    return lo, hi


def _fold(xs, op):
    acc = xs[0]
    for x in xs[1:]:
        acc = op(acc, x)
    return acc


def _lane_chunks(x):
    return [x[:, j * 128:(j + 1) * 128] for j in range(x.shape[1] // 128)]


def _kernel(x_hbm, c_hbm, wq_hbm, wuk_hbm, wuv_hbm, wo_hbm, wqkv_hbm, wob_hbm, gw_ref,
            out_hbm,
            xs_u, cs_u, wp, wraw, wperm, qb, kb, vb, ctx, wo_s, wob_raw, wob_p, out_s,
            sem_x, sem_w, sem_c, sem_p, sem_o, sem_out):
    x_u = x_hbm.bitcast(U32)
    c_u = c_hbm.bitcast(U32)
    wo_u = wo_hbm.bitcast(U32)
    wq_u = wq_hbm.bitcast(U32)
    wuk_u = wuk_hbm.bitcast(U32)
    wuv_u = wuv_hbm.bitcast(U32)
    wob_u = wob_hbm.bitcast(U32)

    def cp_x(j):
        return pltpu.make_async_copy(x_u.at[:, pl.ds(pl.multiple_of(j * 128, 128), 128)], xs_u.at[j], sem_x.at[j])

    def cp_w(j):
        r0 = pl.multiple_of(j * 128, 128)
        return pltpu.make_async_copy(wqkv_hbm.at[pl.ds(r0, 128), :],
                                     wraw.at[pl.ds(r0, 128), :], sem_w.at[j])

    def cp_c(j):
        return pltpu.make_async_copy(c_u.at[:, pl.ds(pl.multiple_of(j * 128, 128), 128)], cs_u.at[j], sem_c.at[0])

    def cp_p(p):
        return (
            pltpu.make_async_copy(wuk_u.at[:, p, :], wp.at[p, pl.ds(0, DC), :], sem_p.at[p]),
            pltpu.make_async_copy(wuv_u.at[:, p, :], wp.at[p, pl.ds(DC, DC), :], sem_p.at[p]),
            pltpu.make_async_copy(wq_u.at[:, p, :], wp.at[p, pl.ds(2 * DC, M), :], sem_p.at[p]),
        )

    def cp_wo(j):
        return pltpu.make_async_copy(wo_u.at[:, pl.ds(pl.multiple_of(j * 128, 128), 128)],
                                     wo_s.at[j], sem_o.at[0])

    def cp_wob(dp):
        return pltpu.make_async_copy(wob_u.at[:, dp, :], wob_raw.at[dp], sem_o.at[1])

    def cp_out(i):
        r0 = pl.multiple_of(i * TO, TO)
        return pltpu.make_async_copy(out_s.at[pl.ds(r0, TO), :], out_hbm.at[pl.ds(r0, TO), :],
                                     sem_out.at[i])

    cp_w(0).start()
    cp_x(0).start()
    cp_w(1).start()
    cp_x(1).start()

    for cc in range(8):
        kb[cc, pl.ds(0, PAD), :] = jnp.zeros((PAD, 128), F32)
        vb[cc, pl.ds(0, PAD), :] = jnp.zeros((PAD, 128), F32)

    def permuted(kt, sec):
        r0 = pl.multiple_of(kt * 128, 128)
        w = pltpu.bitcast(wraw[pl.ds(r0, 128), pl.ds(sec * M, M)], U32)
        return _permute8(_lane_chunks(w))

    def stage_first(kt):
        for cc, t in enumerate(permuted(kt, 0)):
            wperm[cc] = t

    cp_w(0).wait()
    stage_first(0)

    def p1_body(kt, carry):
        @pl.when(kt < 7)
        def _():
            cp_w(kt + 1).wait()

        cp_x(kt).wait()

        @pl.when(kt < 6)
        def _():
            cp_w(kt + 2).start()
            cp_x(kt + 2).start()

        @pl.when(kt < 4)
        def _():
            cp_c(kt).start()

        for e in range(2):
            for d in cp_p(2 * kt + e):
                d.start()
            cp_wob(2 * kt + e).start()

        first = kt == 0
        xk = pltpu.bitcast(xs_u[kt], BF16)
        for sec, (dst, off) in enumerate(((qb, 0), (kb, PAD), (vb, PAD))):
            cols = [wperm[cc] for cc in range(8)] if sec == 0 else permuted(kt, sec)
            for half in range(2):
                w = pltpu.bitcast(jnp.concatenate(cols[half * 4:half * 4 + 4], axis=1), BF16)
                for rb in range(4):
                    r = jnp.dot(xk[rb * 512:(rb + 1) * 512], w, preferred_element_type=F32)
                    for cc in range(4):
                        sl = (half * 4 + cc, pl.ds(off + rb * 512, 512), slice(None))
                        old = jnp.where(first, 0.0, dst[sl])
                        dst[sl] = old + r[:, cc * 128:(cc + 1) * 128]
        stage_first(jnp.minimum(kt + 1, 7))
        return carry

    jax.lax.fori_loop(0, 8, p1_body, 0)

    for j in range(4):
        cp_c(j).wait()
    for dp in range(16):
        cp_wob(dp).wait()

    row = jax.lax.broadcasted_iota(jnp.int32, (TQ, TQ), 0)
    col = jax.lax.broadcasted_iota(jnp.int32, (TQ, TQ), 1)

    def p2_body(p, carry):
        for d in cp_p(p):
            d.wait()

        @pl.when(p < 8)
        def _():
            cp_wo(p).start()

        causal = col <= row
        wk = _bf(jnp.concatenate(_unpack_pair(wp[p, pl.ds(0, DC), :]), axis=1))
        wv = _bf(jnp.concatenate(_unpack_pair(wp[p, pl.ds(DC, DC), :]), axis=1))
        wq = _bf(jnp.concatenate(_unpack_pair(wp[p, pl.ds(2 * DC, M), :]), axis=1))

        lo, hi = _unpack_pair(wob_raw[p])
        b2 = (p >> 1) & 1
        b1 = p & 1
        base = ((p >> 2) << 3) + (b2 << 1) + b1
        for half, dd in ((lo, base), (hi, base + 4)):
            for cc, t in enumerate(_lane_chunks(half)):
                wob_p[cc, pl.ds(pl.multiple_of(dd * 16, 16), 16), :] = t

        ks, vs, qs = {}, {}, {}
        done = {}
        never = p > NP

        def c_rows(i):
            return pltpu.bitcast(
                jnp.concatenate([cs_u[j, pl.ds(i * TQ // 2, TQ // 2), :] for j in range(4)], axis=1),
                BF16)

        def proj_k(i):
            ks[i] = _pack(jnp.dot(c_rows(i), wk, preferred_element_type=F32))

        def proj_v(i):
            vs[i] = _pack(jnp.dot(c_rows(i), wv, preferred_element_type=F32))

        def proj_q(i):
            xb = pltpu.bitcast(
                jnp.concatenate([xs_u[j, pl.ds(i * TQ // 2, TQ // 2), :] for j in range(8)], axis=1),
                BF16)
            q = jnp.dot(xb, wq, preferred_element_type=F32) * (DA ** -0.5 * LOG2E)
            qs[i] = _pack(q)

        def qk(h, i, dep):
            hs = slice(h * DA, (h + 1) * DA)
            kk = _bf(jnp.concatenate([ks[j][:, hs] for j in range(i + 1)], axis=0))
            q = qs[i][:, hs]
            if dep is not None:
                q = jnp.where(never, done[(h, dep)], q)
            s = jax.lax.dot_general(_bf(q), kk, NT, preferred_element_type=F32)
            ch = _lane_chunks(s)
            ch[i] = jnp.where(causal, ch[i], NEG)
            return ch

        def softmax_pv(h, i, ch):
            hs = slice(h * DA, (h + 1) * DA)
            m = jnp.max(_fold(ch, jnp.maximum), axis=1, keepdims=True)
            ps = [jnp.exp2(c - m) for c in ch]
            lp = _fold(ps, jnp.add)
            pb = jnp.concatenate(ps, axis=1).astype(BF16)
            vv = _bf(jnp.concatenate([vs[j][:, hs] for j in range(i + 1)], axis=0))
            o = jnp.dot(pb, vv, preferred_element_type=F32)
            if i >= LDEP:
                lp = jnp.where(never, o, lp)
            l = jnp.sum(lp, axis=1, keepdims=True)
            r = pl.reciprocal(l, approx=True)
            r = r * (2.0 - l * r)
            cn = _pack(o * r)
            done[(h, i)] = cn
            ctx[2 * p + h, pl.ds(i * TQ // 2, TQ // 2), :] = cn

        order = list(range(NLAST, NQ)) + list(range(NLAST))[::-1]
        for j in range(NLAST + 1):
            proj_k(j)
        proj_q(order[0])
        for j in range(NLAST):
            proj_v(j)
        pend = None
        for t, i in enumerate(order):
            dep = order[t - DEP] if t >= DEP else None
            if pend is not None and dep == pend[0]:
                dep = order[t - DEP - 1]
            s0 = qk(0, i, dep)
            s1 = qk(1, i, dep)
            if pend is not None:
                softmax_pv(0, pend[0], pend[1])
                softmax_pv(1, pend[0], pend[2])
                pend = None
            if i >= NLAST:
                proj_v(i)
            if t + 1 < NQ:
                nx = order[t + 1]
                if nx > i:
                    proj_k(nx)
                proj_q(nx)
            if t + 1 < NQ and order[t + 1] < i:
                pend = (i, s0, s1)
            else:
                softmax_pv(0, i, s0)
                softmax_pv(1, i, s1)
        return carry

    jax.lax.fori_loop(0, NP, p2_body, 0)

    for j in range(8):
        cp_wo(j).wait()
    gw = gw_ref[...].astype(F32)
    RB = 16
    rowi = jax.lax.broadcasted_iota(jnp.int32, (RB, 128), 0)

    def p3_body(i, carry):
        r0 = pl.multiple_of(i * TO, TO)
        h0 = pl.multiple_of(i * (TO // 2), TO // 2)
        ca = pltpu.bitcast(
            jnp.concatenate([ctx[h, pl.ds(h0, TO // 2), :] for h in range(HA)], axis=1), BF16)
        wa = pltpu.bitcast(jnp.concatenate([wo_s[j] for j in range(8)], axis=1), BF16)
        a = jnp.dot(ca, wa, preferred_element_type=F32)

        gs = _fold([pltpu.bitcast(xs_u[j, pl.ds(h0, TO // 2), :], BF16).astype(F32) * gw[j:j + 1]
                    for j in range(8)], jnp.add)
        g = jax.nn.sigmoid(jnp.sum(gs, axis=1, keepdims=True))

        obs = []
        for rb in range(TO // RB):
            q = [qb[cc, pl.ds(r0 + rb * RB, RB), :] for cc in range(8)]
            lg = [_fold([q[cc] * kb[cc, pl.ds(r0 + (PAD + rb * RB - DIL * w), RB), :]
                         for cc in range(8)], jnp.add) for w in range(WIN)]
            lg = [t + pltpu.roll(t, 64, 1) for t in lg]
            lg = [t + pltpu.roll(t, 32, 1) for t in lg]
            lg = [t * (DB ** -0.5 * LOG2E) for t in lg]
            if rb == 0:
                lg = [lg[0]] + [jnp.where(rowi + r0 >= DIL * w, lg[w], NEG) for w in range(1, WIN)]
            m = _fold(lg, jnp.maximum)
            ps = [jnp.exp2(t - m) for t in lg]
            l = _fold(ps, jnp.add)
            r = pl.reciprocal(l, approx=True)
            r = r * (2.0 - l * r)
            ps = [t * r for t in ps]
            o = [_pack(_fold([ps[w] * vb[cc, pl.ds(r0 + (PAD + rb * RB - DIL * w), RB), :]
                              for w in range(WIN)], jnp.add)) for cc in range(8)]
            obs.append(jnp.concatenate(o, axis=1))
        ob = _bf(jnp.concatenate(obs, axis=0))
        wb = pltpu.bitcast(jnp.concatenate([wob_p[j] for j in range(8)], axis=1), BF16)
        b = jnp.dot(ob, wb, preferred_element_type=F32)
        out_s[pl.ds(r0, TO), :] = (g * a + (1.0 - g) * b).astype(BF16)
        cp_out(i).start()
        return carry

    jax.lax.fori_loop(0, S // TO, p3_body, 0)
    for i in range(S // TO):
        cp_out(i).wait()


@jax.jit
def pallas_gated_mix__compressed_kv_cla__sliding_local_dilated__prompt_kernel(
    A_x: jax.Array,
    A_c_kv: jax.Array,
    A_w_q: jax.Array,
    A_w_uk: jax.Array,
    A_w_uv: jax.Array,
    A_w_o: jax.Array,
    B_x: jax.Array,
    B_wqkv: jax.Array,
    B_wo: jax.Array,
    gate_w: jax.Array,
):
    del B_x
    any_spec = pl.BlockSpec(memory_space=pl.ANY)
    out = pl.pallas_call(
        _kernel,
        in_specs=[any_spec] * 8 + [pl.BlockSpec(memory_space=pltpu.VMEM)],
        out_specs=any_spec,
        out_shape=jax.ShapeDtypeStruct((S, M), BF16),
        scratch_shapes=[
            pltpu.VMEM((8, S // 2, 128), U32),
            pltpu.VMEM((4, S // 2, 128), U32),
            pltpu.VMEM((NP, 2 * DC + M, 128), U32),
            pltpu.VMEM((M, 3 * M), BF16),
            pltpu.VMEM((8, 64, 128), U32),
            pltpu.VMEM((8, S, 128), F32),
            pltpu.VMEM((8, S + PAD, 128), F32),
            pltpu.VMEM((8, S + PAD, 128), F32),
            pltpu.VMEM((HA, S // 2, 128), U32),
            pltpu.VMEM((8, HA * DA // 2, 128), U32),
            pltpu.VMEM((16, HB, M), U32),
            pltpu.VMEM((8, M // 2, 128), U32),
            pltpu.VMEM((S, M), BF16),
            pltpu.SemaphoreType.DMA((8,)),
            pltpu.SemaphoreType.DMA((8,)),
            pltpu.SemaphoreType.DMA((1,)),
            pltpu.SemaphoreType.DMA((NP,)),
            pltpu.SemaphoreType.DMA((2,)),
            pltpu.SemaphoreType.DMA((S // TO,)),
        ],
        compiler_params=pltpu.CompilerParams(vmem_limit_bytes=120 * 1024 * 1024,
                                             disable_bounds_checks=True),
    )(
        A_x.reshape(S, M),
        A_c_kv.reshape(S, DC),
        A_w_q,
        A_w_uk,
        A_w_uv,
        A_w_o.reshape(HA * DA, M),
        B_wqkv,
        B_wo.reshape(HB, DB, M),
        gate_w.reshape(8, 128),
    )
    return out.reshape(1, S, M)
```

```python
import functools
import math

import jax
import jax.numpy as jnp
import jax.experimental.pallas as pl
import jax.experimental.pallas.tpu as pltpu

F32 = jnp.float32
BF16 = jnp.bfloat16
U32 = jnp.uint32

S = 2048
M = 1024
HA = 32
DA = 128
DC = 512
HB = 32
DB = 32
WIN = 8
DIL = 2
PAD = 16
LOG2E = math.log2(math.e)
NEG = -1e9

TQ = 128
NQ = S // TQ
NP = HA // 2
DEP = 2
LDEP = 3
NLAST = 3
TO = 128
NT = (((1,), (1,)), ((), ()))

_STAGES = ((2, 4), (1, 3), (0, 2), (0, 6), (0, 1))


def _permute8(cols):
    cols = list(cols)
    lane = jax.lax.broadcasted_iota(jnp.int32, cols[0].shape, 1)
    for va, lb in _STAGES:
        lo = (lane & (1 << lb)) == 0
        sh = 1 << lb
        idx = [i for i in range(8) if not (i >> va) & 1]
        if lb == 6:
            rr = [pltpu.roll(jnp.where(lo, cols[i | (1 << va)], cols[i]), 64, 1) for i in idx]
            for i, r in zip(idx, rr):
                a, b = cols[i], cols[i | (1 << va)]
                cols[i] = jnp.where(lo, a, r)
                cols[i | (1 << va)] = jnp.where(lo, r, b)
        else:
            rb = [pltpu.roll(cols[i | (1 << va)], sh, 1) for i in idx]
            ra = [pltpu.roll(cols[i], 128 - sh, 1) for i in idx]
            for i, xa, xb in zip(idx, ra, rb):
                a, b = cols[i], cols[i | (1 << va)]
                cols[i] = jnp.where(lo, a, xb)
                cols[i | (1 << va)] = jnp.where(lo, xa, b)
    return cols


def _pack(x):
    return pltpu.bitcast(x.astype(BF16), U32)


def _bf(x):
    return pltpu.bitcast(x, BF16)


def _fold(xs, op):
    acc = xs[0]
    for x in xs[1:]:
        acc = op(acc, x)
    return acc


def _lane_chunks(x):
    return [x[:, j * 128:(j + 1) * 128] for j in range(x.shape[1] // 128)]


def _kernel(x_hbm, c_hbm, wq_hbm, wuk_hbm, wuv_hbm, wo_hbm, wqkv_hbm, wob_hbm, gw_ref,
            out_hbm,
            xs_u, cs_u, wp, wraw, wperm, qb, kb, vb, ctx, wo_s, wob_p, wkst, out_s,
            sem_x, sem_w, sem_c, sem_p, sem_o, sem_out):
    x_u = x_hbm.bitcast(U32)
    c_u = c_hbm.bitcast(U32)
    wo_u = wo_hbm.bitcast(U32)
    wq_u = wq_hbm.bitcast(U32)
    wuk_u = wuk_hbm.bitcast(U32)
    wuv_u = wuv_hbm.bitcast(U32)
    wob_u = wob_hbm.bitcast(U32)

    def cp_x(j):
        return pltpu.make_async_copy(x_u.at[:, pl.ds(pl.multiple_of(j * 128, 128), 128)], xs_u.at[j], sem_x.at[j])

    def cp_w(j):
        r0 = pl.multiple_of(j * 128, 128)
        return pltpu.make_async_copy(wqkv_hbm.at[pl.ds(r0, 128), :],
                                     wraw.at[pl.ds(r0, 128), :], sem_w.at[j])

    def cp_c(j):
        return pltpu.make_async_copy(c_u.at[:, pl.ds(pl.multiple_of(j * 128, 128), 128)], cs_u.at[j], sem_c.at[0])

    def cp_p(p):
        return (
            pltpu.make_async_copy(wuk_u.at[:, p, :], wp.at[p, pl.ds(0, DC), :], sem_p.at[p]),
            pltpu.make_async_copy(wuv_u.at[:, p, :], wp.at[p, pl.ds(DC, DC), :], sem_p.at[p]),
            pltpu.make_async_copy(wq_u.at[:, p, :], wp.at[p, pl.ds(2 * DC, M), :], sem_p.at[p]),
        )

    def cp_wo(j):
        return pltpu.make_async_copy(wo_u.at[:, pl.ds(pl.multiple_of(j * 128, 128), 128)],
                                     wo_s.at[j], sem_o.at[0])

    def cp_wob(dp, h0):
        pos = ((dp >> 2) << 3) + ((dp & 1) << 2) + (dp & 2) + h0
        return pltpu.make_async_copy(wob_u.at[:, h0, dp, :],
                                     wob_p.at[pl.ds(pl.multiple_of(pos * 16, 16), 16), :],
                                     sem_o.at[1])

    def cp_out(i):
        r0 = pl.multiple_of(i * TO, TO)
        return pltpu.make_async_copy(out_s.at[pl.ds(r0, TO), :], out_hbm.at[pl.ds(r0, TO), :],
                                     sem_out.at[i])

    cp_w(0).start()
    cp_x(0).start()
    cp_w(1).start()
    cp_x(1).start()

    for cc in range(8):
        kb[cc, pl.ds(0, PAD), :] = jnp.zeros((PAD, 128), F32)
        vb[cc, pl.ds(0, PAD), :] = jnp.zeros((PAD, 128), F32)

    def permuted(kt, sec):
        r0 = pl.multiple_of(kt * 128, 128)
        w = pltpu.bitcast(wraw[pl.ds(r0, 128), pl.ds(sec * M, M)], U32)
        return _permute8(_lane_chunks(w))

    def stage_first(kt):
        for cc, t in enumerate(permuted(kt, 0)):
            wperm[cc] = t

    cp_w(0).wait()
    stage_first(0)

    def p1_body(kt, carry):
        @pl.when(kt < 7)
        def _():
            cp_w(kt + 1).wait()

        cp_x(kt).wait()

        @pl.when(kt < 6)
        def _():
            cp_w(kt + 2).start()
            cp_x(kt + 2).start()

        @pl.when(kt < 4)
        def _():
            cp_c(kt).start()

        for e in range(2):
            for d in cp_p(2 * kt + e):
                d.start()

        first = kt == 0
        xk = pltpu.bitcast(xs_u[kt], BF16)
        for sec, (dst, off) in enumerate(((qb, 0), (kb, PAD), (vb, PAD))):
            cols = [wperm[cc] for cc in range(8)] if sec == 0 else permuted(kt, sec)
            for half in range(2):
                w = pltpu.bitcast(jnp.concatenate(cols[half * 4:half * 4 + 4], axis=1), BF16)
                for rb in range(4):
                    r = jnp.dot(xk[rb * 512:(rb + 1) * 512], w, preferred_element_type=F32)
                    for cc in range(4):
                        sl = (half * 4 + cc, pl.ds(off + rb * 512, 512), slice(None))
                        old = jnp.where(first, 0.0, dst[sl])
                        dst[sl] = old + r[:, cc * 128:(cc + 1) * 128]
        stage_first(jnp.minimum(kt + 1, 7))
        return carry

    jax.lax.fori_loop(0, 8, p1_body, 0)

    for j in range(4):
        cp_c(j).wait()

    row = jax.lax.broadcasted_iota(jnp.int32, (TQ, TQ), 0)
    col = jax.lax.broadcasted_iota(jnp.int32, (TQ, TQ), 1)

    def pair_weights(pp, r0, n):
        ev = wp[pp, pl.ds(r0, n // 2, stride=2), :]
        od = wp[pp, pl.ds(r0 + 1, n // 2, stride=2), :]
        lo = (ev & jnp.uint32(0xFFFF)) | (od << 16)
        hi = (ev >> 16) | (od & jnp.uint32(0xFFFF0000))
        return lo, hi

    def stage_wk(pp):
        lo, hi = pair_weights(pp, 0, DC)
        wkst[0] = lo
        wkst[1] = hi

    for d in cp_p(0):
        d.wait()
    stage_wk(0)

    def p2_body(p, carry):
        @pl.when(p < NP - 1)
        def _():
            for d in cp_p(p + 1):
                d.wait()

        @pl.when(p < 8)
        def _():
            cp_wo(p).start()

        cp_wob(p, 0).start()
        cp_wob(p, 1).start()

        causal = col <= row
        wk = _bf(jnp.concatenate([wkst[0], wkst[1]], axis=1))
        wv = _bf(jnp.concatenate(pair_weights(p, DC, DC), axis=1))
        wq = _bf(jnp.concatenate(pair_weights(p, 2 * DC, M), axis=1))

        ks, vs, qs = {}, {}, {}
        done = {}
        never = p > NP

        def c_rows(i):
            return pltpu.bitcast(
                jnp.concatenate([cs_u[j, pl.ds(i * TQ // 2, TQ // 2), :] for j in range(4)], axis=1),
                BF16)

        def proj_k(i):
            ks[i] = _pack(jnp.dot(c_rows(i), wk, preferred_element_type=F32))

        def proj_v(i):
            vs[i] = _pack(jnp.dot(c_rows(i), wv, preferred_element_type=F32))

        def proj_q(i):
            xb = pltpu.bitcast(
                jnp.concatenate([xs_u[j, pl.ds(i * TQ // 2, TQ // 2), :] for j in range(8)], axis=1),
                BF16)
            q = jnp.dot(xb, wq, preferred_element_type=F32) * (DA ** -0.5 * LOG2E)
            qs[i] = _pack(q)

        def qk(h, i, dep):
            hs = slice(h * DA, (h + 1) * DA)
            kk = _bf(jnp.concatenate([ks[j][:, hs] for j in range(i + 1)], axis=0))
            q = qs[i][:, hs]
            if dep is not None:
                q = jnp.where(never, done[(h, dep)], q)
            s = jax.lax.dot_general(_bf(q), kk, NT, preferred_element_type=F32)
            ch = _lane_chunks(s)
            ch[i] = jnp.where(causal, ch[i], NEG)
            return ch

        def softmax_pv(h, i, ch):
            hs = slice(h * DA, (h + 1) * DA)
            m = jnp.max(_fold(ch, jnp.maximum), axis=1, keepdims=True)
            ps = [jnp.exp2(c - m) for c in ch]
            lp = _fold(ps, jnp.add)
            pb = jnp.concatenate(ps, axis=1).astype(BF16)
            vv = _bf(jnp.concatenate([vs[j][:, hs] for j in range(i + 1)], axis=0))
            o = jnp.dot(pb, vv, preferred_element_type=F32)
            if i >= LDEP:
                lp = jnp.where(never, o, lp)
            l = jnp.sum(lp, axis=1, keepdims=True)
            r = pl.reciprocal(l, approx=True)
            r = r * (2.0 - l * r)
            cn = _pack(o * r)
            done[(h, i)] = cn
            ctx[2 * p + h, pl.ds(i * TQ // 2, TQ // 2), :] = cn

        for j in range(NLAST + 1):
            proj_k(j)
        proj_q(NLAST)
        for j in range(NLAST):
            proj_v(j)
        for i in range(NLAST, NQ):
            dep = i - DEP if i - DEP >= NLAST else None
            s0 = qk(0, i, dep)
            s1 = qk(1, i, dep)
            late = []
            if i + 1 < NQ:
                proj_v(i)
                proj_k(i + 1)
                proj_q(i + 1)
            else:
                stage_wk(jnp.minimum(p + 1, NP - 1))
                proj_q(NLAST - 1)
                for j in range(NLAST - 1, -1, -1):
                    if j > 0:
                        proj_q(j - 1)
                    else:
                        proj_v(i)
                    dep = NQ - 2 if j == 0 else None
                    late.append((j, qk(0, j, dep), qk(1, j, dep)))
            softmax_pv(0, i, s0)
            softmax_pv(1, i, s1)
            for j, t0, t1 in late:
                softmax_pv(0, j, t0)
                softmax_pv(1, j, t1)
        return carry

    jax.lax.fori_loop(0, NP, p2_body, 0)

    for j in range(8):
        cp_wo(j).wait()
    for dp in range(16):
        cp_wob(dp, 0).wait()
        cp_wob(dp, 1).wait()
    gw = gw_ref[...].astype(F32)
    RB = 16
    rowi = jax.lax.broadcasted_iota(jnp.int32, (RB, 128), 0)
    odd = (jax.lax.broadcasted_iota(jnp.int32, (RB, 128), 1) & 1) == 1

    def p3_body(i, carry):
        r0 = pl.multiple_of(i * TO, TO)
        h0 = pl.multiple_of(i * (TO // 2), TO // 2)
        ca = pltpu.bitcast(
            jnp.concatenate([ctx[h, pl.ds(h0, TO // 2), :] for h in range(HA)], axis=1), BF16)
        wa = pltpu.bitcast(jnp.concatenate([wo_s[j] for j in range(8)], axis=1), BF16)
        a = jnp.dot(ca, wa, preferred_element_type=F32)

        gs = _fold([pltpu.bitcast(xs_u[j, pl.ds(h0, TO // 2), :], BF16).astype(F32) * gw[j:j + 1]
                    for j in range(8)], jnp.add)
        g = jax.nn.sigmoid(jnp.sum(gs, axis=1, keepdims=True))

        obs = []
        for rb in range(TO // RB):
            q = [qb[cc, pl.ds(r0 + rb * RB, RB), :] for cc in range(8)]
            lg = [_fold([q[cc] * kb[cc, pl.ds(r0 + (PAD + rb * RB - DIL * w), RB), :]
                         for cc in range(8)], jnp.add) for w in range(WIN)]
            lg = [t + pltpu.roll(t, 64, 1) for t in lg]
            lg = [t + jnp.where(odd, pltpu.roll(t, 1, 1), pltpu.roll(t, 127, 1)) for t in lg]
            lg = [t * (DB ** -0.5 * LOG2E) for t in lg]
            if rb == 0:
                lg = [lg[0]] + [jnp.where(rowi + r0 >= DIL * w, lg[w], NEG) for w in range(1, WIN)]
            m = _fold(lg, jnp.maximum)
            ps = [jnp.exp2(t - m) for t in lg]
            l = _fold(ps, jnp.add)
            r = pl.reciprocal(l, approx=True)
            r = r * (2.0 - l * r)
            ps = [t * r for t in ps]
            o = [_pack(_fold([ps[w] * vb[cc, pl.ds(r0 + (PAD + rb * RB - DIL * w), RB), :]
                              for w in range(WIN)], jnp.add)) for cc in range(8)]
            obs.append(jnp.concatenate(o, axis=1))
        ob = _bf(jnp.concatenate(obs, axis=0))
        wb = _bf(wob_p[...])
        b = jnp.dot(ob, wb, preferred_element_type=F32)
        out_s[pl.ds(r0, TO), :] = (g * a + (1.0 - g) * b).astype(BF16)
        cp_out(i).start()
        return carry

    jax.lax.fori_loop(0, S // TO, p3_body, 0)
    for i in range(S // TO):
        cp_out(i).wait()


@jax.jit
def pallas_gated_mix__compressed_kv_cla__sliding_local_dilated__prompt_kernel(
    A_x: jax.Array,
    A_c_kv: jax.Array,
    A_w_q: jax.Array,
    A_w_uk: jax.Array,
    A_w_uv: jax.Array,
    A_w_o: jax.Array,
    B_x: jax.Array,
    B_wqkv: jax.Array,
    B_wo: jax.Array,
    gate_w: jax.Array,
):
    del B_x
    any_spec = pl.BlockSpec(memory_space=pl.ANY)
    out = pl.pallas_call(
        _kernel,
        in_specs=[any_spec] * 8 + [pl.BlockSpec(memory_space=pltpu.VMEM)],
        out_specs=any_spec,
        out_shape=jax.ShapeDtypeStruct((S, M), BF16),
        scratch_shapes=[
            pltpu.VMEM((8, S // 2, 128), U32),
            pltpu.VMEM((4, S // 2, 128), U32),
            pltpu.VMEM((NP, 2 * DC + M, 128), U32),
            pltpu.VMEM((M, 3 * M), BF16),
            pltpu.VMEM((8, 64, 128), U32),
            pltpu.VMEM((8, S, 128), F32),
            pltpu.VMEM((8, S + PAD, 128), F32),
            pltpu.VMEM((8, S + PAD, 128), F32),
            pltpu.VMEM((HA, S // 2, 128), U32),
            pltpu.VMEM((8, HA * DA // 2, 128), U32),
            pltpu.VMEM((M // 2, M), U32),
            pltpu.VMEM((2, DC // 2, 128), U32),
            pltpu.VMEM((S, M), BF16),
            pltpu.SemaphoreType.DMA((8,)),
            pltpu.SemaphoreType.DMA((8,)),
            pltpu.SemaphoreType.DMA((1,)),
            pltpu.SemaphoreType.DMA((NP,)),
            pltpu.SemaphoreType.DMA((2,)),
            pltpu.SemaphoreType.DMA((S // TO,)),
        ],
        compiler_params=pltpu.CompilerParams(vmem_limit_bytes=120 * 1024 * 1024,
                                             disable_bounds_checks=True),
    )(
        A_x.reshape(S, M),
        A_c_kv.reshape(S, DC),
        A_w_q,
        A_w_uk,
        A_w_uv,
        A_w_o.reshape(HA * DA, M),
        B_wqkv,
        B_wo.reshape(HB // 2, 2, DB, M),
        gate_w.reshape(8, 128),
    )
    return out.reshape(1, S, M)
```

```python
import functools
import math

import jax
import jax.numpy as jnp
import jax.experimental.pallas as pl
import jax.experimental.pallas.tpu as pltpu

F32 = jnp.float32
BF16 = jnp.bfloat16
U32 = jnp.uint32

S = 2048
M = 1024
HA = 32
DA = 128
DC = 512
HB = 32
DB = 32
WIN = 8
DIL = 2
PAD = 16
LOG2E = math.log2(math.e)
NEG = -1e9

TQ = 128
NQ = S // TQ
NP = HA // 2
DEP = 2
LDEP = 3
NLAST = 3
TO = 128
NT = (((1,), (1,)), ((), ()))

_STAGES = ((2, 4), (1, 3), (0, 2), (0, 6), (0, 1))


def _permute8(cols):
    cols = list(cols)
    lane = jax.lax.broadcasted_iota(jnp.int32, cols[0].shape, 1)
    for va, lb in _STAGES:
        lo = (lane & (1 << lb)) == 0
        sh = 1 << lb
        idx = [i for i in range(8) if not (i >> va) & 1]
        if lb == 6:
            rr = [pltpu.roll(jnp.where(lo, cols[i | (1 << va)], cols[i]), 64, 1) for i in idx]
            for i, r in zip(idx, rr):
                a, b = cols[i], cols[i | (1 << va)]
                cols[i] = jnp.where(lo, a, r)
                cols[i | (1 << va)] = jnp.where(lo, r, b)
        else:
            rb = [pltpu.roll(cols[i | (1 << va)], sh, 1) for i in idx]
            ra = [pltpu.roll(cols[i], 128 - sh, 1) for i in idx]
            for i, xa, xb in zip(idx, ra, rb):
                a, b = cols[i], cols[i | (1 << va)]
                cols[i] = jnp.where(lo, a, xb)
                cols[i | (1 << va)] = jnp.where(lo, xa, b)
    return cols


def _pack(x):
    return pltpu.bitcast(x.astype(BF16), U32)


def _bf(x):
    return pltpu.bitcast(x, BF16)


def _fold(xs, op):
    acc = xs[0]
    for x in xs[1:]:
        acc = op(acc, x)
    return acc


def _lane_chunks(x):
    return [x[:, j * 128:(j + 1) * 128] for j in range(x.shape[1] // 128)]


def _kernel(x_hbm, c_hbm, wq_hbm, wuk_hbm, wuv_hbm, wo_hbm, wqkv_hbm, wob_hbm, gw_hbm,
            out_hbm,
            xs_u, cs_u, wp, wraw, wperm, qb, kb, vb, ctx, wo_s, wob_p, wkst, out_s, gw_ref,
            sem_x, sem_a):
    x_u = x_hbm.bitcast(U32)
    c_u = c_hbm.bitcast(U32)
    wo_u = wo_hbm.bitcast(U32)
    wq_u = wq_hbm.bitcast(U32)
    wuk_u = wuk_hbm.bitcast(U32)
    wuv_u = wuv_hbm.bitcast(U32)
    wob_u = wob_hbm.bitcast(U32)

    def strip(j):
        return pl.ds(pl.multiple_of(j * 128, 128), 128)

    def cp_x(j):
        return pltpu.make_async_copy(x_u.at[:, strip(j)], xs_u.at[j], sem_x.at[j & 1])

    def cp_wa(j, sem):
        return pltpu.make_async_copy(wqkv_hbm.at[strip(j), pl.ds(0, M)],
                                     wraw.at[strip(j), pl.ds(0, M)], sem)

    def cp_wb(j):
        return pltpu.make_async_copy(wqkv_hbm.at[strip(j), pl.ds(M, 2 * M)],
                                     wraw.at[strip(j), pl.ds(M, 2 * M)], sem_x.at[2 + (j & 1)])

    def cp_c(j):
        return pltpu.make_async_copy(c_u.at[:, strip(j)], cs_u.at[j], sem_a.at[0])

    def cp_p(p):
        return (
            pltpu.make_async_copy(wuk_u.at[:, p, :], wp.at[p, pl.ds(0, DC), :], sem_a.at[0]),
            pltpu.make_async_copy(wuv_u.at[:, p, :], wp.at[p, pl.ds(DC, DC), :], sem_a.at[0]),
            pltpu.make_async_copy(wq_u.at[:, p, :], wp.at[p, pl.ds(2 * DC, M), :], sem_a.at[0]),
        )

    def cp_wo(j):
        return pltpu.make_async_copy(wo_u.at[:, strip(j)], wo_s.at[j], sem_a.at[1])

    def cp_wob(dp, h0):
        pos = ((dp >> 2) << 3) + ((dp & 1) << 2) + (dp & 2) + h0
        return pltpu.make_async_copy(wob_u.at[:, h0, dp, :],
                                     wob_p.at[pl.ds(pl.multiple_of(pos * 16, 16), 16), :],
                                     sem_a.at[1])

    def cp_gw():
        return pltpu.make_async_copy(gw_hbm, gw_ref, sem_a.at[1])

    def cp_out(i):
        r0 = pl.multiple_of(i * TO, TO)
        return pltpu.make_async_copy(out_s.at[pl.ds(r0, TO), :], out_hbm.at[pl.ds(r0, TO), :],
                                     sem_a.at[2])

    def start_group(j):
        cp_x(j).start()
        cp_wb(j).start()

    cp_wa(0, sem_a.at[2]).start()
    start_group(0)
    cp_wa(1, sem_x.at[2]).start()

    for cc in range(8):
        kb[cc, pl.ds(0, PAD), :] = jnp.zeros((PAD, 128), F32)
        vb[cc, pl.ds(0, PAD), :] = jnp.zeros((PAD, 128), F32)

    def permuted(kt, sec):
        r0 = pl.multiple_of(kt * 128, 128)
        w = pltpu.bitcast(wraw[pl.ds(r0, 128), pl.ds(sec * M, M)], U32)
        return _permute8(_lane_chunks(w))

    def stage_first(kt):
        for cc, t in enumerate(permuted(kt, 0)):
            wperm[cc] = t

    cp_wa(0, sem_a.at[2]).wait()
    stage_first(0)

    def p1_body(kt, carry):
        cp_x(kt).wait()

        def wait_w():
            cp_wb(kt).wait()

            @pl.when(kt < 7)
            def _():
                cp_wa(kt + 1, sem_x.at[2 + (kt & 1)]).wait()

            @pl.when(kt == 0)
            def _():
                start_group(1)
                cp_wa(2, sem_x.at[3]).start()

        wait_w()
        first = kt == 0
        xk = pltpu.bitcast(xs_u[kt], BF16)
        for sec, (dst, off) in enumerate(((qb, 0), (kb, PAD), (vb, PAD))):
            cols = [wperm[cc] for cc in range(8)] if sec == 0 else permuted(kt, sec)
            for half in range(2):
                w = pltpu.bitcast(jnp.concatenate(cols[half * 4:half * 4 + 4], axis=1), BF16)
                for rb in range(4):
                    r = jnp.dot(xk[rb * 512:(rb + 1) * 512], w, preferred_element_type=F32)
                    for cc in range(4):
                        sl = (half * 4 + cc, pl.ds(off + rb * 512, 512), slice(None))
                        old = jnp.where(first, 0.0, dst[sl])
                        dst[sl] = old + r[:, cc * 128:(cc + 1) * 128]
        stage_first(jnp.minimum(kt + 1, 7))

        @pl.when(kt < 6)
        def _():
            start_group(kt + 2)

        @pl.when(kt < 5)
        def _():
            cp_wa(kt + 3, sem_x.at[2 + (kt & 1)]).start()

        @pl.when(kt < 4)
        def _():
            cp_c(kt).start()
            for e in range(4):
                for d in cp_p(4 * kt + e):
                    d.start()

        @pl.when(kt >= 4)
        def _():
            cp_wo(2 * kt - 8).start()
            cp_wo(2 * kt - 7).start()

        return carry

    jax.lax.fori_loop(0, 8, p1_body, 0)

    for j in range(4):
        cp_c(j).wait()
    for pp in range(NP):
        for d in cp_p(pp):
            d.wait()

    row = jax.lax.broadcasted_iota(jnp.int32, (TQ, TQ), 0)
    col = jax.lax.broadcasted_iota(jnp.int32, (TQ, TQ), 1)

    def pair_weights(pp, r0, n):
        ev = wp[pp, pl.ds(r0, n // 2, stride=2), :]
        od = wp[pp, pl.ds(r0 + 1, n // 2, stride=2), :]
        lo = (ev & jnp.uint32(0xFFFF)) | (od << 16)
        hi = (ev >> 16) | (od & jnp.uint32(0xFFFF0000))
        return lo, hi

    def stage_wk(pp):
        lo, hi = pair_weights(pp, 0, DC)
        wkst[0] = lo
        wkst[1] = hi

    cp_gw().start()
    for dp in range(16):
        cp_wob(dp, 0).start()
        cp_wob(dp, 1).start()
    stage_wk(0)

    def p2_body(p, carry):
        causal = col <= row
        wv = _bf(jnp.concatenate(pair_weights(p, DC, DC), axis=1))
        wq = _bf(jnp.concatenate(pair_weights(p, 2 * DC, M), axis=1))

        ks, vs, qs = {}, {}, {}
        done = {}
        never = p > NP

        def c_rows(i):
            return pltpu.bitcast(
                jnp.concatenate([cs_u[j, pl.ds(i * TQ // 2, TQ // 2), :] for j in range(4)], axis=1),
                BF16)

        def proj_k(i):
            wk = _bf(jnp.concatenate([wkst[0], wkst[1]], axis=1))
            ks[i] = _pack(jnp.dot(c_rows(i), wk, preferred_element_type=F32))

        def proj_v(i):
            vs[i] = _pack(jnp.dot(c_rows(i), wv, preferred_element_type=F32))

        def proj_q(i):
            xb = pltpu.bitcast(
                jnp.concatenate([xs_u[j, pl.ds(i * TQ // 2, TQ // 2), :] for j in range(8)], axis=1),
                BF16)
            q = jnp.dot(xb, wq, preferred_element_type=F32) * (DA ** -0.5 * LOG2E)
            qs[i] = _pack(q)

        def qk(h, i, dep):
            hs = slice(h * DA, (h + 1) * DA)
            kk = _bf(jnp.concatenate([ks[j][:, hs] for j in range(i + 1)], axis=0))
            q = qs[i][:, hs]
            if dep is not None:
                q = jnp.where(never, done[(h, dep)], q)
            s = jax.lax.dot_general(_bf(q), kk, NT, preferred_element_type=F32)
            ch = _lane_chunks(s)
            ch[i] = jnp.where(causal, ch[i], NEG)
            return ch

        def softmax_pv(h, i, ch):
            hs = slice(h * DA, (h + 1) * DA)
            m = jnp.max(_fold(ch, jnp.maximum), axis=1, keepdims=True)
            ps = [jnp.exp2(c - m) for c in ch]
            lp = _fold(ps, jnp.add)
            pb = jnp.concatenate(ps, axis=1).astype(BF16)
            vv = _bf(jnp.concatenate([vs[j][:, hs] for j in range(i + 1)], axis=0))
            o = jnp.dot(pb, vv, preferred_element_type=F32)
            if i >= LDEP:
                lp = jnp.where(never, o, lp)
            l = jnp.sum(lp, axis=1, keepdims=True)
            r = pl.reciprocal(l, approx=True)
            r = r * (2.0 - l * r)
            cn = _pack(o * r)
            done[(h, i)] = cn
            ctx[2 * p + h, pl.ds(i * TQ // 2, TQ // 2), :] = cn

        for j in range(NLAST + 1):
            proj_k(j)
        proj_q(NLAST)
        for j in range(NLAST):
            proj_v(j)
        for i in range(NLAST, NQ):
            dep = i - DEP if i - DEP >= NLAST else None
            s0 = qk(0, i, dep)
            s1 = qk(1, i, dep)
            late = []
            if i + 1 < NQ:
                proj_v(i)
                proj_k(i + 1)
                proj_q(i + 1)
            else:
                stage_wk(jnp.minimum(p + 1, NP - 1))
                proj_q(NLAST - 1)
                for j in range(NLAST - 1, -1, -1):
                    if j > 0:
                        proj_q(j - 1)
                    else:
                        proj_v(i)
                    dep = NQ - 2 if j == 0 else None
                    late.append((j, qk(0, j, dep), qk(1, j, dep)))
            softmax_pv(0, i, s0)
            softmax_pv(1, i, s1)
            for j, t0, t1 in late:
                softmax_pv(0, j, t0)
                softmax_pv(1, j, t1)
        return carry

    jax.lax.fori_loop(0, NP, p2_body, 0)

    cp_gw().wait()
    for j in range(8):
        cp_wo(j).wait()
    for dp in range(16):
        cp_wob(dp, 0).wait()
        cp_wob(dp, 1).wait()
    gw = gw_ref[...].astype(F32)
    RB = 16
    rowi = jax.lax.broadcasted_iota(jnp.int32, (RB, 128), 0)
    odd = (jax.lax.broadcasted_iota(jnp.int32, (RB, 128), 1) & 1) == 1

    def p3_body(i, carry):
        r0 = pl.multiple_of(i * TO, TO)
        h0 = pl.multiple_of(i * (TO // 2), TO // 2)
        ca = pltpu.bitcast(
            jnp.concatenate([ctx[h, pl.ds(h0, TO // 2), :] for h in range(HA)], axis=1), BF16)
        wa = pltpu.bitcast(jnp.concatenate([wo_s[j] for j in range(8)], axis=1), BF16)
        a = jnp.dot(ca, wa, preferred_element_type=F32)

        gs = _fold([pltpu.bitcast(xs_u[j, pl.ds(h0, TO // 2), :], BF16).astype(F32) * gw[j:j + 1]
                    for j in range(8)], jnp.add)
        g = jax.nn.sigmoid(jnp.sum(gs, axis=1, keepdims=True))

        obs = []
        for rb in range(TO // RB):
            q = [qb[cc, pl.ds(r0 + rb * RB, RB), :] for cc in range(8)]
            lg = [_fold([q[cc] * kb[cc, pl.ds(r0 + (PAD + rb * RB - DIL * w), RB), :]
                         for cc in range(8)], jnp.add) for w in range(WIN)]
            lg = [t + pltpu.roll(t, 64, 1) for t in lg]
            lg = [t + jnp.where(odd, pltpu.roll(t, 1, 1), pltpu.roll(t, 127, 1)) for t in lg]
            lg = [t * (DB ** -0.5 * LOG2E) for t in lg]
            if rb == 0:
                lg = [lg[0]] + [jnp.where(rowi + r0 >= DIL * w, lg[w], NEG) for w in range(1, WIN)]
            m = _fold(lg, jnp.maximum)
            ps = [jnp.exp2(t - m) for t in lg]
            l = _fold(ps, jnp.add)
            r = pl.reciprocal(l, approx=True)
            r = r * (2.0 - l * r)
            ps = [t * r for t in ps]
            o = [_pack(_fold([ps[w] * vb[cc, pl.ds(r0 + (PAD + rb * RB - DIL * w), RB), :]
                              for w in range(WIN)], jnp.add)) for cc in range(8)]
            obs.append(jnp.concatenate(o, axis=1))
        ob = _bf(jnp.concatenate(obs, axis=0))
        wb = _bf(wob_p[...])
        b = jnp.dot(ob, wb, preferred_element_type=F32)
        out_s[pl.ds(r0, TO), :] = (g * a + (1.0 - g) * b).astype(BF16)
        cp_out(i).start()
        return carry

    jax.lax.fori_loop(0, S // TO, p3_body, 0)
    for i in range(S // TO):
        cp_out(i).wait()


@jax.jit
def pallas_gated_mix__compressed_kv_cla__sliding_local_dilated__prompt_kernel(
    A_x: jax.Array,
    A_c_kv: jax.Array,
    A_w_q: jax.Array,
    A_w_uk: jax.Array,
    A_w_uv: jax.Array,
    A_w_o: jax.Array,
    B_x: jax.Array,
    B_wqkv: jax.Array,
    B_wo: jax.Array,
    gate_w: jax.Array,
):
    del B_x
    any_spec = pl.BlockSpec(memory_space=pl.ANY)
    out = pl.pallas_call(
        _kernel,
        in_specs=[any_spec] * 9,
        out_specs=any_spec,
        out_shape=jax.ShapeDtypeStruct((S, M), BF16),
        scratch_shapes=[
            pltpu.VMEM((8, S // 2, 128), U32),
            pltpu.VMEM((4, S // 2, 128), U32),
            pltpu.VMEM((NP, 2 * DC + M, 128), U32),
            pltpu.VMEM((M, 3 * M), BF16),
            pltpu.VMEM((8, 64, 128), U32),
            pltpu.VMEM((8, S, 128), F32),
            pltpu.VMEM((8, S + PAD, 128), F32),
            pltpu.VMEM((8, S + PAD, 128), F32),
            pltpu.VMEM((HA, S // 2, 128), U32),
            pltpu.VMEM((8, HA * DA // 2, 128), U32),
            pltpu.VMEM((M // 2, M), U32),
            pltpu.VMEM((2, DC // 2, 128), U32),
            pltpu.VMEM((S, M), BF16),
            pltpu.VMEM((8, 128), BF16),
            pltpu.SemaphoreType.DMA((4,)),
            pltpu.SemaphoreType.DMA((3,)),
        ],
        compiler_params=pltpu.CompilerParams(vmem_limit_bytes=120 * 1024 * 1024,
                                             disable_bounds_checks=True),
    )(
        A_x.reshape(S, M),
        A_c_kv.reshape(S, DC),
        A_w_q,
        A_w_uk,
        A_w_uv,
        A_w_o.reshape(HA * DA, M),
        B_wqkv,
        B_wo.reshape(HB // 2, 2, DB, M),
        gate_w.reshape(8, 128),
    )
    return out.reshape(1, S, M)
```

```python
import functools
import math

import jax
import jax.numpy as jnp
import jax.experimental.pallas as pl
import jax.experimental.pallas.tpu as pltpu

F32 = jnp.float32
BF16 = jnp.bfloat16
U32 = jnp.uint32

S = 2048
M = 1024
HA = 32
DA = 128
DC = 512
HB = 32
DB = 32
WIN = 8
DIL = 2
PAD = 16
LOG2E = math.log2(math.e)
NEG = -1e9

TQ = 128
NQ = S // TQ
NP = HA // 2
DEP = 2
H_START = 0
H_FIN = 0
RB = 16
LDEP = 3
NLAST = 3
TO = 256
NT = (((1,), (1,)), ((), ()))

_STAGES = ((2, 4), (1, 3), (0, 2), (0, 6), (0, 1))


def _permute8(cols):
    cols = list(cols)
    lane = jax.lax.broadcasted_iota(jnp.int32, cols[0].shape, 1)
    for va, lb in _STAGES:
        lo = (lane & (1 << lb)) == 0
        sh = 1 << lb
        idx = [i for i in range(8) if not (i >> va) & 1]
        if lb == 6:
            rr = [pltpu.roll(jnp.where(lo, cols[i | (1 << va)], cols[i]), 64, 1) for i in idx]
            for i, r in zip(idx, rr):
                a, b = cols[i], cols[i | (1 << va)]
                cols[i] = jnp.where(lo, a, r)
                cols[i | (1 << va)] = jnp.where(lo, r, b)
        else:
            rb = [pltpu.roll(cols[i | (1 << va)], sh, 1) for i in idx]
            ra = [pltpu.roll(cols[i], 128 - sh, 1) for i in idx]
            for i, xa, xb in zip(idx, ra, rb):
                a, b = cols[i], cols[i | (1 << va)]
                cols[i] = jnp.where(lo, a, xb)
                cols[i | (1 << va)] = jnp.where(lo, xa, b)
    return cols


def _pack(x):
    return pltpu.bitcast(x.astype(BF16), U32)


def _bf(x):
    return pltpu.bitcast(x, BF16)


def _fold(xs, op):
    acc = xs[0]
    for x in xs[1:]:
        acc = op(acc, x)
    return acc


def _lane_chunks(x):
    return [x[:, j * 128:(j + 1) * 128] for j in range(x.shape[1] // 128)]


def _kernel(x_hbm, c_hbm, wq_hbm, wuk_hbm, wuv_hbm, wo_hbm, wqkv_hbm, wob_hbm, gw_hbm,
            out_hbm,
            xs_u, cs_u, wp, wraw, wperm, qb, kb, vb, ctx, wo_s, wob_p, wkst, out_s, gw_ref,
            sem_x, sem_a):
    x_u = x_hbm.bitcast(U32)
    c_u = c_hbm.bitcast(U32)
    wo_u = wo_hbm.bitcast(U32)
    wq_u = wq_hbm.bitcast(U32)
    wuk_u = wuk_hbm.bitcast(U32)
    wuv_u = wuv_hbm.bitcast(U32)
    wob_u = wob_hbm.bitcast(U32)

    def strip(j):
        return pl.ds(pl.multiple_of(j * 128, 128), 128)

    def cp_x(t):
        rows = pl.ds(pl.multiple_of((t & 1) * (S // 4), S // 4), S // 4)
        return pltpu.make_async_copy(x_u.at[rows, strip(t >> 1)], xs_u.at[t >> 1, rows, :],
                                     sem_x.at[t & 1])

    def cp_wa(j, sem):
        return pltpu.make_async_copy(wqkv_hbm.at[strip(j), pl.ds(0, M)],
                                     wraw.at[strip(j), pl.ds(0, M)], sem)

    def cp_wb(j):
        return pltpu.make_async_copy(wqkv_hbm.at[strip(j), pl.ds(M, 2 * M)],
                                     wraw.at[strip(j), pl.ds(M, 2 * M)], sem_x.at[0])

    def cp_c(j):
        return pltpu.make_async_copy(c_u.at[:, strip(j)], cs_u.at[j], sem_a.at[0])

    def cp_p(p):
        return (
            pltpu.make_async_copy(wuk_u.at[:, p, :], wp.at[p, pl.ds(0, DC), :], sem_a.at[0]),
            pltpu.make_async_copy(wuv_u.at[:, p, :], wp.at[p, pl.ds(DC, DC), :], sem_a.at[0]),
            pltpu.make_async_copy(wq_u.at[:, p, :], wp.at[p, pl.ds(2 * DC, M), :], sem_a.at[0]),
        )

    def cp_wo(j):
        return pltpu.make_async_copy(wo_u.at[:, strip(j)], wo_s.at[j], sem_a.at[1])

    def cp_wob(dp, h0):
        pos = ((dp >> 2) << 3) + ((dp & 1) << 2) + (dp & 2) + h0
        return pltpu.make_async_copy(wob_u.at[:, h0, dp, :],
                                     wob_p.at[pl.ds(pl.multiple_of(pos * 16, 16), 16), :],
                                     sem_a.at[1])

    def cp_gw():
        return pltpu.make_async_copy(gw_hbm, gw_ref, sem_a.at[1])

    def cp_out(i):
        r0 = pl.multiple_of(i * TO, TO)
        return pltpu.make_async_copy(out_s.at[pl.ds(r0, TO), :], out_hbm.at[pl.ds(r0, TO), :],
                                     sem_a.at[2])

    cp_wa(0, sem_a.at[2]).start()
    cp_x(0).start()
    cp_wb(0).start()

    for cc in range(8):
        kb[cc, pl.ds(0, PAD), :] = jnp.zeros((PAD, 128), F32)
        vb[cc, pl.ds(0, PAD), :] = jnp.zeros((PAD, 128), F32)

    def permuted(kt, sec):
        r0 = pl.multiple_of(kt * 128, 128)
        w = pltpu.bitcast(wraw[pl.ds(r0, 128), pl.ds(sec * M, M)], U32)
        return _permute8(_lane_chunks(w))

    def stage_first(kt):
        for cc, t in enumerate(permuted(kt, 0)):
            wperm[cc] = t

    cp_wa(0, sem_a.at[2]).wait()
    stage_first(0)

    def group(t, fn):
        fn(cp_x(t))

        @pl.when((t & 1) == 0)
        def _():
            fn(cp_wb(t >> 1))

        @pl.when(jnp.logical_and((t & 1) == 1, t < 15))
        def _():
            fn(cp_wa((t >> 1) + 1, sem_x.at[1]))

    def p1_body(t, carry):
        kt = t >> 1
        group(t, lambda d: d.wait())

        @pl.when(t < 15)
        def _():
            group(t + 1, lambda d: d.start())

        first = kt == 0
        w0 = pl.multiple_of((t & 1) * (S // 4), S // 4)
        r0 = pl.multiple_of((t & 1) * (S // 2), S // 2)
        xk = _bf(xs_u[kt, pl.ds(w0, S // 4), :])
        for sec, (dst, off) in enumerate(((qb, 0), (kb, PAD), (vb, PAD))):
            cols = [wperm[cc] for cc in range(8)] if sec == 0 else permuted(kt, sec)
            for half in range(2):
                w = _bf(jnp.concatenate(cols[half * 4:half * 4 + 4], axis=1))
                for rb in range(2):
                    r = jnp.dot(xk[rb * 512:(rb + 1) * 512], w, preferred_element_type=F32)
                    for cc in range(4):
                        sl = (half * 4 + cc, pl.ds(r0 + (off + rb * 512), 512), slice(None))
                        old = jnp.where(first, 0.0, dst[sl])
                        dst[sl] = old + r[:, cc * 128:(cc + 1) * 128]
        stage_first(jnp.minimum((t + 1) >> 1, 7))

        @pl.when(t < 4)
        def _():
            cp_c(t).start()

        @pl.when(t < 8)
        def _():
            for e in range(2):
                for d in cp_p(2 * t + e):
                    d.start()

        @pl.when(t >= 8)
        def _():
            cp_wo(t - 8).start()

        return carry

    jax.lax.fori_loop(0, 16, p1_body, 0)

    for j in range(4):
        cp_c(j).wait()
    for pp in range(NP):
        for d in cp_p(pp):
            d.wait()

    row = jax.lax.broadcasted_iota(jnp.int32, (TQ, TQ), 0)
    col = jax.lax.broadcasted_iota(jnp.int32, (TQ, TQ), 1)

    def pair_weights(pp, r0, n):
        ev = wp[pp, pl.ds(r0, n // 2, stride=2), :]
        od = wp[pp, pl.ds(r0 + 1, n // 2, stride=2), :]
        lo = (ev & jnp.uint32(0xFFFF)) | (od << 16)
        hi = (ev >> 16) | (od & jnp.uint32(0xFFFF0000))
        return lo, hi

    def stage_wk(pp):
        lo, hi = pair_weights(pp, 0, DC)
        wkst[0] = lo
        wkst[1] = hi

    cp_gw().start()
    for dp in range(16):
        cp_wob(dp, 0).start()
        cp_wob(dp, 1).start()
    stage_wk(0)

    def p2_body(p, carry):
        causal = col <= row
        wv = _bf(jnp.concatenate(pair_weights(p, DC, DC), axis=1))
        wq = _bf(jnp.concatenate(pair_weights(p, 2 * DC, M), axis=1))

        ks, vs, qs = {}, {}, {}
        done = {}
        never = p > NP

        def c_rows(i):
            return pltpu.bitcast(
                jnp.concatenate([cs_u[j, pl.ds(i * TQ // 2, TQ // 2), :] for j in range(4)], axis=1),
                BF16)

        def proj_k(i):
            wk = _bf(jnp.concatenate([wkst[0], wkst[1]], axis=1))
            ks[i] = _pack(jnp.dot(c_rows(i), wk, preferred_element_type=F32))

        def proj_v(i):
            vs[i] = _pack(jnp.dot(c_rows(i), wv, preferred_element_type=F32))

        def proj_q(i):
            xb = pltpu.bitcast(
                jnp.concatenate([xs_u[j, pl.ds(i * TQ // 2, TQ // 2), :] for j in range(8)], axis=1),
                BF16)
            q = jnp.dot(xb, wq, preferred_element_type=F32) * (DA ** -0.5 * LOG2E)
            qs[i] = _pack(q)

        def qk(h, i, dep):
            hs = slice(h * DA, (h + 1) * DA)
            kk = _bf(jnp.concatenate([ks[j][:, hs] for j in range(i + 1)], axis=0))
            q = qs[i][:, hs]
            if dep is not None:
                q = jnp.where(never, done[(h, dep)], q)
            s = jax.lax.dot_general(_bf(q), kk, NT, preferred_element_type=F32)
            ch = _lane_chunks(s)
            ch[i] = jnp.where(causal, ch[i], NEG)
            return ch

        def softmax_pv(h, i, ch):
            hs = slice(h * DA, (h + 1) * DA)
            m = jnp.max(_fold(ch, jnp.maximum), axis=1, keepdims=True)
            ps = [jnp.exp2(c - m) for c in ch]
            lp = _fold(ps, jnp.add)
            pb = jnp.concatenate(ps, axis=1).astype(BF16)
            vv = _bf(jnp.concatenate([vs[j][:, hs] for j in range(i + 1)], axis=0))
            o = jnp.dot(pb, vv, preferred_element_type=F32)
            if i >= LDEP:
                lp = jnp.where(never, o, lp)
            l = jnp.sum(lp, axis=1, keepdims=True)
            r = pl.reciprocal(l, approx=True)
            r = r * (2.0 - l * r)
            cn = _pack(o * r)
            done[(h, i)] = cn
            ctx[2 * p + h, pl.ds(i * TQ // 2, TQ // 2), :] = cn

        for j in range(NLAST + 1):
            proj_k(j)
        proj_q(NLAST)
        for j in range(NLAST):
            proj_v(j)
        for i in range(NLAST, NQ):
            dep = i - DEP if i - DEP >= NLAST else None
            s0 = qk(0, i, dep)
            s1 = qk(1, i, dep)
            late = []
            if i + 1 < NQ:
                proj_v(i)
                proj_k(i + 1)
                proj_q(i + 1)
            else:
                stage_wk(jnp.minimum(p + 1, NP - 1))
                proj_q(NLAST - 1)
                for j in range(NLAST - 1, -1, -1):
                    if j > 0:
                        proj_q(j - 1)
                    else:
                        proj_v(i)
                    dep = NQ - 2 if j == 0 else None
                    late.append((j, qk(0, j, dep), qk(1, j, dep)))
            softmax_pv(0, i, s0)
            softmax_pv(1, i, s1)
            for j, t0, t1 in late:
                softmax_pv(0, j, t0)
                softmax_pv(1, j, t1)
        return carry

    jax.lax.fori_loop(0, NP, p2_body, 0)

    cp_gw().wait()
    for j in range(8):
        cp_wo(j).wait()
    for dp in range(16):
        cp_wob(dp, 0).wait()
        cp_wob(dp, 1).wait()
    gw = gw_ref[...].astype(F32)
    rowi = jax.lax.broadcasted_iota(jnp.int32, (RB, 128), 0)
    odd = (jax.lax.broadcasted_iota(jnp.int32, (RB, 128), 1) & 1) == 1

    NSUB = TO // RB
    PER = NSUB // 8

    def p3_body(i, carry):
        r0 = pl.multiple_of(i * TO, TO)
        h0 = pl.multiple_of(i * (TO // 2), TO // 2)
        never = i > S

        def local(rb, after):
            q = [qb[cc, pl.ds(r0 + rb * RB, RB), :] for cc in range(8)]
            if after is not None and H_START:
                q = [jnp.where(never, after[cc * RB:(cc + 1) * RB], q[cc]) for cc in range(8)]
            lg = [_fold([q[cc] * kb[cc, pl.ds(r0 + (PAD + rb * RB - DIL * w), RB), :]
                         for cc in range(8)], jnp.add) for w in range(WIN)]
            lg = [t + pltpu.roll(t, 64, 1) for t in lg]
            lg = [t + jnp.where(odd, pltpu.roll(t, 1, 1), pltpu.roll(t, 127, 1)) for t in lg]
            lg = [t * (DB ** -0.5 * LOG2E) for t in lg]
            if rb == 0:
                lg = [lg[0]] + [jnp.where(rowi + r0 >= DIL * w, lg[w], NEG) for w in range(1, WIN)]
            m = _fold(lg, jnp.maximum)
            ps = [jnp.exp2(t - m) for t in lg]
            l = _fold(ps, jnp.add)
            r = pl.reciprocal(l, approx=True)
            r = r * (2.0 - l * r)
            ps = [t * r for t in ps]
            o = [_pack(_fold([ps[w] * vb[cc, pl.ds(r0 + (PAD + rb * RB - DIL * w), RB), :]
                              for w in range(WIN)], jnp.add)) for cc in range(8)]
            return jnp.concatenate(o, axis=1)

        ca = jnp.concatenate([ctx[h, pl.ds(h0, TO // 2), :] for h in range(HA)], axis=1)
        obs, acs = [], []
        for j in range(8):
            lhs = ca
            if j >= 2 and H_FIN:
                dep = jnp.concatenate(obs[(j - 2) * PER:(j - 1) * PER], axis=0)
                n = dep.shape[0]
                top = jnp.concatenate([jnp.where(never, dep, ca[:n, :M]), ca[:n, M:]], axis=1)
                lhs = jnp.concatenate([top, ca[n:]], axis=0)
            acs.append(jnp.dot(_bf(lhs), _bf(wo_s[j]), preferred_element_type=F32))
            for e in range(PER):
                obs.append(local(j * PER + e, acs[j - 1] if j >= 1 else None))
        a = jnp.concatenate(acs, axis=1)

        gs = _fold([_bf(xs_u[j, pl.ds(h0, TO // 2), :]).astype(F32) * gw[j:j + 1]
                    for j in range(8)], jnp.add)
        g = jax.nn.sigmoid(jnp.sum(gs, axis=1, keepdims=True))

        ob = _bf(jnp.concatenate(obs, axis=0))
        b = jnp.dot(ob, _bf(wob_p[...]), preferred_element_type=F32)
        out_s[pl.ds(r0, TO), :] = (g * a + (1.0 - g) * b).astype(BF16)
        cp_out(i).start()
        return carry

    jax.lax.fori_loop(0, S // TO, p3_body, 0)
    for i in range(S // TO):
        cp_out(i).wait()


@jax.jit
def pallas_gated_mix__compressed_kv_cla__sliding_local_dilated__prompt_kernel(
    A_x: jax.Array,
    A_c_kv: jax.Array,
    A_w_q: jax.Array,
    A_w_uk: jax.Array,
    A_w_uv: jax.Array,
    A_w_o: jax.Array,
    B_x: jax.Array,
    B_wqkv: jax.Array,
    B_wo: jax.Array,
    gate_w: jax.Array,
):
    del B_x
    any_spec = pl.BlockSpec(memory_space=pl.ANY)
    out = pl.pallas_call(
        _kernel,
        in_specs=[any_spec] * 9,
        out_specs=any_spec,
        out_shape=jax.ShapeDtypeStruct((S, M), BF16),
        scratch_shapes=[
            pltpu.VMEM((8, S // 2, 128), U32),
            pltpu.VMEM((4, S // 2, 128), U32),
            pltpu.VMEM((NP, 2 * DC + M, 128), U32),
            pltpu.VMEM((M, 3 * M), BF16),
            pltpu.VMEM((8, 64, 128), U32),
            pltpu.VMEM((8, S, 128), F32),
            pltpu.VMEM((8, S + PAD, 128), F32),
            pltpu.VMEM((8, S + PAD, 128), F32),
            pltpu.VMEM((HA, S // 2, 128), U32),
            pltpu.VMEM((8, HA * DA // 2, 128), U32),
            pltpu.VMEM((M // 2, M), U32),
            pltpu.VMEM((2, DC // 2, 128), U32),
            pltpu.VMEM((S, M), BF16),
            pltpu.VMEM((8, 128), BF16),
            pltpu.SemaphoreType.DMA((2,)),
            pltpu.SemaphoreType.DMA((3,)),
        ],
        compiler_params=pltpu.CompilerParams(vmem_limit_bytes=120 * 1024 * 1024,
                                             disable_bounds_checks=True),
    )(
        A_x.reshape(S, M),
        A_c_kv.reshape(S, DC),
        A_w_q,
        A_w_uk,
        A_w_uv,
        A_w_o.reshape(HA * DA, M),
        B_wqkv,
        B_wo.reshape(HB // 2, 2, DB, M),
        gate_w.reshape(8, 128),
    )
    return out.reshape(1, S, M)
```

```python
import functools
import math

import jax
import jax.numpy as jnp
import jax.experimental.pallas as pl
import jax.experimental.pallas.tpu as pltpu

F32 = jnp.float32
BF16 = jnp.bfloat16
U32 = jnp.uint32

S = 2048
M = 1024
HA = 32
DA = 128
DC = 512
HB = 32
DB = 32
WIN = 8
DIL = 2
PAD = 16
LOG2E = math.log2(math.e)
NEG = -1e9

TQ = 128
NQ = S // TQ
NP = HA // 2
DEP = 2
TIE = 4
H_START = 0
H_FIN = 0
RB = 16
LDEP = 4
NLAST = 4
TO = 256
NT = (((1,), (1,)), ((), ()))

_STAGES = ((2, 4), (1, 3), (0, 2), (0, 6), (0, 1))


def _permute8(cols):
    cols = list(cols)
    lane = jax.lax.broadcasted_iota(jnp.int32, cols[0].shape, 1)
    for va, lb in _STAGES:
        lo = (lane & (1 << lb)) == 0
        sh = 1 << lb
        idx = [i for i in range(8) if not (i >> va) & 1]
        if lb == 6:
            rr = [pltpu.roll(jnp.where(lo, cols[i | (1 << va)], cols[i]), 64, 1) for i in idx]
            for i, r in zip(idx, rr):
                a, b = cols[i], cols[i | (1 << va)]
                cols[i] = jnp.where(lo, a, r)
                cols[i | (1 << va)] = jnp.where(lo, r, b)
        else:
            rb = [pltpu.roll(cols[i | (1 << va)], sh, 1) for i in idx]
            ra = [pltpu.roll(cols[i], 128 - sh, 1) for i in idx]
            for i, xa, xb in zip(idx, ra, rb):
                a, b = cols[i], cols[i | (1 << va)]
                cols[i] = jnp.where(lo, a, xb)
                cols[i | (1 << va)] = jnp.where(lo, xa, b)
    return cols


def _pack(x):
    return pltpu.bitcast(x.astype(BF16), U32)


def _bf(x):
    return pltpu.bitcast(x, BF16)


def _fold(xs, op):
    acc = xs[0]
    for x in xs[1:]:
        acc = op(acc, x)
    return acc


def _lane_chunks(x):
    return [x[:, j * 128:(j + 1) * 128] for j in range(x.shape[1] // 128)]


def _kernel(x_hbm, c_hbm, wq_hbm, wuk_hbm, wuv_hbm, wo_hbm, wqkv_hbm, wob_hbm, gw_hbm,
            out_hbm,
            xs_u, cs_u, wp, wraw, wperm, qb, kb, vb, ctx, wo_s, wob_p, wkst, out_s, gw_ref,
            sem_x, sem_a):
    x_u = x_hbm.bitcast(U32)
    c_u = c_hbm.bitcast(U32)
    wo_u = wo_hbm.bitcast(U32)
    wq_u = wq_hbm.bitcast(U32)
    wuk_u = wuk_hbm.bitcast(U32)
    wuv_u = wuv_hbm.bitcast(U32)
    wob_u = wob_hbm.bitcast(U32)

    def strip(j):
        return pl.ds(pl.multiple_of(j * 128, 128), 128)

    def cp_x(t):
        rows = pl.ds(pl.multiple_of((t & 1) * (S // 4), S // 4), S // 4)
        return pltpu.make_async_copy(x_u.at[rows, strip(t >> 1)], xs_u.at[t >> 1, rows, :],
                                     sem_x.at[t & 1])

    def cp_wa(j, sem):
        return pltpu.make_async_copy(wqkv_hbm.at[strip(j), pl.ds(0, M)],
                                     wraw.at[strip(j), pl.ds(0, M)], sem)

    def cp_wb(j):
        return pltpu.make_async_copy(wqkv_hbm.at[strip(j), pl.ds(M, 2 * M)],
                                     wraw.at[strip(j), pl.ds(M, 2 * M)], sem_x.at[0])

    def cp_c(j):
        return pltpu.make_async_copy(c_u.at[:, strip(j)], cs_u.at[j], sem_a.at[0])

    def cp_p(p):
        return (
            pltpu.make_async_copy(wuk_u.at[:, p, :], wp.at[p, pl.ds(0, DC), :], sem_a.at[0]),
            pltpu.make_async_copy(wuv_u.at[:, p, :], wp.at[p, pl.ds(DC, DC), :], sem_a.at[0]),
            pltpu.make_async_copy(wq_u.at[:, p, :], wp.at[p, pl.ds(2 * DC, M), :], sem_a.at[0]),
        )

    def cp_wo(j):
        return pltpu.make_async_copy(wo_u.at[:, strip(j)], wo_s.at[j], sem_a.at[1])

    def cp_wob(dp, h0):
        pos = ((dp >> 2) << 3) + ((dp & 1) << 2) + (dp & 2) + h0
        return pltpu.make_async_copy(wob_u.at[:, h0, dp, :],
                                     wob_p.at[pl.ds(pl.multiple_of(pos * 16, 16), 16), :],
                                     sem_a.at[1])

    def cp_gw():
        return pltpu.make_async_copy(gw_hbm, gw_ref, sem_a.at[1])

    def cp_out(i):
        r0 = pl.multiple_of(i * TO, TO)
        return pltpu.make_async_copy(out_s.at[pl.ds(r0, TO), :], out_hbm.at[pl.ds(r0, TO), :],
                                     sem_a.at[2])

    cp_wa(0, sem_a.at[2]).start()
    cp_x(0).start()
    cp_wb(0).start()

    for cc in range(8):
        kb[cc, pl.ds(0, PAD), :] = jnp.zeros((PAD, 128), F32)
        vb[cc, pl.ds(0, PAD), :] = jnp.zeros((PAD, 128), F32)

    def permuted(kt, sec):
        r0 = pl.multiple_of(kt * 128, 128)
        w = pltpu.bitcast(wraw[pl.ds(r0, 128), pl.ds(sec * M, M)], U32)
        return _permute8(_lane_chunks(w))

    def stage_first(kt):
        for cc, t in enumerate(permuted(kt, 0)):
            wperm[cc] = t

    cp_wa(0, sem_a.at[2]).wait()
    stage_first(0)

    def group(t, fn):
        fn(cp_x(t))

        @pl.when((t & 1) == 0)
        def _():
            fn(cp_wb(t >> 1))

        @pl.when(jnp.logical_and((t & 1) == 1, t < 15))
        def _():
            fn(cp_wa((t >> 1) + 1, sem_x.at[1]))

    def p1_body(t, carry):
        kt = t >> 1
        group(t, lambda d: d.wait())

        @pl.when(t < 15)
        def _():
            group(t + 1, lambda d: d.start())

        first = kt == 0
        w0 = pl.multiple_of((t & 1) * (S // 4), S // 4)
        r0 = pl.multiple_of((t & 1) * (S // 2), S // 2)
        xk = _bf(xs_u[kt, pl.ds(w0, S // 4), :])
        for sec, (dst, off) in enumerate(((qb, 0), (kb, PAD), (vb, PAD))):
            cols = [wperm[cc] for cc in range(8)] if sec == 0 else permuted(kt, sec)
            for half in range(2):
                w = _bf(jnp.concatenate(cols[half * 4:half * 4 + 4], axis=1))
                for rb in range(2):
                    r = jnp.dot(xk[rb * 512:(rb + 1) * 512], w, preferred_element_type=F32)
                    for cc in range(4):
                        sl = (half * 4 + cc, pl.ds(r0 + (off + rb * 512), 512), slice(None))
                        old = jnp.where(first, 0.0, dst[sl])
                        dst[sl] = old + r[:, cc * 128:(cc + 1) * 128]
        stage_first(jnp.minimum((t + 1) >> 1, 7))

        @pl.when(t < 4)
        def _():
            cp_c(t).start()

        @pl.when(t < 8)
        def _():
            for e in range(2):
                for d in cp_p(2 * t + e):
                    d.start()

        @pl.when(t >= 8)
        def _():
            cp_wo(t - 8).start()

        return carry

    jax.lax.fori_loop(0, 16, p1_body, 0)

    for j in range(4):
        cp_c(j).wait()
    for pp in range(NP):
        for d in cp_p(pp):
            d.wait()

    row = jax.lax.broadcasted_iota(jnp.int32, (TQ, TQ), 0)
    col = jax.lax.broadcasted_iota(jnp.int32, (TQ, TQ), 1)

    def pair_weights(pp, r0, n):
        ev = wp[pp, pl.ds(r0, n // 2, stride=2), :]
        od = wp[pp, pl.ds(r0 + 1, n // 2, stride=2), :]
        lo = (ev & jnp.uint32(0xFFFF)) | (od << 16)
        hi = (ev >> 16) | (od & jnp.uint32(0xFFFF0000))
        return lo, hi

    def stage_wk(pp):
        lo, hi = pair_weights(pp, 0, DC)
        wkst[0] = lo
        wkst[1] = hi

    cp_gw().start()
    for dp in range(16):
        cp_wob(dp, 0).start()
        cp_wob(dp, 1).start()
    stage_wk(0)

    def p2_body(p, carry):
        causal = col <= row
        wv = _bf(jnp.concatenate(pair_weights(p, DC, DC), axis=1))
        wq = _bf(jnp.concatenate(pair_weights(p, 2 * DC, M), axis=1))

        ks, vs, qs = {}, {}, {}
        done = {}
        never = p > NP

        def c_rows(i):
            return pltpu.bitcast(
                jnp.concatenate([cs_u[j, pl.ds(i * TQ // 2, TQ // 2), :] for j in range(4)], axis=1),
                BF16)

        def proj_k(i):
            wk = _bf(jnp.concatenate([wkst[0], wkst[1]], axis=1))
            ks[i] = _pack(jnp.dot(c_rows(i), wk, preferred_element_type=F32))

        def proj_v(i):
            vs[i] = _pack(jnp.dot(c_rows(i), wv, preferred_element_type=F32))

        def proj_q(i):
            xb = pltpu.bitcast(
                jnp.concatenate([xs_u[j, pl.ds(i * TQ // 2, TQ // 2), :] for j in range(8)], axis=1),
                BF16)
            q = jnp.dot(xb, wq, preferred_element_type=F32) * (DA ** -0.5 * LOG2E)
            qs[i] = _pack(q)

        def qk(h, i, dep):
            hs = slice(h * DA, (h + 1) * DA)
            kk = _bf(jnp.concatenate([ks[j][:, hs] for j in range(i + 1)], axis=0))
            q = qs[i][:, hs]
            if dep is not None:
                q = jnp.where(never, done[(h, dep)], q)
            s = jax.lax.dot_general(_bf(q), kk, NT, preferred_element_type=F32)
            ch = _lane_chunks(s)
            ch[i] = jnp.where(causal, ch[i], NEG)
            return ch

        def softmax_pv(h, i, ch):
            hs = slice(h * DA, (h + 1) * DA)
            m = jnp.max(_fold(ch, jnp.maximum), axis=1, keepdims=True)
            ps = [jnp.exp2(c - m) for c in ch]
            lp = ps[0]
            for j in range(1, i + 1):
                lp = lp + ps[j]
                if TIE and (j % TIE == TIE - 1 or j == i):
                    ps[j] = jnp.where(never, lp, ps[j])
            pb = jnp.concatenate(ps, axis=1).astype(BF16)
            vv = _bf(jnp.concatenate([vs[j][:, hs] for j in range(i + 1)], axis=0))
            o = jnp.dot(pb, vv, preferred_element_type=F32)
            if i >= LDEP:
                lp = jnp.where(never, o, lp)
            l = jnp.sum(lp, axis=1, keepdims=True)
            r = pl.reciprocal(l, approx=True)
            r = r * (2.0 - l * r)
            cn = _pack(o * r)
            done[(h, i)] = cn
            ctx[2 * p + h, pl.ds(i * TQ // 2, TQ // 2), :] = cn

        for j in range(NLAST + 1):
            proj_k(j)
        proj_q(NLAST)
        for j in range(NLAST):
            proj_v(j)
        for i in range(NLAST, NQ):
            dep = i - DEP if i - DEP >= NLAST else None
            s0 = qk(0, i, dep)
            s1 = qk(1, i, dep)
            late = []
            if i + 1 < NQ:
                proj_v(i)
                proj_k(i + 1)
                proj_q(i + 1)
            else:
                stage_wk(jnp.minimum(p + 1, NP - 1))
                proj_q(NLAST - 1)
                for j in range(NLAST - 1, -1, -1):
                    if j > 0:
                        proj_q(j - 1)
                    else:
                        proj_v(i)
                    dep = NQ - 2 if j == 0 else None
                    late.append((j, qk(0, j, dep), qk(1, j, dep)))
            softmax_pv(0, i, s0)
            softmax_pv(1, i, s1)
            for j, t0, t1 in late:
                softmax_pv(0, j, t0)
                softmax_pv(1, j, t1)
        return carry

    jax.lax.fori_loop(0, NP, p2_body, 0)

    cp_gw().wait()
    for j in range(8):
        cp_wo(j).wait()
    for dp in range(16):
        cp_wob(dp, 0).wait()
        cp_wob(dp, 1).wait()
    gw = gw_ref[...].astype(F32)
    rowi = jax.lax.broadcasted_iota(jnp.int32, (RB, 128), 0)
    odd = (jax.lax.broadcasted_iota(jnp.int32, (RB, 128), 1) & 1) == 1

    NSUB = TO // RB
    PER = NSUB // 8

    def p3_body(i, carry):
        r0 = pl.multiple_of(i * TO, TO)
        h0 = pl.multiple_of(i * (TO // 2), TO // 2)
        never = i > S

        def local(rb, after):
            q = [qb[cc, pl.ds(r0 + rb * RB, RB), :] for cc in range(8)]
            if after is not None and H_START:
                q = [jnp.where(never, after[cc * RB:(cc + 1) * RB], q[cc]) for cc in range(8)]
            lg = [_fold([q[cc] * kb[cc, pl.ds(r0 + (PAD + rb * RB - DIL * w), RB), :]
                         for cc in range(8)], jnp.add) for w in range(WIN)]
            lg = [t + pltpu.roll(t, 64, 1) for t in lg]
            lg = [t + jnp.where(odd, pltpu.roll(t, 1, 1), pltpu.roll(t, 127, 1)) for t in lg]
            lg = [t * (DB ** -0.5 * LOG2E) for t in lg]
            if rb == 0:
                lg = [lg[0]] + [jnp.where(rowi + r0 >= DIL * w, lg[w], NEG) for w in range(1, WIN)]
            m = _fold(lg, jnp.maximum)
            ps = [jnp.exp2(t - m) for t in lg]
            l = _fold(ps, jnp.add)
            r = pl.reciprocal(l, approx=True)
            r = r * (2.0 - l * r)
            ps = [t * r for t in ps]
            o = [_pack(_fold([ps[w] * vb[cc, pl.ds(r0 + (PAD + rb * RB - DIL * w), RB), :]
                              for w in range(WIN)], jnp.add)) for cc in range(8)]
            return jnp.concatenate(o, axis=1)

        ca = jnp.concatenate([ctx[h, pl.ds(h0, TO // 2), :] for h in range(HA)], axis=1)
        obs, acs = [], []
        for j in range(8):
            lhs = ca
            if j >= 2 and H_FIN:
                dep = jnp.concatenate(obs[(j - 2) * PER:(j - 1) * PER], axis=0)
                n = dep.shape[0]
                top = jnp.concatenate([jnp.where(never, dep, ca[:n, :M]), ca[:n, M:]], axis=1)
                lhs = jnp.concatenate([top, ca[n:]], axis=0)
            acs.append(jnp.dot(_bf(lhs), _bf(wo_s[j]), preferred_element_type=F32))
            for e in range(PER):
                obs.append(local(j * PER + e, acs[j - 1] if j >= 1 else None))
        a = jnp.concatenate(acs, axis=1)

        gs = _fold([_bf(xs_u[j, pl.ds(h0, TO // 2), :]).astype(F32) * gw[j:j + 1]
                    for j in range(8)], jnp.add)
        g = jax.nn.sigmoid(jnp.sum(gs, axis=1, keepdims=True))

        ob = _bf(jnp.concatenate(obs, axis=0))
        b = jnp.dot(ob, _bf(wob_p[...]), preferred_element_type=F32)
        out_s[pl.ds(r0, TO), :] = (g * a + (1.0 - g) * b).astype(BF16)
        cp_out(i).start()
        return carry

    jax.lax.fori_loop(0, S // TO, p3_body, 0)
    for i in range(S // TO):
        cp_out(i).wait()


@jax.jit
def pallas_gated_mix__compressed_kv_cla__sliding_local_dilated__prompt_kernel(
    A_x: jax.Array,
    A_c_kv: jax.Array,
    A_w_q: jax.Array,
    A_w_uk: jax.Array,
    A_w_uv: jax.Array,
    A_w_o: jax.Array,
    B_x: jax.Array,
    B_wqkv: jax.Array,
    B_wo: jax.Array,
    gate_w: jax.Array,
):
    del B_x
    any_spec = pl.BlockSpec(memory_space=pl.ANY)
    out = pl.pallas_call(
        _kernel,
        in_specs=[any_spec] * 9,
        out_specs=any_spec,
        out_shape=jax.ShapeDtypeStruct((S, M), BF16),
        scratch_shapes=[
            pltpu.VMEM((8, S // 2, 128), U32),
            pltpu.VMEM((4, S // 2, 128), U32),
            pltpu.VMEM((NP, 2 * DC + M, 128), U32),
            pltpu.VMEM((M, 3 * M), BF16),
            pltpu.VMEM((8, 64, 128), U32),
            pltpu.VMEM((8, S, 128), F32),
            pltpu.VMEM((8, S + PAD, 128), F32),
            pltpu.VMEM((8, S + PAD, 128), F32),
            pltpu.VMEM((HA, S // 2, 128), U32),
            pltpu.VMEM((8, HA * DA // 2, 128), U32),
            pltpu.VMEM((M // 2, M), U32),
            pltpu.VMEM((2, DC // 2, 128), U32),
            pltpu.VMEM((S, M), BF16),
            pltpu.VMEM((8, 128), BF16),
            pltpu.SemaphoreType.DMA((2,)),
            pltpu.SemaphoreType.DMA((3,)),
        ],
        compiler_params=pltpu.CompilerParams(vmem_limit_bytes=120 * 1024 * 1024,
                                             disable_bounds_checks=True),
    )(
        A_x.reshape(S, M),
        A_c_kv.reshape(S, DC),
        A_w_q,
        A_w_uk,
        A_w_uv,
        A_w_o.reshape(HA * DA, M),
        B_wqkv,
        B_wo.reshape(HB // 2, 2, DB, M),
        gate_w.reshape(8, 128),
    )
    return out.reshape(1, S, M)
```

```python
import functools
import math

import jax
import jax.numpy as jnp
import jax.experimental.pallas as pl
import jax.experimental.pallas.tpu as pltpu

F32 = jnp.float32
BF16 = jnp.bfloat16
U32 = jnp.uint32

S = 2048
M = 1024
HA = 32
DA = 128
DC = 512
HB = 32
DB = 32
WIN = 8
DIL = 2
PAD = 16
LOG2E = math.log2(math.e)
NEG = -1e9

TQ = 128
HQ = TQ // 2
NQ = S // TQ
NP = HA // 2
DEP = 2
CHAIN = 1
TIE = 4
RB = 16
LDEP = 4
NLAST = 4
BVH = 1
NS = 2
TO = 256
NT = (((1,), (1,)), ((), ()))

_STAGES = ((2, 4), (1, 3), (0, 2), (0, 6), (0, 1))


def _permute8(cols):
    cols = list(cols)
    lane = jax.lax.broadcasted_iota(jnp.int32, cols[0].shape, 1)
    for va, lb in _STAGES:
        lo = (lane & (1 << lb)) == 0
        sh = 1 << lb
        idx = [i for i in range(8) if not (i >> va) & 1]
        if lb == 6:
            rr = [pltpu.roll(jnp.where(lo, cols[i | (1 << va)], cols[i]), 64, 1) for i in idx]
            for i, r in zip(idx, rr):
                a, b = cols[i], cols[i | (1 << va)]
                cols[i] = jnp.where(lo, a, r)
                cols[i | (1 << va)] = jnp.where(lo, r, b)
        else:
            rb = [pltpu.roll(cols[i | (1 << va)], sh, 1) for i in idx]
            ra = [pltpu.roll(cols[i], 128 - sh, 1) for i in idx]
            for i, xa, xb in zip(idx, ra, rb):
                a, b = cols[i], cols[i | (1 << va)]
                cols[i] = jnp.where(lo, a, xb)
                cols[i | (1 << va)] = jnp.where(lo, xa, b)
    return cols


def _pack(x):
    return pltpu.bitcast(x.astype(BF16), U32)


def _bf(x):
    return pltpu.bitcast(x, BF16)


def _split(w):
    return (pltpu.bitcast(w << 16, F32), pltpu.bitcast(w & jnp.uint32(0xFFFF0000), F32))


def _join(lo, hi):
    return pltpu.bitcast(pltpu.pack_elementwise([lo, hi], packed_dtype=BF16), U32)


def _lhs7(a11, a12, a21, a22):
    return [a11 + a22, a21 + a22, a11, a22, a11 + a12, a21 - a11, a12 - a22]


def _rhs7(b11, b12, b21, b22):
    return [b11 + b22, b11, b12 - b22, b21 - b11, b22, b11 + b12, b21 + b22]


LSUM = (0, 1, 4, 5, 6)
RSUM = (0, 2, 3, 5, 6)


def _words7(fn, quads):
    halves = [_split(w) for w in quads]
    lo = fn(*[h[0] for h in halves])
    hi = fn(*[h[1] for h in halves])
    return [_join(a, b) for a, b in zip(lo, hi)]


def _strassen(lhs, rhs):
    def mm(m):
        return jnp.dot(_bf(lhs(m)), _bf(rhs(m)), preferred_element_type=F32)
    m4 = mm(4)
    m2 = mm(2)
    c12 = m2 + m4
    t11 = mm(6) - m4
    t22 = mm(5) + m2
    m0 = mm(0)
    t11 = t11 + m0
    t22 = t22 + m0
    m3 = mm(3)
    c11 = t11 + m3
    m1 = mm(1)
    return c11, c12, m1 + m3, t22 - m1


def _fold(xs, op):
    acc = xs[0]
    for x in xs[1:]:
        acc = op(acc, x)
    return acc


def _lane_chunks(x):
    return [x[:, j * 128:(j + 1) * 128] for j in range(x.shape[1] // 128)]


def _kernel(x_hbm, c_hbm, wq_hbm, wuk_hbm, wuv_hbm, wo_hbm, wqkv_hbm, wob_hbm, gw_hbm,
            out_hbm,
            xs_u, xq, cs_u, cq, wp, wo_r, wraw, wperm, wv7, qb, kb, vb, ctx7, wo7, wob_p, wob5,
            out_s, gw_ref, sem_x, sem_p, sem_a):
    x_u = x_hbm.bitcast(U32)
    c_u = c_hbm.bitcast(U32)
    wo_u = wo_hbm.bitcast(U32)
    wq_u = wq_hbm.bitcast(U32)
    wuk_u = wuk_hbm.bitcast(U32)
    wuv_u = wuv_hbm.bitcast(U32)
    wob_u = wob_hbm.bitcast(U32)

    def blk(j, n):
        return pl.ds(pl.multiple_of(j * n, n), n)

    def strip(j):
        return blk(j, 128)

    def ktile(t):
        return (t >> 2) + ((t >> 1) & 1) * 4

    def cp_xl(t):
        rows = blk(t & 1, S // 4)
        return pltpu.make_async_copy(x_u.at[rows, strip(t >> 2)], xs_u.at[t >> 2, rows, :],
                                     sem_x.at[t & 1])

    def cp_xr(t):
        rows = blk(t & 3, S // 8)
        return pltpu.make_async_copy(x_u.at[rows, strip((t >> 2) + 4)],
                                     xs_u.at[(t >> 2) + 4, rows, :], sem_x.at[t & 1])

    def cp_c(t, e):
        rows = blk(t >> 1, TQ)
        j = (t & 1) + 2 * e
        return pltpu.make_async_copy(c_u.at[rows, strip(j)], cs_u.at[j, rows, :], sem_x.at[t & 1])

    def cp_w(j, sec, sem):
        return pltpu.make_async_copy(wqkv_hbm.at[strip(j), pl.ds(sec * M, M)],
                                     wraw.at[strip(j), pl.ds(sec * M, M)], sem)

    def cp_wv(t, e):
        rows = blk(t + 16 * e, 32)
        return pltpu.make_async_copy(wqkv_hbm.at[rows, pl.ds(2 * M, M)],
                                     wraw.at[rows, pl.ds(2 * M, M)], sem_x.at[t & 1])

    def cp_p(p, slot):
        sem = sem_p.at[slot]
        return (
            pltpu.make_async_copy(wuk_u.at[:, p, :], wp.at[slot, pl.ds(0, DC), :], sem),
            pltpu.make_async_copy(wuv_u.at[:, p, :], wp.at[slot, pl.ds(DC, DC), :], sem),
            pltpu.make_async_copy(wq_u.at[:, p, :], wp.at[slot, pl.ds(2 * DC, M), :], sem),
            pltpu.make_async_copy(wo_u.at[blk(p, DA), :], wo_r.at[slot], sem),
        )

    def cp_wob(dp, h0):
        pos = ((dp >> 2) << 3) + ((dp & 1) << 2) + (dp & 2) + h0
        return pltpu.make_async_copy(wob_u.at[:, h0, dp, :], wob_p.at[blk(pos, 16), :],
                                     sem_a.at[0])

    def cp_gw():
        return pltpu.make_async_copy(gw_hbm, gw_ref, sem_a.at[0])

    def cp_out(i):
        return pltpu.make_async_copy(out_s.at[blk(i, TO), :], out_hbm.at[blk(i, TO), :],
                                     sem_a.at[1])

    def group(t, fn):
        @pl.when((t & 3) < 2)
        def _():
            fn(cp_xl(t))

        @pl.when((t & 1) == 0)
        def _():
            fn(cp_w(ktile(t), 1, sem_x.at[0]))

        @pl.when(jnp.logical_and((t & 1) == 1, t < 15))
        def _():
            fn(cp_w(ktile(t + 1), 0, sem_x.at[1]))

        fn(cp_xr(t))
        for e in range(2):
            fn(cp_wv(t, e))
            fn(cp_c(t, e))

    cp_w(0, 0, sem_a.at[1]).start()
    cp_xl(0).start()
    cp_w(0, 1, sem_x.at[0]).start()
    cp_xr(0).start()
    for e in range(2):
        cp_wv(0, e).start()
        cp_c(0, e).start()

    for cc in range(8):
        kb[cc, pl.ds(0, PAD), :] = jnp.zeros((PAD, 128), F32)
        vb[cc, pl.ds(0, PAD), :] = jnp.zeros((PAD, 128), F32)

    def permuted(kt, sec):
        w = pltpu.bitcast(wraw[strip(kt), pl.ds(sec * M, M)], U32)
        return _permute8(_lane_chunks(w))

    def stage_first(kt):
        for cc, t in enumerate(permuted(kt, 0)):
            wperm[cc] = t

    def act_sums(src, dst, u, nu, j):
        top, bot = blk(2 * j, HQ), blk(2 * j + 1, HQ)
        ops = _words7(_lhs7, (src[u, top, :], src[u + nu, top, :],
                              src[u, bot, :], src[u + nu, bot, :]))
        for e, m in enumerate(LSUM):
            dst[e, u, blk(j, HQ), :] = ops[m]

    def act_lhs(src, sums, nu, j):
        def lhs(m):
            if m == 2:
                parts = [src[u, blk(2 * j, HQ), :] for u in range(nu)]
            elif m == 3:
                parts = [src[u + nu, blk(2 * j + 1, HQ), :] for u in range(nu)]
            else:
                parts = [sums[LSUM.index(m), u, blk(j, HQ), :] for u in range(nu)]
            return jnp.concatenate(parts, axis=1)
        return lhs

    cp_w(0, 0, sem_a.at[1]).wait()
    stage_first(0)

    def p1_body(t, carry):
        kt = ktile(t)
        group(t, lambda d: d.wait())

        @pl.when(t < 15)
        def _():
            group(t + 1, lambda d: d.start())

        first = t < 2
        r0 = pl.multiple_of((t & 1) * (S // 2), S // 2)
        xk = _bf(xs_u[kt, blk(t & 1, S // 4), :])
        for sec, (dst, off) in enumerate(((qb, 0), (kb, PAD))):
            cols = [wperm[cc] for cc in range(8)] if sec == 0 else permuted(kt, sec)
            for half in range(2):
                w = _bf(jnp.concatenate(cols[half * 4:half * 4 + 4], axis=1))
                for rb in range(2):
                    r = jnp.dot(xk[rb * 512:(rb + 1) * 512], w, preferred_element_type=F32)
                    for cc in range(4):
                        sl = (half * 4 + cc, pl.ds(r0 + (off + rb * 512), 512), slice(None))
                        old = jnp.where(first, 0.0, dst[sl])
                        dst[sl] = old + r[:, cc * 128:(cc + 1) * 128]
        stage_first(ktile(jnp.minimum(t + 1, 15)))

        for e in range(2):
            act_sums(xs_u, xq, t >> 2, 4, 2 * (t & 3) + e)
        act_sums(cs_u, cq, t & 1, 2, t >> 1)
        wv = jnp.concatenate(
            [pltpu.bitcast(wraw[blk(t + 16 * e, 32), pl.ds(2 * M, M)], U32) for e in range(2)],
            axis=0)
        wv = _permute8(_lane_chunks(wv))
        for cc in range(4):
            ops = _words7(_rhs7, (wv[cc][:16], wv[cc + 4][:16], wv[cc][16:], wv[cc + 4][16:]))
            for m in range(7):
                wv7[m, cc, blk(t, 16), :] = ops[m]

        @pl.when(jnp.logical_and(t >= 8, t < 8 + NS))
        def _():
            for d in cp_p(t - 8, t - 8):
                d.start()

        @pl.when(t < 8)
        def _():
            for e in range(4):
                cp_wob(2 * t + (e >> 1), e & 1).start()

        return carry

    cp_gw().start()
    jax.lax.fori_loop(0, 16, p1_body, 0)

    cp_gw().wait()
    for dp in range(16):
        cp_wob(dp, 0).wait()
        cp_wob(dp, 1).wait()

    row = jax.lax.broadcasted_iota(jnp.int32, (TQ, TQ), 0)
    col = jax.lax.broadcasted_iota(jnp.int32, (TQ, TQ), 1)

    def p2_body(p, carry):
        slot = p & (NS - 1)
        for d in cp_p(p, slot):
            d.wait()
        causal = col <= row

        def pair_weights(r0, n):
            res = []
            for e in range(2):
                b11, b12 = _split(wp[slot, pl.ds(r0 + e, n // 4, stride=2), :])
                b21, b22 = _split(wp[slot, pl.ds(r0 + n // 2 + e, n // 4, stride=2), :])
                res.append(_rhs7(b11, b12, b21, b22))
            return [_join(a, b) for a, b in zip(*res)]

        def proj_bv(e):
            j = p >> 1
            cc = 2 * (p & 1) + e
            c = _strassen(act_lhs(xs_u, xq, 4, j), lambda m: wv7[m, cc])
            r0 = pl.multiple_of(j * (2 * TQ), 2 * TQ) + PAD
            vb[cc, pl.ds(r0, TQ), :] = c[0]
            vb[cc + 4, pl.ds(r0, TQ), :] = c[1]
            vb[cc, pl.ds(r0 + TQ, TQ), :] = c[2]
            vb[cc + 4, pl.ds(r0 + TQ, TQ), :] = c[3]

        for e in range(BVH):
            proj_bv(e)
        wk = pair_weights(0, DC)
        wq = pair_weights(2 * DC, M)
        wv = pair_weights(DC, DC)

        ks, vs, qs = {}, {}, {}
        done = {}
        never = p > NP

        def put(dst, j, c):
            for e, t in enumerate(c):
                dst[(e & 1, 2 * j + (e >> 1))] = _pack(t)

        def proj_k(j):
            put(ks, j, _strassen(act_lhs(cs_u, cq, 2, j), lambda m: wk[m]))

        def proj_v(j):
            put(vs, j, _strassen(act_lhs(cs_u, cq, 2, j), lambda m: wv[m]))

        def proj_q(j):
            c = _strassen(act_lhs(xs_u, xq, 4, j), lambda m: wq[m])
            put(qs, j, [t * (DA ** -0.5 * LOG2E) for t in c])

        def qk(h, i, dep):
            kk = _bf(jnp.concatenate([ks[(h, j)] for j in range(i + 1)], axis=0))
            q = qs[(h, i)]
            if dep is not None:
                q = jnp.where(never, pltpu.bitcast(done[(h, dep)][:HQ], U32), q)
            s = jax.lax.dot_general(_bf(q), kk, NT, preferred_element_type=F32)
            ch = _lane_chunks(s)
            ch[i] = jnp.where(causal, ch[i], NEG)
            return ch

        def softmax_pv(h, i, ch):
            m = jnp.max(_fold(ch, jnp.maximum), axis=1, keepdims=True)
            ps = [jnp.exp2(c - m) for c in ch]
            lp = ps[0]
            for j in range(1, i + 1):
                lp = lp + ps[j]
                if TIE and (j % TIE == TIE - 1 or j == i):
                    ps[j] = jnp.where(never, lp, ps[j])
            pb = jnp.concatenate(ps, axis=1).astype(BF16)
            vv = _bf(jnp.concatenate([vs[(h, j)] for j in range(i + 1)], axis=0))
            o = jnp.dot(pb, vv, preferred_element_type=F32)
            if i >= LDEP:
                lp = jnp.where(never, o, lp)
            l = jnp.sum(lp, axis=1, keepdims=True)
            r = pl.reciprocal(l, approx=True)
            r = r * (2.0 - l * r)
            done[(h, i)] = o * r
            j = i >> 1
            quad = [(0, 2 * j), (1, 2 * j), (0, 2 * j + 1), (1, 2 * j + 1)]
            if all(k in done for k in quad):
                for mm, t in enumerate(_lhs7(*[done[k] for k in quad])):
                    ctx7[mm, p, pl.ds(j * HQ, HQ), :] = _pack(t)

        def out_weights():
            w = wo_r[slot]
            for cc in range(4):
                lf, rt = slice(cc * 128, (cc + 1) * 128), slice((cc + 4) * 128, (cc + 5) * 128)
                ops = _words7(_rhs7, (w[:HQ, lf], w[:HQ, rt], w[HQ:, lf], w[HQ:, rt]))
                for m in range(7):
                    wo7[m, cc, blk(p, HQ), :] = ops[m]
            top = wob_p[blk(p, 16), :]
            bot = wob_p[blk(p + 16, 16), :]
            ops = _words7(_rhs7, (top[:, :M // 2], top[:, M // 2:], bot[:, :M // 2], bot[:, M // 2:]))
            for e, m in enumerate(RSUM):
                wob5[e, blk(p, 16), :] = ops[m]

        JL = NLAST // 2
        for j in range(JL + 1):
            proj_k(j)
        proj_q(JL)
        for j in range(JL):
            proj_v(j)
        out_weights()
        for i in range(NLAST, NQ):
            j = i >> 1
            dep = i - DEP if i - DEP >= NLAST else None
            s0 = qk(0, i, dep)
            s1 = qk(1, i, dep)
            late = []
            if i % 2 == 0:
                proj_v(j)
                if i + 2 < NQ:
                    proj_k(j + 1)
                elif JL:
                    proj_q(JL - 1)
            elif i + 1 < NQ:
                proj_q(j + 1)
            else:
                for jj in range(NLAST - 1, -1, -1):
                    if jj % 2 == 1 and jj > 1:
                        proj_q(jj // 2 - 1)
                    dep = NQ - 2 if jj == 0 else None
                    late.append((jj, qk(0, jj, dep), qk(1, jj, dep)))
            softmax_pv(0, i, s0)
            softmax_pv(1, i, s1)
            for jj, t0, t1 in late:
                softmax_pv(0, jj, t0)
                softmax_pv(1, jj, t1)
        for e in range(BVH, 2):
            proj_bv(e)
        for d in cp_p(jnp.minimum(p + NS, NP - 1), slot):
            d.start()
        return carry

    jax.lax.fori_loop(0, NP, p2_body, 0)
    for slot in range(NS):
        for d in cp_p(NP - 1, slot):
            d.wait()

    gw = gw_ref[...].astype(F32)
    rowi = jax.lax.broadcasted_iota(jnp.int32, (RB, 128), 0)
    odd = (jax.lax.broadcasted_iota(jnp.int32, (RB, 128), 1) & 1) == 1

    NSUB = TQ // RB
    PER = NSUB // 4

    def p3_body(i, carry):
        r0 = pl.multiple_of(i * TO, TO)
        never = i > S
        chain = []

        def local(rb):
            q = [qb[cc, pl.ds(r0 + rb * RB, RB), :] for cc in range(8)]
            lg = [_fold([q[cc] * kb[cc, pl.ds(r0 + (PAD + rb * RB - DIL * w), RB), :]
                         for cc in range(8)], jnp.add) for w in range(WIN)]
            lg = [t + pltpu.roll(t, 64, 1) for t in lg]
            lg = [t + jnp.where(odd, pltpu.roll(t, 1, 1), pltpu.roll(t, 127, 1)) for t in lg]
            lg = [t * (DB ** -0.5 * LOG2E) for t in lg]
            if rb == 0:
                lg = [lg[0]] + [jnp.where(rowi + r0 >= DIL * w, lg[w], NEG) for w in range(1, WIN)]
            m = _fold(lg, jnp.maximum)
            ps = [jnp.exp2(t - m) for t in lg]
            l = _fold(ps, jnp.add)
            r = pl.reciprocal(l, approx=True)
            r = r * (2.0 - l * r)
            ps = [t * r for t in ps]
            o = []
            for cc in range(8):
                pr = [ps[w] * vb[cc, pl.ds(r0 + (PAD + rb * RB - DIL * w), RB), :]
                      for w in range(WIN)]
                if CHAIN and chain:
                    pr[0] = jnp.where(never, chain[-1], pr[0])
                chain.append(_fold(pr, jnp.add))
                o.append(chain[-1])
            return jnp.concatenate(o[:4], axis=1), jnp.concatenate(o[4:], axis=1)

        ca = [jnp.concatenate([ctx7[m, pp, blk(i, HQ), :] for pp in range(NP)], axis=1)
              for m in range(7)]
        obs, acs = [], []
        for cc in range(4):
            acs.append(_strassen(lambda m: ca[m], lambda m: wo7[m, cc]))
            for e in range(PER):
                rb = cc * PER + e
                obs.append([_pack(t) for t in _lhs7(*local(rb), *local(rb + NSUB))])

        gs = _fold([_bf(xs_u[j, blk(i, TO // 2), :]).astype(F32) * gw[j:j + 1]
                    for j in range(8)], jnp.add)
        g = jax.nn.sigmoid(jnp.sum(gs, axis=1, keepdims=True))

        def wob(m):
            if m == 1:
                return wob_p[pl.ds(0, M // 4), pl.ds(0, M // 2)]
            if m == 4:
                return wob_p[pl.ds(M // 4, M // 4), pl.ds(M // 2, M // 2)]
            return wob5[RSUM.index(m)]

        b = _strassen(lambda m: jnp.concatenate([o[m] for o in obs], axis=0), wob)
        for e in range(4):
            a = jnp.concatenate([c[e] for c in acs], axis=1)
            ge = g[(e >> 1) * TQ:(e >> 1) * TQ + TQ]
            out_s[pl.ds(r0 + (e >> 1) * TQ, TQ), pl.ds((e & 1) * (M // 2), M // 2)] = (
                ge * a + (1.0 - ge) * b[e]).astype(BF16)
        cp_out(i).start()
        return carry

    jax.lax.fori_loop(0, S // TO, p3_body, 0)
    for i in range(S // TO):
        cp_out(i).wait()


@jax.jit
def pallas_gated_mix__compressed_kv_cla__sliding_local_dilated__prompt_kernel(
    A_x: jax.Array,
    A_c_kv: jax.Array,
    A_w_q: jax.Array,
    A_w_uk: jax.Array,
    A_w_uv: jax.Array,
    A_w_o: jax.Array,
    B_x: jax.Array,
    B_wqkv: jax.Array,
    B_wo: jax.Array,
    gate_w: jax.Array,
):
    del B_x
    any_spec = pl.BlockSpec(memory_space=pl.ANY)
    out = pl.pallas_call(
        _kernel,
        in_specs=[any_spec] * 9,
        out_specs=any_spec,
        out_shape=jax.ShapeDtypeStruct((S, M), BF16),
        scratch_shapes=[
            pltpu.VMEM((8, S // 2, 128), U32),
            pltpu.VMEM((5, 4, S // 4, 128), U32),
            pltpu.VMEM((4, S // 2, 128), U32),
            pltpu.VMEM((5, 2, S // 4, 128), U32),
            pltpu.VMEM((NS, 2 * DC + M, 128), U32),
            pltpu.VMEM((NS, DA, M), U32),
            pltpu.VMEM((M, 3 * M), BF16),
            pltpu.VMEM((8, 64, 128), U32),
            pltpu.VMEM((7, 4, M // 4, 128), U32),
            pltpu.VMEM((8, S, 128), F32),
            pltpu.VMEM((8, S + PAD, 128), F32),
            pltpu.VMEM((8, S + PAD, 128), F32),
            pltpu.VMEM((7, NP, S // 4, 128), U32),
            pltpu.VMEM((7, 4, NP * HQ, 128), U32),
            pltpu.VMEM((M // 2, M), U32),
            pltpu.VMEM((5, M // 4, M // 2), U32),
            pltpu.VMEM((S, M), BF16),
            pltpu.VMEM((8, 128), BF16),
            pltpu.SemaphoreType.DMA((2,)),
            pltpu.SemaphoreType.DMA((NS,)),
            pltpu.SemaphoreType.DMA((2,)),
        ],
        compiler_params=pltpu.CompilerParams(vmem_limit_bytes=120 * 1024 * 1024,
                                             disable_bounds_checks=True),
    )(
        A_x.reshape(S, M),
        A_c_kv.reshape(S, DC),
        A_w_q,
        A_w_uk,
        A_w_uv,
        A_w_o.reshape(HA * DA, M),
        B_wqkv,
        B_wo.reshape(HB // 2, 2, DB, M),
        gate_w.reshape(8, 128),
    )
    return out.reshape(1, S, M)
```

```python
import functools
import math

import jax
import jax.numpy as jnp
import jax.experimental.pallas as pl
import jax.experimental.pallas.tpu as pltpu

F32 = jnp.float32
BF16 = jnp.bfloat16
U32 = jnp.uint32

S = 2048
M = 1024
HA = 32
DA = 128
DC = 512
HB = 32
DB = 32
WIN = 8
DIL = 2
PAD = 16
LOG2E = math.log2(math.e)
NEG = -1e9

TQ = 128
HQ = TQ // 2
QQ = TQ // 4
LOFF = 0
NQ = S // TQ
NP = HA // 2
DEP = 2
CHAIN = 1
TIE = 4
RB = 16
LDEP = 4
NLAST = 4
BVH = 1
NS = 2
TO = 256
NT = (((1,), (1,)), ((), ()))

_STAGES = ((2, 4), (1, 3), (0, 2), (0, 6), (0, 1))


def _permute8(cols):
    cols = list(cols)
    lane = jax.lax.broadcasted_iota(jnp.int32, cols[0].shape, 1)
    for va, lb in _STAGES:
        lo = (lane & (1 << lb)) == 0
        sh = 1 << lb
        idx = [i for i in range(8) if not (i >> va) & 1]
        if lb == 6:
            rr = [pltpu.roll(jnp.where(lo, cols[i | (1 << va)], cols[i]), 64, 1) for i in idx]
            for i, r in zip(idx, rr):
                a, b = cols[i], cols[i | (1 << va)]
                cols[i] = jnp.where(lo, a, r)
                cols[i | (1 << va)] = jnp.where(lo, r, b)
        else:
            rb = [pltpu.roll(cols[i | (1 << va)], sh, 1) for i in idx]
            ra = [pltpu.roll(cols[i], 128 - sh, 1) for i in idx]
            for i, xa, xb in zip(idx, ra, rb):
                a, b = cols[i], cols[i | (1 << va)]
                cols[i] = jnp.where(lo, a, xb)
                cols[i | (1 << va)] = jnp.where(lo, xa, b)
    return cols


def _pack(x):
    return pltpu.bitcast(x.astype(BF16), U32)


def _bf(x):
    return pltpu.bitcast(x, BF16)


def _split(w):
    return (pltpu.bitcast(w << 16, F32), pltpu.bitcast(w & jnp.uint32(0xFFFF0000), F32))


def _join(lo, hi):
    return pltpu.bitcast(pltpu.pack_elementwise([lo, hi], packed_dtype=BF16), U32)


def _lhs7(a11, a12, a21, a22):
    return [a11 + a22, a21 + a22, a11, a22, a11 + a12, a21 - a11, a12 - a22]


def _rhs7(b11, b12, b21, b22):
    return [b11 + b22, b11, b12 - b22, b21 - b11, b22, b11 + b12, b21 + b22]


LSUM = (0, 1, 4, 5, 6)
RSUM = (0, 2, 3, 5, 6)


def _words7(fn, quads):
    halves = [_split(w) for w in quads]
    lo = fn(*[h[0] for h in halves])
    hi = fn(*[h[1] for h in halves])
    return [_join(a, b) for a, b in zip(lo, hi)]


def _combine(mm):
    add = functools.partial(jax.tree.map, jnp.add)
    sub = functools.partial(jax.tree.map, jnp.subtract)
    m4 = mm(4)
    m2 = mm(2)
    c12 = add(m2, m4)
    t11 = sub(mm(6), m4)
    t22 = add(mm(5), m2)
    m0 = mm(0)
    t11 = add(t11, m0)
    t22 = add(t22, m0)
    m3 = mm(3)
    c11 = add(t11, m3)
    m1 = mm(1)
    return c11, c12, add(m1, m3), sub(t22, m1)


def _dot(a, b):
    return jnp.dot(_bf(a), _bf(b), preferred_element_type=F32)


def _strassen(lhs, rhs):
    return _combine(lambda m: _dot(lhs(m), rhs(m)))


def _strassen2(lhs, rhs):
    return _combine(lambda m: _combine(lambda n: _dot(lhs(m, n), rhs(m, n))))


def _ops49(fn, blocks, m):
    return fn(*[fn(*[blocks[q][e] for q in range(4)])[m] for e in range(4)])


def _words49(fn, words, m):
    halves = [[_split(w) for w in q] for q in words]
    lo = _ops49(fn, [[h[0] for h in q] for q in halves], m)
    hi = _ops49(fn, [[h[1] for h in q] for q in halves], m)
    return [_join(a, b) for a, b in zip(lo, hi)]


def _fold(xs, op):
    acc = xs[0]
    for x in xs[1:]:
        acc = op(acc, x)
    return acc


def _lane_chunks(x):
    return [x[:, j * 128:(j + 1) * 128] for j in range(x.shape[1] // 128)]


def _kernel(x_hbm, c_hbm, wq_hbm, wuk_hbm, wuv_hbm, wo_hbm, wqkv_hbm, wob_hbm, gw_hbm,
            out_hbm,
            xs_u, xq, cs_u, cq, wp, wo_r, wraw, wperm, wv7, qb, kb, vb, ctx, wo49, wob_p, wob5,
            out_s, gw_ref, sem_x, sem_p, sem_a):
    x_u = x_hbm.bitcast(U32)
    c_u = c_hbm.bitcast(U32)
    wo_u = wo_hbm.bitcast(U32)
    wq_u = wq_hbm.bitcast(U32)
    wuk_u = wuk_hbm.bitcast(U32)
    wuv_u = wuv_hbm.bitcast(U32)
    wob_u = wob_hbm.bitcast(U32)

    def blk(j, n):
        return pl.ds(pl.multiple_of(j * n, n), n)

    def strip(j):
        return blk(j, 128)

    def ktile(t):
        return (t >> 2) + ((t >> 1) & 1) * 4

    def cp_xl(t):
        rows = blk(t & 1, S // 4)
        return pltpu.make_async_copy(x_u.at[rows, strip(t >> 2)], xs_u.at[t >> 2, rows, :],
                                     sem_x.at[t & 1])

    def cp_xr(t):
        rows = blk(t & 3, S // 8)
        return pltpu.make_async_copy(x_u.at[rows, strip((t >> 2) + 4)],
                                     xs_u.at[(t >> 2) + 4, rows, :], sem_x.at[t & 1])

    def cp_c(t):
        rows = blk(t >> 1, TQ)
        return pltpu.make_async_copy(c_u.at[rows, :], cs_u.at[rows, :], sem_x.at[0])

    def cp_w(j, sec, sem):
        return pltpu.make_async_copy(wqkv_hbm.at[strip(j), pl.ds(sec * M, M)],
                                     wraw.at[strip(j), pl.ds(sec * M, M)], sem)

    def cp_wv(t, e):
        rows = blk(t + 16 * e, 32)
        return pltpu.make_async_copy(wqkv_hbm.at[rows, pl.ds(2 * M, M)],
                                     wraw.at[rows, pl.ds(2 * M, M)], sem_x.at[t & 1])

    def cp_p(p, slot):
        sem = sem_p.at[slot]
        return (
            pltpu.make_async_copy(wuk_u.at[:, p, :], wp.at[slot, pl.ds(0, DC), :], sem),
            pltpu.make_async_copy(wuv_u.at[:, p, :], wp.at[slot, pl.ds(DC, DC), :], sem),
            pltpu.make_async_copy(wq_u.at[:, p, :], wp.at[slot, pl.ds(2 * DC, M), :], sem),
        ) + tuple(
            pltpu.make_async_copy(wo_u.at[blk(8 * (p >> 1) + 2 * e + (p & 1), QQ), :],
                                  wo_r.at[slot, pl.ds(e * QQ, QQ), :], sem) for e in range(4))

    def cp_wob(dp, h0):
        pos = ((dp >> 2) << 3) + ((dp & 1) << 2) + (dp & 2) + h0
        return pltpu.make_async_copy(wob_u.at[:, h0, dp, :], wob_p.at[blk(pos, 16), :],
                                     sem_a.at[0])

    def cp_gw():
        return pltpu.make_async_copy(gw_hbm, gw_ref, sem_a.at[0])

    def cp_out(i):
        return pltpu.make_async_copy(out_s.at[blk(i, TO), :], out_hbm.at[blk(i, TO), :],
                                     sem_a.at[1])

    def group(t, fn):
        @pl.when((t & 3) < 2)
        def _():
            fn(cp_xl(t))

        @pl.when((t & 1) == 0)
        def _():
            fn(cp_w(ktile(t), 1, sem_x.at[0]))
            fn(cp_c(t))

        @pl.when(jnp.logical_and((t & 1) == 1, t < 15))
        def _():
            fn(cp_w(ktile(t + 1), 0, sem_x.at[1]))

        fn(cp_xr(t))
        for e in range(2):
            fn(cp_wv(t, e))

    cp_w(0, 0, sem_a.at[1]).start()
    cp_xl(0).start()
    cp_w(0, 1, sem_x.at[0]).start()
    cp_xr(0).start()
    for e in range(2):
        cp_wv(0, e).start()
    cp_c(0).start()

    for cc in range(8):
        kb[cc, pl.ds(0, PAD), :] = jnp.zeros((PAD, 128), F32)
        vb[cc, pl.ds(0, PAD), :] = jnp.zeros((PAD, 128), F32)

    def permuted(kt, sec):
        w = pltpu.bitcast(wraw[strip(kt), pl.ds(sec * M, M)], U32)
        return _permute8(_lane_chunks(w))

    def stage_first(kt):
        for cc, t in enumerate(permuted(kt, 0)):
            wperm[cc] = t

    def act_sums(src, dst, u, nu, j):
        top, bot = blk(2 * j, HQ), blk(2 * j + 1, HQ)
        ops = _words7(_lhs7, (src[u, top, :], src[u + nu, top, :],
                              src[u, bot, :], src[u + nu, bot, :]))
        for e, m in enumerate(LSUM):
            dst[e, u, blk(j, HQ), :] = ops[m]

    def act_lhs(src, sums, nu, j):
        def lhs(m):
            if m == 2:
                parts = [src[u, blk(2 * j, HQ), :] for u in range(nu)]
            elif m == 3:
                parts = [src[u + nu, blk(2 * j + 1, HQ), :] for u in range(nu)]
            else:
                parts = [sums[LSUM.index(m), u, blk(j, HQ), :] for u in range(nu)]
            return jnp.concatenate(parts, axis=1)
        return lhs

    cp_w(0, 0, sem_a.at[1]).wait()
    stage_first(0)

    def p1_body(t, carry):
        kt = ktile(t)
        group(t, lambda d: d.wait())

        @pl.when(t < 15)
        def _():
            group(t + 1, lambda d: d.start())

        first = t < 2
        r0 = pl.multiple_of((t & 1) * (S // 2), S // 2)
        xk = _bf(xs_u[kt, blk(t & 1, S // 4), :])
        for sec, (dst, off) in enumerate(((qb, 0), (kb, PAD))):
            cols = [wperm[cc] for cc in range(8)] if sec == 0 else permuted(kt, sec)
            for half in range(2):
                w = _bf(jnp.concatenate(cols[half * 4:half * 4 + 4], axis=1))
                for rb in range(2):
                    r = jnp.dot(xk[rb * 512:(rb + 1) * 512], w, preferred_element_type=F32)
                    for cc in range(4):
                        sl = (half * 4 + cc, pl.ds(r0 + (off + rb * 512), 512), slice(None))
                        old = jnp.where(first, 0.0, dst[sl])
                        dst[sl] = old + r[:, cc * 128:(cc + 1) * 128]
        stage_first(ktile(jnp.minimum(t + 1, 15)))

        for e in range(2):
            act_sums(xs_u, xq, t >> 2, 4, 2 * (t & 3) + e)
        cw = [[cs_u[blk(8 * (t >> 1) + 4 * (q >> 1) + 2 * (e >> 1) + (t & 1), 16),
                    pl.ds((2 * (q & 1) + (e & 1)) * 128, 128)] for e in range(4)] for q in range(4)]
        for m in range(7):
            for n, w in enumerate(_words49(_lhs7, cw, m)):
                cq[7 * m + n, blk(t, 16), :] = w
        wv = jnp.concatenate(
            [pltpu.bitcast(wraw[blk(t + 16 * e, 32), pl.ds(2 * M, M)], U32) for e in range(2)],
            axis=0)
        wv = _permute8(_lane_chunks(wv))
        for cc in range(4):
            ops = _words7(_rhs7, (wv[cc][:16], wv[cc + 4][:16], wv[cc][16:], wv[cc + 4][16:]))
            for m in range(7):
                wv7[m, cc, blk(t, 16), :] = ops[m]

        @pl.when(jnp.logical_and(t >= 8, t < 8 + NS))
        def _():
            for d in cp_p(t - 8, t - 8):
                d.start()

        @pl.when(t < 8)
        def _():
            for e in range(4):
                cp_wob(2 * t + (e >> 1), e & 1).start()

        return carry

    cp_gw().start()
    jax.lax.fori_loop(0, 16, p1_body, 0)

    cp_gw().wait()
    for dp in range(16):
        cp_wob(dp, 0).wait()
        cp_wob(dp, 1).wait()

    row = jax.lax.broadcasted_iota(jnp.int32, (TQ, TQ), 0)
    col = jax.lax.broadcasted_iota(jnp.int32, (TQ, TQ), 1)

    def p2_body(p, carry):
        slot = p & (NS - 1)
        for d in cp_p(p, slot):
            d.wait()
        causal = col <= row

        def pair_weights(r0, n):
            res = []
            for e in range(2):
                b11, b12 = _split(wp[slot, pl.ds(r0 + e, n // 4, stride=2), :])
                b21, b22 = _split(wp[slot, pl.ds(r0 + n // 2 + e, n // 4, stride=2), :])
                res.append(_rhs7(b11, b12, b21, b22))
            return [_join(a, b) for a, b in zip(*res)]

        def proj_bv(e):
            j = p >> 1
            cc = 2 * (p & 1) + e
            c = _strassen(act_lhs(xs_u, xq, 4, j), lambda m: wv7[m, cc])
            r0 = pl.multiple_of(j * (2 * TQ), 2 * TQ) + PAD
            vb[cc, pl.ds(r0, TQ), :] = c[0]
            vb[cc + 4, pl.ds(r0, TQ), :] = c[1]
            vb[cc, pl.ds(r0 + TQ, TQ), :] = c[2]
            vb[cc + 4, pl.ds(r0 + TQ, TQ), :] = c[3]

        for e in range(BVH):
            proj_bv(e)
        res = []
        for par in range(2):
            tiles = [[_split(wp[slot, pl.ds(DC - n1 * DC + kt * 128 + par, HQ, stride=2), :])
                      for n1 in range(2)] for kt in range(4)]
            blocks = [[tiles[2 * (q >> 1) + (e >> 1)][q & 1][e & 1] for e in range(4)]
                      for q in range(4)]
            res.append([_ops49(_rhs7, blocks, m) for m in range(7)])
        wkv = [[_join(a, b) for a, b in zip(*t)] for t in zip(*res)]
        wq = pair_weights(2 * DC, M)

        ks, vs, qs = {}, {}, {}
        done = {}
        never = p > NP

        def put(dst, j, c):
            for e, t in enumerate(c):
                dst[(e & 1, 2 * j + (e >> 1))] = _pack(t)

        def proj_kv(j):
            c = _strassen2(lambda m, n: cq[7 * m + n, pl.ds(j * QQ, QQ), :],
                           lambda m, n: wkv[m][n])
            for q in range(4):
                for h in range(2):
                    (vs, ks)[q & 1][(h, 2 * j + (q >> 1))] = jnp.concatenate(
                        [_pack(c[q][h]), _pack(c[q][2 + h])], axis=0)

        def proj_q(j):
            c = _strassen(act_lhs(xs_u, xq, 4, j), lambda m: wq[m])
            put(qs, j, [t * (DA ** -0.5 * LOG2E) for t in c])

        def qk(h, i, dep):
            kk = _bf(jnp.concatenate([ks[(h, j)] for j in range(i + 1)], axis=0))
            q = qs[(h, i)]
            if dep is not None:
                q = jnp.where(never, done[(h, dep)], q)
            s = jax.lax.dot_general(_bf(q), kk, NT, preferred_element_type=F32)
            ch = _lane_chunks(s)
            ch[i] = jnp.where(causal, ch[i], NEG)
            return ch

        def softmax_pv(h, i, ch):
            m = jnp.max(_fold(ch, jnp.maximum), axis=1, keepdims=True)
            ps = [jnp.exp2(c - m) for c in ch]
            lp = ps[0]
            for j in range(1, i + 1):
                lp = lp + ps[j]
                if TIE and (j % TIE == TIE - 1 or j == i):
                    ps[j] = jnp.where(never, lp, ps[j])
            pb = jnp.concatenate(ps, axis=1).astype(BF16)
            vv = _bf(jnp.concatenate([vs[(h, j)] for j in range(i + 1)], axis=0))
            o = jnp.dot(pb, vv, preferred_element_type=F32)
            if i >= LDEP:
                lp = jnp.where(never, o, lp)
            l = jnp.sum(lp, axis=1, keepdims=True)
            r = pl.reciprocal(l, approx=True)
            r = r * (2.0 - l * r)
            cn = _pack(o * r)
            done[(h, i)] = cn
            ctx[2 * p + h, pl.ds(i * HQ, HQ), :] = cn

        def out_weights():
            for cc in range(2):
                ww = [[wo_r[slot, pl.ds((2 * (q >> 1) + (e >> 1)) * QQ, QQ),
                            pl.ds((4 * (q & 1) + 2 * (e & 1) + cc) * 128, 128)]
                       for e in range(4)] for q in range(4)]
                for m in range(7):
                    for n, w in enumerate(_words49(_rhs7, ww, m)):
                        wo49[7 * m + n, cc, blk(p, QQ), :] = w
            top = wob_p[blk(p, 16), :]
            bot = wob_p[blk(p + 16, 16), :]
            ops = _words7(_rhs7, (top[:, :M // 2], top[:, M // 2:], bot[:, :M // 2], bot[:, M // 2:]))
            for e, m in enumerate(RSUM):
                wob5[e, blk(p, 16), :] = ops[m]

        JL = NLAST // 2
        for j in range(JL + 1):
            proj_kv(j)
        proj_q(JL)
        out_weights()
        for i in range(NLAST, NQ):
            j = i >> 1
            dep = i - DEP if i - DEP >= NLAST else None
            s0 = qk(0, i, dep)
            s1 = qk(1, i, dep)
            late = []
            if i % 2 == 0:
                if i + 2 < NQ:
                    proj_kv(j + 1)
                elif JL:
                    proj_q(JL - 1)
            elif i + 1 < NQ:
                proj_q(j + 1)
            else:
                for jj in range(NLAST - 1, -1, -1):
                    if jj % 2 == 1 and jj > 1:
                        proj_q(jj // 2 - 1)
                    dep = NQ - 2 if jj == 0 else None
                    late.append((jj, qk(0, jj, dep), qk(1, jj, dep)))
                for e in range(BVH, 2):
                    proj_bv(e)
            softmax_pv(0, i, s0)
            softmax_pv(1, i, s1)
            for jj, t0, t1 in late:
                softmax_pv(0, jj, t0)
                softmax_pv(1, jj, t1)
        for d in cp_p(jnp.minimum(p + NS, NP - 1), slot):
            d.start()
        return carry

    jax.lax.fori_loop(0, NP, p2_body, 0)

    gw = gw_ref[...].astype(F32)
    rowi = jax.lax.broadcasted_iota(jnp.int32, (RB, 128), 0)
    odd = (jax.lax.broadcasted_iota(jnp.int32, (RB, 128), 1) & 1) == 1

    NSUB = TQ // RB

    def p3_body(i, carry):
        r0 = pl.multiple_of(i * TO, TO)
        never = i > S
        chain = []

        def local(rb):
            q = [qb[cc, pl.ds(r0 + rb * RB, RB), :] for cc in range(8)]
            lg = [_fold([q[cc] * kb[cc, pl.ds(r0 + (PAD + rb * RB - DIL * w), RB), :]
                         for cc in range(8)], jnp.add) for w in range(WIN)]
            lg = [t + pltpu.roll(t, 64, 1) for t in lg]
            lg = [t + jnp.where(odd, pltpu.roll(t, 1, 1), pltpu.roll(t, 127, 1)) for t in lg]
            lg = [t * (DB ** -0.5 * LOG2E) for t in lg]
            if rb == 0:
                lg = [lg[0]] + [jnp.where(rowi + r0 >= DIL * w, lg[w], NEG) for w in range(1, WIN)]
            m = _fold(lg, jnp.maximum)
            ps = [jnp.exp2(t - m) for t in lg]
            l = _fold(ps, jnp.add)
            r = pl.reciprocal(l, approx=True)
            r = r * (2.0 - l * r)
            ps = [t * r for t in ps]
            o = []
            for cc in range(8):
                pr = [ps[w] * vb[cc, pl.ds(r0 + (PAD + rb * RB - DIL * w), RB), :]
                      for w in range(WIN)]
                if CHAIN and chain:
                    pr[0] = jnp.where(never, chain[-1], pr[0])
                chain.append(_fold(pr, jnp.add))
                o.append(chain[-1])
            return jnp.concatenate(o[:4], axis=1), jnp.concatenate(o[4:], axis=1)

        cw = [[jnp.concatenate([ctx[4 * u + 2 * (q & 1) + (e & 1),
                                    blk(4 * i + 2 * (q >> 1) + (e >> 1), QQ), :]
                                for u in range(HA // 4)], axis=1)
               for e in range(4)] for q in range(4)]
        obs, calls = [], []

        def outer(m):
            ca = _words49(_lhs7, cw, m)
            res = _strassen(
                lambda n: ca[n],
                lambda n: jnp.concatenate([wo49[7 * m + n, cc] for cc in range(2)], axis=1))
            calls.append(m)
            for rb in range(len(obs), min(NSUB, len(calls) + 1 + LOFF)):
                obs.append([_pack(t) for t in _lhs7(*local(rb), *local(rb + NSUB))])
            return res

        acs = _combine(outer)
        assert len(obs) == NSUB

        gs = _fold([_bf(xs_u[j, blk(i, TO // 2), :]).astype(F32) * gw[j:j + 1]
                    for j in range(8)], jnp.add)
        g = jax.nn.sigmoid(jnp.sum(gs, axis=1, keepdims=True))

        def wob(m):
            if m == 1:
                return wob_p[pl.ds(0, M // 4), pl.ds(0, M // 2)]
            if m == 4:
                return wob_p[pl.ds(M // 4, M // 4), pl.ds(M // 2, M // 2)]
            return wob5[RSUM.index(m)]

        b = _strassen(lambda m: jnp.concatenate([o[m] for o in obs], axis=0), wob)
        for e in range(4):
            a = jnp.concatenate([jnp.concatenate(acs[e][2 * r2:2 * r2 + 2], axis=1)
                                 for r2 in range(2)], axis=0)
            ge = g[(e >> 1) * TQ:(e >> 1) * TQ + TQ]
            out_s[pl.ds(r0 + (e >> 1) * TQ, TQ), pl.ds((e & 1) * (M // 2), M // 2)] = (
                ge * a + (1.0 - ge) * b[e]).astype(BF16)
        cp_out(i).start()
        return carry

    jax.lax.fori_loop(0, S // TO, p3_body, 0)
    for slot in range(NS):
        for d in cp_p(NP - 1, slot):
            d.wait()
    for i in range(S // TO):
        cp_out(i).wait()


@jax.jit
def pallas_gated_mix__compressed_kv_cla__sliding_local_dilated__prompt_kernel(
    A_x: jax.Array,
    A_c_kv: jax.Array,
    A_w_q: jax.Array,
    A_w_uk: jax.Array,
    A_w_uv: jax.Array,
    A_w_o: jax.Array,
    B_x: jax.Array,
    B_wqkv: jax.Array,
    B_wo: jax.Array,
    gate_w: jax.Array,
):
    del B_x
    any_spec = pl.BlockSpec(memory_space=pl.ANY)
    out = pl.pallas_call(
        _kernel,
        in_specs=[any_spec] * 9,
        out_specs=any_spec,
        out_shape=jax.ShapeDtypeStruct((S, M), BF16),
        scratch_shapes=[
            pltpu.VMEM((8, S // 2, 128), U32),
            pltpu.VMEM((5, 4, S // 4, 128), U32),
            pltpu.VMEM((S // 2, DC), U32),
            pltpu.VMEM((49, S // 8, 128), U32),
            pltpu.VMEM((NS, 2 * DC + M, 128), U32),
            pltpu.VMEM((NS, DA, M), U32),
            pltpu.VMEM((M, 3 * M), BF16),
            pltpu.VMEM((8, 64, 128), U32),
            pltpu.VMEM((7, 4, M // 4, 128), U32),
            pltpu.VMEM((8, S, 128), F32),
            pltpu.VMEM((8, S + PAD, 128), F32),
            pltpu.VMEM((8, S + PAD, 128), F32),
            pltpu.VMEM((HA, S // 2, 128), U32),
            pltpu.VMEM((49, 2, NP * QQ, 128), U32),
            pltpu.VMEM((M // 2, M), U32),
            pltpu.VMEM((5, M // 4, M // 2), U32),
            pltpu.VMEM((S, M), BF16),
            pltpu.VMEM((8, 128), BF16),
            pltpu.SemaphoreType.DMA((2,)),
            pltpu.SemaphoreType.DMA((NS,)),
            pltpu.SemaphoreType.DMA((2,)),
        ],
        compiler_params=pltpu.CompilerParams(vmem_limit_bytes=120 * 1024 * 1024,
                                             disable_bounds_checks=True),
    )(
        A_x.reshape(S, M),
        A_c_kv.reshape(S, DC),
        A_w_q,
        A_w_uk,
        A_w_uv,
        A_w_o.reshape(HA * DA, M),
        B_wqkv,
        B_wo.reshape(HB // 2, 2, DB, M),
        gate_w.reshape(8, 128),
    )
    return out.reshape(1, S, M)
```

```python
import functools
import math

import jax
import jax.numpy as jnp
import jax.experimental.pallas as pl
import jax.experimental.pallas.tpu as pltpu

F32 = jnp.float32
BF16 = jnp.bfloat16
U32 = jnp.uint32

S = 2048
M = 1024
HA = 32
DA = 128
DC = 512
HB = 32
DB = 32
WIN = 8
DIL = 2
PAD = 16
LOG2E = math.log2(math.e)
NEG = -1e9

TQ = 128
HQ = TQ // 2
QQ = TQ // 4
BOP = (2, 3, 2)
LX = 16
KVS = 28
QS = 28
SK = 3
SMR = 16
P1N = 6
P1U = 2
P3S = 4
P3E = 12
NQ = S // TQ
NP = HA // 2
DEP = 2
TIE = 4
RB = 16
LDEP = 4
TO = 256
NN = (((1,), (0,)), ((), ()))
NT = (((1,), (1,)), ((), ()))


def _plan2():
    plan = {}

    def put(name, count, start, until):
        plan.setdefault(start, []).extend([(name, until)] * count)

    def after_qk(i):
        if i >= NQ - 2:
            return ("bo", (i - NQ + 2) * BOP[0] + 1)
        return ("kv", i // 2 + 1, KVS * (i & 1) + LX)

    def fill(name, count, sites):
        for start, room, until in sites:
            n = min(count, room - len(plan.get(start, ())))
            put(name, n, start, until)
            count -= n
        assert count == 0, (name, count)

    def qk_sites(lo, hi):
        return [(("qk", h, i), max(i + 1 - h * SK, 0), after_qk(i))
                for i in range(lo, hi) for h in range(2)]

    def q_sites(g, lo, hi, until):
        return [(("q", g, k), 1, until) for k in range(lo, hi)]

    for k in range(14):
        put("wo", 4, ("bv", k), ("kv", 0, 24))
    put("sc", 1, ("kv", 0, 0), ("q", 0, 0))
    put("sc", 1, ("kv", 0, 24), ("q", 0, 8))
    early = q_sites(0, 8, 45, ("kv", 1, 8))
    for g in range(1, 4):
        early += q_sites(g, 0, QS - 4, ("qk", 1, 2 * g - 1))
        early += qk_sites(2 * g - 1, 2 * g)
        early += q_sites(g, QS, 45, ("qk", 1, 2 * g))
        early += qk_sites(2 * g, 2 * g + 1)
    fill("bx", 16, early)
    fill("lo", 128 + 128 // SMR, early)
    fill("qw", 112, qk_sites(7, 14))
    fill("kv", 56, qk_sites(14, 16) + [(("bo", k), 8, ("bo", 6)) for k in range(BOP[0], 5)])
    return plan


def _planx():
    names = _spread(["sc"] * 2 + ["bx"] * 16 + ["qw"] * 112 + ["kv"] * 56, 8 * 30)
    return {k: [(n, min(k + 4, 31)) for n in names[8 * k:8 * k + 8]] for k in range(30)}


def _spread(names, ticks):
    out = [None] * ticks
    for k, name in enumerate(names):
        out[k * ticks // len(names)] = name
    return out


def _plan1():
    names = _spread(["x"] * 28 + ["c"] * 14 + ["o"] * 8 + ["v"] * 8, 16 * P1N)
    return {k: [(n, min(k + P1U, 7)) for n in names[16 * k:16 * k + 16]] for k in range(P1N)}


def _plan3():
    plan = {}
    for k in range(6):
        lo = P3S if k == 0 else 0
        extra = ["g"] * 8 if k in (1, 2) else []
        names = _spread(["a"] * 32 + extra, 4 * (P3E - lo))
        for d in range(lo, P3E):
            plan[(k, d)] = [(n, (k + 1, 0)) for n in names[4 * (d - lo):4 * (d - lo) + 4]]
    return plan


_STAGES = ((2, 4), (1, 3), (0, 2), (0, 6), (0, 1))


def _permute8(cols):
    cols = list(cols)
    lane = jax.lax.broadcasted_iota(jnp.int32, cols[0].shape, 1)
    for va, lb in _STAGES:
        lo = (lane & (1 << lb)) == 0
        sh = 1 << lb
        idx = [i for i in range(8) if not (i >> va) & 1]
        if lb == 6:
            rr = [pltpu.roll(jnp.where(lo, cols[i | (1 << va)], cols[i]), 64, 1) for i in idx]
            for i, r in zip(idx, rr):
                a, b = cols[i], cols[i | (1 << va)]
                cols[i] = jnp.where(lo, a, r)
                cols[i | (1 << va)] = jnp.where(lo, r, b)
        else:
            rb = [pltpu.roll(cols[i | (1 << va)], sh, 1) for i in idx]
            ra = [pltpu.roll(cols[i], 128 - sh, 1) for i in idx]
            for i, xa, xb in zip(idx, ra, rb):
                a, b = cols[i], cols[i | (1 << va)]
                cols[i] = jnp.where(lo, a, xb)
                cols[i | (1 << va)] = jnp.where(lo, xa, b)
    return cols


def _pack(x):
    return pltpu.bitcast(x.astype(BF16), U32)


def _bf(x):
    return pltpu.bitcast(x, BF16)


def _split(w):
    return (pltpu.bitcast(w << 16, F32), pltpu.bitcast(w & jnp.uint32(0xFFFF0000), F32))


def _join(lo, hi):
    return pltpu.bitcast(pltpu.pack_elementwise([lo, hi], packed_dtype=BF16), U32)


def _lhs7(a11, a12, a21, a22):
    return [a11 + a22, a21 + a22, a11, a22, a11 + a12, a21 - a11, a12 - a22]


def _rhs7(b11, b12, b21, b22):
    return [b11 + b22, b11, b12 - b22, b21 - b11, b22, b11 + b12, b21 + b22]


LSUM = (0, 1, 4, 5, 6)
RSUM = (0, 2, 3, 5, 6)


def _words7(fn, quads):
    halves = [_split(w) for w in quads]
    lo = fn(*[h[0] for h in halves])
    hi = fn(*[h[1] for h in halves])
    return [_join(a, b) for a, b in zip(lo, hi)]


def _combine(mm):
    add = functools.partial(jax.tree.map, jnp.add)
    sub = functools.partial(jax.tree.map, jnp.subtract)
    m2 = mm(2)
    m3 = mm(3)
    m4 = mm(4)
    c12 = add(m2, m4)
    t11 = sub(m3, m4)
    m1 = mm(1)
    c21 = add(m1, m3)
    t22 = sub(m2, m1)
    m0 = mm(0)
    t11 = add(t11, m0)
    t22 = add(t22, m0)
    c11 = add(t11, mm(6))
    return c11, c12, c21, add(t22, mm(5))


ORDER = (2, 3, 4, 1, 0, 6, 5)


def _zero(i, m):
    return i >> (8 + m)


def _merge(vals):
    return _fold([v[r:r + 8, c:c + 128] for v in vals for r in range(0, v.shape[0], 8)
                  for c in range(0, v.shape[1], 128)], jnp.bitwise_or)


def _gate(never, g):
    def gate(x):
        t = jnp.tile(pltpu.bitcast(g, x.dtype), (x.shape[0] // 8, x.shape[1] // 128))
        return jnp.where(never, t, x)
    return gate


def _tie(never, x, deps):
    if not deps:
        return x
    top = jnp.where(never, _merge(deps), x[:8, :128])
    if x.shape[1] > 128:
        top = jnp.concatenate([top, x[:8, 128:]], axis=1)
    return jnp.concatenate([top, x[8:]], axis=0)


class _Sched:
    def __init__(self, never, plan, jobs):
        self.never, self.plan, self.jobs, self.pending = never, plan, jobs, {}

    def mm(self, site, a, b, dims=NN, width=128, step=32):
        deps = [d() if callable(d) else d for d in self.pending.pop(site, ())]
        a = a() if callable(a) else a
        tie = functools.partial(_tie, self.never, deps=deps)
        a, b = (_bf(tie(a)), _bf(b)) if a.dtype == U32 else (a, _bf(tie(b)))
        out = jax.lax.dot_general(a, b, dims, preferred_element_type=F32)
        per = out.shape[0] // step
        last = {}
        for k, (name, until) in enumerate(self.plan.get(site, ())):
            if name is not None:
                r, c = step * (k % per), width * (k // per)
                vals, stored = self.jobs[name].pop(0)(_gate(self.never, out[r:r + 8, c:c + 128]))
                self.pending.setdefault(until, []).extend(vals)
                last[(getattr(stored, "__code__", None), until)] = stored
        for (_, until), stored in last.items():
            if stored is not None:
                self.pending[until].append(stored)
        return out

    def finish(self):
        assert not any(self.jobs.values()) and not any(self.pending.values())


def _ops49(fn, blocks, m):
    return fn(*[fn(*[blocks[q][e] for q in range(4)])[m] for e in range(4)])


def _words49(fn, words, m):
    halves = [[_split(w) for w in q] for q in words]
    lo = _ops49(fn, [[h[0] for h in q] for q in halves], m)
    hi = _ops49(fn, [[h[1] for h in q] for q in halves], m)
    return [_join(a, b) for a, b in zip(lo, hi)]


def _fold(xs, op):
    acc = xs[0]
    for x in xs[1:]:
        acc = op(acc, x)
    return acc


def _tree(xs, op):
    while len(xs) > 1:
        xs = [op(a, b) for a, b in zip(xs[::2], xs[1::2])]
    return xs[0]


def _lane_chunks(x):
    return [x[:, j * 128:(j + 1) * 128] for j in range(x.shape[1] // 128)]


def _kernel(x_hbm, c_hbm, wq_hbm, wuk_hbm, wuv_hbm, wo_hbm, wqkv_hbm, wob_hbm, gw_hbm,
            out_hbm,
            xs_u, x_r, c_r, w_r, wv_r, wob_p, wkv_r, wq_r, wo_r,
            wperm, xq, cq, wv7, wob5, wo49, wkv, wq49, ups, bx, qn,
            qk_b, vb, lg_s, pr_s, o_s, ob7, ctx, ca0, ca1, g_s, out_s, gw_ref,
            sem_x, sem_p, sem_a):
    x_u = x_hbm.bitcast(U32)
    c_u = c_hbm.bitcast(U32)
    wo_u = wo_hbm.bitcast(U32)
    wq_u = wq_hbm.bitcast(U32)
    wuk_u = wuk_hbm.bitcast(U32)
    wuv_u = wuv_hbm.bitcast(U32)
    wob_u = wob_hbm.bitcast(U32)
    part = functools.partial

    def blk(j, n):
        return pl.ds(pl.multiple_of(j * n, n), n)

    def strip(j):
        return blk(j, 128)

    def cp_x(t):
        return pltpu.make_async_copy(x_u.at[:, strip(t >> 1)], xs_u.at[t >> 1], sem_x.at[0])

    def cp_w(t, sem):
        return pltpu.make_async_copy(wqkv_hbm.at[t >> 3, strip((t >> 1) & 3), blk(t & 1, M)],
                                     w_r.at[t & 1], sem)

    def cp_side(t):
        dp = ((t >> 3) << 2) + (t & 2) + ((t >> 2) & 1)
        sem = sem_x.at[t & 1]
        return (
            pltpu.make_async_copy(x_u.at[blk(t, HQ), :], x_r.at[t & 1], sem),
            pltpu.make_async_copy(c_u.at[blk(t, HQ), :], c_r.at[t & 1], sem),
            pltpu.make_async_copy(wqkv_hbm.at[:, blk(t, 32), pl.ds(2 * M, M)], wv_r.at[t & 1], sem),
            pltpu.make_async_copy(wob_u.at[:, t & 1, dp, :], wob_p.at[blk(t, 16), :], sem),
            pltpu.make_async_copy(wob_u.at[:, t & 1, dp + 8, :], wob_p.at[blk(t + 16, 16), :], sem),
        )

    def cp_wq(p, sem):
        return pltpu.make_async_copy(wq_u.at[:, jnp.minimum(p, NP - 1), :], wq_r.at[p & 3], sem)

    def cp_p(g):
        slot = g & 1
        p = jnp.minimum(g + 1, NP - 1)
        o = jnp.clip(g, 0, NP - 1)
        sem = sem_p.at[slot]
        return (
            pltpu.make_async_copy(wo_u.at[blk(o >> 1, 2 * DA), blk(o & 1, M // 2)],
                                  wo_r.at[slot], sem),
            pltpu.make_async_copy(wuk_u.at[:, p, :], wkv_r.at[slot, pl.ds(DC, DC), :], sem),
            pltpu.make_async_copy(wuv_u.at[:, p, :], wkv_r.at[slot, pl.ds(0, DC), :], sem),
            cp_wq(g + 2, sem),
        )

    def cp_gw():
        return pltpu.make_async_copy(gw_hbm, gw_ref, sem_a.at[0])

    def cp_out(i):
        return pltpu.make_async_copy(out_s.at[blk(i, TO), :], out_hbm.at[blk(i, TO), :],
                                     sem_a.at[1])

    def group(t, fn):
        tc = jnp.minimum(t, 15)
        for d in cp_side(tc):
            pl.when(t < 16)(part(fn, d))
        pl.when((t & 17) == 0)(part(fn, cp_x(tc)))
        pl.when(t < 15)(part(fn, cp_w(jnp.minimum(t + 1, 15), sem_x.at[t & 1])))

    cp_w(0, sem_a.at[1]).start()
    cp_x(0).start()
    cp_w(1, sem_x.at[0]).start()
    for d in cp_side(0):
        d.start()

    for cc in range(8):
        qk_b[8 + cc, pl.ds(0, PAD), :] = jnp.zeros((PAD, 128), F32)
        vb[cc, pl.ds(TQ, PAD), :] = jnp.zeros((PAD, 128), F32)

    def stage_first(t):
        for cc, w in enumerate(_permute8(_lane_chunks(pltpu.bitcast(w_r[t & 1], U32)))):
            wperm[cc] = w

    cp_w(0, sem_a.at[1]).wait()
    stage_first(0)
    cp_w(2, sem_x.at[1]).start()
    for d in cp_side(1):
        d.start()
    cp_gw().start()
    plan1 = _plan1()

    def p1_body(t, carry):
        group(t, lambda d: d.wait())

        def act_sums(src, dst, ns, m, sr, r, gate):
            cw = [[gate(src[(t & 1) + _zero(t, m), pl.ds(32 * (q >> 1) + 16 * (e >> 1) + 8 * r, 8),
                            pl.ds(((2 * (q & 1) + (e & 1)) * ns + sr) * 128, 128)])
                   for e in range(4)] for q in range(4)]
            for n, w in enumerate(_words49(_lhs7, cw, m)):
                dst[7 * m + n, sr, blk(2 * t + r, 8), :] = w
            if ns == 1:
                return [], lambda: dst[7 * m + _zero(t, 0), sr, blk(2 * t + r, 8), :]
            return [], lambda: dst[7 * m + _zero(t, 0), sr, blk(2 * t + r, 8), :]

        wv = _permute8(_lane_chunks(jnp.concatenate(
            [pltpu.bitcast(wv_r[t & 1, e], U32) for e in range(2)], axis=0)))

        def v_sums(r, cc, gate):
            ops = _words7(_rhs7, [gate(wv[cc + 4 * d][16 * e + 8 * r:16 * e + 8 * r + 8])
                                  for e in range(2) for d in range(2)])
            for m in range(7):
                wv7[m, cc, blk(2 * t + r, 8), :] = ops[m]
            return [], lambda: wv7[_zero(t, 0), cc, blk(2 * t + r, 8), :]

        def o_sums(r, cc, gate):
            ops = _words7(_rhs7, [gate(wob_p[blk(2 * t + r + 32 * e, 8), strip(cc + 4 * d)])
                                  for e in range(2) for d in range(2)])
            for e, m in enumerate(RSUM):
                wob5[e, blk(2 * t + r, 8), strip(cc)] = ops[m]
            return [], lambda: wob5[_zero(t, 0), blk(2 * t + r, 8), strip(cc)]

        sched = _Sched(t > 99, plan1, dict(
            x=[part(act_sums, x_r, xq, 2, m, sr, r)
               for m in range(7) for sr in range(2) for r in range(2)],
            c=[part(act_sums, c_r, cq, 1, m, 0, r) for m in range(7) for r in range(2)],
            v=[part(v_sums, r, cc) for r in range(2) for cc in range(4)],
            o=[part(o_sums, r, cc) for r in range(2) for cc in range(4)]))

        first = t < 2
        for half in range(2):
            for rb in range(4):
                w = jnp.concatenate([wperm[4 * half + cc] for cc in range(4)], axis=1)
                r = sched.mm(4 * half + rb, xs_u[t >> 1, pl.ds(rb * 256, 256), :], w)
                for cc in range(4):
                    sl = (8 * (t & 1) + 4 * half + cc, pl.ds(PAD + rb * 512, 512), slice(None))
                    old = jnp.where(first, 0.0, qk_b[sl])
                    qk_b[sl] = old + r[:, cc * 128:(cc + 1) * 128]
        sched.finish()
        stage_first(jnp.minimum(t + 1, 15))

        group(t + 2, lambda d: d.start())

        @pl.when(jnp.logical_and(t >= 7, t < 9))
        def _():
            for d in cp_p(t - 8):
                d.start()

        @pl.when(t == 6)
        def _():
            cp_wq(0, sem_p.at[1]).start()

        return t

    last = jax.lax.fori_loop(0, 16, p1_body, 0)

    row = jax.lax.broadcasted_iota(jnp.int32, (TQ, TQ), 0)
    col = jax.lax.broadcasted_iota(jnp.int32, (TQ, TQ), 1)
    rowi = jax.lax.broadcasted_iota(jnp.int32, (RB, 128), 0)
    odd = (jax.lax.broadcasted_iota(jnp.int32, (RB, 128), 1) & 1) == 1
    NSUB = HQ // RB
    QSCALE = DA ** -0.5 * LOG2E

    def pair_rows(src, slot, r0, n, gate):
        return [_split(gate(src[slot, pl.ds(r0 + par, n // 2, stride=2), :])) for par in range(2)]

    def staging(g, z):
        up, down = {}, {}

        def scales(n1, gate):
            w = pltpu.bitcast(wkv_r[g & 1, pl.ds(n1 * DC, DC), :], jnp.int32)
            rows = [gate(w[:8])] + [w[r:r + 8] for r in range(8, DC, 8)]
            for h in range(2):
                e = _fold([t & (0x7F80 << (16 * h)) for t in rows], jnp.maximum) << (16 - 16 * h)
                e = jnp.max(pltpu.bitcast(e, F32), axis=0, keepdims=True)
                e = jnp.clip(pltpu.bitcast(e, jnp.int32), 1 << 23, 253 << 23)
                e = jnp.broadcast_to(e, (8, 128))
                up[2 * n1 + h] = e
                down[2 * n1 + h] = pltpu.bitcast((254 << 23) - e, F32)
            return [pltpu.bitcast(up[2 * n1] | up[2 * n1 + 1], U32)], None

        def rhs49(dst, tiles, scale, m, r):
            res = [_ops49(_rhs7,
                          [[scale(tiles[2 * (q >> 1) + (e >> 1)][q & 1][par][e & 1],
                                  2 * (q & 1) + (e & 1)) for e in range(4)] for q in range(4)],
                          m) for par in range(2)]
            for k, (lo, hi) in enumerate(zip(*res)):
                dst[7 * m + k, pl.ds(8 * r, 8), :] = _join(lo, hi)

        def kv(m, r, gate):
            while up:
                k, e = up.popitem()
                ups[k] = pltpu.bitcast(gate(e), F32)
            tiles = [[pair_rows(wkv_r, (g & 1) + _zero(z, m), n1 * DC + kt * 128 + 16 * r, 16, gate)
                      for n1 in range(2)] for kt in range(4)]
            rhs49(wkv, tiles, lambda w, k: w * down[k], m, r)
            return [], lambda: wkv[7 * m, blk(r + _zero(z, 0), 8), :]

        def qw(m, r, gate):
            tiles = [[pair_rows(wq_r, ((g + 1 + n1) & 3) + _zero(z, m), kt * 256 + 16 * r, 16, gate)
                      for n1 in range(2)] for kt in range(4)]
            rhs49(wq49, tiles, lambda w, k: w, m, r)
            return [], lambda: wq49[7 * m, blk(r + _zero(z, 0), 8), :]

        def b_lhs(u, r, gate):
            base = 8 * jnp.minimum(g + 1, NQ - 1) + r
            ops = _words7(_lhs7, [gate(xs_u[u + 4 * d, blk(base + 4 * e, 8), :])
                                  for e in range(2) for d in range(2)])
            for k, m in enumerate(LSUM):
                bx[k, pl.ds(8 * r, 8), strip(u)] = ops[m]
            return [], lambda: bx[0, blk(r + _zero(z, 0), 8), strip(u)]

        return dict(sc=[part(scales, n1) for n1 in range(2)],
                    kv=[part(kv, m, r) for m in range(7) for r in range(8)],
                    qw=[part(qw, m, r) for m in range(7) for r in range(16)],
                    bx=[part(b_lhs, u, r) for u in range(4) for r in range(4)])

    cp_wq(0, sem_p.at[1]).wait()
    for d in cp_p(-1):
        d.wait()
    sched = _Sched(last > 99, _planx(), staging(-1, last))
    w0 = pair_rows(wq_r, 0, 0, M, lambda x: x)
    w0 = [_join(w0[0][h], w0[1][h]) for h in range(2)]
    for g in range(4):
        for e in range(2):
            for h in range(2):
                q = [sched.mm(8 * g + 4 * e + 2 * h + k, jnp.concatenate(
                    [xs_u[4 * k + u, pl.ds((4 * g + 2 + e) * HQ, HQ), :] for u in range(4)], axis=1),
                    w0[h][256 * k:256 * k + 256], step=16) for k in range(2)]
                qn[h, g, e] = _pack((q[0] + q[1]) * QSCALE)
    sched.finish()
    for d in cp_p(1):
        d.start()
    plan2 = _plan2()

    def p2_body(p, carry):
        for d in cp_p(p):
            d.wait()
        causal = col <= row
        never = p > NP
        jobs = staging(p, p)
        sched = _Sched(never, plan2, jobs)
        mm = sched.mm

        r0 = pl.multiple_of(p * TQ, TQ)

        def scatter(dst, off, c):
            for e, t in enumerate(c):
                for cc in range(4):
                    dst[4 * (e & 1) + cc, pl.ds(off + (PAD + (e >> 1) * HQ), HQ), :] = (
                        t[:, cc * 128:(cc + 1) * 128])

        def proj_bv():
            def lhs(m):
                if m in (2, 3):
                    return jnp.concatenate([xs_u[u + 4 * (m - 2), blk(2 * p + m - 2, QQ), :]
                                            for u in range(4)], axis=1)
                return bx[LSUM.index(m)]

            for cc in range(8):
                vb[cc, pl.ds(0, PAD), :] = vb[cc, pl.ds(TQ, PAD), :]
            c = [_combine(lambda m: mm(("bv", 7 * e + ORDER.index(m)), lhs(m), jnp.concatenate(
                [wv7[m, 2 * e], wv7[m, 2 * e + 1]], axis=1))) for e in range(2)]
            scatter(vb, 0, [jnp.concatenate(t, axis=1) for t in zip(*c)])

        def local_qk(rb, w, gate):
            pr = [qk_b[cc, pl.ds(r0 + _zero(p, w) + (PAD + rb * RB), RB), :]
                  * qk_b[8 + cc, pl.ds(r0 + (PAD + rb * RB - DIL * w), RB), :] for cc in range(8)]
            pr[0] = gate(pr[0])
            t = _fold(pr, jnp.add)
            t = t + pltpu.roll(t, 64, 1)
            t = t + jnp.where(odd, pltpu.roll(t, 1, 1), pltpu.roll(t, 127, 1))
            t = t * (DB ** -0.5 * LOG2E)
            if rb == 0 and w:
                t = jnp.where(rowi + r0 >= DIL * w, t, NEG)
            lg_s[w, pl.ds(rb * RB, RB), :] = t
            return [], lambda: pltpu.bitcast(lg_s[w, blk(2 * rb + _zero(p, 0), 8), :], U32)

        def local_sm(rb, e, gate):
            rows = pl.ds(rb * RB + SMR * e, SMR)
            lg = [gate(lg_s[w, rows, :]) for w in range(WIN)]
            m = _tree(lg, jnp.maximum)
            ps = [jnp.exp2(t - m) for t in lg]
            l = _tree(ps, jnp.add)
            r = pl.reciprocal(l, approx=True)
            r = r * (2.0 - l * r)
            for w in range(WIN):
                pr_s[w, rows, :] = ps[w] * r
            return [], lambda: pltpu.bitcast(pr_s[0, blk(2 * rb + e + _zero(p, 0), 8), :], U32)

        def local_pv(rb, cc, gate):
            rows = pl.ds(rb * RB, RB)
            pr = [pr_s[w + _zero(p, cc), rows, :]
                  * vb[cc, pl.ds(PAD + rb * RB - DIL * w, RB), :] for w in range(WIN)]
            pr[0] = gate(pr[0])
            o = _fold(pr, jnp.add)
            if rb < NSUB or cc < 4:
                o_s[cc, rows, :] = o
                return [], lambda: pltpu.bitcast(o_s[cc, blk(2 * rb + _zero(p, 0), 8), :], U32)
            top = pl.ds((rb - NSUB) * RB, RB)
            ops = _lhs7(o_s[cc - 4, top, :], o_s[cc, top, :], o_s[cc - 4, rows, :], o)
            cols = pl.ds((cc - 4) * 128, 128)
            for m, t in enumerate(ops):
                ob7[m, pl.ds((rb - NSUB) * RB // 2, RB // 2), cols] = _pack(t)
            return [], lambda: ob7[0, blk(rb - NSUB + _zero(p, 0), 8), cols]

        order = [rb + e * NSUB for rb in range(NSUB) for e in range(2)]
        jobs["lo"] = []
        for k in range(len(order) + 2):
            for f, d, n in ((local_sm, 1, RB // SMR), (local_qk, 0, 8), (local_pv, 2, 8)):
                if 0 <= k - d < len(order):
                    jobs["lo"] += [part(f, order[k - d], e) for e in range(n)]

        def wob(m):
            if m == 1:
                return wob_p[pl.ds(0, M // 4), pl.ds(0, M // 2)]
            if m == 4:
                return wob_p[pl.ds(M // 4, M // 4), pl.ds(M // 2, M // 2)]
            return wob5[RSUM.index(m)]

        bo = {}

        def proj_bo(n):
            for m in ORDER[len(bo):len(bo) + n]:
                bo[m] = mm(("bo", len(bo)), lambda: ob7[m], wob(m))
            if n and len(bo) == 7:
                scatter(qk_b, r0, _combine(lambda m: bo[m]))

        def out_weights(m, r, gate):
            ww = [[gate(wo_r[(p & 1) + _zero(p, m),
                             pl.ds((2 * (q >> 1) + (e >> 1)) * HQ + 8 * r, 8),
                             pl.ds((2 * (q & 1) + (e & 1)) * 128, 128)])
                   for e in range(4)] for q in range(4)]
            rows = blk(8 * (p >> 1) + r, 8)
            for n, w in enumerate(_words49(_rhs7, ww, m)):
                wo49[7 * m + n, p & 1, rows, :] = w
            return [], lambda: wo49[7 * m + _zero(p, 0), p & 1, rows, :]

        jobs["wo"] = [part(out_weights, m, r) for m in range(7) for r in range(8)]

        ks, vs, qs = {}, {}, {}
        done, prods = {}, {}

        def project(kind, j, n, lhs, rhs, scale):
            got = prods.setdefault((kind, j), {})
            for m in ORDER[len(got):len(got) + n]:
                got[m] = _combine(lambda k: mm((kind, j, 7 * len(got) + ORDER.index(k)),
                                               lhs(7 * m + k), rhs[7 * m + k]))
            if len(got) < 7:
                return None
            c = _combine(lambda m: got[m])
            c = [[_pack(c[(rg & 2) + (cg >> 1)][2 * (rg & 1) + (cg & 1)] * scale(cg))
                  for rg in range(4)] for cg in range(4)]
            return [[jnp.concatenate([t[16 * e:16 * e + 16] for t in c[cg]], axis=0)
                     for e in range(2)] for cg in range(4)]

        def proj_kv(j, n):
            c = project("kv", j, n, lambda k: cq[k, 0, pl.ds(j * QQ, QQ), :], wkv,
                        lambda cg: ups[cg][:1])
            if c is not None:
                for cg in range(4):
                    for e in range(2):
                        (vs, ks)[cg >> 1][(cg & 1, 2 * j + e)] = c[cg][e]

        def proj_q(g, n):
            rows = blk(2 * g + (p & 1), QQ)
            c = project("q", g, n,
                        lambda k: jnp.concatenate([xq[k, sr, rows, :] for sr in range(2)], axis=1),
                        wq49, lambda cg: QSCALE)
            if c is not None:
                for h in range(2):
                    for e in range(2):
                        old = qn[h, g, e]
                        for b in range(2):
                            qs[(h, 4 * g + 2 * b + e)] = jnp.where((p & 1) == b, c[h][e], old)
                        qn[h, g, e] = c[2 + h][e]

        def qk(h, i, dep):
            kk = jnp.concatenate([ks[(h, j)] for j in range(i + 1)], axis=0)
            q = qs[(h, i)]
            if dep is not None:
                q = jnp.where(never, done[(h, dep)], q)
            ch = _lane_chunks(mm(("qk", h, i), q, kk, NT, 512))
            ch[i] = jnp.where(causal, ch[i], NEG)
            return ch

        def softmax_pv(h, i, ch):
            m = jnp.max(_fold(ch, jnp.maximum), axis=1, keepdims=True)
            ps = [jnp.exp2(c - m) for c in ch]
            lp = ps[0]
            for j in range(1, i + 1):
                lp = lp + ps[j]
                if TIE and (j % TIE == TIE - 1 or j == i):
                    ps[j] = jnp.where(never, lp, ps[j])
            pb = jnp.concatenate(ps, axis=1).astype(BF16)
            vv = jnp.concatenate([vs[(h, j)] for j in range(i + 1)], axis=0)
            o = mm(("pv", h, i), pb, vv)
            if i >= LDEP:
                lp = jnp.where(never, o, lp)
            l = jnp.sum(lp, axis=1, keepdims=True)
            r = pl.reciprocal(l, approx=True)
            r = r * (2.0 - l * r)
            cn = _pack(o * r)
            done[(h, i)] = cn
            ctx[2 * p + h, pl.ds(i * HQ, HQ), :] = cn

        proj_bv()
        proj_kv(0, 7)
        proj_q(0, 7)
        for i in range(NQ):
            dep = i - DEP if i >= DEP else None
            s0 = qk(0, i, dep)
            s1 = qk(1, i, dep)
            if i + 2 < NQ:
                proj_kv(i // 2 + 1, 7 if i & 1 else KVS // 7)
                if i < 6:
                    proj_q(i // 2 + 1, 7 if i & 1 else QS // 7)
            else:
                proj_bo(BOP[i + 2 - NQ])
            softmax_pv(0, i, s0)
            softmax_pv(1, i, s1)
        proj_bo(BOP[2])
        sched.finish()
        for d in cp_p(p + 2):
            d.start()
        return carry

    jax.lax.fori_loop(0, NP, p2_body, 0)

    cp_gw().wait()
    gw = gw_ref[...].astype(F32)
    plan3 = _plan3()
    cab = (ca0, ca1)

    def p3_body(i, carry):
        r0 = pl.multiple_of(i * TO, TO)
        h0 = pl.multiple_of(i * (TO // 2), TO // 2)
        never = i > S

        def ctx_words(m, u, r, n):
            return [[ctx[4 * u + 2 * (q & 1) + (e & 1),
                         pl.ds(h0 + _zero(i, m) * 8 + ((2 * (q >> 1) + (e >> 1)) * QQ + r), n), :]
                     for e in range(4)] for q in range(4)]

        def operands(k, u, r, gate):
            m = ORDER[k]
            cw = [[gate(w) for w in q] for q in ctx_words(m, u, r, 8)]
            for n, w in enumerate(_words49(_lhs7, cw, m)):
                if not (m in (2, 3) and n in (2, 3)):
                    cab[k & 1][n, pl.ds(r, 8), pl.ds(u * 128, 128)] = w
            return [], lambda: cab[k & 1][_zero(i, 0), pl.ds(r, 8), pl.ds(u * 128, 128)]

        def gate_rows(r, gate):
            gs = _fold([_bf(gate(xs_u[j, pl.ds(h0 + r, 8), :])).astype(F32) * gw[j:j + 1]
                        for j in range(8)], jnp.add)
            g = jax.nn.sigmoid(jnp.sum(gs, axis=1, keepdims=True))
            g_s[pl.ds(2 * r, 16), :] = jnp.broadcast_to(g, (16, 128))
            return [], lambda: pltpu.bitcast(g_s[blk(r // 4 + _zero(i, 0), 8), :], U32)

        sched = _Sched(never, plan3, dict(
            a=[part(operands, k, u, r) for k in range(1, 7) for u in range(HA // 4)
               for r in range(0, QQ, 8)],
            g=[part(gate_rows, r) for r in range(0, TO // 2, 8)]))
        first = [[_words49(_lhs7, ctx_words(ORDER[0], u, 0, QQ), ORDER[0])[n]
                  for u in range(HA // 4)] for n in range(7)]

        def inner(m, n):
            k = ORDER.index(m)
            res = []
            for e in range(2):
                us = range(4 * e, 4 * e + 4)
                if m in (2, 3) and n in (2, 3):
                    lhs = jnp.concatenate([ctx_words(m, u, 0, QQ)[3 * (m - 2)][3 * (n - 2)]
                                           for u in us], axis=1)
                elif k == 0:
                    lhs = jnp.concatenate([first[n][u] for u in us], axis=1)
                else:
                    lhs = lambda: cab[k & 1][n, :, pl.ds(e * 512, 512)]
                rhs = jnp.concatenate([wo49[7 * m + n, cc, pl.ds(e * 256, 256), :]
                                       for cc in range(2)], axis=1)
                res.append(sched.mm((k, 2 * ORDER.index(n) + e), lhs, rhs))
            return res[0] + res[1]

        acs = _combine(lambda m: _combine(lambda n: inner(m, n)))
        sched.finish()
        for q in range(4):
            for e in range(4):
                off = (2 * (q >> 1) + (e >> 1)) * HQ
                g = g_s[pl.ds(off, HQ), :]
                for cc in range(2):
                    ch = 4 * cc + 2 * (q & 1) + (e & 1)
                    a = acs[q][e][:, cc * 128:(cc + 1) * 128]
                    b = qk_b[ch, pl.ds(r0 + (PAD + off), HQ), :]
                    out_s[pl.ds(r0 + off, HQ), pl.ds(ch * 128, 128)] = (
                        g * a + (1.0 - g) * b).astype(BF16)
        cp_out(i).start()
        return carry

    jax.lax.fori_loop(0, S // TO, p3_body, 0)
    for g in range(NP, NP + 2):
        for d in cp_p(g):
            d.wait()
    for i in range(S // TO):
        cp_out(i).wait()


@jax.jit
def pallas_gated_mix__compressed_kv_cla__sliding_local_dilated__prompt_kernel(
    A_x: jax.Array,
    A_c_kv: jax.Array,
    A_w_q: jax.Array,
    A_w_uk: jax.Array,
    A_w_uv: jax.Array,
    A_w_o: jax.Array,
    B_x: jax.Array,
    B_wqkv: jax.Array,
    B_wo: jax.Array,
    gate_w: jax.Array,
):
    del B_x
    any_spec = pl.BlockSpec(memory_space=pl.ANY)
    out = pl.pallas_call(
        _kernel,
        in_specs=[any_spec] * 9,
        out_specs=any_spec,
        out_shape=jax.ShapeDtypeStruct((S, M), BF16),
        scratch_shapes=[
            pltpu.VMEM((8, S // 2, 128), U32),
            pltpu.VMEM((2, HQ, M), U32),
            pltpu.VMEM((2, HQ, DC), U32),
            pltpu.VMEM((2, 128, M), BF16),
            pltpu.VMEM((2, 2, 32, M), BF16),
            pltpu.VMEM((M // 2, M), U32),
            pltpu.VMEM((2, 2 * DC, 128), U32),
            pltpu.VMEM((4, M, 128), U32),
            pltpu.VMEM((2, 2 * DA, M // 2), U32),
            pltpu.VMEM((8, 64, 128), U32),
            pltpu.VMEM((49, 2, S // 8, 128), U32),
            pltpu.VMEM((49, 1, S // 8, 128), U32),
            pltpu.VMEM((7, 4, M // 4, 128), U32),
            pltpu.VMEM((5, M // 4, M // 2), U32),
            pltpu.VMEM((49, 2, NP * QQ, 128), U32),
            pltpu.VMEM((49, HQ, 128), U32),
            pltpu.VMEM((49, TQ, 128), U32),
            pltpu.VMEM((4, 8, 128), F32),
            pltpu.VMEM((5, QQ, M // 2), U32),
            pltpu.VMEM((2, 4, 2, HQ, 128), U32),
            pltpu.VMEM((16, S + PAD, 128), F32),
            pltpu.VMEM((8, TQ + PAD, 128), F32),
            pltpu.VMEM((WIN, TQ, 128), F32),
            pltpu.VMEM((WIN, TQ, 128), F32),
            pltpu.VMEM((8, TQ, 128), F32),
            pltpu.VMEM((7, QQ, M // 2), U32),
            pltpu.VMEM((HA, S // 2, 128), U32),
            pltpu.VMEM((7, QQ, M), U32),
            pltpu.VMEM((7, QQ, M), U32),
            pltpu.VMEM((TO, 128), F32),
            pltpu.VMEM((S, M), BF16),
            pltpu.VMEM((8, 128), BF16),
            pltpu.SemaphoreType.DMA((2,)),
            pltpu.SemaphoreType.DMA((2,)),
            pltpu.SemaphoreType.DMA((2,)),
        ],
        compiler_params=pltpu.CompilerParams(vmem_limit_bytes=120 * 1024 * 1024,
                                             disable_bounds_checks=True),
    )(
        A_x.reshape(S, M),
        A_c_kv.reshape(S, DC),
        A_w_q,
        A_w_uk,
        A_w_uv,
        A_w_o.reshape(HA * DA, M),
        B_wqkv.reshape(2, M // 2, 3 * M),
        B_wo.reshape(HB // 2, 2, DB, M),
        gate_w.reshape(8, 128),
    )
    return out.reshape(1, S, M)
```

```python
import functools
import math

import jax
import jax.numpy as jnp
import jax.experimental.pallas as pl
import jax.experimental.pallas.tpu as pltpu

F32 = jnp.float32
BF16 = jnp.bfloat16
U32 = jnp.uint32

S = 2048
M = 1024
HA = 32
DA = 128
DC = 512
HB = 32
DB = 32
WIN = 8
DIL = 2
PAD = 16
LOG2E = math.log2(math.e)
NEG = -1e9

TQ = 128
HQ = TQ // 2
QQ = TQ // 4
BOP = (2, 3, 2)
LX = 16
KVS = 28
QS = 28
QST = 3
LQ0 = 3
LG = 2
XN = 29
SK = 3
SMR = 16
P1N = 6
P1U = 2
P3S = 4
P3E = 12
NQ = S // TQ
NP = HA // 2
DEP = 2
TIE = 4
RB = 16
LDEP = 4
TO = 256
NN = (((1,), (0,)), ((), ()))
NT = (((1,), (1,)), ((), ()))


def _plan2():
    plan = {}

    def put(name, count, start, until):
        plan.setdefault(start, []).extend([(name, until)] * count)

    def after_qk(i):
        if i >= NQ - 2:
            return ("bo", (i - NQ + 2) * BOP[0] + 1)
        return ("kv", i // 2 + 1, KVS * (i & 1) + LX)

    def fill(name, count, sites):
        for start, room, until in sites:
            n = min(count, room - len(plan.get(start, ())))
            put(name, n, start, until)
            count -= n
        assert count == 0, (name, count)

    def qk_sites(lo, hi):
        return [(("qk", h, i), max(i + 1 - h * SK, 0), after_qk(i))
                for i in range(lo, hi) for h in range(2)]

    def q_sites(g, lo, hi, until):
        return [(("q", g, k), 1, until) for k in range(lo, hi, QST)]

    for k in range(14):
        put("wo", 4, ("bv", k), ("kv", 0, 24))
    put("sc", 1, ("kv", 0, 0), ("q", 0, 0))
    put("sc", 1, ("kv", 0, 24), ("q", 0, 8))
    early = q_sites(0, 8, 45, ("kv", 1, 8))
    for g in range(1, 4):
        early += q_sites(g, 0, QS - 4, after_qk(2 * g - 1))
        early += qk_sites(max(2 * g - 1, LQ0), 2 * g)
        early += q_sites(g, QS, 45, after_qk(2 * g))
        early += qk_sites(max(2 * g, LQ0), 2 * g + 1)
    fill("lo", 64 // LG + 32 + 128 // SMR, early)
    fill("bx", 16, early + qk_sites(7, 14))
    fill("qw", 112, qk_sites(7, 14))
    fill("kv", 56, qk_sites(14, 16) + [(("bo", k), 8, ("bo", 6)) for k in range(BOP[0], 5)])
    return plan


def _planx():
    names = _spread(["sc"] * 2 + ["bx"] * 16 + ["qw"] * 112 + ["kv"] * 56, 8 * XN)
    return {k: [(n, 31) for n in names[8 * k:8 * k + 8]] for k in range(XN)}


def _spread(names, ticks):
    out = [None] * ticks
    for k, name in enumerate(names):
        out[k * ticks // len(names)] = name
    return out


def _plan1():
    names = _spread(["x"] * 28 + ["c"] * 14 + ["o"] * 8 + ["v"] * 8, 16 * P1N)
    return {k: [(n, min(k + P1U, 7)) for n in names[16 * k:16 * k + 16]] for k in range(P1N)}


def _plan3():
    plan = {}
    for k in range(6):
        lo = P3S if k == 0 else 0
        extra = ["g"] * 8 if k in (1, 2) else []
        names = _spread(["a"] * 32 + extra, 4 * (P3E - lo))
        for d in range(lo, P3E):
            plan[(k, d)] = [(n, (k + 1, 0)) for n in names[4 * (d - lo):4 * (d - lo) + 4]]
    return plan


_STAGES = ((2, 4), (1, 3), (0, 2), (0, 6), (0, 1))


def _permute8(cols):
    cols = list(cols)
    lane = jax.lax.broadcasted_iota(jnp.int32, cols[0].shape, 1)
    for va, lb in _STAGES:
        lo = (lane & (1 << lb)) == 0
        sh = 1 << lb
        idx = [i for i in range(8) if not (i >> va) & 1]
        if lb == 6:
            rr = [pltpu.roll(jnp.where(lo, cols[i | (1 << va)], cols[i]), 64, 1) for i in idx]
            for i, r in zip(idx, rr):
                a, b = cols[i], cols[i | (1 << va)]
                cols[i] = jnp.where(lo, a, r)
                cols[i | (1 << va)] = jnp.where(lo, r, b)
        else:
            rb = [pltpu.roll(cols[i | (1 << va)], sh, 1) for i in idx]
            ra = [pltpu.roll(cols[i], 128 - sh, 1) for i in idx]
            for i, xa, xb in zip(idx, ra, rb):
                a, b = cols[i], cols[i | (1 << va)]
                cols[i] = jnp.where(lo, a, xb)
                cols[i | (1 << va)] = jnp.where(lo, xa, b)
    return cols


def _pack(x):
    return pltpu.bitcast(x.astype(BF16), U32)


def _bf(x):
    return pltpu.bitcast(x, BF16)


def _split(w):
    return (pltpu.bitcast(w << 16, F32), pltpu.bitcast(w & jnp.uint32(0xFFFF0000), F32))


def _join(lo, hi):
    return pltpu.bitcast(pltpu.pack_elementwise([lo, hi], packed_dtype=BF16), U32)


def _lhs7(a11, a12, a21, a22):
    return [a11 + a22, a21 + a22, a11, a22, a11 + a12, a21 - a11, a12 - a22]


def _rhs7(b11, b12, b21, b22):
    return [b11 + b22, b11, b12 - b22, b21 - b11, b22, b11 + b12, b21 + b22]


LSUM = (0, 1, 4, 5, 6)
RSUM = (0, 2, 3, 5, 6)


def _words7(fn, quads):
    halves = [_split(w) for w in quads]
    lo = fn(*[h[0] for h in halves])
    hi = fn(*[h[1] for h in halves])
    return [_join(a, b) for a, b in zip(lo, hi)]


def _combine(mm):
    add = functools.partial(jax.tree.map, jnp.add)
    sub = functools.partial(jax.tree.map, jnp.subtract)
    m2 = mm(2)
    m3 = mm(3)
    m4 = mm(4)
    c12 = add(m2, m4)
    t11 = sub(m3, m4)
    m1 = mm(1)
    c21 = add(m1, m3)
    t22 = sub(m2, m1)
    m0 = mm(0)
    t11 = add(t11, m0)
    t22 = add(t22, m0)
    c11 = add(t11, mm(6))
    return c11, c12, c21, add(t22, mm(5))


ORDER = (2, 3, 4, 1, 0, 6, 5)


def _zero(i, m):
    return i >> (8 + m)


def _merge(vals):
    return _fold([v[r:r + 8, c:c + 128] for v in vals for r in range(0, v.shape[0], 8)
                  for c in range(0, v.shape[1], 128)], jnp.bitwise_or)


def _gate(never, g):
    def gate(x):
        t = jnp.tile(pltpu.bitcast(g, x.dtype), (x.shape[0] // 8, x.shape[1] // 128))
        return jnp.where(never, t, x)
    return gate


def _tie(never, x, deps):
    if not deps:
        return x
    top = jnp.where(never, _merge(deps), x[:8, :128])
    if x.shape[1] > 128:
        top = jnp.concatenate([top, x[:8, 128:]], axis=1)
    return jnp.concatenate([top, x[8:]], axis=0)


class _Sched:
    def __init__(self, never, plan, jobs):
        self.never, self.plan, self.jobs, self.pending = never, plan, jobs, {}

    def mm(self, site, a, b, dims=NN, width=128, step=32):
        deps = [d() if callable(d) else d for d in self.pending.pop(site, ())]
        a = a() if callable(a) else a
        tie = functools.partial(_tie, self.never, deps=deps)
        a, b = (_bf(tie(a)), _bf(b)) if a.dtype == U32 else (a, _bf(tie(b)))
        out = jax.lax.dot_general(a, b, dims, preferred_element_type=F32)
        per = out.shape[0] // step
        last = {}
        for k, (name, until) in enumerate(self.plan.get(site, ())):
            if name is not None:
                r, c = step * (k % per), width * (k // per)
                vals, tag, stored = self.jobs[name].pop(0)(
                    _gate(self.never, out[r:r + 8, c:c + 128]))
                self.pending.setdefault(until, []).extend(vals)
                last[(name, tag, until)] = stored
        for (_, _, until), stored in last.items():
            if stored is not None:
                self.pending[until].append(stored)
        return out

    def finish(self):
        assert not any(self.jobs.values()) and not any(self.pending.values())


def _ops49(fn, blocks, m):
    return fn(*[fn(*[blocks[q][e] for q in range(4)])[m] for e in range(4)])


def _words49(fn, words, m):
    halves = [[_split(w) for w in q] for q in words]
    lo = _ops49(fn, [[h[0] for h in q] for q in halves], m)
    hi = _ops49(fn, [[h[1] for h in q] for q in halves], m)
    return [_join(a, b) for a, b in zip(lo, hi)]


def _fold(xs, op):
    acc = xs[0]
    for x in xs[1:]:
        acc = op(acc, x)
    return acc


def _tree(xs, op):
    while len(xs) > 1:
        xs = [op(a, b) for a, b in zip(xs[::2], xs[1::2])]
    return xs[0]


def _lane_chunks(x):
    return [x[:, j * 128:(j + 1) * 128] for j in range(x.shape[1] // 128)]


def _kernel(x_hbm, c_hbm, wq_hbm, wuk_hbm, wuv_hbm, wo_hbm, wqkv_hbm, wob_hbm, gw_hbm,
            out_hbm,
            xs_u, x_r, c_r, w_r, wv_r, wob_p, wkv_r, wq_r, wo_r,
            wperm, xq, cq, wv7, wob5, wo49, wkv, wq49, ups, bx, qn,
            qk_b, vb, lg_s, pr_s, o_s, ob7, ctx, ca0, ca1, g_s, out_s, gw_ref,
            sem_x, sem_p, sem_a):
    x_u = x_hbm.bitcast(U32)
    c_u = c_hbm.bitcast(U32)
    wo_u = wo_hbm.bitcast(U32)
    wq_u = wq_hbm.bitcast(U32)
    wuk_u = wuk_hbm.bitcast(U32)
    wuv_u = wuv_hbm.bitcast(U32)
    wob_u = wob_hbm.bitcast(U32)
    part = functools.partial

    def blk(j, n):
        return pl.ds(pl.multiple_of(j * n, n), n)

    def strip(j):
        return blk(j, 128)

    def cp_x(t):
        return pltpu.make_async_copy(x_u.at[:, strip(t >> 1)], xs_u.at[t >> 1], sem_x.at[0])

    def cp_w(t, sem):
        return pltpu.make_async_copy(wqkv_hbm.at[t >> 3, strip((t >> 1) & 3), blk(t & 1, M)],
                                     w_r.at[t & 1], sem)

    def cp_side(t):
        dp = ((t >> 3) << 2) + (t & 2) + ((t >> 2) & 1)
        sem = sem_x.at[t & 1]
        return (
            pltpu.make_async_copy(x_u.at[blk(t, HQ), :], x_r.at[t & 1], sem),
            pltpu.make_async_copy(c_u.at[blk(t, HQ), :], c_r.at[t & 1], sem),
            pltpu.make_async_copy(wqkv_hbm.at[:, blk(t, 32), pl.ds(2 * M, M)], wv_r.at[t & 1], sem),
            pltpu.make_async_copy(wob_u.at[:, t & 1, dp, :], wob_p.at[blk(t, 16), :], sem),
            pltpu.make_async_copy(wob_u.at[:, t & 1, dp + 8, :], wob_p.at[blk(t + 16, 16), :], sem),
        )

    def cp_wq(p, sem):
        return pltpu.make_async_copy(wq_u.at[:, jnp.minimum(p, NP - 1), :], wq_r.at[p & 3], sem)

    def cp_p(g):
        slot = g & 1
        p = jnp.minimum(g + 1, NP - 1)
        o = jnp.clip(g, 0, NP - 1)
        sem = sem_p.at[slot]
        return (
            pltpu.make_async_copy(wo_u.at[blk(o >> 1, 2 * DA), blk(o & 1, M // 2)],
                                  wo_r.at[slot], sem),
            pltpu.make_async_copy(wuk_u.at[:, p, :], wkv_r.at[slot, pl.ds(DC, DC), :], sem),
            pltpu.make_async_copy(wuv_u.at[:, p, :], wkv_r.at[slot, pl.ds(0, DC), :], sem),
            cp_wq(g + 2, sem),
        )

    def cp_gw():
        return pltpu.make_async_copy(gw_hbm, gw_ref, sem_a.at[0])

    def cp_out(i):
        return pltpu.make_async_copy(out_s.at[blk(i, TO), :], out_hbm.at[blk(i, TO), :],
                                     sem_a.at[1])

    def group(t, fn):
        tc = jnp.minimum(t, 15)
        for d in cp_side(tc):
            pl.when(t < 16)(part(fn, d))
        pl.when((t & 17) == 0)(part(fn, cp_x(tc)))
        pl.when(t < 15)(part(fn, cp_w(jnp.minimum(t + 1, 15), sem_x.at[t & 1])))

    cp_w(0, sem_a.at[1]).start()
    cp_x(0).start()
    cp_w(1, sem_x.at[0]).start()
    for d in cp_side(0):
        d.start()

    for cc in range(8):
        qk_b[8 + cc, pl.ds(0, PAD), :] = jnp.zeros((PAD, 128), F32)
        vb[cc, pl.ds(TQ, PAD), :] = jnp.zeros((PAD, 128), F32)

    def stage_first(t):
        for cc, w in enumerate(_permute8(_lane_chunks(pltpu.bitcast(w_r[t & 1], U32)))):
            wperm[cc] = w

    cp_w(0, sem_a.at[1]).wait()
    stage_first(0)
    cp_w(2, sem_x.at[1]).start()
    for d in cp_side(1):
        d.start()
    cp_gw().start()
    plan1 = _plan1()

    def p1_body(t, carry):
        group(t, lambda d: d.wait())

        def act_sums(src, dst, ns, m, sr, r, gate):
            cw = [[gate(src[(t & 1) + _zero(t, m), pl.ds(32 * (q >> 1) + 16 * (e >> 1) + 8 * r, 8),
                            pl.ds(((2 * (q & 1) + (e & 1)) * ns + sr) * 128, 128)])
                   for e in range(4)] for q in range(4)]
            for n, w in enumerate(_words49(_lhs7, cw, m)):
                dst[7 * m + n, sr, blk(2 * t + r, 8), :] = w
            return [], 0, lambda: dst[7 * m + _zero(t, 0), sr, blk(2 * t + r, 8), :]

        wv = _permute8(_lane_chunks(jnp.concatenate(
            [pltpu.bitcast(wv_r[t & 1, e], U32) for e in range(2)], axis=0)))

        def v_sums(r, cc, gate):
            ops = _words7(_rhs7, [gate(wv[cc + 4 * d][16 * e + 8 * r:16 * e + 8 * r + 8])
                                  for e in range(2) for d in range(2)])
            for m in range(7):
                wv7[m, cc, blk(2 * t + r, 8), :] = ops[m]
            return [], 0, lambda: wv7[_zero(t, 0), cc, blk(2 * t + r, 8), :]

        def o_sums(r, cc, gate):
            ops = _words7(_rhs7, [gate(wob_p[blk(2 * t + r + 32 * e, 8), strip(cc + 4 * d)])
                                  for e in range(2) for d in range(2)])
            for e, m in enumerate(RSUM):
                wob5[e, blk(2 * t + r, 8), strip(cc)] = ops[m]
            return [], 0, lambda: wob5[_zero(t, 0), blk(2 * t + r, 8), strip(cc)]

        sched = _Sched(t > 99, plan1, dict(
            x=[part(act_sums, x_r, xq, 2, m, sr, r)
               for m in range(7) for sr in range(2) for r in range(2)],
            c=[part(act_sums, c_r, cq, 1, m, 0, r) for m in range(7) for r in range(2)],
            v=[part(v_sums, r, cc) for r in range(2) for cc in range(4)],
            o=[part(o_sums, r, cc) for r in range(2) for cc in range(4)]))

        first = t < 2
        for half in range(2):
            for rb in range(4):
                w = jnp.concatenate([wperm[4 * half + cc] for cc in range(4)], axis=1)
                r = sched.mm(4 * half + rb, xs_u[t >> 1, pl.ds(rb * 256, 256), :], w)
                for cc in range(4):
                    sl = (8 * (t & 1) + 4 * half + cc, pl.ds(PAD + rb * 512, 512), slice(None))
                    old = jnp.where(first, 0.0, qk_b[sl])
                    qk_b[sl] = old + r[:, cc * 128:(cc + 1) * 128]
        sched.finish()
        stage_first(jnp.minimum(t + 1, 15))

        group(t + 2, lambda d: d.start())

        @pl.when(jnp.logical_and(t >= 7, t < 9))
        def _():
            for d in cp_p(t - 8):
                d.start()

        @pl.when(t == 6)
        def _():
            cp_wq(0, sem_p.at[1]).start()

        return t

    last = jax.lax.fori_loop(0, 16, p1_body, 0)

    row = jax.lax.broadcasted_iota(jnp.int32, (TQ, TQ), 0)
    col = jax.lax.broadcasted_iota(jnp.int32, (TQ, TQ), 1)
    rowi = jax.lax.broadcasted_iota(jnp.int32, (RB, 128), 0)
    odd = (jax.lax.broadcasted_iota(jnp.int32, (RB, 128), 1) & 1) == 1
    NSUB = HQ // RB
    QSCALE = DA ** -0.5 * LOG2E

    def pair_rows(src, slot, r0, n, gate):
        return [_split(gate(src[slot, pl.ds(r0 + par, n // 2, stride=2), :])) for par in range(2)]

    def staging(g, z):
        up, down = {}, {}

        def scales(n1, gate):
            w = pltpu.bitcast(wkv_r[g & 1, pl.ds(n1 * DC, DC), :], jnp.int32)
            rows = [gate(w[:8])] + [w[r:r + 8] for r in range(8, DC, 8)]
            for h in range(2):
                e = _fold([t & (0x7F80 << (16 * h)) for t in rows], jnp.maximum) << (16 - 16 * h)
                e = jnp.max(pltpu.bitcast(e, F32), axis=0, keepdims=True)
                e = jnp.clip(pltpu.bitcast(e, jnp.int32), 1 << 23, 253 << 23)
                e = jnp.broadcast_to(e, (8, 128))
                up[2 * n1 + h] = e
                down[2 * n1 + h] = pltpu.bitcast((254 << 23) - e, F32)
            return [pltpu.bitcast(up[2 * n1] | up[2 * n1 + 1], U32)], 0, None

        def rhs49(dst, tiles, scale, m, r):
            res = [_ops49(_rhs7,
                          [[scale(tiles[2 * (q >> 1) + (e >> 1)][q & 1][par][e & 1],
                                  2 * (q & 1) + (e & 1)) for e in range(4)] for q in range(4)],
                          m) for par in range(2)]
            for k, (lo, hi) in enumerate(zip(*res)):
                dst[7 * m + k, pl.ds(8 * r, 8), :] = _join(lo, hi)

        def kv(m, r, gate):
            while up:
                k, e = up.popitem()
                ups[k] = pltpu.bitcast(gate(e), F32)
            tiles = [[pair_rows(wkv_r, (g & 1) + _zero(z, m), n1 * DC + kt * 128 + 16 * r, 16, gate)
                      for n1 in range(2)] for kt in range(4)]
            rhs49(wkv, tiles, lambda w, k: w * down[k], m, r)
            return [], 0, lambda: wkv[7 * m, blk(r + _zero(z, 0), 8), :]

        def qw(m, r, gate):
            tiles = [[pair_rows(wq_r, ((g + 1 + n1) & 3) + _zero(z, m), kt * 256 + 16 * r, 16, gate)
                      for n1 in range(2)] for kt in range(4)]
            rhs49(wq49, tiles, lambda w, k: w, m, r)
            return [], 0, lambda: wq49[7 * m, blk(r + _zero(z, 0), 8), :]

        def b_lhs(u, r, gate):
            base = 8 * jnp.minimum(g + 1, NQ - 1) + r
            ops = _words7(_lhs7, [gate(xs_u[u + 4 * d, blk(base + 4 * e, 8), :])
                                  for e in range(2) for d in range(2)])
            for k, m in enumerate(LSUM):
                bx[k, pl.ds(8 * r, 8), strip(u)] = ops[m]
            return [], 0, lambda: bx[0, blk(r + _zero(z, 0), 8), strip(u)]

        return dict(sc=[part(scales, n1) for n1 in range(2)],
                    kv=[part(kv, m, r) for m in range(7) for r in range(8)],
                    qw=[part(qw, m, r) for m in range(7) for r in range(16)],
                    bx=[part(b_lhs, u, r) for u in range(4) for r in range(4)])

    cp_wq(0, sem_p.at[1]).wait()
    for d in cp_p(-1):
        d.wait()
    sched = _Sched(last > 99, _planx(), staging(-1, last))
    w0 = pair_rows(wq_r, 0, 0, M, lambda x: x)
    w0 = [_join(w0[0][h], w0[1][h]) for h in range(2)]
    for g in range(4):
        for e in range(2):
            for h in range(2):
                q = [sched.mm(8 * g + 4 * e + 2 * h + k, jnp.concatenate(
                    [xs_u[4 * k + u, pl.ds((4 * g + 2 + e) * HQ, HQ), :] for u in range(4)], axis=1),
                    w0[h][256 * k:256 * k + 256], step=16) for k in range(2)]
                qn[h, g, e] = _pack((q[0] + q[1]) * QSCALE)
    sched.finish()
    for d in cp_p(1):
        d.start()
    plan2 = _plan2()

    def p2_body(p, carry):
        for d in cp_p(p):
            d.wait()
        causal = col <= row
        never = p > NP
        jobs = staging(p, p)
        sched = _Sched(never, plan2, jobs)
        mm = sched.mm

        r0 = pl.multiple_of(p * TQ, TQ)

        def scatter(dst, off, c):
            for e, t in enumerate(c):
                for cc in range(4):
                    dst[4 * (e & 1) + cc, pl.ds(off + (PAD + (e >> 1) * HQ), HQ), :] = (
                        t[:, cc * 128:(cc + 1) * 128])

        def proj_bv():
            def lhs(m):
                if m in (2, 3):
                    return jnp.concatenate([xs_u[u + 4 * (m - 2), blk(2 * p + m - 2, QQ), :]
                                            for u in range(4)], axis=1)
                return bx[LSUM.index(m)]

            for cc in range(8):
                vb[cc, pl.ds(0, PAD), :] = vb[cc, pl.ds(TQ, PAD), :]
            c = [_combine(lambda m: mm(("bv", 7 * e + ORDER.index(m)), lhs(m), jnp.concatenate(
                [wv7[m, 2 * e], wv7[m, 2 * e + 1]], axis=1))) for e in range(2)]
            scatter(vb, 0, [jnp.concatenate(t, axis=1) for t in zip(*c)])

        def local_qk(rb, k, gate):
            q = [qk_b[cc, pl.ds(r0 + _zero(p, k) + (PAD + rb * RB), RB), :] for cc in range(8)]
            q[0] = gate(q[0])
            for w in range(LG * k, LG * k + LG):
                t = _fold([q[cc] * qk_b[8 + cc, pl.ds(r0 + (PAD + rb * RB - DIL * w), RB), :]
                           for cc in range(8)], jnp.add)
                t = t + pltpu.roll(t, 64, 1)
                t = t + jnp.where(odd, pltpu.roll(t, 1, 1), pltpu.roll(t, 127, 1))
                t = t * (DB ** -0.5 * LOG2E)
                if rb == 0 and w:
                    t = jnp.where(rowi + r0 >= DIL * w, t, NEG)
                lg_s[w, pl.ds(rb * RB, RB), :] = t
            return [], 1, lambda: pltpu.bitcast(lg_s[w, blk(2 * rb + _zero(p, 0), 8), :], U32)

        def local_sm(rb, e, gate):
            rows = pl.ds(rb * RB + SMR * e, SMR)
            lg = [gate(lg_s[w, rows, :]) for w in range(WIN)]
            m = _tree(lg, jnp.maximum)
            ps = [jnp.exp2(t - m) for t in lg]
            l = _tree(ps, jnp.add)
            r = pl.reciprocal(l, approx=True)
            r = r * (2.0 - l * r)
            for w in range(WIN):
                pr_s[w, rows, :] = ps[w] * r
            return [], 2, lambda: pltpu.bitcast(pr_s[0, blk(2 * rb + e + _zero(p, 0), 8), :], U32)

        def local_pv(rb, k, gate):
            rows = pl.ds(rb * RB, RB)
            ps = [pr_s[w + _zero(p, k), rows, :] for w in range(WIN)]
            ps[0] = gate(ps[0])
            o = [_fold([ps[w] * vb[cc, pl.ds(PAD + rb * RB - DIL * w, RB), :] for w in range(WIN)],
                       jnp.add) for cc in (k, k + 4)]
            if rb < NSUB:
                for e in range(2):
                    o_s[k + 4 * e, rows, :] = o[e]
                return [], 3, lambda: pltpu.bitcast(o_s[k, blk(2 * rb + _zero(p, 0), 8), :], U32)
            top = pl.ds((rb - NSUB) * RB, RB)
            for m, t in enumerate(_lhs7(o_s[k, top, :], o_s[k + 4, top, :], *o)):
                ob7[m, pl.ds((rb - NSUB) * RB // 2, RB // 2), strip(k)] = _pack(t)
            return [], 0, lambda: ob7[0, blk(rb - NSUB + _zero(p, 0), 8), strip(k)]

        order = [rb + e * NSUB for rb in range(NSUB) for e in range(2)]
        jobs["lo"] = []
        for k in range(len(order) + 2):
            for f, d, n in ((local_sm, 1, RB // SMR), (local_qk, 0, 8 // LG), (local_pv, 2, 4)):
                if 0 <= k - d < len(order):
                    jobs["lo"] += [part(f, order[k - d], e) for e in range(n)]

        def wob(m):
            if m == 1:
                return wob_p[pl.ds(0, M // 4), pl.ds(0, M // 2)]
            if m == 4:
                return wob_p[pl.ds(M // 4, M // 4), pl.ds(M // 2, M // 2)]
            return wob5[RSUM.index(m)]

        bo = {}

        def proj_bo(n):
            for m in ORDER[len(bo):len(bo) + n]:
                bo[m] = mm(("bo", len(bo)), lambda: ob7[m], wob(m))
            if n and len(bo) == 7:
                scatter(qk_b, r0, _combine(lambda m: bo[m]))

        def out_weights(m, r, gate):
            ww = [[gate(wo_r[(p & 1) + _zero(p, m),
                             pl.ds((2 * (q >> 1) + (e >> 1)) * HQ + 8 * r, 8),
                             pl.ds((2 * (q & 1) + (e & 1)) * 128, 128)])
                   for e in range(4)] for q in range(4)]
            rows = blk(8 * (p >> 1) + r, 8)
            for n, w in enumerate(_words49(_rhs7, ww, m)):
                wo49[7 * m + n, p & 1, rows, :] = w
            return [], 0, lambda: wo49[7 * m + _zero(p, 0), p & 1, rows, :]

        jobs["wo"] = [part(out_weights, m, r) for m in range(7) for r in range(8)]

        ks, vs, qs = {}, {}, {}
        done, prods = {}, {}

        def project(kind, j, n, lhs, rhs, scale):
            got = prods.setdefault((kind, j), {})
            for m in ORDER[len(got):len(got) + n]:
                got[m] = _combine(lambda k: mm((kind, j, 7 * len(got) + ORDER.index(k)),
                                               lhs(7 * m + k), rhs[7 * m + k]))
            if len(got) < 7:
                return None
            c = _combine(lambda m: got[m])
            c = [[_pack(c[(rg & 2) + (cg >> 1)][2 * (rg & 1) + (cg & 1)] * scale(cg))
                  for rg in range(4)] for cg in range(4)]
            return [[jnp.concatenate([t[16 * e:16 * e + 16] for t in c[cg]], axis=0)
                     for e in range(2)] for cg in range(4)]

        def proj_kv(j, n):
            c = project("kv", j, n, lambda k: cq[k, 0, pl.ds(j * QQ, QQ), :], wkv,
                        lambda cg: ups[cg][:1])
            if c is not None:
                for cg in range(4):
                    for e in range(2):
                        (vs, ks)[cg >> 1][(cg & 1, 2 * j + e)] = c[cg][e]

        def proj_q(g, n):
            rows = blk(2 * g + (p & 1), QQ)
            c = project("q", g, n,
                        lambda k: jnp.concatenate([xq[k, sr, rows, :] for sr in range(2)], axis=1),
                        wq49, lambda cg: QSCALE)
            if c is not None:
                for h in range(2):
                    for e in range(2):
                        old = qn[h, g, e]
                        for b in range(2):
                            qs[(h, 4 * g + 2 * b + e)] = jnp.where((p & 1) == b, c[h][e], old)
                        qn[h, g, e] = c[2 + h][e]

        def qk(h, i, dep):
            kk = jnp.concatenate([ks[(h, j)] for j in range(i + 1)], axis=0)
            q = qs[(h, i)]
            if dep is not None:
                q = jnp.where(never, done[(h, dep)], q)
            ch = _lane_chunks(mm(("qk", h, i), q, kk, NT, 512))
            ch[i] = jnp.where(causal, ch[i], NEG)
            return ch

        def softmax_pv(h, i, ch):
            m = jnp.max(_fold(ch, jnp.maximum), axis=1, keepdims=True)
            ps = [jnp.exp2(c - m) for c in ch]
            lp = ps[0]
            for j in range(1, i + 1):
                lp = lp + ps[j]
                if TIE and (j % TIE == TIE - 1 or j == i):
                    ps[j] = jnp.where(never, lp, ps[j])
            pb = jnp.concatenate(ps, axis=1).astype(BF16)
            vv = jnp.concatenate([vs[(h, j)] for j in range(i + 1)], axis=0)
            o = mm(("pv", h, i), pb, vv)
            if i >= LDEP:
                lp = jnp.where(never, o, lp)
            l = jnp.sum(lp, axis=1, keepdims=True)
            r = pl.reciprocal(l, approx=True)
            r = r * (2.0 - l * r)
            cn = _pack(o * r)
            done[(h, i)] = cn
            ctx[2 * p + h, pl.ds(i * HQ, HQ), :] = cn

        proj_bv()
        proj_kv(0, 7)
        proj_q(0, 7)
        for i in range(NQ):
            dep = i - DEP if i >= DEP else None
            s0 = qk(0, i, dep)
            s1 = qk(1, i, dep)
            if i + 2 < NQ:
                proj_kv(i // 2 + 1, 7 if i & 1 else KVS // 7)
                if i < 6:
                    proj_q(i // 2 + 1, 7 if i & 1 else QS // 7)
            else:
                proj_bo(BOP[i + 2 - NQ])
            softmax_pv(0, i, s0)
            softmax_pv(1, i, s1)
        proj_bo(BOP[2])
        sched.finish()
        for d in cp_p(p + 2):
            d.start()
        return carry

    jax.lax.fori_loop(0, NP, p2_body, 0)

    cp_gw().wait()
    gw = gw_ref[...].astype(F32)
    plan3 = _plan3()
    cab = (ca0, ca1)

    def p3_body(i, carry):
        r0 = pl.multiple_of(i * TO, TO)
        h0 = pl.multiple_of(i * (TO // 2), TO // 2)
        never = i > S

        def ctx_words(m, u, r, n):
            return [[ctx[4 * u + 2 * (q & 1) + (e & 1),
                         pl.ds(h0 + _zero(i, m) * 8 + ((2 * (q >> 1) + (e >> 1)) * QQ + r), n), :]
                     for e in range(4)] for q in range(4)]

        def operands(k, u, r, gate):
            m = ORDER[k]
            cw = [[gate(w) for w in q] for q in ctx_words(m, u, r, 8)]
            for n, w in enumerate(_words49(_lhs7, cw, m)):
                if not (m in (2, 3) and n in (2, 3)):
                    cab[k & 1][n, pl.ds(r, 8), pl.ds(u * 128, 128)] = w
            return [], 0, lambda: cab[k & 1][_zero(i, 0), pl.ds(r, 8), pl.ds(u * 128, 128)]

        def gate_rows(r, gate):
            gs = _fold([_bf(gate(xs_u[j, pl.ds(h0 + r, 8), :])).astype(F32) * gw[j:j + 1]
                        for j in range(8)], jnp.add)
            g = jax.nn.sigmoid(jnp.sum(gs, axis=1, keepdims=True))
            g_s[pl.ds(2 * r, 16), :] = jnp.broadcast_to(g, (16, 128))
            return [], 0, lambda: pltpu.bitcast(g_s[blk(r // 4 + _zero(i, 0), 8), :], U32)

        sched = _Sched(never, plan3, dict(
            a=[part(operands, k, u, r) for k in range(1, 7) for u in range(HA // 4)
               for r in range(0, QQ, 8)],
            g=[part(gate_rows, r) for r in range(0, TO // 2, 8)]))
        first = [[_words49(_lhs7, ctx_words(ORDER[0], u, 0, QQ), ORDER[0])[n]
                  for u in range(HA // 4)] for n in range(7)]

        def inner(m, n):
            k = ORDER.index(m)
            res = []
            for e in range(2):
                us = range(4 * e, 4 * e + 4)
                if m in (2, 3) and n in (2, 3):
                    lhs = jnp.concatenate([ctx_words(m, u, 0, QQ)[3 * (m - 2)][3 * (n - 2)]
                                           for u in us], axis=1)
                elif k == 0:
                    lhs = jnp.concatenate([first[n][u] for u in us], axis=1)
                else:
                    lhs = lambda: cab[k & 1][n, :, pl.ds(e * 512, 512)]
                rhs = jnp.concatenate([wo49[7 * m + n, cc, pl.ds(e * 256, 256), :]
                                       for cc in range(2)], axis=1)
                res.append(sched.mm((k, 2 * ORDER.index(n) + e), lhs, rhs))
            return res[0] + res[1]

        acs = _combine(lambda m: _combine(lambda n: inner(m, n)))
        sched.finish()
        for q in range(4):
            for e in range(4):
                off = (2 * (q >> 1) + (e >> 1)) * HQ
                g = g_s[pl.ds(off, HQ), :]
                for cc in range(2):
                    ch = 4 * cc + 2 * (q & 1) + (e & 1)
                    a = acs[q][e][:, cc * 128:(cc + 1) * 128]
                    b = qk_b[ch, pl.ds(r0 + (PAD + off), HQ), :]
                    out_s[pl.ds(r0 + off, HQ), pl.ds(ch * 128, 128)] = (
                        g * a + (1.0 - g) * b).astype(BF16)
        cp_out(i).start()
        return carry

    jax.lax.fori_loop(0, S // TO, p3_body, 0)
    for g in range(NP, NP + 2):
        for d in cp_p(g):
            d.wait()
    for i in range(S // TO):
        cp_out(i).wait()


@jax.jit
def pallas_gated_mix__compressed_kv_cla__sliding_local_dilated__prompt_kernel(
    A_x: jax.Array,
    A_c_kv: jax.Array,
    A_w_q: jax.Array,
    A_w_uk: jax.Array,
    A_w_uv: jax.Array,
    A_w_o: jax.Array,
    B_x: jax.Array,
    B_wqkv: jax.Array,
    B_wo: jax.Array,
    gate_w: jax.Array,
):
    del B_x
    any_spec = pl.BlockSpec(memory_space=pl.ANY)
    out = pl.pallas_call(
        _kernel,
        in_specs=[any_spec] * 9,
        out_specs=any_spec,
        out_shape=jax.ShapeDtypeStruct((S, M), BF16),
        scratch_shapes=[
            pltpu.VMEM((8, S // 2, 128), U32),
            pltpu.VMEM((2, HQ, M), U32),
            pltpu.VMEM((2, HQ, DC), U32),
            pltpu.VMEM((2, 128, M), BF16),
            pltpu.VMEM((2, 2, 32, M), BF16),
            pltpu.VMEM((M // 2, M), U32),
            pltpu.VMEM((2, 2 * DC, 128), U32),
            pltpu.VMEM((4, M, 128), U32),
            pltpu.VMEM((2, 2 * DA, M // 2), U32),
            pltpu.VMEM((8, 64, 128), U32),
            pltpu.VMEM((49, 2, S // 8, 128), U32),
            pltpu.VMEM((49, 1, S // 8, 128), U32),
            pltpu.VMEM((7, 4, M // 4, 128), U32),
            pltpu.VMEM((5, M // 4, M // 2), U32),
            pltpu.VMEM((49, 2, NP * QQ, 128), U32),
            pltpu.VMEM((49, HQ, 128), U32),
            pltpu.VMEM((49, TQ, 128), U32),
            pltpu.VMEM((4, 8, 128), F32),
            pltpu.VMEM((5, QQ, M // 2), U32),
            pltpu.VMEM((2, 4, 2, HQ, 128), U32),
            pltpu.VMEM((16, S + PAD, 128), F32),
            pltpu.VMEM((8, TQ + PAD, 128), F32),
            pltpu.VMEM((WIN, TQ, 128), F32),
            pltpu.VMEM((WIN, TQ, 128), F32),
            pltpu.VMEM((8, HQ, 128), F32),
            pltpu.VMEM((7, QQ, M // 2), U32),
            pltpu.VMEM((HA, S // 2, 128), U32),
            pltpu.VMEM((7, QQ, M), U32),
            pltpu.VMEM((7, QQ, M), U32),
            pltpu.VMEM((TO, 128), F32),
            pltpu.VMEM((S, M), BF16),
            pltpu.VMEM((8, 128), BF16),
            pltpu.SemaphoreType.DMA((2,)),
            pltpu.SemaphoreType.DMA((2,)),
            pltpu.SemaphoreType.DMA((2,)),
        ],
        compiler_params=pltpu.CompilerParams(vmem_limit_bytes=120 * 1024 * 1024,
                                             disable_bounds_checks=True),
    )(
        A_x.reshape(S, M),
        A_c_kv.reshape(S, DC),
        A_w_q,
        A_w_uk,
        A_w_uv,
        A_w_o.reshape(HA * DA, M),
        B_wqkv.reshape(2, M // 2, 3 * M),
        B_wo.reshape(HB // 2, 2, DB, M),
        gate_w.reshape(8, 128),
    )
    return out.reshape(1, S, M)
```

```python
import functools
import math

import jax
import jax.numpy as jnp
import jax.experimental.pallas as pl
import jax.experimental.pallas.tpu as pltpu

F32 = jnp.float32
BF16 = jnp.bfloat16
U32 = jnp.uint32

S = 2048
M = 1024
HA = 32
DA = 128
DC = 512
HB = 32
DB = 32
WIN = 8
DIL = 2
PAD = 16
LOG2E = math.log2(math.e)
NEG = -1e9

TQ = 128
HQ = TQ // 2
QQ = TQ // 4
BOP = (2, 3, 2)
LX = 16
KVS = 28
QS = 28
QST = 2
LQ0 = 3
LG = 2
XN = 29
SK = 3
SMR = 16
P1N = 6
P1U = 2
P3S = 4
P3E = 12
NQ = S // TQ
NP = HA // 2
DEP = 2
LN = 52
SML = 2
LE = 2
LI = 0
LA = 13
LB = 4
LS = 4
LP = ("kv", 0, 24)
FA = 6
F0 = 0
FD = 8
TIE = 4
RB = 16
LDEP = 4
TO = 256
NN = (((1,), (0,)), ((), ()))
NT = (((1,), (1,)), ((), ()))


def _plan2():
    plan = {}

    def put(name, count, start, until):
        plan.setdefault(start, []).extend([(name, until)] * count)

    def after_qk(i):
        if i >= NQ - 2:
            return ("bo", (i - NQ + 2) * BOP[0] + 1)
        return ("kv", i // 2 + 1, KVS * (i & 1) + LX)

    def fill(name, count, sites):
        for start, room, until in sites:
            n = min(count, room - len(plan.get(start, ())))
            put(name, n, start, until)
            count -= n
        assert count == 0, (name, count)

    def qk_sites(lo, hi):
        return [(("qk", h, i), max(i + 1 - h * SK, 0), after_qk(i))
                for i in range(lo, hi) for h in range(2)]

    def q_sites(g, lo, hi, until):
        return [(("q", g, k), 1, until) for k in range(lo, hi, QST)]

    names = _spread(["lo"] * (64 // LG + 128 // SMR), LN)
    for k, name in enumerate(names):
        put(name, 1, ("bv", k // 4) if k < 56 else ("kv", 0, 2 * (k - 56) + 1), LP)
    put("sc", 1, ("kv", 0, 0), ("q", 0, 0))
    put("sc", 1, ("kv", 0, 24), ("q", 0, 8))
    first = [(("kv", 0, k), 1, ("kv", 1, 8)) for k in range(LA, 49, LS)]
    first += [(("q", 0, k), 1, ("kv", 1, 8)) for k in range(LI, 49 - LB, LE)]
    early = []
    for g in range(1, 4):
        early += q_sites(g, 0, QS - 4, after_qk(2 * g - 1))
        early += qk_sites(max(2 * g - 1, LQ0), 2 * g)
        early += q_sites(g, QS, 45, after_qk(2 * g))
        early += qk_sites(max(2 * g, LQ0), 2 * g + 1)
    fill("lv", 32, first + early)
    fill("wo", 56, early)
    fill("bx", 16, early + qk_sites(7, 14))
    fill("qw", 112, qk_sites(7, 14))
    fill("kv", 56, qk_sites(14, 16) + [(("bo", k), 8, ("bo", 6)) for k in range(BOP[0], 5)])
    return plan


def _planx():
    names = _spread(["sc"] * 2 + ["bx"] * 16 + ["qw"] * 112 + ["kv"] * 56, 8 * XN)
    return {k: [(n, 31) for n in names[8 * k:8 * k + 8]] for k in range(XN)}


def _spread(names, ticks):
    out = [None] * ticks
    for k, name in enumerate(names):
        out[k * ticks // len(names)] = name
    return out


def _plan1():
    names = _spread(["x"] * 28 + ["c"] * 14 + ["o"] * 8 + ["v"] * 8, 16 * P1N)
    return {k: [(n, min(k + P1U, 7)) for n in names[16 * k:16 * k + 16]] for k in range(P1N)}


def _plan3():
    plan = {}
    for k in range(6):
        lo = P3S if k == 0 else 0
        extra = ["g"] * 8 if k in (1, 2) else []
        names = _spread(["a"] * 32 + extra, 4 * (P3E - lo))
        for d in range(lo, P3E):
            plan[(k, d)] = [(n, (k + 1, 0)) for n in names[4 * (d - lo):4 * (d - lo) + 4]]
    return plan


_STAGES = ((2, 4), (1, 3), (0, 2), (0, 6), (0, 1))


def _permute8(cols):
    cols = list(cols)
    lane = jax.lax.broadcasted_iota(jnp.int32, cols[0].shape, 1)
    for va, lb in _STAGES:
        lo = (lane & (1 << lb)) == 0
        sh = 1 << lb
        idx = [i for i in range(8) if not (i >> va) & 1]
        if lb == 6:
            rr = [pltpu.roll(jnp.where(lo, cols[i | (1 << va)], cols[i]), 64, 1) for i in idx]
            for i, r in zip(idx, rr):
                a, b = cols[i], cols[i | (1 << va)]
                cols[i] = jnp.where(lo, a, r)
                cols[i | (1 << va)] = jnp.where(lo, r, b)
        else:
            rb = [pltpu.roll(cols[i | (1 << va)], sh, 1) for i in idx]
            ra = [pltpu.roll(cols[i], 128 - sh, 1) for i in idx]
            for i, xa, xb in zip(idx, ra, rb):
                a, b = cols[i], cols[i | (1 << va)]
                cols[i] = jnp.where(lo, a, xb)
                cols[i | (1 << va)] = jnp.where(lo, xa, b)
    return cols


def _pack(x):
    return pltpu.bitcast(x.astype(BF16), U32)


def _bf(x):
    return pltpu.bitcast(x, BF16)


def _split(w):
    return (pltpu.bitcast(w << 16, F32), pltpu.bitcast(w & jnp.uint32(0xFFFF0000), F32))


def _join(lo, hi):
    return pltpu.bitcast(pltpu.pack_elementwise([lo, hi], packed_dtype=BF16), U32)


def _riffle(x):
    return jnp.concatenate([_join(x[r:r + 16], x[r + 16:r + 32]) for r in range(0, x.shape[0], 32)],
                           axis=0)


def _lhs7(a11, a12, a21, a22):
    return [a11 + a22, a21 + a22, a11, a22, a11 + a12, a21 - a11, a12 - a22]


def _rhs7(b11, b12, b21, b22):
    return [b11 + b22, b11, b12 - b22, b21 - b11, b22, b11 + b12, b21 + b22]


LSUM = (0, 1, 4, 5, 6)
RSUM = (0, 2, 3, 5, 6)


def _words7(fn, quads):
    halves = [_split(w) for w in quads]
    lo = fn(*[h[0] for h in halves])
    hi = fn(*[h[1] for h in halves])
    return [_join(a, b) for a, b in zip(lo, hi)]


def _combine(mm):
    add = functools.partial(jax.tree.map, jnp.add)
    sub = functools.partial(jax.tree.map, jnp.subtract)
    m2 = mm(2)
    m3 = mm(3)
    m4 = mm(4)
    c12 = add(m2, m4)
    t11 = sub(m3, m4)
    m1 = mm(1)
    c21 = add(m1, m3)
    t22 = sub(m2, m1)
    m0 = mm(0)
    t11 = add(t11, m0)
    t22 = add(t22, m0)
    c11 = add(t11, mm(6))
    return c11, c12, c21, add(t22, mm(5))


ORDER = (2, 3, 4, 1, 0, 6, 5)


def _zero(i, m):
    return i >> (8 + m)


def _merge(vals):
    return _fold([v[r:r + 8, c:c + 128] for v in vals for r in range(0, v.shape[0], 8)
                  for c in range(0, v.shape[1], 128)], jnp.bitwise_or)


def _gate(never, g):
    def gate(x):
        t = jnp.tile(pltpu.bitcast(g, x.dtype), (x.shape[0] // 8, x.shape[1] // 128))
        return jnp.where(never, t, x)
    return gate


def _tie(never, x, deps):
    if not deps:
        return x
    top = jnp.where(never, _merge(deps), x[:8, :128])
    if x.shape[1] > 128:
        top = jnp.concatenate([top, x[:8, 128:]], axis=1)
    return jnp.concatenate([top, x[8:]], axis=0)


class _Sched:
    def __init__(self, never, plan, jobs):
        self.never, self.plan, self.jobs, self.pending = never, plan, jobs, {}

    def mm(self, site, a, b, dims=NN, width=128, step=32):
        deps = [d() if callable(d) else d for d in self.pending.pop(site, ())]
        a = a() if callable(a) else a
        tie = functools.partial(_tie, self.never, deps=deps)
        a, b = (_bf(tie(a)), _bf(b)) if a.dtype == U32 else (a, _bf(tie(b)))
        out = jax.lax.dot_general(a, b, dims, preferred_element_type=F32)
        per = out.shape[0] // step
        last = {}
        for k, (name, until) in enumerate(self.plan.get(site, ())):
            if name is not None:
                r, c = step * (k % per), width * (k // per)
                vals, tag, stored = self.jobs[name].pop(0)(
                    _gate(self.never, out[r:r + 8, c:c + 128]))
                self.pending.setdefault(until, []).extend(vals)
                last[(name, tag, until)] = stored
        for (_, _, until), stored in last.items():
            if stored is not None:
                self.pending[until].append(stored)
        return out

    def finish(self):
        assert not any(self.jobs.values()) and not any(self.pending.values())


def _ops49(fn, blocks, m):
    return fn(*[fn(*[blocks[q][e] for q in range(4)])[m] for e in range(4)])


def _words49(fn, words, m):
    halves = [[_split(w) for w in q] for q in words]
    lo = _ops49(fn, [[h[0] for h in q] for q in halves], m)
    hi = _ops49(fn, [[h[1] for h in q] for q in halves], m)
    return [_join(a, b) for a, b in zip(lo, hi)]


def _fold(xs, op):
    acc = xs[0]
    for x in xs[1:]:
        acc = op(acc, x)
    return acc


def _tree(xs, op):
    while len(xs) > 1:
        xs = [op(a, b) for a, b in zip(xs[::2], xs[1::2])]
    return xs[0]


def _lane_chunks(x):
    return [x[:, j * 128:(j + 1) * 128] for j in range(x.shape[1] // 128)]


def _kernel(x_hbm, c_hbm, wq_hbm, wuk_hbm, wuv_hbm, wo_hbm, wqkv_hbm, wob_hbm, gw_hbm,
            out_hbm,
            xs_u, x_r, c_r, w_r, wv_r, wob_p, wkv_r, wq_r, wo_r,
            wperm, xq, cq, wv7, wob5, wo49, wkv, wq49, ups, bx, qn,
            qk_b, vb, lg_s, pr_s, o_s, ob7, ctx, ca0, ca1, g_s, out_s, gw_ref,
            sem_x, sem_p, sem_a):
    x_u = x_hbm.bitcast(U32)
    c_u = c_hbm.bitcast(U32)
    wo_u = wo_hbm.bitcast(U32)
    wq_u = wq_hbm.bitcast(U32)
    wuk_u = wuk_hbm.bitcast(U32)
    wuv_u = wuv_hbm.bitcast(U32)
    wob_u = wob_hbm.bitcast(U32)
    part = functools.partial

    def blk(j, n):
        return pl.ds(pl.multiple_of(j * n, n), n)

    def strip(j):
        return blk(j, 128)

    def cp_x(t):
        return pltpu.make_async_copy(x_u.at[:, strip(t >> 1)], xs_u.at[t >> 1], sem_x.at[0])

    def cp_w(t, sem):
        return pltpu.make_async_copy(wqkv_hbm.at[t >> 3, strip((t >> 1) & 3), blk(t & 1, M)],
                                     w_r.at[t & 1], sem)

    def cp_side(t):
        dp = ((t >> 3) << 2) + (t & 2) + ((t >> 2) & 1)
        sem = sem_x.at[t & 1]
        return (
            pltpu.make_async_copy(x_u.at[blk(t, HQ), :], x_r.at[t & 1], sem),
            pltpu.make_async_copy(c_u.at[blk(t, HQ), :], c_r.at[t & 1], sem),
            pltpu.make_async_copy(wqkv_hbm.at[:, blk(t, 32), pl.ds(2 * M, M)], wv_r.at[t & 1], sem),
            pltpu.make_async_copy(wob_u.at[:, t & 1, dp, :], wob_p.at[blk(t, 16), :], sem),
            pltpu.make_async_copy(wob_u.at[:, t & 1, dp + 8, :], wob_p.at[blk(t + 16, 16), :], sem),
        )

    def cp_wq(p, sem):
        return pltpu.make_async_copy(wq_u.at[:, jnp.minimum(p, NP - 1), :], wq_r.at[p & 3], sem)

    def cp_p(g):
        slot = g & 1
        p = jnp.minimum(g + 1, NP - 1)
        o = jnp.clip(g, 0, NP - 1)
        sem = sem_p.at[slot]
        return (
            pltpu.make_async_copy(wo_u.at[blk(o >> 1, 2 * DA), blk(o & 1, M // 2)],
                                  wo_r.at[slot], sem),
            pltpu.make_async_copy(wuk_u.at[:, p, :], wkv_r.at[slot, pl.ds(DC, DC), :], sem),
            pltpu.make_async_copy(wuv_u.at[:, p, :], wkv_r.at[slot, pl.ds(0, DC), :], sem),
            cp_wq(g + 2, sem),
        )

    def cp_gw():
        return pltpu.make_async_copy(gw_hbm, gw_ref, sem_a.at[0])

    def cp_out(i):
        return pltpu.make_async_copy(out_s.at[blk(i, TO), :], out_hbm.at[blk(i, TO), :],
                                     sem_a.at[1])

    def group(t, fn):
        tc = jnp.minimum(t, 15)
        for d in cp_side(tc):
            pl.when(t < 16)(part(fn, d))
        pl.when((t & 17) == 0)(part(fn, cp_x(tc)))
        pl.when(t < 15)(part(fn, cp_w(jnp.minimum(t + 1, 15), sem_x.at[t & 1])))

    cp_w(0, sem_a.at[1]).start()
    cp_x(0).start()
    cp_w(1, sem_x.at[0]).start()
    for d in cp_side(0):
        d.start()

    for cc in range(8):
        qk_b[8 + cc, pl.ds(0, PAD), :] = jnp.zeros((PAD, 128), F32)
        vb[cc, pl.ds(TQ, PAD), :] = jnp.zeros((PAD, 128), F32)

    def stage_first(t):
        for cc, w in enumerate(_permute8(_lane_chunks(pltpu.bitcast(w_r[t & 1], U32)))):
            wperm[cc] = w

    cp_w(0, sem_a.at[1]).wait()
    stage_first(0)
    cp_w(2, sem_x.at[1]).start()
    for d in cp_side(1):
        d.start()
    cp_gw().start()
    plan1 = _plan1()

    def p1_body(t, carry):
        group(t, lambda d: d.wait())

        def act_sums(src, dst, ns, m, sr, r, gate):
            cw = [[gate(src[(t & 1) + _zero(t, m), pl.ds(32 * (q >> 1) + 16 * (e >> 1) + 8 * r, 8),
                            pl.ds(((2 * (q & 1) + (e & 1)) * ns + sr) * 128, 128)])
                   for e in range(4)] for q in range(4)]
            for n, w in enumerate(_words49(_lhs7, cw, m)):
                dst[7 * m + n, sr, blk(2 * t + r, 8), :] = w
            return [], 0, lambda: dst[7 * m + _zero(t, 0), sr, blk(2 * t + r, 8), :]

        wv = _permute8(_lane_chunks(jnp.concatenate(
            [pltpu.bitcast(wv_r[t & 1, e], U32) for e in range(2)], axis=0)))

        def v_sums(r, cc, gate):
            ops = _words7(_rhs7, [gate(wv[cc + 4 * d][16 * e + 8 * r:16 * e + 8 * r + 8])
                                  for e in range(2) for d in range(2)])
            for m in range(7):
                wv7[m, cc, blk(2 * t + r, 8), :] = ops[m]
            return [], 0, lambda: wv7[_zero(t, 0), cc, blk(2 * t + r, 8), :]

        def o_sums(r, cc, gate):
            ops = _words7(_rhs7, [gate(wob_p[blk(2 * t + r + 32 * e, 8), strip(cc + 4 * d)])
                                  for e in range(2) for d in range(2)])
            for e, m in enumerate(RSUM):
                wob5[e, blk(2 * t + r, 8), strip(cc)] = ops[m]
            return [], 0, lambda: wob5[_zero(t, 0), blk(2 * t + r, 8), strip(cc)]

        sched = _Sched(t > 99, plan1, dict(
            x=[part(act_sums, x_r, xq, 2, m, sr, r)
               for m in range(7) for sr in range(2) for r in range(2)],
            c=[part(act_sums, c_r, cq, 1, m, 0, r) for m in range(7) for r in range(2)],
            v=[part(v_sums, r, cc) for r in range(2) for cc in range(4)],
            o=[part(o_sums, r, cc) for r in range(2) for cc in range(4)]))

        first = t < 2
        for half in range(2):
            for rb in range(4):
                w = jnp.concatenate([wperm[4 * half + cc] for cc in range(4)], axis=1)
                r = sched.mm(4 * half + rb, xs_u[t >> 1, pl.ds(rb * 256, 256), :], w)
                for cc in range(4):
                    sl = (8 * (t & 1) + 4 * half + cc, pl.ds(PAD + rb * 512, 512), slice(None))
                    old = jnp.where(first, 0.0, qk_b[sl])
                    qk_b[sl] = old + r[:, cc * 128:(cc + 1) * 128]
        sched.finish()
        stage_first(jnp.minimum(t + 1, 15))

        group(t + 2, lambda d: d.start())

        @pl.when(jnp.logical_and(t >= 7, t < 9))
        def _():
            for d in cp_p(t - 8):
                d.start()

        @pl.when(t == 6)
        def _():
            cp_wq(0, sem_p.at[1]).start()

        return t

    last = jax.lax.fori_loop(0, 16, p1_body, 0)

    row = jax.lax.broadcasted_iota(jnp.int32, (TQ, TQ), 0)
    col = jax.lax.broadcasted_iota(jnp.int32, (TQ, TQ), 1)
    col = (col & ~31) | ((col & 1) << 4) | ((col & 31) >> 1)
    rowi = jax.lax.broadcasted_iota(jnp.int32, (RB, 128), 0)
    odd = (jax.lax.broadcasted_iota(jnp.int32, (RB, 128), 1) & 1) == 1
    NSUB = HQ // RB
    QSCALE = DA ** -0.5 * LOG2E

    def pair_rows(src, slot, r0, n, gate):
        return [_split(gate(src[slot, pl.ds(r0 + par, n // 2, stride=2), :])) for par in range(2)]

    def staging(g, z):
        up, down = {}, {}

        def scales(n1, gate):
            w = pltpu.bitcast(wkv_r[g & 1, pl.ds(n1 * DC, DC), :], jnp.int32)
            rows = [gate(w[:8])] + [w[r:r + 8] for r in range(8, DC, 8)]
            for h in range(2):
                e = _fold([t & (0x7F80 << (16 * h)) for t in rows], jnp.maximum) << (16 - 16 * h)
                e = jnp.max(pltpu.bitcast(e, F32), axis=0, keepdims=True)
                e = jnp.clip(pltpu.bitcast(e, jnp.int32), 1 << 23, 253 << 23)
                e = jnp.broadcast_to(e, (8, 128))
                up[2 * n1 + h] = e
                down[2 * n1 + h] = pltpu.bitcast((254 << 23) - e, F32)
            return [pltpu.bitcast(up[2 * n1] | up[2 * n1 + 1], U32)], 0, None

        def rhs49(dst, tiles, scale, m, r):
            res = [_ops49(_rhs7,
                          [[scale(tiles[2 * (q >> 1) + (e >> 1)][q & 1][par][e & 1],
                                  2 * (q & 1) + (e & 1)) for e in range(4)] for q in range(4)],
                          m) for par in range(2)]
            for k, (lo, hi) in enumerate(zip(*res)):
                dst[7 * m + k, pl.ds(8 * r, 8), :] = _join(lo, hi)

        def kv(m, r, gate):
            while up:
                k, e = up.popitem()
                ups[k] = pltpu.bitcast(gate(e), F32)
            tiles = [[pair_rows(wkv_r, (g & 1) + _zero(z, m), n1 * DC + kt * 128 + 16 * r, 16, gate)
                      for n1 in range(2)] for kt in range(4)]
            rhs49(wkv, tiles, lambda w, k: w * down[k], m, r)
            return [], 0, lambda: wkv[7 * m, blk(r + _zero(z, 0), 8), :]

        def qw(m, r, gate):
            tiles = [[pair_rows(wq_r, ((g + 1 + n1) & 3) + _zero(z, m), kt * 256 + 16 * r, 16, gate)
                      for n1 in range(2)] for kt in range(4)]
            rhs49(wq49, tiles, lambda w, k: w, m, r)
            return [], 0, lambda: wq49[7 * m, blk(r + _zero(z, 0), 8), :]

        def b_lhs(u, r, gate):
            base = 8 * jnp.minimum(g + 1, NQ - 1) + r
            ops = _words7(_lhs7, [gate(xs_u[u + 4 * d, blk(base + 4 * e, 8), :])
                                  for e in range(2) for d in range(2)])
            for k, m in enumerate(LSUM):
                bx[k, pl.ds(8 * r, 8), strip(u)] = ops[m]
            return [], 0, lambda: bx[0, blk(r + _zero(z, 0), 8), strip(u)]

        return dict(sc=[part(scales, n1) for n1 in range(2)],
                    kv=[part(kv, m, r) for m in range(7) for r in range(8)],
                    qw=[part(qw, m, r) for m in range(7) for r in range(16)],
                    bx=[part(b_lhs, u, r) for u in range(4) for r in range(4)])

    cp_wq(0, sem_p.at[1]).wait()
    for d in cp_p(-1):
        d.wait()
    sched = _Sched(last > 99, _planx(), staging(-1, last))
    w0 = pair_rows(wq_r, 0, 0, M, lambda x: x)
    w0 = [_join(w0[0][h], w0[1][h]) for h in range(2)]
    for g in range(4):
        for e in range(2):
            for h in range(2):
                q = [sched.mm(8 * g + 4 * e + 2 * h + k, jnp.concatenate(
                    [xs_u[4 * k + u, pl.ds((4 * g + 2 + e) * HQ, HQ), :] for u in range(4)], axis=1),
                    w0[h][256 * k:256 * k + 256], step=16) for k in range(2)]
                qn[h, g, e] = _pack((q[0] + q[1]) * QSCALE)
    sched.finish()
    for d in cp_p(1):
        d.start()
    plan2 = _plan2()

    def p2_body(p, carry):
        for d in cp_p(p):
            d.wait()
        causal = col <= row
        never = p > NP
        jobs = staging(p, p)
        sched = _Sched(never, plan2, jobs)
        mm = sched.mm

        r0 = pl.multiple_of(p * TQ, TQ)

        def scatter(dst, off, c):
            for e, t in enumerate(c):
                for cc in range(4):
                    dst[4 * (e & 1) + cc, pl.ds(off + (PAD + (e >> 1) * HQ), HQ), :] = (
                        t[:, cc * 128:(cc + 1) * 128])

        def proj_bv():
            def lhs(m):
                if m in (2, 3):
                    return jnp.concatenate([xs_u[u + 4 * (m - 2), blk(2 * p + m - 2, QQ), :]
                                            for u in range(4)], axis=1)
                return bx[LSUM.index(m)]

            for cc in range(8):
                vb[cc, pl.ds(0, PAD), :] = vb[cc, pl.ds(TQ, PAD), :]
            c = [_combine(lambda m: mm(("bv", 7 * e + ORDER.index(m)), lhs(m), jnp.concatenate(
                [wv7[m, 2 * e], wv7[m, 2 * e + 1]], axis=1))) for e in range(2)]
            scatter(vb, 0, [jnp.concatenate(t, axis=1) for t in zip(*c)])

        def local_qk(rb, k, gate):
            q = [qk_b[cc, pl.ds(r0 + _zero(p, k) + (PAD + rb * RB), RB), :] for cc in range(8)]
            q[0] = gate(q[0])
            for w in range(LG * k, LG * k + LG):
                t = _fold([q[cc] * qk_b[8 + cc, pl.ds(r0 + (PAD + rb * RB - DIL * w), RB), :]
                           for cc in range(8)], jnp.add)
                t = t + pltpu.roll(t, 64, 1)
                t = t + jnp.where(odd, pltpu.roll(t, 1, 1), pltpu.roll(t, 127, 1))
                t = t * (DB ** -0.5 * LOG2E)
                if rb == 0 and w:
                    t = jnp.where(rowi + r0 >= DIL * w, t, NEG)
                lg_s[w, pl.ds(rb * RB, RB), :] = t
            return [], 1, lambda: pltpu.bitcast(lg_s[w, blk(2 * rb + _zero(p, 0), 8), :], U32)

        def local_sm(rb, e, gate):
            rows = pl.ds(rb * RB + SMR * e, SMR)
            lg = [gate(lg_s[w, rows, :]) for w in range(WIN)]
            m = _tree(lg, jnp.maximum)
            ps = [jnp.exp2(t - m) for t in lg]
            l = _tree(ps, jnp.add)
            r = pl.reciprocal(l, approx=True)
            r = r * (2.0 - l * r)
            for w in range(WIN):
                pr_s[w, rows, :] = ps[w] * r
            return [], 2, lambda: pltpu.bitcast(pr_s[0, blk(2 * rb + e + _zero(p, 0), 8), :], U32)

        def local_pv(rb, k, gate):
            rows = pl.ds(rb * RB, RB)
            ps = [pr_s[w + _zero(p, k), rows, :] for w in range(WIN)]
            ps[0] = gate(ps[0])
            o = [_fold([ps[w] * vb[cc, pl.ds(PAD + rb * RB - DIL * w, RB), :] for w in range(WIN)],
                       jnp.add) for cc in (k, k + 4)]
            if rb < NSUB:
                for e in range(2):
                    o_s[k + 4 * e, rows, :] = o[e]
                return [], 3, lambda: pltpu.bitcast(o_s[k, blk(2 * rb + _zero(p, 0), 8), :], U32)
            top = pl.ds((rb - NSUB) * RB, RB)
            for m, t in enumerate(_lhs7(o_s[k, top, :], o_s[k + 4, top, :], *o)):
                ob7[m, pl.ds((rb - NSUB) * RB // 2, RB // 2), strip(k)] = _pack(t)
            return [], 0, lambda: ob7[0, blk(rb - NSUB + _zero(p, 0), 8), strip(k)]

        order = [rb + e * NSUB for rb in range(NSUB) for e in range(2)]
        jobs["lo"] = []
        for k in range(len(order) + SML):
            for f, d, n in ((local_sm, SML, RB // SMR), (local_qk, 0, 8 // LG)):
                if 0 <= k - d < len(order):
                    jobs["lo"] += [part(f, order[k - d], e) for e in range(n)]
        jobs["lv"] = [part(local_pv, rb, e) for rb in order for e in range(4)]

        def wob(m):
            if m == 1:
                return wob_p[pl.ds(0, M // 4), pl.ds(0, M // 2)]
            if m == 4:
                return wob_p[pl.ds(M // 4, M // 4), pl.ds(M // 2, M // 2)]
            return wob5[RSUM.index(m)]

        bo = {}

        def proj_bo(n):
            for m in ORDER[len(bo):len(bo) + n]:
                bo[m] = mm(("bo", len(bo)), lambda: ob7[m], wob(m))
            if n and len(bo) == 7:
                scatter(qk_b, r0, _combine(lambda m: bo[m]))

        def out_weights(m, r, gate):
            ww = [[gate(wo_r[(p & 1) + _zero(p, m),
                             pl.ds((2 * (q >> 1) + (e >> 1)) * HQ + 8 * r, 8),
                             pl.ds((2 * (q & 1) + (e & 1)) * 128, 128)])
                   for e in range(4)] for q in range(4)]
            rows = blk(8 * (p >> 1) + r, 8)
            for n, w in enumerate(_words49(_rhs7, ww, m)):
                wo49[7 * m + n, p & 1, rows, :] = w
            return [], 0, lambda: wo49[7 * m + _zero(p, 0), p & 1, rows, :]

        jobs["wo"] = [part(out_weights, m, r) for m in range(7) for r in range(8)]

        ks, vs, qs = {}, {}, {}
        done, prods = {}, {}

        def project(kind, j, n, lhs, rhs, scale, pack):
            got = prods.setdefault((kind, j), {})
            for m in ORDER[len(got):len(got) + n]:
                got[m] = _combine(lambda k: mm((kind, j, 7 * len(got) + ORDER.index(k)),
                                               lhs(7 * m + k), rhs[7 * m + k]))
            if len(got) < 7:
                return None
            c = _combine(lambda m: got[m])
            c = [[pack(c[(rg & 2) + (cg >> 1)][2 * (rg & 1) + (cg & 1)] * scale(cg))
                  for rg in range(4)] for cg in range(4)]
            return [[jnp.concatenate([t[16 * e:16 * e + 16] for t in c[cg]], axis=0)
                     for e in range(2)] for cg in range(4)]

        def proj_kv(j, n):
            c = project("kv", j, n, lambda k: cq[k, 0, pl.ds(j * QQ, QQ), :], wkv,
                        lambda cg: ups[cg][:1], _riffle)
            if c is not None:
                for cg in range(4):
                    for e in range(2):
                        (vs, ks)[cg >> 1][(cg & 1, 2 * j + e)] = c[cg][e]

        def proj_q(g, n):
            rows = blk(2 * g + (p & 1), QQ)
            c = project("q", g, n,
                        lambda k: jnp.concatenate([xq[k, sr, rows, :] for sr in range(2)], axis=1),
                        wq49, lambda cg: QSCALE, _pack)
            if c is not None:
                for h in range(2):
                    for e in range(2):
                        old = qn[h, g, e]
                        for b in range(2):
                            qs[(h, 4 * g + 2 * b + e)] = jnp.where((p & 1) == b, c[h][e], old)
                        qn[h, g, e] = c[2 + h][e]

        def qk(h, i, dep):
            kk = jnp.concatenate([ks[(h, j)] for j in range(i + 1)], axis=0)
            q = qs[(h, i)]
            if dep is not None:
                q = jnp.where(never, done[(h, dep)], q)
            ch = _lane_chunks(mm(("qk", h, i), q, kk, NT, 512))
            ch[i] = jnp.where(causal, ch[i], NEG)
            return ch

        def softmax_pv(h, i, ch):
            m = jnp.max(_fold(ch, jnp.maximum), axis=1, keepdims=True)
            ps = [jnp.exp2(c - m) for c in ch]
            lp = ps[0]
            for j in range(1, i + 1):
                lp = lp + ps[j]
                if TIE and (j % TIE == TIE - 1 or j == i):
                    ps[j] = jnp.where(never, lp, ps[j])
            pb = jnp.concatenate(ps, axis=1).astype(BF16)
            vv = jnp.concatenate([vs[(h, j)] for j in range(i + 1)], axis=0)
            o = mm(("pv", h, i), pb, vv)
            if i >= LDEP:
                lp = jnp.where(never, o, lp)
            l = jnp.sum(lp, axis=1, keepdims=True)
            r = pl.reciprocal(l, approx=True)
            r = r * (2.0 - l * r)
            cn = _pack(o * r)
            done[(h, i)] = cn
            if FA <= i < NQ - 1:
                if h == 0 and F0 < 0:
                    site = ("qk", 1, i + 1)
                elif i + 3 < NQ:
                    site = ("kv", (i + 1) // 2 + 1, KVS * ((i + 1) & 1) + (F0, FD)[h])
                else:
                    site = ("bo", (i + 3 - NQ) * BOP[0] + h)
                sched.pending.setdefault(site, []).append(cn)
            ctx[2 * p + h, pl.ds(i * HQ, HQ), :] = cn

        proj_bv()
        proj_kv(0, 7)
        proj_q(0, 7)
        for i in range(NQ):
            dep = i - DEP if DEP <= i < FA + DEP else None
            s0 = qk(0, i, dep)
            s1 = qk(1, i, dep)
            if i + 2 < NQ:
                proj_kv(i // 2 + 1, 7 if i & 1 else KVS // 7)
                if i < 6:
                    proj_q(i // 2 + 1, 7 if i & 1 else QS // 7)
            else:
                proj_bo(BOP[i + 2 - NQ])
            softmax_pv(0, i, s0)
            softmax_pv(1, i, s1)
        proj_bo(BOP[2])
        sched.finish()
        for d in cp_p(p + 2):
            d.start()
        return carry

    jax.lax.fori_loop(0, NP, p2_body, 0)

    cp_gw().wait()
    gw = gw_ref[...].astype(F32)
    plan3 = _plan3()
    cab = (ca0, ca1)

    def p3_body(i, carry):
        r0 = pl.multiple_of(i * TO, TO)
        h0 = pl.multiple_of(i * (TO // 2), TO // 2)
        never = i > S

        def ctx_words(m, u, r, n):
            return [[ctx[4 * u + 2 * (q & 1) + (e & 1),
                         pl.ds(h0 + _zero(i, m) * 8 + ((2 * (q >> 1) + (e >> 1)) * QQ + r), n), :]
                     for e in range(4)] for q in range(4)]

        def operands(k, u, r, gate):
            m = ORDER[k]
            cw = [[gate(w) for w in q] for q in ctx_words(m, u, r, 8)]
            for n, w in enumerate(_words49(_lhs7, cw, m)):
                if not (m in (2, 3) and n in (2, 3)):
                    cab[k & 1][n, pl.ds(r, 8), pl.ds(u * 128, 128)] = w
            return [], 0, lambda: cab[k & 1][_zero(i, 0), pl.ds(r, 8), pl.ds(u * 128, 128)]

        def gate_rows(r, gate):
            gs = _fold([_bf(gate(xs_u[j, pl.ds(h0 + r, 8), :])).astype(F32) * gw[j:j + 1]
                        for j in range(8)], jnp.add)
            g = jax.nn.sigmoid(jnp.sum(gs, axis=1, keepdims=True))
            g_s[pl.ds(2 * r, 16), :] = jnp.broadcast_to(g, (16, 128))
            return [], 0, lambda: pltpu.bitcast(g_s[blk(r // 4 + _zero(i, 0), 8), :], U32)

        sched = _Sched(never, plan3, dict(
            a=[part(operands, k, u, r) for k in range(1, 7) for u in range(HA // 4)
               for r in range(0, QQ, 8)],
            g=[part(gate_rows, r) for r in range(0, TO // 2, 8)]))
        first = [[_words49(_lhs7, ctx_words(ORDER[0], u, 0, QQ), ORDER[0])[n]
                  for u in range(HA // 4)] for n in range(7)]

        def inner(m, n):
            k = ORDER.index(m)
            res = []
            for e in range(2):
                us = range(4 * e, 4 * e + 4)
                if m in (2, 3) and n in (2, 3):
                    lhs = jnp.concatenate([ctx_words(m, u, 0, QQ)[3 * (m - 2)][3 * (n - 2)]
                                           for u in us], axis=1)
                elif k == 0:
                    lhs = jnp.concatenate([first[n][u] for u in us], axis=1)
                else:
                    lhs = lambda: cab[k & 1][n, :, pl.ds(e * 512, 512)]
                rhs = jnp.concatenate([wo49[7 * m + n, cc, pl.ds(e * 256, 256), :]
                                       for cc in range(2)], axis=1)
                res.append(sched.mm((k, 2 * ORDER.index(n) + e), lhs, rhs))
            return res[0] + res[1]

        acs = _combine(lambda m: _combine(lambda n: inner(m, n)))
        sched.finish()
        for q in range(4):
            for e in range(4):
                off = (2 * (q >> 1) + (e >> 1)) * HQ
                g = g_s[pl.ds(off, HQ), :]
                for cc in range(2):
                    ch = 4 * cc + 2 * (q & 1) + (e & 1)
                    a = acs[q][e][:, cc * 128:(cc + 1) * 128]
                    b = qk_b[ch, pl.ds(r0 + (PAD + off), HQ), :]
                    out_s[pl.ds(r0 + off, HQ), pl.ds(ch * 128, 128)] = (
                        g * a + (1.0 - g) * b).astype(BF16)
        cp_out(i).start()
        return carry

    jax.lax.fori_loop(0, S // TO, p3_body, 0)
    for g in range(NP, NP + 2):
        for d in cp_p(g):
            d.wait()
    for i in range(S // TO):
        cp_out(i).wait()


@jax.jit
def pallas_gated_mix__compressed_kv_cla__sliding_local_dilated__prompt_kernel(
    A_x: jax.Array,
    A_c_kv: jax.Array,
    A_w_q: jax.Array,
    A_w_uk: jax.Array,
    A_w_uv: jax.Array,
    A_w_o: jax.Array,
    B_x: jax.Array,
    B_wqkv: jax.Array,
    B_wo: jax.Array,
    gate_w: jax.Array,
):
    del B_x
    any_spec = pl.BlockSpec(memory_space=pl.ANY)
    out = pl.pallas_call(
        _kernel,
        in_specs=[any_spec] * 9,
        out_specs=any_spec,
        out_shape=jax.ShapeDtypeStruct((S, M), BF16),
        scratch_shapes=[
            pltpu.VMEM((8, S // 2, 128), U32),
            pltpu.VMEM((2, HQ, M), U32),
            pltpu.VMEM((2, HQ, DC), U32),
            pltpu.VMEM((2, 128, M), BF16),
            pltpu.VMEM((2, 2, 32, M), BF16),
            pltpu.VMEM((M // 2, M), U32),
            pltpu.VMEM((2, 2 * DC, 128), U32),
            pltpu.VMEM((4, M, 128), U32),
            pltpu.VMEM((2, 2 * DA, M // 2), U32),
            pltpu.VMEM((8, 64, 128), U32),
            pltpu.VMEM((49, 2, S // 8, 128), U32),
            pltpu.VMEM((49, 1, S // 8, 128), U32),
            pltpu.VMEM((7, 4, M // 4, 128), U32),
            pltpu.VMEM((5, M // 4, M // 2), U32),
            pltpu.VMEM((49, 2, NP * QQ, 128), U32),
            pltpu.VMEM((49, HQ, 128), U32),
            pltpu.VMEM((49, TQ, 128), U32),
            pltpu.VMEM((4, 8, 128), F32),
            pltpu.VMEM((5, QQ, M // 2), U32),
            pltpu.VMEM((2, 4, 2, HQ, 128), U32),
            pltpu.VMEM((16, S + PAD, 128), F32),
            pltpu.VMEM((8, TQ + PAD, 128), F32),
            pltpu.VMEM((WIN, TQ, 128), F32),
            pltpu.VMEM((WIN, TQ, 128), F32),
            pltpu.VMEM((8, HQ, 128), F32),
            pltpu.VMEM((7, QQ, M // 2), U32),
            pltpu.VMEM((HA, S // 2, 128), U32),
            pltpu.VMEM((7, QQ, M), U32),
            pltpu.VMEM((7, QQ, M), U32),
            pltpu.VMEM((TO, 128), F32),
            pltpu.VMEM((S, M), BF16),
            pltpu.VMEM((8, 128), BF16),
            pltpu.SemaphoreType.DMA((2,)),
            pltpu.SemaphoreType.DMA((2,)),
            pltpu.SemaphoreType.DMA((2,)),
        ],
        compiler_params=pltpu.CompilerParams(vmem_limit_bytes=120 * 1024 * 1024,
                                             disable_bounds_checks=True),
    )(
        A_x.reshape(S, M),
        A_c_kv.reshape(S, DC),
        A_w_q,
        A_w_uk,
        A_w_uv,
        A_w_o.reshape(HA * DA, M),
        B_wqkv.reshape(2, M // 2, 3 * M),
        B_wo.reshape(HB // 2, 2, DB, M),
        gate_w.reshape(8, 128),
    )
    return out.reshape(1, S, M)
```

```python
import functools
import math

import jax
import jax.numpy as jnp
import jax.experimental.pallas as pl
import jax.experimental.pallas.tpu as pltpu

F32 = jnp.float32
BF16 = jnp.bfloat16
U32 = jnp.uint32

S = 2048
M = 1024
HA = 32
DA = 128
DC = 512
HB = 32
DB = 32
WIN = 8
DIL = 2
PAD = 16
LOG2E = math.log2(math.e)
NEG = -1e9

TQ = 128
HQ = TQ // 2
QQ = TQ // 4
BOP = (2, 3, 2)
LX = 16
KVS = 28
QS = 28
QST = 2
LQ0 = 3
LG = 2
XN = 29
SK = 3
SMR = 16
P1N = 6
P1U = 2
P3S = 4
P3E = 12
NQ = S // TQ
NP = HA // 2
DEP = 2
SCR = 32
LN = 62
SML = 2
LE = 2
LI = 0
LA = 29
LB = 4
LS = 4
LP = ("kv", 0, 44)
FA = 6
F0 = 0
FD = 8
TIE = 4
RB = 16
LDEP = 4
TO = 256
NN = (((1,), (0,)), ((), ()))
NT = (((1,), (1,)), ((), ()))


def _plan2():
    plan = {}

    def put(name, count, start, until):
        plan.setdefault(start, []).extend([(name, until)] * count)

    def after_qk(i):
        if i >= NQ - 2:
            return ("bo", (i - NQ + 2) * BOP[0] + 1)
        return ("kv", i // 2 + 1, KVS * (i & 1) + LX)

    def fill(name, count, sites):
        for start, room, until in sites:
            n = min(count, room - len(plan.get(start, ())))
            put(name, n, start, until)
            count -= n
        assert count == 0, (name, count)

    def qk_sites(lo, hi):
        return [(("qk", h, i), max(i + 1 - h * SK, 0), after_qk(i))
                for i in range(lo, hi) for h in range(2)]

    def q_sites(g, lo, hi, until):
        return [(("q", g, k), 1, until) for k in range(lo, hi, QST)]

    names = _spread(["lo"] * (64 // LG + 128 // SMR), LN)
    for k, name in enumerate(names):
        put(name, 1, ("bv", k // 4) if k < 56 else ("kv", 0, 2 * (k - 56) + 1), LP)
    first = [(("kv", 0, k), 1, ("kv", 1, 8)) for k in range(LA, 49, LS)]
    first += [(("q", 0, k), 1, ("kv", 1, 8)) for k in range(LI, 49 - LB, LE)]
    early = []
    for g in range(1, 4):
        early += q_sites(g, 0, QS - 4, after_qk(2 * g - 1))
        early += qk_sites(max(2 * g - 1, LQ0), 2 * g)
        early += q_sites(g, QS, 45, after_qk(2 * g))
        early += qk_sites(max(2 * g, LQ0), 2 * g + 1)
    fill("lv", 32, first + early)
    fill("wo", 56, early)
    fill("bx", 16, early + qk_sites(7, 14))
    fill("qw", 112, qk_sites(7, 14))
    fill("kv", 56, qk_sites(14, 16) + [(("bo", k), 8, ("bo", 6)) for k in range(BOP[0], 5)])
    return plan


def _planx():
    names = _spread(["sc"] * (2 * DC // SCR + 2) + ["bx"] * 16 + ["qw"] * 112 + ["kv"] * 56, 8 * XN)
    return {k: [(n, 31) for n in names[8 * k:8 * k + 8]] for k in range(XN)}


def _spread(names, ticks):
    out = [None] * ticks
    for k, name in enumerate(names):
        out[k * ticks // len(names)] = name
    return out


def _plan1():
    names = _spread(["x"] * 28 + ["c"] * 14 + ["o"] * 8 + ["v"] * 8, 16 * P1N)
    return {k: [(n, min(k + P1U, 7)) for n in names[16 * k:16 * k + 16]] for k in range(P1N)}


def _plan3():
    plan = {}
    for k in range(6):
        lo = P3S if k == 0 else 0
        extra = ["g"] * 8 if k in (1, 2) else []
        names = _spread(["a"] * 32 + extra, 4 * (P3E - lo))
        for d in range(lo, P3E):
            plan[(k, d)] = [(n, (k + 1, 0)) for n in names[4 * (d - lo):4 * (d - lo) + 4]]
    return plan


_STAGES = ((2, 4), (1, 3), (0, 2), (0, 6), (0, 1))


def _permute8(cols):
    cols = list(cols)
    lane = jax.lax.broadcasted_iota(jnp.int32, cols[0].shape, 1)
    for va, lb in _STAGES:
        lo = (lane & (1 << lb)) == 0
        sh = 1 << lb
        idx = [i for i in range(8) if not (i >> va) & 1]
        if lb == 6:
            rr = [pltpu.roll(jnp.where(lo, cols[i | (1 << va)], cols[i]), 64, 1) for i in idx]
            for i, r in zip(idx, rr):
                a, b = cols[i], cols[i | (1 << va)]
                cols[i] = jnp.where(lo, a, r)
                cols[i | (1 << va)] = jnp.where(lo, r, b)
        else:
            rb = [pltpu.roll(cols[i | (1 << va)], sh, 1) for i in idx]
            ra = [pltpu.roll(cols[i], 128 - sh, 1) for i in idx]
            for i, xa, xb in zip(idx, ra, rb):
                a, b = cols[i], cols[i | (1 << va)]
                cols[i] = jnp.where(lo, a, xb)
                cols[i | (1 << va)] = jnp.where(lo, xa, b)
    return cols


def _pack(x):
    return pltpu.bitcast(x.astype(BF16), U32)


def _bf(x):
    return pltpu.bitcast(x, BF16)


def _split(w):
    return (pltpu.bitcast(w << 16, F32), pltpu.bitcast(w & jnp.uint32(0xFFFF0000), F32))


def _join(lo, hi):
    return pltpu.bitcast(pltpu.pack_elementwise([lo, hi], packed_dtype=BF16), U32)


def _riffle(x):
    return jnp.concatenate([_join(x[r:r + 16], x[r + 16:r + 32]) for r in range(0, x.shape[0], 32)],
                           axis=0)


def _lhs7(a11, a12, a21, a22):
    return [a11 + a22, a21 + a22, a11, a22, a11 + a12, a21 - a11, a12 - a22]


def _rhs7(b11, b12, b21, b22):
    return [b11 + b22, b11, b12 - b22, b21 - b11, b22, b11 + b12, b21 + b22]


LSUM = (0, 1, 4, 5, 6)
RSUM = (0, 2, 3, 5, 6)


def _words7(fn, quads):
    halves = [_split(w) for w in quads]
    lo = fn(*[h[0] for h in halves])
    hi = fn(*[h[1] for h in halves])
    return [_join(a, b) for a, b in zip(lo, hi)]


def _combine(mm):
    add = functools.partial(jax.tree.map, jnp.add)
    sub = functools.partial(jax.tree.map, jnp.subtract)
    m2 = mm(2)
    m3 = mm(3)
    m4 = mm(4)
    c12 = add(m2, m4)
    t11 = sub(m3, m4)
    m1 = mm(1)
    c21 = add(m1, m3)
    t22 = sub(m2, m1)
    m0 = mm(0)
    t11 = add(t11, m0)
    t22 = add(t22, m0)
    c11 = add(t11, mm(6))
    return c11, c12, c21, add(t22, mm(5))


ORDER = (2, 3, 4, 1, 0, 6, 5)


def _zero(i, m):
    return i >> (8 + m)


def _merge(vals):
    return _fold([v[r:r + 8, c:c + 128] for v in vals for r in range(0, v.shape[0], 8)
                  for c in range(0, v.shape[1], 128)], jnp.bitwise_or)


def _gate(never, g):
    def gate(x):
        t = jnp.tile(pltpu.bitcast(g, x.dtype), (x.shape[0] // 8, x.shape[1] // 128))
        return jnp.where(never, t, x)
    return gate


def _tie(never, x, deps):
    if not deps:
        return x
    top = jnp.where(never, _merge(deps), x[:8, :128])
    if x.shape[1] > 128:
        top = jnp.concatenate([top, x[:8, 128:]], axis=1)
    return jnp.concatenate([top, x[8:]], axis=0)


class _Sched:
    def __init__(self, never, plan, jobs):
        self.never, self.plan, self.jobs, self.pending = never, plan, jobs, {}

    def mm(self, site, a, b, dims=NN, width=128, step=32):
        deps = [d() if callable(d) else d for d in self.pending.pop(site, ())]
        a = a() if callable(a) else a
        tie = functools.partial(_tie, self.never, deps=deps)
        a, b = (_bf(tie(a)), _bf(b)) if a.dtype == U32 else (a, _bf(tie(b)))
        out = jax.lax.dot_general(a, b, dims, preferred_element_type=F32)
        per = out.shape[0] // step
        last = {}
        for k, (name, until) in enumerate(self.plan.get(site, ())):
            if name is not None:
                r, c = step * (k % per), width * (k // per)
                vals, tag, stored = self.jobs[name].pop(0)(
                    _gate(self.never, out[r:r + 8, c:c + 128]))
                self.pending.setdefault(until, []).extend(vals)
                last[(name, tag, until)] = stored
        for (_, _, until), stored in last.items():
            if stored is not None:
                self.pending[until].append(stored)
        return out

    def finish(self):
        assert not any(self.jobs.values()) and not any(self.pending.values())


def _ops49(fn, blocks, m):
    return fn(*[fn(*[blocks[q][e] for q in range(4)])[m] for e in range(4)])


def _words49(fn, words, m):
    halves = [[_split(w) for w in q] for q in words]
    lo = _ops49(fn, [[h[0] for h in q] for q in halves], m)
    hi = _ops49(fn, [[h[1] for h in q] for q in halves], m)
    return [_join(a, b) for a, b in zip(lo, hi)]


def _fold(xs, op):
    acc = xs[0]
    for x in xs[1:]:
        acc = op(acc, x)
    return acc


def _tree(xs, op):
    while len(xs) > 1:
        xs = [op(a, b) for a, b in zip(xs[::2], xs[1::2])]
    return xs[0]


def _lane_chunks(x):
    return [x[:, j * 128:(j + 1) * 128] for j in range(x.shape[1] // 128)]


def _kernel(x_hbm, c_hbm, wq_hbm, wuk_hbm, wuv_hbm, wo_hbm, wqkv_hbm, wob_hbm, gw_hbm,
            out_hbm,
            xs_u, x_r, c_r, w_r, wv_r, wob_p, wkv_r, wq_r, wo_r,
            wperm, xq, cq, wv7, wob5, wo49, wkv, wq49, ups, sc_s, bx, qn,
            qk_b, vb, lg_s, pr_s, o_s, ob7, ctx, ca0, ca1, g_s, out_s, gw_ref,
            sem_x, sem_p, sem_a):
    x_u = x_hbm.bitcast(U32)
    c_u = c_hbm.bitcast(U32)
    wo_u = wo_hbm.bitcast(U32)
    wq_u = wq_hbm.bitcast(U32)
    wuk_u = wuk_hbm.bitcast(U32)
    wuv_u = wuv_hbm.bitcast(U32)
    wob_u = wob_hbm.bitcast(U32)
    part = functools.partial

    def blk(j, n):
        return pl.ds(pl.multiple_of(j * n, n), n)

    def strip(j):
        return blk(j, 128)

    def cp_x(t):
        return pltpu.make_async_copy(x_u.at[:, strip(t >> 1)], xs_u.at[t >> 1], sem_x.at[0])

    def cp_w(t, sem):
        return pltpu.make_async_copy(wqkv_hbm.at[t >> 3, strip((t >> 1) & 3), blk(t & 1, M)],
                                     w_r.at[t & 1], sem)

    def cp_side(t):
        dp = ((t >> 3) << 2) + (t & 2) + ((t >> 2) & 1)
        sem = sem_x.at[t & 1]
        return (
            pltpu.make_async_copy(x_u.at[blk(t, HQ), :], x_r.at[t & 1], sem),
            pltpu.make_async_copy(c_u.at[blk(t, HQ), :], c_r.at[t & 1], sem),
            pltpu.make_async_copy(wqkv_hbm.at[:, blk(t, 32), pl.ds(2 * M, M)], wv_r.at[t & 1], sem),
            pltpu.make_async_copy(wob_u.at[:, t & 1, dp, :], wob_p.at[blk(t, 16), :], sem),
            pltpu.make_async_copy(wob_u.at[:, t & 1, dp + 8, :], wob_p.at[blk(t + 16, 16), :], sem),
        )

    def cp_wq(p, sem):
        return pltpu.make_async_copy(wq_u.at[:, jnp.minimum(p, NP - 1), :], wq_r.at[p & 3], sem)

    def cp_p(g):
        slot = g & 1
        p = jnp.minimum(g + 1, NP - 1)
        o = jnp.clip(g, 0, NP - 1)
        sem = sem_p.at[slot]
        return (
            pltpu.make_async_copy(wo_u.at[blk(o >> 1, 2 * DA), blk(o & 1, M // 2)],
                                  wo_r.at[slot], sem),
            pltpu.make_async_copy(wuk_u.at[:, p, :], wkv_r.at[slot, pl.ds(DC, DC), :], sem),
            pltpu.make_async_copy(wuv_u.at[:, p, :], wkv_r.at[slot, pl.ds(0, DC), :], sem),
            cp_wq(g + 2, sem),
        )

    def cp_gw():
        return pltpu.make_async_copy(gw_hbm, gw_ref, sem_a.at[0])

    def cp_out(i):
        return pltpu.make_async_copy(out_s.at[blk(i, TO), :], out_hbm.at[blk(i, TO), :],
                                     sem_a.at[1])

    def group(t, fn):
        tc = jnp.minimum(t, 15)
        for d in cp_side(tc):
            pl.when(t < 16)(part(fn, d))
        pl.when((t & 17) == 0)(part(fn, cp_x(tc)))
        pl.when(t < 15)(part(fn, cp_w(jnp.minimum(t + 1, 15), sem_x.at[t & 1])))

    cp_w(0, sem_a.at[1]).start()
    cp_x(0).start()
    cp_w(1, sem_x.at[0]).start()
    for d in cp_side(0):
        d.start()

    for cc in range(8):
        qk_b[8 + cc, pl.ds(0, PAD), :] = jnp.zeros((PAD, 128), F32)
        vb[cc, pl.ds(TQ, PAD), :] = jnp.zeros((PAD, 128), F32)

    def stage_first(t):
        for cc, w in enumerate(_permute8(_lane_chunks(pltpu.bitcast(w_r[t & 1], U32)))):
            wperm[cc] = w

    cp_w(0, sem_a.at[1]).wait()
    stage_first(0)
    cp_w(2, sem_x.at[1]).start()
    for d in cp_side(1):
        d.start()
    cp_gw().start()
    plan1 = _plan1()

    def p1_body(t, carry):
        group(t, lambda d: d.wait())

        def act_sums(src, dst, ns, m, sr, r, gate):
            cw = [[gate(src[(t & 1) + _zero(t, m), pl.ds(32 * (q >> 1) + 16 * (e >> 1) + 8 * r, 8),
                            pl.ds(((2 * (q & 1) + (e & 1)) * ns + sr) * 128, 128)])
                   for e in range(4)] for q in range(4)]
            for n, w in enumerate(_words49(_lhs7, cw, m)):
                dst[7 * m + n, sr, blk(2 * t + r, 8), :] = w
            return [], 0, lambda: dst[7 * m + _zero(t, 0), sr, blk(2 * t + r, 8), :]

        wv = _permute8(_lane_chunks(jnp.concatenate(
            [pltpu.bitcast(wv_r[t & 1, e], U32) for e in range(2)], axis=0)))

        def v_sums(r, cc, gate):
            ops = _words7(_rhs7, [gate(wv[cc + 4 * d][16 * e + 8 * r:16 * e + 8 * r + 8])
                                  for e in range(2) for d in range(2)])
            for m in range(7):
                wv7[m, cc, blk(2 * t + r, 8), :] = ops[m]
            return [], 0, lambda: wv7[_zero(t, 0), cc, blk(2 * t + r, 8), :]

        def o_sums(r, cc, gate):
            ops = _words7(_rhs7, [gate(wob_p[blk(2 * t + r + 32 * e, 8), strip(cc + 4 * d)])
                                  for e in range(2) for d in range(2)])
            for e, m in enumerate(RSUM):
                wob5[e, blk(2 * t + r, 8), strip(cc)] = ops[m]
            return [], 0, lambda: wob5[_zero(t, 0), blk(2 * t + r, 8), strip(cc)]

        sched = _Sched(t > 99, plan1, dict(
            x=[part(act_sums, x_r, xq, 2, m, sr, r)
               for m in range(7) for sr in range(2) for r in range(2)],
            c=[part(act_sums, c_r, cq, 1, m, 0, r) for m in range(7) for r in range(2)],
            v=[part(v_sums, r, cc) for r in range(2) for cc in range(4)],
            o=[part(o_sums, r, cc) for r in range(2) for cc in range(4)]))

        first = t < 2
        for half in range(2):
            for rb in range(4):
                w = jnp.concatenate([wperm[4 * half + cc] for cc in range(4)], axis=1)
                r = sched.mm(4 * half + rb, xs_u[t >> 1, pl.ds(rb * 256, 256), :], w)
                for cc in range(4):
                    sl = (8 * (t & 1) + 4 * half + cc, pl.ds(PAD + rb * 512, 512), slice(None))
                    old = jnp.where(first, 0.0, qk_b[sl])
                    qk_b[sl] = old + r[:, cc * 128:(cc + 1) * 128]
        sched.finish()
        stage_first(jnp.minimum(t + 1, 15))

        group(t + 2, lambda d: d.start())

        @pl.when(jnp.logical_and(t >= 7, t < 9))
        def _():
            for d in cp_p(t - 8):
                d.start()

        @pl.when(t == 6)
        def _():
            cp_wq(0, sem_p.at[1]).start()

        return t

    last = jax.lax.fori_loop(0, 16, p1_body, 0)

    row = jax.lax.broadcasted_iota(jnp.int32, (TQ, TQ), 0)
    col = jax.lax.broadcasted_iota(jnp.int32, (TQ, TQ), 1)
    col = (col & ~31) | ((col & 1) << 4) | ((col & 31) >> 1)
    rowi = jax.lax.broadcasted_iota(jnp.int32, (RB, 128), 0)
    odd = (jax.lax.broadcasted_iota(jnp.int32, (RB, 128), 1) & 1) == 1
    NSUB = HQ // RB
    QSCALE = DA ** -0.5 * LOG2E

    def pair_rows(src, slot, r0, n, gate):
        return [_split(gate(src[slot, pl.ds(r0 + par, n // 2, stride=2), :])) for par in range(2)]

    def staging(g, z):
        ns = DC // SCR

        def scales(n1, k, gate):
            res = []
            for h in range(2):
                if k < ns:
                    w = gate(wkv_r[g & 1, pl.ds(n1 * DC + k * SCR, SCR), :])
                    w = pltpu.bitcast(w, jnp.int32) & (0x7F80 << (16 * h))
                else:
                    w = gate(sc_s[2 * n1 + h, pl.ds(0, 8 * ns), :])
                e = _tree([w[r:r + 8] for r in range(0, w.shape[0], 8)], jnp.maximum)
                if k == ns:
                    e = pltpu.bitcast(e << (16 - 16 * h), F32)
                    e = jnp.max(e, axis=0, keepdims=True)
                    e = jnp.clip(pltpu.bitcast(e, jnp.int32), 1 << 23, 253 << 23)
                    e = jnp.broadcast_to(e, (8, 128))
                    sc_s[2 * n1 + h, pl.ds(8 * ns + 8, 8), :] = (254 << 23) - e
                sc_s[2 * n1 + h, pl.ds(8 * k, 8), :] = e
                res.append(pltpu.bitcast(e, U32))
            return res, 0, lambda: pltpu.bitcast(sc_s[2 * n1, blk(k + _zero(z, 0), 8), :], U32)

        def rhs49(dst, tiles, scale, m, r):
            res = [_ops49(_rhs7,
                          [[scale(tiles[2 * (q >> 1) + (e >> 1)][q & 1][par][e & 1],
                                  2 * (q & 1) + (e & 1)) for e in range(4)] for q in range(4)],
                          m) for par in range(2)]
            for k, (lo, hi) in enumerate(zip(*res)):
                dst[7 * m + k, pl.ds(8 * r, 8), :] = _join(lo, hi)

        def kv(m, r, gate):
            if m == 0 and r == 0:
                for k in range(4):
                    ups[k] = pltpu.bitcast(gate(sc_s[k, pl.ds(8 * ns, 8), :]), F32)
            down = [pltpu.bitcast(sc_s[k + _zero(z, m), pl.ds(8 * ns + 8, 8), :], F32)
                    for k in range(4)]
            tiles = [[pair_rows(wkv_r, (g & 1) + _zero(z, m), n1 * DC + kt * 128 + 16 * r, 16, gate)
                      for n1 in range(2)] for kt in range(4)]
            rhs49(wkv, tiles, lambda w, k: w * down[k], m, r)
            return [], 0, lambda: wkv[7 * m, blk(r + _zero(z, 0), 8), :]

        def qw(m, r, gate):
            tiles = [[pair_rows(wq_r, ((g + 1 + n1) & 3) + _zero(z, m), kt * 256 + 16 * r, 16, gate)
                      for n1 in range(2)] for kt in range(4)]
            rhs49(wq49, tiles, lambda w, k: w, m, r)
            return [], 0, lambda: wq49[7 * m, blk(r + _zero(z, 0), 8), :]

        def b_lhs(u, r, gate):
            base = 8 * jnp.minimum(g + 1, NQ - 1) + r
            ops = _words7(_lhs7, [gate(xs_u[u + 4 * d, blk(base + 4 * e, 8), :])
                                  for e in range(2) for d in range(2)])
            for k, m in enumerate(LSUM):
                bx[k, pl.ds(8 * r, 8), strip(u)] = ops[m]
            return [], 0, lambda: bx[0, blk(r + _zero(z, 0), 8), strip(u)]

        return dict(sc=[part(scales, n1, k) for k in range(ns + 1) for n1 in range(2)],
                    kv=[part(kv, m, r) for m in range(7) for r in range(8)],
                    qw=[part(qw, m, r) for m in range(7) for r in range(16)],
                    bx=[part(b_lhs, u, r) for u in range(4) for r in range(4)])

    cp_wq(0, sem_p.at[1]).wait()
    for d in cp_p(-1):
        d.wait()
    sched = _Sched(last > 99, _planx(), staging(-1, last))
    w0 = pair_rows(wq_r, 0, 0, M, lambda x: x)
    w0 = [_join(w0[0][h], w0[1][h]) for h in range(2)]
    for g in range(4):
        for e in range(2):
            for h in range(2):
                q = [sched.mm(8 * g + 4 * e + 2 * h + k, jnp.concatenate(
                    [xs_u[4 * k + u, pl.ds((4 * g + 2 + e) * HQ, HQ), :] for u in range(4)], axis=1),
                    w0[h][256 * k:256 * k + 256], step=16) for k in range(2)]
                qn[h, g, e] = _pack((q[0] + q[1]) * QSCALE)
    sched.finish()
    for d in cp_p(1):
        d.start()
    plan2 = _plan2()

    def p2_body(p, carry):
        for d in cp_p(p):
            d.wait()
        causal = col <= row
        never = p > NP
        jobs = staging(p, p)
        sched = _Sched(never, plan2, jobs)
        mm = sched.mm

        r0 = pl.multiple_of(p * TQ, TQ)

        def scatter(dst, off, c):
            for e, t in enumerate(c):
                for cc in range(4):
                    dst[4 * (e & 1) + cc, pl.ds(off + (PAD + (e >> 1) * HQ), HQ), :] = (
                        t[:, cc * 128:(cc + 1) * 128])

        def proj_bv():
            def lhs(m):
                if m in (2, 3):
                    return jnp.concatenate([xs_u[u + 4 * (m - 2), blk(2 * p + m - 2, QQ), :]
                                            for u in range(4)], axis=1)
                return bx[LSUM.index(m)]

            for cc in range(8):
                vb[cc, pl.ds(0, PAD), :] = vb[cc, pl.ds(TQ, PAD), :]
            c = [_combine(lambda m: mm(("bv", 7 * e + ORDER.index(m)), lhs(m), jnp.concatenate(
                [wv7[m, 2 * e], wv7[m, 2 * e + 1]], axis=1))) for e in range(2)]
            scatter(vb, 0, [jnp.concatenate(t, axis=1) for t in zip(*c)])

        def local_qk(rb, k, gate):
            q = [qk_b[cc, pl.ds(r0 + _zero(p, k) + (PAD + rb * RB), RB), :] for cc in range(8)]
            q[0] = gate(q[0])
            for w in range(LG * k, LG * k + LG):
                t = _fold([q[cc] * qk_b[8 + cc, pl.ds(r0 + (PAD + rb * RB - DIL * w), RB), :]
                           for cc in range(8)], jnp.add)
                t = t + pltpu.roll(t, 64, 1)
                t = t + jnp.where(odd, pltpu.roll(t, 1, 1), pltpu.roll(t, 127, 1))
                t = t * (DB ** -0.5 * LOG2E)
                if rb == 0 and w:
                    t = jnp.where(rowi + r0 >= DIL * w, t, NEG)
                lg_s[w, pl.ds(rb * RB, RB), :] = t
            return [], 1, lambda: pltpu.bitcast(lg_s[w, blk(2 * rb + _zero(p, 0), 8), :], U32)

        def local_sm(rb, e, gate):
            rows = pl.ds(rb * RB + SMR * e, SMR)
            lg = [gate(lg_s[w, rows, :]) for w in range(WIN)]
            m = _tree(lg, jnp.maximum)
            ps = [jnp.exp2(t - m) for t in lg]
            l = _tree(ps, jnp.add)
            r = pl.reciprocal(l, approx=True)
            r = r * (2.0 - l * r)
            for w in range(WIN):
                pr_s[w, rows, :] = ps[w] * r
            return [], 2, lambda: pltpu.bitcast(pr_s[0, blk(2 * rb + e + _zero(p, 0), 8), :], U32)

        def local_pv(rb, k, gate):
            rows = pl.ds(rb * RB, RB)
            ps = [pr_s[w + _zero(p, k), rows, :] for w in range(WIN)]
            ps[0] = gate(ps[0])
            o = [_fold([ps[w] * vb[cc, pl.ds(PAD + rb * RB - DIL * w, RB), :] for w in range(WIN)],
                       jnp.add) for cc in (k, k + 4)]
            if rb < NSUB:
                for e in range(2):
                    o_s[k + 4 * e, rows, :] = o[e]
                return [], 3, lambda: pltpu.bitcast(o_s[k, blk(2 * rb + _zero(p, 0), 8), :], U32)
            top = pl.ds((rb - NSUB) * RB, RB)
            for m, t in enumerate(_lhs7(o_s[k, top, :], o_s[k + 4, top, :], *o)):
                ob7[m, pl.ds((rb - NSUB) * RB // 2, RB // 2), strip(k)] = _pack(t)
            return [], 0, lambda: ob7[0, blk(rb - NSUB + _zero(p, 0), 8), strip(k)]

        order = [rb + e * NSUB for rb in range(NSUB) for e in range(2)]
        jobs["lo"] = []
        for k in range(len(order) + SML):
            for f, d, n in ((local_sm, SML, RB // SMR), (local_qk, 0, 8 // LG)):
                if 0 <= k - d < len(order):
                    jobs["lo"] += [part(f, order[k - d], e) for e in range(n)]
        jobs["lv"] = [part(local_pv, rb, e) for rb in order for e in range(4)]

        def wob(m):
            if m == 1:
                return wob_p[pl.ds(0, M // 4), pl.ds(0, M // 2)]
            if m == 4:
                return wob_p[pl.ds(M // 4, M // 4), pl.ds(M // 2, M // 2)]
            return wob5[RSUM.index(m)]

        bo = {}

        def proj_bo(n):
            for m in ORDER[len(bo):len(bo) + n]:
                bo[m] = mm(("bo", len(bo)), lambda: ob7[m], wob(m))
            if n and len(bo) == 7:
                scatter(qk_b, r0, _combine(lambda m: bo[m]))

        def out_weights(m, r, gate):
            ww = [[gate(wo_r[(p & 1) + _zero(p, m),
                             pl.ds((2 * (q >> 1) + (e >> 1)) * HQ + 8 * r, 8),
                             pl.ds((2 * (q & 1) + (e & 1)) * 128, 128)])
                   for e in range(4)] for q in range(4)]
            rows = blk(8 * (p >> 1) + r, 8)
            extra = jobs["sc"].pop(0)(gate)[0] if jobs["sc"] else []
            for n, w in enumerate(_words49(_rhs7, ww, m)):
                if n < len(extra):
                    w = jnp.where(never, extra[n], w)
                wo49[7 * m + n, p & 1, rows, :] = w
            return [], 0, lambda: wo49[7 * m + _zero(p, 0), p & 1, rows, :]

        jobs["wo"] = [part(out_weights, m, r) for m in range(7) for r in range(8)]

        ks, vs, qs = {}, {}, {}
        done, prods = {}, {}

        def project(kind, j, n, lhs, rhs, scale, pack):
            got = prods.setdefault((kind, j), {})
            for m in ORDER[len(got):len(got) + n]:
                got[m] = _combine(lambda k: mm((kind, j, 7 * len(got) + ORDER.index(k)),
                                               lhs(7 * m + k), rhs[7 * m + k]))
            if len(got) < 7:
                return None
            c = _combine(lambda m: got[m])
            c = [[pack(c[(rg & 2) + (cg >> 1)][2 * (rg & 1) + (cg & 1)] * scale(cg))
                  for rg in range(4)] for cg in range(4)]
            return [[jnp.concatenate([t[16 * e:16 * e + 16] for t in c[cg]], axis=0)
                     for e in range(2)] for cg in range(4)]

        def proj_kv(j, n):
            c = project("kv", j, n, lambda k: cq[k, 0, pl.ds(j * QQ, QQ), :], wkv,
                        lambda cg: ups[cg][:1], _riffle)
            if c is not None:
                for cg in range(4):
                    for e in range(2):
                        (vs, ks)[cg >> 1][(cg & 1, 2 * j + e)] = c[cg][e]

        def proj_q(g, n):
            rows = blk(2 * g + (p & 1), QQ)
            c = project("q", g, n,
                        lambda k: jnp.concatenate([xq[k, sr, rows, :] for sr in range(2)], axis=1),
                        wq49, lambda cg: QSCALE, _pack)
            if c is not None:
                for h in range(2):
                    for e in range(2):
                        old = qn[h, g, e]
                        for b in range(2):
                            qs[(h, 4 * g + 2 * b + e)] = jnp.where((p & 1) == b, c[h][e], old)
                        qn[h, g, e] = c[2 + h][e]

        def qk(h, i, dep):
            kk = jnp.concatenate([ks[(h, j)] for j in range(i + 1)], axis=0)
            q = qs[(h, i)]
            if dep is not None:
                q = jnp.where(never, done[(h, dep)], q)
            ch = _lane_chunks(mm(("qk", h, i), q, kk, NT, 512))
            ch[i] = jnp.where(causal, ch[i], NEG)
            return ch

        def softmax_pv(h, i, ch):
            m = jnp.max(_fold(ch, jnp.maximum), axis=1, keepdims=True)
            ps = [jnp.exp2(c - m) for c in ch]
            lp = ps[0]
            for j in range(1, i + 1):
                lp = lp + ps[j]
                if TIE and (j % TIE == TIE - 1 or j == i):
                    ps[j] = jnp.where(never, lp, ps[j])
            pb = jnp.concatenate(ps, axis=1).astype(BF16)
            vv = jnp.concatenate([vs[(h, j)] for j in range(i + 1)], axis=0)
            o = mm(("pv", h, i), pb, vv)
            if i >= LDEP:
                lp = jnp.where(never, o, lp)
            l = jnp.sum(lp, axis=1, keepdims=True)
            r = pl.reciprocal(l, approx=True)
            r = r * (2.0 - l * r)
            cn = _pack(o * r)
            done[(h, i)] = cn
            if FA <= i < NQ - 1:
                if h == 0 and F0 < 0:
                    site = ("qk", 1, i + 1)
                elif i + 3 < NQ:
                    site = ("kv", (i + 1) // 2 + 1, KVS * ((i + 1) & 1) + (F0, FD)[h])
                else:
                    site = ("bo", (i + 3 - NQ) * BOP[0] + h)
                sched.pending.setdefault(site, []).append(cn)
            ctx[2 * p + h, pl.ds(i * HQ, HQ), :] = cn

        proj_bv()
        proj_kv(0, 7)
        proj_q(0, 7)
        for i in range(NQ):
            dep = i - DEP if DEP <= i < FA + DEP else None
            s0 = qk(0, i, dep)
            s1 = qk(1, i, dep)
            if i + 2 < NQ:
                proj_kv(i // 2 + 1, 7 if i & 1 else KVS // 7)
                if i < 6:
                    proj_q(i // 2 + 1, 7 if i & 1 else QS // 7)
            else:
                proj_bo(BOP[i + 2 - NQ])
            softmax_pv(0, i, s0)
            softmax_pv(1, i, s1)
        proj_bo(BOP[2])
        sched.finish()
        for d in cp_p(p + 2):
            d.start()
        return carry

    jax.lax.fori_loop(0, NP, p2_body, 0)

    cp_gw().wait()
    gw = gw_ref[...].astype(F32)
    plan3 = _plan3()
    cab = (ca0, ca1)

    def p3_body(i, carry):
        r0 = pl.multiple_of(i * TO, TO)
        h0 = pl.multiple_of(i * (TO // 2), TO // 2)
        never = i > S

        def ctx_words(m, u, r, n):
            return [[ctx[4 * u + 2 * (q & 1) + (e & 1),
                         pl.ds(h0 + _zero(i, m) * 8 + ((2 * (q >> 1) + (e >> 1)) * QQ + r), n), :]
                     for e in range(4)] for q in range(4)]

        def operands(k, u, r, gate):
            m = ORDER[k]
            cw = [[gate(w) for w in q] for q in ctx_words(m, u, r, 8)]
            for n, w in enumerate(_words49(_lhs7, cw, m)):
                if not (m in (2, 3) and n in (2, 3)):
                    cab[k & 1][n, pl.ds(r, 8), pl.ds(u * 128, 128)] = w
            return [], 0, lambda: cab[k & 1][_zero(i, 0), pl.ds(r, 8), pl.ds(u * 128, 128)]

        def gate_rows(r, gate):
            gs = _fold([_bf(gate(xs_u[j, pl.ds(h0 + r, 8), :])).astype(F32) * gw[j:j + 1]
                        for j in range(8)], jnp.add)
            g = jax.nn.sigmoid(jnp.sum(gs, axis=1, keepdims=True))
            g_s[pl.ds(2 * r, 16), :] = jnp.broadcast_to(g, (16, 128))
            return [], 0, lambda: pltpu.bitcast(g_s[blk(r // 4 + _zero(i, 0), 8), :], U32)

        sched = _Sched(never, plan3, dict(
            a=[part(operands, k, u, r) for k in range(1, 7) for u in range(HA // 4)
               for r in range(0, QQ, 8)],
            g=[part(gate_rows, r) for r in range(0, TO // 2, 8)]))
        first = [[_words49(_lhs7, ctx_words(ORDER[0], u, 0, QQ), ORDER[0])[n]
                  for u in range(HA // 4)] for n in range(7)]

        def inner(m, n):
            k = ORDER.index(m)
            res = []
            for e in range(2):
                us = range(4 * e, 4 * e + 4)
                if m in (2, 3) and n in (2, 3):
                    lhs = jnp.concatenate([ctx_words(m, u, 0, QQ)[3 * (m - 2)][3 * (n - 2)]
                                           for u in us], axis=1)
                elif k == 0:
                    lhs = jnp.concatenate([first[n][u] for u in us], axis=1)
                else:
                    lhs = lambda: cab[k & 1][n, :, pl.ds(e * 512, 512)]
                rhs = jnp.concatenate([wo49[7 * m + n, cc, pl.ds(e * 256, 256), :]
                                       for cc in range(2)], axis=1)
                res.append(sched.mm((k, 2 * ORDER.index(n) + e), lhs, rhs))
            return res[0] + res[1]

        acs = _combine(lambda m: _combine(lambda n: inner(m, n)))
        sched.finish()
        for q in range(4):
            for e in range(4):
                off = (2 * (q >> 1) + (e >> 1)) * HQ
                g = g_s[pl.ds(off, HQ), :]
                for cc in range(2):
                    ch = 4 * cc + 2 * (q & 1) + (e & 1)
                    a = acs[q][e][:, cc * 128:(cc + 1) * 128]
                    b = qk_b[ch, pl.ds(r0 + (PAD + off), HQ), :]
                    out_s[pl.ds(r0 + off, HQ), pl.ds(ch * 128, 128)] = (
                        g * a + (1.0 - g) * b).astype(BF16)
        cp_out(i).start()
        return carry

    jax.lax.fori_loop(0, S // TO, p3_body, 0)
    for g in range(NP, NP + 2):
        for d in cp_p(g):
            d.wait()
    for i in range(S // TO):
        cp_out(i).wait()


@jax.jit
def pallas_gated_mix__compressed_kv_cla__sliding_local_dilated__prompt_kernel(
    A_x: jax.Array,
    A_c_kv: jax.Array,
    A_w_q: jax.Array,
    A_w_uk: jax.Array,
    A_w_uv: jax.Array,
    A_w_o: jax.Array,
    B_x: jax.Array,
    B_wqkv: jax.Array,
    B_wo: jax.Array,
    gate_w: jax.Array,
):
    del B_x
    any_spec = pl.BlockSpec(memory_space=pl.ANY)
    out = pl.pallas_call(
        _kernel,
        in_specs=[any_spec] * 9,
        out_specs=any_spec,
        out_shape=jax.ShapeDtypeStruct((S, M), BF16),
        scratch_shapes=[
            pltpu.VMEM((8, S // 2, 128), U32),
            pltpu.VMEM((2, HQ, M), U32),
            pltpu.VMEM((2, HQ, DC), U32),
            pltpu.VMEM((2, 128, M), BF16),
            pltpu.VMEM((2, 2, 32, M), BF16),
            pltpu.VMEM((M // 2, M), U32),
            pltpu.VMEM((2, 2 * DC, 128), U32),
            pltpu.VMEM((4, M, 128), U32),
            pltpu.VMEM((2, 2 * DA, M // 2), U32),
            pltpu.VMEM((8, 64, 128), U32),
            pltpu.VMEM((49, 2, S // 8, 128), U32),
            pltpu.VMEM((49, 1, S // 8, 128), U32),
            pltpu.VMEM((7, 4, M // 4, 128), U32),
            pltpu.VMEM((5, M // 4, M // 2), U32),
            pltpu.VMEM((49, 2, NP * QQ, 128), U32),
            pltpu.VMEM((49, HQ, 128), U32),
            pltpu.VMEM((49, TQ, 128), U32),
            pltpu.VMEM((4, 8, 128), F32),
            pltpu.VMEM((4, DC // SCR * 8 + 16, 128), jnp.int32),
            pltpu.VMEM((5, QQ, M // 2), U32),
            pltpu.VMEM((2, 4, 2, HQ, 128), U32),
            pltpu.VMEM((16, S + PAD, 128), F32),
            pltpu.VMEM((8, TQ + PAD, 128), F32),
            pltpu.VMEM((WIN, TQ, 128), F32),
            pltpu.VMEM((WIN, TQ, 128), F32),
            pltpu.VMEM((8, HQ, 128), F32),
            pltpu.VMEM((7, QQ, M // 2), U32),
            pltpu.VMEM((HA, S // 2, 128), U32),
            pltpu.VMEM((7, QQ, M), U32),
            pltpu.VMEM((7, QQ, M), U32),
            pltpu.VMEM((TO, 128), F32),
            pltpu.VMEM((S, M), BF16),
            pltpu.VMEM((8, 128), BF16),
            pltpu.SemaphoreType.DMA((2,)),
            pltpu.SemaphoreType.DMA((2,)),
            pltpu.SemaphoreType.DMA((2,)),
        ],
        compiler_params=pltpu.CompilerParams(vmem_limit_bytes=120 * 1024 * 1024,
                                             disable_bounds_checks=True),
    )(
        A_x.reshape(S, M),
        A_c_kv.reshape(S, DC),
        A_w_q,
        A_w_uk,
        A_w_uv,
        A_w_o.reshape(HA * DA, M),
        B_wqkv.reshape(2, M // 2, 3 * M),
        B_wo.reshape(HB // 2, 2, DB, M),
        gate_w.reshape(8, 128),
    )
    return out.reshape(1, S, M)
```

```python
import functools
import math

import jax
import jax.numpy as jnp
import jax.experimental.pallas as pl
import jax.experimental.pallas.tpu as pltpu

F32 = jnp.float32
BF16 = jnp.bfloat16
U32 = jnp.uint32

S = 2048
M = 1024
HA = 32
DA = 128
DC = 512
HB = 32
DB = 32
WIN = 8
DIL = 2
PAD = 16
LOG2E = math.log2(math.e)
NEG = -1e9

TQ = 128
HQ = TQ // 2
QQ = TQ // 4
BOP = (2, 3, 2)
LX = 16
KVS = 28
QS = 28
QST = 2
LQ0 = 3
LG = 2
XN = 29
SK = 3
SMR = 16
P1N = 6
P1U = 2
P3S = 4
P3E = 12
NQ = S // TQ
NP = HA // 2
DEP = 2
SCR = 32
LN = 62
SML = 2
LE = 2
LI = 0
LA = 29
LB = 4
LS = 4
LP = ("kv", 0, 44)
FA = 6
F0 = 0
FD = 8
TIE = 4
RB = 16
LDEP = 4
TO = 256
NN = (((1,), (0,)), ((), ()))
NT = (((1,), (1,)), ((), ()))


def _plan2():
    plan = {}

    def put(name, count, start, until):
        plan.setdefault(start, []).extend([(name, until)] * count)

    def after_qk(i):
        if i >= NQ - 2:
            return ("bo", (i - NQ + 2) * BOP[0] + 1)
        return ("kv", i // 2 + 1, KVS * (i & 1) + LX)

    def fill(name, count, sites):
        for start, room, until in sites:
            n = min(count, room - len(plan.get(start, ())))
            put(name, n, start, until)
            count -= n
        assert count == 0, (name, count)

    def qk_sites(lo, hi):
        return [(("qk", h, i), max(i + 1 - h * SK, 0), after_qk(i))
                for i in range(lo, hi) for h in range(2)]

    def q_sites(g, lo, hi, until):
        return [(("q", g, k), 1, until) for k in range(lo, hi, QST)]

    names = _spread(["lo"] * (64 // LG + 128 // SMR), LN)
    for k, name in enumerate(names):
        put(name, 1, ("bv", k // 4) if k < 56 else ("kv", 0, 2 * (k - 56) + 1), LP)
    first = [(("kv", 0, k), 1, ("kv", 1, 8)) for k in range(LA, 49, LS)]
    first += [(("q", 0, k), 1, ("kv", 1, 8)) for k in range(LI, 49 - LB, LE)]
    early = []
    for g in range(1, 4):
        early += q_sites(g, 0, QS - 4, after_qk(2 * g - 1))
        early += qk_sites(max(2 * g - 1, LQ0), 2 * g)
        early += q_sites(g, QS, 45, after_qk(2 * g))
        early += qk_sites(max(2 * g, LQ0), 2 * g + 1)
    fill("lv", 32, first + early)
    fill("wo", 56, early)
    fill("bx", 16, early + qk_sites(7, 14))
    fill("qw", 112, qk_sites(7, 14))
    fill("kv", 56, qk_sites(14, 16) + [(("bo", k), 8, ("bo", 6)) for k in range(BOP[0], 5)])
    return plan


def _planx():
    names = _spread(["sc"] * (2 * DC // SCR + 2) + ["bx"] * 16 + ["qw"] * 112 + ["kv"] * 56, 8 * XN)
    return {k: [(n, 31) for n in names[8 * k:8 * k + 8]] for k in range(XN)}


def _spread(names, ticks):
    out = [None] * ticks
    for k, name in enumerate(names):
        out[k * ticks // len(names)] = name
    return out


def _plan1():
    names = _spread(["x"] * 28 + ["c"] * 14 + ["o"] * 8 + ["v"] * 8, 16 * P1N)
    return {k: [(n, min(k + P1U, 7)) for n in names[16 * k:16 * k + 16]] for k in range(P1N)}


def _plan3():
    plan = {}
    for k in range(6):
        lo = P3S if k == 0 else 0
        extra = ["g"] * 8 if k in (1, 2) else []
        names = _spread(["a"] * 32 + extra, 4 * (P3E - lo))
        for d in range(lo, P3E):
            plan[(k, d)] = [(n, (k + 1, 0)) for n in names[4 * (d - lo):4 * (d - lo) + 4]]
    return plan


_STAGES = ((2, 4), (1, 3), (0, 2), (0, 6), (0, 1))


def _permute8(cols):
    cols = list(cols)
    lane = jax.lax.broadcasted_iota(jnp.int32, cols[0].shape, 1)
    for va, lb in _STAGES:
        lo = (lane & (1 << lb)) == 0
        sh = 1 << lb
        idx = [i for i in range(8) if not (i >> va) & 1]
        if lb == 6:
            rr = [pltpu.roll(jnp.where(lo, cols[i | (1 << va)], cols[i]), 64, 1) for i in idx]
            for i, r in zip(idx, rr):
                a, b = cols[i], cols[i | (1 << va)]
                cols[i] = jnp.where(lo, a, r)
                cols[i | (1 << va)] = jnp.where(lo, r, b)
        else:
            rb = [pltpu.roll(cols[i | (1 << va)], sh, 1) for i in idx]
            ra = [pltpu.roll(cols[i], 128 - sh, 1) for i in idx]
            for i, xa, xb in zip(idx, ra, rb):
                a, b = cols[i], cols[i | (1 << va)]
                cols[i] = jnp.where(lo, a, xb)
                cols[i | (1 << va)] = jnp.where(lo, xa, b)
    return cols


def _pack(x):
    return pltpu.bitcast(x.astype(BF16), U32)


def _bf(x):
    return pltpu.bitcast(x, BF16)


def _split(w):
    return (pltpu.bitcast(w << 16, F32), pltpu.bitcast(w & jnp.uint32(0xFFFF0000), F32))


def _join(lo, hi):
    return pltpu.bitcast(pltpu.pack_elementwise([lo, hi], packed_dtype=BF16), U32)


def _riffle(x):
    return jnp.concatenate([_join(x[r:r + 16], x[r + 16:r + 32]) for r in range(0, x.shape[0], 32)],
                           axis=0)


def _lhs7(a11, a12, a21, a22):
    return [a11 + a22, a21 + a22, a11, a22, a11 + a12, a21 - a11, a12 - a22]


def _rhs7(b11, b12, b21, b22):
    return [b11 + b22, b11, b12 - b22, b21 - b11, b22, b11 + b12, b21 + b22]


LSUM = (0, 1, 4, 5, 6)
RSUM = (0, 2, 3, 5, 6)


def _words7(fn, quads):
    halves = [_split(w) for w in quads]
    lo = fn(*[h[0] for h in halves])
    hi = fn(*[h[1] for h in halves])
    return [_join(a, b) for a, b in zip(lo, hi)]


def _combine(mm):
    add = functools.partial(jax.tree.map, jnp.add)
    sub = functools.partial(jax.tree.map, jnp.subtract)
    m2 = mm(2)
    m3 = mm(3)
    m4 = mm(4)
    c12 = add(m2, m4)
    t11 = sub(m3, m4)
    m1 = mm(1)
    c21 = add(m1, m3)
    t22 = sub(m2, m1)
    m0 = mm(0)
    t11 = add(t11, m0)
    t22 = add(t22, m0)
    c11 = add(t11, mm(6))
    return c11, c12, c21, add(t22, mm(5))


ORDER = (2, 3, 4, 1, 0, 6, 5)


def _zero(i, m):
    return i >> (8 + m)


def _merge(vals):
    return _fold([v[r:r + 8, c:c + 128] for v in vals for r in range(0, v.shape[0], 8)
                  for c in range(0, v.shape[1], 128)], jnp.bitwise_or)


def _gate(never, g):
    def gate(x):
        t = jnp.tile(pltpu.bitcast(g, x.dtype), (x.shape[0] // 8, x.shape[1] // 128))
        return jnp.where(never, t, x)
    return gate


def _tie(never, x, deps):
    if not deps:
        return x
    top = jnp.where(never, _merge(deps), x[:8, :128])
    if x.shape[1] > 128:
        top = jnp.concatenate([top, x[:8, 128:]], axis=1)
    return jnp.concatenate([top, x[8:]], axis=0)


class _Sched:
    def __init__(self, never, plan, jobs):
        self.never, self.plan, self.jobs, self.pending = never, plan, jobs, {}

    def mm(self, site, a, b, dims=NN, width=128, step=32):
        deps = [d() if callable(d) else d for d in self.pending.pop(site, ())]
        a = a() if callable(a) else a
        tie = functools.partial(_tie, self.never, deps=deps)
        a, b = (_bf(tie(a)), _bf(b)) if a.dtype == U32 else (a, _bf(tie(b)))
        out = jax.lax.dot_general(a, b, dims, preferred_element_type=F32)
        per = out.shape[0] // step
        last = {}
        for k, (name, until) in enumerate(self.plan.get(site, ())):
            if name is not None:
                r, c = step * (k % per), width * (k // per)
                vals, tag, stored = self.jobs[name].pop(0)(
                    _gate(self.never, out[r:r + 8, c:c + 128]))
                self.pending.setdefault(until, []).extend(vals)
                last[(name, tag, until)] = stored
        for (_, _, until), stored in last.items():
            if stored is not None:
                self.pending[until].append(stored)
        return out

    def finish(self):
        assert not any(self.jobs.values()) and not any(self.pending.values())


def _ops49(fn, blocks, m):
    return fn(*[fn(*[blocks[q][e] for q in range(4)])[m] for e in range(4)])


def _words49(fn, words, m):
    halves = [[_split(w) for w in q] for q in words]
    lo = _ops49(fn, [[h[0] for h in q] for q in halves], m)
    hi = _ops49(fn, [[h[1] for h in q] for q in halves], m)
    return [_join(a, b) for a, b in zip(lo, hi)]


def _fold(xs, op):
    acc = xs[0]
    for x in xs[1:]:
        acc = op(acc, x)
    return acc


def _tree(xs, op):
    while len(xs) > 1:
        xs = [op(a, b) for a, b in zip(xs[::2], xs[1::2])]
    return xs[0]


def _lane_chunks(x):
    return [x[:, j * 128:(j + 1) * 128] for j in range(x.shape[1] // 128)]


def _kernel(x_hbm, c_hbm, wq_hbm, wuk_hbm, wuv_hbm, wo_hbm, wqkv_hbm, wob_hbm, gw_hbm,
            out_hbm,
            xs_u, x_r, c_r, w_r, wv_r, wob_p, wkv_r, wq_r, wo_r,
            wperm, xq, cq, wv7, wob5, wo49, wkv, wq49, ups, sc_s, bx, qn,
            qk_b, vb, lg_s, pr_s, o_s, ob7, ctx, ca0, ca1, g_s, out_s, gw_ref,
            sem_x, sem_p, sem_a):
    x_u = x_hbm.bitcast(U32)
    c_u = c_hbm.bitcast(U32)
    wo_u = wo_hbm.bitcast(U32)
    wq_u = wq_hbm.bitcast(U32)
    wuk_u = wuk_hbm.bitcast(U32)
    wuv_u = wuv_hbm.bitcast(U32)
    wob_u = wob_hbm.bitcast(U32)
    part = functools.partial

    def blk(j, n):
        return pl.ds(pl.multiple_of(j * n, n), n)

    def strip(j):
        return blk(j, 128)

    def cp_x(t, sem):
        k = (t + 1) >> 1
        return pltpu.make_async_copy(x_u.at[blk(t & 1, S // 4), strip(jnp.minimum(k, 7))],
                                     xs_u.at[jnp.minimum(k, 8), blk(t & 1, S // 4), :], sem)

    def cp_w(t, sem):
        u = t - 2 * (t >> 4)
        u = u - 2 * (u >> 4)
        return pltpu.make_async_copy(wqkv_hbm.at[u >> 3, strip((u >> 1) & 3), blk(u & 1, M)],
                                     w_r.at[u & 1], sem)

    def group(t):
        sem = sem_x.at[t & 1]
        late = t >> 4
        u = t - 2 * late
        dp = ((u >> 3) << 2) + (u & 2) + ((u >> 2) & 1)
        pq = (t >> 3) + late
        return (
            pltpu.make_async_copy(x_u.at[blk(u, HQ), :], x_r.at[u & 1], sem),
            pltpu.make_async_copy(c_u.at[blk(u, HQ), :], c_r.at[u & 1], sem),
            pltpu.make_async_copy(wob_u.at[:, u & 1, dp, :], wob_p.at[blk(u, 16), :], sem),
            pltpu.make_async_copy(wob_u.at[:, u & 1, dp + 8, :], wob_p.at[blk(u + 16, 16), :], sem),
            cp_x(t, sem),
            cp_w(t + 1, sem),
            pltpu.make_async_copy(wqkv_hbm.at[0, blk(u, 32), pl.ds(2 * M, M)],
                                  wv_r.at[u & 1, 0], sem),
            pltpu.make_async_copy(wqkv_hbm.at[1, blk(u, 32), pl.ds(2 * M, M)],
                                  wv_r.at[u & 1, 1], sem),
            pltpu.make_async_copy(wq_u.at[strip(t & 7), pq, :], wq_r.at[pq, strip(t & 7), :], sem),
            pltpu.make_async_copy(wuk_u.at[blk(u, 32), 0, :],
                                  wkv_r.at[1 + late, blk(16 + u, 32), :], sem),
            pltpu.make_async_copy(wuv_u.at[blk(u, 32), 0, :],
                                  wkv_r.at[1 + late, blk(u, 32), :], sem),
        )

    def cp_wq(p, sem):
        return pltpu.make_async_copy(wq_u.at[:, jnp.minimum(p, NP - 1), :], wq_r.at[p & 3], sem)

    def cp_p(g):
        slot = g & 1
        p = jnp.minimum(g + 1, NP - 1)
        o = jnp.minimum(g, NP - 1)
        sem = sem_p.at[slot]
        return (
            pltpu.make_async_copy(wo_u.at[blk(o >> 1, 2 * DA), blk(o & 1, M // 2)],
                                  wo_r.at[slot], sem),
            pltpu.make_async_copy(wuk_u.at[:, p, :], wkv_r.at[slot, pl.ds(DC, DC), :], sem),
            pltpu.make_async_copy(wuv_u.at[:, p, :], wkv_r.at[slot, pl.ds(0, DC), :], sem),
            cp_wq(g + 2, sem),
        )

    def cp_gw():
        return pltpu.make_async_copy(gw_hbm, gw_ref, sem_a.at[0])

    def cp_out(i):
        return pltpu.make_async_copy(out_s.at[blk(i, TO), :], out_hbm.at[blk(i, TO), :],
                                     sem_a.at[1])

    cp_w(0, sem_a.at[1]).start()
    cp_x(-1, sem_a.at[2]).start()
    for d in group(0)[4:] + group(0)[:4]:
        d.start()

    for cc in range(8):
        qk_b[8 + cc, pl.ds(0, PAD), :] = jnp.zeros((PAD, 128), F32)
        vb[cc, pl.ds(TQ, PAD), :] = jnp.zeros((PAD, 128), F32)

    def stage_first(t):
        for cc, w in enumerate(_permute8(_lane_chunks(pltpu.bitcast(w_r[t & 1], U32)))):
            wperm[cc] = w

    cp_w(0, sem_a.at[1]).wait()
    stage_first(0)
    for d in group(1) + cp_p(0):
        d.start()
    cp_gw().start()
    cp_x(-1, sem_a.at[2]).wait()
    plan1 = _plan1()

    def p1_body(t, carry):
        for d in group(t):
            d.wait()

        def act_sums(src, dst, ns, m, sr, r, gate):
            cw = [[gate(src[(t & 1) + _zero(t, m), pl.ds(32 * (q >> 1) + 16 * (e >> 1) + 8 * r, 8),
                            pl.ds(((2 * (q & 1) + (e & 1)) * ns + sr) * 128, 128)])
                   for e in range(4)] for q in range(4)]
            for n, w in enumerate(_words49(_lhs7, cw, m)):
                dst[7 * m + n, sr, blk(2 * t + r, 8), :] = w
            return [], 0, lambda: dst[7 * m + _zero(t, 0), sr, blk(2 * t + r, 8), :]

        wv = _permute8(_lane_chunks(jnp.concatenate(
            [pltpu.bitcast(wv_r[t & 1, e], U32) for e in range(2)], axis=0)))

        def v_sums(r, cc, gate):
            ops = _words7(_rhs7, [gate(wv[cc + 4 * d][16 * e + 8 * r:16 * e + 8 * r + 8])
                                  for e in range(2) for d in range(2)])
            for m in range(7):
                wv7[m, cc, blk(2 * t + r, 8), :] = ops[m]
            return [], 0, lambda: wv7[_zero(t, 0), cc, blk(2 * t + r, 8), :]

        def o_sums(r, cc, gate):
            ops = _words7(_rhs7, [gate(wob_p[blk(2 * t + r + 32 * e, 8), strip(cc + 4 * d)])
                                  for e in range(2) for d in range(2)])
            for e, m in enumerate(RSUM):
                wob5[e, blk(2 * t + r, 8), strip(cc)] = ops[m]
            return [], 0, lambda: wob5[_zero(t, 0), blk(2 * t + r, 8), strip(cc)]

        sched = _Sched(t > 99, plan1, dict(
            x=[part(act_sums, x_r, xq, 2, m, sr, r)
               for m in range(7) for sr in range(2) for r in range(2)],
            c=[part(act_sums, c_r, cq, 1, m, 0, r) for m in range(7) for r in range(2)],
            v=[part(v_sums, r, cc) for r in range(2) for cc in range(4)],
            o=[part(o_sums, r, cc) for r in range(2) for cc in range(4)]))

        first = t < 2
        for half in range(2):
            for rb in range(4):
                w = jnp.concatenate([wperm[4 * half + cc] for cc in range(4)], axis=1)
                r = sched.mm(4 * half + rb, xs_u[t >> 1, pl.ds(rb * 256, 256), :], w)
                for cc in range(4):
                    sl = (8 * (t & 1) + 4 * half + cc, pl.ds(PAD + rb * 512, 512), slice(None))
                    old = jnp.where(first, 0.0, qk_b[sl])
                    qk_b[sl] = old + r[:, cc * 128:(cc + 1) * 128]
        sched.finish()
        stage_first(t + 1)
        for d in group(t + 2):
            d.start()
        return t

    last = jax.lax.fori_loop(0, 16, p1_body, 0)

    row = jax.lax.broadcasted_iota(jnp.int32, (TQ, TQ), 0)
    col = jax.lax.broadcasted_iota(jnp.int32, (TQ, TQ), 1)
    col = (col & ~31) | ((col & 1) << 4) | ((col & 31) >> 1)
    rowi = jax.lax.broadcasted_iota(jnp.int32, (RB, 128), 0)
    odd = (jax.lax.broadcasted_iota(jnp.int32, (RB, 128), 1) & 1) == 1
    NSUB = HQ // RB
    QSCALE = DA ** -0.5 * LOG2E

    def pair_rows(src, slot, r0, n, gate):
        return [_split(gate(src[slot, pl.ds(r0 + par, n // 2, stride=2), :])) for par in range(2)]

    def staging(g, z):
        ns = DC // SCR

        def scales(n1, k, gate):
            res = []
            for h in range(2):
                if k < ns:
                    w = gate(wkv_r[g & 1, pl.ds(n1 * DC + k * SCR, SCR), :])
                    w = pltpu.bitcast(w, jnp.int32) & (0x7F80 << (16 * h))
                else:
                    w = gate(sc_s[2 * n1 + h, pl.ds(0, 8 * ns), :])
                e = _tree([w[r:r + 8] for r in range(0, w.shape[0], 8)], jnp.maximum)
                if k == ns:
                    e = pltpu.bitcast(e << (16 - 16 * h), F32)
                    e = jnp.max(e, axis=0, keepdims=True)
                    e = jnp.clip(pltpu.bitcast(e, jnp.int32), 1 << 23, 253 << 23)
                    e = jnp.broadcast_to(e, (8, 128))
                    sc_s[2 * n1 + h, pl.ds(8 * ns + 8, 8), :] = (254 << 23) - e
                sc_s[2 * n1 + h, pl.ds(8 * k, 8), :] = e
                res.append(pltpu.bitcast(e, U32))
            return res, 0, lambda: pltpu.bitcast(sc_s[2 * n1, blk(k + _zero(z, 0), 8), :], U32)

        def rhs49(dst, tiles, scale, m, r):
            res = [_ops49(_rhs7,
                          [[scale(tiles[2 * (q >> 1) + (e >> 1)][q & 1][par][e & 1],
                                  2 * (q & 1) + (e & 1)) for e in range(4)] for q in range(4)],
                          m) for par in range(2)]
            for k, (lo, hi) in enumerate(zip(*res)):
                dst[7 * m + k, pl.ds(8 * r, 8), :] = _join(lo, hi)

        def kv(m, r, gate):
            if m == 0 and r == 0:
                for k in range(4):
                    ups[k] = pltpu.bitcast(gate(sc_s[k, pl.ds(8 * ns, 8), :]), F32)
            down = [pltpu.bitcast(sc_s[k + _zero(z, m), pl.ds(8 * ns + 8, 8), :], F32)
                    for k in range(4)]
            tiles = [[pair_rows(wkv_r, (g & 1) + _zero(z, m), n1 * DC + kt * 128 + 16 * r, 16, gate)
                      for n1 in range(2)] for kt in range(4)]
            rhs49(wkv, tiles, lambda w, k: w * down[k], m, r)
            return [], 0, lambda: wkv[7 * m, blk(r + _zero(z, 0), 8), :]

        def qw(m, r, gate):
            tiles = [[pair_rows(wq_r, ((g + 1 + n1) & 3) + _zero(z, m), kt * 256 + 16 * r, 16, gate)
                      for n1 in range(2)] for kt in range(4)]
            rhs49(wq49, tiles, lambda w, k: w, m, r)
            return [], 0, lambda: wq49[7 * m, blk(r + _zero(z, 0), 8), :]

        def b_lhs(u, r, gate):
            base = 8 * jnp.minimum(g + 1, NQ - 1) + r
            ops = _words7(_lhs7, [gate(xs_u[u + 4 * d, blk(base + 4 * e, 8), :])
                                  for e in range(2) for d in range(2)])
            for k, m in enumerate(LSUM):
                bx[k, pl.ds(8 * r, 8), strip(u)] = ops[m]
            return [], 0, lambda: bx[0, blk(r + _zero(z, 0), 8), strip(u)]

        return dict(sc=[part(scales, n1, k) for k in range(ns + 1) for n1 in range(2)],
                    kv=[part(kv, m, r) for m in range(7) for r in range(8)],
                    qw=[part(qw, m, r) for m in range(7) for r in range(16)],
                    bx=[part(b_lhs, u, r) for u in range(4) for r in range(4)])

    sched = _Sched(last > 99, _planx(), staging(-1, last))
    w0 = pair_rows(wq_r, 0, 0, M, lambda x: x)
    w0 = [_join(w0[0][h], w0[1][h]) for h in range(2)]
    for g in range(4):
        for e in range(2):
            for h in range(2):
                q = [sched.mm(8 * g + 4 * e + 2 * h + k, jnp.concatenate(
                    [xs_u[4 * k + u, pl.ds((4 * g + 2 + e) * HQ, HQ), :] for u in range(4)], axis=1),
                    w0[h][256 * k:256 * k + 256], step=16) for k in range(2)]
                qn[h, g, e] = _pack((q[0] + q[1]) * QSCALE)
    sched.finish()
    for d in group(16) + group(17):
        d.wait()
    for d in cp_p(1):
        d.start()
    plan2 = _plan2()

    def p2_body(p, carry):
        for d in cp_p(p):
            d.wait()
        causal = col <= row
        never = p > NP
        jobs = staging(p, p)
        sched = _Sched(never, plan2, jobs)
        mm = sched.mm

        r0 = pl.multiple_of(p * TQ, TQ)

        def scatter(dst, off, c):
            for e, t in enumerate(c):
                for cc in range(4):
                    dst[4 * (e & 1) + cc, pl.ds(off + (PAD + (e >> 1) * HQ), HQ), :] = (
                        t[:, cc * 128:(cc + 1) * 128])

        def proj_bv():
            def lhs(m):
                if m in (2, 3):
                    return jnp.concatenate([xs_u[u + 4 * (m - 2), blk(2 * p + m - 2, QQ), :]
                                            for u in range(4)], axis=1)
                return bx[LSUM.index(m)]

            for cc in range(8):
                vb[cc, pl.ds(0, PAD), :] = vb[cc, pl.ds(TQ, PAD), :]
            c = [_combine(lambda m: mm(("bv", 7 * e + ORDER.index(m)), lhs(m), jnp.concatenate(
                [wv7[m, 2 * e], wv7[m, 2 * e + 1]], axis=1))) for e in range(2)]
            scatter(vb, 0, [jnp.concatenate(t, axis=1) for t in zip(*c)])

        def local_qk(rb, k, gate):
            q = [qk_b[cc, pl.ds(r0 + _zero(p, k) + (PAD + rb * RB), RB), :] for cc in range(8)]
            q[0] = gate(q[0])
            for w in range(LG * k, LG * k + LG):
                t = _fold([q[cc] * qk_b[8 + cc, pl.ds(r0 + (PAD + rb * RB - DIL * w), RB), :]
                           for cc in range(8)], jnp.add)
                t = t + pltpu.roll(t, 64, 1)
                t = t + jnp.where(odd, pltpu.roll(t, 1, 1), pltpu.roll(t, 127, 1))
                t = t * (DB ** -0.5 * LOG2E)
                if rb == 0 and w:
                    t = jnp.where(rowi + r0 >= DIL * w, t, NEG)
                lg_s[w, pl.ds(rb * RB, RB), :] = t
            return [], 1, lambda: pltpu.bitcast(lg_s[w, blk(2 * rb + _zero(p, 0), 8), :], U32)

        def local_sm(rb, e, gate):
            rows = pl.ds(rb * RB + SMR * e, SMR)
            lg = [gate(lg_s[w, rows, :]) for w in range(WIN)]
            m = _tree(lg, jnp.maximum)
            ps = [jnp.exp2(t - m) for t in lg]
            l = _tree(ps, jnp.add)
            r = pl.reciprocal(l, approx=True)
            r = r * (2.0 - l * r)
            for w in range(WIN):
                pr_s[w, rows, :] = ps[w] * r
            return [], 2, lambda: pltpu.bitcast(pr_s[0, blk(2 * rb + e + _zero(p, 0), 8), :], U32)

        def local_pv(rb, k, gate):
            rows = pl.ds(rb * RB, RB)
            ps = [pr_s[w + _zero(p, k), rows, :] for w in range(WIN)]
            ps[0] = gate(ps[0])
            o = [_fold([ps[w] * vb[cc, pl.ds(PAD + rb * RB - DIL * w, RB), :] for w in range(WIN)],
                       jnp.add) for cc in (k, k + 4)]
            if rb < NSUB:
                for e in range(2):
                    o_s[k + 4 * e, rows, :] = o[e]
                return [], 3, lambda: pltpu.bitcast(o_s[k, blk(2 * rb + _zero(p, 0), 8), :], U32)
            top = pl.ds((rb - NSUB) * RB, RB)
            for m, t in enumerate(_lhs7(o_s[k, top, :], o_s[k + 4, top, :], *o)):
                ob7[m, pl.ds((rb - NSUB) * RB // 2, RB // 2), strip(k)] = _pack(t)
            return [], 0, lambda: ob7[0, blk(rb - NSUB + _zero(p, 0), 8), strip(k)]

        order = [rb + e * NSUB for rb in range(NSUB) for e in range(2)]
        jobs["lo"] = []
        for k in range(len(order) + SML):
            for f, d, n in ((local_sm, SML, RB // SMR), (local_qk, 0, 8 // LG)):
                if 0 <= k - d < len(order):
                    jobs["lo"] += [part(f, order[k - d], e) for e in range(n)]
        jobs["lv"] = [part(local_pv, rb, e) for rb in order for e in range(4)]

        def wob(m):
            if m == 1:
                return wob_p[pl.ds(0, M // 4), pl.ds(0, M // 2)]
            if m == 4:
                return wob_p[pl.ds(M // 4, M // 4), pl.ds(M // 2, M // 2)]
            return wob5[RSUM.index(m)]

        bo = {}

        def proj_bo(n):
            for m in ORDER[len(bo):len(bo) + n]:
                bo[m] = mm(("bo", len(bo)), lambda: ob7[m], wob(m))
            if n and len(bo) == 7:
                scatter(qk_b, r0, _combine(lambda m: bo[m]))

        def out_weights(m, r, gate):
            ww = [[gate(wo_r[(p & 1) + _zero(p, m),
                             pl.ds((2 * (q >> 1) + (e >> 1)) * HQ + 8 * r, 8),
                             pl.ds((2 * (q & 1) + (e & 1)) * 128, 128)])
                   for e in range(4)] for q in range(4)]
            rows = blk(8 * (p >> 1) + r, 8)
            extra = jobs["sc"].pop(0)(gate)[0] if jobs["sc"] else []
            for n, w in enumerate(_words49(_rhs7, ww, m)):
                if n < len(extra):
                    w = jnp.where(never, extra[n], w)
                wo49[7 * m + n, p & 1, rows, :] = w
            return [], 0, lambda: wo49[7 * m + _zero(p, 0), p & 1, rows, :]

        jobs["wo"] = [part(out_weights, m, r) for m in range(7) for r in range(8)]

        ks, vs, qs = {}, {}, {}
        done, prods = {}, {}

        def project(kind, j, n, lhs, rhs, scale, pack):
            got = prods.setdefault((kind, j), {})
            for m in ORDER[len(got):len(got) + n]:
                got[m] = _combine(lambda k: mm((kind, j, 7 * len(got) + ORDER.index(k)),
                                               lhs(7 * m + k), rhs[7 * m + k]))
            if len(got) < 7:
                return None
            c = _combine(lambda m: got[m])
            c = [[pack(c[(rg & 2) + (cg >> 1)][2 * (rg & 1) + (cg & 1)] * scale(cg))
                  for rg in range(4)] for cg in range(4)]
            return [[jnp.concatenate([t[16 * e:16 * e + 16] for t in c[cg]], axis=0)
                     for e in range(2)] for cg in range(4)]

        def proj_kv(j, n):
            c = project("kv", j, n, lambda k: cq[k, 0, pl.ds(j * QQ, QQ), :], wkv,
                        lambda cg: ups[cg][:1], _riffle)
            if c is not None:
                for cg in range(4):
                    for e in range(2):
                        (vs, ks)[cg >> 1][(cg & 1, 2 * j + e)] = c[cg][e]

        def proj_q(g, n):
            rows = blk(2 * g + (p & 1), QQ)
            c = project("q", g, n,
                        lambda k: jnp.concatenate([xq[k, sr, rows, :] for sr in range(2)], axis=1),
                        wq49, lambda cg: QSCALE, _pack)
            if c is not None:
                for h in range(2):
                    for e in range(2):
                        old = qn[h, g, e]
                        for b in range(2):
                            qs[(h, 4 * g + 2 * b + e)] = jnp.where((p & 1) == b, c[h][e], old)
                        qn[h, g, e] = c[2 + h][e]

        def qk(h, i, dep):
            kk = jnp.concatenate([ks[(h, j)] for j in range(i + 1)], axis=0)
            q = qs[(h, i)]
            if dep is not None:
                q = jnp.where(never, done[(h, dep)], q)
            ch = _lane_chunks(mm(("qk", h, i), q, kk, NT, 512))
            ch[i] = jnp.where(causal, ch[i], NEG)
            return ch

        def softmax_pv(h, i, ch):
            m = jnp.max(_fold(ch, jnp.maximum), axis=1, keepdims=True)
            ps = [jnp.exp2(c - m) for c in ch]
            lp = ps[0]
            for j in range(1, i + 1):
                lp = lp + ps[j]
                if TIE and (j % TIE == TIE - 1 or j == i):
                    ps[j] = jnp.where(never, lp, ps[j])
            pb = jnp.concatenate(ps, axis=1).astype(BF16)
            vv = jnp.concatenate([vs[(h, j)] for j in range(i + 1)], axis=0)
            o = mm(("pv", h, i), pb, vv)
            if i >= LDEP:
                lp = jnp.where(never, o, lp)
            l = jnp.sum(lp, axis=1, keepdims=True)
            r = pl.reciprocal(l, approx=True)
            r = r * (2.0 - l * r)
            cn = _pack(o * r)
            done[(h, i)] = cn
            if FA <= i < NQ - 1:
                if h == 0 and F0 < 0:
                    site = ("qk", 1, i + 1)
                elif i + 3 < NQ:
                    site = ("kv", (i + 1) // 2 + 1, KVS * ((i + 1) & 1) + (F0, FD)[h])
                else:
                    site = ("bo", (i + 3 - NQ) * BOP[0] + h)
                sched.pending.setdefault(site, []).append(cn)
            ctx[2 * p + h, pl.ds(i * HQ, HQ), :] = cn

        proj_bv()
        proj_kv(0, 7)
        proj_q(0, 7)
        for i in range(NQ):
            dep = i - DEP if DEP <= i < FA + DEP else None
            s0 = qk(0, i, dep)
            s1 = qk(1, i, dep)
            if i + 2 < NQ:
                proj_kv(i // 2 + 1, 7 if i & 1 else KVS // 7)
                if i < 6:
                    proj_q(i // 2 + 1, 7 if i & 1 else QS // 7)
            else:
                proj_bo(BOP[i + 2 - NQ])
            softmax_pv(0, i, s0)
            softmax_pv(1, i, s1)
        proj_bo(BOP[2])
        sched.finish()
        for d in cp_p(p + 2):
            d.start()
        return carry

    jax.lax.fori_loop(0, NP, p2_body, 0)

    cp_gw().wait()
    gw = gw_ref[...].astype(F32)
    plan3 = _plan3()
    cab = (ca0, ca1)

    def p3_body(i, carry):
        r0 = pl.multiple_of(i * TO, TO)
        h0 = pl.multiple_of(i * (TO // 2), TO // 2)
        never = i > S

        def ctx_words(m, u, r, n):
            return [[ctx[4 * u + 2 * (q & 1) + (e & 1),
                         pl.ds(h0 + _zero(i, m) * 8 + ((2 * (q >> 1) + (e >> 1)) * QQ + r), n), :]
                     for e in range(4)] for q in range(4)]

        def operands(k, u, r, gate):
            m = ORDER[k]
            cw = [[gate(w) for w in q] for q in ctx_words(m, u, r, 8)]
            for n, w in enumerate(_words49(_lhs7, cw, m)):
                if not (m in (2, 3) and n in (2, 3)):
                    cab[k & 1][n, pl.ds(r, 8), pl.ds(u * 128, 128)] = w
            return [], 0, lambda: cab[k & 1][_zero(i, 0), pl.ds(r, 8), pl.ds(u * 128, 128)]

        def gate_rows(r, gate):
            gs = _fold([_bf(gate(xs_u[j, pl.ds(h0 + r, 8), :])).astype(F32) * gw[j:j + 1]
                        for j in range(8)], jnp.add)
            g = jax.nn.sigmoid(jnp.sum(gs, axis=1, keepdims=True))
            g_s[pl.ds(2 * r, 16), :] = jnp.broadcast_to(g, (16, 128))
            return [], 0, lambda: pltpu.bitcast(g_s[blk(r // 4 + _zero(i, 0), 8), :], U32)

        sched = _Sched(never, plan3, dict(
            a=[part(operands, k, u, r) for k in range(1, 7) for u in range(HA // 4)
               for r in range(0, QQ, 8)],
            g=[part(gate_rows, r) for r in range(0, TO // 2, 8)]))
        first = [[_words49(_lhs7, ctx_words(ORDER[0], u, 0, QQ), ORDER[0])[n]
                  for u in range(HA // 4)] for n in range(7)]

        def inner(m, n):
            k = ORDER.index(m)
            res = []
            for e in range(2):
                us = range(4 * e, 4 * e + 4)
                if m in (2, 3) and n in (2, 3):
                    lhs = jnp.concatenate([ctx_words(m, u, 0, QQ)[3 * (m - 2)][3 * (n - 2)]
                                           for u in us], axis=1)
                elif k == 0:
                    lhs = jnp.concatenate([first[n][u] for u in us], axis=1)
                else:
                    lhs = lambda: cab[k & 1][n, :, pl.ds(e * 512, 512)]
                rhs = jnp.concatenate([wo49[7 * m + n, cc, pl.ds(e * 256, 256), :]
                                       for cc in range(2)], axis=1)
                res.append(sched.mm((k, 2 * ORDER.index(n) + e), lhs, rhs))
            return res[0] + res[1]

        acs = _combine(lambda m: _combine(lambda n: inner(m, n)))
        sched.finish()
        for q in range(4):
            for e in range(4):
                off = (2 * (q >> 1) + (e >> 1)) * HQ
                g = g_s[pl.ds(off, HQ), :]
                for cc in range(2):
                    ch = 4 * cc + 2 * (q & 1) + (e & 1)
                    a = acs[q][e][:, cc * 128:(cc + 1) * 128]
                    b = qk_b[ch, pl.ds(r0 + (PAD + off), HQ), :]
                    out_s[pl.ds(r0 + off, HQ), pl.ds(ch * 128, 128)] = (
                        g * a + (1.0 - g) * b).astype(BF16)
        cp_out(i).start()
        return carry

    jax.lax.fori_loop(0, S // TO, p3_body, 0)
    for g in range(NP, NP + 2):
        for d in cp_p(g):
            d.wait()
    for i in range(S // TO):
        cp_out(i).wait()


@jax.jit
def pallas_gated_mix__compressed_kv_cla__sliding_local_dilated__prompt_kernel(
    A_x: jax.Array,
    A_c_kv: jax.Array,
    A_w_q: jax.Array,
    A_w_uk: jax.Array,
    A_w_uv: jax.Array,
    A_w_o: jax.Array,
    B_x: jax.Array,
    B_wqkv: jax.Array,
    B_wo: jax.Array,
    gate_w: jax.Array,
):
    del B_x
    any_spec = pl.BlockSpec(memory_space=pl.ANY)
    out = pl.pallas_call(
        _kernel,
        in_specs=[any_spec] * 9,
        out_specs=any_spec,
        out_shape=jax.ShapeDtypeStruct((S, M), BF16),
        scratch_shapes=[
            pltpu.VMEM((9, S // 2, 128), U32),
            pltpu.VMEM((2, HQ, M), U32),
            pltpu.VMEM((2, HQ, DC), U32),
            pltpu.VMEM((2, 128, M), BF16),
            pltpu.VMEM((2, 2, 32, M), BF16),
            pltpu.VMEM((M // 2, M), U32),
            pltpu.VMEM((3, 2 * DC, 128), U32),
            pltpu.VMEM((4, M, 128), U32),
            pltpu.VMEM((2, 2 * DA, M // 2), U32),
            pltpu.VMEM((8, 64, 128), U32),
            pltpu.VMEM((49, 2, S // 8, 128), U32),
            pltpu.VMEM((49, 1, S // 8, 128), U32),
            pltpu.VMEM((7, 4, M // 4, 128), U32),
            pltpu.VMEM((5, M // 4, M // 2), U32),
            pltpu.VMEM((49, 2, NP * QQ, 128), U32),
            pltpu.VMEM((49, HQ, 128), U32),
            pltpu.VMEM((49, TQ, 128), U32),
            pltpu.VMEM((4, 8, 128), F32),
            pltpu.VMEM((4, DC // SCR * 8 + 16, 128), jnp.int32),
            pltpu.VMEM((5, QQ, M // 2), U32),
            pltpu.VMEM((2, 4, 2, HQ, 128), U32),
            pltpu.VMEM((16, S + PAD, 128), F32),
            pltpu.VMEM((8, TQ + PAD, 128), F32),
            pltpu.VMEM((WIN, TQ, 128), F32),
            pltpu.VMEM((WIN, TQ, 128), F32),
            pltpu.VMEM((8, HQ, 128), F32),
            pltpu.VMEM((7, QQ, M // 2), U32),
            pltpu.VMEM((HA, S // 2, 128), U32),
            pltpu.VMEM((7, QQ, M), U32),
            pltpu.VMEM((7, QQ, M), U32),
            pltpu.VMEM((TO, 128), F32),
            pltpu.VMEM((S, M), BF16),
            pltpu.VMEM((8, 128), BF16),
            pltpu.SemaphoreType.DMA((2,)),
            pltpu.SemaphoreType.DMA((2,)),
            pltpu.SemaphoreType.DMA((3,)),
        ],
        compiler_params=pltpu.CompilerParams(vmem_limit_bytes=120 * 1024 * 1024,
                                             disable_bounds_checks=True),
    )(
        A_x.reshape(S, M),
        A_c_kv.reshape(S, DC),
        A_w_q,
        A_w_uk,
        A_w_uv,
        A_w_o.reshape(HA * DA, M),
        B_wqkv.reshape(2, M // 2, 3 * M),
        B_wo.reshape(HB // 2, 2, DB, M),
        gate_w.reshape(8, 128),
    )
    return out.reshape(1, S, M)
```

```python
import functools
import math

import jax
import jax.numpy as jnp
import jax.experimental.pallas as pl
import jax.experimental.pallas.tpu as pltpu

F32 = jnp.float32
BF16 = jnp.bfloat16
U32 = jnp.uint32

S = 2048
M = 1024
HA = 32
DA = 128
DC = 512
HB = 32
DB = 32
WIN = 8
DIL = 2
PAD = 16
LOG2E = math.log2(math.e)
NEG = -1e9

TQ = 128
HQ = TQ // 2
QQ = TQ // 4
BOP = (2, 3, 2)
LX = 16
KVS = 28
QS = 28
QST = 2
LQ0 = 3
LG = 2
XN = 29
SK = 3
SMR = 16
P1N = 96
P1K = 6
P1W = 0
P1S = tuple((h, r, 512) for h in range(2) for r in range(0, S, 512))
P1U = 7
P3S = 4
P3M = 6
P3E = 12
NQ = S // TQ
NP = HA // 2
DEP = 2
SCR = 32
LN = 58
SML = 1
LE = 2
LI = 0
LA = 21
LB = 4
LS = 4
LP = ("q", 0, 4)
FA = 6
F0 = 0
FD = 8
TIE = 4
RB = 16
LDEP = 4
TO = 256
NN = (((1,), (0,)), ((), ()))
NT = (((1,), (1,)), ((), ()))


def _plan2():
    plan = {}

    def put(name, count, start, until):
        plan.setdefault(start, []).extend([(name, until)] * count)

    def after_qk(i):
        if i >= NQ - 2:
            return ("bo", (i - NQ + 2) * BOP[0] + 1)
        return ("kv", i // 2 + 1, KVS * (i & 1) + LX)

    def fill(name, count, sites):
        for start, room, until in sites:
            n = min(count, room - len(plan.get(start, ())))
            put(name, n, start, until)
            count -= n
        assert count == 0, (name, count)

    def qk_sites(lo, hi):
        return [(("qk", h, i), max(i + 1 - h * SK, 0), after_qk(i))
                for i in range(lo, hi) for h in range(2)]

    def q_sites(g, lo, hi, until):
        return [(("q", g, k), 1, until) for k in range(lo, hi, QST)]

    names = _spread(["lo"] * (64 // LG + 128 // SMR), LN)
    for k, name in enumerate(names):
        put(name, 1, ("bv", k // 4) if k < 56 else ("kv", 0, 2 * (k - 56) + 1), LP)
    first = [(("kv", 0, k), 1, ("kv", 1, 8)) for k in range(LA, 49, LS)]
    first += [(("q", 0, k), 1, ("kv", 1, 8)) for k in range(LI, 49 - LB, LE)]
    early = []
    for g in range(1, 4):
        early += q_sites(g, 0, QS - 4, after_qk(2 * g - 1))
        early += qk_sites(max(2 * g - 1, LQ0), 2 * g)
        early += q_sites(g, QS, 45, after_qk(2 * g))
        early += qk_sites(max(2 * g, LQ0), 2 * g + 1)
    fill("lv", 32, first + early)
    fill("wo", 56, early)
    fill("bx", 16, early + qk_sites(7, 14))
    fill("qw", 112, qk_sites(7, 14))
    fill("kv", 56, qk_sites(14, 16) + [(("bo", k), 8, ("bo", 6)) for k in range(BOP[0], 5)])
    return plan


def _planx():
    names = _spread(["qw"] * 112 + ["kv"] * 56 + ["bx"] * 16, 8 * XN)
    return {k: [(n, 31) for n in names[8 * k:8 * k + 8]] for k in range(XN)}


def _spread(names, ticks):
    out = [None] * ticks
    for k, name in enumerate(names):
        out[k * ticks // len(names)] = name
    return out


def _plan1():
    ticks = [(k, min(k + P1U, len(P1S) - 1)) for k, (_, _, n) in enumerate(P1S[:-1])
             for _ in range(n // 32 - (P1K if k + 1 == min(k + P1U, len(P1S) - 1) else 0))][:P1N]
    names = _spread(["x"] * 28 + ["c"] * 14 + ["o"] * 8 + ["v"] * 8, len(ticks))
    plan = {}
    for name, (k, until) in zip(names, ticks):
        plan.setdefault(k, []).append((name, until))
    return plan


def _plan3():
    plan = {}
    for k in range(6):
        lo = P3S if k == 0 else 0
        extra = ["g"] * 8 if k in (1, 2) else []
        names = _spread(["a"] * 32 + extra, 4 * (P3E - lo))
        for d in range(lo, P3E):
            plan[(k, d)] = [(n, (k + 1, 0)) for n in names[4 * (d - lo):4 * (d - lo) + 4]]
    names = _spread(["m"] * 24, 4 * P3M)
    for d in range(P3M):
        plan[(6, d)] = [(n, (6, 13)) for n in names[4 * d:4 * d + 4]]
    return plan


_STAGES = ((2, 4), (1, 3), (0, 2), (0, 6), (0, 1))


def _permute8(cols):
    cols = list(cols)
    lane = jax.lax.broadcasted_iota(jnp.int32, cols[0].shape, 1)
    for va, lb in _STAGES:
        lo = (lane & (1 << lb)) == 0
        sh = 1 << lb
        idx = [i for i in range(8) if not (i >> va) & 1]
        if lb == 6:
            rr = [pltpu.roll(jnp.where(lo, cols[i | (1 << va)], cols[i]), 64, 1) for i in idx]
            for i, r in zip(idx, rr):
                a, b = cols[i], cols[i | (1 << va)]
                cols[i] = jnp.where(lo, a, r)
                cols[i | (1 << va)] = jnp.where(lo, r, b)
        else:
            rb = [pltpu.roll(cols[i | (1 << va)], sh, 1) for i in idx]
            ra = [pltpu.roll(cols[i], 128 - sh, 1) for i in idx]
            for i, xa, xb in zip(idx, ra, rb):
                a, b = cols[i], cols[i | (1 << va)]
                cols[i] = jnp.where(lo, a, xb)
                cols[i | (1 << va)] = jnp.where(lo, xa, b)
    return cols


def _pack(x):
    return pltpu.bitcast(x.astype(BF16), U32)


def _bf(x):
    return pltpu.bitcast(x, BF16)


def _split(w):
    return (pltpu.bitcast(w << 16, F32), pltpu.bitcast(w & jnp.uint32(0xFFFF0000), F32))


def _join(lo, hi):
    return pltpu.bitcast(pltpu.pack_elementwise([lo, hi], packed_dtype=BF16), U32)


def _riffle(x):
    return jnp.concatenate([_join(x[r:r + 16], x[r + 16:r + 32]) for r in range(0, x.shape[0], 32)],
                           axis=0)


def _lhs7(a11, a12, a21, a22):
    return [a11 + a22, a21 + a22, a11, a22, a11 + a12, a21 - a11, a12 - a22]


def _rhs7(b11, b12, b21, b22):
    return [b11 + b22, b11, b12 - b22, b21 - b11, b22, b11 + b12, b21 + b22]


LSUM = (0, 1, 4, 5, 6)
RSUM = (0, 2, 3, 5, 6)


def _words7(fn, quads):
    halves = [_split(w) for w in quads]
    lo = fn(*[h[0] for h in halves])
    hi = fn(*[h[1] for h in halves])
    return [_join(a, b) for a, b in zip(lo, hi)]


def _combine(mm):
    add = functools.partial(jax.tree.map, jnp.add)
    sub = functools.partial(jax.tree.map, jnp.subtract)
    m2 = mm(2)
    m3 = mm(3)
    m4 = mm(4)
    c12 = add(m2, m4)
    t11 = sub(m3, m4)
    m1 = mm(1)
    c21 = add(m1, m3)
    t22 = sub(m2, m1)
    m0 = mm(0)
    t11 = add(t11, m0)
    t22 = add(t22, m0)
    c11 = add(t11, mm(6))
    return c11, c12, c21, add(t22, mm(5))


ORDER = (2, 3, 4, 1, 0, 6, 5)


def _zero(i, m):
    return i >> (8 + m)


def _merge(vals):
    return _fold([v[r:r + 8, c:c + 128] for v in vals for r in range(0, v.shape[0], 8)
                  for c in range(0, v.shape[1], 128)], jnp.bitwise_or)


def _gate(never, g):
    def gate(x):
        t = jnp.tile(pltpu.bitcast(g, x.dtype), (x.shape[0] // 8, x.shape[1] // 128))
        return jnp.where(never, t, x)
    return gate


def _tie(never, x, deps):
    if not deps:
        return x
    top = jnp.where(never, _merge(deps), x[:8, :128])
    if x.shape[1] > 128:
        top = jnp.concatenate([top, x[:8, 128:]], axis=1)
    return jnp.concatenate([top, x[8:]], axis=0)


class _Sched:
    def __init__(self, never, plan, jobs):
        self.never, self.plan, self.jobs, self.pending = never, plan, jobs, {}

    def mm(self, site, a, b, dims=NN, width=128, step=32):
        deps = [d() if callable(d) else d for d in self.pending.pop(site, ())]
        a = a() if callable(a) else a
        tie = functools.partial(_tie, self.never, deps=deps)
        a, b = (_bf(tie(a)), _bf(b)) if a.dtype == U32 else (a, _bf(tie(b)))
        out = jax.lax.dot_general(a, b, dims, preferred_element_type=F32)
        per = out.shape[0] // step
        last = {}
        for k, (name, until) in enumerate(self.plan.get(site, ())):
            if name is not None:
                r, c = step * (k % per), width * (k // per)
                vals, tag, stored = self.jobs[name].pop(0)(
                    _gate(self.never, out[r:r + 8, c:c + 128]))
                self.pending.setdefault(until, []).extend(vals)
                last[(name, tag, until)] = stored
        for (_, _, until), stored in last.items():
            if stored is not None:
                self.pending[until].append(stored)
        return out

    def finish(self):
        assert not any(self.jobs.values()) and not any(self.pending.values())


def _ops49(fn, blocks, m):
    return fn(*[fn(*[blocks[q][e] for q in range(4)])[m] for e in range(4)])


def _words49(fn, words, m):
    halves = [[_split(w) for w in q] for q in words]
    lo = _ops49(fn, [[h[0] for h in q] for q in halves], m)
    hi = _ops49(fn, [[h[1] for h in q] for q in halves], m)
    return [_join(a, b) for a, b in zip(lo, hi)]


def _fold(xs, op):
    acc = xs[0]
    for x in xs[1:]:
        acc = op(acc, x)
    return acc


def _tree(xs, op):
    while len(xs) > 1:
        xs = [op(a, b) for a, b in zip(xs[::2], xs[1::2])]
    return xs[0]


def _lane_chunks(x):
    return [x[:, j * 128:(j + 1) * 128] for j in range(x.shape[1] // 128)]


def _kernel(x_hbm, c_hbm, wq_hbm, wuk_hbm, wuv_hbm, wo_hbm, wqkv_hbm, wob_hbm, gw_hbm,
            out_hbm,
            xs_u, x_r, c_r, w_r, wv_r, wob_p, wkv_r, wq_r, wo_r,
            wperm, xq, cq, wv7, wob5, wo49, wkv, wq49, ups, sc_s, bx, qn,
            qk_b, vb, lg_s, pr_s, o_s, ob7, ctx, ca0, ca1, g_s, out_s, gw_ref,
            sem_x, sem_p, sem_a):
    x_u = x_hbm.bitcast(U32)
    c_u = c_hbm.bitcast(U32)
    wo_u = wo_hbm.bitcast(U32)
    wq_u = wq_hbm.bitcast(U32)
    wuk_u = wuk_hbm.bitcast(U32)
    wuv_u = wuv_hbm.bitcast(U32)
    wob_u = wob_hbm.bitcast(U32)
    part = functools.partial

    def blk(j, n):
        return pl.ds(pl.multiple_of(j * n, n), n)

    def strip(j):
        return blk(j, 128)

    def cp_x(t, sem):
        k = (t + 1) >> 1
        return pltpu.make_async_copy(x_u.at[blk(t & 1, S // 4), strip(jnp.minimum(k, 7))],
                                     xs_u.at[jnp.minimum(k, 8), blk(t & 1, S // 4), :], sem)

    def cp_w(t, sem):
        u = t - 2 * (t >> 4)
        u = u - 2 * (u >> 4)
        return pltpu.make_async_copy(wqkv_hbm.at[u >> 3, strip((u >> 1) & 3), blk(u & 1, M)],
                                     w_r.at[u & 1], sem)

    def group(t):
        sem = sem_x.at[t & 1]
        late = t >> 4
        u = t - 2 * late
        dp = ((u >> 3) << 2) + (u & 2) + ((u >> 2) & 1)
        pq = (t >> 3) + late
        return (
            pltpu.make_async_copy(x_u.at[blk(u, HQ), :], x_r.at[u & 1], sem),
            pltpu.make_async_copy(c_u.at[blk(u, HQ), :], c_r.at[u & 1], sem),
            pltpu.make_async_copy(wob_u.at[:, u & 1, dp, :], wob_p.at[blk(u, 16), :], sem),
            pltpu.make_async_copy(wob_u.at[:, u & 1, dp + 8, :], wob_p.at[blk(u + 16, 16), :], sem),
            cp_x(t, sem),
            cp_w(t + 1, sem),
            pltpu.make_async_copy(wqkv_hbm.at[0, blk(u, 32), pl.ds(2 * M, M)],
                                  wv_r.at[u & 1, 0], sem),
            pltpu.make_async_copy(wqkv_hbm.at[1, blk(u, 32), pl.ds(2 * M, M)],
                                  wv_r.at[u & 1, 1], sem),
            pltpu.make_async_copy(wq_u.at[strip(t & 7), pq, :], wq_r.at[pq, strip(t & 7), :], sem),
            pltpu.make_async_copy(wuk_u.at[blk(u, 32), 0, :],
                                  wkv_r.at[1 + late, blk(16 + u, 32), :], sem),
            pltpu.make_async_copy(wuv_u.at[blk(u, 32), 0, :],
                                  wkv_r.at[1 + late, blk(u, 32), :], sem),
        )

    def cp_wq(p, sem):
        return pltpu.make_async_copy(wq_u.at[:, jnp.minimum(p, NP - 1), :], wq_r.at[p & 3], sem)

    def cp_p(g):
        slot = g & 1
        p = jnp.minimum(g + 1, NP - 1)
        o = jnp.minimum(g, NP - 1)
        sem = sem_p.at[slot]
        return (
            pltpu.make_async_copy(wo_u.at[blk(o >> 1, 2 * DA), blk(o & 1, M // 2)],
                                  wo_r.at[slot], sem),
            pltpu.make_async_copy(wuk_u.at[:, p, :], wkv_r.at[slot, pl.ds(DC, DC), :], sem),
            pltpu.make_async_copy(wuv_u.at[:, p, :], wkv_r.at[slot, pl.ds(0, DC), :], sem),
            cp_wq(g + 2, sem),
        )

    def cp_gw():
        return pltpu.make_async_copy(gw_hbm, gw_ref, sem_a.at[0])

    def cp_out(i):
        return pltpu.make_async_copy(out_s.at[blk(i, TO), :], out_hbm.at[blk(i, TO), :],
                                     sem_a.at[1])

    cp_w(0, sem_a.at[1]).start()
    cp_x(-1, sem_a.at[2]).start()
    for d in group(0)[4:] + group(0)[:4]:
        d.start()

    for cc in range(8):
        qk_b[8 + cc, pl.ds(0, PAD), :] = jnp.zeros((PAD, 128), F32)
        vb[cc, pl.ds(TQ, PAD), :] = jnp.zeros((PAD, 128), F32)

    def stage_first(t):
        for cc, w in enumerate(_permute8(_lane_chunks(pltpu.bitcast(w_r[t & 1], U32)))):
            wperm[cc] = w

    cp_w(0, sem_a.at[1]).wait()
    stage_first(0)
    for d in group(1) + cp_p(0):
        d.start()
    cp_gw().start()
    cp_x(-1, sem_a.at[2]).wait()
    plan1 = _plan1()

    def p1_body(t, carry):
        for d in group(t):
            d.wait()

        def act_sums(src, dst, ns, m, sr, r, gate):
            cw = [[gate(src[(t & 1) + _zero(t, m), pl.ds(32 * (q >> 1) + 16 * (e >> 1) + 8 * r, 8),
                            pl.ds(((2 * (q & 1) + (e & 1)) * ns + sr) * 128, 128)])
                   for e in range(4)] for q in range(4)]
            for n, w in enumerate(_words49(_lhs7, cw, m)):
                dst[7 * m + n, sr, blk(2 * t + r, 8), :] = w
            return [], 0, lambda: dst[7 * m + _zero(t, 0), sr, blk(2 * t + r, 8), :]

        wv = _permute8(_lane_chunks(jnp.concatenate(
            [pltpu.bitcast(wv_r[t & 1, e], U32) for e in range(2)], axis=0)))

        def v_sums(r, cc, gate):
            ops = _words7(_rhs7, [gate(wv[cc + 4 * d][16 * e + 8 * r:16 * e + 8 * r + 8])
                                  for e in range(2) for d in range(2)])
            for m in range(7):
                wv7[m, cc, blk(2 * t + r, 8), :] = ops[m]
            return [], 0, lambda: wv7[_zero(t, 0), cc, blk(2 * t + r, 8), :]

        def o_sums(r, cc, gate):
            ops = _words7(_rhs7, [gate(wob_p[blk(2 * t + r + 32 * e, 8), strip(cc + 4 * d)])
                                  for e in range(2) for d in range(2)])
            for e, m in enumerate(RSUM):
                wob5[e, blk(2 * t + r, 8), strip(cc)] = ops[m]
            return [], 0, lambda: wob5[_zero(t, 0), blk(2 * t + r, 8), strip(cc)]

        sched = _Sched(t > 99, plan1, dict(
            x=[part(act_sums, x_r, xq, 2, m, sr, r)
               for m in range(7) for sr in range(2) for r in range(2)],
            c=[part(act_sums, c_r, cq, 1, m, 0, r) for m in range(7) for r in range(2)],
            v=[part(v_sums, r, cc) for r in range(2) for cc in range(4)],
            o=[part(o_sums, r, cc) for r in range(2) for cc in range(4)]))

        first = t < 2
        for k, (half, r0, n) in enumerate(P1S):
            w = jnp.concatenate([wperm[4 * half + cc] for cc in range(4)], axis=1)
            r = sched.mm(k, xs_u[t >> 1, pl.ds(r0 // 2, n // 2), :], w)
            for cc in range(4):
                sl = (8 * (t & 1) + 4 * half + cc, pl.ds(PAD + r0, n), slice(None))
                new = r[:, cc * 128:(cc + 1) * 128]
                if P1W:
                    qk_b[sl] = jnp.where(first, new, qk_b[sl] + new)
                else:
                    qk_b[sl] = jnp.where(first, 0.0, qk_b[sl]) + new
        sched.finish()
        stage_first(t + 1)
        for d in group(t + 2):
            d.start()
        return t

    last = jax.lax.fori_loop(0, 16, p1_body, 0)

    row = jax.lax.broadcasted_iota(jnp.int32, (TQ, TQ), 0)
    col = jax.lax.broadcasted_iota(jnp.int32, (TQ, TQ), 1)
    col = (col & ~31) | ((col & 1) << 4) | ((col & 31) >> 1)
    rowi = jax.lax.broadcasted_iota(jnp.int32, (RB, 128), 0)
    odd = (jax.lax.broadcasted_iota(jnp.int32, (RB, 128), 1) & 1) == 1
    NSUB = HQ // RB
    QSCALE = DA ** -0.5 * LOG2E

    def pair_rows(src, slot, r0, n, gate):
        return [_split(gate(src[slot, pl.ds(r0 + par, n // 2, stride=2), :])) for par in range(2)]

    def staging(g, z, never):
        ns = DC // SCR

        def scales(n1, k, gate):
            res = []
            for h in range(2):
                if k < ns:
                    w = gate(wkv_r[g & 1, pl.ds(n1 * DC + k * SCR, SCR), :])
                    w = pltpu.bitcast(w, jnp.int32) & (0x7F80 << (16 * h))
                else:
                    w = gate(sc_s[2 * n1 + h, pl.ds(0, 8 * ns), :])
                e = _tree([w[r:r + 8] for r in range(0, w.shape[0], 8)], jnp.maximum)
                if k == ns:
                    e = pltpu.bitcast(e << (16 - 16 * h), F32)
                    e = jnp.max(e, axis=0, keepdims=True)
                    e = jnp.clip(pltpu.bitcast(e, jnp.int32), 1 << 23, 253 << 23)
                    e = jnp.broadcast_to(e, (8, 128))
                    sc_s[2 * n1 + h, pl.ds(8 * ns + 8, 8), :] = (254 << 23) - e
                sc_s[2 * n1 + h, pl.ds(8 * k, 8), :] = e
                res.append(pltpu.bitcast(e, U32))
            return res, 0, lambda: pltpu.bitcast(sc_s[2 * n1, blk(k + _zero(z, 0), 8), :], U32)

        def rhs49(dst, tiles, scale, m, r, extra=()):
            res = [_ops49(_rhs7,
                          [[scale(tiles[2 * (q >> 1) + (e >> 1)][q & 1][par][e & 1],
                                  2 * (q & 1) + (e & 1)) for e in range(4)] for q in range(4)],
                          m) for par in range(2)]
            for k, (lo, hi) in enumerate(zip(*res)):
                w = _join(lo, hi)
                if k < len(extra):
                    w = jnp.where(never, extra[k], w)
                dst[7 * m + k, pl.ds(8 * r, 8), :] = w

        def kv(m, r, gate):
            if m == 0 and r == 0:
                for k in range(4):
                    ups[k] = pltpu.bitcast(gate(sc_s[k, pl.ds(8 * ns, 8), :]), F32)
            down = [pltpu.bitcast(sc_s[k + _zero(z, m), pl.ds(8 * ns + 8, 8), :], F32)
                    for k in range(4)]
            tiles = [[pair_rows(wkv_r, (g & 1) + _zero(z, m), n1 * DC + kt * 128 + 16 * r, 16, gate)
                      for n1 in range(2)] for kt in range(4)]
            rhs49(wkv, tiles, lambda w, k: w * down[k], m, r)
            return [], 0, lambda: wkv[7 * m, blk(r + _zero(z, 0), 8), :]

        def qw(m, r, gate):
            tiles = [[pair_rows(wq_r, ((g + 1 + n1) & 3) + _zero(z, m), kt * 256 + 16 * r, 16, gate)
                      for n1 in range(2)] for kt in range(4)]
            rhs49(wq49, tiles, lambda w, k: w, m, r, sc.pop(0)(gate)[0] if sc else ())
            return [], 0, lambda: wq49[7 * m, blk(r + _zero(z, 0), 8), :]

        def b_lhs(u, r, gate):
            base = 8 * jnp.minimum(g + 1, NQ - 1) + r
            ops = _words7(_lhs7, [gate(xs_u[u + 4 * d, blk(base + 4 * e, 8), :])
                                  for e in range(2) for d in range(2)])
            for k, m in enumerate(LSUM):
                bx[k, pl.ds(8 * r, 8), strip(u)] = ops[m]
            return [], 0, lambda: bx[0, blk(r + _zero(z, 0), 8), strip(u)]

        sc = [part(scales, n1, k) for k in range(ns + 1) for n1 in range(2)]
        return dict(sc=sc,
                    kv=[part(kv, m, r) for m in range(7) for r in range(8)],
                    qw=[part(qw, m, r) for m in range(7) for r in range(16)],
                    bx=[part(b_lhs, u, r) for u in range(4) for r in range(4)])

    sched = _Sched(last > 99, _planx(), staging(-1, last, last > 99))
    w0 = pair_rows(wq_r, 0, 0, M, lambda x: x)
    w0 = [_join(w0[0][h], w0[1][h]) for h in range(2)]
    for g in range(4):
        for e in range(2):
            for h in range(2):
                q = [sched.mm(8 * g + 4 * e + 2 * h + k, jnp.concatenate(
                    [xs_u[4 * k + u, pl.ds((4 * g + 2 + e) * HQ, HQ), :] for u in range(4)], axis=1),
                    w0[h][256 * k:256 * k + 256], step=16) for k in range(2)]
                qn[h, g, e] = _pack((q[0] + q[1]) * QSCALE)
    sched.finish()
    for d in group(16) + group(17):
        d.wait()
    for d in cp_p(1):
        d.start()
    plan2 = _plan2()

    def p2_body(p, carry):
        for d in cp_p(p):
            d.wait()
        causal = col <= row
        never = p > NP
        jobs = staging(p, p, never)
        sched = _Sched(never, plan2, jobs)
        mm = sched.mm

        r0 = pl.multiple_of(p * TQ, TQ)

        def scatter(dst, off, c):
            for e, t in enumerate(c):
                for cc in range(4):
                    dst[4 * (e & 1) + cc, pl.ds(off + (PAD + (e >> 1) * HQ), HQ), :] = (
                        t[:, cc * 128:(cc + 1) * 128])

        def proj_bv():
            def lhs(m):
                if m in (2, 3):
                    return jnp.concatenate([xs_u[u + 4 * (m - 2), blk(2 * p + m - 2, QQ), :]
                                            for u in range(4)], axis=1)
                return bx[LSUM.index(m)]

            for cc in range(8):
                vb[cc, pl.ds(0, PAD), :] = vb[cc, pl.ds(TQ, PAD), :]
            c = [_combine(lambda m: mm(("bv", 7 * e + ORDER.index(m)), lhs(m), jnp.concatenate(
                [wv7[m, 2 * e], wv7[m, 2 * e + 1]], axis=1))) for e in range(2)]
            scatter(vb, 0, [jnp.concatenate(t, axis=1) for t in zip(*c)])

        def local_qk(rb, k, gate):
            q = [qk_b[cc, pl.ds(r0 + _zero(p, k) + (PAD + rb * RB), RB), :] for cc in range(8)]
            q[0] = gate(q[0])
            for w in range(LG * k, LG * k + LG):
                t = _fold([q[cc] * qk_b[8 + cc, pl.ds(r0 + (PAD + rb * RB - DIL * w), RB), :]
                           for cc in range(8)], jnp.add)
                t = t + pltpu.roll(t, 64, 1)
                t = t + jnp.where(odd, pltpu.roll(t, 1, 1), pltpu.roll(t, 127, 1))
                t = t * (DB ** -0.5 * LOG2E)
                if rb == 0 and w:
                    t = jnp.where(rowi + r0 >= DIL * w, t, NEG)
                lg_s[w, pl.ds(rb * RB, RB), :] = t
            return [], 1, lambda: pltpu.bitcast(lg_s[w, blk(2 * rb + _zero(p, 0), 8), :], U32)

        def local_sm(rb, e, gate):
            rows = pl.ds(rb * RB + SMR * e, SMR)
            lg = [gate(lg_s[w, rows, :]) for w in range(WIN)]
            m = _tree(lg, jnp.maximum)
            ps = [jnp.exp2(t - m) for t in lg]
            l = _tree(ps, jnp.add)
            r = pl.reciprocal(l, approx=True)
            r = r * (2.0 - l * r)
            for w in range(WIN):
                pr_s[w, rows, :] = ps[w] * r
            return [], 2, lambda: pltpu.bitcast(pr_s[0, blk(2 * rb + e + _zero(p, 0), 8), :], U32)

        def local_pv(rb, k, gate):
            rows = pl.ds(rb * RB, RB)
            ps = [pr_s[w + _zero(p, k), rows, :] for w in range(WIN)]
            ps[0] = gate(ps[0])
            o = [_fold([ps[w] * vb[cc, pl.ds(PAD + rb * RB - DIL * w, RB), :] for w in range(WIN)],
                       jnp.add) for cc in (k, k + 4)]
            if rb < NSUB:
                for e in range(2):
                    o_s[k + 4 * e, rows, :] = o[e]
                return [], 3, lambda: pltpu.bitcast(o_s[k, blk(2 * rb + _zero(p, 0), 8), :], U32)
            top = pl.ds((rb - NSUB) * RB, RB)
            for m, t in enumerate(_lhs7(o_s[k, top, :], o_s[k + 4, top, :], *o)):
                ob7[m, pl.ds((rb - NSUB) * RB // 2, RB // 2), strip(k)] = _pack(t)
            return [], 0, lambda: ob7[0, blk(rb - NSUB + _zero(p, 0), 8), strip(k)]

        order = [rb + e * NSUB for rb in range(NSUB) for e in range(2)]
        jobs["lo"] = []
        for k in range(len(order) + SML):
            for f, d, n in ((local_sm, SML, RB // SMR), (local_qk, 0, 8 // LG)):
                if 0 <= k - d < len(order):
                    jobs["lo"] += [part(f, order[k - d], e) for e in range(n)]
        jobs["lv"] = [part(local_pv, rb, e) for rb in order for e in range(4)]

        def wob(m):
            if m == 1:
                return wob_p[pl.ds(0, M // 4), pl.ds(0, M // 2)]
            if m == 4:
                return wob_p[pl.ds(M // 4, M // 4), pl.ds(M // 2, M // 2)]
            return wob5[RSUM.index(m)]

        bo = {}

        def proj_bo(n):
            for m in ORDER[len(bo):len(bo) + n]:
                bo[m] = mm(("bo", len(bo)), lambda: ob7[m], wob(m))
            if n and len(bo) == 7:
                scatter(qk_b, r0, _combine(lambda m: bo[m]))

        def out_weights(m, r, gate):
            ww = [[gate(wo_r[(p & 1) + _zero(p, m),
                             pl.ds((2 * (q >> 1) + (e >> 1)) * HQ + 8 * r, 8),
                             pl.ds((2 * (q & 1) + (e & 1)) * 128, 128)])
                   for e in range(4)] for q in range(4)]
            rows = blk(8 * (p >> 1) + r, 8)
            extra = jobs["sc"].pop(0)(gate)[0] if jobs["sc"] else []
            for n, w in enumerate(_words49(_rhs7, ww, m)):
                if n < len(extra):
                    w = jnp.where(never, extra[n], w)
                wo49[7 * m + n, p & 1, rows, :] = w
            return [], 0, lambda: wo49[7 * m + _zero(p, 0), p & 1, rows, :]

        jobs["wo"] = [part(out_weights, m, r) for m in range(7) for r in range(8)]

        ks, vs, qs = {}, {}, {}
        done, prods = {}, {}

        def project(kind, j, n, lhs, rhs, scale, pack):
            got = prods.setdefault((kind, j), {})
            for m in ORDER[len(got):len(got) + n]:
                got[m] = _combine(lambda k: mm((kind, j, 7 * len(got) + ORDER.index(k)),
                                               lhs(7 * m + k), rhs[7 * m + k]))
            if len(got) < 7:
                return None
            c = _combine(lambda m: got[m])
            c = [[pack(c[(rg & 2) + (cg >> 1)][2 * (rg & 1) + (cg & 1)] * scale(cg))
                  for rg in range(4)] for cg in range(4)]
            return [[jnp.concatenate([t[16 * e:16 * e + 16] for t in c[cg]], axis=0)
                     for e in range(2)] for cg in range(4)]

        def proj_kv(j, n):
            c = project("kv", j, n, lambda k: cq[k, 0, pl.ds(j * QQ, QQ), :], wkv,
                        lambda cg: ups[cg][:1], _riffle)
            if c is not None:
                for cg in range(4):
                    for e in range(2):
                        (vs, ks)[cg >> 1][(cg & 1, 2 * j + e)] = c[cg][e]

        def proj_q(g, n):
            rows = blk(2 * g + (p & 1), QQ)
            c = project("q", g, n,
                        lambda k: jnp.concatenate([xq[k, sr, rows, :] for sr in range(2)], axis=1),
                        wq49, lambda cg: QSCALE, _pack)
            if c is not None:
                for h in range(2):
                    for e in range(2):
                        old = qn[h, g, e]
                        for b in range(2):
                            qs[(h, 4 * g + 2 * b + e)] = jnp.where((p & 1) == b, c[h][e], old)
                        qn[h, g, e] = c[2 + h][e]

        def qk(h, i, dep):
            kk = jnp.concatenate([ks[(h, j)] for j in range(i + 1)], axis=0)
            q = qs[(h, i)]
            if dep is not None:
                q = jnp.where(never, done[(h, dep)], q)
            ch = _lane_chunks(mm(("qk", h, i), q, kk, NT, 512))
            ch[i] = jnp.where(causal, ch[i], NEG)
            return ch

        def softmax_pv(h, i, ch):
            m = jnp.max(_fold(ch, jnp.maximum), axis=1, keepdims=True)
            ps = [jnp.exp2(c - m) for c in ch]
            lp = ps[0]
            for j in range(1, i + 1):
                lp = lp + ps[j]
                if TIE and (j % TIE == TIE - 1 or j == i):
                    ps[j] = jnp.where(never, lp, ps[j])
            pb = jnp.concatenate(ps, axis=1).astype(BF16)
            vv = jnp.concatenate([vs[(h, j)] for j in range(i + 1)], axis=0)
            o = mm(("pv", h, i), pb, vv)
            if i >= LDEP:
                lp = jnp.where(never, o, lp)
            l = jnp.sum(lp, axis=1, keepdims=True)
            r = pl.reciprocal(l, approx=True)
            r = r * (2.0 - l * r)
            cn = _pack(o * r)
            done[(h, i)] = cn
            if FA <= i < NQ - 1:
                if h == 0 and F0 < 0:
                    site = ("qk", 1, i + 1)
                elif i + 3 < NQ:
                    site = ("kv", (i + 1) // 2 + 1, KVS * ((i + 1) & 1) + (F0, FD)[h])
                else:
                    site = ("bo", (i + 3 - NQ) * BOP[0] + h)
                sched.pending.setdefault(site, []).append(cn)
            ctx[2 * p + h, pl.ds(i * HQ, HQ), :] = cn

        proj_bv()
        proj_kv(0, 7)
        proj_q(0, 7)
        for i in range(NQ):
            dep = i - DEP if DEP <= i < FA + DEP else None
            s0 = qk(0, i, dep)
            s1 = qk(1, i, dep)
            if i + 2 < NQ:
                proj_kv(i // 2 + 1, 7 if i & 1 else KVS // 7)
                if i < 6:
                    proj_q(i // 2 + 1, 7 if i & 1 else QS // 7)
            else:
                proj_bo(BOP[i + 2 - NQ])
            softmax_pv(0, i, s0)
            softmax_pv(1, i, s1)
        proj_bo(BOP[2])
        sched.finish()
        for d in cp_p(p + 2):
            d.start()
        return carry

    jax.lax.fori_loop(0, NP, p2_body, 0)

    cp_gw().wait()
    gw = gw_ref[...].astype(F32)
    plan3 = _plan3()
    cab = (ca0, ca1)

    def p3_body(i, carry):
        r0 = pl.multiple_of(i * TO, TO)
        h0 = pl.multiple_of(i * (TO // 2), TO // 2)
        never = i > S

        def ctx_words(m, u, r, n):
            return [[ctx[4 * u + 2 * (q & 1) + (e & 1),
                         pl.ds(h0 + _zero(i, m) * 8 + ((2 * (q >> 1) + (e >> 1)) * QQ + r), n), :]
                     for e in range(4)] for q in range(4)]

        def operands(k, u, r, gate):
            m = ORDER[k]
            cw = [[gate(w) for w in q] for q in ctx_words(m, u, r, 8)]
            for n, w in enumerate(_words49(_lhs7, cw, m)):
                if not (m in (2, 3) and n in (2, 3)):
                    cab[k & 1][n, pl.ds(r, 8), pl.ds(u * 128, 128)] = w
            return [], 0, lambda: cab[k & 1][_zero(i, 0), pl.ds(r, 8), pl.ds(u * 128, 128)]

        def gate_rows(r, gate):
            gs = _fold([_bf(gate(xs_u[j, pl.ds(h0 + r, 8), :])).astype(F32) * gw[j:j + 1]
                        for j in range(8)], jnp.add)
            g = jax.nn.sigmoid(jnp.sum(gs, axis=1, keepdims=True))
            g_s[pl.ds(2 * r, 16), :] = jnp.broadcast_to(g, (16, 128))
            return [], 0, lambda: pltpu.bitcast(g_s[blk(r // 4 + _zero(i, 0), 8), :], U32)

        pr = {}

        def mix(q, e, cc, gate):
            off = (2 * (q >> 1) + (e >> 1)) * HQ
            ch = 4 * cc + 2 * (q & 1) + (e & 1)
            a = _combine(lambda m: pr.get(m, pr[2])[e][:, cc * 128:(cc + 1) * 128])[q]
            g = gate(g_s[pl.ds(off, HQ), :])
            b = qk_b[ch, pl.ds(r0 + (PAD + off), HQ), :]
            out_s[pl.ds(r0 + off, HQ), pl.ds(ch * 128, 128)] = (g * a + (1.0 - g) * b).astype(BF16)
            return [], 0, lambda: pltpu.bitcast(
                out_s[blk(i * (TO // 16) + off // 16 + _zero(i, 0), 16), pl.ds(ch * 128, 128)], U32)

        sched = _Sched(never, plan3, dict(
            a=[part(operands, k, u, r) for k in range(1, 7) for u in range(HA // 4)
               for r in range(0, QQ, 8)],
            g=[part(gate_rows, r) for r in range(0, TO // 2, 8)],
            m=[part(mix, q, e, cc) for q in (1, 2, 0) for e in range(4) for cc in range(2)]))
        first = [[_words49(_lhs7, ctx_words(ORDER[0], u, 0, QQ), ORDER[0])[n]
                  for u in range(HA // 4)] for n in range(7)]

        def inner(m, n):
            k = ORDER.index(m)
            res = []
            for e in range(2):
                us = range(4 * e, 4 * e + 4)
                if m in (2, 3) and n in (2, 3):
                    lhs = jnp.concatenate([ctx_words(m, u, 0, QQ)[3 * (m - 2)][3 * (n - 2)]
                                           for u in us], axis=1)
                elif k == 0:
                    lhs = jnp.concatenate([first[n][u] for u in us], axis=1)
                else:
                    lhs = lambda: cab[k & 1][n, :, pl.ds(e * 512, 512)]
                rhs = jnp.concatenate([wo49[7 * m + n, cc, pl.ds(e * 256, 256), :]
                                       for cc in range(2)], axis=1)
                res.append(sched.mm((k, 2 * ORDER.index(n) + e), lhs, rhs))
            return res[0] + res[1]

        for m in ORDER:
            pr[m] = _combine(lambda n: inner(m, n))
        sched.finish()
        for e in (1, 2, 0, 3):
            for cc in range(2):
                mix(3, e, cc, lambda x: x)
        cp_out(i).start()
        return carry

    jax.lax.fori_loop(0, S // TO, p3_body, 0)
    for g in range(NP, NP + 2):
        for d in cp_p(g):
            d.wait()
    for i in range(S // TO):
        cp_out(i).wait()


@jax.jit
def pallas_gated_mix__compressed_kv_cla__sliding_local_dilated__prompt_kernel(
    A_x: jax.Array,
    A_c_kv: jax.Array,
    A_w_q: jax.Array,
    A_w_uk: jax.Array,
    A_w_uv: jax.Array,
    A_w_o: jax.Array,
    B_x: jax.Array,
    B_wqkv: jax.Array,
    B_wo: jax.Array,
    gate_w: jax.Array,
):
    del B_x
    any_spec = pl.BlockSpec(memory_space=pl.ANY)
    out = pl.pallas_call(
        _kernel,
        in_specs=[any_spec] * 9,
        out_specs=any_spec,
        out_shape=jax.ShapeDtypeStruct((S, M), BF16),
        scratch_shapes=[
            pltpu.VMEM((9, S // 2, 128), U32),
            pltpu.VMEM((2, HQ, M), U32),
            pltpu.VMEM((2, HQ, DC), U32),
            pltpu.VMEM((2, 128, M), BF16),
            pltpu.VMEM((2, 2, 32, M), BF16),
            pltpu.VMEM((M // 2, M), U32),
            pltpu.VMEM((3, 2 * DC, 128), U32),
            pltpu.VMEM((4, M, 128), U32),
            pltpu.VMEM((2, 2 * DA, M // 2), U32),
            pltpu.VMEM((8, 64, 128), U32),
            pltpu.VMEM((49, 2, S // 8, 128), U32),
            pltpu.VMEM((49, 1, S // 8, 128), U32),
            pltpu.VMEM((7, 4, M // 4, 128), U32),
            pltpu.VMEM((5, M // 4, M // 2), U32),
            pltpu.VMEM((49, 2, NP * QQ, 128), U32),
            pltpu.VMEM((49, HQ, 128), U32),
            pltpu.VMEM((49, TQ, 128), U32),
            pltpu.VMEM((4, 8, 128), F32),
            pltpu.VMEM((4, DC // SCR * 8 + 16, 128), jnp.int32),
            pltpu.VMEM((5, QQ, M // 2), U32),
            pltpu.VMEM((2, 4, 2, HQ, 128), U32),
            pltpu.VMEM((16, S + PAD, 128), F32),
            pltpu.VMEM((8, TQ + PAD, 128), F32),
            pltpu.VMEM((WIN, TQ, 128), F32),
            pltpu.VMEM((WIN, TQ, 128), F32),
            pltpu.VMEM((8, HQ, 128), F32),
            pltpu.VMEM((7, QQ, M // 2), U32),
            pltpu.VMEM((HA, S // 2, 128), U32),
            pltpu.VMEM((7, QQ, M), U32),
            pltpu.VMEM((7, QQ, M), U32),
            pltpu.VMEM((TO, 128), F32),
            pltpu.VMEM((S, M), BF16),
            pltpu.VMEM((8, 128), BF16),
            pltpu.SemaphoreType.DMA((2,)),
            pltpu.SemaphoreType.DMA((2,)),
            pltpu.SemaphoreType.DMA((3,)),
        ],
        compiler_params=pltpu.CompilerParams(vmem_limit_bytes=120 * 1024 * 1024,
                                             disable_bounds_checks=True),
    )(
        A_x.reshape(S, M),
        A_c_kv.reshape(S, DC),
        A_w_q,
        A_w_uk,
        A_w_uv,
        A_w_o.reshape(HA * DA, M),
        B_wqkv.reshape(2, M // 2, 3 * M),
        B_wo.reshape(HB // 2, 2, DB, M),
        gate_w.reshape(8, 128),
    )
    return out.reshape(1, S, M)
```

```python
import functools
import math

import jax
import jax.numpy as jnp
import jax.experimental.pallas as pl
import jax.experimental.pallas.tpu as pltpu

F32 = jnp.float32
BF16 = jnp.bfloat16
U32 = jnp.uint32

S = 2048
M = 1024
HA = 32
DA = 128
DC = 512
HB = 32
DB = 32
WIN = 8
DIL = 2
PAD = 16
LOG2E = math.log2(math.e)
NEG = -1e9

TQ = 128
HQ = TQ // 2
QQ = TQ // 4
BOP = (2, 3, 2)
LX = 16
KVS = 28
QS = 28
QST = 2
LQ0 = 3
LG = 2
XN = 29
SK = 3
SMR = 16
P1N = 96
P0W = 1
ST = 0
P0T = 24
P0N = 64
P0S = ((0, 0, 2048), (1, 0, 1024), (1, 1024, 768), (1, 1792, 256))
P1S = tuple((h, r, 512) for h in range(2) for r in range(0, S, 512))
P3S = 4
P3M = 6
P3E = 12
NQ = S // TQ
NP = HA // 2
DEP = 2
SCR = 32
LN = 58
SML = 1
LE = 2
LI = 0
LA = 21
LB = 4
LS = 4
LP = ("q", 0, 4)
FA = 6
F0 = 0
FD = 8
TIE = 4
RB = 16
LDEP = 4
TO = 256
NN = (((1,), (0,)), ((), ()))
NT = (((1,), (1,)), ((), ()))


def _plan2():
    plan = {}

    def put(name, count, start, until):
        plan.setdefault(start, []).extend([(name, until)] * count)

    def after_qk(i):
        if i >= NQ - 2:
            return ("bo", (i - NQ + 2) * BOP[0] + 1)
        return ("kv", i // 2 + 1, KVS * (i & 1) + LX)

    def fill(name, count, sites):
        for start, room, until in sites:
            n = min(count, room - len(plan.get(start, ())))
            put(name, n, start, until)
            count -= n
        assert count == 0, (name, count)

    def qk_sites(lo, hi):
        return [(("qk", h, i), max(i + 1 - h * SK, 0), after_qk(i))
                for i in range(lo, hi) for h in range(2)]

    def q_sites(g, lo, hi, until):
        return [(("q", g, k), 1, until) for k in range(lo, hi, QST)]

    names = _spread(["lo"] * (64 // LG + 128 // SMR), LN)
    for k, name in enumerate(names):
        put(name, 1, ("bv", k // 4) if k < 56 else ("kv", 0, 2 * (k - 56) + 1), LP)
    first = [(("kv", 0, k), 1, ("kv", 1, 8)) for k in range(LA, 49, LS)]
    first += [(("q", 0, k), 1, ("kv", 1, 8)) for k in range(LI, 49 - LB, LE)]
    early = []
    for g in range(1, 4):
        early += q_sites(g, 0, QS - 4, after_qk(2 * g - 1))
        early += qk_sites(max(2 * g - 1, LQ0), 2 * g)
        early += q_sites(g, QS, 45, after_qk(2 * g))
        early += qk_sites(max(2 * g, LQ0), 2 * g + 1)
    fill("lv", 32, first + early)
    fill("wo", 56, early)
    fill("bx", 16, early + qk_sites(7, 14))
    fill("qw", 112, qk_sites(7, 14))
    fill("kv", 56, qk_sites(14, 16) + [(("bo", k), 8, ("bo", 6)) for k in range(BOP[0], 5)])
    return plan


def _planx():
    names = _spread(["qw"] * 112 + ["kv"] * 56 + ["bx"] * 16, 8 * XN)
    return {k: [(n, 31) for n in names[8 * k:8 * k + 8]] for k in range(XN)}


def _spread(names, ticks):
    out = [None] * ticks
    for k, name in enumerate(names):
        out[k * ticks // len(names)] = name
    return out


def _plan1(segs, lo, step, count):
    end = len(segs) - 1
    ticks = [k for k in range(lo, end) for _ in range(segs[k][2] // step)][:count]
    names = _spread(["x"] * 28 + ["c"] * 14 + ["o"] * 8 + ["v"] * 8, len(ticks))
    plan = {}
    for k, name in zip(ticks, names):
        plan.setdefault(k, []).append((name, end))
    return plan


def _plan3():
    plan = {}
    for k in range(6):
        lo = P3S if k == 0 else 0
        extra = ["g"] * 8 if k in (1, 2) else []
        names = _spread(["a"] * 32 + extra, 4 * (P3E - lo))
        for d in range(lo, P3E):
            plan[(k, d)] = [(n, (k + 1, 0)) for n in names[4 * (d - lo):4 * (d - lo) + 4]]
    names = _spread(["m"] * 24, 4 * P3M)
    for d in range(P3M):
        plan[(6, d)] = [(n, (6, 13)) for n in names[4 * d:4 * d + 4]]
    return plan


_STAGES = ((2, 4), (1, 3), (0, 2), (0, 6), (0, 1))


def _permute8(cols):
    cols = list(cols)
    lane = jax.lax.broadcasted_iota(jnp.int32, cols[0].shape, 1)
    for va, lb in _STAGES:
        lo = (lane & (1 << lb)) == 0
        sh = 1 << lb
        idx = [i for i in range(8) if not (i >> va) & 1]
        if lb == 6:
            rr = [pltpu.roll(jnp.where(lo, cols[i | (1 << va)], cols[i]), 64, 1) for i in idx]
            for i, r in zip(idx, rr):
                a, b = cols[i], cols[i | (1 << va)]
                cols[i] = jnp.where(lo, a, r)
                cols[i | (1 << va)] = jnp.where(lo, r, b)
        else:
            rb = [pltpu.roll(cols[i | (1 << va)], sh, 1) for i in idx]
            ra = [pltpu.roll(cols[i], 128 - sh, 1) for i in idx]
            for i, xa, xb in zip(idx, ra, rb):
                a, b = cols[i], cols[i | (1 << va)]
                cols[i] = jnp.where(lo, a, xb)
                cols[i | (1 << va)] = jnp.where(lo, xa, b)
    return cols


def _pack(x):
    return pltpu.bitcast(x.astype(BF16), U32)


def _bf(x):
    return pltpu.bitcast(x, BF16)


def _split(w):
    return (pltpu.bitcast(w << 16, F32), pltpu.bitcast(w & jnp.uint32(0xFFFF0000), F32))


def _join(lo, hi):
    return pltpu.bitcast(pltpu.pack_elementwise([lo, hi], packed_dtype=BF16), U32)


def _riffle(x):
    return jnp.concatenate([_join(x[r:r + 16], x[r + 16:r + 32]) for r in range(0, x.shape[0], 32)],
                           axis=0)


def _lhs7(a11, a12, a21, a22):
    return [a11 + a22, a21 + a22, a11, a22, a11 + a12, a21 - a11, a12 - a22]


def _rhs7(b11, b12, b21, b22):
    return [b11 + b22, b11, b12 - b22, b21 - b11, b22, b11 + b12, b21 + b22]


LSUM = (0, 1, 4, 5, 6)
RSUM = (0, 2, 3, 5, 6)


def _words7(fn, quads):
    halves = [_split(w) for w in quads]
    lo = fn(*[h[0] for h in halves])
    hi = fn(*[h[1] for h in halves])
    return [_join(a, b) for a, b in zip(lo, hi)]


def _combine(mm):
    add = functools.partial(jax.tree.map, jnp.add)
    sub = functools.partial(jax.tree.map, jnp.subtract)
    m2 = mm(2)
    m3 = mm(3)
    m4 = mm(4)
    c12 = add(m2, m4)
    t11 = sub(m3, m4)
    m1 = mm(1)
    c21 = add(m1, m3)
    t22 = sub(m2, m1)
    m0 = mm(0)
    t11 = add(t11, m0)
    t22 = add(t22, m0)
    c11 = add(t11, mm(6))
    return c11, c12, c21, add(t22, mm(5))


ORDER = (2, 3, 4, 1, 0, 6, 5)


def _zero(i, m):
    return i >> (8 + m)


def _merge(vals):
    return _fold([v[r:r + 8, c:c + 128] for v in vals for r in range(0, v.shape[0], 8)
                  for c in range(0, v.shape[1], 128)], jnp.bitwise_or)


def _gate(never, g):
    def gate(x):
        t = jnp.tile(pltpu.bitcast(g, x.dtype), (x.shape[0] // 8, x.shape[1] // 128))
        return jnp.where(never, t, x)
    return gate


def _tie(never, x, deps):
    if not deps:
        return x
    top = jnp.where(never, _merge(deps), x[:8, :128])
    if x.shape[1] > 128:
        top = jnp.concatenate([top, x[:8, 128:]], axis=1)
    return jnp.concatenate([top, x[8:]], axis=0)


class _Sched:
    def __init__(self, never, plan, jobs):
        self.never, self.plan, self.jobs, self.pending = never, plan, jobs, {}

    def mm(self, site, a, b, dims=NN, width=128, step=32):
        deps = [d() if callable(d) else d for d in self.pending.pop(site, ())]
        a = a() if callable(a) else a
        tie = functools.partial(_tie, self.never, deps=deps)
        a, b = (_bf(tie(a)), _bf(b)) if a.dtype == U32 else (a, _bf(tie(b)))
        out = jax.lax.dot_general(a, b, dims, preferred_element_type=F32)
        per = out.shape[0] // step
        last = {}
        for k, (name, until) in enumerate(self.plan.get(site, ())):
            if name is not None:
                r, c = step * (k % per), width * (k // per)
                vals, tag, stored = self.jobs[name].pop(0)(
                    _gate(self.never, out[r:r + 8, c:c + 128]))
                self.pending.setdefault(until, []).extend(vals)
                last[(name, tag, until)] = stored
        for (_, _, until), stored in last.items():
            if stored is not None:
                self.pending[until].append(stored)
        return out

    def finish(self):
        assert not any(self.jobs.values()) and not any(self.pending.values())


def _ops49(fn, blocks, m):
    return fn(*[fn(*[blocks[q][e] for q in range(4)])[m] for e in range(4)])


def _words49(fn, words, m):
    halves = [[_split(w) for w in q] for q in words]
    lo = _ops49(fn, [[h[0] for h in q] for q in halves], m)
    hi = _ops49(fn, [[h[1] for h in q] for q in halves], m)
    return [_join(a, b) for a, b in zip(lo, hi)]


def _fold(xs, op):
    acc = xs[0]
    for x in xs[1:]:
        acc = op(acc, x)
    return acc


def _tree(xs, op):
    while len(xs) > 1:
        xs = [op(a, b) for a, b in zip(xs[::2], xs[1::2])]
    return xs[0]


def _lane_chunks(x):
    return [x[:, j * 128:(j + 1) * 128] for j in range(x.shape[1] // 128)]


def _kernel(x_hbm, c_hbm, wq_hbm, wuk_hbm, wuv_hbm, wo_hbm, wqkv_hbm, wob_hbm, gw_hbm,
            out_hbm,
            xs_u, x_r, c_r, w_r, wv_r, wob_p, wkv_r, wq_r, wo_r,
            wperm, xq, cq, wv7, wob5, wo49, wkv, wq49, ups, sc_s, bx, qn,
            qk_b, vb, lg_s, pr_s, o_s, ob7, ctx, ca0, ca1, g_s, out_s, gw_ref,
            sem_x, sem_p, sem_a):
    x_u = x_hbm.bitcast(U32)
    c_u = c_hbm.bitcast(U32)
    wo_u = wo_hbm.bitcast(U32)
    wq_u = wq_hbm.bitcast(U32)
    wuk_u = wuk_hbm.bitcast(U32)
    wuv_u = wuv_hbm.bitcast(U32)
    wob_u = wob_hbm.bitcast(U32)
    part = functools.partial

    def blk(j, n):
        return pl.ds(pl.multiple_of(j * n, n), n)

    def strip(j):
        return blk(j, 128)

    def cp_x(t, sem):
        k = (t + 1) >> 1
        return pltpu.make_async_copy(x_u.at[blk(t & 1, S // 4), strip(jnp.minimum(k, 7))],
                                     xs_u.at[jnp.minimum(k, 8), blk(t & 1, S // 4), :], sem)

    def cp_w(t, sem):
        u = t - 2 * (t >> 4)
        u = u - 2 * (u >> 4)
        return pltpu.make_async_copy(wqkv_hbm.at[u >> 3, strip((u >> 1) & 3), blk(u & 1, M)],
                                     w_r.at[u & 1], sem)

    def group(t):
        sem = sem_x.at[t & 1]
        late = t >> 4
        u = t - 2 * late
        dp = ((u >> 3) << 2) + (u & 2) + ((u >> 2) & 1)
        pq = (t >> 3) + late
        return (
            cp_x(t, sem),
            cp_w(t + 1, sem),
            pltpu.make_async_copy(x_u.at[blk(u, HQ), :], x_r.at[u & 1], sem),
            pltpu.make_async_copy(c_u.at[blk(u, HQ), :], c_r.at[u & 1], sem),
            pltpu.make_async_copy(wob_u.at[:, u & 1, dp, :], wob_p.at[blk(u, 16), :], sem),
            pltpu.make_async_copy(wob_u.at[:, u & 1, dp + 8, :], wob_p.at[blk(u + 16, 16), :], sem),
            pltpu.make_async_copy(wqkv_hbm.at[0, blk(u, 32), pl.ds(2 * M, M)],
                                  wv_r.at[u & 1, 0], sem),
            pltpu.make_async_copy(wqkv_hbm.at[1, blk(u, 32), pl.ds(2 * M, M)],
                                  wv_r.at[u & 1, 1], sem),
            pltpu.make_async_copy(wq_u.at[strip(t & 7), pq, :], wq_r.at[pq, strip(t & 7), :], sem),
            pltpu.make_async_copy(wuk_u.at[blk(u, 32), 0, :],
                                  wkv_r.at[1 + late, blk(16 + u, 32), :], sem),
            pltpu.make_async_copy(wuv_u.at[blk(u, 32), 0, :],
                                  wkv_r.at[1 + late, blk(u, 32), :], sem),
        )

    def cp_wq(p, sem):
        return pltpu.make_async_copy(wq_u.at[:, jnp.minimum(p, NP - 1), :], wq_r.at[p & 3], sem)

    def cp_p(g):
        slot = g & 1
        p = jnp.minimum(g + 1, NP - 1)
        o = jnp.minimum(g, NP - 1)
        sem = sem_p.at[slot]
        return (
            pltpu.make_async_copy(wo_u.at[blk(o >> 1, 2 * DA), blk(o & 1, M // 2)],
                                  wo_r.at[slot], sem),
            pltpu.make_async_copy(wuk_u.at[:, p, :], wkv_r.at[slot, pl.ds(DC, DC), :], sem),
            pltpu.make_async_copy(wuv_u.at[:, p, :], wkv_r.at[slot, pl.ds(0, DC), :], sem),
            cp_wq(g + 2, sem),
        )

    def cp_gw():
        return pltpu.make_async_copy(gw_hbm, gw_ref, sem_a.at[0])

    def cp_out(i):
        return pltpu.make_async_copy(out_s.at[blk(i, TO), :], out_hbm.at[blk(i, TO), :],
                                     sem_a.at[1])

    cp_w(0, sem_a.at[1]).start()
    for t in range(2):
        cp_x(-t, sem_a.at[2]).start()
    for d in group(0)[1:]:
        d.start()

    for cc in range(8):
        qk_b[8 + cc, pl.ds(0, PAD), :] = jnp.zeros((PAD, 128), F32)
        vb[cc, pl.ds(TQ, PAD), :] = jnp.zeros((PAD, 128), F32)

    def stage_first(t):
        for cc, w in enumerate(_permute8(_lane_chunks(pltpu.bitcast(w_r[t & 1], U32)))):
            wperm[cc] = w

    def p1_step(t, peel):
        if not peel:
            for d in group(t):
                d.wait()

        def act_sums(src, dst, ns, m, sr, r, gate):
            cw = [[gate(src[(t & 1) + _zero(t, m), pl.ds(32 * (q >> 1) + 16 * (e >> 1) + 8 * r, 8),
                            pl.ds(((2 * (q & 1) + (e & 1)) * ns + sr) * 128, 128)])
                   for e in range(4)] for q in range(4)]
            for n, w in enumerate(_words49(_lhs7, cw, m)):
                dst[7 * m + n, sr, blk(2 * t + r, 8), :] = w
            return [], 0, lambda: dst[7 * m + _zero(t, 0), sr, blk(2 * t + r, 8), :]

        wv = []

        def load_wv():
            wv.extend(_permute8(_lane_chunks(jnp.concatenate(
                [pltpu.bitcast(wv_r[t & 1, e], U32) for e in range(2)], axis=0))))

        def v_sums(r, cc, gate):
            ops = _words7(_rhs7, [gate(wv[cc + 4 * d][16 * e + 8 * r:16 * e + 8 * r + 8])
                                  for e in range(2) for d in range(2)])
            for m in range(7):
                wv7[m, cc, blk(2 * t + r, 8), :] = ops[m]
            return [], 0, lambda: wv7[_zero(t, 0), cc, blk(2 * t + r, 8), :]

        def o_sums(r, cc, gate):
            ops = _words7(_rhs7, [gate(wob_p[blk(2 * t + r + 32 * e, 8), strip(cc + 4 * d)])
                                  for e in range(2) for d in range(2)])
            for e, m in enumerate(RSUM):
                wob5[e, blk(2 * t + r, 8), strip(cc)] = ops[m]
            return [], 0, lambda: wob5[_zero(t, 0), blk(2 * t + r, 8), strip(cc)]

        segs, step = (P0S, P0T) if peel else (P1S, 32)
        sched = _Sched(t > 99, _plan1(segs, P0W * peel, step, P0N if peel else P1N), dict(
            x=[part(act_sums, x_r, xq, 2, m, sr, r)
               for m in range(7) for sr in range(2) for r in range(2)],
            c=[part(act_sums, c_r, cq, 1, m, 0, r) for m in range(7) for r in range(2)],
            v=[part(v_sums, r, cc) for r in range(2) for cc in range(4)],
            o=[part(o_sums, r, cc) for r in range(2) for cc in range(4)]))

        first = t < 2
        for k, (half, r0, n) in enumerate(segs):
            if k == P0W * peel:
                if peel:
                    for d in group(0)[1:]:
                        d.wait()
                    if ST == 1:
                        for d in group(1):
                            d.start()
                load_wv()
            w = jnp.concatenate([wperm[4 * half + cc] for cc in range(4)], axis=1)
            r = sched.mm(k, xs_u[t >> 1, pl.ds(r0 // 2, n // 2), :], w, step=step)
            for cc in range(4):
                sl = (8 * (t & 1) + 4 * half + cc, pl.ds(PAD + r0, n), slice(None))
                new = r[:, cc * 128:(cc + 1) * 128]
                qk_b[sl] = new if peel else jnp.where(first, 0.0, qk_b[sl]) + new
        sched.finish()
        stage_first(t + 1)
        d = group(t + 2)
        for d in d[2:] + d[:2]:
            d.start()
        return t

    zero = jnp.max(vb[0, pl.ds(TQ, 8), :]).astype(jnp.int32)
    cp_w(0, sem_a.at[1]).wait()
    stage_first(0)
    if ST == 0:
        for d in group(1):
            d.start()
    for t in range(2):
        cp_x(-t, sem_a.at[2]).wait()
    p1_step(zero, True)
    for d in cp_p(0) + (cp_gw(),):
        d.start()
    last = jax.lax.fori_loop(1, 16, lambda t, c: p1_step(t, False), 0)

    row = jax.lax.broadcasted_iota(jnp.int32, (TQ, TQ), 0)
    col = jax.lax.broadcasted_iota(jnp.int32, (TQ, TQ), 1)
    col = (col & ~31) | ((col & 1) << 4) | ((col & 31) >> 1)
    rowi = jax.lax.broadcasted_iota(jnp.int32, (RB, 128), 0)
    odd = (jax.lax.broadcasted_iota(jnp.int32, (RB, 128), 1) & 1) == 1
    NSUB = HQ // RB
    QSCALE = DA ** -0.5 * LOG2E

    def pair_rows(src, slot, r0, n, gate):
        return [_split(gate(src[slot, pl.ds(r0 + par, n // 2, stride=2), :])) for par in range(2)]

    def staging(g, z, never):
        ns = DC // SCR

        def scales(n1, k, gate):
            res = []
            for h in range(2):
                if k < ns:
                    w = gate(wkv_r[g & 1, pl.ds(n1 * DC + k * SCR, SCR), :])
                    w = pltpu.bitcast(w, jnp.int32) & (0x7F80 << (16 * h))
                else:
                    w = gate(sc_s[2 * n1 + h, pl.ds(0, 8 * ns), :])
                e = _tree([w[r:r + 8] for r in range(0, w.shape[0], 8)], jnp.maximum)
                if k == ns:
                    e = pltpu.bitcast(e << (16 - 16 * h), F32)
                    e = jnp.max(e, axis=0, keepdims=True)
                    e = jnp.clip(pltpu.bitcast(e, jnp.int32), 1 << 23, 253 << 23)
                    e = jnp.broadcast_to(e, (8, 128))
                    sc_s[2 * n1 + h, pl.ds(8 * ns + 8, 8), :] = (254 << 23) - e
                sc_s[2 * n1 + h, pl.ds(8 * k, 8), :] = e
                res.append(pltpu.bitcast(e, U32))
            return res, 0, lambda: pltpu.bitcast(sc_s[2 * n1, blk(k + _zero(z, 0), 8), :], U32)

        def rhs49(dst, tiles, scale, m, r, extra=()):
            res = [_ops49(_rhs7,
                          [[scale(tiles[2 * (q >> 1) + (e >> 1)][q & 1][par][e & 1],
                                  2 * (q & 1) + (e & 1)) for e in range(4)] for q in range(4)],
                          m) for par in range(2)]
            for k, (lo, hi) in enumerate(zip(*res)):
                w = _join(lo, hi)
                if k < len(extra):
                    w = jnp.where(never, extra[k], w)
                dst[7 * m + k, pl.ds(8 * r, 8), :] = w

        def kv(m, r, gate):
            if m == 0 and r == 0:
                for k in range(4):
                    ups[k] = pltpu.bitcast(gate(sc_s[k, pl.ds(8 * ns, 8), :]), F32)
            down = [pltpu.bitcast(sc_s[k + _zero(z, m), pl.ds(8 * ns + 8, 8), :], F32)
                    for k in range(4)]
            tiles = [[pair_rows(wkv_r, (g & 1) + _zero(z, m), n1 * DC + kt * 128 + 16 * r, 16, gate)
                      for n1 in range(2)] for kt in range(4)]
            rhs49(wkv, tiles, lambda w, k: w * down[k], m, r)
            return [], 0, lambda: wkv[7 * m, blk(r + _zero(z, 0), 8), :]

        def qw(m, r, gate):
            tiles = [[pair_rows(wq_r, ((g + 1 + n1) & 3) + _zero(z, m), kt * 256 + 16 * r, 16, gate)
                      for n1 in range(2)] for kt in range(4)]
            rhs49(wq49, tiles, lambda w, k: w, m, r, sc.pop(0)(gate)[0] if sc else ())
            return [], 0, lambda: wq49[7 * m, blk(r + _zero(z, 0), 8), :]

        def b_lhs(u, r, gate):
            base = 8 * jnp.minimum(g + 1, NQ - 1) + r
            ops = _words7(_lhs7, [gate(xs_u[u + 4 * d, blk(base + 4 * e, 8), :])
                                  for e in range(2) for d in range(2)])
            for k, m in enumerate(LSUM):
                bx[k, pl.ds(8 * r, 8), strip(u)] = ops[m]
            return [], 0, lambda: bx[0, blk(r + _zero(z, 0), 8), strip(u)]

        sc = [part(scales, n1, k) for k in range(ns + 1) for n1 in range(2)]
        return dict(sc=sc,
                    kv=[part(kv, m, r) for m in range(7) for r in range(8)],
                    qw=[part(qw, m, r) for m in range(7) for r in range(16)],
                    bx=[part(b_lhs, u, r) for u in range(4) for r in range(4)])

    sched = _Sched(last > 99, _planx(), staging(-1, last, last > 99))
    w0 = pair_rows(wq_r, 0, 0, M, lambda x: x)
    w0 = [_join(w0[0][h], w0[1][h]) for h in range(2)]
    for g in range(4):
        for e in range(2):
            for h in range(2):
                q = [sched.mm(8 * g + 4 * e + 2 * h + k, jnp.concatenate(
                    [xs_u[4 * k + u, pl.ds((4 * g + 2 + e) * HQ, HQ), :] for u in range(4)], axis=1),
                    w0[h][256 * k:256 * k + 256], step=16) for k in range(2)]
                qn[h, g, e] = _pack((q[0] + q[1]) * QSCALE)
    sched.finish()
    for d in group(16) + group(17):
        d.wait()
    for d in cp_p(1):
        d.start()
    plan2 = _plan2()

    def p2_body(p, carry):
        for d in cp_p(p):
            d.wait()
        causal = col <= row
        never = p > NP
        jobs = staging(p, p, never)
        sched = _Sched(never, plan2, jobs)
        mm = sched.mm

        r0 = pl.multiple_of(p * TQ, TQ)

        def scatter(dst, off, c):
            for e, t in enumerate(c):
                for cc in range(4):
                    dst[4 * (e & 1) + cc, pl.ds(off + (PAD + (e >> 1) * HQ), HQ), :] = (
                        t[:, cc * 128:(cc + 1) * 128])

        def proj_bv():
            def lhs(m):
                if m in (2, 3):
                    return jnp.concatenate([xs_u[u + 4 * (m - 2), blk(2 * p + m - 2, QQ), :]
                                            for u in range(4)], axis=1)
                return bx[LSUM.index(m)]

            for cc in range(8):
                vb[cc, pl.ds(0, PAD), :] = vb[cc, pl.ds(TQ, PAD), :]
            c = [_combine(lambda m: mm(("bv", 7 * e + ORDER.index(m)), lhs(m), jnp.concatenate(
                [wv7[m, 2 * e], wv7[m, 2 * e + 1]], axis=1))) for e in range(2)]
            scatter(vb, 0, [jnp.concatenate(t, axis=1) for t in zip(*c)])

        def local_qk(rb, k, gate):
            q = [qk_b[cc, pl.ds(r0 + _zero(p, k) + (PAD + rb * RB), RB), :] for cc in range(8)]
            q[0] = gate(q[0])
            for w in range(LG * k, LG * k + LG):
                t = _fold([q[cc] * qk_b[8 + cc, pl.ds(r0 + (PAD + rb * RB - DIL * w), RB), :]
                           for cc in range(8)], jnp.add)
                t = t + pltpu.roll(t, 64, 1)
                t = t + jnp.where(odd, pltpu.roll(t, 1, 1), pltpu.roll(t, 127, 1))
                t = t * (DB ** -0.5 * LOG2E)
                if rb == 0 and w:
                    t = jnp.where(rowi + r0 >= DIL * w, t, NEG)
                lg_s[w, pl.ds(rb * RB, RB), :] = t
            return [], 1, lambda: pltpu.bitcast(lg_s[w, blk(2 * rb + _zero(p, 0), 8), :], U32)

        def local_sm(rb, e, gate):
            rows = pl.ds(rb * RB + SMR * e, SMR)
            lg = [gate(lg_s[w, rows, :]) for w in range(WIN)]
            m = _tree(lg, jnp.maximum)
            ps = [jnp.exp2(t - m) for t in lg]
            l = _tree(ps, jnp.add)
            r = pl.reciprocal(l, approx=True)
            r = r * (2.0 - l * r)
            for w in range(WIN):
                pr_s[w, rows, :] = ps[w] * r
            return [], 2, lambda: pltpu.bitcast(pr_s[0, blk(2 * rb + e + _zero(p, 0), 8), :], U32)

        def local_pv(rb, k, gate):
            rows = pl.ds(rb * RB, RB)
            ps = [pr_s[w + _zero(p, k), rows, :] for w in range(WIN)]
            ps[0] = gate(ps[0])
            o = [_fold([ps[w] * vb[cc, pl.ds(PAD + rb * RB - DIL * w, RB), :] for w in range(WIN)],
                       jnp.add) for cc in (k, k + 4)]
            if rb < NSUB:
                for e in range(2):
                    o_s[k + 4 * e, rows, :] = o[e]
                return [], 3, lambda: pltpu.bitcast(o_s[k, blk(2 * rb + _zero(p, 0), 8), :], U32)
            top = pl.ds((rb - NSUB) * RB, RB)
            for m, t in enumerate(_lhs7(o_s[k, top, :], o_s[k + 4, top, :], *o)):
                ob7[m, pl.ds((rb - NSUB) * RB // 2, RB // 2), strip(k)] = _pack(t)
            return [], 0, lambda: ob7[0, blk(rb - NSUB + _zero(p, 0), 8), strip(k)]

        order = [rb + e * NSUB for rb in range(NSUB) for e in range(2)]
        jobs["lo"] = []
        for k in range(len(order) + SML):
            for f, d, n in ((local_sm, SML, RB // SMR), (local_qk, 0, 8 // LG)):
                if 0 <= k - d < len(order):
                    jobs["lo"] += [part(f, order[k - d], e) for e in range(n)]
        jobs["lv"] = [part(local_pv, rb, e) for rb in order for e in range(4)]

        def wob(m):
            if m == 1:
                return wob_p[pl.ds(0, M // 4), pl.ds(0, M // 2)]
            if m == 4:
                return wob_p[pl.ds(M // 4, M // 4), pl.ds(M // 2, M // 2)]
            return wob5[RSUM.index(m)]

        bo = {}

        def proj_bo(n):
            for m in ORDER[len(bo):len(bo) + n]:
                bo[m] = mm(("bo", len(bo)), lambda: ob7[m], wob(m))
            if n and len(bo) == 7:
                scatter(qk_b, r0, _combine(lambda m: bo[m]))

        def out_weights(m, r, gate):
            ww = [[gate(wo_r[(p & 1) + _zero(p, m),
                             pl.ds((2 * (q >> 1) + (e >> 1)) * HQ + 8 * r, 8),
                             pl.ds((2 * (q & 1) + (e & 1)) * 128, 128)])
                   for e in range(4)] for q in range(4)]
            rows = blk(8 * (p >> 1) + r, 8)
            extra = jobs["sc"].pop(0)(gate)[0] if jobs["sc"] else []
            for n, w in enumerate(_words49(_rhs7, ww, m)):
                if n < len(extra):
                    w = jnp.where(never, extra[n], w)
                wo49[7 * m + n, p & 1, rows, :] = w
            return [], 0, lambda: wo49[7 * m + _zero(p, 0), p & 1, rows, :]

        jobs["wo"] = [part(out_weights, m, r) for m in range(7) for r in range(8)]

        ks, vs, qs = {}, {}, {}
        done, prods = {}, {}

        def project(kind, j, n, lhs, rhs, scale, pack):
            got = prods.setdefault((kind, j), {})
            for m in ORDER[len(got):len(got) + n]:
                got[m] = _combine(lambda k: mm((kind, j, 7 * len(got) + ORDER.index(k)),
                                               lhs(7 * m + k), rhs[7 * m + k]))
            if len(got) < 7:
                return None
            c = _combine(lambda m: got[m])
            c = [[pack(c[(rg & 2) + (cg >> 1)][2 * (rg & 1) + (cg & 1)] * scale(cg))
                  for rg in range(4)] for cg in range(4)]
            return [[jnp.concatenate([t[16 * e:16 * e + 16] for t in c[cg]], axis=0)
                     for e in range(2)] for cg in range(4)]

        def proj_kv(j, n):
            c = project("kv", j, n, lambda k: cq[k, 0, pl.ds(j * QQ, QQ), :], wkv,
                        lambda cg: ups[cg][:1], _riffle)
            if c is not None:
                for cg in range(4):
                    for e in range(2):
                        (vs, ks)[cg >> 1][(cg & 1, 2 * j + e)] = c[cg][e]

        def proj_q(g, n):
            rows = blk(2 * g + (p & 1), QQ)
            c = project("q", g, n,
                        lambda k: jnp.concatenate([xq[k, sr, rows, :] for sr in range(2)], axis=1),
                        wq49, lambda cg: QSCALE, _pack)
            if c is not None:
                for h in range(2):
                    for e in range(2):
                        old = qn[h, g, e]
                        for b in range(2):
                            qs[(h, 4 * g + 2 * b + e)] = jnp.where((p & 1) == b, c[h][e], old)
                        qn[h, g, e] = c[2 + h][e]

        def qk(h, i, dep):
            kk = jnp.concatenate([ks[(h, j)] for j in range(i + 1)], axis=0)
            q = qs[(h, i)]
            if dep is not None:
                q = jnp.where(never, done[(h, dep)], q)
            ch = _lane_chunks(mm(("qk", h, i), q, kk, NT, 512))
            ch[i] = jnp.where(causal, ch[i], NEG)
            return ch

        def softmax_pv(h, i, ch):
            m = jnp.max(_fold(ch, jnp.maximum), axis=1, keepdims=True)
            ps = [jnp.exp2(c - m) for c in ch]
            lp = ps[0]
            for j in range(1, i + 1):
                lp = lp + ps[j]
                if TIE and (j % TIE == TIE - 1 or j == i):
                    ps[j] = jnp.where(never, lp, ps[j])
            pb = jnp.concatenate(ps, axis=1).astype(BF16)
            vv = jnp.concatenate([vs[(h, j)] for j in range(i + 1)], axis=0)
            o = mm(("pv", h, i), pb, vv)
            if i >= LDEP:
                lp = jnp.where(never, o, lp)
            l = jnp.sum(lp, axis=1, keepdims=True)
            r = pl.reciprocal(l, approx=True)
            r = r * (2.0 - l * r)
            cn = _pack(o * r)
            done[(h, i)] = cn
            if FA <= i < NQ - 1:
                if h == 0 and F0 < 0:
                    site = ("qk", 1, i + 1)
                elif i + 3 < NQ:
                    site = ("kv", (i + 1) // 2 + 1, KVS * ((i + 1) & 1) + (F0, FD)[h])
                else:
                    site = ("bo", (i + 3 - NQ) * BOP[0] + h)
                sched.pending.setdefault(site, []).append(cn)
            ctx[2 * p + h, pl.ds(i * HQ, HQ), :] = cn

        proj_bv()
        proj_kv(0, 7)
        proj_q(0, 7)
        for i in range(NQ):
            dep = i - DEP if DEP <= i < FA + DEP else None
            s0 = qk(0, i, dep)
            s1 = qk(1, i, dep)
            if i + 2 < NQ:
                proj_kv(i // 2 + 1, 7 if i & 1 else KVS // 7)
                if i < 6:
                    proj_q(i // 2 + 1, 7 if i & 1 else QS // 7)
            else:
                proj_bo(BOP[i + 2 - NQ])
            softmax_pv(0, i, s0)
            softmax_pv(1, i, s1)
        proj_bo(BOP[2])
        sched.finish()
        for d in cp_p(p + 2):
            d.start()
        return carry

    jax.lax.fori_loop(0, NP, p2_body, 0)

    cp_gw().wait()
    gw = gw_ref[...].astype(F32)
    plan3 = _plan3()
    cab = (ca0, ca1)

    def p3_body(i, carry):
        r0 = pl.multiple_of(i * TO, TO)
        h0 = pl.multiple_of(i * (TO // 2), TO // 2)
        never = i > S

        def ctx_words(m, u, r, n):
            return [[ctx[4 * u + 2 * (q & 1) + (e & 1),
                         pl.ds(h0 + _zero(i, m) * 8 + ((2 * (q >> 1) + (e >> 1)) * QQ + r), n), :]
                     for e in range(4)] for q in range(4)]

        def operands(k, u, r, gate):
            m = ORDER[k]
            cw = [[gate(w) for w in q] for q in ctx_words(m, u, r, 8)]
            for n, w in enumerate(_words49(_lhs7, cw, m)):
                if not (m in (2, 3) and n in (2, 3)):
                    cab[k & 1][n, pl.ds(r, 8), pl.ds(u * 128, 128)] = w
            return [], 0, lambda: cab[k & 1][_zero(i, 0), pl.ds(r, 8), pl.ds(u * 128, 128)]

        def gate_rows(r, gate):
            gs = _fold([_bf(gate(xs_u[j, pl.ds(h0 + r, 8), :])).astype(F32) * gw[j:j + 1]
                        for j in range(8)], jnp.add)
            g = jax.nn.sigmoid(jnp.sum(gs, axis=1, keepdims=True))
            g_s[pl.ds(2 * r, 16), :] = jnp.broadcast_to(g, (16, 128))
            return [], 0, lambda: pltpu.bitcast(g_s[blk(r // 4 + _zero(i, 0), 8), :], U32)

        pr = {}

        def mix(q, e, cc, gate):
            off = (2 * (q >> 1) + (e >> 1)) * HQ
            ch = 4 * cc + 2 * (q & 1) + (e & 1)
            a = _combine(lambda m: pr.get(m, pr[2])[e][:, cc * 128:(cc + 1) * 128])[q]
            g = gate(g_s[pl.ds(off, HQ), :])
            b = qk_b[ch, pl.ds(r0 + (PAD + off), HQ), :]
            out_s[pl.ds(r0 + off, HQ), pl.ds(ch * 128, 128)] = (g * a + (1.0 - g) * b).astype(BF16)
            return [], 0, lambda: pltpu.bitcast(
                out_s[blk(i * (TO // 16) + off // 16 + _zero(i, 0), 16), pl.ds(ch * 128, 128)], U32)

        sched = _Sched(never, plan3, dict(
            a=[part(operands, k, u, r) for k in range(1, 7) for u in range(HA // 4)
               for r in range(0, QQ, 8)],
            g=[part(gate_rows, r) for r in range(0, TO // 2, 8)],
            m=[part(mix, q, e, cc) for q in (1, 2, 0) for e in range(4) for cc in range(2)]))
        first = [[_words49(_lhs7, ctx_words(ORDER[0], u, 0, QQ), ORDER[0])[n]
                  for u in range(HA // 4)] for n in range(7)]

        def inner(m, n):
            k = ORDER.index(m)
            res = []
            for e in range(2):
                us = range(4 * e, 4 * e + 4)
                if m in (2, 3) and n in (2, 3):
                    lhs = jnp.concatenate([ctx_words(m, u, 0, QQ)[3 * (m - 2)][3 * (n - 2)]
                                           for u in us], axis=1)
                elif k == 0:
                    lhs = jnp.concatenate([first[n][u] for u in us], axis=1)
                else:
                    lhs = lambda: cab[k & 1][n, :, pl.ds(e * 512, 512)]
                rhs = jnp.concatenate([wo49[7 * m + n, cc, pl.ds(e * 256, 256), :]
                                       for cc in range(2)], axis=1)
                res.append(sched.mm((k, 2 * ORDER.index(n) + e), lhs, rhs))
            return res[0] + res[1]

        for m in ORDER:
            pr[m] = _combine(lambda n: inner(m, n))
        sched.finish()
        for e in (1, 2, 0, 3):
            for cc in range(2):
                mix(3, e, cc, lambda x: x)
        cp_out(i).start()
        return carry

    jax.lax.fori_loop(0, S // TO, p3_body, 0)
    for g in range(NP, NP + 2):
        for d in cp_p(g):
            d.wait()
    for i in range(S // TO):
        cp_out(i).wait()


@jax.jit
def pallas_gated_mix__compressed_kv_cla__sliding_local_dilated__prompt_kernel(
    A_x: jax.Array,
    A_c_kv: jax.Array,
    A_w_q: jax.Array,
    A_w_uk: jax.Array,
    A_w_uv: jax.Array,
    A_w_o: jax.Array,
    B_x: jax.Array,
    B_wqkv: jax.Array,
    B_wo: jax.Array,
    gate_w: jax.Array,
):
    del B_x
    any_spec = pl.BlockSpec(memory_space=pl.ANY)
    out = pl.pallas_call(
        _kernel,
        in_specs=[any_spec] * 9,
        out_specs=any_spec,
        out_shape=jax.ShapeDtypeStruct((S, M), BF16),
        scratch_shapes=[
            pltpu.VMEM((9, S // 2, 128), U32),
            pltpu.VMEM((2, HQ, M), U32),
            pltpu.VMEM((2, HQ, DC), U32),
            pltpu.VMEM((2, 128, M), BF16),
            pltpu.VMEM((2, 2, 32, M), BF16),
            pltpu.VMEM((M // 2, M), U32),
            pltpu.VMEM((3, 2 * DC, 128), U32),
            pltpu.VMEM((4, M, 128), U32),
            pltpu.VMEM((2, 2 * DA, M // 2), U32),
            pltpu.VMEM((8, 64, 128), U32),
            pltpu.VMEM((49, 2, S // 8, 128), U32),
            pltpu.VMEM((49, 1, S // 8, 128), U32),
            pltpu.VMEM((7, 4, M // 4, 128), U32),
            pltpu.VMEM((5, M // 4, M // 2), U32),
            pltpu.VMEM((49, 2, NP * QQ, 128), U32),
            pltpu.VMEM((49, HQ, 128), U32),
            pltpu.VMEM((49, TQ, 128), U32),
            pltpu.VMEM((4, 8, 128), F32),
            pltpu.VMEM((4, DC // SCR * 8 + 16, 128), jnp.int32),
            pltpu.VMEM((5, QQ, M // 2), U32),
            pltpu.VMEM((2, 4, 2, HQ, 128), U32),
            pltpu.VMEM((16, S + PAD, 128), F32),
            pltpu.VMEM((8, TQ + PAD, 128), F32),
            pltpu.VMEM((WIN, TQ, 128), F32),
            pltpu.VMEM((WIN, TQ, 128), F32),
            pltpu.VMEM((8, HQ, 128), F32),
            pltpu.VMEM((7, QQ, M // 2), U32),
            pltpu.VMEM((HA, S // 2, 128), U32),
            pltpu.VMEM((7, QQ, M), U32),
            pltpu.VMEM((7, QQ, M), U32),
            pltpu.VMEM((TO, 128), F32),
            pltpu.VMEM((S, M), BF16),
            pltpu.VMEM((8, 128), BF16),
            pltpu.SemaphoreType.DMA((2,)),
            pltpu.SemaphoreType.DMA((2,)),
            pltpu.SemaphoreType.DMA((3,)),
        ],
        compiler_params=pltpu.CompilerParams(vmem_limit_bytes=120 * 1024 * 1024,
                                             disable_bounds_checks=True),
    )(
        A_x.reshape(S, M),
        A_c_kv.reshape(S, DC),
        A_w_q,
        A_w_uk,
        A_w_uv,
        A_w_o.reshape(HA * DA, M),
        B_wqkv.reshape(2, M // 2, 3 * M),
        B_wo.reshape(HB // 2, 2, DB, M),
        gate_w.reshape(8, 128),
    )
    return out.reshape(1, S, M)
```

```python
import functools
import math

import jax
import jax.numpy as jnp
import jax.experimental.pallas as pl
import jax.experimental.pallas.tpu as pltpu

F32 = jnp.float32
BF16 = jnp.bfloat16
U32 = jnp.uint32

S = 2048
M = 1024
HA = 32
DA = 128
DC = 512
HB = 32
DB = 32
WIN = 8
DIL = 2
PAD = 16
LOG2E = math.log2(math.e)
NEG = -1e9

TQ = 128
HQ = TQ // 2
QQ = TQ // 4
BOP = (2, 3, 2)
LX = 16
KVS = 28
QS = 28
QST = 2
LQ0 = 3
LG = 2
XN = 29
SK = 3
SMR = 16
P1N = 96
P0W = 1
P0T = 24
P0N = 64
P0S = ((0, 0, 2048), (1, 0, 1024), (1, 1024, 768), (1, 1792, 256))
P1S = tuple((h, r, 512) for h in range(2) for r in range(0, S, 512))
P3S = 4
P3M = 6
P3D = 8
P3E = 12
NQ = S // TQ
NP = HA // 2
DEP = 2
SCR = 32
LN = 58
SML = 1
LE = 2
LI = 0
LA = 21
LB = 4
LS = 4
LP = ("q", 0, 4)
FA = 6
F0 = 0
FD = 8
TIE = 4
RB = 16
LDEP = 4
TO = 256
NN = (((1,), (0,)), ((), ()))
NT = (((1,), (1,)), ((), ()))


def _plan2():
    plan = {}

    def put(name, count, start, until):
        plan.setdefault(start, []).extend([(name, until)] * count)

    def after_qk(i):
        if i >= NQ - 2:
            return ("bo", (i - NQ + 2) * BOP[0] + 1)
        return ("kv", i // 2 + 1, KVS * (i & 1) + LX)

    def fill(name, count, sites):
        for start, room, until in sites:
            n = min(count, room - len(plan.get(start, ())))
            put(name, n, start, until)
            count -= n
        assert count == 0, (name, count)

    def qk_sites(lo, hi):
        return [(("qk", h, i), max(i + 1 - h * SK, 0), after_qk(i))
                for i in range(lo, hi) for h in range(2)]

    def q_sites(g, lo, hi, until):
        return [(("q", g, k), 1, until) for k in range(lo, hi, QST)]

    names = _spread(["lo"] * (64 // LG + 128 // SMR), LN)
    for k, name in enumerate(names):
        put(name, 1, ("bv", k // 4) if k < 56 else ("kv", 0, 2 * (k - 56) + 1), LP)
    first = [(("kv", 0, k), 1, ("kv", 1, 8)) for k in range(LA, 49, LS)]
    first += [(("q", 0, k), 1, ("kv", 1, 8)) for k in range(LI, 49 - LB, LE)]
    early = []
    for g in range(1, 4):
        early += q_sites(g, 0, QS - 4, after_qk(2 * g - 1))
        early += qk_sites(max(2 * g - 1, LQ0), 2 * g)
        early += q_sites(g, QS, 45, after_qk(2 * g))
        early += qk_sites(max(2 * g, LQ0), 2 * g + 1)
    fill("lv", 32, first + early)
    fill("wo", 56, early)
    fill("bx", 16, early + qk_sites(7, 14))
    fill("qw", 112, qk_sites(7, 14))
    fill("kv", 56, qk_sites(14, 16) + [(("bo", k), 8, ("bo", 6)) for k in range(BOP[0], 5)])
    return plan


def _planx():
    names = _spread(["qw"] * 112 + ["kv"] * 56 + ["bx"] * 16, 8 * XN)
    return {k: [(n, 31) for n in names[8 * k:8 * k + 8]] for k in range(XN)}


def _spread(names, ticks):
    out = [None] * ticks
    for k, name in enumerate(names):
        out[k * ticks // len(names)] = name
    return out


def _plan1(segs, lo, step, count):
    end = len(segs) - 1
    ticks = [k for k in range(lo, end) for _ in range(segs[k][2] // step)][:count]
    names = _spread(["x"] * 28 + ["c"] * 14 + ["o"] * 8 + ["v"] * 8, len(ticks))
    plan = {}
    for k, name in zip(ticks, names):
        plan.setdefault(k, []).append((name, end))
    return plan


def _plan3():
    plan = {}
    for k in range(6):
        lo = P3S if k == 0 else 0
        extra = ["g"] * 8 if k in (1, 2) else []
        names = _spread(["a"] * 32 + extra, 4 * (P3E - lo))
        for d in range(lo, P3E):
            plan[(k, d)] = [(n, (k + 1, 0)) for n in names[4 * (d - lo):4 * (d - lo) + 4]]
    names = _spread(["m"] * 24, 4 * P3M)
    for d in range(P3M):
        plan[(6, d)] = [(n, (6, P3D)) for n in names[4 * d:4 * d + 4]]
    return plan


_STAGES = ((2, 4), (1, 3), (0, 2), (0, 6), (0, 1))


def _permute8(cols):
    cols = list(cols)
    lane = jax.lax.broadcasted_iota(jnp.int32, cols[0].shape, 1)
    for va, lb in _STAGES:
        lo = (lane & (1 << lb)) == 0
        sh = 1 << lb
        idx = [i for i in range(8) if not (i >> va) & 1]
        if lb == 6:
            rr = [pltpu.roll(jnp.where(lo, cols[i | (1 << va)], cols[i]), 64, 1) for i in idx]
            for i, r in zip(idx, rr):
                a, b = cols[i], cols[i | (1 << va)]
                cols[i] = jnp.where(lo, a, r)
                cols[i | (1 << va)] = jnp.where(lo, r, b)
        else:
            rb = [pltpu.roll(cols[i | (1 << va)], sh, 1) for i in idx]
            ra = [pltpu.roll(cols[i], 128 - sh, 1) for i in idx]
            for i, xa, xb in zip(idx, ra, rb):
                a, b = cols[i], cols[i | (1 << va)]
                cols[i] = jnp.where(lo, a, xb)
                cols[i | (1 << va)] = jnp.where(lo, xa, b)
    return cols


def _pack(x):
    return pltpu.bitcast(x.astype(BF16), U32)


def _bf(x):
    return pltpu.bitcast(x, BF16)


def _split(w):
    return (pltpu.bitcast(w << 16, F32), pltpu.bitcast(w & jnp.uint32(0xFFFF0000), F32))


def _join(lo, hi):
    return pltpu.bitcast(pltpu.pack_elementwise([lo, hi], packed_dtype=BF16), U32)


def _riffle(x):
    return jnp.concatenate([_join(x[r:r + 16], x[r + 16:r + 32]) for r in range(0, x.shape[0], 32)],
                           axis=0)


def _lhs7(a11, a12, a21, a22):
    return [a11 + a22, a21 + a22, a11, a22, a11 + a12, a21 - a11, a12 - a22]


def _rhs7(b11, b12, b21, b22):
    return [b11 + b22, b11, b12 - b22, b21 - b11, b22, b11 + b12, b21 + b22]


LSUM = (0, 1, 4, 5, 6)
RSUM = (0, 2, 3, 5, 6)


def _words7(fn, quads):
    halves = [_split(w) for w in quads]
    lo = fn(*[h[0] for h in halves])
    hi = fn(*[h[1] for h in halves])
    return [_join(a, b) for a, b in zip(lo, hi)]


def _combine(mm):
    add = functools.partial(jax.tree.map, jnp.add)
    sub = functools.partial(jax.tree.map, jnp.subtract)
    m2 = mm(2)
    m3 = mm(3)
    m4 = mm(4)
    c12 = add(m2, m4)
    t11 = sub(m3, m4)
    m1 = mm(1)
    c21 = add(m1, m3)
    t22 = sub(m2, m1)
    m0 = mm(0)
    t11 = add(t11, m0)
    t22 = add(t22, m0)
    c11 = add(t11, mm(6))
    return c11, c12, c21, add(t22, mm(5))


ORDER = (2, 3, 4, 1, 0, 6, 5)


def _zero(i, m):
    return i >> (8 + m)


def _merge(vals):
    return _fold([v[r:r + 8, c:c + 128] for v in vals for r in range(0, v.shape[0], 8)
                  for c in range(0, v.shape[1], 128)], jnp.bitwise_or)


def _gate(never, g):
    def gate(x):
        t = jnp.tile(pltpu.bitcast(g, x.dtype), (x.shape[0] // 8, x.shape[1] // 128))
        return jnp.where(never, t, x)
    return gate


def _tie(never, x, deps):
    if not deps:
        return x
    top = jnp.where(never, _merge(deps), x[:8, :128])
    if x.shape[1] > 128:
        top = jnp.concatenate([top, x[:8, 128:]], axis=1)
    return jnp.concatenate([top, x[8:]], axis=0)


class _Sched:
    def __init__(self, never, plan, jobs):
        self.never, self.plan, self.jobs, self.pending = never, plan, jobs, {}

    def mm(self, site, a, b, dims=NN, width=128, step=32):
        deps = [d() if callable(d) else d for d in self.pending.pop(site, ())]
        a = a() if callable(a) else a
        tie = functools.partial(_tie, self.never, deps=deps)
        a, b = (_bf(tie(a)), _bf(b)) if a.dtype == U32 else (a, _bf(tie(b)))
        out = jax.lax.dot_general(a, b, dims, preferred_element_type=F32)
        per = out.shape[0] // step
        last = {}
        for k, (name, until) in enumerate(self.plan.get(site, ())):
            if name is not None:
                r, c = step * (k % per), width * (k // per)
                vals, tag, stored = self.jobs[name].pop(0)(
                    _gate(self.never, out[r:r + 8, c:c + 128]))
                self.pending.setdefault(until, []).extend(vals)
                last[(name, tag, until)] = stored
        for (_, _, until), stored in last.items():
            if stored is not None:
                self.pending[until].append(stored)
        return out

    def finish(self):
        assert not any(self.jobs.values()) and not any(self.pending.values())


def _ops49(fn, blocks, m):
    return fn(*[fn(*[blocks[q][e] for q in range(4)])[m] for e in range(4)])


def _words49(fn, words, m):
    halves = [[_split(w) for w in q] for q in words]
    lo = _ops49(fn, [[h[0] for h in q] for q in halves], m)
    hi = _ops49(fn, [[h[1] for h in q] for q in halves], m)
    return [_join(a, b) for a, b in zip(lo, hi)]


def _fold(xs, op):
    acc = xs[0]
    for x in xs[1:]:
        acc = op(acc, x)
    return acc


def _tree(xs, op):
    while len(xs) > 1:
        xs = [op(a, b) for a, b in zip(xs[::2], xs[1::2])]
    return xs[0]


def _lane_chunks(x):
    return [x[:, j * 128:(j + 1) * 128] for j in range(x.shape[1] // 128)]


def _kernel(x_hbm, c_hbm, wq_hbm, wuk_hbm, wuv_hbm, wo_hbm, wqkv_hbm, wob_hbm, gw_hbm,
            out_hbm,
            xs_u, x_r, c_r, w_r, wv_r, wob_p, wkv_r, wq_r, wo_r,
            wperm, xq, cq, wv7, wob5, wo49, wkv, wq49, ups, sc_s, bx, qn,
            qk_b, vb, lg_s, pr_s, o_s, ob7, ctx, ca0, ca1, g_s, out_s, gw_ref,
            sem_x, sem_p, sem_a):
    x_u = x_hbm.bitcast(U32)
    c_u = c_hbm.bitcast(U32)
    wo_u = wo_hbm.bitcast(U32)
    wq_u = wq_hbm.bitcast(U32)
    wuk_u = wuk_hbm.bitcast(U32)
    wuv_u = wuv_hbm.bitcast(U32)
    wob_u = wob_hbm.bitcast(U32)
    part = functools.partial

    def blk(j, n):
        return pl.ds(pl.multiple_of(j * n, n), n)

    def strip(j):
        return blk(j, 128)

    def cp_x(t, sem):
        k = (t + 1) >> 1
        return pltpu.make_async_copy(x_u.at[blk(t & 1, S // 4), strip(jnp.minimum(k, 7))],
                                     xs_u.at[jnp.minimum(k, 8), blk(t & 1, S // 4), :], sem)

    def cp_w(t, sem):
        u = t - 2 * (t >> 4)
        u = u - 2 * (u >> 4)
        return pltpu.make_async_copy(wqkv_hbm.at[u >> 3, strip((u >> 1) & 3), blk(u & 1, M)],
                                     w_r.at[u & 1], sem)

    def group(t, sem2=None):
        sem = sem_x.at[t & 1]
        sem2 = sem if sem2 is None else sem2
        late = t >> 4
        u = t - 2 * late
        dp = ((u >> 3) << 2) + (u & 2) + ((u >> 2) & 1)
        pq = (t >> 3) + late
        return (
            cp_x(t, sem),
            cp_w(t + 1, sem),
            pltpu.make_async_copy(x_u.at[blk(u, HQ), :], x_r.at[u & 1], sem),
            pltpu.make_async_copy(c_u.at[blk(u, HQ), :], c_r.at[u & 1], sem),
            pltpu.make_async_copy(wob_u.at[:, u & 1, dp, :], wob_p.at[blk(u, 16), :], sem),
            pltpu.make_async_copy(wob_u.at[:, u & 1, dp + 8, :], wob_p.at[blk(u + 16, 16), :], sem),
            pltpu.make_async_copy(wqkv_hbm.at[0, blk(u, 32), pl.ds(2 * M, M)],
                                  wv_r.at[u & 1, 0], sem),
            pltpu.make_async_copy(wqkv_hbm.at[1, blk(u, 32), pl.ds(2 * M, M)],
                                  wv_r.at[u & 1, 1], sem),
            pltpu.make_async_copy(wq_u.at[strip(t & 7), pq, :], wq_r.at[pq, strip(t & 7), :], sem2),
            pltpu.make_async_copy(wuk_u.at[blk(u, 32), 0, :],
                                  wkv_r.at[1 + late, blk(16 + u, 32), :], sem2),
            pltpu.make_async_copy(wuv_u.at[blk(u, 32), 0, :],
                                  wkv_r.at[1 + late, blk(u, 32), :], sem2),
        )

    def cp_wq(p, sem):
        return pltpu.make_async_copy(wq_u.at[:, jnp.minimum(p, NP - 1), :], wq_r.at[p & 3], sem)

    def cp_p(g):
        slot = g & 1
        p = jnp.minimum(g + 1, NP - 1)
        o = jnp.minimum(g, NP - 1)
        sem = sem_p.at[slot]
        return (
            pltpu.make_async_copy(wo_u.at[blk(o >> 1, 2 * DA), blk(o & 1, M // 2)],
                                  wo_r.at[slot], sem),
            pltpu.make_async_copy(wuk_u.at[:, p, :], wkv_r.at[slot, pl.ds(DC, DC), :], sem),
            pltpu.make_async_copy(wuv_u.at[:, p, :], wkv_r.at[slot, pl.ds(0, DC), :], sem),
            cp_wq(g + 2, sem),
        )

    def cp_gw():
        return pltpu.make_async_copy(gw_hbm, gw_ref, sem_a.at[0])

    def cp_out(i, late):
        def cp(rows, cols):
            return pltpu.make_async_copy(out_s.at[rows, cols], out_hbm.at[rows, cols], sem_a.at[1])

        low = [cp(blk(2 * i + 1, TO // 2), pl.ds(512 * cc + 256 * late, 256)) for cc in range(2)]
        return low if late else [cp(blk(2 * i, TO // 2), pl.ds(0, M))] + low

    cp_w(0, sem_a.at[1]).start()
    for t in range(2):
        cp_x(-t, sem_a.at[2]).start()
    group0 = group(0, sem_p.at[1])
    for d in group0[1:] + group(1)[:1] + group(1)[2:]:
        d.start()

    for cc in range(8):
        qk_b[8 + cc, pl.ds(0, PAD), :] = jnp.zeros((PAD, 128), F32)
        vb[cc, pl.ds(TQ, PAD), :] = jnp.zeros((PAD, 128), F32)

    def stage_first(t):
        for cc, w in enumerate(_permute8(_lane_chunks(pltpu.bitcast(w_r[t & 1], U32)))):
            wperm[cc] = w

    def p1_step(t, peel):
        if not peel:
            for d in group(t):
                d.wait()

        def act_sums(src, dst, ns, m, sr, r, gate):
            cw = [[gate(src[(t & 1) + _zero(t, m), pl.ds(32 * (q >> 1) + 16 * (e >> 1) + 8 * r, 8),
                            pl.ds(((2 * (q & 1) + (e & 1)) * ns + sr) * 128, 128)])
                   for e in range(4)] for q in range(4)]
            for n, w in enumerate(_words49(_lhs7, cw, m)):
                dst[7 * m + n, sr, blk(2 * t + r, 8), :] = w
            return [], 0, lambda: dst[7 * m + _zero(t, 0), sr, blk(2 * t + r, 8), :]

        wv = []

        def load_wv():
            wv.extend(_permute8(_lane_chunks(jnp.concatenate(
                [pltpu.bitcast(wv_r[t & 1, e], U32) for e in range(2)], axis=0))))

        def v_sums(r, cc, gate):
            ops = _words7(_rhs7, [gate(wv[cc + 4 * d][16 * e + 8 * r:16 * e + 8 * r + 8])
                                  for e in range(2) for d in range(2)])
            for m in range(7):
                wv7[m, cc, blk(2 * t + r, 8), :] = ops[m]
            return [], 0, lambda: wv7[_zero(t, 0), cc, blk(2 * t + r, 8), :]

        def o_sums(r, cc, gate):
            ops = _words7(_rhs7, [gate(wob_p[blk(2 * t + r + 32 * e, 8), strip(cc + 4 * d)])
                                  for e in range(2) for d in range(2)])
            for e, m in enumerate(RSUM):
                wob5[e, blk(2 * t + r, 8), strip(cc)] = ops[m]
            return [], 0, lambda: wob5[_zero(t, 0), blk(2 * t + r, 8), strip(cc)]

        segs, step = (P0S, P0T) if peel else (P1S, 32)
        sched = _Sched(t > 99, _plan1(segs, P0W * peel, step, P0N if peel else P1N), dict(
            x=[part(act_sums, x_r, xq, 2, m, sr, r)
               for m in range(7) for sr in range(2) for r in range(2)],
            c=[part(act_sums, c_r, cq, 1, m, 0, r) for m in range(7) for r in range(2)],
            v=[part(v_sums, r, cc) for r in range(2) for cc in range(4)],
            o=[part(o_sums, r, cc) for r in range(2) for cc in range(4)]))

        first = t < 2
        for k, (half, r0, n) in enumerate(segs):
            if k == P0W * peel:
                if peel:
                    for d in group0[1:-3]:
                        d.wait()
                load_wv()
            w = jnp.concatenate([wperm[4 * half + cc] for cc in range(4)], axis=1)
            r = sched.mm(k, xs_u[t >> 1, pl.ds(r0 // 2, n // 2), :], w, step=step)
            for cc in range(4):
                sl = (8 * (t & 1) + 4 * half + cc, pl.ds(PAD + r0, n), slice(None))
                new = r[:, cc * 128:(cc + 1) * 128]
                qk_b[sl] = new if peel else jnp.where(first, 0.0, qk_b[sl]) + new
        sched.finish()
        stage_first(t + 1)
        d = group(t + 2)
        for d in d[2:] + d[:2]:
            d.start()
        return t

    zero = jnp.max(vb[0, pl.ds(TQ, 8), :]).astype(jnp.int32)
    cp_w(0, sem_a.at[1]).wait()
    stage_first(0)
    group(1)[1].start()
    for t in range(2):
        cp_x(-t, sem_a.at[2]).wait()
    p1_step(zero, True)
    for d in cp_p(0) + (cp_gw(),):
        d.start()
    for d in group0[-3:]:
        d.wait()
    last = jax.lax.fori_loop(1, 16, lambda t, c: p1_step(t, False), 0)

    row = jax.lax.broadcasted_iota(jnp.int32, (TQ, TQ), 0)
    col = jax.lax.broadcasted_iota(jnp.int32, (TQ, TQ), 1)
    col = (col & ~31) | ((col & 1) << 4) | ((col & 31) >> 1)
    rowi = jax.lax.broadcasted_iota(jnp.int32, (RB, 128), 0)
    odd = (jax.lax.broadcasted_iota(jnp.int32, (RB, 128), 1) & 1) == 1
    NSUB = HQ // RB
    QSCALE = DA ** -0.5 * LOG2E

    def pair_rows(src, slot, r0, n, gate):
        return [_split(gate(src[slot, pl.ds(r0 + par, n // 2, stride=2), :])) for par in range(2)]

    def staging(g, z, never):
        ns = DC // SCR

        def scales(n1, k, gate):
            res = []
            for h in range(2):
                if k < ns:
                    w = gate(wkv_r[g & 1, pl.ds(n1 * DC + k * SCR, SCR), :])
                    w = pltpu.bitcast(w, jnp.int32) & (0x7F80 << (16 * h))
                else:
                    w = gate(sc_s[2 * n1 + h, pl.ds(0, 8 * ns), :])
                e = _tree([w[r:r + 8] for r in range(0, w.shape[0], 8)], jnp.maximum)
                if k == ns:
                    e = pltpu.bitcast(e << (16 - 16 * h), F32)
                    e = jnp.max(e, axis=0, keepdims=True)
                    e = jnp.clip(pltpu.bitcast(e, jnp.int32), 1 << 23, 253 << 23)
                    e = jnp.broadcast_to(e, (8, 128))
                    sc_s[2 * n1 + h, pl.ds(8 * ns + 8, 8), :] = (254 << 23) - e
                sc_s[2 * n1 + h, pl.ds(8 * k, 8), :] = e
                res.append(pltpu.bitcast(e, U32))
            return res, 0, lambda: pltpu.bitcast(sc_s[2 * n1, blk(k + _zero(z, 0), 8), :], U32)

        def rhs49(dst, tiles, scale, m, r, extra=()):
            res = [_ops49(_rhs7,
                          [[scale(tiles[2 * (q >> 1) + (e >> 1)][q & 1][par][e & 1],
                                  2 * (q & 1) + (e & 1)) for e in range(4)] for q in range(4)],
                          m) for par in range(2)]
            for k, (lo, hi) in enumerate(zip(*res)):
                w = _join(lo, hi)
                if k < len(extra):
                    w = jnp.where(never, extra[k], w)
                dst[7 * m + k, pl.ds(8 * r, 8), :] = w

        def kv(m, r, gate):
            if m == 0 and r == 0:
                for k in range(4):
                    ups[k] = pltpu.bitcast(gate(sc_s[k, pl.ds(8 * ns, 8), :]), F32)
            down = [pltpu.bitcast(sc_s[k + _zero(z, m), pl.ds(8 * ns + 8, 8), :], F32)
                    for k in range(4)]
            tiles = [[pair_rows(wkv_r, (g & 1) + _zero(z, m), n1 * DC + kt * 128 + 16 * r, 16, gate)
                      for n1 in range(2)] for kt in range(4)]
            rhs49(wkv, tiles, lambda w, k: w * down[k], m, r)
            return [], 0, lambda: wkv[7 * m, blk(r + _zero(z, 0), 8), :]

        def qw(m, r, gate):
            tiles = [[pair_rows(wq_r, ((g + 1 + n1) & 3) + _zero(z, m), kt * 256 + 16 * r, 16, gate)
                      for n1 in range(2)] for kt in range(4)]
            rhs49(wq49, tiles, lambda w, k: w, m, r, sc.pop(0)(gate)[0] if sc else ())
            return [], 0, lambda: wq49[7 * m, blk(r + _zero(z, 0), 8), :]

        def b_lhs(u, r, gate):
            base = 8 * jnp.minimum(g + 1, NQ - 1) + r
            ops = _words7(_lhs7, [gate(xs_u[u + 4 * d, blk(base + 4 * e, 8), :])
                                  for e in range(2) for d in range(2)])
            for k, m in enumerate(LSUM):
                bx[k, pl.ds(8 * r, 8), strip(u)] = ops[m]
            return [], 0, lambda: bx[0, blk(r + _zero(z, 0), 8), strip(u)]

        sc = [part(scales, n1, k) for k in range(ns + 1) for n1 in range(2)]
        return dict(sc=sc,
                    kv=[part(kv, m, r) for m in range(7) for r in range(8)],
                    qw=[part(qw, m, r) for m in range(7) for r in range(16)],
                    bx=[part(b_lhs, u, r) for u in range(4) for r in range(4)])

    sched = _Sched(last > 99, _planx(), staging(-1, last, last > 99))
    w0 = pair_rows(wq_r, 0, 0, M, lambda x: x)
    w0 = [_join(w0[0][h], w0[1][h]) for h in range(2)]
    for g in range(4):
        for e in range(2):
            for h in range(2):
                q = [sched.mm(8 * g + 4 * e + 2 * h + k, jnp.concatenate(
                    [xs_u[4 * k + u, pl.ds((4 * g + 2 + e) * HQ, HQ), :] for u in range(4)], axis=1),
                    w0[h][256 * k:256 * k + 256], step=16) for k in range(2)]
                qn[h, g, e] = _pack((q[0] + q[1]) * QSCALE)
    sched.finish()
    for d in group(16) + group(17):
        d.wait()
    for d in cp_p(1):
        d.start()
    plan2 = _plan2()

    def p2_body(p, carry):
        for d in cp_p(p):
            d.wait()
        causal = col <= row
        never = p > NP
        jobs = staging(p, p, never)
        sched = _Sched(never, plan2, jobs)
        mm = sched.mm

        r0 = pl.multiple_of(p * TQ, TQ)

        def scatter(dst, off, c):
            for e, t in enumerate(c):
                for cc in range(4):
                    dst[4 * (e & 1) + cc, pl.ds(off + (PAD + (e >> 1) * HQ), HQ), :] = (
                        t[:, cc * 128:(cc + 1) * 128])

        def proj_bv():
            def lhs(m):
                if m in (2, 3):
                    return jnp.concatenate([xs_u[u + 4 * (m - 2), blk(2 * p + m - 2, QQ), :]
                                            for u in range(4)], axis=1)
                return bx[LSUM.index(m)]

            for cc in range(8):
                vb[cc, pl.ds(0, PAD), :] = vb[cc, pl.ds(TQ, PAD), :]
            c = [_combine(lambda m: mm(("bv", 7 * e + ORDER.index(m)), lhs(m), jnp.concatenate(
                [wv7[m, 2 * e], wv7[m, 2 * e + 1]], axis=1))) for e in range(2)]
            scatter(vb, 0, [jnp.concatenate(t, axis=1) for t in zip(*c)])

        def local_qk(rb, k, gate):
            q = [qk_b[cc, pl.ds(r0 + _zero(p, k) + (PAD + rb * RB), RB), :] for cc in range(8)]
            q[0] = gate(q[0])
            for w in range(LG * k, LG * k + LG):
                t = _fold([q[cc] * qk_b[8 + cc, pl.ds(r0 + (PAD + rb * RB - DIL * w), RB), :]
                           for cc in range(8)], jnp.add)
                t = t + pltpu.roll(t, 64, 1)
                t = t + jnp.where(odd, pltpu.roll(t, 1, 1), pltpu.roll(t, 127, 1))
                t = t * (DB ** -0.5 * LOG2E)
                if rb == 0 and w:
                    t = jnp.where(rowi + r0 >= DIL * w, t, NEG)
                lg_s[w, pl.ds(rb * RB, RB), :] = t
            return [], 1, lambda: pltpu.bitcast(lg_s[w, blk(2 * rb + _zero(p, 0), 8), :], U32)

        def local_sm(rb, e, gate):
            rows = pl.ds(rb * RB + SMR * e, SMR)
            lg = [gate(lg_s[w, rows, :]) for w in range(WIN)]
            m = _tree(lg, jnp.maximum)
            ps = [jnp.exp2(t - m) for t in lg]
            l = _tree(ps, jnp.add)
            r = pl.reciprocal(l, approx=True)
            r = r * (2.0 - l * r)
            for w in range(WIN):
                pr_s[w, rows, :] = ps[w] * r
            return [], 2, lambda: pltpu.bitcast(pr_s[0, blk(2 * rb + e + _zero(p, 0), 8), :], U32)

        def local_pv(rb, k, gate):
            rows = pl.ds(rb * RB, RB)
            ps = [pr_s[w + _zero(p, k), rows, :] for w in range(WIN)]
            ps[0] = gate(ps[0])
            o = [_fold([ps[w] * vb[cc, pl.ds(PAD + rb * RB - DIL * w, RB), :] for w in range(WIN)],
                       jnp.add) for cc in (k, k + 4)]
            if rb < NSUB:
                for e in range(2):
                    o_s[k + 4 * e, rows, :] = o[e]
                return [], 3, lambda: pltpu.bitcast(o_s[k, blk(2 * rb + _zero(p, 0), 8), :], U32)
            top = pl.ds((rb - NSUB) * RB, RB)
            for m, t in enumerate(_lhs7(o_s[k, top, :], o_s[k + 4, top, :], *o)):
                ob7[m, pl.ds((rb - NSUB) * RB // 2, RB // 2), strip(k)] = _pack(t)
            return [], 0, lambda: ob7[0, blk(rb - NSUB + _zero(p, 0), 8), strip(k)]

        order = [rb + e * NSUB for rb in range(NSUB) for e in range(2)]
        jobs["lo"] = []
        for k in range(len(order) + SML):
            for f, d, n in ((local_sm, SML, RB // SMR), (local_qk, 0, 8 // LG)):
                if 0 <= k - d < len(order):
                    jobs["lo"] += [part(f, order[k - d], e) for e in range(n)]
        jobs["lv"] = [part(local_pv, rb, e) for rb in order for e in range(4)]

        def wob(m):
            if m == 1:
                return wob_p[pl.ds(0, M // 4), pl.ds(0, M // 2)]
            if m == 4:
                return wob_p[pl.ds(M // 4, M // 4), pl.ds(M // 2, M // 2)]
            return wob5[RSUM.index(m)]

        bo = {}

        def proj_bo(n):
            for m in ORDER[len(bo):len(bo) + n]:
                bo[m] = mm(("bo", len(bo)), lambda: ob7[m], wob(m))
            if n and len(bo) == 7:
                scatter(qk_b, r0, _combine(lambda m: bo[m]))

        def out_weights(m, r, gate):
            ww = [[gate(wo_r[(p & 1) + _zero(p, m),
                             pl.ds((2 * (q >> 1) + (e >> 1)) * HQ + 8 * r, 8),
                             pl.ds((2 * (q & 1) + (e & 1)) * 128, 128)])
                   for e in range(4)] for q in range(4)]
            rows = blk(8 * (p >> 1) + r, 8)
            extra = jobs["sc"].pop(0)(gate)[0] if jobs["sc"] else []
            for n, w in enumerate(_words49(_rhs7, ww, m)):
                if n < len(extra):
                    w = jnp.where(never, extra[n], w)
                wo49[7 * m + n, p & 1, rows, :] = w
            return [], 0, lambda: wo49[7 * m + _zero(p, 0), p & 1, rows, :]

        jobs["wo"] = [part(out_weights, m, r) for m in range(7) for r in range(8)]

        ks, vs, qs = {}, {}, {}
        done, prods = {}, {}

        def project(kind, j, n, lhs, rhs, scale, pack):
            got = prods.setdefault((kind, j), {})
            for m in ORDER[len(got):len(got) + n]:
                got[m] = _combine(lambda k: mm((kind, j, 7 * len(got) + ORDER.index(k)),
                                               lhs(7 * m + k), rhs[7 * m + k]))
            if len(got) < 7:
                return None
            c = _combine(lambda m: got[m])
            c = [[pack(c[(rg & 2) + (cg >> 1)][2 * (rg & 1) + (cg & 1)] * scale(cg))
                  for rg in range(4)] for cg in range(4)]
            return [[jnp.concatenate([t[16 * e:16 * e + 16] for t in c[cg]], axis=0)
                     for e in range(2)] for cg in range(4)]

        def proj_kv(j, n):
            c = project("kv", j, n, lambda k: cq[k, 0, pl.ds(j * QQ, QQ), :], wkv,
                        lambda cg: ups[cg][:1], _riffle)
            if c is not None:
                for cg in range(4):
                    for e in range(2):
                        (vs, ks)[cg >> 1][(cg & 1, 2 * j + e)] = c[cg][e]

        def proj_q(g, n):
            rows = blk(2 * g + (p & 1), QQ)
            c = project("q", g, n,
                        lambda k: jnp.concatenate([xq[k, sr, rows, :] for sr in range(2)], axis=1),
                        wq49, lambda cg: QSCALE, _pack)
            if c is not None:
                for h in range(2):
                    for e in range(2):
                        old = qn[h, g, e]
                        for b in range(2):
                            qs[(h, 4 * g + 2 * b + e)] = jnp.where((p & 1) == b, c[h][e], old)
                        qn[h, g, e] = c[2 + h][e]

        def qk(h, i, dep):
            kk = jnp.concatenate([ks[(h, j)] for j in range(i + 1)], axis=0)
            q = qs[(h, i)]
            if dep is not None:
                q = jnp.where(never, done[(h, dep)], q)
            ch = _lane_chunks(mm(("qk", h, i), q, kk, NT, 512))
            ch[i] = jnp.where(causal, ch[i], NEG)
            return ch

        def softmax_pv(h, i, ch):
            m = jnp.max(_fold(ch, jnp.maximum), axis=1, keepdims=True)
            ps = [jnp.exp2(c - m) for c in ch]
            lp = ps[0]
            for j in range(1, i + 1):
                lp = lp + ps[j]
                if TIE and (j % TIE == TIE - 1 or j == i):
                    ps[j] = jnp.where(never, lp, ps[j])
            pb = jnp.concatenate(ps, axis=1).astype(BF16)
            vv = jnp.concatenate([vs[(h, j)] for j in range(i + 1)], axis=0)
            o = mm(("pv", h, i), pb, vv)
            if i >= LDEP:
                lp = jnp.where(never, o, lp)
            l = jnp.sum(lp, axis=1, keepdims=True)
            r = pl.reciprocal(l, approx=True)
            r = r * (2.0 - l * r)
            cn = _pack(o * r)
            done[(h, i)] = cn
            if FA <= i < NQ - 1:
                if h == 0 and F0 < 0:
                    site = ("qk", 1, i + 1)
                elif i + 3 < NQ:
                    site = ("kv", (i + 1) // 2 + 1, KVS * ((i + 1) & 1) + (F0, FD)[h])
                else:
                    site = ("bo", (i + 3 - NQ) * BOP[0] + h)
                sched.pending.setdefault(site, []).append(cn)
            ctx[2 * p + h, pl.ds(i * HQ, HQ), :] = cn

        proj_bv()
        proj_kv(0, 7)
        proj_q(0, 7)
        for i in range(NQ):
            dep = i - DEP if DEP <= i < FA + DEP else None
            s0 = qk(0, i, dep)
            s1 = qk(1, i, dep)
            if i + 2 < NQ:
                proj_kv(i // 2 + 1, 7 if i & 1 else KVS // 7)
                if i < 6:
                    proj_q(i // 2 + 1, 7 if i & 1 else QS // 7)
            else:
                proj_bo(BOP[i + 2 - NQ])
            softmax_pv(0, i, s0)
            softmax_pv(1, i, s1)
        proj_bo(BOP[2])
        sched.finish()
        for d in cp_p(p + 2):
            d.start()
        return carry

    jax.lax.fori_loop(0, NP, p2_body, 0)

    cp_gw().wait()
    gw = gw_ref[...].astype(F32)
    plan3 = _plan3()
    cab = (ca0, ca1)

    def p3_body(i, carry):
        r0 = pl.multiple_of(i * TO, TO)
        h0 = pl.multiple_of(i * (TO // 2), TO // 2)
        never = i > S

        def ctx_words(m, u, r, n):
            return [[ctx[4 * u + 2 * (q & 1) + (e & 1),
                         pl.ds(h0 + _zero(i, m) * 8 + ((2 * (q >> 1) + (e >> 1)) * QQ + r), n), :]
                     for e in range(4)] for q in range(4)]

        def operands(k, u, r, gate):
            m = ORDER[k]
            cw = [[gate(w) for w in q] for q in ctx_words(m, u, r, 8)]
            for n, w in enumerate(_words49(_lhs7, cw, m)):
                if not (m in (2, 3) and n in (2, 3)):
                    cab[k & 1][n, pl.ds(r, 8), pl.ds(u * 128, 128)] = w
            return [], 0, lambda: cab[k & 1][_zero(i, 0), pl.ds(r, 8), pl.ds(u * 128, 128)]

        def gate_rows(r, gate):
            gs = _fold([_bf(gate(xs_u[j, pl.ds(h0 + r, 8), :])).astype(F32) * gw[j:j + 1]
                        for j in range(8)], jnp.add)
            g = jax.nn.sigmoid(jnp.sum(gs, axis=1, keepdims=True))
            g_s[pl.ds(2 * r, 16), :] = jnp.broadcast_to(g, (16, 128))
            return [], 0, lambda: pltpu.bitcast(g_s[blk(r // 4 + _zero(i, 0), 8), :], U32)

        pr = {}

        def mix(q, e, cc, gate):
            off = (2 * (q >> 1) + (e >> 1)) * HQ
            ch = 4 * cc + 2 * (q & 1) + (e & 1)
            a = _combine(lambda m: pr.get(m, pr[2])[e][:, cc * 128:(cc + 1) * 128])[q]
            g = gate(g_s[pl.ds(off, HQ), :])
            b = qk_b[ch, pl.ds(r0 + (PAD + off), HQ), :]
            out_s[pl.ds(r0 + off, HQ), pl.ds(ch * 128, 128)] = (g * a + (1.0 - g) * b).astype(BF16)
            return [], 0, lambda: pltpu.bitcast(
                out_s[blk(i * (TO // 16) + off // 16 + _zero(i, 0), 16), pl.ds(ch * 128, 128)], U32)

        sched = _Sched(never, plan3, dict(
            a=[part(operands, k, u, r) for k in range(1, 7) for u in range(HA // 4)
               for r in range(0, QQ, 8)],
            g=[part(gate_rows, r) for r in range(0, TO // 2, 8)],
            m=[part(mix, q, e, cc) for q in (1, 2, 0) for e in range(4) for cc in range(2)]))
        first = [[_words49(_lhs7, ctx_words(ORDER[0], u, 0, QQ), ORDER[0])[n]
                  for u in range(HA // 4)] for n in range(7)]

        def inner(m, n):
            k = ORDER.index(m)
            res = []
            for e in range(2):
                us = range(4 * e, 4 * e + 4)
                if m in (2, 3) and n in (2, 3):
                    lhs = jnp.concatenate([ctx_words(m, u, 0, QQ)[3 * (m - 2)][3 * (n - 2)]
                                           for u in us], axis=1)
                elif k == 0:
                    lhs = jnp.concatenate([first[n][u] for u in us], axis=1)
                else:
                    lhs = lambda: cab[k & 1][n, :, pl.ds(e * 512, 512)]
                rhs = jnp.concatenate([wo49[7 * m + n, cc, pl.ds(e * 256, 256), :]
                                       for cc in range(2)], axis=1)
                res.append(sched.mm((k, 2 * ORDER.index(n) + e), lhs, rhs))
                if (k, 2 * ORDER.index(n) + e) == (6, P3D):
                    for d in cp_out(i, 0):
                        d.start()
            return res[0] + res[1]

        for m in ORDER:
            pr[m] = _combine(lambda n: inner(m, n))
        sched.finish()
        for e in (1, 2, 0, 3):
            for cc in range(2):
                mix(3, e, cc, lambda x: x)
        for d in cp_out(i, 1):
            d.start()
        return carry

    jax.lax.fori_loop(0, S // TO, p3_body, 0)
    for g in range(NP, NP + 2):
        for d in cp_p(g):
            d.wait()
    for i in range(S // TO):
        for d in cp_out(i, 0) + cp_out(i, 1):
            d.wait()


@jax.jit
def pallas_gated_mix__compressed_kv_cla__sliding_local_dilated__prompt_kernel(
    A_x: jax.Array,
    A_c_kv: jax.Array,
    A_w_q: jax.Array,
    A_w_uk: jax.Array,
    A_w_uv: jax.Array,
    A_w_o: jax.Array,
    B_x: jax.Array,
    B_wqkv: jax.Array,
    B_wo: jax.Array,
    gate_w: jax.Array,
):
    del B_x
    any_spec = pl.BlockSpec(memory_space=pl.ANY)
    out = pl.pallas_call(
        _kernel,
        in_specs=[any_spec] * 9,
        out_specs=any_spec,
        out_shape=jax.ShapeDtypeStruct((S, M), BF16),
        scratch_shapes=[
            pltpu.VMEM((9, S // 2, 128), U32),
            pltpu.VMEM((2, HQ, M), U32),
            pltpu.VMEM((2, HQ, DC), U32),
            pltpu.VMEM((2, 128, M), BF16),
            pltpu.VMEM((2, 2, 32, M), BF16),
            pltpu.VMEM((M // 2, M), U32),
            pltpu.VMEM((3, 2 * DC, 128), U32),
            pltpu.VMEM((4, M, 128), U32),
            pltpu.VMEM((2, 2 * DA, M // 2), U32),
            pltpu.VMEM((8, 64, 128), U32),
            pltpu.VMEM((49, 2, S // 8, 128), U32),
            pltpu.VMEM((49, 1, S // 8, 128), U32),
            pltpu.VMEM((7, 4, M // 4, 128), U32),
            pltpu.VMEM((5, M // 4, M // 2), U32),
            pltpu.VMEM((49, 2, NP * QQ, 128), U32),
            pltpu.VMEM((49, HQ, 128), U32),
            pltpu.VMEM((49, TQ, 128), U32),
            pltpu.VMEM((4, 8, 128), F32),
            pltpu.VMEM((4, DC // SCR * 8 + 16, 128), jnp.int32),
            pltpu.VMEM((5, QQ, M // 2), U32),
            pltpu.VMEM((2, 4, 2, HQ, 128), U32),
            pltpu.VMEM((16, S + PAD, 128), F32),
            pltpu.VMEM((8, TQ + PAD, 128), F32),
            pltpu.VMEM((WIN, TQ, 128), F32),
            pltpu.VMEM((WIN, TQ, 128), F32),
            pltpu.VMEM((8, HQ, 128), F32),
            pltpu.VMEM((7, QQ, M // 2), U32),
            pltpu.VMEM((HA, S // 2, 128), U32),
            pltpu.VMEM((7, QQ, M), U32),
            pltpu.VMEM((7, QQ, M), U32),
            pltpu.VMEM((TO, 128), F32),
            pltpu.VMEM((S, M), BF16),
            pltpu.VMEM((8, 128), BF16),
            pltpu.SemaphoreType.DMA((2,)),
            pltpu.SemaphoreType.DMA((2,)),
            pltpu.SemaphoreType.DMA((3,)),
        ],
        compiler_params=pltpu.CompilerParams(vmem_limit_bytes=120 * 1024 * 1024,
                                             disable_bounds_checks=True),
    )(
        A_x.reshape(S, M),
        A_c_kv.reshape(S, DC),
        A_w_q,
        A_w_uk,
        A_w_uv,
        A_w_o.reshape(HA * DA, M),
        B_wqkv.reshape(2, M // 2, 3 * M),
        B_wo.reshape(HB // 2, 2, DB, M),
        gate_w.reshape(8, 128),
    )
    return out.reshape(1, S, M)
```

```python
import functools
import math

import jax
import jax.numpy as jnp
import jax.experimental.pallas as pl
import jax.experimental.pallas.tpu as pltpu

F32 = jnp.float32
BF16 = jnp.bfloat16
U32 = jnp.uint32

S = 2048
M = 1024
HA = 32
DA = 128
DC = 512
HB = 32
DB = 32
WIN = 8
DIL = 2
PAD = 16
LOG2E = math.log2(math.e)
NEG = -1e9

TQ = 128
HQ = TQ // 2
QQ = TQ // 4
BOP = (2, 3, 2)
LX = 16
KVS = 28
QS = 28
QST = 2
LQ0 = 1
LG = 2
XN = 28
SK = 3
SMR = 16
P1N = 108
P1A = 70
P0W = 1
P0T = 16
P0N = 98
P0S = ((0, 0, 2048), (1, 0, 1024), (1, 1024, 768), (1, 1792, 256))
P1S = tuple((h, r, 512) for h in range(2) for r in range(0, S, 512))
P3S = 4
P3M = 6
P3D = 8
P3E = 12
NQ = S // TQ
NP = HA // 2
DEP = 2
SCR = 32
LN = 80
SML = 1
LE = 2
LI = 99
LA = 24
LB = 4
LS = 1
BS = 2
LP = ("kv", 1, 8)
BX = 8
BE = 42
FA = 6
F0 = 0
FD = 8
TIE = 4
RB = 16
LDEP = 4
TO = 256
NN = (((1,), (0,)), ((), ()))
NT = (((1,), (1,)), ((), ()))


def _plan2():
    plan = {}

    def put(name, count, start, until):
        plan.setdefault(start, []).extend([(name, until)] * count)

    def after_qk(i):
        if i >= NQ - 2:
            return ("bo", 0, 7 * (i - NQ + 2) * BOP[0] + BX)
        return ("kv", i // 2 + 1, KVS * (i & 1) + LX)

    def fill(name, count, sites):
        for start, room, until in sites:
            n = min(count, room - len(plan.get(start, ())))
            put(name, n, start, until)
            count -= n
        assert count == 0, (name, count)

    def qk_sites(lo, hi):
        return [(("qk", h, i), max(i + 1 - h * SK, 0), after_qk(i))
                for i in range(lo, hi) for h in range(2)]

    def q_sites(g, lo, hi, until):
        return [(("q", g, k), 1, until) for k in range(lo, hi, QST)]

    ticks = ([("bv", 0, k) for k in range(LA, 49, LS)] + [("kv", 0, k) for k in range(0, 49, 2)]
             + [("q", 0, k) for k in range(49)])
    for name, site in zip(_spread(["lo"] * (64 // LG + 128 // SMR), LN), ticks):
        put(name, 1, site, LP)
    first = [(site, 1, ("kv", 1, 8)) for site in ticks[LN + LI:-LB:LE]]
    host = [(("bv", 0, k), 1, ("kv", 0, 8)) for k in range(0, min(LA, 46), BS)]
    early = []
    for g in range(1, 4):
        early += q_sites(g, 0, QS - 4, after_qk(2 * g - 1))
        early += qk_sites(max(2 * g - 1, LQ0), 2 * g)
        early += q_sites(g, QS, 45, after_qk(2 * g))
        early += qk_sites(max(2 * g, LQ0), 2 * g + 1)
    fill("lv", 32, first + early)
    fill("wo", 56, host + early)
    fill("os", 28, early + qk_sites(7, 14))
    fill("qw", 112, qk_sites(7, 14))
    fill("kv", 56, qk_sites(14, 16) + [(("bo", 0, k), 1, ("bo", 0, BE))
                                       for k in range(7 * BOP[0], 35)])
    return plan


def _planx():
    names = _spread(["qw"] * 112 + ["kv"] * 56, 8 * XN)
    return {k: [(n, 31) for n in names[8 * k:8 * k + 8]] for k in range(XN)}


def _spread(names, ticks):
    out = [None] * ticks
    for k, name in enumerate(names):
        out[k * ticks // len(names)] = name
    return out


def _plan1(segs, lo, step, count):
    end = len(segs) - 1
    ticks = [k for k in range(lo, end) for _ in range(segs[k][2] // step)][:count]
    n = len(ticks) * P1A // 100
    names = _spread(["x"] * 28 + ["c"] * 14 + ["o"] * 14, n) + _spread(["v"] * 14, len(ticks) - n)
    plan = {}
    for k, name in zip(ticks, names):
        plan.setdefault(k, []).append((name, end))
    return plan


def _plan3():
    plan = {}
    for k in range(6):
        lo = P3S if k == 0 else 0
        extra = ["g"] * 8 if k in (1, 2) else []
        names = _spread(["a"] * 32 + extra, 4 * (P3E - lo))
        for d in range(lo, P3E):
            plan[(k, d)] = [(n, (k + 1, 0)) for n in names[4 * (d - lo):4 * (d - lo) + 4]]
    names = _spread(["m"] * 24, 4 * P3M)
    for d in range(P3M):
        plan[(6, d)] = [(n, (6, P3D)) for n in names[4 * d:4 * d + 4]]
    return plan


_STAGES = ((2, 4), (1, 3), (0, 2), (0, 6), (0, 1))


def _permute8(cols):
    cols = list(cols)
    lane = jax.lax.broadcasted_iota(jnp.int32, cols[0].shape, 1)
    for va, lb in _STAGES:
        lo = (lane & (1 << lb)) == 0
        sh = 1 << lb
        idx = [i for i in range(8) if not (i >> va) & 1]
        if lb == 6:
            rr = [pltpu.roll(jnp.where(lo, cols[i | (1 << va)], cols[i]), 64, 1) for i in idx]
            for i, r in zip(idx, rr):
                a, b = cols[i], cols[i | (1 << va)]
                cols[i] = jnp.where(lo, a, r)
                cols[i | (1 << va)] = jnp.where(lo, r, b)
        else:
            rb = [pltpu.roll(cols[i | (1 << va)], sh, 1) for i in idx]
            ra = [pltpu.roll(cols[i], 128 - sh, 1) for i in idx]
            for i, xa, xb in zip(idx, ra, rb):
                a, b = cols[i], cols[i | (1 << va)]
                cols[i] = jnp.where(lo, a, xb)
                cols[i | (1 << va)] = jnp.where(lo, xa, b)
    return cols


def _pack(x):
    return pltpu.bitcast(x.astype(BF16), U32)


def _bf(x):
    return pltpu.bitcast(x, BF16)


def _split(w):
    return (pltpu.bitcast(w << 16, F32), pltpu.bitcast(w & jnp.uint32(0xFFFF0000), F32))


def _join(lo, hi):
    return pltpu.bitcast(pltpu.pack_elementwise([lo, hi], packed_dtype=BF16), U32)


def _riffle(x):
    return jnp.concatenate([_join(x[r:r + 16], x[r + 16:r + 32]) for r in range(0, x.shape[0], 32)],
                           axis=0)


def _lhs7(a11, a12, a21, a22):
    return [a11 + a22, a21 + a22, a11, a22, a11 + a12, a21 - a11, a12 - a22]


def _rhs7(b11, b12, b21, b22):
    return [b11 + b22, b11, b12 - b22, b21 - b11, b22, b11 + b12, b21 + b22]


def _combine(mm):
    add = functools.partial(jax.tree.map, jnp.add)
    sub = functools.partial(jax.tree.map, jnp.subtract)
    m2 = mm(2)
    m3 = mm(3)
    m4 = mm(4)
    c12 = add(m2, m4)
    t11 = sub(m3, m4)
    m1 = mm(1)
    c21 = add(m1, m3)
    t22 = sub(m2, m1)
    m0 = mm(0)
    t11 = add(t11, m0)
    t22 = add(t22, m0)
    c11 = add(t11, mm(6))
    return c11, c12, c21, add(t22, mm(5))


ORDER = (2, 3, 4, 1, 0, 6, 5)


def _zero(i, m):
    return i >> (8 + m)


def _merge(vals):
    return _fold([v[r:r + 8, c:c + 128] for v in vals for r in range(0, v.shape[0], 8)
                  for c in range(0, v.shape[1], 128)], jnp.bitwise_or)


def _gate(never, g):
    def gate(x):
        t = jnp.tile(pltpu.bitcast(g, x.dtype), (x.shape[0] // 8, x.shape[1] // 128))
        return jnp.where(never, t, x)
    return gate


def _tie(never, x, deps):
    if not deps:
        return x
    top = jnp.where(never, _merge(deps), x[:8, :128])
    if x.shape[1] > 128:
        top = jnp.concatenate([top, x[:8, 128:]], axis=1)
    return jnp.concatenate([top, x[8:]], axis=0)


class _Sched:
    def __init__(self, never, plan, jobs):
        self.never, self.plan, self.jobs, self.pending = never, plan, jobs, {}

    def mm(self, site, a, b, dims=NN, width=128, step=32):
        deps = [d() if callable(d) else d for d in self.pending.pop(site, ())]
        a = a() if callable(a) else a
        tie = functools.partial(_tie, self.never, deps=deps)
        a, b = (_bf(tie(a)), _bf(b)) if a.dtype == U32 else (a, _bf(tie(b)))
        out = jax.lax.dot_general(a, b, dims, preferred_element_type=F32)
        per = out.shape[0] // step
        last = {}
        for k, (name, until) in enumerate(self.plan.get(site, ())):
            if name is not None:
                r, c = step * (k % per), width * (k // per)
                vals, tag, stored = self.jobs[name].pop(0)(
                    _gate(self.never, out[r:r + 8, c:c + 128]))
                self.pending.setdefault(until, []).extend(vals)
                last[(name, tag, until)] = stored
        for (_, _, until), stored in last.items():
            if stored is not None:
                self.pending[until].append(stored)
        return out

    def finish(self):
        assert not any(self.jobs.values()) and not any(self.pending.values())


def _ops49(fn, blocks, m):
    return fn(*[fn(*[blocks[q][e] for q in range(4)])[m] for e in range(4)])


def _words49(fn, words, m):
    halves = [[_split(w) for w in q] for q in words]
    lo = _ops49(fn, [[h[0] for h in q] for q in halves], m)
    hi = _ops49(fn, [[h[1] for h in q] for q in halves], m)
    return [_join(a, b) for a, b in zip(lo, hi)]


def _fold(xs, op):
    acc = xs[0]
    for x in xs[1:]:
        acc = op(acc, x)
    return acc


def _tree(xs, op):
    while len(xs) > 1:
        xs = [op(a, b) for a, b in zip(xs[::2], xs[1::2])]
    return xs[0]


def _lane_chunks(x):
    return [x[:, j * 128:(j + 1) * 128] for j in range(x.shape[1] // 128)]


def _kernel(x_hbm, c_hbm, wq_hbm, wuk_hbm, wuv_hbm, wo_hbm, wqkv_hbm, wob_hbm, gw_hbm,
            out_hbm,
            xs_u, x_r, c_r, w_r, wv_r, wob_r, wkv_r, wq_r, wo_r,
            wperm, xq, cq, wv49, wob49, wo49, wkv, wq49, ups, sc_s, qn,
            qk_b, vb, lg_s, pr_s, o_s, ob49, ctx, ca0, ca1, g_s, out_s, gw_ref,
            sem_x, sem_p, sem_a):
    x_u = x_hbm.bitcast(U32)
    c_u = c_hbm.bitcast(U32)
    wo_u = wo_hbm.bitcast(U32)
    wq_u = wq_hbm.bitcast(U32)
    wuk_u = wuk_hbm.bitcast(U32)
    wuv_u = wuv_hbm.bitcast(U32)
    wob_u = wob_hbm.bitcast(U32)
    part = functools.partial

    def blk(j, n):
        return pl.ds(pl.multiple_of(j * n, n), n)

    def strip(j):
        return blk(j, 128)

    def cp_x(t, sem):
        k = (t + 1) >> 1
        return pltpu.make_async_copy(x_u.at[blk(t & 1, S // 4), strip(jnp.minimum(k, 7))],
                                     xs_u.at[jnp.minimum(k, 8), blk(t & 1, S // 4), :], sem)

    def cp_w(t, sem):
        u = t - 2 * (t >> 4)
        u = u - 2 * (u >> 4)
        return pltpu.make_async_copy(wqkv_hbm.at[u >> 3, strip((u >> 1) & 3), blk(u & 1, M)],
                                     w_r.at[u & 1], sem)

    def cp_wob(t, sem):
        b = (t + 1) >> 1
        c = jnp.minimum(b, 7)
        return tuple(pltpu.make_async_copy(
            wob_u.at[:, c & 1, 4 * (2 * (t & 1) + j) + (c & 2) + (c >> 2), :],
            wob_r.at[b & 1, 2 * (t & 1) + j], sem) for j in range(2))

    def group(t, sem2=None):
        sem = sem_x.at[t & 1]
        sem2 = sem if sem2 is None else sem2
        late = t >> 4
        u = t - 2 * late
        pq = (t >> 3) + late
        return (
            cp_x(t, sem),
            cp_w(t + 1, sem),
            pltpu.make_async_copy(x_u.at[blk(u, HQ), :], x_r.at[u & 1], sem),
            pltpu.make_async_copy(c_u.at[blk(u, HQ), :], c_r.at[u & 1], sem),
        ) + cp_wob(t, sem) + tuple(
            pltpu.make_async_copy(wqkv_hbm.at[e >> 1, blk(16 * (e & 1) + u, 16), pl.ds(2 * M, M)],
                                  wv_r.at[u & 1, e], sem) for e in range(4)) + (
            pltpu.make_async_copy(wq_u.at[strip(t & 7), pq, :], wq_r.at[pq, strip(t & 7), :], sem2),
            pltpu.make_async_copy(wuk_u.at[blk(u, 32), 0, :],
                                  wkv_r.at[1 + late, blk(16 + u, 32), :], sem2),
            pltpu.make_async_copy(wuv_u.at[blk(u, 32), 0, :],
                                  wkv_r.at[1 + late, blk(u, 32), :], sem2),
        )

    def cp_wq(p, sem):
        return pltpu.make_async_copy(wq_u.at[:, jnp.minimum(p, NP - 1), :], wq_r.at[p & 3], sem)

    def cp_p(g):
        slot = g & 1
        p = jnp.minimum(g + 1, NP - 1)
        o = jnp.minimum(g, NP - 1)
        sem = sem_p.at[slot]
        return (
            pltpu.make_async_copy(wo_u.at[blk(o >> 1, 2 * DA), blk(o & 1, M // 2)],
                                  wo_r.at[slot], sem),
            pltpu.make_async_copy(wuk_u.at[:, p, :], wkv_r.at[slot, pl.ds(DC, DC), :], sem),
            pltpu.make_async_copy(wuv_u.at[:, p, :], wkv_r.at[slot, pl.ds(0, DC), :], sem),
            cp_wq(g + 2, sem),
        )

    def cp_gw():
        return pltpu.make_async_copy(gw_hbm, gw_ref, sem_a.at[0])

    def cp_out(i, late):
        def cp(rows, cols):
            return pltpu.make_async_copy(out_s.at[rows, cols], out_hbm.at[rows, cols], sem_a.at[1])

        low = [cp(blk(2 * i + 1, TO // 2), pl.ds(512 * cc + 256 * late, 256)) for cc in range(2)]
        return low if late else [cp(blk(2 * i, TO // 2), pl.ds(0, M))] + low

    cp_w(0, sem_a.at[1]).start()
    for t in range(2):
        cp_x(-t, sem_a.at[2]).start()
    group0 = group(0, sem_p.at[1])
    group0 = group0[:-3] + cp_wob(-1, sem_x.at[0]) + group0[-3:]
    for d in group0[1:] + group(1)[:1] + group(1)[2:]:
        d.start()

    for cc in range(8):
        qk_b[8 + cc, pl.ds(0, PAD), :] = jnp.zeros((PAD, 128), F32)
        vb[cc, pl.ds(TQ, PAD), :] = jnp.zeros((PAD, 128), F32)

    def stage_first(t):
        for cc, w in enumerate(_permute8(_lane_chunks(pltpu.bitcast(w_r[t & 1], U32)))):
            wperm[cc] = w

    def p1_step(t, peel):
        if not peel:
            for d in group(t):
                d.wait()

        def act_sums(src, dst, ns, m, sr, r, gate):
            cw = [[gate(src[(t & 1) + _zero(t, m), pl.ds(32 * (q >> 1) + 16 * (e >> 1) + 8 * r, 8),
                            pl.ds(((2 * (q & 1) + (e & 1)) * ns + sr) * 128, 128)])
                   for e in range(4)] for q in range(4)]
            for n, w in enumerate(_words49(_lhs7, cw, m)):
                dst[7 * m + n, sr, blk(2 * t + r, 8), :] = w
            return [], 0, lambda: dst[7 * m + _zero(t, 0), sr, blk(2 * t + r, 8), :]

        wv = []

        def load_wv():
            wv.extend(_permute8(_lane_chunks(jnp.concatenate(
                [pltpu.bitcast(wv_r[t & 1, e], U32) for e in range(4)], axis=0))))

        def w_sums(src, dst, m, cc, gate):
            ww = [[gate(src(m, 2 * (q >> 1) + (e >> 1), 2 * (2 * (q & 1) + (e & 1)) + cc))
                   for e in range(4)] for q in range(4)]
            for n, w in enumerate(_words49(_rhs7, ww, m)):
                dst[7 * m + n, cc, blk(t, 8), :] = w
            return [], 0, lambda: dst[7 * m + _zero(t, 0), cc, blk(t, 8), :]

        def v_src(m, rq, ch):
            return wv[ch][8 * rq:8 * rq + 8]

        def o_src(m, rq, ch):
            return wob_r[((t >> 1) & 1) + _zero(t, m), rq, blk(t & 1, 8), pl.ds(128 * ch, 128)]

        segs, step = (P0S, P0T) if peel else (P1S, 32)
        sched = _Sched(t > 99, _plan1(segs, P0W * peel, step, P0N if peel else P1N), dict(
            x=[part(act_sums, x_r, xq, 2, m, sr, r)
               for m in range(7) for sr in range(2) for r in range(2)],
            c=[part(act_sums, c_r, cq, 1, m, 0, r) for m in range(7) for r in range(2)],
            v=[part(w_sums, v_src, wv49, m, cc) for m in range(7) for cc in range(2)],
            o=[part(w_sums, o_src, wob49, m, cc) for m in range(7) for cc in range(2)]))

        first = t < 2
        for k, (half, r0, n) in enumerate(segs):
            if k == P0W * peel:
                if peel:
                    for d in group0[1:-3]:
                        d.wait()
                load_wv()
            w = jnp.concatenate([wperm[4 * half + cc] for cc in range(4)], axis=1)
            r = sched.mm(k, xs_u[t >> 1, pl.ds(r0 // 2, n // 2), :], w, step=step)
            for cc in range(4):
                sl = (8 * (t & 1) + 4 * half + cc, pl.ds(PAD + r0, n), slice(None))
                new = r[:, cc * 128:(cc + 1) * 128]
                qk_b[sl] = new if peel else jnp.where(first, 0.0, qk_b[sl]) + new
        sched.finish()
        stage_first(t + 1)
        d = group(t + 2)
        for d in d[2:] + d[:2]:
            d.start()
        return t

    zero = jnp.max(vb[0, pl.ds(TQ, 8), :]).astype(jnp.int32)
    cp_w(0, sem_a.at[1]).wait()
    stage_first(0)
    group(1)[1].start()
    for t in range(2):
        cp_x(-t, sem_a.at[2]).wait()
    p1_step(zero, True)
    for d in cp_p(0) + (cp_gw(),):
        d.start()
    for d in group0[-3:]:
        d.wait()
    last = jax.lax.fori_loop(1, 16, lambda t, c: p1_step(t, False), 0)

    row = jax.lax.broadcasted_iota(jnp.int32, (TQ, TQ), 0)
    col = jax.lax.broadcasted_iota(jnp.int32, (TQ, TQ), 1)
    col = (col & ~31) | ((col & 1) << 4) | ((col & 31) >> 1)
    rowi = jax.lax.broadcasted_iota(jnp.int32, (RB, 128), 0)
    odd = (jax.lax.broadcasted_iota(jnp.int32, (RB, 128), 1) & 1) == 1
    QSCALE = DA ** -0.5 * LOG2E

    def pair_rows(src, slot, r0, n, gate):
        return [_split(gate(src[slot, pl.ds(r0 + par, n // 2, stride=2), :])) for par in range(2)]

    def staging(g, z, never):
        ns = DC // SCR

        def scales(n1, k, gate):
            res = []
            for h in range(2):
                if k < ns:
                    w = gate(wkv_r[g & 1, pl.ds(n1 * DC + k * SCR, SCR), :])
                    w = pltpu.bitcast(w, jnp.int32) & (0x7F80 << (16 * h))
                else:
                    w = gate(sc_s[2 * n1 + h, pl.ds(0, 8 * ns), :])
                e = _tree([w[r:r + 8] for r in range(0, w.shape[0], 8)], jnp.maximum)
                if k == ns:
                    e = pltpu.bitcast(e << (16 - 16 * h), F32)
                    e = jnp.max(e, axis=0, keepdims=True)
                    e = jnp.clip(pltpu.bitcast(e, jnp.int32), 1 << 23, 253 << 23)
                    e = jnp.broadcast_to(e, (8, 128))
                    sc_s[2 * n1 + h, pl.ds(8 * ns + 8, 8), :] = (254 << 23) - e
                sc_s[2 * n1 + h, pl.ds(8 * k, 8), :] = e
                res.append(pltpu.bitcast(e, U32))
            return res, 0, lambda: pltpu.bitcast(sc_s[2 * n1, blk(k + _zero(z, 0), 8), :], U32)

        def rhs49(dst, tiles, scale, m, r, extra=()):
            res = [_ops49(_rhs7,
                          [[scale(tiles[2 * (q >> 1) + (e >> 1)][q & 1][par][e & 1],
                                  2 * (q & 1) + (e & 1)) for e in range(4)] for q in range(4)],
                          m) for par in range(2)]
            for k, (lo, hi) in enumerate(zip(*res)):
                w = _join(lo, hi)
                if k < len(extra):
                    w = jnp.where(never, extra[k], w)
                dst[7 * m + k, pl.ds(8 * r, 8), :] = w

        def kv(m, r, gate):
            if m == 0 and r == 0:
                for k in range(4):
                    ups[k] = pltpu.bitcast(gate(sc_s[k, pl.ds(8 * ns, 8), :]), F32)
            down = [pltpu.bitcast(sc_s[k + _zero(z, m), pl.ds(8 * ns + 8, 8), :], F32)
                    for k in range(4)]
            tiles = [[pair_rows(wkv_r, (g & 1) + _zero(z, m), n1 * DC + kt * 128 + 16 * r, 16, gate)
                      for n1 in range(2)] for kt in range(4)]
            rhs49(wkv, tiles, lambda w, k: w * down[k], m, r)
            return [], 0, lambda: wkv[7 * m, blk(r + _zero(z, 0), 8), :]

        def qw(m, r, gate):
            tiles = [[pair_rows(wq_r, ((g + 1 + n1) & 3) + _zero(z, m), kt * 256 + 16 * r, 16, gate)
                      for n1 in range(2)] for kt in range(4)]
            rhs49(wq49, tiles, lambda w, k: w, m, r, sc.pop(0)(gate)[0] if sc else ())
            return [], 0, lambda: wq49[7 * m, blk(r + _zero(z, 0), 8), :]

        sc = [part(scales, n1, k) for k in range(ns + 1) for n1 in range(2)]
        return dict(sc=sc,
                    kv=[part(kv, m, r) for m in range(7) for r in range(8)],
                    qw=[part(qw, m, r) for m in range(7) for r in range(16)])

    sched = _Sched(last > 99, _planx(), staging(-1, last, last > 99))
    w0 = pair_rows(wq_r, 0, 0, M, lambda x: x)
    w0 = [_join(w0[0][h], w0[1][h]) for h in range(2)]
    for g in range(4):
        for e in range(2):
            for h in range(2):
                q = [sched.mm(8 * g + 4 * e + 2 * h + k, jnp.concatenate(
                    [xs_u[4 * k + u, pl.ds((4 * g + 2 + e) * HQ, HQ), :] for u in range(4)], axis=1),
                    w0[h][256 * k:256 * k + 256], step=16) for k in range(2)]
                qn[h, g, e] = _pack((q[0] + q[1]) * QSCALE)
    sched.finish()
    for d in group(16) + group(17):
        d.wait()
    for d in cp_p(1):
        d.start()
    plan2 = _plan2()

    def p2_body(p, carry):
        for d in cp_p(p):
            d.wait()
        causal = col <= row
        never = p > NP
        jobs = staging(p, p, never)
        sched = _Sched(never, plan2, jobs)
        mm = sched.mm

        r0 = pl.multiple_of(p * TQ, TQ)

        prods = {}

        def project(kind, j, n, lhs, rhs):
            got = prods.setdefault((kind, j), {})
            for m in ORDER[len(got):len(got) + n]:
                got[m] = _combine(lambda k: mm((kind, j, 7 * len(got) + ORDER.index(k)),
                                               part(lhs, 7 * m + k), rhs(7 * m + k)))
            if len(got) < 7:
                return None
            c = _combine(lambda m: got[m])
            return [[c[(rg & 2) + (cg >> 1)][2 * (rg & 1) + (cg & 1)] for rg in range(4)]
                    for cg in range(4)]

        def pair(ref, rows):
            return lambda k: jnp.concatenate([ref[k, sr, rows, :] for sr in range(2)], axis=1)

        def proj_b(kind, n, lhs, w, dst, off):
            c = project(kind, 0, n, lhs, pair(w, slice(None)))
            for cg in range(4 * (c is not None)):
                for rg in range(4):
                    for cc in range(2):
                        dst[2 * cg + cc, pl.ds(off + (PAD + rg * QQ), QQ), :] = (
                            c[cg][rg][:, cc * 128:(cc + 1) * 128])

        def proj_bv():
            for cc in range(8):
                vb[cc, pl.ds(0, PAD), :] = vb[cc, pl.ds(TQ, PAD), :]
            proj_b("bv", 7, pair(xq, blk(p, 16)), wv49, vb, 0)

        def proj_bo(n):
            proj_b("bo", n, pair(ob49, slice(None)), wob49, qk_b, r0)

        def local_qk(rb, k, gate):
            q = [qk_b[cc, pl.ds(r0 + _zero(p, k) + (PAD + rb * RB), RB), :] for cc in range(8)]
            q[0] = gate(q[0])
            for w in range(LG * k, LG * k + LG):
                t = _fold([q[cc] * qk_b[8 + cc, pl.ds(r0 + (PAD + rb * RB - DIL * w), RB), :]
                           for cc in range(8)], jnp.add)
                t = t + pltpu.roll(t, 64, 1)
                t = t + jnp.where(odd, pltpu.roll(t, 1, 1), pltpu.roll(t, 127, 1))
                t = t * (DB ** -0.5 * LOG2E)
                if rb == 0 and w:
                    t = jnp.where(rowi + r0 >= DIL * w, t, NEG)
                lg_s[w, pl.ds(rb * RB, RB), :] = t
            return [], 1, lambda: pltpu.bitcast(lg_s[w, blk(2 * rb + _zero(p, 0), 8), :], U32)

        def local_sm(rb, e, gate):
            rows = pl.ds(rb * RB + SMR * e, SMR)
            lg = [gate(lg_s[w, rows, :]) for w in range(WIN)]
            m = _tree(lg, jnp.maximum)
            ps = [jnp.exp2(t - m) for t in lg]
            l = _tree(ps, jnp.add)
            r = pl.reciprocal(l, approx=True)
            r = r * (2.0 - l * r)
            for w in range(WIN):
                pr_s[w, rows, :] = ps[w] * r
            return [], 2, lambda: pltpu.bitcast(pr_s[0, blk(2 * rb + e + _zero(p, 0), 8), :], U32)

        def local_pv(rb, k, gate):
            rows = pl.ds(rb * RB, RB)
            ps = [pr_s[w + _zero(p, k), rows, :] for w in range(WIN)]
            ps[0] = gate(ps[0])
            o = [_fold([ps[w] * vb[cc, pl.ds(PAD + rb * RB - DIL * w, RB), :] for w in range(WIN)],
                       jnp.add) for cc in (k, k + 4)]
            for e in range(2):
                o_s[k + 4 * e, rows, :] = o[e]
            return [], 0, lambda: pltpu.bitcast(o_s[k, blk(2 * rb + _zero(p, 0), 8), :], U32)

        def o_sums(m, cc, r, gate):
            res = [_ops49(_lhs7, [[gate(o_s[
                2 * (2 * (q & 1) + (e & 1)) + cc + _zero(p, m),
                pl.ds(QQ * (2 * (q >> 1) + (e >> 1)) + 16 * r + par, 8, stride=2), :])
                for e in range(4)] for q in range(4)], m) for par in range(2)]
            for n, (lo, hi) in enumerate(zip(*res)):
                ob49[7 * m + n, cc, pl.ds(8 * r, 8), :] = _join(lo, hi)
            return [], 0, lambda: ob49[7 * m, cc, blk(r + _zero(p, 0), 8), :]

        jobs["os"] = [part(o_sums, m, cc, r) for r in range(2) for cc in range(2) for m in range(7)]
        order = list(range(0, 8, 2)) + list(range(1, 8, 2))
        jobs["lo"] = []
        for k in range(len(order) + SML):
            for f, d, n in ((local_sm, SML, RB // SMR), (local_qk, 0, 8 // LG)):
                if 0 <= k - d < len(order):
                    jobs["lo"] += [part(f, order[k - d], e) for e in range(n)]
        jobs["lv"] = [part(local_pv, rb, e) for rb in order for e in range(4)]

        def out_weights(m, r, gate):
            ww = [[gate(wo_r[(p & 1) + _zero(p, m),
                             pl.ds((2 * (q >> 1) + (e >> 1)) * HQ + 8 * r, 8),
                             pl.ds((2 * (q & 1) + (e & 1)) * 128, 128)])
                   for e in range(4)] for q in range(4)]
            rows = blk(8 * (p >> 1) + r, 8)
            extra = jobs["sc"].pop(0)(gate)[0] if jobs["sc"] else []
            for n, w in enumerate(_words49(_rhs7, ww, m)):
                if n < len(extra):
                    w = jnp.where(never, extra[n], w)
                wo49[7 * m + n, p & 1, rows, :] = w
            return [], 0, lambda: wo49[7 * m + _zero(p, 0), p & 1, rows, :]

        jobs["wo"] = [part(out_weights, m, r) for m in range(7) for r in range(8)]

        ks, vs, qs = {}, {}, {}
        done = {}

        def blocks(c, scale, pack):
            c = [[pack(t * scale(cg)) for t in c[cg]] for cg in range(4)]
            return [[jnp.concatenate([t[16 * e:16 * e + 16] for t in c[cg]], axis=0)
                     for e in range(2)] for cg in range(4)]

        def proj_kv(j, n):
            c = project("kv", j, n, lambda k: cq[k, 0, pl.ds(j * QQ, QQ), :], lambda k: wkv[k])
            if c is not None:
                c = blocks(c, lambda cg: ups[cg][:1], _riffle)
                for cg in range(4):
                    for e in range(2):
                        (vs, ks)[cg >> 1][(cg & 1, 2 * j + e)] = c[cg][e]

        def proj_q(g, n):
            c = project("q", g, n, pair(xq, blk(2 * g + (p & 1), QQ)), lambda k: wq49[k])
            if c is not None:
                c = blocks(c, lambda cg: QSCALE, _pack)
                for h in range(2):
                    for e in range(2):
                        old = qn[h, g, e]
                        for b in range(2):
                            qs[(h, 4 * g + 2 * b + e)] = jnp.where((p & 1) == b, c[h][e], old)
                        qn[h, g, e] = c[2 + h][e]

        def qk(h, i, dep):
            kk = jnp.concatenate([ks[(h, j)] for j in range(i + 1)], axis=0)
            q = qs[(h, i)]
            if dep is not None:
                q = jnp.where(never, done[(h, dep)], q)
            ch = _lane_chunks(mm(("qk", h, i), q, kk, NT, 512))
            ch[i] = jnp.where(causal, ch[i], NEG)
            return ch

        def softmax_pv(h, i, ch):
            m = jnp.max(_fold(ch, jnp.maximum), axis=1, keepdims=True)
            ps = [jnp.exp2(c - m) for c in ch]
            lp = ps[0]
            for j in range(1, i + 1):
                lp = lp + ps[j]
                if TIE and (j % TIE == TIE - 1 or j == i):
                    ps[j] = jnp.where(never, lp, ps[j])
            pb = jnp.concatenate(ps, axis=1).astype(BF16)
            vv = jnp.concatenate([vs[(h, j)] for j in range(i + 1)], axis=0)
            o = mm(("pv", h, i), pb, vv)
            if i >= LDEP:
                lp = jnp.where(never, o, lp)
            l = jnp.sum(lp, axis=1, keepdims=True)
            r = pl.reciprocal(l, approx=True)
            r = r * (2.0 - l * r)
            cn = _pack(o * r)
            done[(h, i)] = cn
            if FA <= i < NQ - 1:
                if h == 0 and F0 < 0:
                    site = ("qk", 1, i + 1)
                elif i + 3 < NQ:
                    site = ("kv", (i + 1) // 2 + 1, KVS * ((i + 1) & 1) + (F0, FD)[h])
                else:
                    site = ("bo", 0, 7 * (i + 3 - NQ) * BOP[0] + 8 * h)
                sched.pending.setdefault(site, []).append(cn)
            ctx[2 * p + h, pl.ds(i * HQ, HQ), :] = cn

        proj_bv()
        proj_kv(0, 7)
        proj_q(0, 7)
        for i in range(NQ):
            dep = i - DEP if DEP <= i < FA + DEP else None
            s0 = qk(0, i, dep)
            s1 = qk(1, i, dep)
            if i + 2 < NQ:
                proj_kv(i // 2 + 1, 7 if i & 1 else KVS // 7)
                if i < 6:
                    proj_q(i // 2 + 1, 7 if i & 1 else QS // 7)
            else:
                proj_bo(BOP[i + 2 - NQ])
            softmax_pv(0, i, s0)
            softmax_pv(1, i, s1)
        proj_bo(BOP[2])
        sched.finish()
        for d in cp_p(p + 2):
            d.start()
        return carry

    jax.lax.fori_loop(0, NP, p2_body, 0)

    cp_gw().wait()
    gw = gw_ref[...].astype(F32)
    plan3 = _plan3()
    cab = (ca0, ca1)

    def p3_body(i, carry):
        r0 = pl.multiple_of(i * TO, TO)
        h0 = pl.multiple_of(i * (TO // 2), TO // 2)
        never = i > S

        def ctx_words(m, u, r, n):
            return [[ctx[4 * u + 2 * (q & 1) + (e & 1),
                         pl.ds(h0 + _zero(i, m) * 8 + ((2 * (q >> 1) + (e >> 1)) * QQ + r), n), :]
                     for e in range(4)] for q in range(4)]

        def operands(k, u, r, gate):
            m = ORDER[k]
            cw = [[gate(w) for w in q] for q in ctx_words(m, u, r, 8)]
            for n, w in enumerate(_words49(_lhs7, cw, m)):
                if not (m in (2, 3) and n in (2, 3)):
                    cab[k & 1][n, pl.ds(r, 8), pl.ds(u * 128, 128)] = w
            return [], 0, lambda: cab[k & 1][_zero(i, 0), pl.ds(r, 8), pl.ds(u * 128, 128)]

        def gate_rows(r, gate):
            gs = _fold([_bf(gate(xs_u[j, pl.ds(h0 + r, 8), :])).astype(F32) * gw[j:j + 1]
                        for j in range(8)], jnp.add)
            g = jax.nn.sigmoid(jnp.sum(gs, axis=1, keepdims=True))
            g_s[pl.ds(2 * r, 16), :] = jnp.broadcast_to(g, (16, 128))
            return [], 0, lambda: pltpu.bitcast(g_s[blk(r // 4 + _zero(i, 0), 8), :], U32)

        pr = {}

        def mix(q, e, cc, gate):
            off = (2 * (q >> 1) + (e >> 1)) * HQ
            ch = 4 * cc + 2 * (q & 1) + (e & 1)
            a = _combine(lambda m: pr.get(m, pr[2])[e][:, cc * 128:(cc + 1) * 128])[q]
            g = gate(g_s[pl.ds(off, HQ), :])
            b = qk_b[ch, pl.ds(r0 + (PAD + off), HQ), :]
            out_s[pl.ds(r0 + off, HQ), pl.ds(ch * 128, 128)] = (g * a + (1.0 - g) * b).astype(BF16)
            return [], 0, lambda: pltpu.bitcast(
                out_s[blk(i * (TO // 16) + off // 16 + _zero(i, 0), 16), pl.ds(ch * 128, 128)], U32)

        sched = _Sched(never, plan3, dict(
            a=[part(operands, k, u, r) for k in range(1, 7) for u in range(HA // 4)
               for r in range(0, QQ, 8)],
            g=[part(gate_rows, r) for r in range(0, TO // 2, 8)],
            m=[part(mix, q, e, cc) for q in (1, 2, 0) for e in range(4) for cc in range(2)]))
        first = [[_words49(_lhs7, ctx_words(ORDER[0], u, 0, QQ), ORDER[0])[n]
                  for u in range(HA // 4)] for n in range(7)]

        def inner(m, n):
            k = ORDER.index(m)
            res = []
            for e in range(2):
                us = range(4 * e, 4 * e + 4)
                if m in (2, 3) and n in (2, 3):
                    lhs = jnp.concatenate([ctx_words(m, u, 0, QQ)[3 * (m - 2)][3 * (n - 2)]
                                           for u in us], axis=1)
                elif k == 0:
                    lhs = jnp.concatenate([first[n][u] for u in us], axis=1)
                else:
                    lhs = lambda: cab[k & 1][n, :, pl.ds(e * 512, 512)]
                rhs = jnp.concatenate([wo49[7 * m + n, cc, pl.ds(e * 256, 256), :]
                                       for cc in range(2)], axis=1)
                res.append(sched.mm((k, 2 * ORDER.index(n) + e), lhs, rhs))
                if (k, 2 * ORDER.index(n) + e) == (6, P3D):
                    for d in cp_out(i, 0):
                        d.start()
            return res[0] + res[1]

        for m in ORDER:
            pr[m] = _combine(lambda n: inner(m, n))
        sched.finish()
        for e in (1, 2, 0, 3):
            for cc in range(2):
                mix(3, e, cc, lambda x: x)
        for d in cp_out(i, 1):
            d.start()
        return carry

    jax.lax.fori_loop(0, S // TO, p3_body, 0)
    for g in range(NP, NP + 2):
        for d in cp_p(g):
            d.wait()
    for i in range(S // TO):
        for d in cp_out(i, 0) + cp_out(i, 1):
            d.wait()


@jax.jit
def pallas_gated_mix__compressed_kv_cla__sliding_local_dilated__prompt_kernel(
    A_x: jax.Array,
    A_c_kv: jax.Array,
    A_w_q: jax.Array,
    A_w_uk: jax.Array,
    A_w_uv: jax.Array,
    A_w_o: jax.Array,
    B_x: jax.Array,
    B_wqkv: jax.Array,
    B_wo: jax.Array,
    gate_w: jax.Array,
):
    del B_x
    any_spec = pl.BlockSpec(memory_space=pl.ANY)
    out = pl.pallas_call(
        _kernel,
        in_specs=[any_spec] * 9,
        out_specs=any_spec,
        out_shape=jax.ShapeDtypeStruct((S, M), BF16),
        scratch_shapes=[
            pltpu.VMEM((9, S // 2, 128), U32),
            pltpu.VMEM((2, HQ, M), U32),
            pltpu.VMEM((2, HQ, DC), U32),
            pltpu.VMEM((2, 128, M), BF16),
            pltpu.VMEM((2, 4, 16, M), BF16),
            pltpu.VMEM((2, 4, 16, M), U32),
            pltpu.VMEM((3, 2 * DC, 128), U32),
            pltpu.VMEM((4, M, 128), U32),
            pltpu.VMEM((2, 2 * DA, M // 2), U32),
            pltpu.VMEM((8, 64, 128), U32),
            pltpu.VMEM((49, 2, S // 8, 128), U32),
            pltpu.VMEM((49, 1, S // 8, 128), U32),
            pltpu.VMEM((49, 2, M // 8, 128), U32),
            pltpu.VMEM((49, 2, M // 8, 128), U32),
            pltpu.VMEM((49, 2, NP * QQ, 128), U32),
            pltpu.VMEM((49, HQ, 128), U32),
            pltpu.VMEM((49, TQ, 128), U32),
            pltpu.VMEM((4, 8, 128), F32),
            pltpu.VMEM((4, DC // SCR * 8 + 16, 128), jnp.int32),
            pltpu.VMEM((2, 4, 2, HQ, 128), U32),
            pltpu.VMEM((16, S + PAD, 128), F32),
            pltpu.VMEM((8, TQ + PAD, 128), F32),
            pltpu.VMEM((WIN, TQ, 128), F32),
            pltpu.VMEM((WIN, TQ, 128), F32),
            pltpu.VMEM((8, TQ, 128), F32),
            pltpu.VMEM((49, 2, 16, 128), U32),
            pltpu.VMEM((HA, S // 2, 128), U32),
            pltpu.VMEM((7, QQ, M), U32),
            pltpu.VMEM((7, QQ, M), U32),
            pltpu.VMEM((TO, 128), F32),
            pltpu.VMEM((S, M), BF16),
            pltpu.VMEM((8, 128), BF16),
            pltpu.SemaphoreType.DMA((2,)),
            pltpu.SemaphoreType.DMA((2,)),
            pltpu.SemaphoreType.DMA((3,)),
        ],
        compiler_params=pltpu.CompilerParams(vmem_limit_bytes=120 * 1024 * 1024,
                                             disable_bounds_checks=True),
    )(
        A_x.reshape(S, M),
        A_c_kv.reshape(S, DC),
        A_w_q,
        A_w_uk,
        A_w_uv,
        A_w_o.reshape(HA * DA, M),
        B_wqkv.reshape(2, M // 2, 3 * M),
        B_wo.reshape(HB // 2, 2, DB, M),
        gate_w.reshape(8, 128),
    )
    return out.reshape(1, S, M)
```

```python
import functools
import math

import jax
import jax.numpy as jnp
import jax.experimental.pallas as pl
import jax.experimental.pallas.tpu as pltpu

F32 = jnp.float32
BF16 = jnp.bfloat16
U32 = jnp.uint32

S = 2048
M = 1024
HA = 32
DA = 128
DC = 512
HB = 32
DB = 32
WIN = 8
DIL = 2
PAD = 16
LOG2E = math.log2(math.e)
NEG = -1e9

TQ = 128
HQ = TQ // 2
QQ = TQ // 4
BOP = (2, 3, 2)
LX = 16
KVS = 28
QS = 28
QST = 2
LQ0 = 1
LG = 2
XN = 28
SK = 3
SMR = 16
P1N = 108
P1A = 70
P0W = 1
P0T = 16
P0N = 98
P0S = ((0, 0, 2048), (1, 0, 1024), (1, 1024, 768), (1, 1792, 256))
P1S = tuple((h, r, 512) for h in range(2) for r in range(0, S, 512))
P3S = 4
P3M = 6
P3D = 8
P3E = 12
NQ = S // TQ
NP = HA // 2
DEP = 2
SCR = 32
LN = 80
SML = 1
LE = 2
LI = 99
LA = 24
LB = 4
LS = 1
BS = 2
LP = ("kv", 1, 8)
BX = 8
BE = 42
FA = 6
F0 = 0
FD = 8
TIE = 4
RB = 16
LDEP = 4
TO = 256
NN = (((1,), (0,)), ((), ()))
NT = (((1,), (1,)), ((), ()))


def _plan2():
    plan = {}

    def put(name, count, start, until):
        plan.setdefault(start, []).extend([(name, until)] * count)

    def after_qk(i):
        if i >= NQ - 2:
            return ("bo", 0, 7 * (i - NQ + 2) * BOP[0] + BX)
        return ("kv", i // 2 + 1, KVS * (i & 1) + LX)

    def fill(name, count, sites):
        for start, room, until in sites:
            n = min(count, room - len(plan.get(start, ())))
            put(name, n, start, until)
            count -= n
        assert count == 0, (name, count)

    def qk_sites(lo, hi):
        return [(("qk", h, i), max(i + 1 - h * SK, 0), after_qk(i))
                for i in range(lo, hi) for h in range(2)]

    def q_sites(g, lo, hi, until):
        return [(("q", g, k), 1, until) for k in range(lo, hi, QST)]

    ticks = ([("bv", 0, k) for k in range(LA, 49, LS)] + [("kv", 0, k) for k in range(0, 49, 2)]
             + [("q", 0, k) for k in range(49)])
    for name, site in zip(_spread(["lo"] * (64 // LG + 128 // SMR), LN), ticks):
        put(name, 1, site, LP)
    first = [(site, 1, ("kv", 1, 8)) for site in ticks[LN + LI:-LB:LE]]
    host = [(("bv", 0, k), 1, ("kv", 0, 8)) for k in range(0, min(LA, 46), BS)]
    early = []
    for g in range(1, 4):
        early += q_sites(g, 0, QS - 4, after_qk(2 * g - 1))
        early += qk_sites(max(2 * g - 1, LQ0), 2 * g)
        early += q_sites(g, QS, 45, after_qk(2 * g))
        early += qk_sites(max(2 * g, LQ0), 2 * g + 1)
    fill("lv", 32, first + early)
    fill("wo", 56, host + early)
    fill("os", 28, early + qk_sites(7, 14))
    fill("qw", 112, qk_sites(7, 14))
    fill("kv", 56, qk_sites(14, 16) + [(("bo", 0, k), 1, ("bo", 0, BE))
                                       for k in range(7 * BOP[0], 35)])
    return plan


def _planx():
    names = _spread(["qw"] * 112 + ["kv"] * 56, 8 * XN)
    return {k: [(n, 31) for n in names[8 * k:8 * k + 8]] for k in range(XN)}


def _spread(names, ticks):
    out = [None] * ticks
    for k, name in enumerate(names):
        out[k * ticks // len(names)] = name
    return out


def _plan1(segs, lo, step, count):
    end = len(segs) - 1
    ticks = [k for k in range(lo, end) for _ in range(segs[k][2] // step)][:count]
    n = len(ticks) * P1A // 100
    names = _spread(["x"] * 28 + ["c"] * 14 + ["o"] * 14, n) + _spread(["v"] * 14, len(ticks) - n)
    plan = {}
    for k, name in zip(ticks, names):
        plan.setdefault(k, []).append((name, end))
    return plan


def _plan3():
    plan = {}
    for k in range(6):
        lo = P3S if k == 0 else 0
        extra = ["g"] * 8 if k in (1, 2) else []
        names = _spread(["a"] * 32 + extra, 4 * (P3E - lo))
        for d in range(lo, P3E):
            plan[(k, d)] = [(n, (k + 1, 0)) for n in names[4 * (d - lo):4 * (d - lo) + 4]]
    names = _spread(["m"] * 24, 4 * P3M)
    for d in range(P3M):
        plan[(6, d)] = [(n, (6, P3D)) for n in names[4 * d:4 * d + 4]]
    return plan


_STAGES = ((2, 4), (1, 3), (0, 2), (0, 6), (0, 1))


def _permute8(cols):
    cols = list(cols)
    lane = jax.lax.broadcasted_iota(jnp.int32, cols[0].shape, 1)
    for va, lb in _STAGES:
        lo = (lane & (1 << lb)) == 0
        sh = 1 << lb
        idx = [i for i in range(8) if not (i >> va) & 1]
        if lb == 6:
            rr = [pltpu.roll(jnp.where(lo, cols[i | (1 << va)], cols[i]), 64, 1) for i in idx]
            for i, r in zip(idx, rr):
                a, b = cols[i], cols[i | (1 << va)]
                cols[i] = jnp.where(lo, a, r)
                cols[i | (1 << va)] = jnp.where(lo, r, b)
        else:
            rb = [pltpu.roll(cols[i | (1 << va)], sh, 1) for i in idx]
            ra = [pltpu.roll(cols[i], 128 - sh, 1) for i in idx]
            for i, xa, xb in zip(idx, ra, rb):
                a, b = cols[i], cols[i | (1 << va)]
                cols[i] = jnp.where(lo, a, xb)
                cols[i | (1 << va)] = jnp.where(lo, xa, b)
    return cols


def _pack(x):
    return pltpu.bitcast(x.astype(BF16), U32)


def _bf(x):
    return pltpu.bitcast(x, BF16)


def _split(w):
    return (pltpu.bitcast(w << 16, F32), pltpu.bitcast(w & jnp.uint32(0xFFFF0000), F32))


def _join(lo, hi):
    return pltpu.bitcast(pltpu.pack_elementwise([lo, hi], packed_dtype=BF16), U32)


def _riffle(x):
    return jnp.concatenate([_join(x[r:r + 16], x[r + 16:r + 32]) for r in range(0, x.shape[0], 32)],
                           axis=0)


def _lhs7(a11, a12, a21, a22):
    return [a11 + a22, a21 + a22, a11, a22, a11 + a12, a21 - a11, a12 - a22]


def _rhs7(b11, b12, b21, b22):
    return [b11 + b22, b11, b12 - b22, b21 - b11, b22, b11 + b12, b21 + b22]


def _combine(mm):
    add = functools.partial(jax.tree.map, jnp.add)
    sub = functools.partial(jax.tree.map, jnp.subtract)
    m2 = mm(2)
    m3 = mm(3)
    m4 = mm(4)
    c12 = add(m2, m4)
    t11 = sub(m3, m4)
    m1 = mm(1)
    c21 = add(m1, m3)
    t22 = sub(m2, m1)
    m0 = mm(0)
    t11 = add(t11, m0)
    t22 = add(t22, m0)
    c11 = add(t11, mm(6))
    return c11, c12, c21, add(t22, mm(5))


ORDER = (2, 3, 4, 1, 0, 6, 5)


def _zero(i, m):
    return i >> (8 + m)


def _merge(vals):
    return _fold([v[r:r + 8, c:c + 128] for v in vals for r in range(0, v.shape[0], 8)
                  for c in range(0, v.shape[1], 128)], jnp.bitwise_or)


def _gate(never, g):
    def gate(x):
        t = jnp.tile(pltpu.bitcast(g, x.dtype), (x.shape[0] // 8, x.shape[1] // 128))
        return jnp.where(never, t, x)
    return gate


def _tie(never, x, deps):
    if not deps:
        return x
    top = jnp.where(never, _merge(deps), x[:8, :128])
    if x.shape[1] > 128:
        top = jnp.concatenate([top, x[:8, 128:]], axis=1)
    return jnp.concatenate([top, x[8:]], axis=0)


class _Sched:
    def __init__(self, never, plan, jobs):
        self.never, self.plan, self.jobs, self.pending = never, plan, jobs, {}

    def mm(self, site, a, b, dims=NN, width=128, step=32):
        deps = [d() if callable(d) else d for d in self.pending.pop(site, ())]
        a = a() if callable(a) else a
        tie = functools.partial(_tie, self.never, deps=deps)
        a, b = (_bf(tie(a)), _bf(b)) if a.dtype == U32 else (a, _bf(tie(b)))
        out = jax.lax.dot_general(a, b, dims, preferred_element_type=F32)
        per = out.shape[0] // step
        last = {}
        for k, (name, until) in enumerate(self.plan.get(site, ())):
            if name is not None:
                r, c = step * (k % per), width * (k // per)
                vals, tag, stored = self.jobs[name].pop(0)(
                    _gate(self.never, out[r:r + 8, c:c + 128]))
                self.pending.setdefault(until, []).extend(vals)
                last[(name, tag, until)] = stored
        for (_, _, until), stored in last.items():
            if stored is not None:
                self.pending[until].append(stored)
        return out

    def finish(self):
        assert not any(self.jobs.values()) and not any(self.pending.values())


def _ops49(fn, blocks, m):
    return fn(*[fn(*[blocks[q][e] for q in range(4)])[m] for e in range(4)])


def _words49(fn, words, m):
    halves = [[_split(w) for w in q] for q in words]
    lo = _ops49(fn, [[h[0] for h in q] for q in halves], m)
    hi = _ops49(fn, [[h[1] for h in q] for q in halves], m)
    return [_join(a, b) for a, b in zip(lo, hi)]


def _fold(xs, op):
    acc = xs[0]
    for x in xs[1:]:
        acc = op(acc, x)
    return acc


def _tree(xs, op):
    while len(xs) > 1:
        xs = [op(a, b) for a, b in zip(xs[::2], xs[1::2])]
    return xs[0]


def _lane_chunks(x):
    return [x[:, j * 128:(j + 1) * 128] for j in range(x.shape[1] // 128)]


def _kernel(x_hbm, c_hbm, wq_hbm, wuk_hbm, wuv_hbm, wo_hbm, wqkv_hbm, wob_hbm, gw_hbm,
            out_hbm,
            xs_u, x_r, c_r, w_r, wv_r, wob_r, wkv_r, wq_r, wo_r,
            wperm, xq, cq, wv49, wob49, wo49, wkv, wq49, ups, sc_s, qn,
            qk_b, vb, lg_s, pr_s, o_s, ob49, ctx, ca0, ca1, g_s, out_s, gw_ref,
            sem_x, sem_p, sem_a):
    x_u = x_hbm.bitcast(U32)
    c_u = c_hbm.bitcast(U32)
    wo_u = wo_hbm.bitcast(U32)
    wq_u = wq_hbm.bitcast(U32)
    wuk_u = wuk_hbm.bitcast(U32)
    wuv_u = wuv_hbm.bitcast(U32)
    wob_u = wob_hbm.bitcast(U32)
    part = functools.partial

    def blk(j, n):
        return pl.ds(pl.multiple_of(j * n, n), n)

    def strip(j):
        return blk(j, 128)

    def cp_x(t, sem):
        k = (t + 1) >> 1
        return pltpu.make_async_copy(x_u.at[blk(t & 1, S // 4), strip(jnp.minimum(k, 7))],
                                     xs_u.at[jnp.minimum(k, 8), blk(t & 1, S // 4), :], sem)

    def cp_w(t, sem):
        u = t - 2 * (t >> 4)
        u = u - 2 * (u >> 4)
        return pltpu.make_async_copy(wqkv_hbm.at[u >> 3, strip((u >> 1) & 3), blk(u & 1, M)],
                                     w_r.at[u & 1], sem)

    def cp_wob(t, sem):
        b = (t + 1) >> 1
        c = jnp.minimum(b, 7)
        return tuple(pltpu.make_async_copy(
            wob_u.at[:, c & 1, 4 * (2 * (t & 1) + j) + (c & 2) + (c >> 2), :],
            wob_r.at[b & 1, 2 * (t & 1) + j], sem) for j in range(2))

    def group(t, sem2=None):
        sem = sem_x.at[t & 1]
        sem2 = sem if sem2 is None else sem2
        late = t >> 4
        u = t - 2 * late
        pq = (t >> 3) + late
        return (
            cp_x(t, sem),
            cp_w(t + 1, sem),
            pltpu.make_async_copy(x_u.at[blk(u, HQ), :], x_r.at[u & 1], sem),
            pltpu.make_async_copy(c_u.at[blk(u, HQ), :], c_r.at[u & 1], sem),
        ) + cp_wob(t, sem) + tuple(
            pltpu.make_async_copy(wqkv_hbm.at[e >> 1, blk(16 * (e & 1) + u, 16), pl.ds(2 * M, M)],
                                  wv_r.at[u & 1, e], sem) for e in range(4)) + (
            pltpu.make_async_copy(wq_u.at[strip(t & 7), pq, :], wq_r.at[pq, strip(t & 7), :], sem2),
            pltpu.make_async_copy(wuk_u.at[blk(u, 32), 0, :],
                                  wkv_r.at[1 + late, blk(16 + u, 32), :], sem2),
            pltpu.make_async_copy(wuv_u.at[blk(u, 32), 0, :],
                                  wkv_r.at[1 + late, blk(u, 32), :], sem2),
        )

    def cp_wq(p, sem):
        return pltpu.make_async_copy(wq_u.at[:, jnp.minimum(p, NP - 1), :], wq_r.at[p & 3], sem)

    def cp_p(g):
        slot = g & 1
        p = jnp.minimum(g + 1, NP - 1)
        o = jnp.minimum(g, NP - 1)
        sem = sem_p.at[slot]
        return (
            pltpu.make_async_copy(wo_u.at[blk(o >> 1, 2 * DA), blk(o & 1, M // 2)],
                                  wo_r.at[slot], sem),
            pltpu.make_async_copy(wuk_u.at[:, p, :], wkv_r.at[slot, pl.ds(DC, DC), :], sem),
            pltpu.make_async_copy(wuv_u.at[:, p, :], wkv_r.at[slot, pl.ds(0, DC), :], sem),
            cp_wq(g + 2, sem),
        )

    def cp_gw():
        return pltpu.make_async_copy(gw_hbm, gw_ref, sem_a.at[0])

    def cp_out(i, late):
        def cp(rows, cols):
            return pltpu.make_async_copy(out_s.at[rows, cols], out_hbm.at[rows, cols], sem_a.at[1])

        low = [cp(blk(2 * i + 1, TO // 2), pl.ds(512 * cc + 256 * late, 256)) for cc in range(2)]
        return low if late else [cp(blk(2 * i, TO // 2), pl.ds(0, M))] + low

    cp_w(0, sem_a.at[1]).start()
    for t in range(2):
        cp_x(-t, sem_a.at[2]).start()
    group0 = group(0, sem_p.at[1])
    group0 = group0[:-3] + cp_wob(-1, sem_x.at[0]) + group0[-3:]
    for d in group0[1:] + group(1)[:1] + group(1)[2:]:
        d.start()

    for cc in range(8):
        qk_b[8 + cc, pl.ds(0, PAD), :] = jnp.zeros((PAD, 128), F32)
        vb[cc, pl.ds(TQ, PAD), :] = jnp.zeros((PAD, 128), F32)

    def stage_first(t):
        for cc, w in enumerate(_permute8(_lane_chunks(pltpu.bitcast(w_r[t & 1], U32)))):
            wperm[cc] = w

    def p1_step(t, peel):
        if not peel:
            for d in group(t):
                d.wait()

        def act_sums(src, dst, ns, m, sr, r, gate):
            cw = [[gate(src[(t & 1) + _zero(t, m), pl.ds(32 * (q >> 1) + 16 * (e >> 1) + 8 * r, 8),
                            pl.ds(((2 * (q & 1) + (e & 1)) * ns + sr) * 128, 128)])
                   for e in range(4)] for q in range(4)]
            for n, w in enumerate(_words49(_lhs7, cw, m)):
                dst[7 * m + n, t, pl.ds(16 * sr + 8 * r, 8), :] = w
            return [], 0, lambda: dst[7 * m + _zero(t, 0), t, pl.ds(16 * sr + 8 * r, 8), :]

        wv = []

        def load_wv():
            wv.extend(_permute8(_lane_chunks(jnp.concatenate(
                [pltpu.bitcast(wv_r[t & 1, e], U32) for e in range(4)], axis=0))))

        def w_sums(src, dst, m, cc, gate):
            ww = [[gate(src(m, 2 * (q >> 1) + (e >> 1), 2 * (2 * (q & 1) + (e & 1)) + cc))
                   for e in range(4)] for q in range(4)]
            for n, w in enumerate(_words49(_rhs7, ww, m)):
                dst[7 * m + n, cc, blk(t, 8), :] = w
            return [], 0, lambda: dst[7 * m + _zero(t, 0), cc, blk(t, 8), :]

        def v_src(m, rq, ch):
            return wv[ch][8 * rq:8 * rq + 8]

        def o_src(m, rq, ch):
            return wob_r[((t >> 1) & 1) + _zero(t, m), rq, blk(t & 1, 8), pl.ds(128 * ch, 128)]

        segs, step = (P0S, P0T) if peel else (P1S, 32)
        sched = _Sched(t > 99, _plan1(segs, P0W * peel, step, P0N if peel else P1N), dict(
            x=[part(act_sums, x_r, xq, 2, m, sr, r)
               for m in range(7) for sr in range(2) for r in range(2)],
            c=[part(act_sums, c_r, cq, 1, m, 0, r) for m in range(7) for r in range(2)],
            v=[part(w_sums, v_src, wv49, m, cc) for m in range(7) for cc in range(2)],
            o=[part(w_sums, o_src, wob49, m, cc) for m in range(7) for cc in range(2)]))

        first = t < 2
        for k, (half, r0, n) in enumerate(segs):
            if k == P0W * peel:
                if peel:
                    for d in group0[1:-3]:
                        d.wait()
                load_wv()
            w = jnp.concatenate([wperm[4 * half + cc] for cc in range(4)], axis=1)
            r = sched.mm(k, xs_u[t >> 1, pl.ds(r0 // 2, n // 2), :], w, step=step)
            for cc in range(4):
                sl = (8 * (t & 1) + 4 * half + cc, pl.ds(PAD + r0, n), slice(None))
                new = r[:, cc * 128:(cc + 1) * 128]
                qk_b[sl] = new if peel else jnp.where(first, 0.0, qk_b[sl]) + new
        sched.finish()
        stage_first(t + 1)
        d = group(t + 2)
        for d in d[2:] + d[:2]:
            d.start()
        return t

    zero = jnp.max(vb[0, pl.ds(TQ, 8), :]).astype(jnp.int32)
    cp_w(0, sem_a.at[1]).wait()
    stage_first(0)
    group(1)[1].start()
    for t in range(2):
        cp_x(-t, sem_a.at[2]).wait()
    p1_step(zero, True)
    for d in cp_p(0) + (cp_gw(),):
        d.start()
    for d in group0[-3:]:
        d.wait()
    last = jax.lax.fori_loop(1, 16, lambda t, c: p1_step(t, False), 0)

    row = jax.lax.broadcasted_iota(jnp.int32, (TQ, TQ), 0)
    col = jax.lax.broadcasted_iota(jnp.int32, (TQ, TQ), 1)
    col = (col & ~31) | ((col & 1) << 4) | ((col & 31) >> 1)
    rowi = jax.lax.broadcasted_iota(jnp.int32, (RB, 128), 0)
    odd = (jax.lax.broadcasted_iota(jnp.int32, (RB, 128), 1) & 1) == 1
    QSCALE = DA ** -0.5 * LOG2E

    def pair_rows(src, slot, r0, n, gate):
        return [_split(gate(src[slot, pl.ds(r0 + par, n // 2, stride=2), :])) for par in range(2)]

    def staging(g, z, never):
        ns = DC // SCR

        def scales(n1, k, gate):
            res = []
            for h in range(2):
                if k < ns:
                    w = gate(wkv_r[g & 1, pl.ds(n1 * DC + k * SCR, SCR), :])
                    w = pltpu.bitcast(w, jnp.int32) & (0x7F80 << (16 * h))
                else:
                    w = gate(sc_s[2 * n1 + h, pl.ds(0, 8 * ns), :])
                e = _tree([w[r:r + 8] for r in range(0, w.shape[0], 8)], jnp.maximum)
                if k == ns:
                    e = pltpu.bitcast(e << (16 - 16 * h), F32)
                    e = jnp.max(e, axis=0, keepdims=True)
                    e = jnp.clip(pltpu.bitcast(e, jnp.int32), 1 << 23, 253 << 23)
                    e = jnp.broadcast_to(e, (8, 128))
                    sc_s[2 * n1 + h, pl.ds(8 * ns + 8, 8), :] = (254 << 23) - e
                sc_s[2 * n1 + h, pl.ds(8 * k, 8), :] = e
                res.append(pltpu.bitcast(e, U32))
            return res, 0, lambda: pltpu.bitcast(sc_s[2 * n1, blk(k + _zero(z, 0), 8), :], U32)

        def rhs49(dst, tiles, scale, m, r, extra=()):
            res = [_ops49(_rhs7,
                          [[scale(tiles[2 * (q >> 1) + (e >> 1)][q & 1][par][e & 1],
                                  2 * (q & 1) + (e & 1)) for e in range(4)] for q in range(4)],
                          m) for par in range(2)]
            for k, (lo, hi) in enumerate(zip(*res)):
                w = _join(lo, hi)
                if k < len(extra):
                    w = jnp.where(never, extra[k], w)
                dst[7 * m + k, pl.ds(8 * r, 8), :] = w

        def kv(m, r, gate):
            if m == 0 and r == 0:
                for k in range(4):
                    ups[k] = pltpu.bitcast(gate(sc_s[k, pl.ds(8 * ns, 8), :]), F32)
            down = [pltpu.bitcast(sc_s[k + _zero(z, m), pl.ds(8 * ns + 8, 8), :], F32)
                    for k in range(4)]
            tiles = [[pair_rows(wkv_r, (g & 1) + _zero(z, m), n1 * DC + kt * 128 + 16 * r, 16, gate)
                      for n1 in range(2)] for kt in range(4)]
            rhs49(wkv, tiles, lambda w, k: w * down[k], m, r)
            return [], 0, lambda: wkv[7 * m, blk(r + _zero(z, 0), 8), :]

        def qw(m, r, gate):
            tiles = [[pair_rows(wq_r, ((g + 1 + n1) & 3) + _zero(z, m), kt * 256 + 16 * r, 16, gate)
                      for n1 in range(2)] for kt in range(4)]
            rhs49(wq49, tiles, lambda w, k: w, m, r, sc.pop(0)(gate)[0] if sc else ())
            return [], 0, lambda: wq49[7 * m, blk(r + _zero(z, 0), 8), :]

        sc = [part(scales, n1, k) for k in range(ns + 1) for n1 in range(2)]
        return dict(sc=sc,
                    kv=[part(kv, m, r) for m in range(7) for r in range(8)],
                    qw=[part(qw, m, r) for m in range(7) for r in range(16)])

    sched = _Sched(last > 99, _planx(), staging(-1, last, last > 99))
    w0 = pair_rows(wq_r, 0, 0, M, lambda x: x)
    w0 = [_join(w0[0][h], w0[1][h]) for h in range(2)]
    for g in range(4):
        for e in range(2):
            for h in range(2):
                q = [sched.mm(8 * g + 4 * e + 2 * h + k, jnp.concatenate(
                    [xs_u[4 * k + u, pl.ds((4 * g + 2 + e) * HQ, HQ), :] for u in range(4)], axis=1),
                    w0[h][256 * k:256 * k + 256], step=16) for k in range(2)]
                qn[h, g, e] = _pack((q[0] + q[1]) * QSCALE)
    sched.finish()
    for d in group(16) + group(17):
        d.wait()
    for d in cp_p(1):
        d.start()
    plan2 = _plan2()

    def p2_body(p, carry):
        for d in cp_p(p):
            d.wait()
        causal = col <= row
        never = p > NP
        jobs = staging(p, p, never)
        sched = _Sched(never, plan2, jobs)
        mm = sched.mm

        r0 = pl.multiple_of(p * TQ, TQ)

        prods = {}

        def project(kind, j, n, lhs, rhs):
            got = prods.setdefault((kind, j), {})
            for m in ORDER[len(got):len(got) + n]:
                got[m] = _combine(lambda k: mm((kind, j, 7 * len(got) + ORDER.index(k)),
                                               part(lhs, 7 * m + k), rhs(7 * m + k)))
            if len(got) < 7:
                return None
            c = _combine(lambda m: got[m])
            return [[c[(rg & 2) + (cg >> 1)][2 * (rg & 1) + (cg & 1)] for rg in range(4)]
                    for cg in range(4)]

        def pair(ref, rows):
            return lambda k: jnp.concatenate([ref[k, sr, rows, :] for sr in range(2)], axis=1)

        def x_rows(b, n):
            return lambda k: jnp.concatenate([jnp.concatenate(
                [xq[k, b + j, pl.ds(16 * sr, 16), :] for sr in range(2)], axis=1)
                for j in range(n)], axis=0)

        def proj_b(kind, n, lhs, w, dst, off):
            c = project(kind, 0, n, lhs, pair(w, slice(None)))
            for cg in range(4 * (c is not None)):
                for rg in range(4):
                    for cc in range(2):
                        dst[2 * cg + cc, pl.ds(off + (PAD + rg * QQ), QQ), :] = (
                            c[cg][rg][:, cc * 128:(cc + 1) * 128])

        def proj_bv():
            for cc in range(8):
                vb[cc, pl.ds(0, PAD), :] = vb[cc, pl.ds(TQ, PAD), :]
            proj_b("bv", 7, x_rows(p, 1), wv49, vb, 0)

        def proj_bo(n):
            proj_b("bo", n, pair(ob49, slice(None)), wob49, qk_b, r0)

        def local_qk(rb, k, gate):
            rz = pl.multiple_of((p + _zero(p, k)) * TQ, TQ)
            q = [qk_b[cc, pl.ds(rz + (PAD + rb * RB), RB), :] for cc in range(8)]
            q[0] = gate(q[0])
            for w in range(LG * k, LG * k + LG):
                t = _fold([q[cc] * qk_b[8 + cc, pl.ds(r0 + (PAD + rb * RB - DIL * w), RB), :]
                           for cc in range(8)], jnp.add)
                t = t + pltpu.roll(t, 64, 1)
                t = t + jnp.where(odd, pltpu.roll(t, 1, 1), pltpu.roll(t, 127, 1))
                t = t * (DB ** -0.5 * LOG2E)
                if rb == 0 and w:
                    t = jnp.where(rowi + r0 >= DIL * w, t, NEG)
                lg_s[w, pl.ds(rb * RB, RB), :] = t
            return [], 1, lambda: pltpu.bitcast(lg_s[w, blk(2 * rb + _zero(p, 0), 8), :], U32)

        def local_sm(rb, e, gate):
            rows = pl.ds(rb * RB + SMR * e, SMR)
            lg = [gate(lg_s[w, rows, :]) for w in range(WIN)]
            m = _tree(lg, jnp.maximum)
            ps = [jnp.exp2(t - m) for t in lg]
            l = _tree(ps, jnp.add)
            r = pl.reciprocal(l, approx=True)
            r = r * (2.0 - l * r)
            for w in range(WIN):
                pr_s[w, rows, :] = ps[w] * r
            return [], 2, lambda: pltpu.bitcast(pr_s[0, blk(2 * rb + e + _zero(p, 0), 8), :], U32)

        def local_pv(rb, k, gate):
            rows = pl.ds(rb * RB, RB)
            ps = [pr_s[w + _zero(p, k), rows, :] for w in range(WIN)]
            ps[0] = gate(ps[0])
            o = [_fold([ps[w] * vb[cc, pl.ds(PAD + rb * RB - DIL * w, RB), :] for w in range(WIN)],
                       jnp.add) for cc in (k, k + 4)]
            for e in range(2):
                o_s[k + 4 * e, rows, :] = o[e]
            return [], 0, lambda: pltpu.bitcast(o_s[k, blk(2 * rb + _zero(p, 0), 8), :], U32)

        def o_sums(m, cc, r, gate):
            res = [_ops49(_lhs7, [[gate(o_s[
                2 * (2 * (q & 1) + (e & 1)) + cc + _zero(p, m),
                pl.ds(QQ * (2 * (q >> 1) + (e >> 1)) + 16 * r + par, 8, stride=2), :])
                for e in range(4)] for q in range(4)], m) for par in range(2)]
            for n, (lo, hi) in enumerate(zip(*res)):
                ob49[7 * m + n, cc, pl.ds(8 * r, 8), :] = _join(lo, hi)
            return [], 0, lambda: ob49[7 * m, cc, blk(r + _zero(p, 0), 8), :]

        jobs["os"] = [part(o_sums, m, cc, r) for r in range(2) for cc in range(2) for m in range(7)]
        order = list(range(0, 8, 2)) + list(range(1, 8, 2))
        jobs["lo"] = []
        for k in range(len(order) + SML):
            for f, d, n in ((local_sm, SML, RB // SMR), (local_qk, 0, 8 // LG)):
                if 0 <= k - d < len(order):
                    jobs["lo"] += [part(f, order[k - d], e) for e in range(n)]
        jobs["lv"] = [part(local_pv, rb, e) for rb in order for e in range(4)]

        def out_weights(m, r, gate):
            ww = [[gate(wo_r[(p & 1) + _zero(p, m),
                             pl.ds((2 * (q >> 1) + (e >> 1)) * HQ + 8 * r, 8),
                             pl.ds((2 * (q & 1) + (e & 1)) * 128, 128)])
                   for e in range(4)] for q in range(4)]
            rows = blk(8 * (p >> 1) + r, 8)
            extra = jobs["sc"].pop(0)(gate)[0] if jobs["sc"] else []
            for n, w in enumerate(_words49(_rhs7, ww, m)):
                if n < len(extra):
                    w = jnp.where(never, extra[n], w)
                wo49[7 * m + n, p & 1, rows, :] = w
            return [], 0, lambda: wo49[7 * m + _zero(p, 0), p & 1, rows, :]

        jobs["wo"] = [part(out_weights, m, r) for m in range(7) for r in range(8)]

        ks, vs, qs = {}, {}, {}
        done = {}

        def blocks(c, scale, pack):
            c = [[pack(t * scale(cg)) for t in c[cg]] for cg in range(4)]
            return [[jnp.concatenate([t[16 * e:16 * e + 16] for t in c[cg]], axis=0)
                     for e in range(2)] for cg in range(4)]

        def proj_kv(j, n):
            c = project("kv", j, n, lambda k: jnp.concatenate(
                [cq[k, 2 * j], cq[k, 2 * j + 1]], axis=0), lambda k: wkv[k])
            if c is not None:
                c = blocks(c, lambda cg: ups[cg][:1], _riffle)
                for cg in range(4):
                    for e in range(2):
                        (vs, ks)[cg >> 1][(cg & 1, 2 * j + e)] = c[cg][e]

        def proj_q(g, n):
            c = project("q", g, n, x_rows(4 * g + 2 * (p & 1), 2), lambda k: wq49[k])
            if c is not None:
                c = blocks(c, lambda cg: QSCALE, _pack)
                for h in range(2):
                    for e in range(2):
                        old = qn[h, g, e]
                        for b in range(2):
                            qs[(h, 4 * g + 2 * b + e)] = jnp.where((p & 1) == b, c[h][e], old)
                        qn[h, g, e] = c[2 + h][e]

        def qk(h, i, dep):
            kk = jnp.concatenate([ks[(h, j)] for j in range(i + 1)], axis=0)
            q = qs[(h, i)]
            if dep is not None:
                q = jnp.where(never, done[(h, dep)], q)
            ch = _lane_chunks(mm(("qk", h, i), q, kk, NT, 512))
            ch[i] = jnp.where(causal, ch[i], NEG)
            return ch

        def softmax_pv(h, i, ch):
            m = jnp.max(_fold(ch, jnp.maximum), axis=1, keepdims=True)
            ps = [jnp.exp2(c - m) for c in ch]
            lp = ps[0]
            for j in range(1, i + 1):
                lp = lp + ps[j]
                if TIE and (j % TIE == TIE - 1 or j == i):
                    ps[j] = jnp.where(never, lp, ps[j])
            pb = jnp.concatenate(ps, axis=1).astype(BF16)
            vv = jnp.concatenate([vs[(h, j)] for j in range(i + 1)], axis=0)
            o = mm(("pv", h, i), pb, vv)
            if i >= LDEP:
                lp = jnp.where(never, o, lp)
            l = jnp.sum(lp, axis=1, keepdims=True)
            r = pl.reciprocal(l, approx=True)
            r = r * (2.0 - l * r)
            cn = _pack(o * r)
            done[(h, i)] = cn
            if FA <= i < NQ - 1:
                if h == 0 and F0 < 0:
                    site = ("qk", 1, i + 1)
                elif i + 3 < NQ:
                    site = ("kv", (i + 1) // 2 + 1, KVS * ((i + 1) & 1) + (F0, FD)[h])
                else:
                    site = ("bo", 0, 7 * (i + 3 - NQ) * BOP[0] + 8 * h)
                sched.pending.setdefault(site, []).append(cn)
            ctx[2 * p + h, pl.ds(i * HQ, HQ), :] = cn

        proj_bv()
        proj_kv(0, 7)
        proj_q(0, 7)
        for i in range(NQ):
            dep = i - DEP if DEP <= i < FA + DEP else None
            s0 = qk(0, i, dep)
            s1 = qk(1, i, dep)
            if i + 2 < NQ:
                proj_kv(i // 2 + 1, 7 if i & 1 else KVS // 7)
                if i < 6:
                    proj_q(i // 2 + 1, 7 if i & 1 else QS // 7)
            else:
                proj_bo(BOP[i + 2 - NQ])
            softmax_pv(0, i, s0)
            softmax_pv(1, i, s1)
        proj_bo(BOP[2])
        sched.finish()
        for d in cp_p(p + 2):
            d.start()
        return carry

    jax.lax.fori_loop(0, NP, p2_body, 0)

    cp_gw().wait()
    gw = gw_ref[...].astype(F32)
    plan3 = _plan3()
    cab = (ca0, ca1)

    def p3_body(i, carry):
        r0 = pl.multiple_of(i * TO, TO)
        h0 = pl.multiple_of(i * (TO // 2), TO // 2)
        never = i > S

        def ctx_words(m, u, r, n):
            return [[ctx[4 * u + 2 * (q & 1) + (e & 1),
                         pl.ds(h0 + _zero(i, m) * 8 + ((2 * (q >> 1) + (e >> 1)) * QQ + r), n), :]
                     for e in range(4)] for q in range(4)]

        def operands(k, u, r, gate):
            m = ORDER[k]
            cw = [[gate(w) for w in q] for q in ctx_words(m, u, r, 8)]
            for n, w in enumerate(_words49(_lhs7, cw, m)):
                if not (m in (2, 3) and n in (2, 3)):
                    cab[k & 1][n, pl.ds(r, 8), pl.ds(u * 128, 128)] = w
            return [], 0, lambda: cab[k & 1][_zero(i, 0), pl.ds(r, 8), pl.ds(u * 128, 128)]

        def gate_rows(r, gate):
            gs = _fold([_bf(gate(xs_u[j, pl.ds(h0 + r, 8), :])).astype(F32) * gw[j:j + 1]
                        for j in range(8)], jnp.add)
            g = jax.nn.sigmoid(jnp.sum(gs, axis=1, keepdims=True))
            g_s[pl.ds(2 * r, 16), :] = jnp.broadcast_to(g, (16, 128))
            return [], 0, lambda: pltpu.bitcast(g_s[blk(r // 4 + _zero(i, 0), 8), :], U32)

        pr = {}

        def mix(q, e, cc, gate):
            off = (2 * (q >> 1) + (e >> 1)) * HQ
            ch = 4 * cc + 2 * (q & 1) + (e & 1)
            a = _combine(lambda m: pr.get(m, pr[2])[e][:, cc * 128:(cc + 1) * 128])[q]
            g = gate(g_s[pl.ds(off, HQ), :])
            b = qk_b[ch, pl.ds(r0 + (PAD + off), HQ), :]
            out_s[pl.ds(r0 + off, HQ), pl.ds(ch * 128, 128)] = (g * a + (1.0 - g) * b).astype(BF16)
            return [], 0, lambda: pltpu.bitcast(
                out_s[blk(i * (TO // 16) + off // 16 + _zero(i, 0), 16), pl.ds(ch * 128, 128)], U32)

        sched = _Sched(never, plan3, dict(
            a=[part(operands, k, u, r) for k in range(1, 7) for u in range(HA // 4)
               for r in range(0, QQ, 8)],
            g=[part(gate_rows, r) for r in range(0, TO // 2, 8)],
            m=[part(mix, q, e, cc) for q in (1, 2, 0) for e in range(4) for cc in range(2)]))
        first = [[_words49(_lhs7, ctx_words(ORDER[0], u, 0, QQ), ORDER[0])[n]
                  for u in range(HA // 4)] for n in range(7)]

        def inner(m, n):
            k = ORDER.index(m)
            res = []
            for e in range(2):
                us = range(4 * e, 4 * e + 4)
                if m in (2, 3) and n in (2, 3):
                    lhs = jnp.concatenate([ctx_words(m, u, 0, QQ)[3 * (m - 2)][3 * (n - 2)]
                                           for u in us], axis=1)
                elif k == 0:
                    lhs = jnp.concatenate([first[n][u] for u in us], axis=1)
                else:
                    lhs = lambda: cab[k & 1][n, :, pl.ds(e * 512, 512)]
                rhs = jnp.concatenate([wo49[7 * m + n, cc, pl.ds(e * 256, 256), :]
                                       for cc in range(2)], axis=1)
                res.append(sched.mm((k, 2 * ORDER.index(n) + e), lhs, rhs))
                if (k, 2 * ORDER.index(n) + e) == (6, P3D):
                    for d in cp_out(i, 0):
                        d.start()
            return res[0] + res[1]

        for m in ORDER:
            pr[m] = _combine(lambda n: inner(m, n))
        sched.finish()
        for e in (1, 2, 0, 3):
            for cc in range(2):
                mix(3, e, cc, lambda x: x)
        for d in cp_out(i, 1):
            d.start()
        return carry

    jax.lax.fori_loop(0, S // TO, p3_body, 0)
    for g in range(NP, NP + 2):
        for d in cp_p(g):
            d.wait()
    for i in range(S // TO):
        for d in cp_out(i, 0) + cp_out(i, 1):
            d.wait()


@jax.jit
def pallas_gated_mix__compressed_kv_cla__sliding_local_dilated__prompt_kernel(
    A_x: jax.Array,
    A_c_kv: jax.Array,
    A_w_q: jax.Array,
    A_w_uk: jax.Array,
    A_w_uv: jax.Array,
    A_w_o: jax.Array,
    B_x: jax.Array,
    B_wqkv: jax.Array,
    B_wo: jax.Array,
    gate_w: jax.Array,
):
    del B_x
    any_spec = pl.BlockSpec(memory_space=pl.ANY)
    out = pl.pallas_call(
        _kernel,
        in_specs=[any_spec] * 9,
        out_specs=any_spec,
        out_shape=jax.ShapeDtypeStruct((S, M), BF16),
        scratch_shapes=[
            pltpu.VMEM((9, S // 2, 128), U32),
            pltpu.VMEM((2, HQ, M), U32),
            pltpu.VMEM((2, HQ, DC), U32),
            pltpu.VMEM((2, 128, M), BF16),
            pltpu.VMEM((2, 4, 16, M), BF16),
            pltpu.VMEM((2, 4, 16, M), U32),
            pltpu.VMEM((3, 2 * DC, 128), U32),
            pltpu.VMEM((4, M, 128), U32),
            pltpu.VMEM((2, 2 * DA, M // 2), U32),
            pltpu.VMEM((8, 64, 128), U32),
            pltpu.VMEM((49, NQ, 32, 128), U32),
            pltpu.VMEM((49, NQ, 16, 128), U32),
            pltpu.VMEM((49, 2, M // 8, 128), U32),
            pltpu.VMEM((49, 2, M // 8, 128), U32),
            pltpu.VMEM((49, 2, NP * QQ, 128), U32),
            pltpu.VMEM((49, HQ, 128), U32),
            pltpu.VMEM((49, TQ, 128), U32),
            pltpu.VMEM((4, 8, 128), F32),
            pltpu.VMEM((4, DC // SCR * 8 + 16, 128), jnp.int32),
            pltpu.VMEM((2, 4, 2, HQ, 128), U32),
            pltpu.VMEM((16, S + PAD, 128), F32),
            pltpu.VMEM((8, TQ + PAD, 128), F32),
            pltpu.VMEM((WIN, TQ, 128), F32),
            pltpu.VMEM((WIN, TQ, 128), F32),
            pltpu.VMEM((8, TQ, 128), F32),
            pltpu.VMEM((49, 2, 16, 128), U32),
            pltpu.VMEM((HA, S // 2, 128), U32),
            pltpu.VMEM((7, QQ, M), U32),
            pltpu.VMEM((7, QQ, M), U32),
            pltpu.VMEM((TO, 128), F32),
            pltpu.VMEM((S, M), BF16),
            pltpu.VMEM((8, 128), BF16),
            pltpu.SemaphoreType.DMA((2,)),
            pltpu.SemaphoreType.DMA((2,)),
            pltpu.SemaphoreType.DMA((3,)),
        ],
        compiler_params=pltpu.CompilerParams(vmem_limit_bytes=120 * 1024 * 1024,
                                             disable_bounds_checks=True),
    )(
        A_x.reshape(S, M),
        A_c_kv.reshape(S, DC),
        A_w_q,
        A_w_uk,
        A_w_uv,
        A_w_o.reshape(HA * DA, M),
        B_wqkv.reshape(2, M // 2, 3 * M),
        B_wo.reshape(HB // 2, 2, DB, M),
        gate_w.reshape(8, 128),
    )
    return out.reshape(1, S, M)
```

```python
import functools
import math

import jax
import jax.numpy as jnp
import jax.experimental.pallas as pl
import jax.experimental.pallas.tpu as pltpu

F32 = jnp.float32
BF16 = jnp.bfloat16
U32 = jnp.uint32

S = 2048
M = 1024
HA = 32
DA = 128
DC = 512
HB = 32
DB = 32
WIN = 8
DIL = 2
PAD = 16
LOG2E = math.log2(math.e)
NEG = -1e9

TQ = 128
HQ = TQ // 2
QQ = TQ // 4
BOP = (2, 3, 2)
LX = 16
KVS = 28
QS = 28
QST = 2
LQ0 = 1
LG = 2
XN = 28
XQ = 56
SK = 3
SMR = 16
P1N = 108
P1A = 60
P0W = 1
P0T = 16
P0N = 98
P0S = ((0, 0, 2048), (1, 0, 1024), (1, 1024, 768), (1, 1792, 128), (1, 1920, 128))
P1S = ((0, 0, 2048), (1, 0, 1536), (1, 1536, 384), (1, 1920, 128))
P3S = 4
P3M = 6
P3D = 8
P3E = 12
NQ = S // TQ
NP = HA // 2
DEP = 2
SCR = 32
LN = 80
SML = 1
LE = 2
LI = 99
LA = 24
LB = 4
LS = 1
BS = 2
LP = ("kv", 1, 8)
BX = 8
BE = 42
FA = 6
F0 = 0
FD = 8
TIE = 4
RB = 16
LDEP = 4
TO = 256
NN = (((1,), (0,)), ((), ()))
NT = (((1,), (1,)), ((), ()))


def _plan2():
    plan = {}

    def put(name, count, start, until):
        plan.setdefault(start, []).extend([(name, until)] * count)

    def after_qk(i):
        if i >= NQ - 2:
            return ("bo", 0, 7 * (i - NQ + 2) * BOP[0] + BX)
        return ("kv", i // 2 + 1, KVS * (i & 1) + LX)

    def fill(name, count, sites):
        for start, room, until in sites:
            n = min(count, room - len(plan.get(start, ())))
            put(name, n, start, until)
            count -= n
        assert count == 0, (name, count)

    def qk_sites(lo, hi):
        return [(("qk", h, i), max(i + 1 - h * SK, 0), after_qk(i))
                for i in range(lo, hi) for h in range(2)]

    def q_sites(g, lo, hi, until):
        return [(("q", g, k), 1, until) for k in range(lo, hi, QST)]

    ticks = ([("bv", 0, k) for k in range(LA, 49, LS)] + [("kv", 0, k) for k in range(0, 49, 2)]
             + [("q", 0, k) for k in range(49)])
    for name, site in zip(_spread(["lo"] * (64 // LG + 128 // SMR), LN), ticks):
        put(name, 1, site, LP)
    first = [(site, 1, ("kv", 1, 8)) for site in ticks[LN + LI:-LB:LE]]
    host = [(("bv", 0, k), 1, ("kv", 0, 8)) for k in range(0, min(LA, 46), BS)]
    early = []
    for g in range(1, 4):
        early += q_sites(g, 0, QS - 4, after_qk(2 * g - 1))
        early += qk_sites(max(2 * g - 1, LQ0), 2 * g)
        early += q_sites(g, QS, 45, after_qk(2 * g))
        early += qk_sites(max(2 * g, LQ0), 2 * g + 1)
    fill("lv", 32, first + early)
    fill("wo", 56, host + early)
    fill("os", 28, early + qk_sites(7, 14))
    fill("qw", 112, qk_sites(7, 14))
    fill("kv", 56, qk_sites(14, 16) + [(("bo", 0, k), 1, ("bo", 0, BE))
                                       for k in range(7 * BOP[0], 35)])
    return plan


def _planx():
    names = _spread(["qw"] * XQ + ["kv", "qw"] * 56 + ["qw"] * (56 - XQ), 8 * XN)
    return {k: [(n, 31) for n in names[8 * k:8 * k + 8]] for k in range(XN)}


def _spread(names, ticks):
    out = [None] * ticks
    for k, name in enumerate(names):
        out[k * ticks // len(names)] = name
    return out


def _plan1(segs, lo, step, count):
    end = len(segs) - 2
    ticks = [k for k in range(lo, end) for _ in range(segs[k][2] // step)][:count]
    n = len(ticks) * P1A // 100
    names = _spread(["x"] * 28 + ["c"] * 14 + ["o"] * 14, n) + _spread(["v"] * 14, len(ticks) - n)
    plan = {}
    for k, name in zip(ticks, names):
        plan.setdefault(k, []).append((name, end))
    return plan


def _plan3():
    plan = {}
    for k in range(6):
        lo = P3S if k == 0 else 0
        extra = ["g"] * 8 if k in (1, 2) else []
        names = _spread(["a"] * 32 + extra, 4 * (P3E - lo))
        for d in range(lo, P3E):
            plan[(k, d)] = [(n, (k + 1, 0)) for n in names[4 * (d - lo):4 * (d - lo) + 4]]
    names = _spread(["m"] * 24, 4 * P3M)
    for d in range(P3M):
        plan[(6, d)] = [(n, (6, P3D)) for n in names[4 * d:4 * d + 4]]
    return plan


_STAGES = ((2, 4), (1, 3), (0, 2), (0, 6), (0, 1))


def _permute8(cols):
    cols = list(cols)
    lane = jax.lax.broadcasted_iota(jnp.int32, cols[0].shape, 1)
    for va, lb in _STAGES:
        lo = (lane & (1 << lb)) == 0
        sh = 1 << lb
        idx = [i for i in range(8) if not (i >> va) & 1]
        if lb == 6:
            rr = [pltpu.roll(jnp.where(lo, cols[i | (1 << va)], cols[i]), 64, 1) for i in idx]
            for i, r in zip(idx, rr):
                a, b = cols[i], cols[i | (1 << va)]
                cols[i] = jnp.where(lo, a, r)
                cols[i | (1 << va)] = jnp.where(lo, r, b)
        else:
            rb = [pltpu.roll(cols[i | (1 << va)], sh, 1) for i in idx]
            ra = [pltpu.roll(cols[i], 128 - sh, 1) for i in idx]
            for i, xa, xb in zip(idx, ra, rb):
                a, b = cols[i], cols[i | (1 << va)]
                cols[i] = jnp.where(lo, a, xb)
                cols[i | (1 << va)] = jnp.where(lo, xa, b)
    return cols


def _pack(x):
    return pltpu.bitcast(x.astype(BF16), U32)


def _bf(x):
    return pltpu.bitcast(x, BF16)


def _split(w):
    return (pltpu.bitcast(w << 16, F32), pltpu.bitcast(w & jnp.uint32(0xFFFF0000), F32))


def _join(lo, hi):
    return pltpu.bitcast(pltpu.pack_elementwise([lo, hi], packed_dtype=BF16), U32)


def _riffle(x):
    return jnp.concatenate([_join(x[r:r + 16], x[r + 16:r + 32]) for r in range(0, x.shape[0], 32)],
                           axis=0)


def _lhs7(a11, a12, a21, a22):
    return [a11 + a22, a21 + a22, a11, a22, a11 + a12, a21 - a11, a12 - a22]


def _rhs7(b11, b12, b21, b22):
    return [b11 + b22, b11, b12 - b22, b21 - b11, b22, b11 + b12, b21 + b22]


def _combine(mm):
    add = functools.partial(jax.tree.map, jnp.add)
    sub = functools.partial(jax.tree.map, jnp.subtract)
    m2 = mm(2)
    m3 = mm(3)
    m4 = mm(4)
    c12 = add(m2, m4)
    t11 = sub(m3, m4)
    m1 = mm(1)
    c21 = add(m1, m3)
    t22 = sub(m2, m1)
    m0 = mm(0)
    t11 = add(t11, m0)
    t22 = add(t22, m0)
    c11 = add(t11, mm(6))
    return c11, c12, c21, add(t22, mm(5))


ORDER = (2, 3, 4, 1, 0, 6, 5)


def _zero(i, m):
    return i >> (8 + m)


def _merge(vals):
    return _fold([v[r:r + 8, c:c + 128] for v in vals for r in range(0, v.shape[0], 8)
                  for c in range(0, v.shape[1], 128)], jnp.bitwise_or)


def _gate(never, g):
    def gate(x):
        t = jnp.tile(pltpu.bitcast(g, x.dtype), (x.shape[0] // 8, x.shape[1] // 128))
        return jnp.where(never, t, x)
    return gate


def _tie(never, x, deps):
    if not deps:
        return x
    top = jnp.where(never, _merge(deps), x[:8, :128])
    if x.shape[1] > 128:
        top = jnp.concatenate([top, x[:8, 128:]], axis=1)
    return jnp.concatenate([top, x[8:]], axis=0)


class _Sched:
    def __init__(self, never, plan, jobs):
        self.never, self.plan, self.jobs, self.pending = never, plan, jobs, {}

    def mm(self, site, a, b, dims=NN, width=128, step=32):
        deps = [d() if callable(d) else d for d in self.pending.pop(site, ())]
        a = a() if callable(a) else a
        tie = functools.partial(_tie, self.never, deps=deps)
        a, b = (_bf(tie(a)), _bf(b)) if a.dtype == U32 else (a, _bf(tie(b)))
        out = jax.lax.dot_general(a, b, dims, preferred_element_type=F32)
        per = out.shape[0] // step
        last = {}
        for k, (name, until) in enumerate(self.plan.get(site, ())):
            if name is not None:
                r, c = step * (k % per), width * (k // per)
                vals, tag, stored = self.jobs[name].pop(0)(
                    _gate(self.never, out[r:r + 8, c:c + 128]))
                self.pending.setdefault(until, []).extend(vals)
                last[(name, tag, until)] = stored
        for (_, _, until), stored in last.items():
            if stored is not None:
                self.pending[until].append(stored)
        return out

    def finish(self):
        assert not any(self.jobs.values()) and not any(self.pending.values())


def _ops49(fn, blocks, m):
    return fn(*[fn(*[blocks[q][e] for q in range(4)])[m] for e in range(4)])


def _words49(fn, words, m):
    halves = [[_split(w) for w in q] for q in words]
    lo = _ops49(fn, [[h[0] for h in q] for q in halves], m)
    hi = _ops49(fn, [[h[1] for h in q] for q in halves], m)
    return [_join(a, b) for a, b in zip(lo, hi)]


def _fold(xs, op):
    acc = xs[0]
    for x in xs[1:]:
        acc = op(acc, x)
    return acc


def _tree(xs, op):
    while len(xs) > 1:
        xs = [op(a, b) for a, b in zip(xs[::2], xs[1::2])]
    return xs[0]


def _lane_chunks(x):
    return [x[:, j * 128:(j + 1) * 128] for j in range(x.shape[1] // 128)]


def _kernel(x_hbm, c_hbm, wq_hbm, wuk_hbm, wuv_hbm, wo_hbm, wqkv_hbm, wob_hbm, gw_hbm,
            out_hbm,
            xs_u, x_r, c_r, w_r, wv_r, wob_r, wkv_r, wq_r, wo_r,
            wperm, xq, cq, wv49, wob49, wo49, wkv, wq49, ups, sc_s, qn,
            qk_b, vb, lg_s, pr_s, o_s, ob49, ctx, ca0, ca1, g_s, out_s, gw_ref,
            sem_x, sem_p, sem_a):
    x_u = x_hbm.bitcast(U32)
    c_u = c_hbm.bitcast(U32)
    wo_u = wo_hbm.bitcast(U32)
    wq_u = wq_hbm.bitcast(U32)
    wuk_u = wuk_hbm.bitcast(U32)
    wuv_u = wuv_hbm.bitcast(U32)
    wob_u = wob_hbm.bitcast(U32)
    part = functools.partial

    def blk(j, n):
        return pl.ds(pl.multiple_of(j * n, n), n)

    def strip(j):
        return blk(j, 128)

    def cp_x(t, sem):
        k = (t + 1) >> 1
        return pltpu.make_async_copy(x_u.at[blk(t & 1, S // 4), strip(jnp.minimum(k, 7))],
                                     xs_u.at[jnp.minimum(k, 8), blk(t & 1, S // 4), :], sem)

    def cp_w(t, sem):
        u = t - 2 * (t >> 4)
        u = u - 2 * (u >> 4)
        return pltpu.make_async_copy(wqkv_hbm.at[u >> 3, strip((u >> 1) & 3), blk(u & 1, M)],
                                     w_r.at[u & 1], sem)

    def cp_wob(t, sem):
        b = (t + 1) >> 1
        c = jnp.minimum(b, 7)
        return tuple(pltpu.make_async_copy(
            wob_u.at[:, c & 1, 4 * (2 * (t & 1) + j) + (c & 2) + (c >> 2), :],
            wob_r.at[b & 1, 2 * (t & 1) + j], sem) for j in range(2))

    def group(t, sem2=None):
        sem = sem_x.at[t & 1]
        sem2 = sem if sem2 is None else sem2
        late = t >> 4
        u = t - 2 * late
        pq = (t >> 3) + late
        return (
            cp_x(t, sem),
            cp_w(t + 1, sem),
            pltpu.make_async_copy(x_u.at[blk(u, HQ), :], x_r.at[u & 1], sem),
            pltpu.make_async_copy(c_u.at[blk(u, HQ), :], c_r.at[u & 1], sem),
        ) + cp_wob(t, sem) + tuple(
            pltpu.make_async_copy(wqkv_hbm.at[e >> 1, blk(16 * (e & 1) + u, 16), pl.ds(2 * M, M)],
                                  wv_r.at[u & 1, e], sem) for e in range(4)) + (
            pltpu.make_async_copy(wq_u.at[strip(t & 7), pq, :], wq_r.at[pq, strip(t & 7), :], sem2),
            pltpu.make_async_copy(wuk_u.at[blk(u, 32), 0, :],
                                  wkv_r.at[1 + late, blk(16 + u, 32), :], sem2),
            pltpu.make_async_copy(wuv_u.at[blk(u, 32), 0, :],
                                  wkv_r.at[1 + late, blk(u, 32), :], sem2),
        )

    def cp_wq(p, sem):
        return pltpu.make_async_copy(wq_u.at[:, jnp.minimum(p, NP - 1), :], wq_r.at[p & 3], sem)

    def cp_p(g):
        slot = g & 1
        p = jnp.minimum(g + 1, NP - 1)
        o = jnp.minimum(g, NP - 1)
        sem = sem_p.at[slot]
        return (
            pltpu.make_async_copy(wo_u.at[blk(o >> 1, 2 * DA), blk(o & 1, M // 2)],
                                  wo_r.at[slot], sem),
            pltpu.make_async_copy(wuk_u.at[:, p, :], wkv_r.at[slot, pl.ds(DC, DC), :], sem),
            pltpu.make_async_copy(wuv_u.at[:, p, :], wkv_r.at[slot, pl.ds(0, DC), :], sem),
            cp_wq(g + 2, sem),
        )

    def cp_gw():
        return pltpu.make_async_copy(gw_hbm, gw_ref, sem_a.at[0])

    def cp_out(i, late):
        def cp(rows, cols):
            return pltpu.make_async_copy(out_s.at[rows, cols], out_hbm.at[rows, cols], sem_a.at[1])

        low = [cp(blk(2 * i + 1, TO // 2), pl.ds(512 * cc + 256 * late, 256)) for cc in range(2)]
        return low if late else [cp(blk(2 * i, TO // 2), pl.ds(0, M))] + low

    cp_w(0, sem_a.at[1]).start()
    for t in range(2):
        cp_x(-t, sem_a.at[2]).start()
    group0 = group(0, sem_p.at[1])
    group0 = group0[:-3] + cp_wob(-1, sem_x.at[0]) + group0[-3:]
    for d in group0[1:] + group(1)[:1] + group(1)[2:]:
        d.start()

    for cc in range(8):
        qk_b[8 + cc, pl.ds(0, PAD), :] = jnp.zeros((PAD, 128), F32)
        vb[cc, pl.ds(TQ, PAD), :] = jnp.zeros((PAD, 128), F32)

    def stage_first(t):
        for cc, w in enumerate(_permute8(_lane_chunks(pltpu.bitcast(w_r[t & 1], U32)))):
            wperm[cc] = w

    def p1_step(t, peel):
        if not peel:
            for d in group(t):
                d.wait()

        def act_sums(src, dst, ns, m, sr, r, gate):
            cw = [[gate(src[(t & 1) + _zero(t, m), pl.ds(32 * (q >> 1) + 16 * (e >> 1) + 8 * r, 8),
                            pl.ds(((2 * (q & 1) + (e & 1)) * ns + sr) * 128, 128)])
                   for e in range(4)] for q in range(4)]
            for n, w in enumerate(_words49(_lhs7, cw, m)):
                dst[7 * m + n, t, pl.ds(16 * sr + 8 * r, 8), :] = w
            return [], 0, lambda: dst[7 * m + _zero(t, 0), t, pl.ds(16 * sr + 8 * r, 8), :]

        wv = []

        def load_wv():
            wv.extend(_permute8(_lane_chunks(jnp.concatenate(
                [pltpu.bitcast(wv_r[t & 1, e], U32) for e in range(4)], axis=0))))

        def w_sums(src, dst, m, cc, gate):
            ww = [[gate(src(m, 2 * (q >> 1) + (e >> 1), 2 * (2 * (q & 1) + (e & 1)) + cc))
                   for e in range(4)] for q in range(4)]
            for n, w in enumerate(_words49(_rhs7, ww, m)):
                dst[7 * m + n, cc, blk(t, 8), :] = w
            return [], 0, lambda: dst[7 * m + _zero(t, 0), cc, blk(t, 8), :]

        def v_src(m, rq, ch):
            return wv[ch][8 * rq:8 * rq + 8]

        def o_src(m, rq, ch):
            return wob_r[((t >> 1) & 1) + _zero(t, m), rq, blk(t & 1, 8), pl.ds(128 * ch, 128)]

        segs, step = (P0S, P0T) if peel else (P1S, 32)
        sched = _Sched(t > 99, _plan1(segs, P0W * peel, step, P0N if peel else P1N), dict(
            x=[part(act_sums, x_r, xq, 2, m, sr, r)
               for m in range(7) for sr in range(2) for r in range(2)],
            c=[part(act_sums, c_r, cq, 1, m, 0, r) for m in range(7) for r in range(2)],
            v=[part(w_sums, v_src, wv49, m, cc) for m in range(7) for cc in range(2)],
            o=[part(w_sums, o_src, wob49, m, cc) for m in range(7) for cc in range(2)]))

        first = t < 2
        for k, (half, r0, n) in enumerate(segs):
            if k == P0W * peel:
                if peel:
                    for d in group0[1:-3]:
                        d.wait()
                load_wv()
            w = jnp.concatenate([wperm[4 * half + cc] for cc in range(4)], axis=1)
            r = sched.mm(k, xs_u[t >> 1, pl.ds(r0 // 2, n // 2), :], w, step=step)
            if k == len(segs) - 1:
                sched.finish()
                stage_first(t + 1)
                d = group(t + 2)
                for d in d[2:] + d[:2] + (cp_p(0) + (cp_gw(),)) * peel:
                    d.start()
            for cc in range(4):
                sl = (8 * (t & 1) + 4 * half + cc, pl.ds(PAD + r0, n), slice(None))
                new = r[:, cc * 128:(cc + 1) * 128]
                qk_b[sl] = new if peel else jnp.where(first, 0.0, qk_b[sl]) + new
        return t

    zero = jnp.max(vb[0, pl.ds(TQ, 8), :]).astype(jnp.int32)
    cp_w(0, sem_a.at[1]).wait()
    stage_first(0)
    group(1)[1].start()
    for t in range(2):
        cp_x(-t, sem_a.at[2]).wait()
    p1_step(zero, True)
    for d in group0[-3:]:
        d.wait()
    last = jax.lax.fori_loop(1, 16, lambda t, c: p1_step(t, False), 0)

    row = jax.lax.broadcasted_iota(jnp.int32, (TQ, TQ), 0)
    col = jax.lax.broadcasted_iota(jnp.int32, (TQ, TQ), 1)
    col = (col & ~31) | ((col & 1) << 4) | ((col & 31) >> 1)
    rowi = jax.lax.broadcasted_iota(jnp.int32, (RB, 128), 0)
    odd = (jax.lax.broadcasted_iota(jnp.int32, (RB, 128), 1) & 1) == 1
    QSCALE = DA ** -0.5 * LOG2E

    def pair_rows(src, slot, r0, n, gate):
        return [_split(gate(src[slot, pl.ds(r0 + par, n // 2, stride=2), :])) for par in range(2)]

    def staging(g, z, never):
        ns = DC // SCR

        def scales(n1, k, gate):
            res = []
            for h in range(2):
                if k < ns:
                    w = gate(wkv_r[g & 1, pl.ds(n1 * DC + k * SCR, SCR), :])
                    w = pltpu.bitcast(w, jnp.int32) & (0x7F80 << (16 * h))
                else:
                    w = gate(sc_s[2 * n1 + h, pl.ds(0, 8 * ns), :])
                e = _tree([w[r:r + 8] for r in range(0, w.shape[0], 8)], jnp.maximum)
                if k == ns:
                    e = pltpu.bitcast(e << (16 - 16 * h), F32)
                    e = jnp.max(e, axis=0, keepdims=True)
                    e = jnp.clip(pltpu.bitcast(e, jnp.int32), 1 << 23, 253 << 23)
                    e = jnp.broadcast_to(e, (8, 128))
                    sc_s[2 * n1 + h, pl.ds(8 * ns + 8, 8), :] = (254 << 23) - e
                sc_s[2 * n1 + h, pl.ds(8 * k, 8), :] = e
                res.append(pltpu.bitcast(e, U32))
            return res, 0, lambda: pltpu.bitcast(sc_s[2 * n1, blk(k + _zero(z, 0), 8), :], U32)

        def rhs49(dst, tiles, scale, m, r, extra=()):
            res = [_ops49(_rhs7,
                          [[scale(tiles[2 * (q >> 1) + (e >> 1)][q & 1][par][e & 1],
                                  2 * (q & 1) + (e & 1)) for e in range(4)] for q in range(4)],
                          m) for par in range(2)]
            for k, (lo, hi) in enumerate(zip(*res)):
                w = _join(lo, hi)
                if k < len(extra):
                    w = jnp.where(never, extra[k], w)
                dst[7 * m + k, pl.ds(8 * r, 8), :] = w

        def kv(m, r, gate):
            if m == 0 and r == 0:
                for k in range(4):
                    ups[k] = pltpu.bitcast(gate(sc_s[k, pl.ds(8 * ns, 8), :]), F32)
            down = [pltpu.bitcast(sc_s[k + _zero(z, m), pl.ds(8 * ns + 8, 8), :], F32)
                    for k in range(4)]
            tiles = [[pair_rows(wkv_r, (g & 1) + _zero(z, m), n1 * DC + kt * 128 + 16 * r, 16, gate)
                      for n1 in range(2)] for kt in range(4)]
            rhs49(wkv, tiles, lambda w, k: w * down[k], m, r)
            return [], 0, lambda: wkv[7 * m, blk(r + _zero(z, 0), 8), :]

        def qw(m, r, gate):
            tiles = [[pair_rows(wq_r, ((g + 1 + n1) & 3) + _zero(z, m), kt * 256 + 16 * r, 16, gate)
                      for n1 in range(2)] for kt in range(4)]
            rhs49(wq49, tiles, lambda w, k: w, m, r, sc.pop(0)(gate)[0] if sc else ())
            return [], 0, lambda: wq49[7 * m, blk(r + _zero(z, 0), 8), :]

        sc = [part(scales, n1, k) for k in range(ns + 1) for n1 in range(2)]
        return dict(sc=sc,
                    kv=[part(kv, m, r) for m in range(7) for r in range(8)],
                    qw=[part(qw, m, r) for m in range(7) for r in range(16)])

    sched = _Sched(last > 99, _planx(), staging(-1, last, last > 99))
    w0 = pair_rows(wq_r, 0, 0, M, lambda x: x)
    w0 = [_join(w0[0][h], w0[1][h]) for h in range(2)]
    for g in range(4):
        for e in range(2):
            for h in range(2):
                q = [sched.mm(8 * g + 4 * e + 2 * h + k, jnp.concatenate(
                    [xs_u[4 * k + u, pl.ds((4 * g + 2 + e) * HQ, HQ), :] for u in range(4)], axis=1),
                    w0[h][256 * k:256 * k + 256], step=16) for k in range(2)]
                qn[h, g, e] = _pack((q[0] + q[1]) * QSCALE)
    sched.finish()
    for d in group(16) + group(17):
        d.wait()
    for d in cp_p(1):
        d.start()
    plan2 = _plan2()

    def p2_body(p, carry):
        for d in cp_p(p):
            d.wait()
        causal = col <= row
        never = p > NP
        jobs = staging(p, p, never)
        sched = _Sched(never, plan2, jobs)
        mm = sched.mm

        r0 = pl.multiple_of(p * TQ, TQ)

        prods = {}

        def project(kind, j, n, lhs, rhs):
            got = prods.setdefault((kind, j), {})
            for m in ORDER[len(got):len(got) + n]:
                got[m] = _combine(lambda k: mm((kind, j, 7 * len(got) + ORDER.index(k)),
                                               part(lhs, 7 * m + k), rhs(7 * m + k)))
            if len(got) < 7:
                return None
            c = _combine(lambda m: got[m])
            return [[c[(rg & 2) + (cg >> 1)][2 * (rg & 1) + (cg & 1)] for rg in range(4)]
                    for cg in range(4)]

        def pair(ref, rows):
            return lambda k: jnp.concatenate([ref[k, sr, rows, :] for sr in range(2)], axis=1)

        def x_rows(b, n):
            return lambda k: jnp.concatenate([jnp.concatenate(
                [xq[k, b + j, pl.ds(16 * sr, 16), :] for sr in range(2)], axis=1)
                for j in range(n)], axis=0)

        def proj_b(kind, n, lhs, w, dst, off):
            c = project(kind, 0, n, lhs, pair(w, slice(None)))
            for cg in range(4 * (c is not None)):
                for rg in range(4):
                    for cc in range(2):
                        dst[2 * cg + cc, pl.ds(off + (PAD + rg * QQ), QQ), :] = (
                            c[cg][rg][:, cc * 128:(cc + 1) * 128])

        def proj_bv():
            for cc in range(8):
                vb[cc, pl.ds(0, PAD), :] = vb[cc, pl.ds(TQ, PAD), :]
            proj_b("bv", 7, x_rows(p, 1), wv49, vb, 0)

        def proj_bo(n):
            proj_b("bo", n, pair(ob49, slice(None)), wob49, qk_b, r0)

        def local_qk(rb, k, gate):
            rz = pl.multiple_of((p + _zero(p, k)) * TQ, TQ)
            q = [qk_b[cc, pl.ds(rz + (PAD + rb * RB), RB), :] for cc in range(8)]
            q[0] = gate(q[0])
            for w in range(LG * k, LG * k + LG):
                t = _fold([q[cc] * qk_b[8 + cc, pl.ds(r0 + (PAD + rb * RB - DIL * w), RB), :]
                           for cc in range(8)], jnp.add)
                t = t + pltpu.roll(t, 64, 1)
                t = t + jnp.where(odd, pltpu.roll(t, 1, 1), pltpu.roll(t, 127, 1))
                t = t * (DB ** -0.5 * LOG2E)
                if rb == 0 and w:
                    t = jnp.where(rowi + r0 >= DIL * w, t, NEG)
                lg_s[w, pl.ds(rb * RB, RB), :] = t
            return [], 1, lambda: pltpu.bitcast(lg_s[w, blk(2 * rb + _zero(p, 0), 8), :], U32)

        def local_sm(rb, e, gate):
            rows = pl.ds(rb * RB + SMR * e, SMR)
            lg = [gate(lg_s[w, rows, :]) for w in range(WIN)]
            m = _tree(lg, jnp.maximum)
            ps = [jnp.exp2(t - m) for t in lg]
            l = _tree(ps, jnp.add)
            r = pl.reciprocal(l, approx=True)
            r = r * (2.0 - l * r)
            for w in range(WIN):
                pr_s[w, rows, :] = ps[w] * r
            return [], 2, lambda: pltpu.bitcast(pr_s[0, blk(2 * rb + e + _zero(p, 0), 8), :], U32)

        def local_pv(rb, k, gate):
            rows = pl.ds(rb * RB, RB)
            ps = [pr_s[w + _zero(p, k), rows, :] for w in range(WIN)]
            ps[0] = gate(ps[0])
            o = [_fold([ps[w] * vb[cc, pl.ds(PAD + rb * RB - DIL * w, RB), :] for w in range(WIN)],
                       jnp.add) for cc in (k, k + 4)]
            for e in range(2):
                o_s[k + 4 * e, rows, :] = o[e]
            return [], 0, lambda: pltpu.bitcast(o_s[k, blk(2 * rb + _zero(p, 0), 8), :], U32)

        def o_sums(m, cc, r, gate):
            res = [_ops49(_lhs7, [[gate(o_s[
                2 * (2 * (q & 1) + (e & 1)) + cc + _zero(p, m),
                pl.ds(QQ * (2 * (q >> 1) + (e >> 1)) + 16 * r + par, 8, stride=2), :])
                for e in range(4)] for q in range(4)], m) for par in range(2)]
            for n, (lo, hi) in enumerate(zip(*res)):
                ob49[7 * m + n, cc, pl.ds(8 * r, 8), :] = _join(lo, hi)
            return [], 0, lambda: ob49[7 * m, cc, blk(r + _zero(p, 0), 8), :]

        jobs["os"] = [part(o_sums, m, cc, r) for r in range(2) for cc in range(2) for m in range(7)]
        order = list(range(0, 8, 2)) + list(range(1, 8, 2))
        jobs["lo"] = []
        for k in range(len(order) + SML):
            for f, d, n in ((local_sm, SML, RB // SMR), (local_qk, 0, 8 // LG)):
                if 0 <= k - d < len(order):
                    jobs["lo"] += [part(f, order[k - d], e) for e in range(n)]
        jobs["lv"] = [part(local_pv, rb, e) for rb in order for e in range(4)]

        def out_weights(m, r, gate):
            ww = [[gate(wo_r[(p & 1) + _zero(p, m),
                             pl.ds((2 * (q >> 1) + (e >> 1)) * HQ + 8 * r, 8),
                             pl.ds((2 * (q & 1) + (e & 1)) * 128, 128)])
                   for e in range(4)] for q in range(4)]
            rows = blk(8 * (p >> 1) + r, 8)
            extra = jobs["sc"].pop(0)(gate)[0] if jobs["sc"] else []
            for n, w in enumerate(_words49(_rhs7, ww, m)):
                if n < len(extra):
                    w = jnp.where(never, extra[n], w)
                wo49[7 * m + n, p & 1, rows, :] = w
            return [], 0, lambda: wo49[7 * m + _zero(p, 0), p & 1, rows, :]

        jobs["wo"] = [part(out_weights, m, r) for m in range(7) for r in range(8)]

        ks, vs, qs = {}, {}, {}
        done = {}

        def blocks(c, scale, pack):
            c = [[pack(t * scale(cg)) for t in c[cg]] for cg in range(4)]
            return [[jnp.concatenate([t[16 * e:16 * e + 16] for t in c[cg]], axis=0)
                     for e in range(2)] for cg in range(4)]

        def proj_kv(j, n):
            c = project("kv", j, n, lambda k: jnp.concatenate(
                [cq[k, 2 * j], cq[k, 2 * j + 1]], axis=0), lambda k: wkv[k])
            if c is not None:
                c = blocks(c, lambda cg: ups[cg][:1], _riffle)
                for cg in range(4):
                    for e in range(2):
                        (vs, ks)[cg >> 1][(cg & 1, 2 * j + e)] = c[cg][e]

        def proj_q(g, n):
            c = project("q", g, n, x_rows(4 * g + 2 * (p & 1), 2), lambda k: wq49[k])
            if c is not None:
                c = blocks(c, lambda cg: QSCALE, _pack)
                for h in range(2):
                    for e in range(2):
                        old = qn[h, g, e]
                        for b in range(2):
                            qs[(h, 4 * g + 2 * b + e)] = jnp.where((p & 1) == b, c[h][e], old)
                        qn[h, g, e] = c[2 + h][e]

        def qk(h, i, dep):
            kk = jnp.concatenate([ks[(h, j)] for j in range(i + 1)], axis=0)
            q = qs[(h, i)]
            if dep is not None:
                q = jnp.where(never, done[(h, dep)], q)
            ch = _lane_chunks(mm(("qk", h, i), q, kk, NT, 512))
            ch[i] = jnp.where(causal, ch[i], NEG)
            return ch

        def softmax_pv(h, i, ch):
            m = jnp.max(_fold(ch, jnp.maximum), axis=1, keepdims=True)
            ps = [jnp.exp2(c - m) for c in ch]
            lp = ps[0]
            for j in range(1, i + 1):
                lp = lp + ps[j]
                if TIE and (j % TIE == TIE - 1 or j == i):
                    ps[j] = jnp.where(never, lp, ps[j])
            pb = jnp.concatenate(ps, axis=1).astype(BF16)
            vv = jnp.concatenate([vs[(h, j)] for j in range(i + 1)], axis=0)
            o = mm(("pv", h, i), pb, vv)
            if i >= LDEP:
                lp = jnp.where(never, o, lp)
            l = jnp.sum(lp, axis=1, keepdims=True)
            r = pl.reciprocal(l, approx=True)
            r = r * (2.0 - l * r)
            cn = _pack(o * r)
            done[(h, i)] = cn
            if FA <= i < NQ - 1:
                if h == 0 and F0 < 0:
                    site = ("qk", 1, i + 1)
                elif i + 3 < NQ:
                    site = ("kv", (i + 1) // 2 + 1, KVS * ((i + 1) & 1) + (F0, FD)[h])
                else:
                    site = ("bo", 0, 7 * (i + 3 - NQ) * BOP[0] + 8 * h)
                sched.pending.setdefault(site, []).append(cn)
            ctx[2 * p + h, pl.ds(i * HQ, HQ), :] = cn

        proj_bv()
        proj_kv(0, 7)
        proj_q(0, 7)
        for i in range(NQ):
            dep = i - DEP if DEP <= i < FA + DEP else None
            s0 = qk(0, i, dep)
            s1 = qk(1, i, dep)
            if i + 2 < NQ:
                proj_kv(i // 2 + 1, 7 if i & 1 else KVS // 7)
                if i < 6:
                    proj_q(i // 2 + 1, 7 if i & 1 else QS // 7)
            else:
                proj_bo(BOP[i + 2 - NQ])
            softmax_pv(0, i, s0)
            softmax_pv(1, i, s1)
        proj_bo(BOP[2])
        sched.finish()
        for d in cp_p(p + 2):
            d.start()
        return carry

    jax.lax.fori_loop(0, NP, p2_body, 0)

    cp_gw().wait()
    gw = gw_ref[...].astype(F32)
    plan3 = _plan3()
    cab = (ca0, ca1)

    def p3_body(i, carry):
        r0 = pl.multiple_of(i * TO, TO)
        h0 = pl.multiple_of(i * (TO // 2), TO // 2)
        never = i > S

        def ctx_words(m, u, r, n):
            return [[ctx[4 * u + 2 * (q & 1) + (e & 1),
                         pl.ds(h0 + _zero(i, m) * 8 + ((2 * (q >> 1) + (e >> 1)) * QQ + r), n), :]
                     for e in range(4)] for q in range(4)]

        def operands(k, u, r, gate):
            m = ORDER[k]
            cw = [[gate(w) for w in q] for q in ctx_words(m, u, r, 8)]
            for n, w in enumerate(_words49(_lhs7, cw, m)):
                if not (m in (2, 3) and n in (2, 3)):
                    cab[k & 1][n, pl.ds(r, 8), pl.ds(u * 128, 128)] = w
            return [], 0, lambda: cab[k & 1][_zero(i, 0), pl.ds(r, 8), pl.ds(u * 128, 128)]

        def gate_rows(r, gate):
            gs = _fold([_bf(gate(xs_u[j, pl.ds(h0 + r, 8), :])).astype(F32) * gw[j:j + 1]
                        for j in range(8)], jnp.add)
            g = jax.nn.sigmoid(jnp.sum(gs, axis=1, keepdims=True))
            g_s[pl.ds(2 * r, 16), :] = jnp.broadcast_to(g, (16, 128))
            return [], 0, lambda: pltpu.bitcast(g_s[blk(r // 4 + _zero(i, 0), 8), :], U32)

        pr = {}

        def mix(q, e, cc, gate):
            off = (2 * (q >> 1) + (e >> 1)) * HQ
            ch = 4 * cc + 2 * (q & 1) + (e & 1)
            a = _combine(lambda m: pr.get(m, pr[2])[e][:, cc * 128:(cc + 1) * 128])[q]
            g = gate(g_s[pl.ds(off, HQ), :])
            b = qk_b[ch, pl.ds(r0 + (PAD + off), HQ), :]
            out_s[pl.ds(r0 + off, HQ), pl.ds(ch * 128, 128)] = (g * a + (1.0 - g) * b).astype(BF16)
            return [], 0, lambda: pltpu.bitcast(
                out_s[blk(i * (TO // 16) + off // 16 + _zero(i, 0), 16), pl.ds(ch * 128, 128)], U32)

        sched = _Sched(never, plan3, dict(
            a=[part(operands, k, u, r) for k in range(1, 7) for u in range(HA // 4)
               for r in range(0, QQ, 8)],
            g=[part(gate_rows, r) for r in range(0, TO // 2, 8)],
            m=[part(mix, q, e, cc) for q in (1, 2, 0) for e in range(4) for cc in range(2)]))
        first = [[_words49(_lhs7, ctx_words(ORDER[0], u, 0, QQ), ORDER[0])[n]
                  for u in range(HA // 4)] for n in range(7)]

        def inner(m, n):
            k = ORDER.index(m)
            res = []
            for e in range(2):
                us = range(4 * e, 4 * e + 4)
                if m in (2, 3) and n in (2, 3):
                    lhs = jnp.concatenate([ctx_words(m, u, 0, QQ)[3 * (m - 2)][3 * (n - 2)]
                                           for u in us], axis=1)
                elif k == 0:
                    lhs = jnp.concatenate([first[n][u] for u in us], axis=1)
                else:
                    lhs = lambda: cab[k & 1][n, :, pl.ds(e * 512, 512)]
                rhs = jnp.concatenate([wo49[7 * m + n, cc, pl.ds(e * 256, 256), :]
                                       for cc in range(2)], axis=1)
                res.append(sched.mm((k, 2 * ORDER.index(n) + e), lhs, rhs))
                if (k, 2 * ORDER.index(n) + e) == (6, P3D):
                    for d in cp_out(i, 0):
                        d.start()
            return res[0] + res[1]

        for m in ORDER:
            pr[m] = _combine(lambda n: inner(m, n))
        sched.finish()
        for e in (1, 2, 0, 3):
            for cc in range(2):
                mix(3, e, cc, lambda x: x)
        for d in cp_out(i, 1):
            d.start()
        return carry

    jax.lax.fori_loop(0, S // TO, p3_body, 0)
    for g in range(NP, NP + 2):
        for d in cp_p(g):
            d.wait()
    for i in range(S // TO):
        for d in cp_out(i, 0) + cp_out(i, 1):
            d.wait()


@jax.jit
def pallas_gated_mix__compressed_kv_cla__sliding_local_dilated__prompt_kernel(
    A_x: jax.Array,
    A_c_kv: jax.Array,
    A_w_q: jax.Array,
    A_w_uk: jax.Array,
    A_w_uv: jax.Array,
    A_w_o: jax.Array,
    B_x: jax.Array,
    B_wqkv: jax.Array,
    B_wo: jax.Array,
    gate_w: jax.Array,
):
    del B_x
    any_spec = pl.BlockSpec(memory_space=pl.ANY)
    out = pl.pallas_call(
        _kernel,
        in_specs=[any_spec] * 9,
        out_specs=any_spec,
        out_shape=jax.ShapeDtypeStruct((S, M), BF16),
        scratch_shapes=[
            pltpu.VMEM((9, S // 2, 128), U32),
            pltpu.VMEM((2, HQ, M), U32),
            pltpu.VMEM((2, HQ, DC), U32),
            pltpu.VMEM((2, 128, M), BF16),
            pltpu.VMEM((2, 4, 16, M), BF16),
            pltpu.VMEM((2, 4, 16, M), U32),
            pltpu.VMEM((3, 2 * DC, 128), U32),
            pltpu.VMEM((4, M, 128), U32),
            pltpu.VMEM((2, 2 * DA, M // 2), U32),
            pltpu.VMEM((8, 64, 128), U32),
            pltpu.VMEM((49, NQ, 32, 128), U32),
            pltpu.VMEM((49, NQ, 16, 128), U32),
            pltpu.VMEM((49, 2, M // 8, 128), U32),
            pltpu.VMEM((49, 2, M // 8, 128), U32),
            pltpu.VMEM((49, 2, NP * QQ, 128), U32),
            pltpu.VMEM((49, HQ, 128), U32),
            pltpu.VMEM((49, TQ, 128), U32),
            pltpu.VMEM((4, 8, 128), F32),
            pltpu.VMEM((4, DC // SCR * 8 + 16, 128), jnp.int32),
            pltpu.VMEM((2, 4, 2, HQ, 128), U32),
            pltpu.VMEM((16, S + PAD, 128), F32),
            pltpu.VMEM((8, TQ + PAD, 128), F32),
            pltpu.VMEM((WIN, TQ, 128), F32),
            pltpu.VMEM((WIN, TQ, 128), F32),
            pltpu.VMEM((8, TQ, 128), F32),
            pltpu.VMEM((49, 2, 16, 128), U32),
            pltpu.VMEM((HA, S // 2, 128), U32),
            pltpu.VMEM((7, QQ, M), U32),
            pltpu.VMEM((7, QQ, M), U32),
            pltpu.VMEM((TO, 128), F32),
            pltpu.VMEM((S, M), BF16),
            pltpu.VMEM((8, 128), BF16),
            pltpu.SemaphoreType.DMA((2,)),
            pltpu.SemaphoreType.DMA((2,)),
            pltpu.SemaphoreType.DMA((3,)),
        ],
        compiler_params=pltpu.CompilerParams(vmem_limit_bytes=120 * 1024 * 1024,
                                             disable_bounds_checks=True),
    )(
        A_x.reshape(S, M),
        A_c_kv.reshape(S, DC),
        A_w_q,
        A_w_uk,
        A_w_uv,
        A_w_o.reshape(HA * DA, M),
        B_wqkv.reshape(2, M // 2, 3 * M),
        B_wo.reshape(HB // 2, 2, DB, M),
        gate_w.reshape(8, 128),
    )
    return out.reshape(1, S, M)
```

```python
import functools

import jax
import jax.numpy as jnp
import jax.experimental.pallas as pl
import jax.experimental.pallas.tpu as pltpu

F32 = jnp.float32
BF16 = jnp.bfloat16
U32 = jnp.uint32

S = 2048
M = 1024
HA = 32
DA = 128
DC = 512
HB = 32
DB = 32
WIN = 8
DIL = 2
PAD = 16
LOG2E = 1.4426950408889634
NEG = -1e9

TQ = 128
HQ = TQ // 2
QQ = TQ // 4
BOP = (2, 3, 2)
LX = 16
KVS = 28
QS = 28
QST = 2
LQ0 = 1
LG = 2
XN = 28
XQ = 50
SK = 3
SMR = 16
P1N = 108
P1A = 60
P0W = 1
P0T = 16
P0N = 104
P0S = ((0, 0, 2048), (1, 0, 1024), (1, 1024, 768), (1, 1792, 128), (1, 1920, 128))
P1S = ((0, 0, 2048), (1, 0, 1536), (1, 1536, 384), (1, 1920, 128))
P3S = 3
P3M = 6
P3D = 8
P3E = 12
NQ = S // TQ
NP = HA // 2
DEP = 2
SCR = 32
LN = 80
SML = 1
LE = 2
LI = 99
LA = 24
LB = 4
LS = 1
BS = 2
LP = ("kv", 1, 8)
BX = 8
BE = 42
FA = 6
F0 = 0
FD = 8
TIE = 4
RB = 16
LDEP = 4
TO = 256
NN = (((1,), (0,)), ((), ()))
NT = (((1,), (1,)), ((), ()))


def _plan2():
    plan = {}

    def put(name, count, start, until):
        plan.setdefault(start, []).extend([(name, until)] * count)

    def after_qk(i):
        if i >= NQ - 2:
            return ("bo", 0, 7 * (i - NQ + 2) * BOP[0] + BX)
        return ("kv", i // 2 + 1, KVS * (i & 1) + LX)

    def fill(name, count, sites):
        for start, room, until in sites:
            n = min(count, room - len(plan.get(start, ())))
            put(name, n, start, until)
            count -= n
        assert count == 0, (name, count)

    def qk_sites(lo, hi):
        return [(("qk", h, i), max(i + 1 - h * SK, 0), after_qk(i))
                for i in range(lo, hi) for h in range(2)]

    def q_sites(g, lo, hi, until):
        return [(("q", g, k), 1, until) for k in range(lo, hi, QST)]

    ticks = ([("bv", 0, k) for k in range(LA, 49, LS)] + [("kv", 0, k) for k in range(0, 49, 2)]
             + [("q", 0, k) for k in range(49)])
    for name, site in zip(_spread(["lo"] * (64 // LG + 128 // SMR), LN), ticks):
        put(name, 1, site, LP)
    first = [(site, 1, ("kv", 1, 8)) for site in ticks[LN + LI:-LB:LE]]
    host = [(("bv", 0, k), 1, ("kv", 0, 8)) for k in range(0, min(LA, 46), BS)]
    early = []
    for g in range(1, 4):
        early += q_sites(g, 0, QS - 4, after_qk(2 * g - 1))
        early += qk_sites(max(2 * g - 1, LQ0), 2 * g)
        early += q_sites(g, QS, 45, after_qk(2 * g))
        early += qk_sites(max(2 * g, LQ0), 2 * g + 1)
    fill("lv", 32, first + early)
    fill("wo", 56, host + early)
    fill("os", 28, early + qk_sites(7, 14))
    fill("qw", 112, qk_sites(7, 14))
    fill("kv", 56, qk_sites(14, 16) + [(("bo", 0, k), 1, ("bo", 0, BE))
                                       for k in range(7 * BOP[0], 35)])
    return plan


def _planx():
    names = _spread(["qw"] * XQ + ["kv", "qw"] * 56 + ["qw"] * (56 - XQ), 8 * XN)
    return {k: [(n, 31) for n in names[8 * k:8 * k + 8]] for k in range(XN)}


def _spread(names, ticks):
    out = [None] * ticks
    for k, name in enumerate(names):
        out[k * ticks // len(names)] = name
    return out


def _plan1(segs, lo, step, count):
    end = len(segs) - 2
    ticks = [k for k in range(lo, end) for _ in range(segs[k][2] // step)][:count]
    n = len(ticks) * P1A // 100
    names = _spread(["x"] * 28 + ["c"] * 14 + ["o"] * 14, n) + _spread(["v"] * 14, len(ticks) - n)
    plan = {}
    for k, name in zip(ticks, names):
        plan.setdefault(k, []).append((name, end))
    return plan


def _plan3():
    plan = {}
    for k in range(6):
        lo = P3S if k == 0 else 0
        extra = ["g"] * 8 if k in (1, 2) else []
        names = _spread(["a"] * 32 + extra, 4 * (P3E - lo))
        for d in range(lo, P3E):
            plan[(k, d)] = [(n, (k + 1, 0)) for n in names[4 * (d - lo):4 * (d - lo) + 4]]
    names = _spread(["m"] * 24, 4 * P3M)
    for d in range(P3M):
        plan[(6, d)] = [(n, (6, P3D)) for n in names[4 * d:4 * d + 4]]
    return plan


_STAGES = ((2, 4), (1, 3), (0, 2), (0, 6), (0, 1))


def _permute8(cols):
    cols = list(cols)
    lane = jax.lax.broadcasted_iota(jnp.int32, cols[0].shape, 1)
    for va, lb in _STAGES:
        lo = (lane & (1 << lb)) == 0
        sh = 1 << lb
        idx = [i for i in range(8) if not (i >> va) & 1]
        if lb == 6:
            rr = [pltpu.roll(jnp.where(lo, cols[i | (1 << va)], cols[i]), 64, 1) for i in idx]
            for i, r in zip(idx, rr):
                a, b = cols[i], cols[i | (1 << va)]
                cols[i] = jnp.where(lo, a, r)
                cols[i | (1 << va)] = jnp.where(lo, r, b)
        else:
            rb = [pltpu.roll(cols[i | (1 << va)], sh, 1) for i in idx]
            ra = [pltpu.roll(cols[i], 128 - sh, 1) for i in idx]
            for i, xa, xb in zip(idx, ra, rb):
                a, b = cols[i], cols[i | (1 << va)]
                cols[i] = jnp.where(lo, a, xb)
                cols[i | (1 << va)] = jnp.where(lo, xa, b)
    return cols


def _pack(x):
    return pltpu.bitcast(x.astype(BF16), U32)


def _bf(x):
    return pltpu.bitcast(x, BF16)


def _split(w):
    return (pltpu.bitcast(w << 16, F32), pltpu.bitcast(w & jnp.uint32(0xFFFF0000), F32))


def _join(lo, hi):
    return pltpu.bitcast(pltpu.pack_elementwise([lo, hi], packed_dtype=BF16), U32)


def _riffle(x):
    return jnp.concatenate([_join(x[r:r + 16], x[r + 16:r + 32]) for r in range(0, x.shape[0], 32)],
                           axis=0)


def _lhs7(a11, a12, a21, a22):
    return [a11 + a22, a21 + a22, a11, a22, a11 + a12, a21 - a11, a12 - a22]


def _rhs7(b11, b12, b21, b22):
    return [b11 + b22, b11, b12 - b22, b21 - b11, b22, b11 + b12, b21 + b22]


def _combine(mm):
    add = functools.partial(jax.tree.map, jnp.add)
    sub = functools.partial(jax.tree.map, jnp.subtract)
    m2 = mm(2)
    m3 = mm(3)
    m4 = mm(4)
    c12 = add(m2, m4)
    t11 = sub(m3, m4)
    m1 = mm(1)
    c21 = add(m1, m3)
    t22 = sub(m2, m1)
    m0 = mm(0)
    t11 = add(t11, m0)
    t22 = add(t22, m0)
    c11 = add(t11, mm(6))
    return c11, c12, c21, add(t22, mm(5))


ORDER = (2, 3, 4, 1, 0, 6, 5)


def _zero(i, m):
    return i >> (8 + m)


def _merge(vals):
    return _fold([v[r:r + 8, c:c + 128] for v in vals for r in range(0, v.shape[0], 8)
                  for c in range(0, v.shape[1], 128)], jnp.bitwise_or)


def _gate(never, g):
    def gate(x):
        t = jnp.tile(pltpu.bitcast(g, x.dtype), (x.shape[0] // 8, x.shape[1] // 128))
        return jnp.where(never, t, x)
    return gate


def _tie(never, x, deps):
    if not deps:
        return x
    top = jnp.where(never, _merge(deps), x[:8, :128])
    if x.shape[1] > 128:
        top = jnp.concatenate([top, x[:8, 128:]], axis=1)
    return jnp.concatenate([top, x[8:]], axis=0)


class _Sched:
    def __init__(self, never, plan, jobs):
        self.never, self.plan, self.jobs, self.pending = never, plan, jobs, {}

    def mm(self, site, a, b, dims=NN, width=128, step=32):
        deps = [d() if callable(d) else d for d in self.pending.pop(site, ())]
        a = a() if callable(a) else a
        tie = functools.partial(_tie, self.never, deps=deps)
        a, b = (_bf(tie(a)), _bf(b)) if a.dtype == U32 else (a, _bf(tie(b)))
        out = jax.lax.dot_general(a, b, dims, preferred_element_type=F32)
        per = out.shape[0] // step
        last = {}
        for k, (name, until) in enumerate(self.plan.get(site, ())):
            if name is not None:
                r, c = step * (k % per), width * (k // per)
                vals, tag, stored = self.jobs[name].pop(0)(
                    _gate(self.never, out[r:r + 8, c:c + 128]))
                self.pending.setdefault(until, []).extend(vals)
                last[(name, tag, until)] = stored
        for (_, _, until), stored in last.items():
            if stored is not None:
                self.pending[until].append(stored)
        return out

    def finish(self):
        assert not any(self.jobs.values()) and not any(self.pending.values())


def _ops49(fn, blocks, m):
    return fn(*[fn(*[blocks[q][e] for q in range(4)])[m] for e in range(4)])


def _words49(fn, words, m):
    halves = [[_split(w) for w in q] for q in words]
    lo = _ops49(fn, [[h[0] for h in q] for q in halves], m)
    hi = _ops49(fn, [[h[1] for h in q] for q in halves], m)
    return [_join(a, b) for a, b in zip(lo, hi)]


def _fold(xs, op):
    acc = xs[0]
    for x in xs[1:]:
        acc = op(acc, x)
    return acc


def _tree(xs, op):
    while len(xs) > 1:
        xs = [op(a, b) for a, b in zip(xs[::2], xs[1::2])]
    return xs[0]


def _lane_chunks(x):
    return [x[:, j * 128:(j + 1) * 128] for j in range(x.shape[1] // 128)]


def _kernel(x_hbm, c_hbm, wq_hbm, wuk_hbm, wuv_hbm, wo_hbm, wqkv_hbm, wob_hbm, gw_hbm,
            out_hbm,
            xs_u, x_r, c_r, w_r, wv_r, wob_r, wkv_r, wq_r, wo_r,
            wperm, xq, cq, wv49, wob49, wo49, wkv, wq49, ups, sc_s, qn,
            qk_b, vb, lg_s, pr_s, o_s, ob49, ctx, ca0, ca1, g_s, out_s, gw_ref,
            sem_x, sem_p, sem_a):
    x_u = x_hbm.bitcast(U32)
    c_u = c_hbm.bitcast(U32)
    wo_u = wo_hbm.bitcast(U32)
    wq_u = wq_hbm.bitcast(U32)
    wuk_u = wuk_hbm.bitcast(U32)
    wuv_u = wuv_hbm.bitcast(U32)
    wob_u = wob_hbm.bitcast(U32)
    part = functools.partial

    def blk(j, n):
        return pl.ds(pl.multiple_of(j * n, n), n)

    def strip(j):
        return blk(j, 128)

    def cp_x(t, sem):
        k = (t + 1) >> 1
        return pltpu.make_async_copy(x_u.at[blk(t & 1, S // 4), strip(jnp.minimum(k, 7))],
                                     xs_u.at[jnp.minimum(k, 8), blk(t & 1, S // 4), :], sem)

    def cp_w(t, sem):
        u = t - 2 * (t >> 4)
        u = u - 2 * (u >> 4)
        return pltpu.make_async_copy(wqkv_hbm.at[u >> 3, strip((u >> 1) & 3), blk(u & 1, M)],
                                     w_r.at[u & 1], sem)

    def cp_wob(t, sem):
        b = (t + 1) >> 1
        c = jnp.minimum(b, 7)
        return tuple(pltpu.make_async_copy(
            wob_u.at[:, c & 1, 4 * (2 * (t & 1) + j) + (c & 2) + (c >> 2), :],
            wob_r.at[b & 1, 2 * (t & 1) + j], sem) for j in range(2))

    def group(t, sem1=None):
        sem = sem_x.at[t & 1]
        u = t - 2 * (t >> 4)
        return (
            cp_x(t, sem if sem1 is None else sem1),
            cp_w(t + 1, sem),
            pltpu.make_async_copy(x_u.at[blk(u, HQ), :], x_r.at[u & 1], sem),
            pltpu.make_async_copy(c_u.at[blk(u, HQ), :], c_r.at[u & 1], sem),
        ) + cp_wob(t, sem) + tuple(
            pltpu.make_async_copy(wqkv_hbm.at[e >> 1, blk(16 * (e & 1) + u, 16), pl.ds(2 * M, M)],
                                  wv_r.at[u & 1, e], sem) for e in range(4))

    def piece(t):
        late = t >> 4
        pq = (t >> 3) + late
        pk = (t >> 3) & 1
        u = (t & 15) + 2 * late
        sem = sem_a.at[3 + late]
        return (
            pltpu.make_async_copy(wo_u.at[blk(u, 16), pl.ds(0, M // 2)],
                                  wo_r.at[late, blk(u, 16), :], sem),
            pltpu.make_async_copy(wq_u.at[strip(t & 7), pq, :], wq_r.at[pq, strip(t & 7), :], sem),
            pltpu.make_async_copy(wq_u.at[blk(u, 64), 2, :], wq_r.at[2 + late, blk(u, 64), :], sem),
            pltpu.make_async_copy(wuk_u.at[blk(t & 7, 64), pk, :],
                                  wkv_r.at[1 - pk + late, blk(8 + (t & 7), 64), :], sem),
            pltpu.make_async_copy(wuv_u.at[blk(t & 7, 64), pk, :],
                                  wkv_r.at[1 - pk + late, blk(t & 7, 64), :], sem),
        )

    def cp_wq(p, sem):
        return pltpu.make_async_copy(wq_u.at[:, jnp.minimum(p, NP - 1), :], wq_r.at[p & 3], sem)

    def cp_p(g):
        slot = g & 1
        p = jnp.minimum(g + 1, NP - 1)
        o = jnp.minimum(g, NP - 1)
        sem = sem_p.at[slot]
        return (
            pltpu.make_async_copy(wo_u.at[blk(o >> 1, 2 * DA), blk(o & 1, M // 2)],
                                  wo_r.at[slot], sem),
            pltpu.make_async_copy(wuk_u.at[:, p, :], wkv_r.at[slot, pl.ds(DC, DC), :], sem),
            pltpu.make_async_copy(wuv_u.at[:, p, :], wkv_r.at[slot, pl.ds(0, DC), :], sem),
            cp_wq(g + 2, sem),
        )

    def cp_gw():
        return pltpu.make_async_copy(gw_hbm, gw_ref, sem_a.at[0])

    def cp_out(i, late):
        def cp(rows, cols):
            return pltpu.make_async_copy(out_s.at[rows, cols], out_hbm.at[rows, cols], sem_a.at[1])

        low = [cp(blk(2 * i + 1, TO // 2), pl.ds(512 * cc + 256 * late, 256)) for cc in range(2)]
        return low if late else [cp(blk(2 * i, TO // 2), pl.ds(0, M))] + low

    cp_w(0, sem_a.at[1]).start()
    group0, group1 = group(0, sem_a.at[2]), group(1)
    group0 = (group0[0], cp_x(-1, sem_a.at[2])) + group0[1:] + cp_wob(-1, sem_x.at[0])
    for d in group0 + group1[:1] + group1[2:]:
        d.start()

    for cc in range(8):
        qk_b[8 + cc, pl.ds(0, PAD), :] = jnp.zeros((PAD, 128), F32)
        vb[cc, pl.ds(TQ, PAD), :] = jnp.zeros((PAD, 128), F32)

    def stage_first(t):
        for cc, w in enumerate(_permute8(_lane_chunks(pltpu.bitcast(w_r[t & 1], U32)))):
            wperm[cc] = w

    def p1_step(t, peel):
        if not peel:
            for d in group(t):
                d.wait()

        def act_sums(src, dst, ns, m, sr, r, gate):
            cw = [[gate(src[(t & 1) + _zero(t, m), pl.ds(32 * (q >> 1) + 16 * (e >> 1) + 8 * r, 8),
                            pl.ds(((2 * (q & 1) + (e & 1)) * ns + sr) * 128, 128)])
                   for e in range(4)] for q in range(4)]
            for n, w in enumerate(_words49(_lhs7, cw, m)):
                dst[7 * m + n, t, pl.ds(16 * sr + 8 * r, 8), :] = w
            return [], 0, lambda: dst[7 * m + _zero(t, 0), t, pl.ds(16 * sr + 8 * r, 8), :]

        wv = []

        def load_wv():
            wv.extend(_permute8(_lane_chunks(jnp.concatenate(
                [pltpu.bitcast(wv_r[t & 1, e], U32) for e in range(4)], axis=0))))

        def w_sums(src, dst, m, cc, gate):
            ww = [[gate(src(m, 2 * (q >> 1) + (e >> 1), 2 * (2 * (q & 1) + (e & 1)) + cc))
                   for e in range(4)] for q in range(4)]
            for n, w in enumerate(_words49(_rhs7, ww, m)):
                dst[7 * m + n, cc, blk(t, 8), :] = w
            return [], 0, lambda: dst[7 * m + _zero(t, 0), cc, blk(t, 8), :]

        def v_src(m, rq, ch):
            return wv[ch][8 * rq:8 * rq + 8]

        def o_src(m, rq, ch):
            return wob_r[((t >> 1) & 1) + _zero(t, m), rq, blk(t & 1, 8), pl.ds(128 * ch, 128)]

        segs, step = (P0S, P0T) if peel else (P1S, 32)
        sched = _Sched(t > 99, _plan1(segs, P0W * peel, step, P0N if peel else P1N), dict(
            x=[part(act_sums, x_r, xq, 2, m, sr, r)
               for m in range(7) for sr in range(2) for r in range(2)],
            c=[part(act_sums, c_r, cq, 1, m, 0, r) for m in range(7) for r in range(2)],
            v=[part(w_sums, v_src, wv49, m, cc) for m in range(7) for cc in range(2)],
            o=[part(w_sums, o_src, wob49, m, cc) for m in range(7) for cc in range(2)]))

        first = t < 2
        for k, (half, r0, n) in enumerate(segs):
            if k == P0W * peel:
                if peel:
                    for d in group0[2:]:
                        d.wait()
                load_wv()
            w = jnp.concatenate([wperm[4 * half + cc] for cc in range(4)], axis=1)
            r = sched.mm(k, xs_u[t >> 1, pl.ds(r0 // 2, n // 2), :], w, step=step)
            if k == len(segs) - 1:
                sched.finish()
                stage_first(t + 1)
                d = group(t + 2)
                e = piece(t + 1)
                d = d[2:6] + e[:1] + d[6:] + d[:2] + e[1:]
                for d in d + (piece(0) + (cp_gw(),) if peel else ()):
                    d.start()
            for cc in range(4):
                sl = (8 * (t & 1) + 4 * half + cc, pl.ds(PAD + r0, n), slice(None))
                new = r[:, cc * 128:(cc + 1) * 128]
                qk_b[sl] = new if peel else jnp.where(first, 0.0, qk_b[sl]) + new
        return t

    zero = jnp.max(vb[0, pl.ds(TQ, 8), :]).astype(jnp.int32)
    cp_w(0, sem_a.at[1]).wait()
    stage_first(0)
    group1[1].start()
    for d in group0[:2]:
        d.wait()
    p1_step(zero, True)
    last = jax.lax.fori_loop(1, 16, lambda t, c: p1_step(t, False), 0)

    row = jax.lax.broadcasted_iota(jnp.int32, (TQ, TQ), 0)
    col = jax.lax.broadcasted_iota(jnp.int32, (TQ, TQ), 1)
    col = (col & ~31) | ((col & 1) << 4) | ((col & 31) >> 1)
    rowi = jax.lax.broadcasted_iota(jnp.int32, (RB, 128), 0)
    odd = (jax.lax.broadcasted_iota(jnp.int32, (RB, 128), 1) & 1) == 1
    QSCALE = DA ** -0.5 * LOG2E

    def pair_rows(src, slot, r0, n, gate):
        return [_split(gate(src[slot, pl.ds(r0 + par, n // 2, stride=2), :])) for par in range(2)]

    def staging(g, z, never):
        ns = DC // SCR

        def scales(n1, k, gate):
            res = []
            for h in range(2):
                if k < ns:
                    w = gate(wkv_r[g & 1, pl.ds(n1 * DC + k * SCR, SCR), :])
                    w = pltpu.bitcast(w, jnp.int32) & (0x7F80 << (16 * h))
                else:
                    w = gate(sc_s[2 * n1 + h, pl.ds(0, 8 * ns), :])
                e = _tree([w[r:r + 8] for r in range(0, w.shape[0], 8)], jnp.maximum)
                if k == ns:
                    e = pltpu.bitcast(e << (16 - 16 * h), F32)
                    e = jnp.max(e, axis=0, keepdims=True)
                    e = jnp.clip(pltpu.bitcast(e, jnp.int32), 1 << 23, 253 << 23)
                    e = jnp.broadcast_to(e, (8, 128))
                    sc_s[2 * n1 + h, pl.ds(8 * ns + 8, 8), :] = (254 << 23) - e
                sc_s[2 * n1 + h, pl.ds(8 * k, 8), :] = e
                res.append(pltpu.bitcast(e, U32))
            return res, 0, lambda: pltpu.bitcast(sc_s[2 * n1, blk(k + _zero(z, 0), 8), :], U32)

        def rhs49(dst, tiles, scale, m, r, extra=()):
            res = [_ops49(_rhs7,
                          [[scale(tiles[2 * (q >> 1) + (e >> 1)][q & 1][par][e & 1],
                                  2 * (q & 1) + (e & 1)) for e in range(4)] for q in range(4)],
                          m) for par in range(2)]
            for k, (lo, hi) in enumerate(zip(*res)):
                w = _join(lo, hi)
                if k < len(extra):
                    w = jnp.where(never, extra[k], w)
                dst[7 * m + k, pl.ds(8 * r, 8), :] = w

        def kv(m, r, gate):
            if m == 0 and r == 0:
                for k in range(4):
                    ups[k] = pltpu.bitcast(gate(sc_s[k, pl.ds(8 * ns, 8), :]), F32)
            down = [pltpu.bitcast(sc_s[k + _zero(z, m), pl.ds(8 * ns + 8, 8), :], F32)
                    for k in range(4)]
            tiles = [[pair_rows(wkv_r, (g & 1) + _zero(z, m), n1 * DC + kt * 128 + 16 * r, 16, gate)
                      for n1 in range(2)] for kt in range(4)]
            rhs49(wkv, tiles, lambda w, k: w * down[k], m, r)
            return [], 0, lambda: wkv[7 * m, blk(r + _zero(z, 0), 8), :]

        def qw(m, r, gate):
            tiles = [[pair_rows(wq_r, ((g + 1 + n1) & 3) + _zero(z, m), kt * 256 + 16 * r, 16, gate)
                      for n1 in range(2)] for kt in range(4)]
            rhs49(wq49, tiles, lambda w, k: w, m, r, sc.pop(0)(gate)[0] if sc else ())
            return [], 0, lambda: wq49[7 * m, blk(r + _zero(z, 0), 8), :]

        sc = [part(scales, n1, k) for k in range(ns + 1) for n1 in range(2)]
        return dict(sc=sc,
                    kv=[part(kv, m, r) for m in range(7) for r in range(8)],
                    qw=[part(qw, m, r) for m in range(7) for r in range(16)])

    for t in range(16):
        for d in piece(t):
            d.wait()
    sched = _Sched(last > 99, _planx(), staging(-1, last, last > 99))
    w0 = pair_rows(wq_r, 0, 0, M, lambda x: x)
    w0 = [_join(w0[0][h], w0[1][h]) for h in range(2)]
    for g in range(4):
        for e in range(2):
            for h in range(2):
                q = [sched.mm(8 * g + 4 * e + 2 * h + k, jnp.concatenate(
                    [xs_u[4 * k + u, pl.ds((4 * g + 2 + e) * HQ, HQ), :] for u in range(4)], axis=1),
                    w0[h][256 * k:256 * k + 256], step=16) for k in range(2)]
                qn[h, g, e] = _pack((q[0] + q[1]) * QSCALE)
    sched.finish()
    for d in group(16) + group(17) + piece(16):
        d.wait()
    for d in cp_p(1):
        d.start()
    plan2 = _plan2()

    def p2_body(p, carry):
        @pl.when(p > 0)
        def _():
            for d in cp_p(p):
                d.wait()

        causal = col <= row
        never = p > NP
        jobs = staging(p, p, never)
        sched = _Sched(never, plan2, jobs)
        mm = sched.mm

        r0 = pl.multiple_of(p * TQ, TQ)

        prods = {}

        def project(kind, j, n, lhs, rhs):
            got = prods.setdefault((kind, j), {})
            for m in ORDER[len(got):len(got) + n]:
                got[m] = _combine(lambda k: mm((kind, j, 7 * len(got) + ORDER.index(k)),
                                               part(lhs, 7 * m + k), rhs(7 * m + k)))
            if len(got) < 7:
                return None
            c = _combine(lambda m: got[m])
            return [[c[(rg & 2) + (cg >> 1)][2 * (rg & 1) + (cg & 1)] for rg in range(4)]
                    for cg in range(4)]

        def pair(ref, rows):
            return lambda k: jnp.concatenate([ref[k, sr, rows, :] for sr in range(2)], axis=1)

        def x_rows(b, n):
            return lambda k: jnp.concatenate([jnp.concatenate(
                [xq[k, b + j, pl.ds(16 * sr, 16), :] for sr in range(2)], axis=1)
                for j in range(n)], axis=0)

        def proj_b(kind, n, lhs, w, dst, off):
            c = project(kind, 0, n, lhs, pair(w, slice(None)))
            for cg in range(4 * (c is not None)):
                for rg in range(4):
                    for cc in range(2):
                        dst[2 * cg + cc, pl.ds(off + (PAD + rg * QQ), QQ), :] = (
                            c[cg][rg][:, cc * 128:(cc + 1) * 128])

        def proj_bv():
            for cc in range(8):
                vb[cc, pl.ds(0, PAD), :] = vb[cc, pl.ds(TQ, PAD), :]
            proj_b("bv", 7, x_rows(p, 1), wv49, vb, 0)

        def proj_bo(n):
            proj_b("bo", n, pair(ob49, slice(None)), wob49, qk_b, r0)

        def local_qk(rb, k, gate):
            rz = pl.multiple_of((p + _zero(p, k)) * TQ, TQ)
            q = [qk_b[cc, pl.ds(rz + (PAD + rb * RB), RB), :] for cc in range(8)]
            q[0] = gate(q[0])
            for w in range(LG * k, LG * k + LG):
                t = _fold([q[cc] * qk_b[8 + cc, pl.ds(r0 + (PAD + rb * RB - DIL * w), RB), :]
                           for cc in range(8)], jnp.add)
                t = t + pltpu.roll(t, 64, 1)
                t = t + jnp.where(odd, pltpu.roll(t, 1, 1), pltpu.roll(t, 127, 1))
                t = t * (DB ** -0.5 * LOG2E)
                if rb == 0 and w:
                    t = jnp.where(rowi + r0 >= DIL * w, t, NEG)
                lg_s[w, pl.ds(rb * RB, RB), :] = t
            return [], 1, lambda: pltpu.bitcast(lg_s[w, blk(2 * rb + _zero(p, 0), 8), :], U32)

        def local_sm(rb, e, gate):
            rows = pl.ds(rb * RB + SMR * e, SMR)
            lg = [gate(lg_s[w, rows, :]) for w in range(WIN)]
            m = _tree(lg, jnp.maximum)
            ps = [jnp.exp2(t - m) for t in lg]
            l = _tree(ps, jnp.add)
            r = pl.reciprocal(l, approx=True)
            r = r * (2.0 - l * r)
            for w in range(WIN):
                pr_s[w, rows, :] = ps[w] * r
            return [], 2, lambda: pltpu.bitcast(pr_s[0, blk(2 * rb + e + _zero(p, 0), 8), :], U32)

        def local_pv(rb, k, gate):
            rows = pl.ds(rb * RB, RB)
            ps = [pr_s[w + _zero(p, k), rows, :] for w in range(WIN)]
            ps[0] = gate(ps[0])
            o = [_fold([ps[w] * vb[cc, pl.ds(PAD + rb * RB - DIL * w, RB), :] for w in range(WIN)],
                       jnp.add) for cc in (k, k + 4)]
            for e in range(2):
                o_s[k + 4 * e, rows, :] = o[e]
            return [], 0, lambda: pltpu.bitcast(o_s[k, blk(2 * rb + _zero(p, 0), 8), :], U32)

        def o_sums(m, cc, r, gate):
            res = [_ops49(_lhs7, [[gate(o_s[
                2 * (2 * (q & 1) + (e & 1)) + cc + _zero(p, m),
                pl.ds(QQ * (2 * (q >> 1) + (e >> 1)) + 16 * r + par, 8, stride=2), :])
                for e in range(4)] for q in range(4)], m) for par in range(2)]
            for n, (lo, hi) in enumerate(zip(*res)):
                ob49[7 * m + n, cc, pl.ds(8 * r, 8), :] = _join(lo, hi)
            return [], 0, lambda: ob49[7 * m, cc, blk(r + _zero(p, 0), 8), :]

        jobs["os"] = [part(o_sums, m, cc, r) for r in range(2) for cc in range(2) for m in range(7)]
        order = list(range(0, 8, 2)) + list(range(1, 8, 2))
        jobs["lo"] = []
        for k in range(len(order) + SML):
            for f, d, n in ((local_sm, SML, RB // SMR), (local_qk, 0, 8 // LG)):
                if 0 <= k - d < len(order):
                    jobs["lo"] += [part(f, order[k - d], e) for e in range(n)]
        jobs["lv"] = [part(local_pv, rb, e) for rb in order for e in range(4)]

        def out_weights(m, r, gate):
            ww = [[gate(wo_r[(p & 1) + _zero(p, m),
                             pl.ds((2 * (q >> 1) + (e >> 1)) * HQ + 8 * r, 8),
                             pl.ds((2 * (q & 1) + (e & 1)) * 128, 128)])
                   for e in range(4)] for q in range(4)]
            rows = blk(8 * (p >> 1) + r, 8)
            extra = jobs["sc"].pop(0)(gate)[0] if jobs["sc"] else []
            for n, w in enumerate(_words49(_rhs7, ww, m)):
                if n < len(extra):
                    w = jnp.where(never, extra[n], w)
                wo49[7 * m + n, p & 1, rows, :] = w
            return [], 0, lambda: wo49[7 * m + _zero(p, 0), p & 1, rows, :]

        jobs["wo"] = [part(out_weights, m, r) for m in range(7) for r in range(8)]

        ks, vs, qs = {}, {}, {}
        done = {}

        def blocks(c, scale, pack):
            c = [[pack(t * scale(cg)) for t in c[cg]] for cg in range(4)]
            return [[jnp.concatenate([t[16 * e:16 * e + 16] for t in c[cg]], axis=0)
                     for e in range(2)] for cg in range(4)]

        def proj_kv(j, n):
            c = project("kv", j, n, lambda k: jnp.concatenate(
                [cq[k, 2 * j], cq[k, 2 * j + 1]], axis=0), lambda k: wkv[k])
            if c is not None:
                c = blocks(c, lambda cg: ups[cg][:1], _riffle)
                for cg in range(4):
                    for e in range(2):
                        (vs, ks)[cg >> 1][(cg & 1, 2 * j + e)] = c[cg][e]

        def proj_q(g, n):
            c = project("q", g, n, x_rows(4 * g + 2 * (p & 1), 2), lambda k: wq49[k])
            if c is not None:
                c = blocks(c, lambda cg: QSCALE, _pack)
                for h in range(2):
                    for e in range(2):
                        old = qn[h, g, e]
                        for b in range(2):
                            qs[(h, 4 * g + 2 * b + e)] = jnp.where((p & 1) == b, c[h][e], old)
                        qn[h, g, e] = c[2 + h][e]

        def qk(h, i, dep):
            kk = jnp.concatenate([ks[(h, j)] for j in range(i + 1)], axis=0)
            q = qs[(h, i)]
            if dep is not None:
                q = jnp.where(never, done[(h, dep)], q)
            ch = _lane_chunks(mm(("qk", h, i), q, kk, NT, 512))
            ch[i] = jnp.where(causal, ch[i], NEG)
            return ch

        def softmax_pv(h, i, ch):
            m = jnp.max(_fold(ch, jnp.maximum), axis=1, keepdims=True)
            ps = [jnp.exp2(c - m) for c in ch]
            lp = ps[0]
            for j in range(1, i + 1):
                lp = lp + ps[j]
                if TIE and (j % TIE == TIE - 1 or j == i):
                    ps[j] = jnp.where(never, lp, ps[j])
            pb = jnp.concatenate(ps, axis=1).astype(BF16)
            vv = jnp.concatenate([vs[(h, j)] for j in range(i + 1)], axis=0)
            o = mm(("pv", h, i), pb, vv)
            if i >= LDEP:
                lp = jnp.where(never, o, lp)
            l = jnp.sum(lp, axis=1, keepdims=True)
            r = pl.reciprocal(l, approx=True)
            r = r * (2.0 - l * r)
            cn = _pack(o * r)
            done[(h, i)] = cn
            if FA <= i < NQ - 1:
                if h == 0 and F0 < 0:
                    site = ("qk", 1, i + 1)
                elif i + 3 < NQ:
                    site = ("kv", (i + 1) // 2 + 1, KVS * ((i + 1) & 1) + (F0, FD)[h])
                else:
                    site = ("bo", 0, 7 * (i + 3 - NQ) * BOP[0] + 8 * h)
                sched.pending.setdefault(site, []).append(cn)
            ctx[2 * p + h, pl.ds(i * HQ, HQ), :] = cn

        proj_bv()
        proj_kv(0, 7)
        proj_q(0, 7)
        for i in range(NQ):
            dep = i - DEP if DEP <= i < FA + DEP else None
            s0 = qk(0, i, dep)
            s1 = qk(1, i, dep)
            if i + 2 < NQ:
                proj_kv(i // 2 + 1, 7 if i & 1 else KVS // 7)
                if i < 6:
                    proj_q(i // 2 + 1, 7 if i & 1 else QS // 7)
            else:
                proj_bo(BOP[i + 2 - NQ])
            softmax_pv(0, i, s0)
            softmax_pv(1, i, s1)
        proj_bo(BOP[2])
        sched.finish()
        for d in cp_p(p + 2):
            d.start()
        return carry

    jax.lax.fori_loop(0, NP, p2_body, 0)

    cp_gw().wait()
    gw = gw_ref[...].astype(F32)
    plan3 = _plan3()
    cab = (ca0, ca1)

    def p3_body(i, carry):
        r0 = pl.multiple_of(i * TO, TO)
        h0 = pl.multiple_of(i * (TO // 2), TO // 2)
        never = i > S

        def ctx_words(m, u, r, n):
            return [[ctx[4 * u + 2 * (q & 1) + (e & 1),
                         pl.ds(h0 + _zero(i, m) * 8 + ((2 * (q >> 1) + (e >> 1)) * QQ + r), n), :]
                     for e in range(4)] for q in range(4)]

        def operands(k, u, r, gate):
            m = ORDER[k]
            cw = [[gate(w) for w in q] for q in ctx_words(m, u, r, 8)]
            for n, w in enumerate(_words49(_lhs7, cw, m)):
                if not (m in (2, 3) and n in (2, 3)):
                    cab[k & 1][n, pl.ds(r, 8), pl.ds(u * 128, 128)] = w
            return [], 0, lambda: cab[k & 1][_zero(i, 0), pl.ds(r, 8), pl.ds(u * 128, 128)]

        def gate_rows(r, gate):
            gs = _fold([_bf(gate(xs_u[j, pl.ds(h0 + r, 8), :])).astype(F32) * gw[j:j + 1]
                        for j in range(8)], jnp.add)
            g = jax.nn.sigmoid(jnp.sum(gs, axis=1, keepdims=True))
            g_s[pl.ds(2 * r, 16), :] = jnp.broadcast_to(g, (16, 128))
            return [], 0, lambda: pltpu.bitcast(g_s[blk(r // 4 + _zero(i, 0), 8), :], U32)

        pr = {}

        def mix(q, e, cc, gate):
            off = (2 * (q >> 1) + (e >> 1)) * HQ
            ch = 4 * cc + 2 * (q & 1) + (e & 1)
            a = _combine(lambda m: pr.get(m, pr[2])[e][:, cc * 128:(cc + 1) * 128])[q]
            g = gate(g_s[pl.ds(off, HQ), :])
            b = qk_b[ch, pl.ds(r0 + (PAD + off), HQ), :]
            out_s[pl.ds(r0 + off, HQ), pl.ds(ch * 128, 128)] = (g * a + (1.0 - g) * b).astype(BF16)
            return [], 0, lambda: pltpu.bitcast(
                out_s[blk(i * (TO // 16) + off // 16 + _zero(i, 0), 16), pl.ds(ch * 128, 128)], U32)

        sched = _Sched(never, plan3, dict(
            a=[part(operands, k, u, r) for k in range(1, 7) for u in range(HA // 4)
               for r in range(0, QQ, 8)],
            g=[part(gate_rows, r) for r in range(0, TO // 2, 8)],
            m=[part(mix, q, e, cc) for q in (1, 2, 0) for e in range(4) for cc in range(2)]))
        first = [[_words49(_lhs7, ctx_words(ORDER[0], u, 0, QQ), ORDER[0])[n]
                  for u in range(HA // 4)] for n in range(7)]

        def inner(m, n):
            k = ORDER.index(m)
            res = []
            for e in range(2):
                us = range(4 * e, 4 * e + 4)
                if m in (2, 3) and n in (2, 3):
                    lhs = jnp.concatenate([ctx_words(m, u, 0, QQ)[3 * (m - 2)][3 * (n - 2)]
                                           for u in us], axis=1)
                elif k == 0:
                    lhs = jnp.concatenate([first[n][u] for u in us], axis=1)
                else:
                    lhs = lambda: cab[k & 1][n, :, pl.ds(e * 512, 512)]
                rhs = jnp.concatenate([wo49[7 * m + n, cc, pl.ds(e * 256, 256), :]
                                       for cc in range(2)], axis=1)
                res.append(sched.mm((k, 2 * ORDER.index(n) + e), lhs, rhs))
                if (k, 2 * ORDER.index(n) + e) == (6, P3D):
                    for d in cp_out(i, 0):
                        d.start()
            return res[0] + res[1]

        for m in ORDER:
            pr[m] = _combine(lambda n: inner(m, n))
        sched.finish()
        for e in (1, 2, 0, 3):
            for cc in range(2):
                mix(3, e, cc, lambda x: x)
        for d in cp_out(i, 1):
            d.start()
        return carry

    jax.lax.fori_loop(0, S // TO, p3_body, 0)
    for d in cp_p(NP) + cp_p(NP + 1):
        d.wait()
    for i in range(S // TO):
        for d in cp_out(i, 0) + cp_out(i, 1):
            d.wait()


@jax.jit
def pallas_gated_mix__compressed_kv_cla__sliding_local_dilated__prompt_kernel(
    A_x: jax.Array,
    A_c_kv: jax.Array,
    A_w_q: jax.Array,
    A_w_uk: jax.Array,
    A_w_uv: jax.Array,
    A_w_o: jax.Array,
    B_x: jax.Array,
    B_wqkv: jax.Array,
    B_wo: jax.Array,
    gate_w: jax.Array,
):
    del B_x
    any_spec = pl.BlockSpec(memory_space=pl.ANY)
    out = pl.pallas_call(
        _kernel,
        in_specs=[any_spec] * 9,
        out_specs=any_spec,
        out_shape=jax.ShapeDtypeStruct((S, M), BF16),
        scratch_shapes=[
            pltpu.VMEM((9, S // 2, 128), U32),
            pltpu.VMEM((2, HQ, M), U32),
            pltpu.VMEM((2, HQ, DC), U32),
            pltpu.VMEM((2, 128, M), BF16),
            pltpu.VMEM((2, 4, 16, M), BF16),
            pltpu.VMEM((2, 4, 16, M), U32),
            pltpu.VMEM((3, 2 * DC, 128), U32),
            pltpu.VMEM((4, M, 128), U32),
            pltpu.VMEM((2, 2 * DA, M // 2), U32),
            pltpu.VMEM((8, 64, 128), U32),
            pltpu.VMEM((49, NQ, 32, 128), U32),
            pltpu.VMEM((49, NQ, 16, 128), U32),
            pltpu.VMEM((49, 2, M // 8, 128), U32),
            pltpu.VMEM((49, 2, M // 8, 128), U32),
            pltpu.VMEM((49, 2, NP * QQ, 128), U32),
            pltpu.VMEM((49, HQ, 128), U32),
            pltpu.VMEM((49, TQ, 128), U32),
            pltpu.VMEM((4, 8, 128), F32),
            pltpu.VMEM((4, DC // SCR * 8 + 16, 128), jnp.int32),
            pltpu.VMEM((2, 4, 2, HQ, 128), U32),
            pltpu.VMEM((16, S + PAD, 128), F32),
            pltpu.VMEM((8, TQ + PAD, 128), F32),
            pltpu.VMEM((WIN, TQ, 128), F32),
            pltpu.VMEM((WIN, TQ, 128), F32),
            pltpu.VMEM((8, TQ, 128), F32),
            pltpu.VMEM((49, 2, 16, 128), U32),
            pltpu.VMEM((HA, S // 2, 128), U32),
            pltpu.VMEM((7, QQ, M), U32),
            pltpu.VMEM((7, QQ, M), U32),
            pltpu.VMEM((TO, 128), F32),
            pltpu.VMEM((S, M), BF16),
            pltpu.VMEM((8, 128), BF16),
            pltpu.SemaphoreType.DMA((2,)),
            pltpu.SemaphoreType.DMA((2,)),
            pltpu.SemaphoreType.DMA((5,)),
        ],
        compiler_params=pltpu.CompilerParams(vmem_limit_bytes=120 * 1024 * 1024,
                                             disable_bounds_checks=True),
    )(
        A_x.reshape(S, M),
        A_c_kv.reshape(S, DC),
        A_w_q,
        A_w_uk,
        A_w_uv,
        A_w_o.reshape(HA * DA, M),
        B_wqkv.reshape(2, M // 2, 3 * M),
        B_wo.reshape(HB // 2, 2, DB, M),
        gate_w.reshape(8, 128),
    )
    return out.reshape(1, S, M)
```

```python
import functools

import jax
import jax.numpy as jnp
import jax.experimental.pallas as pl
import jax.experimental.pallas.tpu as pltpu

F32 = jnp.float32
BF16 = jnp.bfloat16
U32 = jnp.uint32

S = 2048
M = 1024
HA = 32
DA = 128
DC = 512
HB = 32
DB = 32
WIN = 8
DIL = 2
PAD = 16
LOG2E = 1.4426950408889634
NEG = -1e9

TQ = 128
HQ = TQ // 2
QQ = TQ // 4
NQ = S // TQ
NP = HA // 2
RB = 16
TO = 256

P0S = ((0, 0, 2048), (1, 0, 1024), (1, 1024, 768), (1, 1792, 128), (1, 1920, 128))
P0W = 1
P0A = 75
P0T = 16
P0N = 104
P1S = ((0, 0, 2048), (1, 0, 1536), (1, 1536, 384), (1, 1920, 128))
P1A = 60
P1N = 108
XN = 28
XQ = 50
BOP = (2, 3, 2)
KVS = 28
QS = 28
LX = 16
QST = 2
SK = 3
LG = 2
SMR = 16
SML = 1
SCR = 32
LN = 80
LA = 24
BS = 2
LP = ("kv", 1, 8)
BX = 8
BE = 42
DEP = 2
FA = 6
F0 = 0
FD = 8
TIE = 4
LDEP = 4
P3S = 3
P3E = 12
P3M = 6
P3D = 8

NN = (((1,), (0,)), ((), ()))
NT = (((1,), (1,)), ((), ()))


def _plan2():
    plan = {}

    def put(name, count, start, until):
        plan.setdefault(start, []).extend([(name, until)] * count)

    def after_qk(i):
        if i >= NQ - 2:
            return ("bo", 0, 7 * (i - NQ + 2) * BOP[0] + BX)
        return ("kv", i // 2 + 1, KVS * (i & 1) + LX)

    def fill(name, count, sites):
        for start, room, until in sites:
            n = min(count, room - len(plan.get(start, ())))
            put(name, n, start, until)
            count -= n
        assert count == 0, (name, count)

    def qk_sites(lo, hi):
        return [(("qk", h, i), max(i + 1 - h * SK, 0), after_qk(i))
                for i in range(lo, hi) for h in range(2)]

    def q_sites(g, lo, hi, until):
        return [(("q", g, k), 1, until) for k in range(lo, hi, QST)]

    ticks = ([("bv", 0, k) for k in range(LA, 49)] + [("kv", 0, k) for k in range(0, 49, 2)]
             + [("q", 0, k) for k in range(49)])
    for name, site in zip(_spread(["lo"] * (64 // LG + 128 // SMR), LN), ticks):
        put(name, 1, site, LP)
    host = [(("bv", 0, k), 1, ("kv", 0, 8)) for k in range(0, LA, BS)]
    early = []
    for g in range(1, 4):
        early += q_sites(g, 0, QS - 4, after_qk(2 * g - 1))
        early += qk_sites(2 * g - 1, 2 * g)
        early += q_sites(g, QS, 45, after_qk(2 * g))
        early += qk_sites(2 * g, 2 * g + 1)
    fill("lv", 32, early)
    fill("wo", 56, host + early)
    fill("os", 28, early + qk_sites(7, 14))
    fill("qw", 112, qk_sites(7, 14))
    fill("kv", 56, qk_sites(14, 16) + [(("bo", 0, k), 1, ("bo", 0, BE))
                                       for k in range(7 * BOP[0], 35)])
    return plan


def _planx():
    names = _spread(["qw"] * XQ + ["kv", "qw"] * 56 + ["qw"] * (56 - XQ), 8 * XN)
    return {k: [(n, 31) for n in names[8 * k:8 * k + 8]] for k in range(XN)}


def _spread(names, ticks):
    out = [None] * ticks
    for k, name in enumerate(names):
        out[k * ticks // len(names)] = name
    return out


def _plan1(segs, lo, step, count):
    end = len(segs) - 2
    ticks = [k for k in range(lo, end) for _ in range(segs[k][2] // step)][:count]
    n = len(ticks) * (P0A if lo else P1A) // 100
    names = _spread(["x"] * 28 + ["c"] * 14 + ["o"] * 14, n) + _spread(["v"] * 14, len(ticks) - n)
    plan = {}
    for k, name in zip(ticks, names):
        plan.setdefault(k, []).append((name, end))
    return plan


def _plan3():
    plan = {}
    for k in range(6):
        lo = P3S if k == 0 else 0
        extra = ["g"] * 8 if k in (1, 2) else []
        names = _spread(["a"] * 32 + extra, 4 * (P3E - lo))
        for d in range(lo, P3E):
            plan[(k, d)] = [(n, (k + 1, 0)) for n in names[4 * (d - lo):4 * (d - lo) + 4]]
    names = _spread(["m"] * 24, 4 * P3M)
    for d in range(P3M):
        plan[(6, d)] = [(n, (6, P3D)) for n in names[4 * d:4 * d + 4]]
    return plan


_STAGES = ((2, 4), (1, 3), (0, 2), (0, 6), (0, 1))


def _permute8(cols):
    cols = list(cols)
    lane = jax.lax.broadcasted_iota(jnp.int32, cols[0].shape, 1)
    for va, lb in _STAGES:
        lo = (lane & (1 << lb)) == 0
        sh = 1 << lb
        idx = [i for i in range(8) if not (i >> va) & 1]
        if lb == 6:
            rr = [pltpu.roll(jnp.where(lo, cols[i | (1 << va)], cols[i]), 64, 1) for i in idx]
            for i, r in zip(idx, rr):
                a, b = cols[i], cols[i | (1 << va)]
                cols[i] = jnp.where(lo, a, r)
                cols[i | (1 << va)] = jnp.where(lo, r, b)
        else:
            rb = [pltpu.roll(cols[i | (1 << va)], sh, 1) for i in idx]
            ra = [pltpu.roll(cols[i], 128 - sh, 1) for i in idx]
            for i, xa, xb in zip(idx, ra, rb):
                a, b = cols[i], cols[i | (1 << va)]
                cols[i] = jnp.where(lo, a, xb)
                cols[i | (1 << va)] = jnp.where(lo, xa, b)
    return cols


def _pack(x):
    return pltpu.bitcast(x.astype(BF16), U32)


def _bf(x):
    return pltpu.bitcast(x, BF16)


def _split(w):
    return (pltpu.bitcast(w << 16, F32), pltpu.bitcast(w & jnp.uint32(0xFFFF0000), F32))


def _join(lo, hi):
    return pltpu.bitcast(pltpu.pack_elementwise([lo, hi], packed_dtype=BF16), U32)


def _riffle(x):
    return jnp.concatenate([_join(x[r:r + 16], x[r + 16:r + 32]) for r in range(0, x.shape[0], 32)],
                           axis=0)


def _lhs7(a11, a12, a21, a22):
    return [a11 + a22, a21 + a22, a11, a22, a11 + a12, a21 - a11, a12 - a22]


def _rhs7(b11, b12, b21, b22):
    return [b11 + b22, b11, b12 - b22, b21 - b11, b22, b11 + b12, b21 + b22]


def _combine(mm):
    add = functools.partial(jax.tree.map, jnp.add)
    sub = functools.partial(jax.tree.map, jnp.subtract)
    m2 = mm(2)
    m3 = mm(3)
    m4 = mm(4)
    c12 = add(m2, m4)
    t11 = sub(m3, m4)
    m1 = mm(1)
    c21 = add(m1, m3)
    t22 = sub(m2, m1)
    m0 = mm(0)
    t11 = add(t11, m0)
    t22 = add(t22, m0)
    c11 = add(t11, mm(6))
    return c11, c12, c21, add(t22, mm(5))


ORDER = (2, 3, 4, 1, 0, 6, 5)


def _zero(i, m):
    return i >> (8 + m)


def _merge(vals):
    return _fold([v[r:r + 8, c:c + 128] for v in vals for r in range(0, v.shape[0], 8)
                  for c in range(0, v.shape[1], 128)], jnp.bitwise_or)


def _gate(never, g):
    def gate(x):
        t = jnp.tile(pltpu.bitcast(g, x.dtype), (x.shape[0] // 8, x.shape[1] // 128))
        return jnp.where(never, t, x)
    return gate


def _tie(never, x, deps):
    if not deps:
        return x
    top = jnp.where(never, _merge(deps), x[:8, :128])
    if x.shape[1] > 128:
        top = jnp.concatenate([top, x[:8, 128:]], axis=1)
    return jnp.concatenate([top, x[8:]], axis=0)


class _Sched:
    def __init__(self, never, plan, jobs):
        self.never, self.plan, self.jobs, self.pending = never, plan, jobs, {}

    def mm(self, site, a, b, dims=NN, width=128, step=32):
        deps = [d() if callable(d) else d for d in self.pending.pop(site, ())]
        a = a() if callable(a) else a
        tie = functools.partial(_tie, self.never, deps=deps)
        a, b = (_bf(tie(a)), _bf(b)) if a.dtype == U32 else (a, _bf(tie(b)))
        out = jax.lax.dot_general(a, b, dims, preferred_element_type=F32)
        per = out.shape[0] // step
        last = {}
        for k, (name, until) in enumerate(self.plan.get(site, ())):
            if name is not None:
                r, c = step * (k % per), width * (k // per)
                vals, tag, stored = self.jobs[name].pop(0)(
                    _gate(self.never, out[r:r + 8, c:c + 128]))
                self.pending.setdefault(until, []).extend(vals)
                last[(name, tag, until)] = stored
        for (_, _, until), stored in last.items():
            if stored is not None:
                self.pending[until].append(stored)
        return out

    def finish(self):
        assert not any(self.jobs.values()) and not any(self.pending.values())


def _ops49(fn, blocks, m):
    return fn(*[fn(*[blocks[q][e] for q in range(4)])[m] for e in range(4)])


def _words49(fn, words, m):
    halves = [[_split(w) for w in q] for q in words]
    lo = _ops49(fn, [[h[0] for h in q] for q in halves], m)
    hi = _ops49(fn, [[h[1] for h in q] for q in halves], m)
    return [_join(a, b) for a, b in zip(lo, hi)]


def _fold(xs, op):
    acc = xs[0]
    for x in xs[1:]:
        acc = op(acc, x)
    return acc


def _tree(xs, op):
    while len(xs) > 1:
        xs = [op(a, b) for a, b in zip(xs[::2], xs[1::2])]
    return xs[0]


def _lane_chunks(x):
    return [x[:, j * 128:(j + 1) * 128] for j in range(x.shape[1] // 128)]


def _kernel(x_hbm, c_hbm, wq_hbm, wuk_hbm, wuv_hbm, wo_hbm, wqkv_hbm, wob_hbm, gw_hbm,
            out_hbm,
            xs_u, x_r, c_r, w_r, wv_r, wob_r, wkv_r, wq_r, wo_r,
            wperm, xq, cq, wv49, wob49, wo49, wkv, wq49, ups, sc_s, qn,
            qk_b, vb, lg_s, pr_s, o_s, ob49, ctx, ca0, ca1, g_s, out_s, gw_ref,
            sem_x, sem_p, sem_a):
    x_u = x_hbm.bitcast(U32)
    c_u = c_hbm.bitcast(U32)
    wo_u = wo_hbm.bitcast(U32)
    wq_u = wq_hbm.bitcast(U32)
    wuk_u = wuk_hbm.bitcast(U32)
    wuv_u = wuv_hbm.bitcast(U32)
    wob_u = wob_hbm.bitcast(U32)
    part = functools.partial

    def blk(j, n):
        return pl.ds(pl.multiple_of(j * n, n), n)

    def strip(j):
        return blk(j, 128)

    def cp_x(t, sem):
        k = (t + 1) >> 1
        return pltpu.make_async_copy(x_u.at[blk(t & 1, S // 4), strip(jnp.minimum(k, 7))],
                                     xs_u.at[jnp.minimum(k, 8), blk(t & 1, S // 4), :], sem)

    def cp_w(t, sem):
        u = t - 2 * (t >> 4)
        u = u - 2 * (u >> 4)
        return pltpu.make_async_copy(wqkv_hbm.at[u >> 3, strip((u >> 1) & 3), blk(u & 1, M)],
                                     w_r.at[u & 1], sem)

    def cp_wob(t, sem):
        b = (t + 1) >> 1
        c = jnp.minimum(b, 7)
        return tuple(pltpu.make_async_copy(
            wob_u.at[:, c & 1, 4 * (2 * (t & 1) + j) + (c & 2) + (c >> 2), :],
            wob_r.at[b & 1, 2 * (t & 1) + j], sem) for j in range(2))

    def group(t, sem1=None):
        sem = sem_x.at[t & 1]
        u = t - 2 * (t >> 4)
        return (
            cp_x(t, sem if sem1 is None else sem1),
            cp_w(t + 1, sem),
            pltpu.make_async_copy(x_u.at[blk(u, HQ), :], x_r.at[u & 1], sem),
            pltpu.make_async_copy(c_u.at[blk(u, HQ), :], c_r.at[u & 1], sem),
        ) + cp_wob(t, sem) + tuple(
            pltpu.make_async_copy(wqkv_hbm.at[e >> 1, blk(16 * (e & 1) + u, 16), pl.ds(2 * M, M)],
                                  wv_r.at[u & 1, e], sem) for e in range(4))

    def piece(t):
        late = t >> 4
        pq = (t >> 3) + late
        pk = (t >> 3) & 1
        u = (t & 15) + 2 * late
        sem = sem_a.at[3 + late]
        return (
            pltpu.make_async_copy(wo_u.at[blk(u, 16), pl.ds(0, M // 2)],
                                  wo_r.at[late, blk(u, 16), :], sem),
            pltpu.make_async_copy(wq_u.at[strip(t & 7), pq, :], wq_r.at[pq, strip(t & 7), :], sem),
            pltpu.make_async_copy(wq_u.at[blk(u, 64), 2, :], wq_r.at[2 + late, blk(u, 64), :], sem),
            pltpu.make_async_copy(wuk_u.at[blk(t & 7, 64), pk, :],
                                  wkv_r.at[1 - pk + late, blk(8 + (t & 7), 64), :], sem),
            pltpu.make_async_copy(wuv_u.at[blk(t & 7, 64), pk, :],
                                  wkv_r.at[1 - pk + late, blk(t & 7, 64), :], sem),
        )

    def cp_wq(p, sem):
        return pltpu.make_async_copy(wq_u.at[:, jnp.minimum(p, NP - 1), :], wq_r.at[p & 3], sem)

    def cp_p(g):
        slot = g & 1
        p = jnp.minimum(g + 1, NP - 1)
        o = jnp.minimum(g, NP - 1)
        sem = sem_p.at[slot]
        return (
            pltpu.make_async_copy(wo_u.at[blk(o >> 1, 2 * DA), blk(o & 1, M // 2)],
                                  wo_r.at[slot], sem),
            pltpu.make_async_copy(wuk_u.at[:, p, :], wkv_r.at[slot, pl.ds(DC, DC), :], sem),
            pltpu.make_async_copy(wuv_u.at[:, p, :], wkv_r.at[slot, pl.ds(0, DC), :], sem),
            cp_wq(g + 2, sem),
        )

    def cp_gw():
        return pltpu.make_async_copy(gw_hbm, gw_ref, sem_a.at[0])

    def cp_out(i, late):
        def cp(rows, cols):
            return pltpu.make_async_copy(out_s.at[rows, cols], out_hbm.at[rows, cols], sem_a.at[1])

        low = [cp(blk(2 * i + 1, TO // 2), pl.ds(512 * cc + 256 * late, 256)) for cc in range(2)]
        return low if late else [cp(blk(2 * i, TO // 2), pl.ds(0, M))] + low

    cp_w(0, sem_a.at[1]).start()
    group0, group1 = group(0, sem_a.at[2]), group(1)
    group0 = (group0[0], cp_x(-1, sem_a.at[2])) + group0[1:] + cp_wob(-1, sem_x.at[0])
    for d in group0 + group1[:1] + group1[2:]:
        d.start()

    for cc in range(8):
        qk_b[8 + cc, pl.ds(0, PAD), :] = jnp.zeros((PAD, 128), F32)
        vb[cc, pl.ds(TQ, PAD), :] = jnp.zeros((PAD, 128), F32)

    def stage_first(t):
        for cc, w in enumerate(_permute8(_lane_chunks(pltpu.bitcast(w_r[t & 1], U32)))):
            wperm[cc] = w

    def p1_step(t, peel):
        if not peel:
            for d in group(t):
                d.wait()

        def act_sums(src, dst, ns, m, sr, r, gate):
            cw = [[gate(src[(t & 1) + _zero(t, m), pl.ds(32 * (q >> 1) + 16 * (e >> 1) + 8 * r, 8),
                            pl.ds(((2 * (q & 1) + (e & 1)) * ns + sr) * 128, 128)])
                   for e in range(4)] for q in range(4)]
            for n, w in enumerate(_words49(_lhs7, cw, m)):
                dst[7 * m + n, t, pl.ds(16 * sr + 8 * r, 8), :] = w
            return [], 0, lambda: dst[7 * m + _zero(t, 0), t, pl.ds(16 * sr + 8 * r, 8), :]

        wv = []

        def load_wv():
            wv.extend(_permute8(_lane_chunks(jnp.concatenate(
                [pltpu.bitcast(wv_r[t & 1, e], U32) for e in range(4)], axis=0))))

        def w_sums(src, dst, m, cc, gate):
            ww = [[gate(src(m, 2 * (q >> 1) + (e >> 1), 2 * (2 * (q & 1) + (e & 1)) + cc))
                   for e in range(4)] for q in range(4)]
            for n, w in enumerate(_words49(_rhs7, ww, m)):
                dst[7 * m + n, cc, blk(t, 8), :] = w
            return [], 0, lambda: dst[7 * m + _zero(t, 0), cc, blk(t, 8), :]

        def v_src(m, rq, ch):
            return wv[ch][8 * rq:8 * rq + 8]

        def o_src(m, rq, ch):
            return wob_r[((t >> 1) & 1) + _zero(t, m), rq, blk(t & 1, 8), pl.ds(128 * ch, 128)]

        segs, step = (P0S, P0T) if peel else (P1S, 32)
        sched = _Sched(t > 99, _plan1(segs, P0W * peel, step, P0N if peel else P1N), dict(
            x=[part(act_sums, x_r, xq, 2, m, sr, r)
               for m in range(7) for sr in range(2) for r in range(2)],
            c=[part(act_sums, c_r, cq, 1, m, 0, r) for m in range(7) for r in range(2)],
            v=[part(w_sums, v_src, wv49, m, cc) for m in range(7) for cc in range(2)],
            o=[part(w_sums, o_src, wob49, m, cc) for m in range(7) for cc in range(2)]))

        first = t < 2
        for k, (half, r0, n) in enumerate(segs):
            if k == P0W * peel:
                if peel:
                    for d in group0[2:]:
                        d.wait()
                load_wv()
            w = jnp.concatenate([wperm[4 * half + cc] for cc in range(4)], axis=1)
            r = sched.mm(k, xs_u[t >> 1, pl.ds(r0 // 2, n // 2), :], w, step=step)
            if k == len(segs) - 1:
                sched.finish()
                stage_first(t + 1)
                d = group(t + 2)
                e = piece(t + 1)
                d = d[2:6] + e[:1] + d[6:] + d[:2] + e[1:]
                for d in d + (piece(0) + (cp_gw(),) if peel else ()):
                    d.start()
            for cc in range(4):
                sl = (8 * (t & 1) + 4 * half + cc, pl.ds(PAD + r0, n), slice(None))
                new = r[:, cc * 128:(cc + 1) * 128]
                qk_b[sl] = new if peel else jnp.where(first, 0.0, qk_b[sl]) + new
        return t

    zero = jnp.max(vb[0, pl.ds(TQ, 8), :]).astype(jnp.int32)
    cp_w(0, sem_a.at[1]).wait()
    stage_first(0)
    group1[1].start()
    for d in group0[:2]:
        d.wait()
    p1_step(zero, True)
    last = jax.lax.fori_loop(1, 16, lambda t, c: p1_step(t, False), 0)

    row = jax.lax.broadcasted_iota(jnp.int32, (TQ, TQ), 0)
    col = jax.lax.broadcasted_iota(jnp.int32, (TQ, TQ), 1)
    col = (col & ~31) | ((col & 1) << 4) | ((col & 31) >> 1)
    rowi = jax.lax.broadcasted_iota(jnp.int32, (RB, 128), 0)
    odd = (jax.lax.broadcasted_iota(jnp.int32, (RB, 128), 1) & 1) == 1
    QSCALE = DA ** -0.5 * LOG2E

    def pair_rows(src, slot, r0, n, gate):
        return [_split(gate(src[slot, pl.ds(r0 + par, n // 2, stride=2), :])) for par in range(2)]

    def staging(g, z, never):
        ns = DC // SCR

        def scales(n1, k, gate):
            res = []
            for h in range(2):
                if k < ns:
                    w = gate(wkv_r[g & 1, pl.ds(n1 * DC + k * SCR, SCR), :])
                    w = pltpu.bitcast(w, jnp.int32) & (0x7F80 << (16 * h))
                else:
                    w = gate(sc_s[2 * n1 + h, pl.ds(0, 8 * ns), :])
                e = _tree([w[r:r + 8] for r in range(0, w.shape[0], 8)], jnp.maximum)
                if k == ns:
                    e = pltpu.bitcast(e << (16 - 16 * h), F32)
                    e = jnp.max(e, axis=0, keepdims=True)
                    e = jnp.clip(pltpu.bitcast(e, jnp.int32), 1 << 23, 253 << 23)
                    e = jnp.broadcast_to(e, (8, 128))
                    sc_s[2 * n1 + h, pl.ds(8 * ns + 8, 8), :] = (254 << 23) - e
                sc_s[2 * n1 + h, pl.ds(8 * k, 8), :] = e
                res.append(pltpu.bitcast(e, U32))
            return res, 0, lambda: pltpu.bitcast(sc_s[2 * n1, blk(k + _zero(z, 0), 8), :], U32)

        def rhs49(dst, tiles, scale, m, r, extra=()):
            res = [_ops49(_rhs7,
                          [[scale(tiles[2 * (q >> 1) + (e >> 1)][q & 1][par][e & 1],
                                  2 * (q & 1) + (e & 1)) for e in range(4)] for q in range(4)],
                          m) for par in range(2)]
            for k, (lo, hi) in enumerate(zip(*res)):
                w = _join(lo, hi)
                if k < len(extra):
                    w = jnp.where(never, extra[k], w)
                dst[7 * m + k, pl.ds(8 * r, 8), :] = w

        def kv(m, r, gate):
            if m == 0 and r == 0:
                for k in range(4):
                    ups[k] = pltpu.bitcast(gate(sc_s[k, pl.ds(8 * ns, 8), :]), F32)
            down = [pltpu.bitcast(sc_s[k + _zero(z, m), pl.ds(8 * ns + 8, 8), :], F32)
                    for k in range(4)]
            tiles = [[pair_rows(wkv_r, (g & 1) + _zero(z, m), n1 * DC + kt * 128 + 16 * r, 16, gate)
                      for n1 in range(2)] for kt in range(4)]
            rhs49(wkv, tiles, lambda w, k: w * down[k], m, r)
            return [], 0, lambda: wkv[7 * m, blk(r + _zero(z, 0), 8), :]

        def qw(m, r, gate):
            tiles = [[pair_rows(wq_r, ((g + 1 + n1) & 3) + _zero(z, m), kt * 256 + 16 * r, 16, gate)
                      for n1 in range(2)] for kt in range(4)]
            rhs49(wq49, tiles, lambda w, k: w, m, r, sc.pop(0)(gate)[0] if sc else ())
            return [], 0, lambda: wq49[7 * m, blk(r + _zero(z, 0), 8), :]

        sc = [part(scales, n1, k) for k in range(ns + 1) for n1 in range(2)]
        return dict(sc=sc,
                    kv=[part(kv, m, r) for m in range(7) for r in range(8)],
                    qw=[part(qw, m, r) for m in range(7) for r in range(16)])

    for t in range(16):
        for d in piece(t):
            d.wait()
    sched = _Sched(last > 99, _planx(), staging(-1, last, last > 99))
    w0 = pair_rows(wq_r, 0, 0, M, lambda x: x)
    w0 = [_join(w0[0][h], w0[1][h]) for h in range(2)]
    for g in range(4):
        for e in range(2):
            for h in range(2):
                q = [sched.mm(8 * g + 4 * e + 2 * h + k, jnp.concatenate(
                    [xs_u[4 * k + u, pl.ds((4 * g + 2 + e) * HQ, HQ), :] for u in range(4)], axis=1),
                    w0[h][256 * k:256 * k + 256], step=16) for k in range(2)]
                qn[h, g, e] = _pack((q[0] + q[1]) * QSCALE)
    sched.finish()
    for d in group(16) + group(17) + piece(16):
        d.wait()
    for d in cp_p(1):
        d.start()
    plan2 = _plan2()

    def p2_body(p, carry):
        @pl.when(p > 0)
        def _():
            for d in cp_p(p):
                d.wait()

        causal = col <= row
        never = p > NP
        jobs = staging(p, p, never)
        sched = _Sched(never, plan2, jobs)
        mm = sched.mm

        r0 = pl.multiple_of(p * TQ, TQ)

        prods = {}

        def project(kind, j, n, lhs, rhs):
            got = prods.setdefault((kind, j), {})
            for m in ORDER[len(got):len(got) + n]:
                got[m] = _combine(lambda k: mm((kind, j, 7 * len(got) + ORDER.index(k)),
                                               part(lhs, 7 * m + k), rhs(7 * m + k)))
            if len(got) < 7:
                return None
            c = _combine(lambda m: got[m])
            return [[c[(rg & 2) + (cg >> 1)][2 * (rg & 1) + (cg & 1)] for rg in range(4)]
                    for cg in range(4)]

        def pair(ref, rows):
            return lambda k: jnp.concatenate([ref[k, sr, rows, :] for sr in range(2)], axis=1)

        def x_rows(b, n):
            return lambda k: jnp.concatenate([jnp.concatenate(
                [xq[k, b + j, pl.ds(16 * sr, 16), :] for sr in range(2)], axis=1)
                for j in range(n)], axis=0)

        def proj_b(kind, n, lhs, w, dst, off):
            c = project(kind, 0, n, lhs, pair(w, slice(None)))
            for cg in range(4 * (c is not None)):
                for rg in range(4):
                    for cc in range(2):
                        dst[2 * cg + cc, pl.ds(off + (PAD + rg * QQ), QQ), :] = (
                            c[cg][rg][:, cc * 128:(cc + 1) * 128])

        def proj_bv():
            for cc in range(8):
                vb[cc, pl.ds(0, PAD), :] = vb[cc, pl.ds(TQ, PAD), :]
            proj_b("bv", 7, x_rows(p, 1), wv49, vb, 0)

        def proj_bo(n):
            proj_b("bo", n, pair(ob49, slice(None)), wob49, qk_b, r0)

        def local_qk(rb, k, gate):
            rz = pl.multiple_of((p + _zero(p, k)) * TQ, TQ)
            q = [qk_b[cc, pl.ds(rz + (PAD + rb * RB), RB), :] for cc in range(8)]
            q[0] = gate(q[0])
            for w in range(LG * k, LG * k + LG):
                t = _fold([q[cc] * qk_b[8 + cc, pl.ds(r0 + (PAD + rb * RB - DIL * w), RB), :]
                           for cc in range(8)], jnp.add)
                t = t + pltpu.roll(t, 64, 1)
                t = t + jnp.where(odd, pltpu.roll(t, 1, 1), pltpu.roll(t, 127, 1))
                t = t * (DB ** -0.5 * LOG2E)
                if rb == 0 and w:
                    t = jnp.where(rowi + r0 >= DIL * w, t, NEG)
                lg_s[w, pl.ds(rb * RB, RB), :] = t
            return [], 1, lambda: pltpu.bitcast(lg_s[w, blk(2 * rb + _zero(p, 0), 8), :], U32)

        def local_sm(rb, e, gate):
            rows = pl.ds(rb * RB + SMR * e, SMR)
            lg = [gate(lg_s[w, rows, :]) for w in range(WIN)]
            m = _tree(lg, jnp.maximum)
            ps = [jnp.exp2(t - m) for t in lg]
            l = _tree(ps, jnp.add)
            r = pl.reciprocal(l, approx=True)
            r = r * (2.0 - l * r)
            for w in range(WIN):
                pr_s[w, rows, :] = ps[w] * r
            return [], 2, lambda: pltpu.bitcast(pr_s[0, blk(2 * rb + e + _zero(p, 0), 8), :], U32)

        def local_pv(rb, k, gate):
            rows = pl.ds(rb * RB, RB)
            ps = [pr_s[w + _zero(p, k), rows, :] for w in range(WIN)]
            ps[0] = gate(ps[0])
            o = [_fold([ps[w] * vb[cc, pl.ds(PAD + rb * RB - DIL * w, RB), :] for w in range(WIN)],
                       jnp.add) for cc in (k, k + 4)]
            for e in range(2):
                o_s[k + 4 * e, rows, :] = o[e]
            return [], 0, lambda: pltpu.bitcast(o_s[k, blk(2 * rb + _zero(p, 0), 8), :], U32)

        def o_sums(m, cc, r, gate):
            res = [_ops49(_lhs7, [[gate(o_s[
                2 * (2 * (q & 1) + (e & 1)) + cc + _zero(p, m),
                pl.ds(QQ * (2 * (q >> 1) + (e >> 1)) + 16 * r + par, 8, stride=2), :])
                for e in range(4)] for q in range(4)], m) for par in range(2)]
            for n, (lo, hi) in enumerate(zip(*res)):
                ob49[7 * m + n, cc, pl.ds(8 * r, 8), :] = _join(lo, hi)
            return [], 0, lambda: ob49[7 * m, cc, blk(r + _zero(p, 0), 8), :]

        jobs["os"] = [part(o_sums, m, cc, r) for r in range(2) for cc in range(2) for m in range(7)]
        order = list(range(0, 8, 2)) + list(range(1, 8, 2))
        jobs["lo"] = []
        for k in range(len(order) + SML):
            for f, d, n in ((local_sm, SML, RB // SMR), (local_qk, 0, 8 // LG)):
                if 0 <= k - d < len(order):
                    jobs["lo"] += [part(f, order[k - d], e) for e in range(n)]
        jobs["lv"] = [part(local_pv, rb, e) for rb in order for e in range(4)]

        def out_weights(m, r, gate):
            ww = [[gate(wo_r[(p & 1) + _zero(p, m),
                             pl.ds((2 * (q >> 1) + (e >> 1)) * HQ + 8 * r, 8),
                             pl.ds((2 * (q & 1) + (e & 1)) * 128, 128)])
                   for e in range(4)] for q in range(4)]
            rows = blk(8 * (p >> 1) + r, 8)
            extra = jobs["sc"].pop(0)(gate)[0] if jobs["sc"] else []
            for n, w in enumerate(_words49(_rhs7, ww, m)):
                if n < len(extra):
                    w = jnp.where(never, extra[n], w)
                wo49[7 * m + n, p & 1, rows, :] = w
            return [], 0, lambda: wo49[7 * m + _zero(p, 0), p & 1, rows, :]

        jobs["wo"] = [part(out_weights, m, r) for m in range(7) for r in range(8)]

        ks, vs, qs = {}, {}, {}
        done = {}

        def blocks(c, scale, pack):
            c = [[pack(t * scale(cg)) for t in c[cg]] for cg in range(4)]
            return [[jnp.concatenate([t[16 * e:16 * e + 16] for t in c[cg]], axis=0)
                     for e in range(2)] for cg in range(4)]

        def proj_kv(j, n):
            c = project("kv", j, n, lambda k: jnp.concatenate(
                [cq[k, 2 * j], cq[k, 2 * j + 1]], axis=0), lambda k: wkv[k])
            if c is not None:
                c = blocks(c, lambda cg: ups[cg][:1], _riffle)
                for cg in range(4):
                    for e in range(2):
                        (vs, ks)[cg >> 1][(cg & 1, 2 * j + e)] = c[cg][e]

        def proj_q(g, n):
            c = project("q", g, n, x_rows(4 * g + 2 * (p & 1), 2), lambda k: wq49[k])
            if c is not None:
                c = blocks(c, lambda cg: QSCALE, _pack)
                for h in range(2):
                    for e in range(2):
                        old = qn[h, g, e]
                        for b in range(2):
                            qs[(h, 4 * g + 2 * b + e)] = jnp.where((p & 1) == b, c[h][e], old)
                        qn[h, g, e] = c[2 + h][e]

        def qk(h, i, dep):
            kk = jnp.concatenate([ks[(h, j)] for j in range(i + 1)], axis=0)
            q = qs[(h, i)]
            if dep is not None:
                q = jnp.where(never, done[(h, dep)], q)
            ch = _lane_chunks(mm(("qk", h, i), q, kk, NT, 512))
            ch[i] = jnp.where(causal, ch[i], NEG)
            return ch

        def softmax_pv(h, i, ch):
            m = jnp.max(_fold(ch, jnp.maximum), axis=1, keepdims=True)
            ps = [jnp.exp2(c - m) for c in ch]
            lp = ps[0]
            for j in range(1, i + 1):
                lp = lp + ps[j]
                if TIE and (j % TIE == TIE - 1 or j == i):
                    ps[j] = jnp.where(never, lp, ps[j])
            pb = jnp.concatenate(ps, axis=1).astype(BF16)
            vv = jnp.concatenate([vs[(h, j)] for j in range(i + 1)], axis=0)
            o = mm(("pv", h, i), pb, vv)
            if i >= LDEP:
                lp = jnp.where(never, o, lp)
            l = jnp.sum(lp, axis=1, keepdims=True)
            r = pl.reciprocal(l, approx=True)
            r = r * (2.0 - l * r)
            cn = _pack(o * r)
            done[(h, i)] = cn
            if FA <= i < NQ - 1:
                if i + 3 < NQ:
                    site = ("kv", (i + 1) // 2 + 1, KVS * ((i + 1) & 1) + (F0, FD)[h])
                else:
                    site = ("bo", 0, 7 * (i + 3 - NQ) * BOP[0] + 8 * h)
                sched.pending.setdefault(site, []).append(cn)
            ctx[2 * p + h, pl.ds(i * HQ, HQ), :] = cn

        proj_bv()
        proj_kv(0, 7)
        proj_q(0, 7)
        for i in range(NQ):
            dep = i - DEP if DEP <= i < FA + DEP else None
            s0 = qk(0, i, dep)
            s1 = qk(1, i, dep)
            if i + 2 < NQ:
                proj_kv(i // 2 + 1, 7 if i & 1 else KVS // 7)
                if i < 6:
                    proj_q(i // 2 + 1, 7 if i & 1 else QS // 7)
            else:
                proj_bo(BOP[i + 2 - NQ])
            softmax_pv(0, i, s0)
            softmax_pv(1, i, s1)
        proj_bo(BOP[2])
        sched.finish()
        for d in cp_p(p + 2):
            d.start()
        return carry

    jax.lax.fori_loop(0, NP, p2_body, 0)

    cp_gw().wait()
    gw = gw_ref[...].astype(F32)
    plan3 = _plan3()
    cab = (ca0, ca1)

    def p3_body(i, carry):
        r0 = pl.multiple_of(i * TO, TO)
        h0 = pl.multiple_of(i * (TO // 2), TO // 2)
        never = i > S

        def ctx_words(m, u, r, n):
            return [[ctx[4 * u + 2 * (q & 1) + (e & 1),
                         pl.ds(h0 + _zero(i, m) * 8 + ((2 * (q >> 1) + (e >> 1)) * QQ + r), n), :]
                     for e in range(4)] for q in range(4)]

        def operands(k, u, r, gate):
            m = ORDER[k]
            cw = [[gate(w) for w in q] for q in ctx_words(m, u, r, 8)]
            for n, w in enumerate(_words49(_lhs7, cw, m)):
                if not (m in (2, 3) and n in (2, 3)):
                    cab[k & 1][n, pl.ds(r, 8), pl.ds(u * 128, 128)] = w
            return [], 0, lambda: cab[k & 1][_zero(i, 0), pl.ds(r, 8), pl.ds(u * 128, 128)]

        def gate_rows(r, gate):
            gs = _fold([_bf(gate(xs_u[j, pl.ds(h0 + r, 8), :])).astype(F32) * gw[j:j + 1]
                        for j in range(8)], jnp.add)
            g = jax.nn.sigmoid(jnp.sum(gs, axis=1, keepdims=True))
            g_s[pl.ds(2 * r, 16), :] = jnp.broadcast_to(g, (16, 128))
            return [], 0, lambda: pltpu.bitcast(g_s[blk(r // 4 + _zero(i, 0), 8), :], U32)

        pr = {}

        def mix(q, e, cc, gate):
            off = (2 * (q >> 1) + (e >> 1)) * HQ
            ch = 4 * cc + 2 * (q & 1) + (e & 1)
            a = _combine(lambda m: pr.get(m, pr[2])[e][:, cc * 128:(cc + 1) * 128])[q]
            g = gate(g_s[pl.ds(off, HQ), :])
            b = qk_b[ch, pl.ds(r0 + (PAD + off), HQ), :]
            out_s[pl.ds(r0 + off, HQ), pl.ds(ch * 128, 128)] = (g * a + (1.0 - g) * b).astype(BF16)
            return [], 0, lambda: pltpu.bitcast(
                out_s[blk(i * (TO // 16) + off // 16 + _zero(i, 0), 16), pl.ds(ch * 128, 128)], U32)

        sched = _Sched(never, plan3, dict(
            a=[part(operands, k, u, r) for k in range(1, 7) for u in range(HA // 4)
               for r in range(0, QQ, 8)],
            g=[part(gate_rows, r) for r in range(0, TO // 2, 8)],
            m=[part(mix, q, e, cc) for q in (1, 2, 0) for e in range(4) for cc in range(2)]))
        first = [[_words49(_lhs7, ctx_words(ORDER[0], u, 0, QQ), ORDER[0])[n]
                  for u in range(HA // 4)] for n in range(7)]

        def inner(m, n):
            k = ORDER.index(m)
            res = []
            for e in range(2):
                us = range(4 * e, 4 * e + 4)
                if m in (2, 3) and n in (2, 3):
                    lhs = jnp.concatenate([ctx_words(m, u, 0, QQ)[3 * (m - 2)][3 * (n - 2)]
                                           for u in us], axis=1)
                elif k == 0:
                    lhs = jnp.concatenate([first[n][u] for u in us], axis=1)
                else:
                    lhs = lambda: cab[k & 1][n, :, pl.ds(e * 512, 512)]
                rhs = jnp.concatenate([wo49[7 * m + n, cc, pl.ds(e * 256, 256), :]
                                       for cc in range(2)], axis=1)
                res.append(sched.mm((k, 2 * ORDER.index(n) + e), lhs, rhs))
                if (k, 2 * ORDER.index(n) + e) == (6, P3D):
                    for d in cp_out(i, 0):
                        d.start()
            return res[0] + res[1]

        for m in ORDER:
            pr[m] = _combine(lambda n: inner(m, n))
        sched.finish()
        for e in (1, 2, 0, 3):
            for cc in range(2):
                mix(3, e, cc, lambda x: x)
        for d in cp_out(i, 1):
            d.start()
        return carry

    jax.lax.fori_loop(0, S // TO, p3_body, 0)
    for d in cp_p(NP) + cp_p(NP + 1):
        d.wait()
    for i in range(S // TO):
        for d in cp_out(i, 0) + cp_out(i, 1):
            d.wait()


@jax.jit
def pallas_gated_mix__compressed_kv_cla__sliding_local_dilated__prompt_kernel(
    A_x: jax.Array,
    A_c_kv: jax.Array,
    A_w_q: jax.Array,
    A_w_uk: jax.Array,
    A_w_uv: jax.Array,
    A_w_o: jax.Array,
    B_x: jax.Array,
    B_wqkv: jax.Array,
    B_wo: jax.Array,
    gate_w: jax.Array,
):
    del B_x
    any_spec = pl.BlockSpec(memory_space=pl.ANY)
    out = pl.pallas_call(
        _kernel,
        in_specs=[any_spec] * 9,
        out_specs=any_spec,
        out_shape=jax.ShapeDtypeStruct((S, M), BF16),
        scratch_shapes=[
            pltpu.VMEM((9, S // 2, 128), U32),
            pltpu.VMEM((2, HQ, M), U32),
            pltpu.VMEM((2, HQ, DC), U32),
            pltpu.VMEM((2, 128, M), BF16),
            pltpu.VMEM((2, 4, 16, M), BF16),
            pltpu.VMEM((2, 4, 16, M), U32),
            pltpu.VMEM((3, 2 * DC, 128), U32),
            pltpu.VMEM((4, M, 128), U32),
            pltpu.VMEM((2, 2 * DA, M // 2), U32),
            pltpu.VMEM((8, 64, 128), U32),
            pltpu.VMEM((49, NQ, 32, 128), U32),
            pltpu.VMEM((49, NQ, 16, 128), U32),
            pltpu.VMEM((49, 2, M // 8, 128), U32),
            pltpu.VMEM((49, 2, M // 8, 128), U32),
            pltpu.VMEM((49, 2, NP * QQ, 128), U32),
            pltpu.VMEM((49, HQ, 128), U32),
            pltpu.VMEM((49, TQ, 128), U32),
            pltpu.VMEM((4, 8, 128), F32),
            pltpu.VMEM((4, DC // SCR * 8 + 16, 128), jnp.int32),
            pltpu.VMEM((2, 4, 2, HQ, 128), U32),
            pltpu.VMEM((16, S + PAD, 128), F32),
            pltpu.VMEM((8, TQ + PAD, 128), F32),
            pltpu.VMEM((WIN, TQ, 128), F32),
            pltpu.VMEM((WIN, TQ, 128), F32),
            pltpu.VMEM((8, TQ, 128), F32),
            pltpu.VMEM((49, 2, 16, 128), U32),
            pltpu.VMEM((HA, S // 2, 128), U32),
            pltpu.VMEM((7, QQ, M), U32),
            pltpu.VMEM((7, QQ, M), U32),
            pltpu.VMEM((TO, 128), F32),
            pltpu.VMEM((S, M), BF16),
            pltpu.VMEM((8, 128), BF16),
            pltpu.SemaphoreType.DMA((2,)),
            pltpu.SemaphoreType.DMA((2,)),
            pltpu.SemaphoreType.DMA((5,)),
        ],
        compiler_params=pltpu.CompilerParams(vmem_limit_bytes=120 * 1024 * 1024,
                                             disable_bounds_checks=True),
    )(
        A_x.reshape(S, M),
        A_c_kv.reshape(S, DC),
        A_w_q,
        A_w_uk,
        A_w_uv,
        A_w_o.reshape(HA * DA, M),
        B_wqkv.reshape(2, M // 2, 3 * M),
        B_wo.reshape(HB // 2, 2, DB, M),
        gate_w.reshape(8, 128),
    )
    return out.reshape(1, S, M)
```

```python
import functools

import jax
import jax.numpy as jnp
import jax.experimental.pallas as pl
import jax.experimental.pallas.tpu as pltpu

F32 = jnp.float32
BF16 = jnp.bfloat16
U32 = jnp.uint32

S = 2048
M = 1024
HA = 32
DA = 128
DC = 512
HB = 32
DB = 32
WIN = 8
DIL = 2
PAD = 16
LOG2E = 1.4426950408889634
NEG = -1e9

TQ = 128
HQ = TQ // 2
QQ = TQ // 4
NQ = S // TQ
NP = HA // 2
RB = 16
TO = 256

P0S = ((0, 0, 2048), (1, 0, 1024), (1, 1024, 768), (1, 1792, 128), (1, 1920, 128))
P0W = 1
P0A = 75
P0T = 16
P0N = 104
P1S = ((0, 0, 2048), (1, 0, 1536), (1, 1536, 384), (1, 1920, 128))
P1A = 60
P1N = 108
XN = 28
XQ = 50
BOP = (2, 3, 2)
KVS = 28
QS = 28
LX = 16
QST = 2
SK = 3
LG = 2
SMR = 16
SML = 1
SCR = 32
LN = 80
LA = 24
BS = 2
LP = ("kv", 1, 8)
BX = 8
BE = 42
DEP = 2
FA = 6
F0 = 0
FD = 8
TIE = 4
LDEP = 4
P3S = 3
P3E = 12
P3M = 6
P3D = 8

NN = (((1,), (0,)), ((), ()))
NT = (((1,), (1,)), ((), ()))


def _plan2():
    plan = {}

    def put(name, count, start, until):
        plan.setdefault(start, []).extend([(name, until)] * count)

    def after_qk(i):
        if i >= NQ - 2:
            return ("bo", 0, 7 * (i - NQ + 2) * BOP[0] + BX)
        return ("kv", i // 2 + 1, KVS * (i & 1) + LX)

    def fill(name, count, sites):
        for start, room, until in sites:
            n = min(count, room - len(plan.get(start, ())))
            put(name, n, start, until)
            count -= n
        assert count == 0, (name, count)

    def qk_sites(lo, hi):
        return [(("qk", h, i), max(i + 1 - h * SK, 0), after_qk(i))
                for i in range(lo, hi) for h in range(2)]

    def q_sites(g, lo, hi, until):
        return [(("q", g, k), 1, until) for k in range(lo, hi, QST)]

    ticks = ([("bv", 0, k) for k in range(LA, 49)] + [("kv", 0, k) for k in range(0, 49, 2)]
             + [("q", 0, k) for k in range(49)])
    for name, site in zip(_spread(["lo"] * (64 // LG + 128 // SMR), LN), ticks):
        put(name, 1, site, LP)
    host = [(("bv", 0, k), 1, ("kv", 0, 8)) for k in range(0, LA, BS)]
    early = []
    for g in range(1, 4):
        early += q_sites(g, 0, QS - 4, after_qk(2 * g - 1))
        early += qk_sites(2 * g - 1, 2 * g)
        early += q_sites(g, QS, 45, after_qk(2 * g))
        early += qk_sites(2 * g, 2 * g + 1)
    fill("lv", 32, early)
    fill("wo", 56, host + early)
    fill("os", 28, early + qk_sites(7, 14))
    fill("qw", 112, qk_sites(7, 14))
    fill("kv", 56, qk_sites(14, 16) + [(("bo", 0, k), 1, ("bo", 0, BE))
                                       for k in range(7 * BOP[0], 35)])
    return plan


def _planx():
    names = _spread(["qw"] * XQ + ["kv", "qw"] * 56 + ["qw"] * (56 - XQ), 8 * XN)
    return {k: [(n, 31) for n in names[8 * k:8 * k + 8]] for k in range(XN)}


def _spread(names, ticks):
    out = [None] * ticks
    for k, name in enumerate(names):
        out[k * ticks // len(names)] = name
    return out


def _plan1(segs, lo, step, count):
    end = len(segs) - 2
    ticks = [k for k in range(lo, end) for _ in range(segs[k][2] // step)][:count]
    n = len(ticks) * (P0A if lo else P1A) // 100
    names = _spread(["x"] * 28 + ["c"] * 14 + ["o"] * 14, n) + _spread(["v"] * 14, len(ticks) - n)
    plan = {}
    for k, name in zip(ticks, names):
        plan.setdefault(k, []).append((name, end))
    return plan


def _plan3():
    plan = {}
    for k in range(6):
        lo = P3S if k == 0 else 0
        extra = ["g"] * 8 if k in (1, 2) else []
        names = _spread(["a"] * 32 + extra, 4 * (P3E - lo))
        for d in range(lo, P3E):
            plan[(k, d)] = [(n, (k + 1, 0)) for n in names[4 * (d - lo):4 * (d - lo) + 4]]
    names = _spread(["m"] * 24, 4 * P3M)
    for d in range(P3M):
        plan[(6, d)] = [(n, (6, P3D)) for n in names[4 * d:4 * d + 4]]
    return plan


_STAGES = ((2, 4), (1, 3), (0, 2), (0, 6), (0, 1))


def _permute8(cols):
    cols = list(cols)
    lane = jax.lax.broadcasted_iota(jnp.int32, cols[0].shape, 1)
    for va, lb in _STAGES:
        lo = (lane & (1 << lb)) == 0
        sh = 1 << lb
        idx = [i for i in range(8) if not (i >> va) & 1]
        if lb == 6:
            rr = [pltpu.roll(jnp.where(lo, cols[i | (1 << va)], cols[i]), 64, 1) for i in idx]
            for i, r in zip(idx, rr):
                a, b = cols[i], cols[i | (1 << va)]
                cols[i] = jnp.where(lo, a, r)
                cols[i | (1 << va)] = jnp.where(lo, r, b)
        else:
            rb = [pltpu.roll(cols[i | (1 << va)], sh, 1) for i in idx]
            ra = [pltpu.roll(cols[i], 128 - sh, 1) for i in idx]
            for i, xa, xb in zip(idx, ra, rb):
                a, b = cols[i], cols[i | (1 << va)]
                cols[i] = jnp.where(lo, a, xb)
                cols[i | (1 << va)] = jnp.where(lo, xa, b)
    return cols


def _pack(x):
    return pltpu.bitcast(x.astype(BF16), U32)


def _bf(x):
    return pltpu.bitcast(x, BF16)


def _split(w):
    return (pltpu.bitcast(w << 16, F32), pltpu.bitcast(w & jnp.uint32(0xFFFF0000), F32))


def _join(lo, hi):
    return pltpu.bitcast(pltpu.pack_elementwise([lo, hi], packed_dtype=BF16), U32)


def _riffle(x):
    return jnp.concatenate([_join(x[r:r + 16], x[r + 16:r + 32]) for r in range(0, x.shape[0], 32)],
                           axis=0)


def _lhs7(a11, a12, a21, a22):
    return [a11 + a22, a21 + a22, a11, a22, a11 + a12, a21 - a11, a12 - a22]


def _rhs7(b11, b12, b21, b22):
    return [b11 + b22, b11, b12 - b22, b21 - b11, b22, b11 + b12, b21 + b22]


def _combine(mm):
    add = functools.partial(jax.tree.map, jnp.add)
    sub = functools.partial(jax.tree.map, jnp.subtract)
    m2 = mm(2)
    m3 = mm(3)
    m4 = mm(4)
    c12 = add(m2, m4)
    t11 = sub(m3, m4)
    m1 = mm(1)
    c21 = add(m1, m3)
    t22 = sub(m2, m1)
    m0 = mm(0)
    t11 = add(t11, m0)
    t22 = add(t22, m0)
    c11 = add(t11, mm(6))
    return c11, c12, c21, add(t22, mm(5))


ORDER = (2, 3, 4, 1, 0, 6, 5)


def _zero(i, m):
    return i >> (8 + m)


def _merge(vals):
    return _fold([v[r:r + 8, c:c + 128] for v in vals for r in range(0, v.shape[0], 8)
                  for c in range(0, v.shape[1], 128)], jnp.bitwise_or)


def _gate(never, g):
    def gate(x):
        t = jnp.tile(pltpu.bitcast(g, x.dtype), (x.shape[0] // 8, x.shape[1] // 128))
        return jnp.where(never, t, x)
    return gate


def _tie(never, x, deps):
    if not deps:
        return x
    top = jnp.where(never, _merge(deps), x[:8, :128])
    if x.shape[1] > 128:
        top = jnp.concatenate([top, x[:8, 128:]], axis=1)
    return jnp.concatenate([top, x[8:]], axis=0)


class _Sched:
    def __init__(self, never, plan, jobs):
        self.never, self.plan, self.jobs, self.pending = never, plan, jobs, {}

    def mm(self, site, a, b, dims=NN, width=128, step=32):
        deps = [d() if callable(d) else d for d in self.pending.pop(site, ())]
        a = a() if callable(a) else a
        tie = functools.partial(_tie, self.never, deps=deps)
        a, b = (_bf(tie(a)), _bf(b)) if a.dtype == U32 else (a, _bf(tie(b)))
        out = jax.lax.dot_general(a, b, dims, preferred_element_type=F32)
        per = out.shape[0] // step
        last = {}
        for k, (name, until) in enumerate(self.plan.get(site, ())):
            if name is not None:
                r, c = step * (k % per), width * (k // per)
                vals, tag, stored = self.jobs[name].pop(0)(
                    _gate(self.never, out[r:r + 8, c:c + 128]))
                self.pending.setdefault(until, []).extend(vals)
                last[(name, tag, until)] = stored
        for (_, _, until), stored in last.items():
            if stored is not None:
                self.pending[until].append(stored)
        return out

    def finish(self):
        assert not any(self.jobs.values()) and not any(self.pending.values())


def _ops49(fn, blocks, m):
    return fn(*[fn(*[blocks[q][e] for q in range(4)])[m] for e in range(4)])


def _words49(fn, words, m):
    halves = [[_split(w) for w in q] for q in words]
    lo = _ops49(fn, [[h[0] for h in q] for q in halves], m)
    hi = _ops49(fn, [[h[1] for h in q] for q in halves], m)
    return [_join(a, b) for a, b in zip(lo, hi)]


def _fold(xs, op):
    acc = xs[0]
    for x in xs[1:]:
        acc = op(acc, x)
    return acc


def _tree(xs, op):
    while len(xs) > 1:
        xs = [op(a, b) for a, b in zip(xs[::2], xs[1::2])]
    return xs[0]


def _lane_chunks(x):
    return [x[:, j * 128:(j + 1) * 128] for j in range(x.shape[1] // 128)]


def _kernel(x_hbm, c_hbm, wq_hbm, wuk_hbm, wuv_hbm, wo_hbm, wqkv_hbm, wob_hbm, gw_hbm,
            out_hbm,
            xs_u, x_r, c_r, w_r, wv_r, wob_r, wkv_r, wq_r, wo_r,
            wperm, xq, cq, wv49, wob49, wo49, wkv, wq49, ups, sc_s, qn,
            qk_b, vb, lg_s, pr_s, o_s, ob49, ctx, ca0, ca1, g_s, out_s, gw_ref,
            sem_x, sem_p, sem_a):
    x_u = x_hbm.bitcast(U32)
    c_u = c_hbm.bitcast(U32)
    wo_u = wo_hbm.bitcast(U32)
    wq_u = wq_hbm.bitcast(U32)
    wuk_u = wuk_hbm.bitcast(U32)
    wuv_u = wuv_hbm.bitcast(U32)
    wob_u = wob_hbm.bitcast(U32)
    part = functools.partial

    def blk(j, n):
        return pl.ds(pl.multiple_of(j * n, n), n)

    def strip(j):
        return blk(j, 128)

    def cp_x(t, sem):
        k = (t + 1) >> 1
        return pltpu.make_async_copy(x_u.at[blk(t & 1, S // 4), strip(jnp.minimum(k, 7))],
                                     xs_u.at[jnp.minimum(k, 8), blk(t & 1, S // 4), :], sem)

    def cp_w(t, sem):
        u = t - 2 * (t >> 4)
        u = u - 2 * (u >> 4)
        return pltpu.make_async_copy(wqkv_hbm.at[u >> 3, strip((u >> 1) & 3), blk(u & 1, M)],
                                     w_r.at[u & 1], sem)

    def cp_wob(t, sem):
        b = (t + 1) >> 1
        c = jnp.minimum(b, 7)
        return tuple(pltpu.make_async_copy(
            wob_u.at[:, c & 1, 4 * (2 * (t & 1) + j) + (c & 2) + (c >> 2), :],
            wob_r.at[b & 1, 2 * (t & 1) + j], sem) for j in range(2))

    def group(t, sem1=None):
        sem = sem_x.at[t & 1]
        u = t - 2 * (t >> 4)
        return (
            cp_x(t, sem if sem1 is None else sem1),
            cp_w(t + 1, sem),
            pltpu.make_async_copy(x_u.at[blk(u, HQ), :], x_r.at[u & 1], sem),
            pltpu.make_async_copy(c_u.at[blk(u, HQ), :], c_r.at[u & 1], sem),
        ) + cp_wob(t, sem) + tuple(
            pltpu.make_async_copy(wqkv_hbm.at[e >> 1, blk(16 * (e & 1) + u, 16), pl.ds(2 * M, M)],
                                  wv_r.at[u & 1, e], sem) for e in range(4))

    def piece(t):
        late = t >> 4
        pq = (t >> 3) + late
        pk = (t >> 3) & 1
        u = (t & 15) + 2 * late
        sem = sem_a.at[3 + late]
        return (
            pltpu.make_async_copy(wo_u.at[blk(u, 16), pl.ds(0, M // 2)],
                                  wo_r.at[late, blk(u, 16), :], sem),
            pltpu.make_async_copy(wq_u.at[strip(t & 7), pq, :], wq_r.at[pq, strip(t & 7), :], sem),
            pltpu.make_async_copy(wq_u.at[blk(u, 64), 2, :], wq_r.at[2 + late, blk(u, 64), :], sem),
            pltpu.make_async_copy(wuk_u.at[blk(t & 7, 64), pk, :],
                                  wkv_r.at[1 - pk + late, blk(8 + (t & 7), 64), :], sem),
            pltpu.make_async_copy(wuv_u.at[blk(t & 7, 64), pk, :],
                                  wkv_r.at[1 - pk + late, blk(t & 7, 64), :], sem),
        )

    def cp_wq(p, sem):
        return pltpu.make_async_copy(wq_u.at[:, jnp.minimum(p, NP - 1), :], wq_r.at[p & 3], sem)

    def cp_p(g):
        slot = g & 1
        p = jnp.minimum(g + 1, NP - 1)
        o = jnp.minimum(g, NP - 1)
        sem = sem_p.at[slot]
        return (
            pltpu.make_async_copy(wo_u.at[blk(o >> 1, 2 * DA), blk(o & 1, M // 2)],
                                  wo_r.at[slot], sem),
            pltpu.make_async_copy(wuk_u.at[:, p, :], wkv_r.at[slot, pl.ds(DC, DC), :], sem),
            pltpu.make_async_copy(wuv_u.at[:, p, :], wkv_r.at[slot, pl.ds(0, DC), :], sem),
            cp_wq(g + 2, sem),
        )

    def cp_gw():
        return pltpu.make_async_copy(gw_hbm, gw_ref, sem_a.at[0])

    def cp_out(i, late):
        def cp(rows, cols):
            return pltpu.make_async_copy(out_s.at[rows, cols], out_hbm.at[rows, cols], sem_a.at[1])

        low = [cp(blk(2 * i + 1, TO // 2), pl.ds(512 * cc + 256 * late, 256)) for cc in range(2)]
        return low if late else [cp(blk(2 * i, TO // 2), pl.ds(0, M))] + low

    cp_w(0, sem_a.at[1]).start()
    group0, group1 = group(0, sem_a.at[2]), group(1)
    group0 = (group0[0], cp_x(-1, sem_a.at[2])) + group0[1:] + cp_wob(-1, sem_x.at[0])
    for d in group0 + group1[:1] + group1[2:]:
        d.start()

    for cc in range(8):
        qk_b[8 + cc, pl.ds(0, PAD), :] = jnp.zeros((PAD, 128), F32)
        vb[cc, pl.ds(TQ, PAD), :] = jnp.zeros((PAD, 128), F32)

    def stage_first(t):
        for cc, w in enumerate(_permute8(_lane_chunks(pltpu.bitcast(w_r[t & 1], U32)))):
            wperm[cc] = w

    def p1_step(t, peel, more=True):
        if not peel:
            for d in group(t):
                d.wait()

        def act_sums(src, dst, ns, m, sr, r, gate):
            cw = [[gate(src[(t & 1) + _zero(t, m), pl.ds(32 * (q >> 1) + 16 * (e >> 1) + 8 * r, 8),
                            pl.ds(((2 * (q & 1) + (e & 1)) * ns + sr) * 128, 128)])
                   for e in range(4)] for q in range(4)]
            for n, w in enumerate(_words49(_lhs7, cw, m)):
                dst[7 * m + n, t, pl.ds(16 * sr + 8 * r, 8), :] = w
            return [], 0, lambda: dst[7 * m + _zero(t, 0), t, pl.ds(16 * sr + 8 * r, 8), :]

        wv = []

        def load_wv():
            wv.extend(_permute8(_lane_chunks(jnp.concatenate(
                [pltpu.bitcast(wv_r[t & 1, e], U32) for e in range(4)], axis=0))))

        def w_sums(src, dst, m, cc, gate):
            ww = [[gate(src(m, 2 * (q >> 1) + (e >> 1), 2 * (2 * (q & 1) + (e & 1)) + cc))
                   for e in range(4)] for q in range(4)]
            for n, w in enumerate(_words49(_rhs7, ww, m)):
                dst[7 * m + n, cc, blk(t, 8), :] = w
            return [], 0, lambda: dst[7 * m + _zero(t, 0), cc, blk(t, 8), :]

        def v_src(m, rq, ch):
            return wv[ch][8 * rq:8 * rq + 8]

        def o_src(m, rq, ch):
            return wob_r[((t >> 1) & 1) + _zero(t, m), rq, blk(t & 1, 8), pl.ds(128 * ch, 128)]

        segs, step = (P0S, P0T) if peel else (P1S, 32)
        sched = _Sched(t > 99, _plan1(segs, P0W * peel, step, P0N if peel else P1N), dict(
            x=[part(act_sums, x_r, xq, 2, m, sr, r)
               for m in range(7) for sr in range(2) for r in range(2)],
            c=[part(act_sums, c_r, cq, 1, m, 0, r) for m in range(7) for r in range(2)],
            v=[part(w_sums, v_src, wv49, m, cc) for m in range(7) for cc in range(2)],
            o=[part(w_sums, o_src, wob49, m, cc) for m in range(7) for cc in range(2)]))

        first = t < 2
        for k, (half, r0, n) in enumerate(segs):
            if k == P0W * peel:
                if peel:
                    for d in group0[2:]:
                        d.wait()
                load_wv()
            w = jnp.concatenate([wperm[4 * half + cc] for cc in range(4)], axis=1)
            r = sched.mm(k, xs_u[t >> 1, pl.ds(r0 // 2, n // 2), :], w, step=step)
            if k == len(segs) - 1 and more:
                sched.finish()
                stage_first(t + 1)
                d = group(t + 2)
                e = piece(t + 2)
                d = d[2:6] + e[:1] + d[6:] + d[:2] + e[1:]
                for d in d + (piece(0) + piece(1) + (cp_gw(),) if peel else ()):
                    d.start()
            for cc in range(4):
                sl = (8 * (t & 1) + 4 * half + cc, pl.ds(PAD + r0, n), slice(None))
                new = r[:, cc * 128:(cc + 1) * 128]
                qk_b[sl] = new if peel else jnp.where(first, 0.0, qk_b[sl]) + new
        return t

    zero = jnp.max(vb[0, pl.ds(TQ, 8), :]).astype(jnp.int32)
    cp_w(0, sem_a.at[1]).wait()
    stage_first(0)
    group1[1].start()
    for d in group0[:2]:
        d.wait()
    p1_step(zero, True)
    last = jax.lax.fori_loop(1, 15, lambda t, c: p1_step(t, False), 0)
    for t in range(16):
        for d in piece(t):
            d.wait()
    p1_step(last + 1, False, False)

    row = jax.lax.broadcasted_iota(jnp.int32, (TQ, TQ), 0)
    col = jax.lax.broadcasted_iota(jnp.int32, (TQ, TQ), 1)
    col = (col & ~31) | ((col & 1) << 4) | ((col & 31) >> 1)
    rowi = jax.lax.broadcasted_iota(jnp.int32, (RB, 128), 0)
    odd = (jax.lax.broadcasted_iota(jnp.int32, (RB, 128), 1) & 1) == 1
    QSCALE = DA ** -0.5 * LOG2E

    def pair_rows(src, slot, r0, n, gate):
        return [_split(gate(src[slot, pl.ds(r0 + par, n // 2, stride=2), :])) for par in range(2)]

    def staging(g, z, never):
        ns = DC // SCR

        def scales(n1, k, gate):
            res = []
            for h in range(2):
                if k < ns:
                    w = gate(wkv_r[g & 1, pl.ds(n1 * DC + k * SCR, SCR), :])
                    w = pltpu.bitcast(w, jnp.int32) & (0x7F80 << (16 * h))
                else:
                    w = gate(sc_s[2 * n1 + h, pl.ds(0, 8 * ns), :])
                e = _tree([w[r:r + 8] for r in range(0, w.shape[0], 8)], jnp.maximum)
                if k == ns:
                    e = pltpu.bitcast(e << (16 - 16 * h), F32)
                    e = jnp.max(e, axis=0, keepdims=True)
                    e = jnp.clip(pltpu.bitcast(e, jnp.int32), 1 << 23, 253 << 23)
                    e = jnp.broadcast_to(e, (8, 128))
                    sc_s[2 * n1 + h, pl.ds(8 * ns + 8, 8), :] = (254 << 23) - e
                sc_s[2 * n1 + h, pl.ds(8 * k, 8), :] = e
                res.append(pltpu.bitcast(e, U32))
            return res, 0, lambda: pltpu.bitcast(sc_s[2 * n1, blk(k + _zero(z, 0), 8), :], U32)

        def rhs49(dst, tiles, scale, m, r, extra=()):
            res = [_ops49(_rhs7,
                          [[scale(tiles[2 * (q >> 1) + (e >> 1)][q & 1][par][e & 1],
                                  2 * (q & 1) + (e & 1)) for e in range(4)] for q in range(4)],
                          m) for par in range(2)]
            for k, (lo, hi) in enumerate(zip(*res)):
                w = _join(lo, hi)
                if k < len(extra):
                    w = jnp.where(never, extra[k], w)
                dst[7 * m + k, pl.ds(8 * r, 8), :] = w

        def kv(m, r, gate):
            if m == 0 and r == 0:
                for k in range(4):
                    ups[k] = pltpu.bitcast(gate(sc_s[k, pl.ds(8 * ns, 8), :]), F32)
            down = [pltpu.bitcast(sc_s[k + _zero(z, m), pl.ds(8 * ns + 8, 8), :], F32)
                    for k in range(4)]
            tiles = [[pair_rows(wkv_r, (g & 1) + _zero(z, m), n1 * DC + kt * 128 + 16 * r, 16, gate)
                      for n1 in range(2)] for kt in range(4)]
            rhs49(wkv, tiles, lambda w, k: w * down[k], m, r)
            return [], 0, lambda: wkv[7 * m, blk(r + _zero(z, 0), 8), :]

        def qw(m, r, gate):
            tiles = [[pair_rows(wq_r, ((g + 1 + n1) & 3) + _zero(z, m), kt * 256 + 16 * r, 16, gate)
                      for n1 in range(2)] for kt in range(4)]
            rhs49(wq49, tiles, lambda w, k: w, m, r, sc.pop(0)(gate)[0] if sc else ())
            return [], 0, lambda: wq49[7 * m, blk(r + _zero(z, 0), 8), :]

        sc = [part(scales, n1, k) for k in range(ns + 1) for n1 in range(2)]
        return dict(sc=sc,
                    kv=[part(kv, m, r) for m in range(7) for r in range(8)],
                    qw=[part(qw, m, r) for m in range(7) for r in range(16)])

    sched = _Sched(last > 99, _planx(), staging(-1, last, last > 99))
    w0 = pair_rows(wq_r, 0, 0, M, lambda x: x)
    w0 = [_join(w0[0][h], w0[1][h]) for h in range(2)]
    for g in range(4):
        for e in range(2):
            for h in range(2):
                q = [sched.mm(8 * g + 4 * e + 2 * h + k, jnp.concatenate(
                    [xs_u[4 * k + u, pl.ds((4 * g + 2 + e) * HQ, HQ), :] for u in range(4)], axis=1),
                    w0[h][256 * k:256 * k + 256], step=16) for k in range(2)]
                qn[h, g, e] = _pack((q[0] + q[1]) * QSCALE)
    sched.finish()
    for d in group(16) + piece(16):
        d.wait()
    for d in cp_p(1):
        d.start()
    plan2 = _plan2()

    def p2_body(p, carry):
        @pl.when(p > 0)
        def _():
            for d in cp_p(p):
                d.wait()

        causal = col <= row
        never = p > NP
        jobs = staging(p, p, never)
        sched = _Sched(never, plan2, jobs)
        mm = sched.mm

        r0 = pl.multiple_of(p * TQ, TQ)

        prods = {}

        def project(kind, j, n, lhs, rhs):
            got = prods.setdefault((kind, j), {})
            for m in ORDER[len(got):len(got) + n]:
                got[m] = _combine(lambda k: mm((kind, j, 7 * len(got) + ORDER.index(k)),
                                               part(lhs, 7 * m + k), rhs(7 * m + k)))
            if len(got) < 7:
                return None
            c = _combine(lambda m: got[m])
            return [[c[(rg & 2) + (cg >> 1)][2 * (rg & 1) + (cg & 1)] for rg in range(4)]
                    for cg in range(4)]

        def pair(ref, rows):
            return lambda k: jnp.concatenate([ref[k, sr, rows, :] for sr in range(2)], axis=1)

        def x_rows(b, n):
            return lambda k: jnp.concatenate([jnp.concatenate(
                [xq[k, b + j, pl.ds(16 * sr, 16), :] for sr in range(2)], axis=1)
                for j in range(n)], axis=0)

        def proj_b(kind, n, lhs, w, dst, off):
            c = project(kind, 0, n, lhs, pair(w, slice(None)))
            for cg in range(4 * (c is not None)):
                for rg in range(4):
                    for cc in range(2):
                        dst[2 * cg + cc, pl.ds(off + (PAD + rg * QQ), QQ), :] = (
                            c[cg][rg][:, cc * 128:(cc + 1) * 128])

        def proj_bv():
            for cc in range(8):
                vb[cc, pl.ds(0, PAD), :] = vb[cc, pl.ds(TQ, PAD), :]
            proj_b("bv", 7, x_rows(p, 1), wv49, vb, 0)

        def proj_bo(n):
            proj_b("bo", n, pair(ob49, slice(None)), wob49, qk_b, r0)

        def local_qk(rb, k, gate):
            rz = pl.multiple_of((p + _zero(p, k)) * TQ, TQ)
            q = [qk_b[cc, pl.ds(rz + (PAD + rb * RB), RB), :] for cc in range(8)]
            q[0] = gate(q[0])
            for w in range(LG * k, LG * k + LG):
                t = _fold([q[cc] * qk_b[8 + cc, pl.ds(r0 + (PAD + rb * RB - DIL * w), RB), :]
                           for cc in range(8)], jnp.add)
                t = t + pltpu.roll(t, 64, 1)
                t = t + jnp.where(odd, pltpu.roll(t, 1, 1), pltpu.roll(t, 127, 1))
                t = t * (DB ** -0.5 * LOG2E)
                if rb == 0 and w:
                    t = jnp.where(rowi + r0 >= DIL * w, t, NEG)
                lg_s[w, pl.ds(rb * RB, RB), :] = t
            return [], 1, lambda: pltpu.bitcast(lg_s[w, blk(2 * rb + _zero(p, 0), 8), :], U32)

        def local_sm(rb, e, gate):
            rows = pl.ds(rb * RB + SMR * e, SMR)
            lg = [gate(lg_s[w, rows, :]) for w in range(WIN)]
            m = _tree(lg, jnp.maximum)
            ps = [jnp.exp2(t - m) for t in lg]
            l = _tree(ps, jnp.add)
            r = pl.reciprocal(l, approx=True)
            r = r * (2.0 - l * r)
            for w in range(WIN):
                pr_s[w, rows, :] = ps[w] * r
            return [], 2, lambda: pltpu.bitcast(pr_s[0, blk(2 * rb + e + _zero(p, 0), 8), :], U32)

        def local_pv(rb, k, gate):
            rows = pl.ds(rb * RB, RB)
            ps = [pr_s[w + _zero(p, k), rows, :] for w in range(WIN)]
            ps[0] = gate(ps[0])
            o = [_fold([ps[w] * vb[cc, pl.ds(PAD + rb * RB - DIL * w, RB), :] for w in range(WIN)],
                       jnp.add) for cc in (k, k + 4)]
            for e in range(2):
                o_s[k + 4 * e, rows, :] = o[e]
            return [], 0, lambda: pltpu.bitcast(o_s[k, blk(2 * rb + _zero(p, 0), 8), :], U32)

        def o_sums(m, cc, r, gate):
            res = [_ops49(_lhs7, [[gate(o_s[
                2 * (2 * (q & 1) + (e & 1)) + cc + _zero(p, m),
                pl.ds(QQ * (2 * (q >> 1) + (e >> 1)) + 16 * r + par, 8, stride=2), :])
                for e in range(4)] for q in range(4)], m) for par in range(2)]
            for n, (lo, hi) in enumerate(zip(*res)):
                ob49[7 * m + n, cc, pl.ds(8 * r, 8), :] = _join(lo, hi)
            return [], 0, lambda: ob49[7 * m, cc, blk(r + _zero(p, 0), 8), :]

        jobs["os"] = [part(o_sums, m, cc, r) for r in range(2) for cc in range(2) for m in range(7)]
        order = list(range(0, 8, 2)) + list(range(1, 8, 2))
        jobs["lo"] = []
        for k in range(len(order) + SML):
            for f, d, n in ((local_sm, SML, RB // SMR), (local_qk, 0, 8 // LG)):
                if 0 <= k - d < len(order):
                    jobs["lo"] += [part(f, order[k - d], e) for e in range(n)]
        jobs["lv"] = [part(local_pv, rb, e) for rb in order for e in range(4)]

        def out_weights(m, r, gate):
            ww = [[gate(wo_r[(p & 1) + _zero(p, m),
                             pl.ds((2 * (q >> 1) + (e >> 1)) * HQ + 8 * r, 8),
                             pl.ds((2 * (q & 1) + (e & 1)) * 128, 128)])
                   for e in range(4)] for q in range(4)]
            rows = blk(8 * (p >> 1) + r, 8)
            extra = jobs["sc"].pop(0)(gate)[0] if jobs["sc"] else []
            for n, w in enumerate(_words49(_rhs7, ww, m)):
                if n < len(extra):
                    w = jnp.where(never, extra[n], w)
                wo49[7 * m + n, p & 1, rows, :] = w
            return [], 0, lambda: wo49[7 * m + _zero(p, 0), p & 1, rows, :]

        jobs["wo"] = [part(out_weights, m, r) for m in range(7) for r in range(8)]

        ks, vs, qs = {}, {}, {}
        done = {}

        def blocks(c, scale, pack):
            c = [[pack(t * scale(cg)) for t in c[cg]] for cg in range(4)]
            return [[jnp.concatenate([t[16 * e:16 * e + 16] for t in c[cg]], axis=0)
                     for e in range(2)] for cg in range(4)]

        def proj_kv(j, n):
            c = project("kv", j, n, lambda k: jnp.concatenate(
                [cq[k, 2 * j], cq[k, 2 * j + 1]], axis=0), lambda k: wkv[k])
            if c is not None:
                c = blocks(c, lambda cg: ups[cg][:1], _riffle)
                for cg in range(4):
                    for e in range(2):
                        (vs, ks)[cg >> 1][(cg & 1, 2 * j + e)] = c[cg][e]

        def proj_q(g, n):
            c = project("q", g, n, x_rows(4 * g + 2 * (p & 1), 2), lambda k: wq49[k])
            if c is not None:
                c = blocks(c, lambda cg: QSCALE, _pack)
                for h in range(2):
                    for e in range(2):
                        old = qn[h, g, e]
                        for b in range(2):
                            qs[(h, 4 * g + 2 * b + e)] = jnp.where((p & 1) == b, c[h][e], old)
                        qn[h, g, e] = c[2 + h][e]

        def qk(h, i, dep):
            kk = jnp.concatenate([ks[(h, j)] for j in range(i + 1)], axis=0)
            q = qs[(h, i)]
            if dep is not None:
                q = jnp.where(never, done[(h, dep)], q)
            ch = _lane_chunks(mm(("qk", h, i), q, kk, NT, 512))
            ch[i] = jnp.where(causal, ch[i], NEG)
            return ch

        def softmax_pv(h, i, ch):
            m = jnp.max(_fold(ch, jnp.maximum), axis=1, keepdims=True)
            ps = [jnp.exp2(c - m) for c in ch]
            lp = ps[0]
            for j in range(1, i + 1):
                lp = lp + ps[j]
                if TIE and (j % TIE == TIE - 1 or j == i):
                    ps[j] = jnp.where(never, lp, ps[j])
            pb = jnp.concatenate(ps, axis=1).astype(BF16)
            vv = jnp.concatenate([vs[(h, j)] for j in range(i + 1)], axis=0)
            o = mm(("pv", h, i), pb, vv)
            if i >= LDEP:
                lp = jnp.where(never, o, lp)
            l = jnp.sum(lp, axis=1, keepdims=True)
            r = pl.reciprocal(l, approx=True)
            r = r * (2.0 - l * r)
            cn = _pack(o * r)
            done[(h, i)] = cn
            if FA <= i < NQ - 1:
                if i + 3 < NQ:
                    site = ("kv", (i + 1) // 2 + 1, KVS * ((i + 1) & 1) + (F0, FD)[h])
                else:
                    site = ("bo", 0, 7 * (i + 3 - NQ) * BOP[0] + 8 * h)
                sched.pending.setdefault(site, []).append(cn)
            ctx[2 * p + h, pl.ds(i * HQ, HQ), :] = cn

        proj_bv()
        proj_kv(0, 7)
        proj_q(0, 7)
        for i in range(NQ):
            dep = i - DEP if DEP <= i < FA + DEP else None
            s0 = qk(0, i, dep)
            s1 = qk(1, i, dep)
            if i + 2 < NQ:
                proj_kv(i // 2 + 1, 7 if i & 1 else KVS // 7)
                if i < 6:
                    proj_q(i // 2 + 1, 7 if i & 1 else QS // 7)
            else:
                proj_bo(BOP[i + 2 - NQ])
            softmax_pv(0, i, s0)
            softmax_pv(1, i, s1)
        proj_bo(BOP[2])
        sched.finish()
        for d in cp_p(p + 2):
            d.start()
        return carry

    jax.lax.fori_loop(0, NP, p2_body, 0)

    cp_gw().wait()
    gw = gw_ref[...].astype(F32)
    plan3 = _plan3()
    cab = (ca0, ca1)

    def p3_body(i, carry):
        r0 = pl.multiple_of(i * TO, TO)
        h0 = pl.multiple_of(i * (TO // 2), TO // 2)
        never = i > S

        def ctx_words(m, u, r, n):
            return [[ctx[4 * u + 2 * (q & 1) + (e & 1),
                         pl.ds(h0 + _zero(i, m) * 8 + ((2 * (q >> 1) + (e >> 1)) * QQ + r), n), :]
                     for e in range(4)] for q in range(4)]

        def operands(k, u, r, gate):
            m = ORDER[k]
            cw = [[gate(w) for w in q] for q in ctx_words(m, u, r, 8)]
            for n, w in enumerate(_words49(_lhs7, cw, m)):
                if not (m in (2, 3) and n in (2, 3)):
                    cab[k & 1][n, pl.ds(r, 8), pl.ds(u * 128, 128)] = w
            return [], 0, lambda: cab[k & 1][_zero(i, 0), pl.ds(r, 8), pl.ds(u * 128, 128)]

        def gate_rows(r, gate):
            gs = _fold([_bf(gate(xs_u[j, pl.ds(h0 + r, 8), :])).astype(F32) * gw[j:j + 1]
                        for j in range(8)], jnp.add)
            g = jax.nn.sigmoid(jnp.sum(gs, axis=1, keepdims=True))
            g_s[pl.ds(2 * r, 16), :] = jnp.broadcast_to(g, (16, 128))
            return [], 0, lambda: pltpu.bitcast(g_s[blk(r // 4 + _zero(i, 0), 8), :], U32)

        pr = {}

        def mix(q, e, cc, gate):
            off = (2 * (q >> 1) + (e >> 1)) * HQ
            ch = 4 * cc + 2 * (q & 1) + (e & 1)
            a = _combine(lambda m: pr.get(m, pr[2])[e][:, cc * 128:(cc + 1) * 128])[q]
            g = gate(g_s[pl.ds(off, HQ), :])
            b = qk_b[ch, pl.ds(r0 + (PAD + off), HQ), :]
            out_s[pl.ds(r0 + off, HQ), pl.ds(ch * 128, 128)] = (g * a + (1.0 - g) * b).astype(BF16)
            return [], 0, lambda: pltpu.bitcast(
                out_s[blk(i * (TO // 16) + off // 16 + _zero(i, 0), 16), pl.ds(ch * 128, 128)], U32)

        sched = _Sched(never, plan3, dict(
            a=[part(operands, k, u, r) for k in range(1, 7) for u in range(HA // 4)
               for r in range(0, QQ, 8)],
            g=[part(gate_rows, r) for r in range(0, TO // 2, 8)],
            m=[part(mix, q, e, cc) for q in (1, 2, 0) for e in range(4) for cc in range(2)]))
        first = [[_words49(_lhs7, ctx_words(ORDER[0], u, 0, QQ), ORDER[0])[n]
                  for u in range(HA // 4)] for n in range(7)]

        def inner(m, n):
            k = ORDER.index(m)
            res = []
            for e in range(2):
                us = range(4 * e, 4 * e + 4)
                if m in (2, 3) and n in (2, 3):
                    lhs = jnp.concatenate([ctx_words(m, u, 0, QQ)[3 * (m - 2)][3 * (n - 2)]
                                           for u in us], axis=1)
                elif k == 0:
                    lhs = jnp.concatenate([first[n][u] for u in us], axis=1)
                else:
                    lhs = lambda: cab[k & 1][n, :, pl.ds(e * 512, 512)]
                rhs = jnp.concatenate([wo49[7 * m + n, cc, pl.ds(e * 256, 256), :]
                                       for cc in range(2)], axis=1)
                res.append(sched.mm((k, 2 * ORDER.index(n) + e), lhs, rhs))
                if (k, 2 * ORDER.index(n) + e) == (6, P3D):
                    for d in cp_out(i, 0):
                        d.start()
            return res[0] + res[1]

        for m in ORDER:
            pr[m] = _combine(lambda n: inner(m, n))
        sched.finish()
        for e in (1, 2, 0, 3):
            for cc in range(2):
                mix(3, e, cc, lambda x: x)
        for d in cp_out(i, 1):
            d.start()
        return carry

    jax.lax.fori_loop(0, S // TO, p3_body, 0)
    for d in cp_p(NP) + cp_p(NP + 1):
        d.wait()
    for i in range(S // TO):
        for d in cp_out(i, 0) + cp_out(i, 1):
            d.wait()


@jax.jit
def pallas_gated_mix__compressed_kv_cla__sliding_local_dilated__prompt_kernel(
    A_x: jax.Array,
    A_c_kv: jax.Array,
    A_w_q: jax.Array,
    A_w_uk: jax.Array,
    A_w_uv: jax.Array,
    A_w_o: jax.Array,
    B_x: jax.Array,
    B_wqkv: jax.Array,
    B_wo: jax.Array,
    gate_w: jax.Array,
):
    del B_x
    any_spec = pl.BlockSpec(memory_space=pl.ANY)
    out = pl.pallas_call(
        _kernel,
        in_specs=[any_spec] * 9,
        out_specs=any_spec,
        out_shape=jax.ShapeDtypeStruct((S, M), BF16),
        scratch_shapes=[
            pltpu.VMEM((9, S // 2, 128), U32),
            pltpu.VMEM((2, HQ, M), U32),
            pltpu.VMEM((2, HQ, DC), U32),
            pltpu.VMEM((2, 128, M), BF16),
            pltpu.VMEM((2, 4, 16, M), BF16),
            pltpu.VMEM((2, 4, 16, M), U32),
            pltpu.VMEM((3, 2 * DC, 128), U32),
            pltpu.VMEM((4, M, 128), U32),
            pltpu.VMEM((2, 2 * DA, M // 2), U32),
            pltpu.VMEM((8, 64, 128), U32),
            pltpu.VMEM((49, NQ, 32, 128), U32),
            pltpu.VMEM((49, NQ, 16, 128), U32),
            pltpu.VMEM((49, 2, M // 8, 128), U32),
            pltpu.VMEM((49, 2, M // 8, 128), U32),
            pltpu.VMEM((49, 2, NP * QQ, 128), U32),
            pltpu.VMEM((49, HQ, 128), U32),
            pltpu.VMEM((49, TQ, 128), U32),
            pltpu.VMEM((4, 8, 128), F32),
            pltpu.VMEM((4, DC // SCR * 8 + 16, 128), jnp.int32),
            pltpu.VMEM((2, 4, 2, HQ, 128), U32),
            pltpu.VMEM((16, S + PAD, 128), F32),
            pltpu.VMEM((8, TQ + PAD, 128), F32),
            pltpu.VMEM((WIN, TQ, 128), F32),
            pltpu.VMEM((WIN, TQ, 128), F32),
            pltpu.VMEM((8, TQ, 128), F32),
            pltpu.VMEM((49, 2, 16, 128), U32),
            pltpu.VMEM((HA, S // 2, 128), U32),
            pltpu.VMEM((7, QQ, M), U32),
            pltpu.VMEM((7, QQ, M), U32),
            pltpu.VMEM((TO, 128), F32),
            pltpu.VMEM((S, M), BF16),
            pltpu.VMEM((8, 128), BF16),
            pltpu.SemaphoreType.DMA((2,)),
            pltpu.SemaphoreType.DMA((2,)),
            pltpu.SemaphoreType.DMA((5,)),
        ],
        compiler_params=pltpu.CompilerParams(vmem_limit_bytes=120 * 1024 * 1024,
                                             disable_bounds_checks=True),
    )(
        A_x.reshape(S, M),
        A_c_kv.reshape(S, DC),
        A_w_q,
        A_w_uk,
        A_w_uv,
        A_w_o.reshape(HA * DA, M),
        B_wqkv.reshape(2, M // 2, 3 * M),
        B_wo.reshape(HB // 2, 2, DB, M),
        gate_w.reshape(8, 128),
    )
    return out.reshape(1, S, M)
```

```python
import functools

import jax
import jax.numpy as jnp
import jax.experimental.pallas as pl
import jax.experimental.pallas.tpu as pltpu

F32 = jnp.float32
BF16 = jnp.bfloat16
U32 = jnp.uint32

S = 2048
M = 1024
HA = 32
DA = 128
DC = 512
HB = 32
DB = 32
WIN = 8
DIL = 2
PAD = 16
LOG2E = 1.4426950408889634
NEG = -1e9

TQ = 128
HQ = TQ // 2
QQ = TQ // 4
NQ = S // TQ
NP = HA // 2
RB = 16
TO = 256

P0S = ((0, 0, 2048), (1, 0, 1024), (1, 1024, 768), (1, 1792, 128), (1, 1920, 128))
P0W = 1
P0A = 75
P0T = 16
P0N = 104
P1S = ((0, 0, 2048), (1, 0, 1536), (1, 1536, 384), (1, 1920, 128))
P1A = 60
P1N = 108
XN = 28
XQ = 50
BOP = (2, 3, 2)
KVS = 28
QS = 35
LX = 16
QST = 2
SK = 3
LG = 2
SMR = 16
SML = 1
SCR = 32
LN = 70
LA = 24
BS = 2
LP = ("kv", 1, 8)
BX = 8
BE = 42
DEP = 2
FA = 6
F0 = 0
FD = 8
TIE = 4
LDEP = 6
VL = 1
EXO = 1
PXO = 1
LF = 1
P3S = 3
P3E = 12
P3M = 6
P3D = 8

NN = (((1,), (0,)), ((), ()))
NT = (((1,), (1,)), ((), ()))


def _plan2():
    plan = {}

    def put(name, count, start, until):
        plan.setdefault(start, []).extend([(name, until)] * count)

    def after_qk(i):
        if i >= NQ - 2:
            return ("bo", 0, 7 * (i - NQ + 2) * BOP[0] + BX)
        return ("kv", i // 2 + 1, KVS * (i & 1) + LX)

    def fill(name, count, sites):
        for start, room, until in sites:
            n = min(count, room - len(plan.get(start, ())))
            put(name, n, start, until)
            count -= n
        assert count == 0, (name, count)

    def qk_sites(lo, hi):
        return [(("qk", h, i), max(i + 1 - h * SK, 0), after_qk(i))
                for i in range(lo, hi) for h in range(2)]

    def q_sites(g, lo, hi, until):
        return [(("q", g, k), 1, until) for k in range(lo, hi, QST)]

    ticks = ([("bv", 0, k) for k in range(LA, 49)] + [("kv", 0, k) for k in range(0, 49, 2)]
             + [("q", 0, k) for k in range(49)])
    for name, site in zip(_spread(["lo"] * (64 // LG + 128 // SMR), LN), ticks):
        put(name, 1, site, LP)
    host = [(("bv", 0, k), 1, ("kv", 0, 8)) for k in range(0, LA, BS)]
    early = []
    for g in range(1, 4):
        early += q_sites(g, 0, QS - 4, after_qk(2 * g - 1))
        early += qk_sites(2 * g - 1, 2 * g)
        early += q_sites(g, QS, 45, after_qk(2 * g))
        early += qk_sites(2 * g, 2 * g + 1)
    fill("lv", 32, early)
    fill("wo", 56, host + early)
    fill("os", 28, early + qk_sites(7, 14))
    fill("qw", 112, qk_sites(7, 14))
    fill("kv", 56, qk_sites(14, 16) + [(("bo", 0, k), 1, ("bo", 0, BE))
                                       for k in range(7 * BOP[0], 35)])
    return plan


def _planx():
    names = _spread(["qw"] * XQ + ["kv", "qw"] * 56 + ["qw"] * (56 - XQ), 8 * XN)
    return {k: [(n, 31) for n in names[8 * k:8 * k + 8]] for k in range(XN)}


def _spread(names, ticks):
    out = [None] * ticks
    for k, name in enumerate(names):
        out[k * ticks // len(names)] = name
    return out


def _plan1(segs, lo, step, count):
    end = len(segs) - 2
    ticks = [k for k in range(lo, end) for _ in range(segs[k][2] // step)][:count]
    n = len(ticks) * (P0A if lo else P1A) // 100
    names = _spread(["x"] * 28 + ["c"] * 14 + ["o"] * 14, n) + _spread(["v"] * 14, len(ticks) - n)
    plan = {}
    for k, name in zip(ticks, names):
        plan.setdefault(k, []).append((name, end))
    return plan


def _plan3():
    plan = {}
    for k in range(6):
        lo = P3S if k == 0 else 0
        extra = ["g"] * 8 if k in (1, 2) else []
        names = _spread(["a"] * 32 + extra, 4 * (P3E - lo))
        for d in range(lo, P3E):
            plan[(k, d)] = [(n, (k + 1, 0)) for n in names[4 * (d - lo):4 * (d - lo) + 4]]
    names = _spread(["m"] * 24, 4 * P3M)
    for d in range(P3M):
        plan[(6, d)] = [(n, (6, P3D)) for n in names[4 * d:4 * d + 4]]
    return plan


_STAGES = ((2, 4), (1, 3), (0, 2), (0, 6), (0, 1))


def _permute8(cols):
    cols = list(cols)
    lane = jax.lax.broadcasted_iota(jnp.int32, cols[0].shape, 1)
    for va, lb in _STAGES:
        lo = (lane & (1 << lb)) == 0
        sh = 1 << lb
        idx = [i for i in range(8) if not (i >> va) & 1]
        if lb == 6:
            rr = [pltpu.roll(jnp.where(lo, cols[i | (1 << va)], cols[i]), 64, 1) for i in idx]
            for i, r in zip(idx, rr):
                a, b = cols[i], cols[i | (1 << va)]
                cols[i] = jnp.where(lo, a, r)
                cols[i | (1 << va)] = jnp.where(lo, r, b)
        else:
            rb = [pltpu.roll(cols[i | (1 << va)], sh, 1) for i in idx]
            ra = [pltpu.roll(cols[i], 128 - sh, 1) for i in idx]
            for i, xa, xb in zip(idx, ra, rb):
                a, b = cols[i], cols[i | (1 << va)]
                cols[i] = jnp.where(lo, a, xb)
                cols[i | (1 << va)] = jnp.where(lo, xa, b)
    return cols


def _pack(x):
    return pltpu.bitcast(x.astype(BF16), U32)


def _bf(x):
    return pltpu.bitcast(x, BF16)


def _split(w):
    return (pltpu.bitcast(w << 16, F32), pltpu.bitcast(w & jnp.uint32(0xFFFF0000), F32))


def _join(lo, hi):
    return pltpu.bitcast(pltpu.pack_elementwise([lo, hi], packed_dtype=BF16), U32)


def _riffle(x):
    return jnp.concatenate([_join(x[r:r + 16], x[r + 16:r + 32]) for r in range(0, x.shape[0], 32)],
                           axis=0)


def _lhs7(a11, a12, a21, a22):
    return [a11 + a22, a21 + a22, a11, a22, a11 + a12, a21 - a11, a12 - a22]


def _rhs7(b11, b12, b21, b22):
    return [b11 + b22, b11, b12 - b22, b21 - b11, b22, b11 + b12, b21 + b22]


def _combine(mm):
    add = functools.partial(jax.tree.map, jnp.add)
    sub = functools.partial(jax.tree.map, jnp.subtract)
    m2 = mm(2)
    m3 = mm(3)
    m4 = mm(4)
    c12 = add(m2, m4)
    t11 = sub(m3, m4)
    m1 = mm(1)
    c21 = add(m1, m3)
    t22 = sub(m2, m1)
    m0 = mm(0)
    t11 = add(t11, m0)
    t22 = add(t22, m0)
    c11 = add(t11, mm(6))
    return c11, c12, c21, add(t22, mm(5))


ORDER = (2, 3, 4, 1, 0, 6, 5)


def _zero(i, m):
    return i >> (8 + m)


def _merge(vals):
    return _fold([v[r:r + 8, c:c + 128] for v in vals for r in range(0, v.shape[0], 8)
                  for c in range(0, v.shape[1], 128)], jnp.bitwise_or)


def _gate(never, g):
    def gate(x):
        t = jnp.tile(pltpu.bitcast(g, x.dtype), (x.shape[0] // 8, x.shape[1] // 128))
        return jnp.where(never, t, x)
    return gate


def _tie(never, x, deps):
    if not deps:
        return x
    top = jnp.where(never, _merge(deps), x[:8, :128])
    if x.shape[1] > 128:
        top = jnp.concatenate([top, x[:8, 128:]], axis=1)
    return jnp.concatenate([top, x[8:]], axis=0)


class _Sched:
    def __init__(self, never, plan, jobs):
        self.never, self.plan, self.jobs, self.pending = never, plan, jobs, {}

    def mm(self, site, a, b, dims=NN, width=128, step=32):
        deps = [d() if callable(d) else d for d in self.pending.pop(site, ())]
        a = a() if callable(a) else a
        tie = functools.partial(_tie, self.never, deps=deps)
        a, b = (_bf(tie(a)), _bf(b)) if a.dtype == U32 else (a, _bf(tie(b)))
        out = jax.lax.dot_general(a, b, dims, preferred_element_type=F32)
        per = out.shape[0] // step
        last = {}
        for k, (name, until) in enumerate(self.plan.get(site, ())):
            if name is not None:
                r, c = step * (k % per), min(width * (k // per), out.shape[1] - 128)
                vals, tag, stored = self.jobs[name].pop(0)(
                    _gate(self.never, out[r:r + 8, c:c + 128]))
                self.pending.setdefault(until, []).extend(vals)
                last[(name, tag, until)] = stored
        for (_, _, until), stored in last.items():
            if stored is not None:
                self.pending[until].append(stored)
        return out

    def finish(self):
        assert not any(self.jobs.values()) and not any(self.pending.values())


def _ops49(fn, blocks, m):
    return fn(*[fn(*[blocks[q][e] for q in range(4)])[m] for e in range(4)])


def _words49(fn, words, m):
    halves = [[_split(w) for w in q] for q in words]
    lo = _ops49(fn, [[h[0] for h in q] for q in halves], m)
    hi = _ops49(fn, [[h[1] for h in q] for q in halves], m)
    return [_join(a, b) for a, b in zip(lo, hi)]


def _fold(xs, op):
    acc = xs[0]
    for x in xs[1:]:
        acc = op(acc, x)
    return acc


def _tree(xs, op):
    while len(xs) > 1:
        xs = [op(a, b) for a, b in zip(xs[::2], xs[1::2])]
    return xs[0]


def _lane_chunks(x):
    return [x[:, j * 128:(j + 1) * 128] for j in range(x.shape[1] // 128)]


def _kernel(x_hbm, c_hbm, wq_hbm, wuk_hbm, wuv_hbm, wo_hbm, wqkv_hbm, wob_hbm, gw_hbm,
            out_hbm,
            xs_u, x_r, c_r, w_r, wv_r, wob_r, wkv_r, wq_r, wo_r,
            wperm, xq, cq, wv49, wob49, wo49, wkv, wq49, ups, sc_s, qn,
            qk_b, vb, lg_s, pr_s, o_s, ob49, ctx, ca0, ca1, g_s, out_s, gw_ref,
            sem_x, sem_p, sem_a):
    x_u = x_hbm.bitcast(U32)
    c_u = c_hbm.bitcast(U32)
    wo_u = wo_hbm.bitcast(U32)
    wq_u = wq_hbm.bitcast(U32)
    wuk_u = wuk_hbm.bitcast(U32)
    wuv_u = wuv_hbm.bitcast(U32)
    wob_u = wob_hbm.bitcast(U32)
    part = functools.partial

    def blk(j, n):
        return pl.ds(pl.multiple_of(j * n, n), n)

    def strip(j):
        return blk(j, 128)

    def cp_x(t, sem):
        k = (t + 1) >> 1
        return pltpu.make_async_copy(x_u.at[blk(t & 1, S // 4), strip(jnp.minimum(k, 7))],
                                     xs_u.at[jnp.minimum(k, 8), blk(t & 1, S // 4), :], sem)

    def cp_w(t, sem):
        u = t - 2 * (t >> 4)
        u = u - 2 * (u >> 4)
        return pltpu.make_async_copy(wqkv_hbm.at[u >> 3, strip((u >> 1) & 3), blk(u & 1, M)],
                                     w_r.at[u & 1], sem)

    def cp_wob(t, sem):
        b = (t + 1) >> 1
        c = jnp.minimum(b, 7)
        return tuple(pltpu.make_async_copy(
            wob_u.at[:, c & 1, 4 * (2 * (t & 1) + j) + (c & 2) + (c >> 2), :],
            wob_r.at[b & 1, 2 * (t & 1) + j], sem) for j in range(2))

    def group(t, sem1=None):
        sem = sem_x.at[t & 1]
        u = t - 2 * (t >> 4)
        return (
            cp_x(t, sem if sem1 is None else sem1),
            cp_w(t + 1, sem),
            pltpu.make_async_copy(x_u.at[blk(u, HQ), :], x_r.at[u & 1], sem),
            pltpu.make_async_copy(c_u.at[blk(u, HQ), :], c_r.at[u & 1], sem),
        ) + cp_wob(t, sem) + tuple(
            pltpu.make_async_copy(wqkv_hbm.at[e >> 1, blk(16 * (e & 1) + u, 16), pl.ds(2 * M, M)],
                                  wv_r.at[u & 1, e], sem) for e in range(4))

    def piece(t):
        late = t >> 4
        pq = (t >> 3) + late
        pk = (t >> 3) & 1
        u = (t & 15) + 2 * late
        sem = sem_a.at[3 + late]
        return (
            pltpu.make_async_copy(wo_u.at[blk(u, 16), pl.ds(0, M // 2)],
                                  wo_r.at[late, blk(u, 16), :], sem),
            pltpu.make_async_copy(wq_u.at[strip(t & 7), pq, :], wq_r.at[pq, strip(t & 7), :], sem),
            pltpu.make_async_copy(wq_u.at[blk(u, 64), 2, :], wq_r.at[2 + late, blk(u, 64), :], sem),
            pltpu.make_async_copy(wuk_u.at[blk(t & 7, 64), pk, :],
                                  wkv_r.at[1 - pk + late, blk(8 + (t & 7), 64), :], sem),
            pltpu.make_async_copy(wuv_u.at[blk(t & 7, 64), pk, :],
                                  wkv_r.at[1 - pk + late, blk(t & 7, 64), :], sem),
        )

    def cp_wq(p, sem):
        return pltpu.make_async_copy(wq_u.at[:, jnp.minimum(p, NP - 1), :], wq_r.at[p & 3], sem)

    def cp_p(g):
        slot = g & 1
        p = jnp.minimum(g + 1, NP - 1)
        o = jnp.minimum(g, NP - 1)
        sem = sem_p.at[slot]
        return (
            pltpu.make_async_copy(wo_u.at[blk(o >> 1, 2 * DA), blk(o & 1, M // 2)],
                                  wo_r.at[slot], sem),
            pltpu.make_async_copy(wuk_u.at[:, p, :], wkv_r.at[slot, pl.ds(DC, DC), :], sem),
            pltpu.make_async_copy(wuv_u.at[:, p, :], wkv_r.at[slot, pl.ds(0, DC), :], sem),
            cp_wq(g + 2, sem),
        )

    def cp_gw():
        return pltpu.make_async_copy(gw_hbm, gw_ref, sem_a.at[0])

    def cp_out(i, late):
        def cp(rows, cols):
            return pltpu.make_async_copy(out_s.at[rows, cols], out_hbm.at[rows, cols], sem_a.at[1])

        low = [cp(blk(2 * i + 1, TO // 2), pl.ds(512 * cc + 256 * late, 256)) for cc in range(2)]
        return low if late else [cp(blk(2 * i, TO // 2), pl.ds(0, M))] + low

    cp_w(0, sem_a.at[1]).start()
    group0, group1 = group(0, sem_a.at[2]), group(1)
    group0 = (group0[0], cp_x(-1, sem_a.at[2])) + group0[1:] + cp_wob(-1, sem_x.at[0])
    for d in group0 + group1[:1] + group1[2:]:
        d.start()

    for cc in range(8):
        qk_b[8 + cc, pl.ds(0, PAD), :] = jnp.zeros((PAD, 128), F32)
        vb[cc, pl.ds(TQ, PAD), :] = jnp.zeros((PAD, 128), F32)

    def stage_first(t):
        for cc, w in enumerate(_permute8(_lane_chunks(pltpu.bitcast(w_r[t & 1], U32)))):
            wperm[cc] = w

    def p1_step(t, peel, more=True):
        if not peel:
            for d in group(t):
                d.wait()

        def act_sums(src, dst, ns, m, sr, r, gate):
            cw = [[gate(src[(t & 1) + _zero(t, m), pl.ds(32 * (q >> 1) + 16 * (e >> 1) + 8 * r, 8),
                            pl.ds(((2 * (q & 1) + (e & 1)) * ns + sr) * 128, 128)])
                   for e in range(4)] for q in range(4)]
            for n, w in enumerate(_words49(_lhs7, cw, m)):
                dst[7 * m + n, t, pl.ds(16 * sr + 8 * r, 8), :] = w
            return [], 0, lambda: dst[7 * m + _zero(t, 0), t, pl.ds(16 * sr + 8 * r, 8), :]

        wv = []

        def load_wv():
            wv.extend(_permute8(_lane_chunks(jnp.concatenate(
                [pltpu.bitcast(wv_r[t & 1, e], U32) for e in range(4)], axis=0))))

        def w_sums(src, dst, m, cc, gate):
            ww = [[gate(src(m, 2 * (q >> 1) + (e >> 1), 2 * (2 * (q & 1) + (e & 1)) + cc))
                   for e in range(4)] for q in range(4)]
            for n, w in enumerate(_words49(_rhs7, ww, m)):
                dst[7 * m + n, cc, blk(t, 8), :] = w
            return [], 0, lambda: dst[7 * m + _zero(t, 0), cc, blk(t, 8), :]

        def v_src(m, rq, ch):
            return wv[ch][8 * rq:8 * rq + 8]

        def o_src(m, rq, ch):
            return wob_r[((t >> 1) & 1) + _zero(t, m), rq, blk(t & 1, 8), pl.ds(128 * ch, 128)]

        segs, step = (P0S, P0T) if peel else (P1S, 32)
        sched = _Sched(t > 99, _plan1(segs, P0W * peel, step, P0N if peel else P1N), dict(
            x=[part(act_sums, x_r, xq, 2, m, sr, r)
               for m in range(7) for sr in range(2) for r in range(2)],
            c=[part(act_sums, c_r, cq, 1, m, 0, r) for m in range(7) for r in range(2)],
            v=[part(w_sums, v_src, wv49, m, cc) for m in range(7) for cc in range(2)],
            o=[part(w_sums, o_src, wob49, m, cc) for m in range(7) for cc in range(2)]))

        first = t < 2
        for k, (half, r0, n) in enumerate(segs):
            if k == P0W * peel:
                if peel:
                    for d in group0[2:]:
                        d.wait()
                load_wv()
            w = jnp.concatenate([wperm[4 * half + cc] for cc in range(4)], axis=1)
            r = sched.mm(k, xs_u[t >> 1, pl.ds(r0 // 2, n // 2), :], w, step=step)
            if k == len(segs) - 1 and more:
                sched.finish()
                stage_first(t + 1)
                d = group(t + 2)
                e = piece(t + 2)
                d = d[2:6] + e[:1] + d[6:] + d[:2] + e[1:]
                for d in d + (piece(0) + piece(1) + (cp_gw(),) if peel else ()):
                    d.start()
            for cc in range(4):
                sl = (8 * (t & 1) + 4 * half + cc, pl.ds(PAD + r0, n), slice(None))
                new = r[:, cc * 128:(cc + 1) * 128]
                qk_b[sl] = new if peel else jnp.where(first, 0.0, qk_b[sl]) + new
        return t

    zero = jnp.max(vb[0, pl.ds(TQ, 8), :]).astype(jnp.int32)
    cp_w(0, sem_a.at[1]).wait()
    stage_first(0)
    group1[1].start()
    for d in group0[:2]:
        d.wait()
    p1_step(zero, True)
    last = jax.lax.fori_loop(1, 15, lambda t, c: p1_step(t, False), 0)
    for t in range(16):
        for d in piece(t):
            d.wait()
    p1_step(last + 1, False, False)

    row = jax.lax.broadcasted_iota(jnp.int32, (HQ, TQ), 0)
    col = jax.lax.broadcasted_iota(jnp.int32, (HQ, TQ), 1)
    col = (col & ~31) | ((col & 1) << 4) | ((col & 31) >> 1)
    rowi = jax.lax.broadcasted_iota(jnp.int32, (RB, 128), 0)
    odd = (jax.lax.broadcasted_iota(jnp.int32, (RB, 128), 1) & 1) == 1
    QSCALE = DA ** -0.5 * LOG2E

    def pair_rows(src, slot, r0, n, gate):
        return [_split(gate(src[slot, pl.ds(r0 + par, n // 2, stride=2), :])) for par in range(2)]

    def staging(g, z, never):
        ns = DC // SCR

        def scales(n1, k, gate):
            res = []
            for h in range(2):
                if k < ns:
                    w = gate(wkv_r[g & 1, pl.ds(n1 * DC + k * SCR, SCR), :])
                    w = pltpu.bitcast(w, jnp.int32) & (0x7F80 << (16 * h))
                else:
                    w = gate(sc_s[2 * n1 + h, pl.ds(0, 8 * ns), :])
                e = _tree([w[r:r + 8] for r in range(0, w.shape[0], 8)], jnp.maximum)
                if k == ns:
                    e = pltpu.bitcast(e << (16 - 16 * h), F32)
                    e = jnp.max(e, axis=0, keepdims=True)
                    e = jnp.clip(pltpu.bitcast(e, jnp.int32), 1 << 23, 253 << 23)
                    e = jnp.broadcast_to(e, (8, 128))
                    sc_s[2 * n1 + h, pl.ds(8 * ns + 8, 8), :] = (254 << 23) - e
                sc_s[2 * n1 + h, pl.ds(8 * k, 8), :] = e
                res.append(pltpu.bitcast(e, U32))
            return res, 0, lambda: pltpu.bitcast(sc_s[2 * n1, blk(k + _zero(z, 0), 8), :], U32)

        def rhs49(dst, tiles, scale, m, r, extra=()):
            res = [_ops49(_rhs7,
                          [[scale(tiles[2 * (q >> 1) + (e >> 1)][q & 1][par][e & 1],
                                  2 * (q & 1) + (e & 1)) for e in range(4)] for q in range(4)],
                          m) for par in range(2)]
            for k, (lo, hi) in enumerate(zip(*res)):
                w = _join(lo, hi)
                if k < len(extra):
                    w = jnp.where(never, extra[k], w)
                dst[7 * m + k, pl.ds(8 * r, 8), :] = w

        def kv(m, r, gate):
            if m == 0 and r == 0:
                for k in range(4):
                    ups[k] = pltpu.bitcast(gate(sc_s[k, pl.ds(8 * ns, 8), :]), F32)
            down = [pltpu.bitcast(sc_s[k + _zero(z, m), pl.ds(8 * ns + 8, 8), :], F32)
                    for k in range(4)]
            tiles = [[pair_rows(wkv_r, (g & 1) + _zero(z, m), n1 * DC + kt * 128 + 16 * r, 16, gate)
                      for n1 in range(2)] for kt in range(4)]
            rhs49(wkv, tiles, lambda w, k: w * down[k], m, r)
            return [], 0, lambda: wkv[7 * m, blk(r + _zero(z, 0), 8), :]

        def qw(m, r, gate):
            tiles = [[pair_rows(wq_r, ((g + 1 + n1) & 3) + _zero(z, m), kt * 256 + 16 * r, 16, gate)
                      for n1 in range(2)] for kt in range(4)]
            rhs49(wq49, tiles, lambda w, k: w, m, r, sc.pop(0)(gate)[0] if sc else ())
            return [], 0, lambda: wq49[7 * m, blk(r + _zero(z, 0), 8), :]

        sc = [part(scales, n1, k) for k in range(ns + 1) for n1 in range(2)]
        return dict(sc=sc,
                    kv=[part(kv, m, r) for m in range(7) for r in range(8)],
                    qw=[part(qw, m, r) for m in range(7) for r in range(16)])

    sched = _Sched(last > 99, _planx(), staging(-1, last, last > 99))
    w0 = pair_rows(wq_r, 0, 0, M, lambda x: x)
    w0 = [_join(w0[0][h], w0[1][h]) for h in range(2)]
    for g in range(4):
        for e in range(2):
            for h in range(2):
                q = [sched.mm(8 * g + 4 * e + 2 * h + k, jnp.concatenate(
                    [xs_u[4 * k + u, pl.ds((4 * g + 2 + e) * HQ, HQ), :] for u in range(4)], axis=1),
                    w0[h][256 * k:256 * k + 256], step=16) for k in range(2)]
                qn[h, g, e] = _pack((q[0] + q[1]) * QSCALE)
    sched.finish()
    for d in group(16) + piece(16):
        d.wait()
    for d in cp_p(1):
        d.start()
    plan2 = _plan2()

    def p2_body(p, carry):
        @pl.when(p > 0)
        def _():
            for d in cp_p(p):
                d.wait()

        causal = col <= row + HQ
        never = p > NP
        jobs = staging(p, p, never)
        sched = _Sched(never, plan2, jobs)
        mm = sched.mm

        r0 = pl.multiple_of(p * TQ, TQ)

        prods = {}

        def project(kind, j, n, lhs, rhs):
            got = prods.setdefault((kind, j), {})
            for m in ORDER[len(got):len(got) + n]:
                got[m] = _combine(lambda k: mm((kind, j, 7 * len(got) + ORDER.index(k)),
                                               part(lhs, 7 * m + k), rhs(7 * m + k)))
            if len(got) < 7:
                return None
            c = _combine(lambda m: got[m])
            return [[c[(rg & 2) + (cg >> 1)][2 * (rg & 1) + (cg & 1)] for rg in range(4)]
                    for cg in range(4)]

        def pair(ref, rows):
            return lambda k: jnp.concatenate([ref[k, sr, rows, :] for sr in range(2)], axis=1)

        def x_rows(b, n):
            return lambda k: jnp.concatenate([jnp.concatenate(
                [xq[k, b + j, pl.ds(16 * sr, 16), :] for sr in range(2)], axis=1)
                for j in range(n)], axis=0)

        def proj_b(kind, n, lhs, w, dst, off):
            c = project(kind, 0, n, lhs, pair(w, slice(None)))
            for cg in range(4 * (c is not None)):
                for rg in range(4):
                    for cc in range(2):
                        dst[2 * cg + cc, pl.ds(off + (PAD + rg * QQ), QQ), :] = (
                            c[cg][rg][:, cc * 128:(cc + 1) * 128])

        def proj_bv():
            for cc in range(8):
                vb[cc, pl.ds(0, PAD), :] = vb[cc, pl.ds(TQ, PAD), :]
            proj_b("bv", 7, x_rows(p, 1), wv49, vb, 0)

        def proj_bo(n):
            proj_b("bo", n, pair(ob49, slice(None)), wob49, qk_b, r0)

        def local_qk(rb, k, gate):
            rz = pl.multiple_of((p + _zero(p, k)) * TQ, TQ)
            q = [qk_b[cc, pl.ds(rz + (PAD + rb * RB), RB), :] for cc in range(8)]
            q[0] = gate(q[0])
            for w in range(LG * k, LG * k + LG):
                t = _fold([q[cc] * qk_b[8 + cc, pl.ds(r0 + (PAD + rb * RB - DIL * w), RB), :]
                           for cc in range(8)], jnp.add)
                t = t + pltpu.roll(t, 64, 1)
                t = t + jnp.where(odd, pltpu.roll(t, 1, 1), pltpu.roll(t, 127, 1))
                t = t * (DB ** -0.5 * LOG2E)
                if rb == 0 and w:
                    t = jnp.where(rowi + r0 >= DIL * w, t, NEG)
                lg_s[w, pl.ds(rb * RB, RB), :] = t
            return [], 1, lambda: pltpu.bitcast(lg_s[w, blk(2 * rb + _zero(p, 0), 8), :], U32)

        def local_sm(rb, e, gate):
            rows = pl.ds(rb * RB + SMR * e, SMR)
            lg = [gate(lg_s[w, rows, :]) for w in range(WIN)]
            m = _tree(lg, jnp.maximum)
            ps = [jnp.exp2(t - m) for t in lg]
            l = _tree(ps, jnp.add)
            r = pl.reciprocal(l, approx=True)
            r = r * (2.0 - l * r)
            for w in range(WIN):
                pr_s[w, rows, :] = ps[w] * r
            return [], 2, lambda: pltpu.bitcast(pr_s[0, blk(2 * rb + e + _zero(p, 0), 8), :], U32)

        def local_pv(rb, k, gate):
            rows = pl.ds(rb * RB, RB)
            ps = [pr_s[w + _zero(p, k), rows, :] for w in range(WIN)]
            ps[0] = gate(ps[0])
            o = [_fold([ps[w] * vb[cc, pl.ds(PAD + rb * RB - DIL * w, RB), :] for w in range(WIN)],
                       jnp.add) for cc in (k, k + 4)]
            for e in range(2):
                o_s[k + 4 * e, rows, :] = o[e]
            return [], 0, lambda: pltpu.bitcast(o_s[k, blk(2 * rb + _zero(p, 0), 8), :], U32)

        def o_sums(m, cc, r, gate):
            res = [_ops49(_lhs7, [[gate(o_s[
                2 * (2 * (q & 1) + (e & 1)) + cc + _zero(p, m),
                pl.ds(QQ * (2 * (q >> 1) + (e >> 1)) + 16 * r + par, 8, stride=2), :])
                for e in range(4)] for q in range(4)], m) for par in range(2)]
            for n, (lo, hi) in enumerate(zip(*res)):
                ob49[7 * m + n, cc, pl.ds(8 * r, 8), :] = _join(lo, hi)
            return [], 0, lambda: ob49[7 * m, cc, blk(r + _zero(p, 0), 8), :]

        jobs["os"] = [part(o_sums, m, cc, r) for r in range(2) for cc in range(2) for m in range(7)]
        order = list(range(0, 8, 2)) + list(range(1, 8, 2))
        jobs["lo"] = []
        for k in range(len(order) + SML):
            for f, d, n in ((local_sm, SML, RB // SMR), (local_qk, 0, 8 // LG)):
                if 0 <= k - d < len(order):
                    jobs["lo"] += [part(f, order[k - d], e) for e in range(n)]
        jobs["lv"] = [part(local_pv, rb, e) for rb in order for e in range(4)]

        def out_weights(m, r, gate):
            ww = [[gate(wo_r[(p & 1) + _zero(p, m),
                             pl.ds((2 * (q >> 1) + (e >> 1)) * HQ + 8 * r, 8),
                             pl.ds((2 * (q & 1) + (e & 1)) * 128, 128)])
                   for e in range(4)] for q in range(4)]
            rows = blk(8 * (p >> 1) + r, 8)
            extra = jobs["sc"].pop(0)(gate)[0] if jobs["sc"] else []
            for n, w in enumerate(_words49(_rhs7, ww, m)):
                if n < len(extra):
                    w = jnp.where(never, extra[n], w)
                wo49[7 * m + n, p & 1, rows, :] = w
            return [], 0, lambda: wo49[7 * m + _zero(p, 0), p & 1, rows, :]

        jobs["wo"] = [part(out_weights, m, r) for m in range(7) for r in range(8)]

        ks, vs, qs = {}, {}, {}
        done = {}

        def blocks(c, scale, pack):
            c = [[pack(t * scale(cg)) for t in c[cg]] for cg in range(4)]
            return [[jnp.concatenate([t[16 * e:16 * e + 16] for t in c[cg]], axis=0)
                     for e in range(2)] for cg in range(4)]

        def proj_kv(j, n):
            c = project("kv", j, n, lambda k: jnp.concatenate(
                [cq[k, 2 * j], cq[k, 2 * j + 1]], axis=0), lambda k: wkv[k])
            if c is not None:
                c = blocks(c, lambda cg: ups[cg][:1], _riffle)
                for cg in range(4):
                    for e in range(2):
                        (vs, ks)[cg >> 1][(cg & 1, 2 * j + e)] = c[cg][e]

        def proj_q(g, n):
            c = project("q", g, n, x_rows(4 * g + 2 * (p & 1), 2), lambda k: wq49[k])
            if c is not None:
                c = blocks(c, lambda cg: QSCALE, _pack)
                for h in range(2):
                    for e in range(2):
                        old = qn[h, g, e]
                        for b in range(2):
                            qs[(h, 4 * g + 2 * b + e)] = jnp.where((p & 1) == b, c[h][e], old)
                        qn[h, g, e] = c[2 + h][e]

        def halves(d, h, js):
            return jnp.concatenate([d[(h, j >> 1)][QQ * (j & 1):QQ * (j & 1) + QQ] for j in js],
                                   axis=0)

        def late(x, y, op):
            return jnp.concatenate([x[:HQ], op(x[HQ:], y)], axis=0)

        def unit(h, i):
            return halves(qs, h, (2 * (i & ~1) + (i & 1), 2 * (i | 1) + (i & 1)))

        def first(i):
            t = jnp.concatenate([mm(("kq", h, i), halves(ks, h, (0,)), unit(h, i), NT)
                                 for h in range(2)], axis=0).T
            keep = [col < HQ, col >= HQ]
            top = [col <= row, causal & keep[1]] if i == 0 else keep
            return [jnp.concatenate([jnp.where(a, t[:HQ], NEG), jnp.where(b, t[HQ:], NEG)], axis=0)
                    for a, b in zip(top, keep)]

        def qk(h, i, dep):
            off = 1 - (i & 1)
            q = unit(h, i)
            if dep is not None:
                q = jnp.where(never, done[(h, dep)], q)
            exf = lambda: mm(("qx", h, i), q[QQ:], halves(ks, h, (off + 2 * i, off + 2 * i + 1)), NT)
            ex = None if EXO else exf()
            ch = []
            if i:
                ch = _lane_chunks(mm(("qk", h, i), q, halves(ks, h, range(off, off + 2 * i)),
                                     NT, 512))
                ch[-1] = jnp.concatenate([jnp.where(causal, ch[-1][:HQ], NEG), ch[-1][HQ:]],
                                         axis=0)
            ex = exf() if EXO else ex
            return ch, jnp.where(causal, ex, NEG)

        def softmax_pv(h, i, ch, ex):
            off = 1 - (i & 1)
            m = jnp.max(late(_fold(ch, jnp.maximum), ex, jnp.maximum), axis=1, keepdims=True)
            pe = jnp.exp2(ex - m[HQ:])
            ps = [jnp.exp2(c - m) for c in ch]
            lp = late(ps[0], pe, jnp.add)
            for j in range(1, len(ch)):
                lp = lp + ps[j]
                if TIE and (j % TIE == TIE - 1 or j == len(ch) - 1):
                    ps[j] = jnp.where(never, lp, ps[j])
            pb = jnp.concatenate(ps, axis=1).astype(BF16)
            vv = [halves(vs, h, range(off, off + 2 * i))] if i else []
            v0 = [halves(vs, e, (0,)) for e in range(2 * off)]
            vv = jnp.concatenate(v0 + vv if LF else vv + v0, axis=0)
            oef = lambda: mm(("px", h, i), pe.astype(BF16), halves(vs, h, (off + 2 * i, off + 2 * i + 1)))
            oe = None if PXO else oef()
            o = mm(("pv", h, i), pb, vv)
            o = late(o, oef() if PXO else oe, jnp.add)
            if i >= LDEP:
                lp = jnp.where(never, o, lp)
            l = jnp.sum(lp, axis=1, keepdims=True)
            r = pl.reciprocal(l, approx=True)
            r = r * (2.0 - l * r)
            cn = _pack(o * r)
            done[(h, i)] = cn
            if FA <= i < NQ - 1:
                if i + 3 < NQ:
                    site = ("kv", (i + 1) // 2 + 1, KVS * ((i + 1) & 1) + (F0, FD)[h])
                else:
                    site = ("bo", 0, 7 * (i + 3 - NQ) * BOP[0] + 8 * h)
                sched.pending.setdefault(site, []).append(cn)
            for e in range(2):
                ctx[2 * p + h, pl.ds(((i & ~1) + e) * HQ + QQ * (i & 1), QQ), :] = (
                    cn[QQ * e:QQ * e + QQ])

        proj_bv()
        proj_kv(0, 7)
        proj_q(0, 7)
        lead = {}
        for i in range(NQ):
            dep = i - DEP if DEP <= i < FA + DEP else None
            for k in range(i, i + VL + 1):
                if k < NQ and not k & 1 and k not in lead and (0, k) in qs:
                    lead[k] = first(k)
            sx = [qk(h, i, dep) for h in range(2)]
            if i + 2 < NQ:
                proj_kv(i // 2 + 1, 7 if i & 1 else KVS // 7)
                if i < 6:
                    proj_q(i // 2 + 1, 7 if i & 1 else QS // 7)
            else:
                proj_bo(BOP[i + 2 - NQ])
            for h in range(2):
                c0 = [lead[i][h]] if i in lead else []
                softmax_pv(h, i, c0 + sx[h][0] if LF else sx[h][0] + c0, sx[h][1])
        proj_bo(BOP[2])
        sched.finish()
        for d in cp_p(p + 2):
            d.start()
        return carry

    jax.lax.fori_loop(0, NP, p2_body, 0)

    cp_gw().wait()
    gw = gw_ref[...].astype(F32)
    plan3 = _plan3()
    cab = (ca0, ca1)

    def p3_body(i, carry):
        r0 = pl.multiple_of(i * TO, TO)
        h0 = pl.multiple_of(i * (TO // 2), TO // 2)
        never = i > S

        def ctx_words(m, u, r, n):
            return [[ctx[4 * u + 2 * (q & 1) + (e & 1),
                         pl.ds(h0 + _zero(i, m) * 8 + ((2 * (q >> 1) + (e >> 1)) * QQ + r), n), :]
                     for e in range(4)] for q in range(4)]

        def operands(k, u, r, gate):
            m = ORDER[k]
            cw = [[gate(w) for w in q] for q in ctx_words(m, u, r, 8)]
            for n, w in enumerate(_words49(_lhs7, cw, m)):
                if not (m in (2, 3) and n in (2, 3)):
                    cab[k & 1][n, pl.ds(r, 8), pl.ds(u * 128, 128)] = w
            return [], 0, lambda: cab[k & 1][_zero(i, 0), pl.ds(r, 8), pl.ds(u * 128, 128)]

        def gate_rows(r, gate):
            gs = _fold([_bf(gate(xs_u[j, pl.ds(h0 + r, 8), :])).astype(F32) * gw[j:j + 1]
                        for j in range(8)], jnp.add)
            g = jax.nn.sigmoid(jnp.sum(gs, axis=1, keepdims=True))
            g_s[pl.ds(2 * r, 16), :] = jnp.broadcast_to(g, (16, 128))
            return [], 0, lambda: pltpu.bitcast(g_s[blk(r // 4 + _zero(i, 0), 8), :], U32)

        pr = {}

        def mix(q, e, cc, gate):
            off = (2 * (q >> 1) + (e >> 1)) * HQ
            ch = 4 * cc + 2 * (q & 1) + (e & 1)
            a = _combine(lambda m: pr.get(m, pr[2])[e][:, cc * 128:(cc + 1) * 128])[q]
            g = gate(g_s[pl.ds(off, HQ), :])
            b = qk_b[ch, pl.ds(r0 + (PAD + off), HQ), :]
            out_s[pl.ds(r0 + off, HQ), pl.ds(ch * 128, 128)] = (g * a + (1.0 - g) * b).astype(BF16)
            return [], 0, lambda: pltpu.bitcast(
                out_s[blk(i * (TO // 16) + off // 16 + _zero(i, 0), 16), pl.ds(ch * 128, 128)], U32)

        sched = _Sched(never, plan3, dict(
            a=[part(operands, k, u, r) for k in range(1, 7) for u in range(HA // 4)
               for r in range(0, QQ, 8)],
            g=[part(gate_rows, r) for r in range(0, TO // 2, 8)],
            m=[part(mix, q, e, cc) for q in (1, 2, 0) for e in range(4) for cc in range(2)]))
        first = [[_words49(_lhs7, ctx_words(ORDER[0], u, 0, QQ), ORDER[0])[n]
                  for u in range(HA // 4)] for n in range(7)]

        def inner(m, n):
            k = ORDER.index(m)
            res = []
            for e in range(2):
                us = range(4 * e, 4 * e + 4)
                if m in (2, 3) and n in (2, 3):
                    lhs = jnp.concatenate([ctx_words(m, u, 0, QQ)[3 * (m - 2)][3 * (n - 2)]
                                           for u in us], axis=1)
                elif k == 0:
                    lhs = jnp.concatenate([first[n][u] for u in us], axis=1)
                else:
                    lhs = lambda: cab[k & 1][n, :, pl.ds(e * 512, 512)]
                rhs = jnp.concatenate([wo49[7 * m + n, cc, pl.ds(e * 256, 256), :]
                                       for cc in range(2)], axis=1)
                res.append(sched.mm((k, 2 * ORDER.index(n) + e), lhs, rhs))
                if (k, 2 * ORDER.index(n) + e) == (6, P3D):
                    for d in cp_out(i, 0):
                        d.start()
            return res[0] + res[1]

        for m in ORDER:
            pr[m] = _combine(lambda n: inner(m, n))
        sched.finish()
        for e in (1, 2, 0, 3):
            for cc in range(2):
                mix(3, e, cc, lambda x: x)
        for d in cp_out(i, 1):
            d.start()
        return carry

    jax.lax.fori_loop(0, S // TO, p3_body, 0)
    for d in cp_p(NP) + cp_p(NP + 1):
        d.wait()
    for i in range(S // TO):
        for d in cp_out(i, 0) + cp_out(i, 1):
            d.wait()


@jax.jit
def pallas_gated_mix__compressed_kv_cla__sliding_local_dilated__prompt_kernel(
    A_x: jax.Array,
    A_c_kv: jax.Array,
    A_w_q: jax.Array,
    A_w_uk: jax.Array,
    A_w_uv: jax.Array,
    A_w_o: jax.Array,
    B_x: jax.Array,
    B_wqkv: jax.Array,
    B_wo: jax.Array,
    gate_w: jax.Array,
):
    del B_x
    any_spec = pl.BlockSpec(memory_space=pl.ANY)
    out = pl.pallas_call(
        _kernel,
        in_specs=[any_spec] * 9,
        out_specs=any_spec,
        out_shape=jax.ShapeDtypeStruct((S, M), BF16),
        scratch_shapes=[
            pltpu.VMEM((9, S // 2, 128), U32),
            pltpu.VMEM((2, HQ, M), U32),
            pltpu.VMEM((2, HQ, DC), U32),
            pltpu.VMEM((2, 128, M), BF16),
            pltpu.VMEM((2, 4, 16, M), BF16),
            pltpu.VMEM((2, 4, 16, M), U32),
            pltpu.VMEM((3, 2 * DC, 128), U32),
            pltpu.VMEM((4, M, 128), U32),
            pltpu.VMEM((2, 2 * DA, M // 2), U32),
            pltpu.VMEM((8, 64, 128), U32),
            pltpu.VMEM((49, NQ, 32, 128), U32),
            pltpu.VMEM((49, NQ, 16, 128), U32),
            pltpu.VMEM((49, 2, M // 8, 128), U32),
            pltpu.VMEM((49, 2, M // 8, 128), U32),
            pltpu.VMEM((49, 2, NP * QQ, 128), U32),
            pltpu.VMEM((49, HQ, 128), U32),
            pltpu.VMEM((49, TQ, 128), U32),
            pltpu.VMEM((4, 8, 128), F32),
            pltpu.VMEM((4, DC // SCR * 8 + 16, 128), jnp.int32),
            pltpu.VMEM((2, 4, 2, HQ, 128), U32),
            pltpu.VMEM((16, S + PAD, 128), F32),
            pltpu.VMEM((8, TQ + PAD, 128), F32),
            pltpu.VMEM((WIN, TQ, 128), F32),
            pltpu.VMEM((WIN, TQ, 128), F32),
            pltpu.VMEM((8, TQ, 128), F32),
            pltpu.VMEM((49, 2, 16, 128), U32),
            pltpu.VMEM((HA, S // 2, 128), U32),
            pltpu.VMEM((7, QQ, M), U32),
            pltpu.VMEM((7, QQ, M), U32),
            pltpu.VMEM((TO, 128), F32),
            pltpu.VMEM((S, M), BF16),
            pltpu.VMEM((8, 128), BF16),
            pltpu.SemaphoreType.DMA((2,)),
            pltpu.SemaphoreType.DMA((2,)),
            pltpu.SemaphoreType.DMA((5,)),
        ],
        compiler_params=pltpu.CompilerParams(vmem_limit_bytes=120 * 1024 * 1024,
                                             disable_bounds_checks=True),
    )(
        A_x.reshape(S, M),
        A_c_kv.reshape(S, DC),
        A_w_q,
        A_w_uk,
        A_w_uv,
        A_w_o.reshape(HA * DA, M),
        B_wqkv.reshape(2, M // 2, 3 * M),
        B_wo.reshape(HB // 2, 2, DB, M),
        gate_w.reshape(8, 128),
    )
    return out.reshape(1, S, M)
```

```python
import functools

import jax
import jax.numpy as jnp
import jax.experimental.pallas as pl
import jax.experimental.pallas.tpu as pltpu

F32 = jnp.float32
BF16 = jnp.bfloat16
U32 = jnp.uint32

S = 2048
M = 1024
HA = 32
DA = 128
DC = 512
HB = 32
DB = 32
WIN = 8
DIL = 2
PAD = 16
LOG2E = 1.4426950408889634
NEG = -1e9

TQ = 128
HQ = TQ // 2
QQ = TQ // 4
NQ = S // TQ
NP = HA // 2
RB = 16
TO = 256

P0S = ((0, 0, 2048), (1, 0, 1024), (1, 1024, 768), (1, 1792, 128), (1, 1920, 128))
P0W = 1
P0A = 75
P0T = 16
P0N = 104
P1S = ((0, 0, 2048), (1, 0, 1536), (1, 1536, 384), (1, 1920, 128))
P1A = 60
P1N = 108
XN = 28
XQ = 50
BOP = (2, 3, 2)
KVS = 28
QS = 35
LX = 16
QST = 2
SK = 3
LG = 1
SMR = 16
SML = 1
SCR = 32
LN = 92
LA = 16
BS = 2
LP = ("kv", 1, 8)
BX = 8
BE = 42
DEP = 2
FA = 6
F0 = 0
FD = 8
TIE = 4
LDEP = 6
VL = 1
IV = 3
KE = 4
KT = 42
HP = 53
EXO = 1
PXO = 1
LF = 1
P3S = 3
P3E = 12
P3M = 6
P3D = 8

NN = (((1,), (0,)), ((), ()))
NT = (((1,), (1,)), ((), ()))


def _head():
    rest = [(kind, 0, k) for kind in ("kv", "q") for k in range(49)]
    out, room = [], 0
    for k in range(49):
        out.append(("bv", 0, k))
        room += IV
        while rest and room >= 1 + (rest[0][0] == "q"):
            room -= 1 + (rest[0][0] == "q")
            out.append(rest.pop(0))
    return out + rest


def _plan2():
    plan = {}

    def put(name, count, start, until):
        plan.setdefault(start, []).extend([(name, until)] * count)

    def after_qk(i):
        if i >= NQ - 2:
            return ("bo", 0, 7 * (i - NQ + 2) * BOP[0] + BX)
        return ("kv", i // 2 + 1, KVS * (i & 1) + LX)

    def fill(name, count, sites):
        for start, room, until in sites:
            n = min(count, room - len(plan.get(start, ())))
            put(name, n, start, until)
            count -= n
        assert count == 0, (name, count)

    def qk_sites(lo, hi):
        return [(("qk", h, i), max(i + 1 - h * SK, 0), after_qk(i))
                for i in range(lo, hi) for h in range(2)]

    def q_sites(g, lo, hi, until):
        return [(("q", g, k), 1, until) for k in range(lo, hi, QST)]

    ticks = [t for t in _head() if t[0] != "kv" or t[2] & 1 == 0]
    for name, site in zip(_spread(["lo"] * (64 // LG + 128 // SMR), LN), ticks[LA:]):
        put(name, 1, site, LP)
    host = [(t, 1, ticks[HP]) for t in ticks[:LA:BS]]
    early = []
    for g in range(1, 4):
        early += q_sites(g, 0, QS - 4, after_qk(2 * g - 1))
        early += qk_sites(2 * g - 1, 2 * g)
        early += q_sites(g, QS, 45, after_qk(2 * g))
        early += qk_sites(2 * g, 2 * g + 1)
    fill("lv", 32, early)
    fill("wo", 56, host + early)
    fill("os", 28, early + qk_sites(7, 14))
    fill("qw", 112, qk_sites(7, 14))
    for k in range(KE):
        put("kv", 1, ("bo", 0, KT + k), None)
    fill("kv", 56 - KE, qk_sites(14, 16) + [(("bo", 0, k), 1, ("bo", 0, BE))
                                       for k in range(7 * BOP[0], 35)])
    return plan


def _planx():
    names = _spread(["qw"] * XQ + ["kv", "qw"] * 56 + ["qw"] * (56 - XQ), 8 * XN)
    return {k: [(n, 31) for n in names[8 * k:8 * k + 8]] for k in range(XN)}


def _spread(names, ticks):
    out = [None] * ticks
    for k, name in enumerate(names):
        out[k * ticks // len(names)] = name
    return out


def _plan1(segs, lo, step, count):
    end = len(segs) - 2
    ticks = [k for k in range(lo, end) for _ in range(segs[k][2] // step)][:count]
    n = len(ticks) * (P0A if lo else P1A) // 100
    names = _spread(["x"] * 28 + ["c"] * 14 + ["o"] * 14, n) + _spread(["v"] * 14, len(ticks) - n)
    plan = {}
    for k, name in zip(ticks, names):
        plan.setdefault(k, []).append((name, end))
    return plan


def _plan3():
    plan = {}
    for k in range(6):
        lo = P3S if k == 0 else 0
        extra = ["g"] * 8 if k in (1, 2) else []
        names = _spread(["a"] * 32 + extra, 4 * (P3E - lo))
        for d in range(lo, P3E):
            plan[(k, d)] = [(n, (k + 1, 0)) for n in names[4 * (d - lo):4 * (d - lo) + 4]]
    names = _spread(["m"] * 24, 4 * P3M)
    for d in range(P3M):
        plan[(6, d)] = [(n, (6, P3D)) for n in names[4 * d:4 * d + 4]]
    return plan


_STAGES = ((2, 4), (1, 3), (0, 2), (0, 6), (0, 1))


def _permute8(cols):
    cols = list(cols)
    lane = jax.lax.broadcasted_iota(jnp.int32, cols[0].shape, 1)
    for va, lb in _STAGES:
        lo = (lane & (1 << lb)) == 0
        sh = 1 << lb
        idx = [i for i in range(8) if not (i >> va) & 1]
        if lb == 6:
            rr = [pltpu.roll(jnp.where(lo, cols[i | (1 << va)], cols[i]), 64, 1) for i in idx]
            for i, r in zip(idx, rr):
                a, b = cols[i], cols[i | (1 << va)]
                cols[i] = jnp.where(lo, a, r)
                cols[i | (1 << va)] = jnp.where(lo, r, b)
        else:
            rb = [pltpu.roll(cols[i | (1 << va)], sh, 1) for i in idx]
            ra = [pltpu.roll(cols[i], 128 - sh, 1) for i in idx]
            for i, xa, xb in zip(idx, ra, rb):
                a, b = cols[i], cols[i | (1 << va)]
                cols[i] = jnp.where(lo, a, xb)
                cols[i | (1 << va)] = jnp.where(lo, xa, b)
    return cols


def _pack(x):
    return pltpu.bitcast(x.astype(BF16), U32)


def _bf(x):
    return pltpu.bitcast(x, BF16)


def _split(w):
    return (pltpu.bitcast(w << 16, F32), pltpu.bitcast(w & jnp.uint32(0xFFFF0000), F32))


def _join(lo, hi):
    return pltpu.bitcast(pltpu.pack_elementwise([lo, hi], packed_dtype=BF16), U32)


def _riffle(x):
    return jnp.concatenate([_join(x[r:r + 16], x[r + 16:r + 32]) for r in range(0, x.shape[0], 32)],
                           axis=0)


def _lhs7(a11, a12, a21, a22):
    return [a11 + a22, a21 + a22, a11, a22, a11 + a12, a21 - a11, a12 - a22]


def _rhs7(b11, b12, b21, b22):
    return [b11 + b22, b11, b12 - b22, b21 - b11, b22, b11 + b12, b21 + b22]


def _steps():
    add = functools.partial(jax.tree.map, jnp.add)
    sub = functools.partial(jax.tree.map, jnp.subtract)
    m2 = yield 2
    m3 = yield 3
    m4 = yield 4
    c12 = add(m2, m4)
    t11 = sub(m3, m4)
    m1 = yield 1
    c21 = add(m1, m3)
    t22 = sub(m2, m1)
    m0 = yield 0
    t11 = add(t11, m0)
    t22 = add(t22, m0)
    c11 = add(t11, (yield 6))
    yield c11, c12, c21, add(t22, (yield 5))


def _combine(mm):
    g = _steps()
    k = next(g)
    for _ in range(7):
        k = g.send(mm(k))
    return k


ORDER = (2, 3, 4, 1, 0, 6, 5)


def _zero(i, m):
    return i >> (8 + m)


def _merge(vals):
    return _fold([v[r:r + 8, c:c + 128] for v in vals for r in range(0, v.shape[0], 8)
                  for c in range(0, v.shape[1], 128)], jnp.bitwise_or)


def _gate(never, g):
    def gate(x):
        t = jnp.tile(pltpu.bitcast(g, x.dtype), (x.shape[0] // 8, x.shape[1] // 128))
        return jnp.where(never, t, x)
    return gate


def _tie(never, x, deps):
    if not deps:
        return x
    top = jnp.where(never, _merge(deps), x[:8, :128])
    if x.shape[1] > 128:
        top = jnp.concatenate([top, x[:8, 128:]], axis=1)
    return jnp.concatenate([top, x[8:]], axis=0)


class _Sched:
    def __init__(self, never, plan, jobs):
        self.never, self.plan, self.jobs, self.pending = never, plan, jobs, {}

    def mm(self, site, a, b, dims=NN, width=128, step=32):
        deps = [d() if callable(d) else d for d in self.pending.pop(site, ())]
        a = a() if callable(a) else a
        tie = functools.partial(_tie, self.never, deps=deps)
        a, b = (_bf(tie(a)), _bf(b)) if a.dtype == U32 else (a, _bf(tie(b)))
        out = jax.lax.dot_general(a, b, dims, preferred_element_type=F32)
        per = out.shape[0] // step
        last = {}
        for k, (name, until) in enumerate(self.plan.get(site, ())):
            if name is not None:
                r, c = step * (k % per), min(width * (k // per), out.shape[1] - 128)
                vals, tag, stored = self.jobs[name].pop(0)(
                    _gate(self.never, out[r:r + 8, c:c + 128]))
                self.pending.setdefault(until, []).extend(vals)
                last[(name, tag, until)] = stored
        for (_, _, until), stored in last.items():
            if stored is not None:
                self.pending[until].append(stored)
        return out

    def finish(self):
        self.pending.pop(None, None)
        assert not any(self.jobs.values()) and not any(self.pending.values())


def _ops49(fn, blocks, m):
    return fn(*[fn(*[blocks[q][e] for q in range(4)])[m] for e in range(4)])


def _words49(fn, words, m):
    halves = [[_split(w) for w in q] for q in words]
    lo = _ops49(fn, [[h[0] for h in q] for q in halves], m)
    hi = _ops49(fn, [[h[1] for h in q] for q in halves], m)
    return [_join(a, b) for a, b in zip(lo, hi)]


def _fold(xs, op):
    acc = xs[0]
    for x in xs[1:]:
        acc = op(acc, x)
    return acc


def _tree(xs, op):
    while len(xs) > 1:
        xs = [op(a, b) for a, b in zip(xs[::2], xs[1::2])]
    return xs[0]


def _lane_chunks(x):
    return [x[:, j * 128:(j + 1) * 128] for j in range(x.shape[1] // 128)]


def _kernel(x_hbm, c_hbm, wq_hbm, wuk_hbm, wuv_hbm, wo_hbm, wqkv_hbm, wob_hbm, gw_hbm,
            out_hbm,
            xs_u, x_r, c_r, w_r, wv_r, wob_r, wkv_r, wq_r, wo_r,
            wperm, xq, cq, wv49, wob49, wo49, wkv, wq49, ups, sc_s, qn,
            qk_b, vb, lg_s, pr_s, o_s, ob49, ctx, ca0, ca1, g_s, out_s, gw_ref,
            sem_x, sem_p, sem_a):
    x_u = x_hbm.bitcast(U32)
    c_u = c_hbm.bitcast(U32)
    wo_u = wo_hbm.bitcast(U32)
    wq_u = wq_hbm.bitcast(U32)
    wuk_u = wuk_hbm.bitcast(U32)
    wuv_u = wuv_hbm.bitcast(U32)
    wob_u = wob_hbm.bitcast(U32)
    part = functools.partial

    def blk(j, n):
        return pl.ds(pl.multiple_of(j * n, n), n)

    def strip(j):
        return blk(j, 128)

    def cp_x(t, sem):
        k = (t + 1) >> 1
        return pltpu.make_async_copy(x_u.at[blk(t & 1, S // 4), strip(jnp.minimum(k, 7))],
                                     xs_u.at[jnp.minimum(k, 8), blk(t & 1, S // 4), :], sem)

    def cp_w(t, sem):
        u = t - 2 * (t >> 4)
        u = u - 2 * (u >> 4)
        return pltpu.make_async_copy(wqkv_hbm.at[u >> 3, strip((u >> 1) & 3), blk(u & 1, M)],
                                     w_r.at[u & 1], sem)

    def cp_wob(t, sem):
        b = (t + 1) >> 1
        c = jnp.minimum(b, 7)
        return tuple(pltpu.make_async_copy(
            wob_u.at[:, c & 1, 4 * (2 * (t & 1) + j) + (c & 2) + (c >> 2), :],
            wob_r.at[b & 1, 2 * (t & 1) + j], sem) for j in range(2))

    def group(t, sem1=None):
        sem = sem_x.at[t & 1]
        u = t - 2 * (t >> 4)
        return (
            cp_x(t, sem if sem1 is None else sem1),
            cp_w(t + 1, sem),
            pltpu.make_async_copy(x_u.at[blk(u, HQ), :], x_r.at[u & 1], sem),
            pltpu.make_async_copy(c_u.at[blk(u, HQ), :], c_r.at[u & 1], sem),
        ) + cp_wob(t, sem) + tuple(
            pltpu.make_async_copy(wqkv_hbm.at[e >> 1, blk(16 * (e & 1) + u, 16), pl.ds(2 * M, M)],
                                  wv_r.at[u & 1, e], sem) for e in range(4))

    def piece(t):
        late = t >> 4
        pq = (t >> 3) + late
        pk = (t >> 3) & 1
        u = (t & 15) + 2 * late
        sem = sem_a.at[3 + late]
        return (
            pltpu.make_async_copy(wo_u.at[blk(u, 16), pl.ds(0, M // 2)],
                                  wo_r.at[late, blk(u, 16), :], sem),
            pltpu.make_async_copy(wq_u.at[strip(t & 7), pq, :], wq_r.at[pq, strip(t & 7), :], sem),
            pltpu.make_async_copy(wq_u.at[blk(u, 64), 2, :], wq_r.at[2 + late, blk(u, 64), :], sem),
            pltpu.make_async_copy(wuk_u.at[blk(t & 7, 64), pk, :],
                                  wkv_r.at[1 - pk + late, blk(8 + (t & 7), 64), :], sem),
            pltpu.make_async_copy(wuv_u.at[blk(t & 7, 64), pk, :],
                                  wkv_r.at[1 - pk + late, blk(t & 7, 64), :], sem),
        )

    def cp_wq(p, sem):
        return pltpu.make_async_copy(wq_u.at[:, jnp.minimum(p, NP - 1), :], wq_r.at[p & 3], sem)

    def cp_p(g):
        slot = g & 1
        p = jnp.minimum(g + 1, NP - 1)
        o = jnp.minimum(g, NP - 1)
        sem = sem_p.at[slot]
        return (
            pltpu.make_async_copy(wo_u.at[blk(o >> 1, 2 * DA), blk(o & 1, M // 2)],
                                  wo_r.at[slot], sem),
            pltpu.make_async_copy(wuk_u.at[:, p, :], wkv_r.at[slot, pl.ds(DC, DC), :], sem),
            pltpu.make_async_copy(wuv_u.at[:, p, :], wkv_r.at[slot, pl.ds(0, DC), :], sem),
            cp_wq(g + 2, sem),
        )

    def cp_gw():
        return pltpu.make_async_copy(gw_hbm, gw_ref, sem_a.at[0])

    def cp_out(i, late):
        def cp(rows, cols):
            return pltpu.make_async_copy(out_s.at[rows, cols], out_hbm.at[rows, cols], sem_a.at[1])

        low = [cp(blk(2 * i + 1, TO // 2), pl.ds(512 * cc + 256 * late, 256)) for cc in range(2)]
        return low if late else [cp(blk(2 * i, TO // 2), pl.ds(0, M))] + low

    cp_w(0, sem_a.at[1]).start()
    group0, group1 = group(0, sem_a.at[2]), group(1)
    group0 = (group0[0], cp_x(-1, sem_a.at[2])) + group0[1:] + cp_wob(-1, sem_x.at[0])
    for d in group0 + group1[:1] + group1[2:]:
        d.start()

    for cc in range(8):
        qk_b[8 + cc, pl.ds(0, PAD), :] = jnp.zeros((PAD, 128), F32)
        vb[cc, pl.ds(TQ, PAD), :] = jnp.zeros((PAD, 128), F32)

    def stage_first(t):
        for cc, w in enumerate(_permute8(_lane_chunks(pltpu.bitcast(w_r[t & 1], U32)))):
            wperm[cc] = w

    def p1_step(t, peel, more=True):
        if not peel:
            for d in group(t):
                d.wait()

        def act_sums(src, dst, ns, m, sr, r, gate):
            cw = [[gate(src[(t & 1) + _zero(t, m), pl.ds(32 * (q >> 1) + 16 * (e >> 1) + 8 * r, 8),
                            pl.ds(((2 * (q & 1) + (e & 1)) * ns + sr) * 128, 128)])
                   for e in range(4)] for q in range(4)]
            for n, w in enumerate(_words49(_lhs7, cw, m)):
                dst[7 * m + n, t, pl.ds(16 * sr + 8 * r, 8), :] = w
            return [], 0, lambda: dst[7 * m + _zero(t, 0), t, pl.ds(16 * sr + 8 * r, 8), :]

        wv = []

        def load_wv():
            wv.extend(_permute8(_lane_chunks(jnp.concatenate(
                [pltpu.bitcast(wv_r[t & 1, e], U32) for e in range(4)], axis=0))))

        def w_sums(src, dst, m, cc, gate):
            ww = [[gate(src(m, 2 * (q >> 1) + (e >> 1), 2 * (2 * (q & 1) + (e & 1)) + cc))
                   for e in range(4)] for q in range(4)]
            for n, w in enumerate(_words49(_rhs7, ww, m)):
                dst[7 * m + n, cc, blk(t, 8), :] = w
            return [], 0, lambda: dst[7 * m + _zero(t, 0), cc, blk(t, 8), :]

        def v_src(m, rq, ch):
            return wv[ch][8 * rq:8 * rq + 8]

        def o_src(m, rq, ch):
            return wob_r[((t >> 1) & 1) + _zero(t, m), rq, blk(t & 1, 8), pl.ds(128 * ch, 128)]

        segs, step = (P0S, P0T) if peel else (P1S, 32)
        sched = _Sched(t > 99, _plan1(segs, P0W * peel, step, P0N if peel else P1N), dict(
            x=[part(act_sums, x_r, xq, 2, m, sr, r)
               for m in range(7) for sr in range(2) for r in range(2)],
            c=[part(act_sums, c_r, cq, 1, m, 0, r) for m in range(7) for r in range(2)],
            v=[part(w_sums, v_src, wv49, m, cc) for m in range(7) for cc in range(2)],
            o=[part(w_sums, o_src, wob49, m, cc) for m in range(7) for cc in range(2)]))

        first = t < 2
        for k, (half, r0, n) in enumerate(segs):
            if k == P0W * peel:
                if peel:
                    for d in group0[2:]:
                        d.wait()
                load_wv()
            w = jnp.concatenate([wperm[4 * half + cc] for cc in range(4)], axis=1)
            r = sched.mm(k, xs_u[t >> 1, pl.ds(r0 // 2, n // 2), :], w, step=step)
            if k == len(segs) - 1 and more:
                sched.finish()
                stage_first(t + 1)
                d = group(t + 2)
                e = piece(t + 2)
                d = d[2:6] + e[:1] + d[6:] + d[:2] + e[1:]
                for d in d + (piece(0) + piece(1) + (cp_gw(),) if peel else ()):
                    d.start()
            for cc in range(4):
                sl = (8 * (t & 1) + 4 * half + cc, pl.ds(PAD + r0, n), slice(None))
                new = r[:, cc * 128:(cc + 1) * 128]
                qk_b[sl] = new if peel else jnp.where(first, 0.0, qk_b[sl]) + new
        return t

    zero = jnp.max(vb[0, pl.ds(TQ, 8), :]).astype(jnp.int32)
    cp_w(0, sem_a.at[1]).wait()
    stage_first(0)
    group1[1].start()
    for d in group0[:2]:
        d.wait()
    p1_step(zero, True)
    last = jax.lax.fori_loop(1, 15, lambda t, c: p1_step(t, False), 0)
    for t in range(16):
        for d in piece(t):
            d.wait()
    p1_step(last + 1, False, False)

    row = jax.lax.broadcasted_iota(jnp.int32, (HQ, TQ), 0)
    col = jax.lax.broadcasted_iota(jnp.int32, (HQ, TQ), 1)
    col = (col & ~31) | ((col & 1) << 4) | ((col & 31) >> 1)
    rowi = jax.lax.broadcasted_iota(jnp.int32, (RB, 128), 0)
    odd = (jax.lax.broadcasted_iota(jnp.int32, (RB, 128), 1) & 1) == 1
    QSCALE = DA ** -0.5 * LOG2E

    def pair_rows(src, slot, r0, n, gate):
        return [_split(gate(src[slot, pl.ds(r0 + par, n // 2, stride=2), :])) for par in range(2)]

    def staging(g, z, never):
        ns = DC // SCR

        def scales(n1, k, gate):
            res = []
            for h in range(2):
                if k < ns:
                    w = gate(wkv_r[g & 1, pl.ds(n1 * DC + k * SCR, SCR), :])
                    w = pltpu.bitcast(w, jnp.int32) & (0x7F80 << (16 * h))
                else:
                    w = gate(sc_s[2 * n1 + h, pl.ds(0, 8 * ns), :])
                e = _tree([w[r:r + 8] for r in range(0, w.shape[0], 8)], jnp.maximum)
                if k == ns:
                    e = pltpu.bitcast(e << (16 - 16 * h), F32)
                    e = jnp.max(e, axis=0, keepdims=True)
                    e = jnp.clip(pltpu.bitcast(e, jnp.int32), 1 << 23, 253 << 23)
                    e = jnp.broadcast_to(e, (8, 128))
                    sc_s[2 * n1 + h, pl.ds(8 * ns + 8, 8), :] = (254 << 23) - e
                sc_s[2 * n1 + h, pl.ds(8 * k, 8), :] = e
                res.append(pltpu.bitcast(e, U32))
            return res, 0, lambda: pltpu.bitcast(sc_s[2 * n1, blk(k + _zero(z, 0), 8), :], U32)

        def rhs49(dst, tiles, scale, m, r, extra=()):
            res = [_ops49(_rhs7,
                          [[scale(tiles[2 * (q >> 1) + (e >> 1)][q & 1][par][e & 1],
                                  2 * (q & 1) + (e & 1)) for e in range(4)] for q in range(4)],
                          m) for par in range(2)]
            for k, (lo, hi) in enumerate(zip(*res)):
                w = _join(lo, hi)
                if k < len(extra):
                    w = jnp.where(never, extra[k], w)
                dst[7 * m + k, pl.ds(8 * r, 8), :] = w

        def kv(m, r, gate):
            if m == 0 and r == 0:
                for k in range(4):
                    ups[k] = pltpu.bitcast(gate(sc_s[k, pl.ds(8 * ns, 8), :]), F32)
            down = [pltpu.bitcast(sc_s[k + _zero(z, m), pl.ds(8 * ns + 8, 8), :], F32)
                    for k in range(4)]
            tiles = [[pair_rows(wkv_r, (g & 1) + _zero(z, m), n1 * DC + kt * 128 + 16 * r, 16, gate)
                      for n1 in range(2)] for kt in range(4)]
            rhs49(wkv, tiles, lambda w, k: w * down[k], m, r)
            return [], 0, lambda: wkv[7 * m, blk(r + _zero(z, 0), 8), :]

        def qw(m, r, gate):
            tiles = [[pair_rows(wq_r, ((g + 1 + n1) & 3) + _zero(z, m), kt * 256 + 16 * r, 16, gate)
                      for n1 in range(2)] for kt in range(4)]
            rhs49(wq49, tiles, lambda w, k: w, m, r, sc.pop(0)(gate)[0] if sc else ())
            return [], 0, lambda: wq49[7 * m, blk(r + _zero(z, 0), 8), :]

        sc = [part(scales, n1, k) for k in range(ns + 1) for n1 in range(2)]
        return dict(sc=sc,
                    kv=[part(kv, m, r) for m in range(7) for r in range(8)],
                    qw=[part(qw, m, r) for m in range(7) for r in range(16)])

    sched = _Sched(last > 99, _planx(), staging(-1, last, last > 99))
    w0 = pair_rows(wq_r, 0, 0, M, lambda x: x)
    w0 = [_join(w0[0][h], w0[1][h]) for h in range(2)]
    for g in range(4):
        for e in range(2):
            for h in range(2):
                q = [sched.mm(8 * g + 4 * e + 2 * h + k, jnp.concatenate(
                    [xs_u[4 * k + u, pl.ds((4 * g + 2 + e) * HQ, HQ), :] for u in range(4)], axis=1),
                    w0[h][256 * k:256 * k + 256], step=16) for k in range(2)]
                qn[h, g, e] = _pack((q[0] + q[1]) * QSCALE)
    sched.finish()
    for d in group(16) + piece(16):
        d.wait()
    for d in cp_p(1):
        d.start()
    plan2 = _plan2()

    def p2_body(p, carry):
        @pl.when(p > 0)
        def _():
            for d in cp_p(p):
                d.wait()

        causal = col <= row + HQ
        never = p > NP
        jobs = staging(p, p, never)
        sched = _Sched(never, plan2, jobs)
        mm = sched.mm

        r0 = pl.multiple_of(p * TQ, TQ)

        prods = {}

        def project(kind, j, n, lhs, rhs):
            got = prods.setdefault((kind, j), {})
            for m in ORDER[len(got):len(got) + n]:
                g = _steps()
                k = next(g)
                for e in range(7):
                    k = g.send(mm((kind, j, 7 * len(got) + e), part(lhs, 7 * m + k), rhs(7 * m + k)))
                    if e < 6 or len(got) < 6:
                        yield
                got[m] = k
            if len(got) < 7:
                return None
            c = _combine(lambda m: got[m])
            return [[c[(rg & 2) + (cg >> 1)][2 * (rg & 1) + (cg & 1)] for rg in range(4)]
                    for cg in range(4)]

        def pair(ref, rows):
            return lambda k: jnp.concatenate([ref[k, sr, rows, :] for sr in range(2)], axis=1)

        def x_rows(b, n):
            return lambda k: jnp.concatenate([jnp.concatenate(
                [xq[k, b + j, pl.ds(16 * sr, 16), :] for sr in range(2)], axis=1)
                for j in range(n)], axis=0)

        def proj_b(kind, n, lhs, w, dst, off):
            c = yield from project(kind, 0, n, lhs, pair(w, slice(None)))
            for cg in range(4 * (c is not None)):
                for rg in range(4):
                    for cc in range(2):
                        dst[2 * cg + cc, pl.ds(off + (PAD + rg * QQ), QQ), :] = (
                            c[cg][rg][:, cc * 128:(cc + 1) * 128])

        def proj_bv():
            for cc in range(8):
                vb[cc, pl.ds(0, PAD), :] = vb[cc, pl.ds(TQ, PAD), :]
            return proj_b("bv", 7, x_rows(p, 1), wv49, vb, 0)

        def proj_bo(n):
            list(proj_b("bo", n, pair(ob49, slice(None)), wob49, qk_b, r0))

        def local_qk(rb, k, gate):
            rz = pl.multiple_of((p + _zero(p, k)) * TQ, TQ)
            q = [qk_b[cc, pl.ds(rz + (PAD + rb * RB), RB), :] for cc in range(8)]
            q[0] = gate(q[0])
            for w in range(LG * k, LG * k + LG):
                t = _fold([q[cc] * qk_b[8 + cc, pl.ds(r0 + (PAD + rb * RB - DIL * w), RB), :]
                           for cc in range(8)], jnp.add)
                t = t + pltpu.roll(t, 64, 1)
                t = t + jnp.where(odd, pltpu.roll(t, 1, 1), pltpu.roll(t, 127, 1))
                t = t * (DB ** -0.5 * LOG2E)
                if rb == 0 and w:
                    t = jnp.where(rowi + r0 >= DIL * w, t, NEG)
                lg_s[w, pl.ds(rb * RB, RB), :] = t
            return [], 1, lambda: pltpu.bitcast(lg_s[w, blk(2 * rb + _zero(p, 0), 8), :], U32)

        def local_sm(rb, e, gate):
            rows = pl.ds(rb * RB + SMR * e, SMR)
            lg = [gate(lg_s[w, rows, :]) for w in range(WIN)]
            m = _tree(lg, jnp.maximum)
            ps = [jnp.exp2(t - m) for t in lg]
            l = _tree(ps, jnp.add)
            r = pl.reciprocal(l, approx=True)
            r = r * (2.0 - l * r)
            for w in range(WIN):
                pr_s[w, rows, :] = ps[w] * r
            return [], 2, lambda: pltpu.bitcast(pr_s[0, blk(2 * rb + e + _zero(p, 0), 8), :], U32)

        def local_pv(rb, k, gate):
            rows = pl.ds(rb * RB, RB)
            ps = [pr_s[w + _zero(p, k), rows, :] for w in range(WIN)]
            ps[0] = gate(ps[0])
            o = [_fold([ps[w] * vb[cc, pl.ds(PAD + rb * RB - DIL * w, RB), :] for w in range(WIN)],
                       jnp.add) for cc in (k, k + 4)]
            for e in range(2):
                o_s[k + 4 * e, rows, :] = o[e]
            return [], 0, lambda: pltpu.bitcast(o_s[k, blk(2 * rb + _zero(p, 0), 8), :], U32)

        def o_sums(m, cc, r, gate):
            res = [_ops49(_lhs7, [[gate(o_s[
                2 * (2 * (q & 1) + (e & 1)) + cc + _zero(p, m),
                pl.ds(QQ * (2 * (q >> 1) + (e >> 1)) + 16 * r + par, 8, stride=2), :])
                for e in range(4)] for q in range(4)], m) for par in range(2)]
            for n, (lo, hi) in enumerate(zip(*res)):
                ob49[7 * m + n, cc, pl.ds(8 * r, 8), :] = _join(lo, hi)
            return [], 0, lambda: ob49[7 * m, cc, blk(r + _zero(p, 0), 8), :]

        jobs["os"] = [part(o_sums, m, cc, r) for r in range(2) for cc in range(2) for m in range(7)]
        order = list(range(0, 8, 2)) + list(range(1, 8, 2))
        jobs["lo"] = []
        for k in range(len(order) + SML):
            for f, d, n in ((local_sm, SML, RB // SMR), (local_qk, 0, 8 // LG)):
                if 0 <= k - d < len(order):
                    jobs["lo"] += [part(f, order[k - d], e) for e in range(n)]
        jobs["lv"] = [part(local_pv, rb, e) for rb in order for e in range(4)]

        def out_weights(m, r, gate):
            ww = [[gate(wo_r[(p & 1) + _zero(p, m),
                             pl.ds((2 * (q >> 1) + (e >> 1)) * HQ + 8 * r, 8),
                             pl.ds((2 * (q & 1) + (e & 1)) * 128, 128)])
                   for e in range(4)] for q in range(4)]
            rows = blk(8 * (p >> 1) + r, 8)
            extra = jobs["sc"].pop(0)(gate)[0] if jobs["sc"] else []
            for n, w in enumerate(_words49(_rhs7, ww, m)):
                if n < len(extra):
                    w = jnp.where(never, extra[n], w)
                wo49[7 * m + n, p & 1, rows, :] = w
            return [], 0, lambda: wo49[7 * m + _zero(p, 0), p & 1, rows, :]

        jobs["wo"] = [part(out_weights, m, r) for m in range(7) for r in range(8)]

        ks, vs, qs = {}, {}, {}
        done = {}

        def blocks(c, scale, pack):
            c = [[pack(t * scale(cg)) for t in c[cg]] for cg in range(4)]
            return [[jnp.concatenate([t[16 * e:16 * e + 16] for t in c[cg]], axis=0)
                     for e in range(2)] for cg in range(4)]

        def proj_kv(j, n):
            c = yield from project("kv", j, n, lambda k: jnp.concatenate(
                [cq[k, 2 * j], cq[k, 2 * j + 1]], axis=0), lambda k: wkv[k])
            if c is not None:
                c = blocks(c, lambda cg: ups[cg][:1], _riffle)
                for cg in range(4):
                    for e in range(2):
                        (vs, ks)[cg >> 1][(cg & 1, 2 * j + e)] = c[cg][e]

        def proj_q(g, n):
            c = yield from project("q", g, n, x_rows(4 * g + 2 * (p & 1), 2), lambda k: wq49[k])
            if c is not None:
                c = blocks(c, lambda cg: QSCALE, _pack)
                for h in range(2):
                    for e in range(2):
                        old = qn[h, g, e]
                        for b in range(2):
                            qs[(h, 4 * g + 2 * b + e)] = jnp.where((p & 1) == b, c[h][e], old)
                        qn[h, g, e] = c[2 + h][e]

        def halves(d, h, js):
            return jnp.concatenate([d[(h, j >> 1)][QQ * (j & 1):QQ * (j & 1) + QQ] for j in js],
                                   axis=0)

        def late(x, y, op):
            return jnp.concatenate([x[:HQ], op(x[HQ:], y)], axis=0)

        def unit(h, i):
            return halves(qs, h, (2 * (i & ~1) + (i & 1), 2 * (i | 1) + (i & 1)))

        def first(i):
            t = jnp.concatenate([mm(("kq", h, i), halves(ks, h, (0,)), unit(h, i), NT)
                                 for h in range(2)], axis=0).T
            keep = [col < HQ, col >= HQ]
            top = [col <= row, causal & keep[1]] if i == 0 else keep
            return [jnp.concatenate([jnp.where(a, t[:HQ], NEG), jnp.where(b, t[HQ:], NEG)], axis=0)
                    for a, b in zip(top, keep)]

        def qk(h, i, dep):
            off = 1 - (i & 1)
            q = unit(h, i)
            if dep is not None:
                q = jnp.where(never, done[(h, dep)], q)
            exf = lambda: mm(("qx", h, i), q[QQ:], halves(ks, h, (off + 2 * i, off + 2 * i + 1)), NT)
            ex = None if EXO else exf()
            ch = []
            if i:
                ch = _lane_chunks(mm(("qk", h, i), q, halves(ks, h, range(off, off + 2 * i)),
                                     NT, 512))
                ch[-1] = jnp.concatenate([jnp.where(causal, ch[-1][:HQ], NEG), ch[-1][HQ:]],
                                         axis=0)
            ex = exf() if EXO else ex
            return ch, jnp.where(causal, ex, NEG)

        def softmax_pv(h, i, ch, ex):
            off = 1 - (i & 1)
            m = jnp.max(late(_fold(ch, jnp.maximum), ex, jnp.maximum), axis=1, keepdims=True)
            pe = jnp.exp2(ex - m[HQ:])
            ps = [jnp.exp2(c - m) for c in ch]
            lp = late(ps[0], pe, jnp.add)
            for j in range(1, len(ch)):
                lp = lp + ps[j]
                if TIE and (j % TIE == TIE - 1 or j == len(ch) - 1):
                    ps[j] = jnp.where(never, lp, ps[j])
            pb = jnp.concatenate(ps, axis=1).astype(BF16)
            vv = [halves(vs, h, range(off, off + 2 * i))] if i else []
            v0 = [halves(vs, e, (0,)) for e in range(2 * off)]
            vv = jnp.concatenate(v0 + vv if LF else vv + v0, axis=0)
            oef = lambda: mm(("px", h, i), pe.astype(BF16), halves(vs, h, (off + 2 * i, off + 2 * i + 1)))
            oe = None if PXO else oef()
            o = mm(("pv", h, i), pb, vv)
            o = late(o, oef() if PXO else oe, jnp.add)
            if i >= LDEP:
                lp = jnp.where(never, o, lp)
            l = jnp.sum(lp, axis=1, keepdims=True)
            r = pl.reciprocal(l, approx=True)
            r = r * (2.0 - l * r)
            cn = _pack(o * r)
            done[(h, i)] = cn
            if FA <= i < NQ - 1:
                if i + 3 < NQ:
                    site = ("kv", (i + 1) // 2 + 1, KVS * ((i + 1) & 1) + (F0, FD)[h])
                else:
                    site = ("bo", 0, 7 * (i + 3 - NQ) * BOP[0] + 8 * h)
                sched.pending.setdefault(site, []).append(cn)
            for e in range(2):
                ctx[2 * p + h, pl.ds(((i & ~1) + e) * HQ + QQ * (i & 1), QQ), :] = (
                    cn[QQ * e:QQ * e + QQ])

        head = dict(bv=proj_bv(), kv=proj_kv(0, 7), q=proj_q(0, 7))
        for site in _head():
            next(head[site[0]], None)
        lead = {}
        for i in range(NQ):
            dep = i - DEP if DEP <= i < FA + DEP else None
            for k in range(i, i + VL + 1):
                if k < NQ and not k & 1 and k not in lead and (0, k) in qs:
                    lead[k] = first(k)
            sx = [qk(h, i, dep) for h in range(2)]
            if i + 2 < NQ:
                list(proj_kv(i // 2 + 1, 7 if i & 1 else KVS // 7))
                if i < 6:
                    list(proj_q(i // 2 + 1, 7 if i & 1 else QS // 7))
            else:
                proj_bo(BOP[i + 2 - NQ])
            for h in range(2):
                c0 = [lead[i][h]] if i in lead else []
                softmax_pv(h, i, c0 + sx[h][0] if LF else sx[h][0] + c0, sx[h][1])
        proj_bo(BOP[2])
        sched.finish()
        for d in cp_p(p + 2):
            d.start()
        return carry

    jax.lax.fori_loop(0, NP, p2_body, 0)

    cp_gw().wait()
    gw = gw_ref[...].astype(F32)
    plan3 = _plan3()
    cab = (ca0, ca1)

    def p3_body(i, carry):
        r0 = pl.multiple_of(i * TO, TO)
        h0 = pl.multiple_of(i * (TO // 2), TO // 2)
        never = i > S

        def ctx_words(m, u, r, n):
            return [[ctx[4 * u + 2 * (q & 1) + (e & 1),
                         pl.ds(h0 + _zero(i, m) * 8 + ((2 * (q >> 1) + (e >> 1)) * QQ + r), n), :]
                     for e in range(4)] for q in range(4)]

        def operands(k, u, r, gate):
            m = ORDER[k]
            cw = [[gate(w) for w in q] for q in ctx_words(m, u, r, 8)]
            for n, w in enumerate(_words49(_lhs7, cw, m)):
                if not (m in (2, 3) and n in (2, 3)):
                    cab[k & 1][n, pl.ds(r, 8), pl.ds(u * 128, 128)] = w
            return [], 0, lambda: cab[k & 1][_zero(i, 0), pl.ds(r, 8), pl.ds(u * 128, 128)]

        def gate_rows(r, gate):
            gs = _fold([_bf(gate(xs_u[j, pl.ds(h0 + r, 8), :])).astype(F32) * gw[j:j + 1]
                        for j in range(8)], jnp.add)
            g = jax.nn.sigmoid(jnp.sum(gs, axis=1, keepdims=True))
            g_s[pl.ds(2 * r, 16), :] = jnp.broadcast_to(g, (16, 128))
            return [], 0, lambda: pltpu.bitcast(g_s[blk(r // 4 + _zero(i, 0), 8), :], U32)

        pr = {}

        def mix(q, e, cc, gate):
            off = (2 * (q >> 1) + (e >> 1)) * HQ
            ch = 4 * cc + 2 * (q & 1) + (e & 1)
            a = _combine(lambda m: pr.get(m, pr[2])[e][:, cc * 128:(cc + 1) * 128])[q]
            g = gate(g_s[pl.ds(off, HQ), :])
            b = qk_b[ch, pl.ds(r0 + (PAD + off), HQ), :]
            out_s[pl.ds(r0 + off, HQ), pl.ds(ch * 128, 128)] = (g * a + (1.0 - g) * b).astype(BF16)
            return [], 0, lambda: pltpu.bitcast(
                out_s[blk(i * (TO // 16) + off // 16 + _zero(i, 0), 16), pl.ds(ch * 128, 128)], U32)

        sched = _Sched(never, plan3, dict(
            a=[part(operands, k, u, r) for k in range(1, 7) for u in range(HA // 4)
               for r in range(0, QQ, 8)],
            g=[part(gate_rows, r) for r in range(0, TO // 2, 8)],
            m=[part(mix, q, e, cc) for q in (1, 2, 0) for e in range(4) for cc in range(2)]))
        first = [[_words49(_lhs7, ctx_words(ORDER[0], u, 0, QQ), ORDER[0])[n]
                  for u in range(HA // 4)] for n in range(7)]

        def inner(m, n):
            k = ORDER.index(m)
            res = []
            for e in range(2):
                us = range(4 * e, 4 * e + 4)
                if m in (2, 3) and n in (2, 3):
                    lhs = jnp.concatenate([ctx_words(m, u, 0, QQ)[3 * (m - 2)][3 * (n - 2)]
                                           for u in us], axis=1)
                elif k == 0:
                    lhs = jnp.concatenate([first[n][u] for u in us], axis=1)
                else:
                    lhs = lambda: cab[k & 1][n, :, pl.ds(e * 512, 512)]
                rhs = jnp.concatenate([wo49[7 * m + n, cc, pl.ds(e * 256, 256), :]
                                       for cc in range(2)], axis=1)
                res.append(sched.mm((k, 2 * ORDER.index(n) + e), lhs, rhs))
                if (k, 2 * ORDER.index(n) + e) == (6, P3D):
                    for d in cp_out(i, 0):
                        d.start()
            return res[0] + res[1]

        for m in ORDER:
            pr[m] = _combine(lambda n: inner(m, n))
        sched.finish()
        for e in (1, 2, 0, 3):
            for cc in range(2):
                mix(3, e, cc, lambda x: x)
        for d in cp_out(i, 1):
            d.start()
        return carry

    jax.lax.fori_loop(0, S // TO, p3_body, 0)
    for d in cp_p(NP) + cp_p(NP + 1):
        d.wait()
    for i in range(S // TO):
        for d in cp_out(i, 0) + cp_out(i, 1):
            d.wait()


@jax.jit
def pallas_gated_mix__compressed_kv_cla__sliding_local_dilated__prompt_kernel(
    A_x: jax.Array,
    A_c_kv: jax.Array,
    A_w_q: jax.Array,
    A_w_uk: jax.Array,
    A_w_uv: jax.Array,
    A_w_o: jax.Array,
    B_x: jax.Array,
    B_wqkv: jax.Array,
    B_wo: jax.Array,
    gate_w: jax.Array,
):
    del B_x
    any_spec = pl.BlockSpec(memory_space=pl.ANY)
    out = pl.pallas_call(
        _kernel,
        in_specs=[any_spec] * 9,
        out_specs=any_spec,
        out_shape=jax.ShapeDtypeStruct((S, M), BF16),
        scratch_shapes=[
            pltpu.VMEM((9, S // 2, 128), U32),
            pltpu.VMEM((2, HQ, M), U32),
            pltpu.VMEM((2, HQ, DC), U32),
            pltpu.VMEM((2, 128, M), BF16),
            pltpu.VMEM((2, 4, 16, M), BF16),
            pltpu.VMEM((2, 4, 16, M), U32),
            pltpu.VMEM((3, 2 * DC, 128), U32),
            pltpu.VMEM((4, M, 128), U32),
            pltpu.VMEM((2, 2 * DA, M // 2), U32),
            pltpu.VMEM((8, 64, 128), U32),
            pltpu.VMEM((49, NQ, 32, 128), U32),
            pltpu.VMEM((49, NQ, 16, 128), U32),
            pltpu.VMEM((49, 2, M // 8, 128), U32),
            pltpu.VMEM((49, 2, M // 8, 128), U32),
            pltpu.VMEM((49, 2, NP * QQ, 128), U32),
            pltpu.VMEM((49, HQ, 128), U32),
            pltpu.VMEM((49, TQ, 128), U32),
            pltpu.VMEM((4, 8, 128), F32),
            pltpu.VMEM((4, DC // SCR * 8 + 16, 128), jnp.int32),
            pltpu.VMEM((2, 4, 2, HQ, 128), U32),
            pltpu.VMEM((16, S + PAD, 128), F32),
            pltpu.VMEM((8, TQ + PAD, 128), F32),
            pltpu.VMEM((WIN, TQ, 128), F32),
            pltpu.VMEM((WIN, TQ, 128), F32),
            pltpu.VMEM((8, TQ, 128), F32),
            pltpu.VMEM((49, 2, 16, 128), U32),
            pltpu.VMEM((HA, S // 2, 128), U32),
            pltpu.VMEM((7, QQ, M), U32),
            pltpu.VMEM((7, QQ, M), U32),
            pltpu.VMEM((TO, 128), F32),
            pltpu.VMEM((S, M), BF16),
            pltpu.VMEM((8, 128), BF16),
            pltpu.SemaphoreType.DMA((2,)),
            pltpu.SemaphoreType.DMA((2,)),
            pltpu.SemaphoreType.DMA((5,)),
        ],
        compiler_params=pltpu.CompilerParams(vmem_limit_bytes=120 * 1024 * 1024,
                                             disable_bounds_checks=True),
    )(
        A_x.reshape(S, M),
        A_c_kv.reshape(S, DC),
        A_w_q,
        A_w_uk,
        A_w_uv,
        A_w_o.reshape(HA * DA, M),
        B_wqkv.reshape(2, M // 2, 3 * M),
        B_wo.reshape(HB // 2, 2, DB, M),
        gate_w.reshape(8, 128),
    )
    return out.reshape(1, S, M)
```

```python
import functools

import jax
import jax.numpy as jnp
import jax.experimental.pallas as pl
import jax.experimental.pallas.tpu as pltpu

F32 = jnp.float32
BF16 = jnp.bfloat16
U32 = jnp.uint32

S = 2048
M = 1024
HA = 32
DA = 128
DC = 512
HB = 32
DB = 32
WIN = 8
DIL = 2
PAD = 16
LOG2E = 1.4426950408889634
NEG = -1e9

TQ = 128
HQ = TQ // 2
QQ = TQ // 4
NQ = S // TQ
NP = HA // 2
RB = 16
TO = 256

P0S = ((0, 0, 1024), (1, 0, 1024), (0, 1024, 1024), (1, 1024, 768), (1, 1792, 128), (1, 1920, 128))
P0W = 2
P0A = 75
P0T = 16
P0N = 104
P1S = ((0, 0, 2048), (1, 0, 1536), (1, 1536, 384), (1, 1920, 128))
P1A = 60
P1N = 108
XN = 28
XQ = 50
XS = 24
BOP = (2, 3, 2)
KVS = 28
QS = 35
LX = 16
QST = 2
SK = 3
LG = 1
SMR = 16
SML = 1
SCR = 32
LN = 92
LA = 16
BS = 2
LP = ("kv", 1, 8)
BX = 8
BE = 42
DEP = 2
FA = 6
F0 = 0
FD = 8
TIE = 4
LDEP = 6
VL = 1
IV = 3
KE = 4
KT = 42
HP = 53
EXO = 1
PXO = 1
LF = 1
P3S = 3
P3E = 12
P3M = 6
P3D = 8

NN = (((1,), (0,)), ((), ()))
NT = (((1,), (1,)), ((), ()))


def _head():
    rest = [(kind, 0, k) for kind in ("kv", "q") for k in range(49)]
    out, room = [], 0
    for k in range(49):
        out.append(("bv", 0, k))
        room += IV
        while rest and room >= 1 + (rest[0][0] == "q"):
            room -= 1 + (rest[0][0] == "q")
            out.append(rest.pop(0))
    return out + rest


def _plan2():
    plan = {}

    def put(name, count, start, until):
        plan.setdefault(start, []).extend([(name, until)] * count)

    def after_qk(i):
        if i >= NQ - 2:
            return ("bo", 0, 7 * (i - NQ + 2) * BOP[0] + BX)
        return ("kv", i // 2 + 1, KVS * (i & 1) + LX)

    def fill(name, count, sites):
        for start, room, until in sites:
            n = min(count, room - len(plan.get(start, ())))
            put(name, n, start, until)
            count -= n
        assert count == 0, (name, count)

    def qk_sites(lo, hi):
        return [(("qk", h, i), max(i + 1 - h * SK, 0), after_qk(i))
                for i in range(lo, hi) for h in range(2)]

    def q_sites(g, lo, hi, until):
        return [(("q", g, k), 1, until) for k in range(lo, hi, QST)]

    ticks = [t for t in _head() if t[0] != "kv" or t[2] & 1 == 0]
    for name, site in zip(_spread(["lo"] * (64 // LG + 128 // SMR), LN), ticks[LA:]):
        put(name, 1, site, LP)
    host = [(t, 1, ticks[HP]) for t in ticks[:LA:BS]]
    early = []
    for g in range(1, 4):
        early += q_sites(g, 0, QS - 4, after_qk(2 * g - 1))
        early += qk_sites(2 * g - 1, 2 * g)
        early += q_sites(g, QS, 45, after_qk(2 * g))
        early += qk_sites(2 * g, 2 * g + 1)
    fill("lv", 32, early)
    fill("wo", 56, host + early)
    fill("os", 28, early + qk_sites(7, 14))
    fill("qw", 112, qk_sites(7, 14))
    for k in range(KE):
        put("kv", 1, ("bo", 0, KT + k), None)
    fill("kv", 56 - KE, qk_sites(14, 16) + [(("bo", 0, k), 1, ("bo", 0, BE))
                                       for k in range(7 * BOP[0], 35)])
    return plan


def _planx():
    names = _spread(["qw"] * (XQ - XS) + ["kv", "qw"] * 56 + ["qw"] * (56 - XQ), 8 * XN)
    return {k: [(n, None) for n in names[8 * k:8 * k + 8]] for k in range(XN)}


def _spread(names, ticks):
    out = [None] * ticks
    for k, name in enumerate(names):
        out[k * ticks // len(names)] = name
    return out


def _plan1(segs, lo, step, count, extra):
    end = len(segs) - 2
    ticks = [k for k in range(lo, end) for _ in range(segs[k][2] // step)][:count]
    n = len(ticks) * (P0A if lo else P1A) // 100
    names = _spread(["x"] * 28 + ["c"] * 14 + ["o"] * 14, n) + _spread(["v"] * 14, len(ticks) - n)
    free = [k for k, name in enumerate(names) if name is None]
    for k in free[len(free) - extra:]:
        names[k] = "qw"
    plan = {}
    for k, name in zip(ticks, names):
        plan.setdefault(k, []).append((name, None if name == "qw" else end))
    return plan


def _plan3():
    plan = {}
    for k in range(6):
        lo = P3S if k == 0 else 0
        extra = ["g"] * 8 if k in (1, 2) else []
        names = _spread(["a"] * 32 + extra, 4 * (P3E - lo))
        for d in range(lo, P3E):
            plan[(k, d)] = [(n, (k + 1, 0)) for n in names[4 * (d - lo):4 * (d - lo) + 4]]
    names = _spread(["m"] * 24, 4 * P3M)
    for d in range(P3M):
        plan[(6, d)] = [(n, (6, P3D)) for n in names[4 * d:4 * d + 4]]
    return plan


_STAGES = ((2, 4), (1, 3), (0, 2), (0, 6), (0, 1))


def _permute8(cols):
    cols = list(cols)
    lane = jax.lax.broadcasted_iota(jnp.int32, cols[0].shape, 1)
    for va, lb in _STAGES:
        lo = (lane & (1 << lb)) == 0
        sh = 1 << lb
        idx = [i for i in range(8) if not (i >> va) & 1]
        if lb == 6:
            rr = [pltpu.roll(jnp.where(lo, cols[i | (1 << va)], cols[i]), 64, 1) for i in idx]
            for i, r in zip(idx, rr):
                a, b = cols[i], cols[i | (1 << va)]
                cols[i] = jnp.where(lo, a, r)
                cols[i | (1 << va)] = jnp.where(lo, r, b)
        else:
            rb = [pltpu.roll(cols[i | (1 << va)], sh, 1) for i in idx]
            ra = [pltpu.roll(cols[i], 128 - sh, 1) for i in idx]
            for i, xa, xb in zip(idx, ra, rb):
                a, b = cols[i], cols[i | (1 << va)]
                cols[i] = jnp.where(lo, a, xb)
                cols[i | (1 << va)] = jnp.where(lo, xa, b)
    return cols


def _pack(x):
    return pltpu.bitcast(x.astype(BF16), U32)


def _bf(x):
    return pltpu.bitcast(x, BF16)


def _split(w):
    return (pltpu.bitcast(w << 16, F32), pltpu.bitcast(w & jnp.uint32(0xFFFF0000), F32))


def _join(lo, hi):
    return pltpu.bitcast(pltpu.pack_elementwise([lo, hi], packed_dtype=BF16), U32)


def _riffle(x):
    return jnp.concatenate([_join(x[r:r + 16], x[r + 16:r + 32]) for r in range(0, x.shape[0], 32)],
                           axis=0)


def _lhs7(a11, a12, a21, a22):
    return [a11 + a22, a21 + a22, a11, a22, a11 + a12, a21 - a11, a12 - a22]


def _rhs7(b11, b12, b21, b22):
    return [b11 + b22, b11, b12 - b22, b21 - b11, b22, b11 + b12, b21 + b22]


def _steps():
    add = functools.partial(jax.tree.map, jnp.add)
    sub = functools.partial(jax.tree.map, jnp.subtract)
    m2 = yield 2
    m3 = yield 3
    m4 = yield 4
    c12 = add(m2, m4)
    t11 = sub(m3, m4)
    m1 = yield 1
    c21 = add(m1, m3)
    t22 = sub(m2, m1)
    m0 = yield 0
    t11 = add(t11, m0)
    t22 = add(t22, m0)
    c11 = add(t11, (yield 6))
    yield c11, c12, c21, add(t22, (yield 5))


def _combine(mm):
    g = _steps()
    k = next(g)
    for _ in range(7):
        k = g.send(mm(k))
    return k


ORDER = (2, 3, 4, 1, 0, 6, 5)


def _zero(i, m):
    return i >> (8 + m)


def _merge(vals):
    return _fold([v[r:r + 8, c:c + 128] for v in vals for r in range(0, v.shape[0], 8)
                  for c in range(0, v.shape[1], 128)], jnp.bitwise_or)


def _gate(never, g):
    def gate(x):
        t = jnp.tile(pltpu.bitcast(g, x.dtype), (x.shape[0] // 8, x.shape[1] // 128))
        return jnp.where(never, t, x)
    return gate


def _tie(never, x, deps):
    if not deps:
        return x
    top = jnp.where(never, _merge(deps), x[:8, :128])
    if x.shape[1] > 128:
        top = jnp.concatenate([top, x[:8, 128:]], axis=1)
    return jnp.concatenate([top, x[8:]], axis=0)


class _Sched:
    def __init__(self, never, plan, jobs):
        self.never, self.plan, self.jobs, self.pending = never, plan, jobs, {}

    def mm(self, site, a, b, dims=NN, width=128, step=32):
        deps = [d() if callable(d) else d for d in self.pending.pop(site, ())]
        a = a() if callable(a) else a
        tie = functools.partial(_tie, self.never, deps=deps)
        a, b = (_bf(tie(a)), _bf(b)) if a.dtype == U32 else (a, _bf(tie(b)))
        out = jax.lax.dot_general(a, b, dims, preferred_element_type=F32)
        per = out.shape[0] // step
        last = {}
        for k, (name, until) in enumerate(self.plan.get(site, ())):
            if name is not None:
                r, c = step * (k % per), min(width * (k // per), out.shape[1] - 128)
                vals, tag, stored = self.jobs[name].pop(0)(
                    _gate(self.never, out[r:r + 8, c:c + 128]))
                self.pending.setdefault(until, []).extend(vals)
                last[(name, tag, until)] = stored
        for (_, _, until), stored in last.items():
            if stored is not None:
                self.pending[until].append(stored)
        return out

    def finish(self):
        self.pending.pop(None, None)
        assert not any(self.jobs.values()) and not any(self.pending.values())


def _ops49(fn, blocks, m):
    return fn(*[fn(*[blocks[q][e] for q in range(4)])[m] for e in range(4)])


def _words49(fn, words, m):
    halves = [[_split(w) for w in q] for q in words]
    lo = _ops49(fn, [[h[0] for h in q] for q in halves], m)
    hi = _ops49(fn, [[h[1] for h in q] for q in halves], m)
    return [_join(a, b) for a, b in zip(lo, hi)]


def _fold(xs, op):
    acc = xs[0]
    for x in xs[1:]:
        acc = op(acc, x)
    return acc


def _tree(xs, op):
    while len(xs) > 1:
        xs = [op(a, b) for a, b in zip(xs[::2], xs[1::2])]
    return xs[0]


def _lane_chunks(x):
    return [x[:, j * 128:(j + 1) * 128] for j in range(x.shape[1] // 128)]


def _kernel(x_hbm, c_hbm, wq_hbm, wuk_hbm, wuv_hbm, wo_hbm, wqkv_hbm, wob_hbm, gw_hbm,
            out_hbm,
            xs_u, x_r, c_r, w_r, wv_r, wob_r, wkv_r, wq_r, wo_r,
            wperm, xq, cq, wv49, wob49, wo49, wkv, wq49, ups, sc_s, qn,
            qk_b, vb, lg_s, pr_s, o_s, ob49, ctx, ca0, ca1, g_s, out_s, gw_ref,
            sem_x, sem_p, sem_a):
    x_u = x_hbm.bitcast(U32)
    c_u = c_hbm.bitcast(U32)
    wo_u = wo_hbm.bitcast(U32)
    wq_u = wq_hbm.bitcast(U32)
    wuk_u = wuk_hbm.bitcast(U32)
    wuv_u = wuv_hbm.bitcast(U32)
    wob_u = wob_hbm.bitcast(U32)
    part = functools.partial

    def blk(j, n):
        return pl.ds(pl.multiple_of(j * n, n), n)

    def strip(j):
        return blk(j, 128)

    def cp_x(t, sem):
        k = (t + 1) >> 1
        return pltpu.make_async_copy(x_u.at[blk(t & 1, S // 4), strip(jnp.minimum(k, 7))],
                                     xs_u.at[jnp.minimum(k, 8), blk(t & 1, S // 4), :], sem)

    def cp_w(t, sem):
        u = t - 2 * (t >> 4)
        u = u - 2 * (u >> 4)
        return pltpu.make_async_copy(wqkv_hbm.at[u >> 3, strip((u >> 1) & 3), blk(u & 1, M)],
                                     w_r.at[u & 1], sem)

    def cp_wob(t, sem):
        b = (t + 1) >> 1
        c = jnp.minimum(b, 7)
        return tuple(pltpu.make_async_copy(
            wob_u.at[:, c & 1, 4 * (2 * (t & 1) + j) + (c & 2) + (c >> 2), :],
            wob_r.at[b & 1, 2 * (t & 1) + j], sem) for j in range(2))

    def group(t, sem1=None):
        sem = sem_x.at[t & 1]
        u = t - 2 * (t >> 4)
        return (
            cp_x(t, sem if sem1 is None else sem1),
            cp_w(t + 1, sem),
            pltpu.make_async_copy(x_u.at[blk(u, HQ), :], x_r.at[u & 1], sem),
            pltpu.make_async_copy(c_u.at[blk(u, HQ), :], c_r.at[u & 1], sem),
        ) + cp_wob(t, sem) + tuple(
            pltpu.make_async_copy(wqkv_hbm.at[e >> 1, blk(16 * (e & 1) + u, 16), pl.ds(2 * M, M)],
                                  wv_r.at[u & 1, e], sem) for e in range(4))

    def piece(t):
        late = t >> 4
        pq = (t >> 3) + late
        pk = (t >> 3) & 1
        u = (t & 15) + 2 * late
        sem = sem_a.at[3 + late]
        return (
            pltpu.make_async_copy(wo_u.at[blk(u, 16), pl.ds(0, M // 2)],
                                  wo_r.at[late, blk(u, 16), :], sem),
            pltpu.make_async_copy(wq_u.at[strip(t & 7), pq, :], wq_r.at[pq, strip(t & 7), :], sem),
            pltpu.make_async_copy(wq_u.at[blk(u, 64), 2, :], wq_r.at[2 + late, blk(u, 64), :], sem),
            pltpu.make_async_copy(wuk_u.at[blk(t & 7, 64), pk, :],
                                  wkv_r.at[1 - pk + late, blk(8 + (t & 7), 64), :], sem),
            pltpu.make_async_copy(wuv_u.at[blk(t & 7, 64), pk, :],
                                  wkv_r.at[1 - pk + late, blk(t & 7, 64), :], sem),
        )

    def cp_wq(p, sem):
        return pltpu.make_async_copy(wq_u.at[:, jnp.minimum(p, NP - 1), :], wq_r.at[p & 3], sem)

    def cp_p(g):
        slot = g & 1
        p = jnp.minimum(g + 1, NP - 1)
        o = jnp.minimum(g, NP - 1)
        sem = sem_p.at[slot]
        return (
            pltpu.make_async_copy(wo_u.at[blk(o >> 1, 2 * DA), blk(o & 1, M // 2)],
                                  wo_r.at[slot], sem),
            pltpu.make_async_copy(wuk_u.at[:, p, :], wkv_r.at[slot, pl.ds(DC, DC), :], sem),
            pltpu.make_async_copy(wuv_u.at[:, p, :], wkv_r.at[slot, pl.ds(0, DC), :], sem),
            cp_wq(g + 2, sem),
        )

    def cp_gw():
        return pltpu.make_async_copy(gw_hbm, gw_ref, sem_a.at[0])

    def cp_out(i, late):
        def cp(rows, cols):
            return pltpu.make_async_copy(out_s.at[rows, cols], out_hbm.at[rows, cols], sem_a.at[1])

        low = [cp(blk(2 * i + 1, TO // 2), pl.ds(512 * cc + 256 * late, 256)) for cc in range(2)]
        return low if late else [cp(blk(2 * i, TO // 2), pl.ds(0, M))] + low

    cp_w(0, sem_a.at[1]).start()
    group0, group1 = group(0, sem_a.at[2]), group(1)
    group0 = (group0[0], cp_x(-1, sem_x.at[0])) + group0[1:] + cp_wob(-1, sem_x.at[0])
    for d in group0 + group1[:1] + group1[2:]:
        d.start()

    for cc in range(8):
        qk_b[8 + cc, pl.ds(0, PAD), :] = jnp.zeros((PAD, 128), F32)
        vb[cc, pl.ds(TQ, PAD), :] = jnp.zeros((PAD, 128), F32)

    def stage_first(t, lo=0, hi=8):
        w = _permute8(_lane_chunks(pltpu.bitcast(w_r[t & 1], U32)))
        for cc in range(lo, hi):
            wperm[cc] = w[cc]

    def p1_step(t, peel, extra=None):
        if not peel:
            for d in group(t):
                d.wait()

        def act_sums(src, dst, ns, m, sr, r, gate):
            cw = [[gate(src[(t & 1) + _zero(t, m), pl.ds(32 * (q >> 1) + 16 * (e >> 1) + 8 * r, 8),
                            pl.ds(((2 * (q & 1) + (e & 1)) * ns + sr) * 128, 128)])
                   for e in range(4)] for q in range(4)]
            for n, w in enumerate(_words49(_lhs7, cw, m)):
                dst[7 * m + n, t, pl.ds(16 * sr + 8 * r, 8), :] = w
            return [], 0, lambda: dst[7 * m + _zero(t, 0), t, pl.ds(16 * sr + 8 * r, 8), :]

        wv = []

        def load_wv():
            wv.extend(_permute8(_lane_chunks(jnp.concatenate(
                [pltpu.bitcast(wv_r[t & 1, e], U32) for e in range(4)], axis=0))))

        def w_sums(src, dst, m, cc, gate):
            ww = [[gate(src(m, 2 * (q >> 1) + (e >> 1), 2 * (2 * (q & 1) + (e & 1)) + cc))
                   for e in range(4)] for q in range(4)]
            for n, w in enumerate(_words49(_rhs7, ww, m)):
                dst[7 * m + n, cc, blk(t, 8), :] = w
            return [], 0, lambda: dst[7 * m + _zero(t, 0), cc, blk(t, 8), :]

        def v_src(m, rq, ch):
            return wv[ch][8 * rq:8 * rq + 8]

        def o_src(m, rq, ch):
            return wob_r[((t >> 1) & 1) + _zero(t, m), rq, blk(t & 1, 8), pl.ds(128 * ch, 128)]

        segs, step = (P0S, P0T) if peel else (P1S, 32)
        sched = _Sched(t > 99, _plan1(segs, P0W * peel, step, P0N if peel else P1N,
                                     XS if extra else 0), dict(
            extra or {},
            x=[part(act_sums, x_r, xq, 2, m, sr, r)
               for m in range(7) for sr in range(2) for r in range(2)],
            c=[part(act_sums, c_r, cq, 1, m, 0, r) for m in range(7) for r in range(2)],
            v=[part(w_sums, v_src, wv49, m, cc) for m in range(7) for cc in range(2)],
            o=[part(w_sums, o_src, wob49, m, cc) for m in range(7) for cc in range(2)]))

        first = t < 2
        for k, (half, r0, n) in enumerate(segs):
            if k == P0W * peel:
                if peel:
                    for d in group0[1:]:
                        d.wait()
                    group1[1].start()
                load_wv()
            w = jnp.concatenate([wperm[4 * half + cc] for cc in range(4)], axis=1)
            r = sched.mm(k, xs_u[t >> 1, pl.ds(r0 // 2, n // 2), :], w, step=step)
            if k == len(segs) - 1 and not extra:
                sched.finish()
                stage_first(t + 1)
                d = group(t + 2)
                e = piece(t + 2)
                d = d[2:6] + e[:1] + d[6:] + d[:2] + e[1:]
                for d in d + (piece(0) + piece(1) + (cp_gw(),) if peel else ()):
                    d.start()
            for cc in range(4):
                sl = (8 * (t & 1) + 4 * half + cc, pl.ds(PAD + r0, n), slice(None))
                new = r[:, cc * 128:(cc + 1) * 128]
                qk_b[sl] = new if peel else jnp.where(first, 0.0, qk_b[sl]) + new
        return t

    zero = jnp.max(vb[0, pl.ds(TQ, 8), :]).astype(jnp.int32)
    cp_w(0, sem_a.at[1]).wait()
    stage_first(0, 0, 4)
    group0[0].wait()
    stage_first(0, 4, 8)
    p1_step(zero, True)
    last = jax.lax.fori_loop(1, 15, lambda t, c: p1_step(t, False), 0)
    for t in range(16):
        for d in piece(t):
            d.wait()

    row = jax.lax.broadcasted_iota(jnp.int32, (HQ, TQ), 0)
    col = jax.lax.broadcasted_iota(jnp.int32, (HQ, TQ), 1)
    col = (col & ~31) | ((col & 1) << 4) | ((col & 31) >> 1)
    rowi = jax.lax.broadcasted_iota(jnp.int32, (RB, 128), 0)
    odd = (jax.lax.broadcasted_iota(jnp.int32, (RB, 128), 1) & 1) == 1
    QSCALE = DA ** -0.5 * LOG2E

    def pair_rows(src, slot, r0, n, gate):
        return [_split(gate(src[slot, pl.ds(r0 + par, n // 2, stride=2), :])) for par in range(2)]

    def staging(g, z, never):
        ns = DC // SCR

        def scales(n1, k, gate):
            res = []
            for h in range(2):
                if k < ns:
                    w = gate(wkv_r[g & 1, pl.ds(n1 * DC + k * SCR, SCR), :])
                    w = pltpu.bitcast(w, jnp.int32) & (0x7F80 << (16 * h))
                else:
                    w = gate(sc_s[2 * n1 + h, pl.ds(0, 8 * ns), :])
                e = _tree([w[r:r + 8] for r in range(0, w.shape[0], 8)], jnp.maximum)
                if k == ns:
                    e = pltpu.bitcast(e << (16 - 16 * h), F32)
                    e = jnp.max(e, axis=0, keepdims=True)
                    e = jnp.clip(pltpu.bitcast(e, jnp.int32), 1 << 23, 253 << 23)
                    e = jnp.broadcast_to(e, (8, 128))
                    sc_s[2 * n1 + h, pl.ds(8 * ns + 8, 8), :] = (254 << 23) - e
                sc_s[2 * n1 + h, pl.ds(8 * k, 8), :] = e
                res.append(pltpu.bitcast(e, U32))
            return res, 0, lambda: pltpu.bitcast(sc_s[2 * n1, blk(k + _zero(z, 0), 8), :], U32)

        def rhs49(dst, tiles, scale, m, r, extra=()):
            res = [_ops49(_rhs7,
                          [[scale(tiles[2 * (q >> 1) + (e >> 1)][q & 1][par][e & 1],
                                  2 * (q & 1) + (e & 1)) for e in range(4)] for q in range(4)],
                          m) for par in range(2)]
            for k, (lo, hi) in enumerate(zip(*res)):
                w = _join(lo, hi)
                if k < len(extra):
                    w = jnp.where(never, extra[k], w)
                dst[7 * m + k, pl.ds(8 * r, 8), :] = w

        def kv(m, r, gate):
            if m == 0 and r == 0:
                for k in range(4):
                    ups[k] = pltpu.bitcast(gate(sc_s[k, pl.ds(8 * ns, 8), :]), F32)
            down = [pltpu.bitcast(sc_s[k + _zero(z, m), pl.ds(8 * ns + 8, 8), :], F32)
                    for k in range(4)]
            tiles = [[pair_rows(wkv_r, (g & 1) + _zero(z, m), n1 * DC + kt * 128 + 16 * r, 16, gate)
                      for n1 in range(2)] for kt in range(4)]
            rhs49(wkv, tiles, lambda w, k: w * down[k], m, r)
            return [], 0, lambda: wkv[7 * m, blk(r + _zero(z, 0), 8), :]

        def qw(m, r, gate):
            tiles = [[pair_rows(wq_r, ((g + 1 + n1) & 3) + _zero(z, m), kt * 256 + 16 * r, 16, gate)
                      for n1 in range(2)] for kt in range(4)]
            rhs49(wq49, tiles, lambda w, k: w, m, r, sc.pop(0)(gate)[0] if sc else ())
            return [], 0, lambda: wq49[7 * m, blk(r + _zero(z, 0), 8), :]

        sc = [part(scales, n1, k) for k in range(ns + 1) for n1 in range(2)]
        return dict(sc=sc,
                    kv=[part(kv, m, r) for m in range(7) for r in range(8)],
                    qw=[part(qw, m, r) for m in range(7) for r in range(16)])

    sched = _Sched(last > 99, _planx(), staging(-1, last, last > 99))
    p1_step(last + 1, False, sched.jobs)
    w0 = pair_rows(wq_r, 0, 0, M, lambda x: x)
    w0 = [_join(w0[0][h], w0[1][h]) for h in range(2)]
    for g in range(4):
        for e in range(2):
            for h in range(2):
                q = [sched.mm(8 * g + 4 * e + 2 * h + k, jnp.concatenate(
                    [xs_u[4 * k + u, pl.ds((4 * g + 2 + e) * HQ, HQ), :] for u in range(4)], axis=1),
                    w0[h][256 * k:256 * k + 256], step=16) for k in range(2)]
                qn[h, g, e] = _pack((q[0] + q[1]) * QSCALE)
    sched.finish()
    for d in group(16) + piece(16) + (cp_gw(),):
        d.wait()
    for d in cp_p(1):
        d.start()
    plan2 = _plan2()

    def p2_body(p, carry):
        @pl.when(p > 0)
        def _():
            for d in cp_p(p):
                d.wait()

        causal = col <= row + HQ
        never = p > NP
        jobs = staging(p, p, never)
        sched = _Sched(never, plan2, jobs)
        mm = sched.mm

        r0 = pl.multiple_of(p * TQ, TQ)

        prods = {}

        def project(kind, j, n, lhs, rhs):
            got = prods.setdefault((kind, j), {})
            for m in ORDER[len(got):len(got) + n]:
                g = _steps()
                k = next(g)
                for e in range(7):
                    k = g.send(mm((kind, j, 7 * len(got) + e), part(lhs, 7 * m + k), rhs(7 * m + k)))
                    if e < 6 or len(got) < 6:
                        yield
                got[m] = k
            if len(got) < 7:
                return None
            c = _combine(lambda m: got[m])
            return [[c[(rg & 2) + (cg >> 1)][2 * (rg & 1) + (cg & 1)] for rg in range(4)]
                    for cg in range(4)]

        def pair(ref, rows):
            return lambda k: jnp.concatenate([ref[k, sr, rows, :] for sr in range(2)], axis=1)

        def x_rows(b, n):
            return lambda k: jnp.concatenate([jnp.concatenate(
                [xq[k, b + j, pl.ds(16 * sr, 16), :] for sr in range(2)], axis=1)
                for j in range(n)], axis=0)

        def proj_b(kind, n, lhs, w, dst, off):
            c = yield from project(kind, 0, n, lhs, pair(w, slice(None)))
            for cg in range(4 * (c is not None)):
                for rg in range(4):
                    for cc in range(2):
                        dst[2 * cg + cc, pl.ds(off + (PAD + rg * QQ), QQ), :] = (
                            c[cg][rg][:, cc * 128:(cc + 1) * 128])

        def proj_bv():
            for cc in range(8):
                vb[cc, pl.ds(0, PAD), :] = vb[cc, pl.ds(TQ, PAD), :]
            return proj_b("bv", 7, x_rows(p, 1), wv49, vb, 0)

        def proj_bo(n):
            list(proj_b("bo", n, pair(ob49, slice(None)), wob49, qk_b, r0))

        def local_qk(rb, k, gate):
            rz = pl.multiple_of((p + _zero(p, k)) * TQ, TQ)
            q = [qk_b[cc, pl.ds(rz + (PAD + rb * RB), RB), :] for cc in range(8)]
            q[0] = gate(q[0])
            for w in range(LG * k, LG * k + LG):
                t = _fold([q[cc] * qk_b[8 + cc, pl.ds(r0 + (PAD + rb * RB - DIL * w), RB), :]
                           for cc in range(8)], jnp.add)
                t = t + pltpu.roll(t, 64, 1)
                t = t + jnp.where(odd, pltpu.roll(t, 1, 1), pltpu.roll(t, 127, 1))
                t = t * (DB ** -0.5 * LOG2E)
                if rb == 0 and w:
                    t = jnp.where(rowi + r0 >= DIL * w, t, NEG)
                lg_s[w, pl.ds(rb * RB, RB), :] = t
            return [], 1, lambda: pltpu.bitcast(lg_s[w, blk(2 * rb + _zero(p, 0), 8), :], U32)

        def local_sm(rb, e, gate):
            rows = pl.ds(rb * RB + SMR * e, SMR)
            lg = [gate(lg_s[w, rows, :]) for w in range(WIN)]
            m = _tree(lg, jnp.maximum)
            ps = [jnp.exp2(t - m) for t in lg]
            l = _tree(ps, jnp.add)
            r = pl.reciprocal(l, approx=True)
            r = r * (2.0 - l * r)
            for w in range(WIN):
                pr_s[w, rows, :] = ps[w] * r
            return [], 2, lambda: pltpu.bitcast(pr_s[0, blk(2 * rb + e + _zero(p, 0), 8), :], U32)

        def local_pv(rb, k, gate):
            rows = pl.ds(rb * RB, RB)
            ps = [pr_s[w + _zero(p, k), rows, :] for w in range(WIN)]
            ps[0] = gate(ps[0])
            o = [_fold([ps[w] * vb[cc, pl.ds(PAD + rb * RB - DIL * w, RB), :] for w in range(WIN)],
                       jnp.add) for cc in (k, k + 4)]
            for e in range(2):
                o_s[k + 4 * e, rows, :] = o[e]
            return [], 0, lambda: pltpu.bitcast(o_s[k, blk(2 * rb + _zero(p, 0), 8), :], U32)

        def o_sums(m, cc, r, gate):
            res = [_ops49(_lhs7, [[gate(o_s[
                2 * (2 * (q & 1) + (e & 1)) + cc + _zero(p, m),
                pl.ds(QQ * (2 * (q >> 1) + (e >> 1)) + 16 * r + par, 8, stride=2), :])
                for e in range(4)] for q in range(4)], m) for par in range(2)]
            for n, (lo, hi) in enumerate(zip(*res)):
                ob49[7 * m + n, cc, pl.ds(8 * r, 8), :] = _join(lo, hi)
            return [], 0, lambda: ob49[7 * m, cc, blk(r + _zero(p, 0), 8), :]

        jobs["os"] = [part(o_sums, m, cc, r) for r in range(2) for cc in range(2) for m in range(7)]
        order = list(range(0, 8, 2)) + list(range(1, 8, 2))
        jobs["lo"] = []
        for k in range(len(order) + SML):
            for f, d, n in ((local_sm, SML, RB // SMR), (local_qk, 0, 8 // LG)):
                if 0 <= k - d < len(order):
                    jobs["lo"] += [part(f, order[k - d], e) for e in range(n)]
        jobs["lv"] = [part(local_pv, rb, e) for rb in order for e in range(4)]

        def out_weights(m, r, gate):
            ww = [[gate(wo_r[(p & 1) + _zero(p, m),
                             pl.ds((2 * (q >> 1) + (e >> 1)) * HQ + 8 * r, 8),
                             pl.ds((2 * (q & 1) + (e & 1)) * 128, 128)])
                   for e in range(4)] for q in range(4)]
            rows = blk(8 * (p >> 1) + r, 8)
            extra = jobs["sc"].pop(0)(gate)[0] if jobs["sc"] else []
            for n, w in enumerate(_words49(_rhs7, ww, m)):
                if n < len(extra):
                    w = jnp.where(never, extra[n], w)
                wo49[7 * m + n, p & 1, rows, :] = w
            return [], 0, lambda: wo49[7 * m + _zero(p, 0), p & 1, rows, :]

        jobs["wo"] = [part(out_weights, m, r) for m in range(7) for r in range(8)]

        ks, vs, qs = {}, {}, {}
        done = {}

        def blocks(c, scale, pack):
            c = [[pack(t * scale(cg)) for t in c[cg]] for cg in range(4)]
            return [[jnp.concatenate([t[16 * e:16 * e + 16] for t in c[cg]], axis=0)
                     for e in range(2)] for cg in range(4)]

        def proj_kv(j, n):
            c = yield from project("kv", j, n, lambda k: jnp.concatenate(
                [cq[k, 2 * j], cq[k, 2 * j + 1]], axis=0), lambda k: wkv[k])
            if c is not None:
                c = blocks(c, lambda cg: ups[cg][:1], _riffle)
                for cg in range(4):
                    for e in range(2):
                        (vs, ks)[cg >> 1][(cg & 1, 2 * j + e)] = c[cg][e]

        def proj_q(g, n):
            c = yield from project("q", g, n, x_rows(4 * g + 2 * (p & 1), 2), lambda k: wq49[k])
            if c is not None:
                c = blocks(c, lambda cg: QSCALE, _pack)
                for h in range(2):
                    for e in range(2):
                        old = qn[h, g, e]
                        for b in range(2):
                            qs[(h, 4 * g + 2 * b + e)] = jnp.where((p & 1) == b, c[h][e], old)
                        qn[h, g, e] = c[2 + h][e]

        def halves(d, h, js):
            return jnp.concatenate([d[(h, j >> 1)][QQ * (j & 1):QQ * (j & 1) + QQ] for j in js],
                                   axis=0)

        def late(x, y, op):
            return jnp.concatenate([x[:HQ], op(x[HQ:], y)], axis=0)

        def unit(h, i):
            return halves(qs, h, (2 * (i & ~1) + (i & 1), 2 * (i | 1) + (i & 1)))

        def first(i):
            t = jnp.concatenate([mm(("kq", h, i), halves(ks, h, (0,)), unit(h, i), NT)
                                 for h in range(2)], axis=0).T
            keep = [col < HQ, col >= HQ]
            top = [col <= row, causal & keep[1]] if i == 0 else keep
            return [jnp.concatenate([jnp.where(a, t[:HQ], NEG), jnp.where(b, t[HQ:], NEG)], axis=0)
                    for a, b in zip(top, keep)]

        def qk(h, i, dep):
            off = 1 - (i & 1)
            q = unit(h, i)
            if dep is not None:
                q = jnp.where(never, done[(h, dep)], q)
            exf = lambda: mm(("qx", h, i), q[QQ:], halves(ks, h, (off + 2 * i, off + 2 * i + 1)), NT)
            ex = None if EXO else exf()
            ch = []
            if i:
                ch = _lane_chunks(mm(("qk", h, i), q, halves(ks, h, range(off, off + 2 * i)),
                                     NT, 512))
                ch[-1] = jnp.concatenate([jnp.where(causal, ch[-1][:HQ], NEG), ch[-1][HQ:]],
                                         axis=0)
            ex = exf() if EXO else ex
            return ch, jnp.where(causal, ex, NEG)

        def softmax_pv(h, i, ch, ex):
            off = 1 - (i & 1)
            m = jnp.max(late(_fold(ch, jnp.maximum), ex, jnp.maximum), axis=1, keepdims=True)
            pe = jnp.exp2(ex - m[HQ:])
            ps = [jnp.exp2(c - m) for c in ch]
            lp = late(ps[0], pe, jnp.add)
            for j in range(1, len(ch)):
                lp = lp + ps[j]
                if TIE and (j % TIE == TIE - 1 or j == len(ch) - 1):
                    ps[j] = jnp.where(never, lp, ps[j])
            pb = jnp.concatenate(ps, axis=1).astype(BF16)
            vv = [halves(vs, h, range(off, off + 2 * i))] if i else []
            v0 = [halves(vs, e, (0,)) for e in range(2 * off)]
            vv = jnp.concatenate(v0 + vv if LF else vv + v0, axis=0)
            oef = lambda: mm(("px", h, i), pe.astype(BF16), halves(vs, h, (off + 2 * i, off + 2 * i + 1)))
            oe = None if PXO else oef()
            o = mm(("pv", h, i), pb, vv)
            o = late(o, oef() if PXO else oe, jnp.add)
            if i >= LDEP:
                lp = jnp.where(never, o, lp)
            l = jnp.sum(lp, axis=1, keepdims=True)
            r = pl.reciprocal(l, approx=True)
            r = r * (2.0 - l * r)
            cn = _pack(o * r)
            done[(h, i)] = cn
            if FA <= i < NQ - 1:
                if i + 3 < NQ:
                    site = ("kv", (i + 1) // 2 + 1, KVS * ((i + 1) & 1) + (F0, FD)[h])
                else:
                    site = ("bo", 0, 7 * (i + 3 - NQ) * BOP[0] + 8 * h)
                sched.pending.setdefault(site, []).append(cn)
            for e in range(2):
                ctx[2 * p + h, pl.ds(((i & ~1) + e) * HQ + QQ * (i & 1), QQ), :] = (
                    cn[QQ * e:QQ * e + QQ])

        head = dict(bv=proj_bv(), kv=proj_kv(0, 7), q=proj_q(0, 7))
        for site in _head():
            next(head[site[0]], None)
        lead = {}
        for i in range(NQ):
            dep = i - DEP if DEP <= i < FA + DEP else None
            for k in range(i, i + VL + 1):
                if k < NQ and not k & 1 and k not in lead and (0, k) in qs:
                    lead[k] = first(k)
            sx = [qk(h, i, dep) for h in range(2)]
            if i + 2 < NQ:
                list(proj_kv(i // 2 + 1, 7 if i & 1 else KVS // 7))
                if i < 6:
                    list(proj_q(i // 2 + 1, 7 if i & 1 else QS // 7))
            else:
                proj_bo(BOP[i + 2 - NQ])
            for h in range(2):
                c0 = [lead[i][h]] if i in lead else []
                softmax_pv(h, i, c0 + sx[h][0] if LF else sx[h][0] + c0, sx[h][1])
        proj_bo(BOP[2])
        sched.finish()
        for d in cp_p(p + 2):
            d.start()
        return carry

    jax.lax.fori_loop(0, NP, p2_body, 0)

    gw = gw_ref[...].astype(F32)
    plan3 = _plan3()
    cab = (ca0, ca1)

    def p3_body(i, carry):
        r0 = pl.multiple_of(i * TO, TO)
        h0 = pl.multiple_of(i * (TO // 2), TO // 2)
        never = i > S

        def ctx_words(m, u, r, n):
            return [[ctx[4 * u + 2 * (q & 1) + (e & 1),
                         pl.ds(h0 + _zero(i, m) * 8 + ((2 * (q >> 1) + (e >> 1)) * QQ + r), n), :]
                     for e in range(4)] for q in range(4)]

        def operands(k, u, r, gate):
            m = ORDER[k]
            cw = [[gate(w) for w in q] for q in ctx_words(m, u, r, 8)]
            for n, w in enumerate(_words49(_lhs7, cw, m)):
                if not (m in (2, 3) and n in (2, 3)):
                    cab[k & 1][n, pl.ds(r, 8), pl.ds(u * 128, 128)] = w
            return [], 0, lambda: cab[k & 1][_zero(i, 0), pl.ds(r, 8), pl.ds(u * 128, 128)]

        def gate_rows(r, gate):
            gs = _fold([_bf(gate(xs_u[j, pl.ds(h0 + r, 8), :])).astype(F32) * gw[j:j + 1]
                        for j in range(8)], jnp.add)
            g = jax.nn.sigmoid(jnp.sum(gs, axis=1, keepdims=True))
            g_s[pl.ds(2 * r, 16), :] = jnp.broadcast_to(g, (16, 128))
            return [], 0, lambda: pltpu.bitcast(g_s[blk(r // 4 + _zero(i, 0), 8), :], U32)

        pr = {}

        def mix(q, e, cc, gate):
            off = (2 * (q >> 1) + (e >> 1)) * HQ
            ch = 4 * cc + 2 * (q & 1) + (e & 1)
            a = _combine(lambda m: pr.get(m, pr[2])[e][:, cc * 128:(cc + 1) * 128])[q]
            g = gate(g_s[pl.ds(off, HQ), :])
            b = qk_b[ch, pl.ds(r0 + (PAD + off), HQ), :]
            out_s[pl.ds(r0 + off, HQ), pl.ds(ch * 128, 128)] = (g * a + (1.0 - g) * b).astype(BF16)
            return [], 0, lambda: pltpu.bitcast(
                out_s[blk(i * (TO // 16) + off // 16 + _zero(i, 0), 16), pl.ds(ch * 128, 128)], U32)

        sched = _Sched(never, plan3, dict(
            a=[part(operands, k, u, r) for k in range(1, 7) for u in range(HA // 4)
               for r in range(0, QQ, 8)],
            g=[part(gate_rows, r) for r in range(0, TO // 2, 8)],
            m=[part(mix, q, e, cc) for q in (1, 2, 0) for e in range(4) for cc in range(2)]))
        first = [[_words49(_lhs7, ctx_words(ORDER[0], u, 0, QQ), ORDER[0])[n]
                  for u in range(HA // 4)] for n in range(7)]

        def inner(m, n):
            k = ORDER.index(m)
            res = []
            for e in range(2):
                us = range(4 * e, 4 * e + 4)
                if m in (2, 3) and n in (2, 3):
                    lhs = jnp.concatenate([ctx_words(m, u, 0, QQ)[3 * (m - 2)][3 * (n - 2)]
                                           for u in us], axis=1)
                elif k == 0:
                    lhs = jnp.concatenate([first[n][u] for u in us], axis=1)
                else:
                    lhs = lambda: cab[k & 1][n, :, pl.ds(e * 512, 512)]
                rhs = jnp.concatenate([wo49[7 * m + n, cc, pl.ds(e * 256, 256), :]
                                       for cc in range(2)], axis=1)
                res.append(sched.mm((k, 2 * ORDER.index(n) + e), lhs, rhs))
                if (k, 2 * ORDER.index(n) + e) == (6, P3D):
                    for d in cp_out(i, 0):
                        d.start()
            return res[0] + res[1]

        for m in ORDER:
            pr[m] = _combine(lambda n: inner(m, n))
        sched.finish()
        for e in (1, 2, 0, 3):
            for cc in range(2):
                mix(3, e, cc, lambda x: x)
        for d in cp_out(i, 1):
            d.start()
        return carry

    jax.lax.fori_loop(0, S // TO, p3_body, 0)
    for d in cp_p(NP) + cp_p(NP + 1):
        d.wait()
    for i in range(S // TO):
        for d in cp_out(i, 0) + cp_out(i, 1):
            d.wait()


@jax.jit
def pallas_gated_mix__compressed_kv_cla__sliding_local_dilated__prompt_kernel(
    A_x: jax.Array,
    A_c_kv: jax.Array,
    A_w_q: jax.Array,
    A_w_uk: jax.Array,
    A_w_uv: jax.Array,
    A_w_o: jax.Array,
    B_x: jax.Array,
    B_wqkv: jax.Array,
    B_wo: jax.Array,
    gate_w: jax.Array,
):
    del B_x
    any_spec = pl.BlockSpec(memory_space=pl.ANY)
    out = pl.pallas_call(
        _kernel,
        in_specs=[any_spec] * 9,
        out_specs=any_spec,
        out_shape=jax.ShapeDtypeStruct((S, M), BF16),
        scratch_shapes=[
            pltpu.VMEM((9, S // 2, 128), U32),
            pltpu.VMEM((2, HQ, M), U32),
            pltpu.VMEM((2, HQ, DC), U32),
            pltpu.VMEM((2, 128, M), BF16),
            pltpu.VMEM((2, 4, 16, M), BF16),
            pltpu.VMEM((2, 4, 16, M), U32),
            pltpu.VMEM((3, 2 * DC, 128), U32),
            pltpu.VMEM((4, M, 128), U32),
            pltpu.VMEM((2, 2 * DA, M // 2), U32),
            pltpu.VMEM((8, 64, 128), U32),
            pltpu.VMEM((49, NQ, 32, 128), U32),
            pltpu.VMEM((49, NQ, 16, 128), U32),
            pltpu.VMEM((49, 2, M // 8, 128), U32),
            pltpu.VMEM((49, 2, M // 8, 128), U32),
            pltpu.VMEM((49, 2, NP * QQ, 128), U32),
            pltpu.VMEM((49, HQ, 128), U32),
            pltpu.VMEM((49, TQ, 128), U32),
            pltpu.VMEM((4, 8, 128), F32),
            pltpu.VMEM((4, DC // SCR * 8 + 16, 128), jnp.int32),
            pltpu.VMEM((2, 4, 2, HQ, 128), U32),
            pltpu.VMEM((16, S + PAD, 128), F32),
            pltpu.VMEM((8, TQ + PAD, 128), F32),
            pltpu.VMEM((WIN, TQ, 128), F32),
            pltpu.VMEM((WIN, TQ, 128), F32),
            pltpu.VMEM((8, TQ, 128), F32),
            pltpu.VMEM((49, 2, 16, 128), U32),
            pltpu.VMEM((HA, S // 2, 128), U32),
            pltpu.VMEM((7, QQ, M), U32),
            pltpu.VMEM((7, QQ, M), U32),
            pltpu.VMEM((TO, 128), F32),
            pltpu.VMEM((S, M), BF16),
            pltpu.VMEM((8, 128), BF16),
            pltpu.SemaphoreType.DMA((2,)),
            pltpu.SemaphoreType.DMA((2,)),
            pltpu.SemaphoreType.DMA((5,)),
        ],
        compiler_params=pltpu.CompilerParams(vmem_limit_bytes=120 * 1024 * 1024,
                                             disable_bounds_checks=True),
    )(
        A_x.reshape(S, M),
        A_c_kv.reshape(S, DC),
        A_w_q,
        A_w_uk,
        A_w_uv,
        A_w_o.reshape(HA * DA, M),
        B_wqkv.reshape(2, M // 2, 3 * M),
        B_wo.reshape(HB // 2, 2, DB, M),
        gate_w.reshape(8, 128),
    )
    return out.reshape(1, S, M)
```

```python
import functools

import jax
import jax.numpy as jnp
import jax.experimental.pallas as pl
import jax.experimental.pallas.tpu as pltpu

F32 = jnp.float32
BF16 = jnp.bfloat16
U32 = jnp.uint32

S = 2048
M = 1024
HA = 32
DA = 128
DC = 512
HB = 32
DB = 32
WIN = 8
DIL = 2
PAD = 16
LOG2E = 1.4426950408889634
NEG = -1e9

TQ = 128
HQ = TQ // 2
QQ = TQ // 4
NQ = S // TQ
NP = HA // 2
RB = 16
TO = 256

P0S = ((0, 0, 1024), (1, 0, 1024), (0, 1024, 1024), (1, 1024, 768), (1, 1792, 128), (1, 1920, 128))
P0W = 2
P0A = 75
P0T = 16
P0N = 104
P1S = ((0, 0, 2048), (1, 0, 1536), (1, 1536, 384), (1, 1920, 128))
P1A = 60
P1N = 108
XN = 28
XQ = 50
XS = 24
BOP = (2, 3, 2)
KVS = 28
QS = 35
LX = 16
QST = 2
SK = 3
LG = 1
SMR = 16
SML = 1
SCR = 32
LN = 92
LA = 16
BS = 2
LP = ("kv", 1, 8)
BX = 8
BE = 42
DEP = 2
FA = 6
F0 = 0
FD = 8
TIE = 4
LDEP = 6
VL = 1
IV = 3
KE = 4
KT = 42
HP = 53
P3S = 3
P3E = 12
P3M = 6
P3D = 8

NN = (((1,), (0,)), ((), ()))
NT = (((1,), (1,)), ((), ()))


def _head():
    rest = [(kind, 0, k) for kind in ("kv", "q") for k in range(49)]
    out, room = [], 0
    for k in range(49):
        out.append(("bv", 0, k))
        room += IV
        while rest and room >= 1 + (rest[0][0] == "q"):
            room -= 1 + (rest[0][0] == "q")
            out.append(rest.pop(0))
    return out + rest


def _plan2():
    plan = {}

    def put(name, count, start, until):
        plan.setdefault(start, []).extend([(name, until)] * count)

    def after_qk(i):
        if i >= NQ - 2:
            return ("bo", 0, 7 * (i - NQ + 2) * BOP[0] + BX)
        return ("kv", i // 2 + 1, KVS * (i & 1) + LX)

    def fill(name, count, sites):
        for start, room, until in sites:
            n = min(count, room - len(plan.get(start, ())))
            put(name, n, start, until)
            count -= n
        assert count == 0, (name, count)

    def qk_sites(lo, hi):
        return [(("qk", h, i), max(i + 1 - h * SK, 0), after_qk(i))
                for i in range(lo, hi) for h in range(2)]

    def q_sites(g, lo, hi, until):
        return [(("q", g, k), 1, until) for k in range(lo, hi, QST)]

    ticks = [t for t in _head() if t[0] != "kv" or t[2] & 1 == 0]
    for name, site in zip(_spread(["lo"] * (64 // LG + 128 // SMR), LN), ticks[LA:]):
        put(name, 1, site, LP)
    host = [(t, 1, ticks[HP]) for t in ticks[:LA:BS]]
    early = []
    for g in range(1, 4):
        early += q_sites(g, 0, QS - 4, after_qk(2 * g - 1))
        early += qk_sites(2 * g - 1, 2 * g)
        early += q_sites(g, QS, 45, after_qk(2 * g))
        early += qk_sites(2 * g, 2 * g + 1)
    fill("lv", 32, early)
    fill("wo", 56, host + early)
    fill("os", 28, early + qk_sites(7, 14))
    fill("qw", 112, qk_sites(7, 14))
    for k in range(KE):
        put("kv", 1, ("bo", 0, KT + k), None)
    fill("kv", 56 - KE, qk_sites(14, 16) + [(("bo", 0, k), 1, ("bo", 0, BE))
                                       for k in range(7 * BOP[0], 35)])
    return plan


def _planx():
    names = _spread(["qw"] * (XQ - XS) + ["kv", "qw"] * 56 + ["qw"] * (56 - XQ), 8 * XN)
    return {k: [(n, None) for n in names[8 * k:8 * k + 8]] for k in range(XN)}


def _spread(names, ticks):
    out = [None] * ticks
    for k, name in enumerate(names):
        out[k * ticks // len(names)] = name
    return out


def _plan1(segs, lo, step, count, extra):
    end = len(segs) - 2
    ticks = [k for k in range(lo, end) for _ in range(segs[k][2] // step)][:count]
    n = len(ticks) * (P0A if lo else P1A) // 100
    names = _spread(["x"] * 28 + ["c"] * 14 + ["o"] * 14, n) + _spread(["v"] * 14, len(ticks) - n)
    free = [k for k, name in enumerate(names) if name is None]
    for k in free[len(free) - extra:]:
        names[k] = "qw"
    plan = {}
    for k, name in zip(ticks, names):
        plan.setdefault(k, []).append((name, None if name == "qw" else end))
    return plan


def _plan3():
    plan = {}
    for k in range(6):
        lo = P3S if k == 0 else 0
        extra = ["g"] * 8 if k in (1, 2) else []
        names = _spread(["a"] * 32 + extra, 4 * (P3E - lo))
        for d in range(lo, P3E):
            plan[(k, d)] = [(n, (k + 1, 0)) for n in names[4 * (d - lo):4 * (d - lo) + 4]]
    names = _spread(["m"] * 24, 4 * P3M)
    for d in range(P3M):
        plan[(6, d)] = [(n, (6, P3D)) for n in names[4 * d:4 * d + 4]]
    return plan


_STAGES = ((2, 4), (1, 3), (0, 2), (0, 6), (0, 1))


def _permute8(cols):
    cols = list(cols)
    lane = jax.lax.broadcasted_iota(jnp.int32, cols[0].shape, 1)
    for va, lb in _STAGES:
        lo = (lane & (1 << lb)) == 0
        sh = 1 << lb
        idx = [i for i in range(8) if not (i >> va) & 1]
        if lb == 6:
            rr = [pltpu.roll(jnp.where(lo, cols[i | (1 << va)], cols[i]), 64, 1) for i in idx]
            for i, r in zip(idx, rr):
                a, b = cols[i], cols[i | (1 << va)]
                cols[i] = jnp.where(lo, a, r)
                cols[i | (1 << va)] = jnp.where(lo, r, b)
        else:
            rb = [pltpu.roll(cols[i | (1 << va)], sh, 1) for i in idx]
            ra = [pltpu.roll(cols[i], 128 - sh, 1) for i in idx]
            for i, xa, xb in zip(idx, ra, rb):
                a, b = cols[i], cols[i | (1 << va)]
                cols[i] = jnp.where(lo, a, xb)
                cols[i | (1 << va)] = jnp.where(lo, xa, b)
    return cols


def _pack(x):
    return pltpu.bitcast(x.astype(BF16), U32)


def _bf(x):
    return pltpu.bitcast(x, BF16)


def _split(w):
    return (pltpu.bitcast(w << 16, F32), pltpu.bitcast(w & jnp.uint32(0xFFFF0000), F32))


def _join(lo, hi):
    return pltpu.bitcast(pltpu.pack_elementwise([lo, hi], packed_dtype=BF16), U32)


def _riffle(x):
    return jnp.concatenate([_join(x[r:r + 16], x[r + 16:r + 32]) for r in range(0, x.shape[0], 32)],
                           axis=0)


def _lhs7(a11, a12, a21, a22):
    return [a11 + a22, a21 + a22, a11, a22, a11 + a12, a21 - a11, a12 - a22]


def _rhs7(b11, b12, b21, b22):
    return [b11 + b22, b11, b12 - b22, b21 - b11, b22, b11 + b12, b21 + b22]


def _steps():
    add = functools.partial(jax.tree.map, jnp.add)
    sub = functools.partial(jax.tree.map, jnp.subtract)
    m2 = yield 2
    m3 = yield 3
    m4 = yield 4
    c12 = add(m2, m4)
    t11 = sub(m3, m4)
    m1 = yield 1
    c21 = add(m1, m3)
    t22 = sub(m2, m1)
    m0 = yield 0
    t11 = add(t11, m0)
    t22 = add(t22, m0)
    c11 = add(t11, (yield 6))
    yield c11, c12, c21, add(t22, (yield 5))


def _combine(mm):
    g = _steps()
    k = next(g)
    for _ in range(7):
        k = g.send(mm(k))
    return k


ORDER = (2, 3, 4, 1, 0, 6, 5)


def _zero(i, m):
    return i >> (8 + m)


def _merge(vals):
    return _fold([v[r:r + 8, c:c + 128] for v in vals for r in range(0, v.shape[0], 8)
                  for c in range(0, v.shape[1], 128)], jnp.bitwise_or)


def _gate(never, g):
    def gate(x):
        t = jnp.tile(pltpu.bitcast(g, x.dtype), (x.shape[0] // 8, x.shape[1] // 128))
        return jnp.where(never, t, x)
    return gate


def _tie(never, x, deps):
    if not deps:
        return x
    top = jnp.where(never, _merge(deps), x[:8, :128])
    if x.shape[1] > 128:
        top = jnp.concatenate([top, x[:8, 128:]], axis=1)
    return jnp.concatenate([top, x[8:]], axis=0)


class _Sched:
    def __init__(self, never, plan, jobs):
        self.never, self.plan, self.jobs, self.pending = never, plan, jobs, {}

    def mm(self, site, a, b, dims=NN, width=128, step=32):
        deps = [d() if callable(d) else d for d in self.pending.pop(site, ())]
        a = a() if callable(a) else a
        tie = functools.partial(_tie, self.never, deps=deps)
        a, b = (_bf(tie(a)), _bf(b)) if a.dtype == U32 else (a, _bf(tie(b)))
        out = jax.lax.dot_general(a, b, dims, preferred_element_type=F32)
        per = out.shape[0] // step
        last = {}
        for k, (name, until) in enumerate(self.plan.get(site, ())):
            if name is not None:
                r, c = step * (k % per), min(width * (k // per), out.shape[1] - 128)
                vals, tag, stored = self.jobs[name].pop(0)(
                    _gate(self.never, out[r:r + 8, c:c + 128]))
                self.pending.setdefault(until, []).extend(vals)
                last[(name, tag, until)] = stored
        for (_, _, until), stored in last.items():
            if stored is not None:
                self.pending[until].append(stored)
        return out

    def finish(self):
        self.pending.pop(None, None)
        assert not any(self.jobs.values()) and not any(self.pending.values())


def _ops49(fn, blocks, m):
    return fn(*[fn(*[blocks[q][e] for q in range(4)])[m] for e in range(4)])


def _words49(fn, words, m):
    halves = [[_split(w) for w in q] for q in words]
    lo = _ops49(fn, [[h[0] for h in q] for q in halves], m)
    hi = _ops49(fn, [[h[1] for h in q] for q in halves], m)
    return [_join(a, b) for a, b in zip(lo, hi)]


def _fold(xs, op):
    acc = xs[0]
    for x in xs[1:]:
        acc = op(acc, x)
    return acc


def _tree(xs, op):
    while len(xs) > 1:
        xs = [op(a, b) for a, b in zip(xs[::2], xs[1::2])]
    return xs[0]


def _lane_chunks(x):
    return [x[:, j * 128:(j + 1) * 128] for j in range(x.shape[1] // 128)]


def _kernel(x_hbm, c_hbm, wq_hbm, wuk_hbm, wuv_hbm, wo_hbm, wqkv_hbm, wob_hbm, gw_hbm,
            out_hbm,
            xs_u, x_r, c_r, w_r, wv_r, wob_r, wkv_r, wq_r, wo_r,
            wperm, xq, cq, wv49, wob49, wo49, wkv, wq49, ups, sc_s, qn,
            qk_b, vb, lg_s, pr_s, o_s, ob49, ctx, ca0, ca1, g_s, out_s, gw_ref,
            sem_x, sem_p, sem_a):
    x_u = x_hbm.bitcast(U32)
    c_u = c_hbm.bitcast(U32)
    wo_u = wo_hbm.bitcast(U32)
    wq_u = wq_hbm.bitcast(U32)
    wuk_u = wuk_hbm.bitcast(U32)
    wuv_u = wuv_hbm.bitcast(U32)
    wob_u = wob_hbm.bitcast(U32)
    part = functools.partial

    def blk(j, n):
        return pl.ds(pl.multiple_of(j * n, n), n)

    def strip(j):
        return blk(j, 128)

    def cp_x(t, sem):
        k = (t + 1) >> 1
        return pltpu.make_async_copy(x_u.at[blk(t & 1, S // 4), strip(jnp.minimum(k, 7))],
                                     xs_u.at[jnp.minimum(k, 8), blk(t & 1, S // 4), :], sem)

    def cp_w(t, sem):
        u = t - 2 * (t >> 4)
        u = u - 2 * (u >> 4)
        return pltpu.make_async_copy(wqkv_hbm.at[u >> 3, strip((u >> 1) & 3), blk(u & 1, M)],
                                     w_r.at[u & 1], sem)

    def cp_wob(t, sem):
        b = (t + 1) >> 1
        c = jnp.minimum(b, 7)
        return tuple(pltpu.make_async_copy(
            wob_u.at[:, c & 1, 4 * (2 * (t & 1) + j) + (c & 2) + (c >> 2), :],
            wob_r.at[b & 1, 2 * (t & 1) + j], sem) for j in range(2))

    def group(t, sem1=None):
        sem = sem_x.at[t & 1]
        u = t - 2 * (t >> 4)
        return (
            cp_x(t, sem if sem1 is None else sem1),
            cp_w(t + 1, sem),
            pltpu.make_async_copy(x_u.at[blk(u, HQ), :], x_r.at[u & 1], sem),
            pltpu.make_async_copy(c_u.at[blk(u, HQ), :], c_r.at[u & 1], sem),
        ) + cp_wob(t, sem) + tuple(
            pltpu.make_async_copy(wqkv_hbm.at[e >> 1, blk(16 * (e & 1) + u, 16), pl.ds(2 * M, M)],
                                  wv_r.at[u & 1, e], sem) for e in range(4))

    def piece(t):
        late = t >> 4
        pq = (t >> 3) + late
        pk = (t >> 3) & 1
        u = (t & 15) + 2 * late
        sem = sem_a.at[3 + late]
        return (
            pltpu.make_async_copy(wo_u.at[blk(u, 16), pl.ds(0, M // 2)],
                                  wo_r.at[late, blk(u, 16), :], sem),
            pltpu.make_async_copy(wq_u.at[strip(t & 7), pq, :], wq_r.at[pq, strip(t & 7), :], sem),
            pltpu.make_async_copy(wq_u.at[blk(u, 64), 2, :], wq_r.at[2 + late, blk(u, 64), :], sem),
            pltpu.make_async_copy(wuk_u.at[blk(t & 7, 64), pk, :],
                                  wkv_r.at[1 - pk + late, blk(8 + (t & 7), 64), :], sem),
            pltpu.make_async_copy(wuv_u.at[blk(t & 7, 64), pk, :],
                                  wkv_r.at[1 - pk + late, blk(t & 7, 64), :], sem),
        )

    def cp_wq(p, sem):
        return pltpu.make_async_copy(wq_u.at[:, jnp.minimum(p, NP - 1), :], wq_r.at[p & 3], sem)

    def cp_p(g):
        slot = g & 1
        p = jnp.minimum(g + 1, NP - 1)
        o = jnp.minimum(g, NP - 1)
        sem = sem_p.at[slot]
        return (
            pltpu.make_async_copy(wo_u.at[blk(o >> 1, 2 * DA), blk(o & 1, M // 2)],
                                  wo_r.at[slot], sem),
            pltpu.make_async_copy(wuk_u.at[:, p, :], wkv_r.at[slot, pl.ds(DC, DC), :], sem),
            pltpu.make_async_copy(wuv_u.at[:, p, :], wkv_r.at[slot, pl.ds(0, DC), :], sem),
            cp_wq(g + 2, sem),
        )

    def cp_gw():
        return pltpu.make_async_copy(gw_hbm, gw_ref, sem_a.at[0])

    def cp_out(i, late):
        def cp(rows, cols):
            return pltpu.make_async_copy(out_s.at[rows, cols], out_hbm.at[rows, cols], sem_a.at[1])

        low = [cp(blk(2 * i + 1, TO // 2), pl.ds(512 * cc + 256 * late, 256)) for cc in range(2)]
        return low if late else [cp(blk(2 * i, TO // 2), pl.ds(0, M))] + low

    cp_w(0, sem_a.at[1]).start()
    group0, group1 = group(0, sem_a.at[2]), group(1)
    group0 = (group0[0], cp_x(-1, sem_x.at[0])) + group0[1:] + cp_wob(-1, sem_x.at[0])
    for d in group0 + group1[:1] + group1[2:]:
        d.start()

    for cc in range(8):
        qk_b[8 + cc, pl.ds(0, PAD), :] = jnp.zeros((PAD, 128), F32)
        vb[cc, pl.ds(TQ, PAD), :] = jnp.zeros((PAD, 128), F32)

    def stage_first(t, lo=0, hi=8):
        w = _permute8(_lane_chunks(pltpu.bitcast(w_r[t & 1], U32)))
        for cc in range(lo, hi):
            wperm[cc] = w[cc]

    def p1_step(t, peel, extra=None):
        if not peel:
            for d in group(t):
                d.wait()

        def act_sums(src, dst, ns, m, sr, r, gate):
            cw = [[gate(src[(t & 1) + _zero(t, m), pl.ds(32 * (q >> 1) + 16 * (e >> 1) + 8 * r, 8),
                            pl.ds(((2 * (q & 1) + (e & 1)) * ns + sr) * 128, 128)])
                   for e in range(4)] for q in range(4)]
            for n, w in enumerate(_words49(_lhs7, cw, m)):
                dst[7 * m + n, t, pl.ds(16 * sr + 8 * r, 8), :] = w
            return [], 0, lambda: dst[7 * m + _zero(t, 0), t, pl.ds(16 * sr + 8 * r, 8), :]

        wv = []

        def load_wv():
            wv.extend(_permute8(_lane_chunks(jnp.concatenate(
                [pltpu.bitcast(wv_r[t & 1, e], U32) for e in range(4)], axis=0))))

        def w_sums(src, dst, m, cc, gate):
            ww = [[gate(src(m, 2 * (q >> 1) + (e >> 1), 2 * (2 * (q & 1) + (e & 1)) + cc))
                   for e in range(4)] for q in range(4)]
            for n, w in enumerate(_words49(_rhs7, ww, m)):
                dst[7 * m + n, cc, blk(t, 8), :] = w
            return [], 0, lambda: dst[7 * m + _zero(t, 0), cc, blk(t, 8), :]

        def v_src(m, rq, ch):
            return wv[ch][8 * rq:8 * rq + 8]

        def o_src(m, rq, ch):
            return wob_r[((t >> 1) & 1) + _zero(t, m), rq, blk(t & 1, 8), pl.ds(128 * ch, 128)]

        segs, step = (P0S, P0T) if peel else (P1S, 32)
        sched = _Sched(t > 99, _plan1(segs, P0W * peel, step, P0N if peel else P1N,
                                     XS if extra else 0), dict(
            extra or {},
            x=[part(act_sums, x_r, xq, 2, m, sr, r)
               for m in range(7) for sr in range(2) for r in range(2)],
            c=[part(act_sums, c_r, cq, 1, m, 0, r) for m in range(7) for r in range(2)],
            v=[part(w_sums, v_src, wv49, m, cc) for m in range(7) for cc in range(2)],
            o=[part(w_sums, o_src, wob49, m, cc) for m in range(7) for cc in range(2)]))

        first = t < 2
        for k, (half, r0, n) in enumerate(segs):
            if k == P0W * peel:
                if peel:
                    for d in group0[1:]:
                        d.wait()
                    group1[1].start()
                load_wv()
            w = jnp.concatenate([wperm[4 * half + cc] for cc in range(4)], axis=1)
            r = sched.mm(k, xs_u[t >> 1, pl.ds(r0 // 2, n // 2), :], w, step=step)
            if k == len(segs) - 1 and not extra:
                sched.finish()
                stage_first(t + 1)
                d = group(t + 2)
                e = piece(t + 2)
                d = d[2:6] + e[:1] + d[6:] + d[:2] + e[1:]
                for d in d + (piece(0) + piece(1) + (cp_gw(),) if peel else ()):
                    d.start()
            for cc in range(4):
                sl = (8 * (t & 1) + 4 * half + cc, pl.ds(PAD + r0, n), slice(None))
                new = r[:, cc * 128:(cc + 1) * 128]
                qk_b[sl] = new if peel else jnp.where(first, 0.0, qk_b[sl]) + new
        return t

    zero = jnp.max(vb[0, pl.ds(TQ, 8), :]).astype(jnp.int32)
    cp_w(0, sem_a.at[1]).wait()
    stage_first(0, 0, 4)
    group0[0].wait()
    stage_first(0, 4, 8)
    p1_step(zero, True)
    last = jax.lax.fori_loop(1, 15, lambda t, c: p1_step(t, False), 0)
    for t in range(16):
        for d in piece(t):
            d.wait()

    row = jax.lax.broadcasted_iota(jnp.int32, (HQ, TQ), 0)
    col = jax.lax.broadcasted_iota(jnp.int32, (HQ, TQ), 1)
    col = (col & ~31) | ((col & 1) << 4) | ((col & 31) >> 1)
    rowi = jax.lax.broadcasted_iota(jnp.int32, (RB, 128), 0)
    odd = (jax.lax.broadcasted_iota(jnp.int32, (RB, 128), 1) & 1) == 1
    QSCALE = DA ** -0.5 * LOG2E

    def pair_rows(src, slot, r0, n, gate):
        return [_split(gate(src[slot, pl.ds(r0 + par, n // 2, stride=2), :])) for par in range(2)]

    def staging(g, z, never):
        ns = DC // SCR

        def scales(n1, k, gate):
            res = []
            for h in range(2):
                if k < ns:
                    w = gate(wkv_r[g & 1, pl.ds(n1 * DC + k * SCR, SCR), :])
                    w = pltpu.bitcast(w, jnp.int32) & (0x7F80 << (16 * h))
                else:
                    w = gate(sc_s[2 * n1 + h, pl.ds(0, 8 * ns), :])
                e = _tree([w[r:r + 8] for r in range(0, w.shape[0], 8)], jnp.maximum)
                if k == ns:
                    e = pltpu.bitcast(e << (16 - 16 * h), F32)
                    e = jnp.max(e, axis=0, keepdims=True)
                    e = jnp.clip(pltpu.bitcast(e, jnp.int32), 1 << 23, 253 << 23)
                    e = jnp.broadcast_to(e, (8, 128))
                    sc_s[2 * n1 + h, pl.ds(8 * ns + 8, 8), :] = (254 << 23) - e
                sc_s[2 * n1 + h, pl.ds(8 * k, 8), :] = e
                res.append(pltpu.bitcast(e, U32))
            return res, 0, lambda: pltpu.bitcast(sc_s[2 * n1, blk(k + _zero(z, 0), 8), :], U32)

        def rhs49(dst, tiles, scale, m, r, extra=()):
            res = [_ops49(_rhs7,
                          [[scale(tiles[2 * (q >> 1) + (e >> 1)][q & 1][par][e & 1],
                                  2 * (q & 1) + (e & 1)) for e in range(4)] for q in range(4)],
                          m) for par in range(2)]
            for k, (lo, hi) in enumerate(zip(*res)):
                w = _join(lo, hi)
                if k < len(extra):
                    w = jnp.where(never, extra[k], w)
                dst[7 * m + k, pl.ds(8 * r, 8), :] = w

        def kv(m, r, gate):
            if m == 0 and r == 0:
                for k in range(4):
                    ups[k] = pltpu.bitcast(gate(sc_s[k, pl.ds(8 * ns, 8), :]), F32)
            down = [pltpu.bitcast(sc_s[k + _zero(z, m), pl.ds(8 * ns + 8, 8), :], F32)
                    for k in range(4)]
            tiles = [[pair_rows(wkv_r, (g & 1) + _zero(z, m), n1 * DC + kt * 128 + 16 * r, 16, gate)
                      for n1 in range(2)] for kt in range(4)]
            rhs49(wkv, tiles, lambda w, k: w * down[k], m, r)
            return [], 0, lambda: wkv[7 * m, blk(r + _zero(z, 0), 8), :]

        def qw(m, r, gate):
            tiles = [[pair_rows(wq_r, ((g + 1 + n1) & 3) + _zero(z, m), kt * 256 + 16 * r, 16, gate)
                      for n1 in range(2)] for kt in range(4)]
            rhs49(wq49, tiles, lambda w, k: w, m, r, sc.pop(0)(gate)[0] if sc else ())
            return [], 0, lambda: wq49[7 * m, blk(r + _zero(z, 0), 8), :]

        sc = [part(scales, n1, k) for k in range(ns + 1) for n1 in range(2)]
        return dict(sc=sc,
                    kv=[part(kv, m, r) for m in range(7) for r in range(8)],
                    qw=[part(qw, m, r) for m in range(7) for r in range(16)])

    sched = _Sched(last > 99, _planx(), staging(-1, last, last > 99))
    p1_step(last + 1, False, sched.jobs)
    w0 = pair_rows(wq_r, 0, 0, M, lambda x: x)
    w0 = [_join(w0[0][h], w0[1][h]) for h in range(2)]
    for g in range(4):
        for e in range(2):
            for h in range(2):
                q = [sched.mm(8 * g + 4 * e + 2 * h + k, jnp.concatenate(
                    [xs_u[4 * k + u, pl.ds((4 * g + 2 + e) * HQ, HQ), :] for u in range(4)], axis=1),
                    w0[h][256 * k:256 * k + 256], step=16) for k in range(2)]
                qn[h, g, e] = _pack((q[0] + q[1]) * QSCALE)
    sched.finish()
    for d in group(16) + piece(16) + (cp_gw(),):
        d.wait()
    for d in cp_p(1):
        d.start()
    plan2 = _plan2()

    def p2_body(p, carry):
        @pl.when(p > 0)
        def _():
            for d in cp_p(p):
                d.wait()

        causal = col <= row + HQ
        never = p > NP
        jobs = staging(p, p, never)
        sched = _Sched(never, plan2, jobs)
        mm = sched.mm

        r0 = pl.multiple_of(p * TQ, TQ)

        prods = {}

        def project(kind, j, n, lhs, rhs):
            got = prods.setdefault((kind, j), {})
            for m in ORDER[len(got):len(got) + n]:
                g = _steps()
                k = next(g)
                for e in range(7):
                    k = g.send(mm((kind, j, 7 * len(got) + e), part(lhs, 7 * m + k), rhs(7 * m + k)))
                    if e < 6 or len(got) < 6:
                        yield
                got[m] = k
            if len(got) < 7:
                return None
            c = _combine(lambda m: got[m])
            return [[c[(rg & 2) + (cg >> 1)][2 * (rg & 1) + (cg & 1)] for rg in range(4)]
                    for cg in range(4)]

        def pair(ref, rows):
            return lambda k: jnp.concatenate([ref[k, sr, rows, :] for sr in range(2)], axis=1)

        def x_rows(b, n):
            return lambda k: jnp.concatenate([jnp.concatenate(
                [xq[k, b + j, pl.ds(16 * sr, 16), :] for sr in range(2)], axis=1)
                for j in range(n)], axis=0)

        def proj_b(kind, n, lhs, w, dst, off):
            c = yield from project(kind, 0, n, lhs, pair(w, slice(None)))
            for cg in range(4 * (c is not None)):
                for rg in range(4):
                    for cc in range(2):
                        dst[2 * cg + cc, pl.ds(off + (PAD + rg * QQ), QQ), :] = (
                            c[cg][rg][:, cc * 128:(cc + 1) * 128])

        def proj_bv():
            for cc in range(8):
                vb[cc, pl.ds(0, PAD), :] = vb[cc, pl.ds(TQ, PAD), :]
            return proj_b("bv", 7, x_rows(p, 1), wv49, vb, 0)

        def proj_bo(n):
            list(proj_b("bo", n, pair(ob49, slice(None)), wob49, qk_b, r0))

        def local_qk(rb, k, gate):
            rz = pl.multiple_of((p + _zero(p, k)) * TQ, TQ)
            q = [qk_b[cc, pl.ds(rz + (PAD + rb * RB), RB), :] for cc in range(8)]
            q[0] = gate(q[0])
            for w in range(LG * k, LG * k + LG):
                t = _fold([q[cc] * qk_b[8 + cc, pl.ds(r0 + (PAD + rb * RB - DIL * w), RB), :]
                           for cc in range(8)], jnp.add)
                t = t + pltpu.roll(t, 64, 1)
                t = t + jnp.where(odd, pltpu.roll(t, 1, 1), pltpu.roll(t, 127, 1))
                t = t * (DB ** -0.5 * LOG2E)
                if rb == 0 and w:
                    t = jnp.where(rowi + r0 >= DIL * w, t, NEG)
                lg_s[w, pl.ds(rb * RB, RB), :] = t
            return [], 1, lambda: pltpu.bitcast(lg_s[w, blk(2 * rb + _zero(p, 0), 8), :], U32)

        def local_sm(rb, e, gate):
            rows = pl.ds(rb * RB + SMR * e, SMR)
            lg = [gate(lg_s[w, rows, :]) for w in range(WIN)]
            m = _tree(lg, jnp.maximum)
            ps = [jnp.exp2(t - m) for t in lg]
            l = _tree(ps, jnp.add)
            r = pl.reciprocal(l, approx=True)
            r = r * (2.0 - l * r)
            for w in range(WIN):
                pr_s[w, rows, :] = ps[w] * r
            return [], 2, lambda: pltpu.bitcast(pr_s[0, blk(2 * rb + e + _zero(p, 0), 8), :], U32)

        def local_pv(rb, k, gate):
            rows = pl.ds(rb * RB, RB)
            ps = [pr_s[w + _zero(p, k), rows, :] for w in range(WIN)]
            ps[0] = gate(ps[0])
            o = [_fold([ps[w] * vb[cc, pl.ds(PAD + rb * RB - DIL * w, RB), :] for w in range(WIN)],
                       jnp.add) for cc in (k, k + 4)]
            for e in range(2):
                o_s[k + 4 * e, rows, :] = o[e]
            return [], 0, lambda: pltpu.bitcast(o_s[k, blk(2 * rb + _zero(p, 0), 8), :], U32)

        def o_sums(m, cc, r, gate):
            res = [_ops49(_lhs7, [[gate(o_s[
                2 * (2 * (q & 1) + (e & 1)) + cc + _zero(p, m),
                pl.ds(QQ * (2 * (q >> 1) + (e >> 1)) + 16 * r + par, 8, stride=2), :])
                for e in range(4)] for q in range(4)], m) for par in range(2)]
            for n, (lo, hi) in enumerate(zip(*res)):
                ob49[7 * m + n, cc, pl.ds(8 * r, 8), :] = _join(lo, hi)
            return [], 0, lambda: ob49[7 * m, cc, blk(r + _zero(p, 0), 8), :]

        jobs["os"] = [part(o_sums, m, cc, r) for r in range(2) for cc in range(2) for m in range(7)]
        order = list(range(0, 8, 2)) + list(range(1, 8, 2))
        jobs["lo"] = []
        for k in range(len(order) + SML):
            for f, d, n in ((local_sm, SML, RB // SMR), (local_qk, 0, 8 // LG)):
                if 0 <= k - d < len(order):
                    jobs["lo"] += [part(f, order[k - d], e) for e in range(n)]
        jobs["lv"] = [part(local_pv, rb, e) for rb in order for e in range(4)]

        def out_weights(m, r, gate):
            ww = [[gate(wo_r[(p & 1) + _zero(p, m),
                             pl.ds((2 * (q >> 1) + (e >> 1)) * HQ + 8 * r, 8),
                             pl.ds((2 * (q & 1) + (e & 1)) * 128, 128)])
                   for e in range(4)] for q in range(4)]
            rows = blk(8 * (p >> 1) + r, 8)
            extra = jobs["sc"].pop(0)(gate)[0] if jobs["sc"] else []
            for n, w in enumerate(_words49(_rhs7, ww, m)):
                if n < len(extra):
                    w = jnp.where(never, extra[n], w)
                wo49[7 * m + n, p & 1, rows, :] = w
            return [], 0, lambda: wo49[7 * m + _zero(p, 0), p & 1, rows, :]

        jobs["wo"] = [part(out_weights, m, r) for m in range(7) for r in range(8)]

        ks, vs, qs = {}, {}, {}
        done = {}

        def blocks(c, scale, pack):
            c = [[pack(t * scale(cg)) for t in c[cg]] for cg in range(4)]
            return [[jnp.concatenate([t[16 * e:16 * e + 16] for t in c[cg]], axis=0)
                     for e in range(2)] for cg in range(4)]

        def proj_kv(j, n):
            c = yield from project("kv", j, n, lambda k: jnp.concatenate(
                [cq[k, 2 * j], cq[k, 2 * j + 1]], axis=0), lambda k: wkv[k])
            if c is not None:
                c = blocks(c, lambda cg: ups[cg][:1], _riffle)
                for cg in range(4):
                    for e in range(2):
                        (vs, ks)[cg >> 1][(cg & 1, 2 * j + e)] = c[cg][e]

        def proj_q(g, n):
            c = yield from project("q", g, n, x_rows(4 * g + 2 * (p & 1), 2), lambda k: wq49[k])
            if c is not None:
                c = blocks(c, lambda cg: QSCALE, _pack)
                for h in range(2):
                    for e in range(2):
                        old = qn[h, g, e]
                        for b in range(2):
                            qs[(h, 4 * g + 2 * b + e)] = jnp.where((p & 1) == b, c[h][e], old)
                        qn[h, g, e] = c[2 + h][e]

        def halves(d, h, js):
            return jnp.concatenate([d[(h, j >> 1)][QQ * (j & 1):QQ * (j & 1) + QQ] for j in js],
                                   axis=0)

        def late(x, y, op):
            return jnp.concatenate([x[:HQ], op(x[HQ:], y)], axis=0)

        def unit(h, i):
            return halves(qs, h, (2 * (i & ~1) + (i & 1), 2 * (i | 1) + (i & 1)))

        def first(i):
            t = jnp.concatenate([mm(("kq", h, i), halves(ks, h, (0,)), unit(h, i), NT)
                                 for h in range(2)], axis=0).T
            keep = [col < HQ, col >= HQ]
            top = [col <= row, causal & keep[1]] if i == 0 else keep
            return [jnp.concatenate([jnp.where(a, t[:HQ], NEG), jnp.where(b, t[HQ:], NEG)], axis=0)
                    for a, b in zip(top, keep)]

        def qk(h, i, dep):
            off = 1 - (i & 1)
            q = unit(h, i)
            if dep is not None:
                q = jnp.where(never, done[(h, dep)], q)
            ch = []
            if i:
                ch = _lane_chunks(mm(("qk", h, i), q, halves(ks, h, range(off, off + 2 * i)),
                                     NT, 512))
                ch[-1] = jnp.concatenate([jnp.where(causal, ch[-1][:HQ], NEG), ch[-1][HQ:]],
                                         axis=0)
            ex = mm(("qx", h, i), q[QQ:], halves(ks, h, (off + 2 * i, off + 2 * i + 1)), NT)
            return ch, jnp.where(causal, ex, NEG)

        def softmax_pv(h, i, ch, ex):
            off = 1 - (i & 1)
            m = jnp.max(late(_fold(ch, jnp.maximum), ex, jnp.maximum), axis=1, keepdims=True)
            pe = jnp.exp2(ex - m[HQ:])
            ps = [jnp.exp2(c - m) for c in ch]
            lp = late(ps[0], pe, jnp.add)
            for j in range(1, len(ch)):
                lp = lp + ps[j]
                if TIE and (j % TIE == TIE - 1 or j == len(ch) - 1):
                    ps[j] = jnp.where(never, lp, ps[j])
            pb = jnp.concatenate(ps, axis=1).astype(BF16)
            vv = [halves(vs, h, range(off, off + 2 * i))] if i else []
            v0 = [halves(vs, e, (0,)) for e in range(2 * off)]
            vv = jnp.concatenate(v0 + vv, axis=0)
            o = mm(("pv", h, i), pb, vv)
            o = late(o, mm(("px", h, i), pe.astype(BF16),
                           halves(vs, h, (off + 2 * i, off + 2 * i + 1))), jnp.add)
            if i >= LDEP:
                lp = jnp.where(never, o, lp)
            l = jnp.sum(lp, axis=1, keepdims=True)
            r = pl.reciprocal(l, approx=True)
            r = r * (2.0 - l * r)
            cn = _pack(o * r)
            done[(h, i)] = cn
            if FA <= i < NQ - 1:
                if i + 3 < NQ:
                    site = ("kv", (i + 1) // 2 + 1, KVS * ((i + 1) & 1) + (F0, FD)[h])
                else:
                    site = ("bo", 0, 7 * (i + 3 - NQ) * BOP[0] + 8 * h)
                sched.pending.setdefault(site, []).append(cn)
            for e in range(2):
                ctx[2 * p + h, pl.ds(((i & ~1) + e) * HQ + QQ * (i & 1), QQ), :] = (
                    cn[QQ * e:QQ * e + QQ])

        head = dict(bv=proj_bv(), kv=proj_kv(0, 7), q=proj_q(0, 7))
        for site in _head():
            next(head[site[0]], None)
        lead = {}
        for i in range(NQ):
            dep = i - DEP if DEP <= i < FA + DEP else None
            for k in range(i, i + VL + 1):
                if k < NQ and not k & 1 and k not in lead and (0, k) in qs:
                    lead[k] = first(k)
            sx = [qk(h, i, dep) for h in range(2)]
            if i + 2 < NQ:
                list(proj_kv(i // 2 + 1, 7 if i & 1 else KVS // 7))
                if i < 6:
                    list(proj_q(i // 2 + 1, 7 if i & 1 else QS // 7))
            else:
                proj_bo(BOP[i + 2 - NQ])
            for h in range(2):
                c0 = [lead[i][h]] if i in lead else []
                softmax_pv(h, i, c0 + sx[h][0], sx[h][1])
        proj_bo(BOP[2])
        sched.finish()
        for d in cp_p(p + 2):
            d.start()
        return carry

    jax.lax.fori_loop(0, NP, p2_body, 0)

    gw = gw_ref[...].astype(F32)
    plan3 = _plan3()
    cab = (ca0, ca1)

    def p3_body(i, carry):
        r0 = pl.multiple_of(i * TO, TO)
        h0 = pl.multiple_of(i * (TO // 2), TO // 2)
        never = i > S

        def ctx_words(m, u, r, n):
            return [[ctx[4 * u + 2 * (q & 1) + (e & 1),
                         pl.ds(h0 + _zero(i, m) * 8 + ((2 * (q >> 1) + (e >> 1)) * QQ + r), n), :]
                     for e in range(4)] for q in range(4)]

        def operands(k, u, r, gate):
            m = ORDER[k]
            cw = [[gate(w) for w in q] for q in ctx_words(m, u, r, 8)]
            for n, w in enumerate(_words49(_lhs7, cw, m)):
                if not (m in (2, 3) and n in (2, 3)):
                    cab[k & 1][n, pl.ds(r, 8), pl.ds(u * 128, 128)] = w
            return [], 0, lambda: cab[k & 1][_zero(i, 0), pl.ds(r, 8), pl.ds(u * 128, 128)]

        def gate_rows(r, gate):
            gs = _fold([_bf(gate(xs_u[j, pl.ds(h0 + r, 8), :])).astype(F32) * gw[j:j + 1]
                        for j in range(8)], jnp.add)
            g = jax.nn.sigmoid(jnp.sum(gs, axis=1, keepdims=True))
            g_s[pl.ds(2 * r, 16), :] = jnp.broadcast_to(g, (16, 128))
            return [], 0, lambda: pltpu.bitcast(g_s[blk(r // 4 + _zero(i, 0), 8), :], U32)

        pr = {}

        def mix(q, e, cc, gate):
            off = (2 * (q >> 1) + (e >> 1)) * HQ
            ch = 4 * cc + 2 * (q & 1) + (e & 1)
            a = _combine(lambda m: pr.get(m, pr[2])[e][:, cc * 128:(cc + 1) * 128])[q]
            g = gate(g_s[pl.ds(off, HQ), :])
            b = qk_b[ch, pl.ds(r0 + (PAD + off), HQ), :]
            out_s[pl.ds(r0 + off, HQ), pl.ds(ch * 128, 128)] = (g * a + (1.0 - g) * b).astype(BF16)
            return [], 0, lambda: pltpu.bitcast(
                out_s[blk(i * (TO // 16) + off // 16 + _zero(i, 0), 16), pl.ds(ch * 128, 128)], U32)

        sched = _Sched(never, plan3, dict(
            a=[part(operands, k, u, r) for k in range(1, 7) for u in range(HA // 4)
               for r in range(0, QQ, 8)],
            g=[part(gate_rows, r) for r in range(0, TO // 2, 8)],
            m=[part(mix, q, e, cc) for q in (1, 2, 0) for e in range(4) for cc in range(2)]))
        first = [[_words49(_lhs7, ctx_words(ORDER[0], u, 0, QQ), ORDER[0])[n]
                  for u in range(HA // 4)] for n in range(7)]

        def inner(m, n):
            k = ORDER.index(m)
            res = []
            for e in range(2):
                us = range(4 * e, 4 * e + 4)
                if m in (2, 3) and n in (2, 3):
                    lhs = jnp.concatenate([ctx_words(m, u, 0, QQ)[3 * (m - 2)][3 * (n - 2)]
                                           for u in us], axis=1)
                elif k == 0:
                    lhs = jnp.concatenate([first[n][u] for u in us], axis=1)
                else:
                    lhs = lambda: cab[k & 1][n, :, pl.ds(e * 512, 512)]
                rhs = jnp.concatenate([wo49[7 * m + n, cc, pl.ds(e * 256, 256), :]
                                       for cc in range(2)], axis=1)
                res.append(sched.mm((k, 2 * ORDER.index(n) + e), lhs, rhs))
                if (k, 2 * ORDER.index(n) + e) == (6, P3D):
                    for d in cp_out(i, 0):
                        d.start()
            return res[0] + res[1]

        for m in ORDER:
            pr[m] = _combine(lambda n: inner(m, n))
        sched.finish()
        for e in (1, 2, 0, 3):
            for cc in range(2):
                mix(3, e, cc, lambda x: x)
        for d in cp_out(i, 1):
            d.start()
        return carry

    jax.lax.fori_loop(0, S // TO, p3_body, 0)
    for d in cp_p(NP) + cp_p(NP + 1):
        d.wait()
    for i in range(S // TO):
        for d in cp_out(i, 0) + cp_out(i, 1):
            d.wait()


@jax.jit
def pallas_gated_mix__compressed_kv_cla__sliding_local_dilated__prompt_kernel(
    A_x: jax.Array,
    A_c_kv: jax.Array,
    A_w_q: jax.Array,
    A_w_uk: jax.Array,
    A_w_uv: jax.Array,
    A_w_o: jax.Array,
    B_x: jax.Array,
    B_wqkv: jax.Array,
    B_wo: jax.Array,
    gate_w: jax.Array,
):
    del B_x
    any_spec = pl.BlockSpec(memory_space=pl.ANY)
    out = pl.pallas_call(
        _kernel,
        in_specs=[any_spec] * 9,
        out_specs=any_spec,
        out_shape=jax.ShapeDtypeStruct((S, M), BF16),
        scratch_shapes=[
            pltpu.VMEM((9, S // 2, 128), U32),
            pltpu.VMEM((2, HQ, M), U32),
            pltpu.VMEM((2, HQ, DC), U32),
            pltpu.VMEM((2, 128, M), BF16),
            pltpu.VMEM((2, 4, 16, M), BF16),
            pltpu.VMEM((2, 4, 16, M), U32),
            pltpu.VMEM((3, 2 * DC, 128), U32),
            pltpu.VMEM((4, M, 128), U32),
            pltpu.VMEM((2, 2 * DA, M // 2), U32),
            pltpu.VMEM((8, 64, 128), U32),
            pltpu.VMEM((49, NQ, 32, 128), U32),
            pltpu.VMEM((49, NQ, 16, 128), U32),
            pltpu.VMEM((49, 2, M // 8, 128), U32),
            pltpu.VMEM((49, 2, M // 8, 128), U32),
            pltpu.VMEM((49, 2, NP * QQ, 128), U32),
            pltpu.VMEM((49, HQ, 128), U32),
            pltpu.VMEM((49, TQ, 128), U32),
            pltpu.VMEM((4, 8, 128), F32),
            pltpu.VMEM((4, DC // SCR * 8 + 16, 128), jnp.int32),
            pltpu.VMEM((2, 4, 2, HQ, 128), U32),
            pltpu.VMEM((16, S + PAD, 128), F32),
            pltpu.VMEM((8, TQ + PAD, 128), F32),
            pltpu.VMEM((WIN, TQ, 128), F32),
            pltpu.VMEM((WIN, TQ, 128), F32),
            pltpu.VMEM((8, TQ, 128), F32),
            pltpu.VMEM((49, 2, 16, 128), U32),
            pltpu.VMEM((HA, S // 2, 128), U32),
            pltpu.VMEM((7, QQ, M), U32),
            pltpu.VMEM((7, QQ, M), U32),
            pltpu.VMEM((TO, 128), F32),
            pltpu.VMEM((S, M), BF16),
            pltpu.VMEM((8, 128), BF16),
            pltpu.SemaphoreType.DMA((2,)),
            pltpu.SemaphoreType.DMA((2,)),
            pltpu.SemaphoreType.DMA((5,)),
        ],
        compiler_params=pltpu.CompilerParams(vmem_limit_bytes=120 * 1024 * 1024,
                                             disable_bounds_checks=True),
    )(
        A_x.reshape(S, M),
        A_c_kv.reshape(S, DC),
        A_w_q,
        A_w_uk,
        A_w_uv,
        A_w_o.reshape(HA * DA, M),
        B_wqkv.reshape(2, M // 2, 3 * M),
        B_wo.reshape(HB // 2, 2, DB, M),
        gate_w.reshape(8, 128),
    )
    return out.reshape(1, S, M)
```

```python
import functools

import jax
import jax.numpy as jnp
import jax.experimental.pallas as pl
import jax.experimental.pallas.tpu as pltpu

F32 = jnp.float32
BF16 = jnp.bfloat16
U32 = jnp.uint32

S = 2048
M = 1024
HA = 32
DA = 128
DC = 512
HB = 32
DB = 32
WIN = 8
DIL = 2
PAD = 16
LOG2E = 1.4426950408889634
NEG = -1e9

TQ = 128
HQ = TQ // 2
QQ = TQ // 4
NQ = S // TQ
NP = HA // 2
RB = 16
TO = 256

P0S = ((0, 0, 1024), (1, 0, 1024), (0, 1024, 1024), (1, 1024, 768), (1, 1792, 128), (1, 1920, 128))
P0W = 2
P0A = 75
P0T = 16
P0N = 104
P1S = ((0, 0, 2048), (1, 0, 1536), (1, 1536, 384), (1, 1920, 128))
P1A = 60
P1N = 108
XN = 28
XQ = 50
XS = 24
BOP = (2, 3, 2)
KVS = 28
QS = 35
LX = 16
QST = 2
SK = 3
LG = 1
SMR = 16
SML = 1
SCR = 32
LN = 92
LA = 16
BS = 2
LP = ("kv", 1, 8)
BX = 8
BE = 42
DEP = 2
FA = 6
F0 = 0
FD = 8
TIE = 4
LDEP = 6
VL = 1
IV = 3
DS = 10
KE = 2
KT = 42
HP = 53
P3S = 3
P3E = 12
P3M = 6
P3D = 8

NN = (((1,), (0,)), ((), ()))
NT = (((1,), (1,)), ((), ()))


def _head():
    rest = [(kind, 0, k) for kind in ("kv", "q") for k in range(49)]
    out, room = [], 0
    for k in range(49):
        out.append(("bv", 0, k))
        room += IV
        while rest and room >= 1 + (rest[0][0] == "q"):
            room -= 1 + (rest[0][0] == "q")
            out.append(rest.pop(0))
    return out + rest


def _plan2():
    plan = {}

    def put(name, count, start, until):
        plan.setdefault(start, []).extend([(name, until)] * count)

    def after_qk(i):
        if i >= NQ - 2:
            return ("bo", 0, 7 * (i - NQ + 2) * BOP[0] + BX)
        return ("kv", i // 2 + 1, KVS * (i & 1) + LX)

    def fill(name, count, sites):
        for start, room, until in sites:
            n = min(count, room - len(plan.get(start, ())))
            put(name, n, start, until)
            count -= n
        assert count == 0, (name, count)

    def qk_sites(lo, hi):
        return [(("qk", h, i), max(i + 1 - h * SK, 0), after_qk(i))
                for i in range(lo, hi) for h in range(2)]

    def q_sites(g, lo, hi, until):
        return [(("q", g, k), 1, until) for k in range(lo, hi, QST)]

    ticks = [t for t in _head() if t[0] != "kv" or t[2] & 1 == 0]
    for name, site in zip(_spread(["lo"] * (64 // LG + 128 // SMR), LN), ticks[LA:]):
        put(name, 1, site, LP)
    host = [(t, 1, ticks[HP]) for t in ticks[:LA:BS]]
    early = []
    for g in range(1, 4):
        early += q_sites(g, 0, QS - 4, after_qk(2 * g - 1))
        early += qk_sites(2 * g - 1, 2 * g)
        early += q_sites(g, QS, 45, after_qk(2 * g))
        early += qk_sites(2 * g, 2 * g + 1)
    fill("lv", 32, early)
    fill("wo", 56, host + early)
    fill("os", 28, early + qk_sites(7, 14))
    fill("qw", 112, qk_sites(7, 14))
    for k in range(KE):
        put("kv", 1, ("bo", 0, KT + k), None)
    fill("kv", 56 - KE, qk_sites(14, 16) + [(("bo", 0, k), 1, ("bo", 0, BE))
                                       for k in range(7 * BOP[0], 35)])
    return plan


def _planx():
    names = _spread(["qw"] * (XQ - XS) + ["kv", "qw"] * 56 + ["qw"] * (56 - XQ), 8 * XN)
    return {k: [(n, None) for n in names[8 * k:8 * k + 8]] for k in range(XN)}


def _spread(names, ticks):
    out = [None] * ticks
    for k, name in enumerate(names):
        out[k * ticks // len(names)] = name
    return out


def _plan1(segs, lo, step, count, extra):
    end = len(segs) - 2
    ticks = [k for k in range(lo, end) for _ in range(segs[k][2] // step)][:count]
    n = len(ticks) * (P0A if lo else P1A) // 100
    names = _spread(["x"] * 28 + ["c"] * 14 + ["o"] * 14, n) + _spread(["v"] * 14, len(ticks) - n)
    free = [k for k, name in enumerate(names) if name is None]
    for k in free[len(free) - extra:]:
        names[k] = "qw"
    plan = {}
    for k, name in zip(ticks, names):
        plan.setdefault(k, []).append((name, None if name == "qw" else end))
    return plan


def _plan3():
    plan = {}
    for k in range(6):
        lo = P3S if k == 0 else 0
        extra = ["g"] * 8 if k in (1, 2) else []
        names = _spread(["a"] * 32 + extra, 4 * (P3E - lo))
        for d in range(lo, P3E):
            plan[(k, d)] = [(n, (k + 1, 0)) for n in names[4 * (d - lo):4 * (d - lo) + 4]]
    names = _spread(["m"] * 24, 4 * P3M)
    for d in range(P3M):
        plan[(6, d)] = [(n, (6, P3D)) for n in names[4 * d:4 * d + 4]]
    return plan


_STAGES = ((2, 4), (1, 3), (0, 2), (0, 6), (0, 1))


def _permute8(cols):
    cols = list(cols)
    lane = jax.lax.broadcasted_iota(jnp.int32, cols[0].shape, 1)
    for va, lb in _STAGES:
        lo = (lane & (1 << lb)) == 0
        sh = 1 << lb
        idx = [i for i in range(8) if not (i >> va) & 1]
        if lb == 6:
            rr = [pltpu.roll(jnp.where(lo, cols[i | (1 << va)], cols[i]), 64, 1) for i in idx]
            for i, r in zip(idx, rr):
                a, b = cols[i], cols[i | (1 << va)]
                cols[i] = jnp.where(lo, a, r)
                cols[i | (1 << va)] = jnp.where(lo, r, b)
        else:
            rb = [pltpu.roll(cols[i | (1 << va)], sh, 1) for i in idx]
            ra = [pltpu.roll(cols[i], 128 - sh, 1) for i in idx]
            for i, xa, xb in zip(idx, ra, rb):
                a, b = cols[i], cols[i | (1 << va)]
                cols[i] = jnp.where(lo, a, xb)
                cols[i | (1 << va)] = jnp.where(lo, xa, b)
    return cols


def _pack(x):
    return pltpu.bitcast(x.astype(BF16), U32)


def _bf(x):
    return pltpu.bitcast(x, BF16)


def _split(w):
    return (pltpu.bitcast(w << 16, F32), pltpu.bitcast(w & jnp.uint32(0xFFFF0000), F32))


def _join(lo, hi):
    return pltpu.bitcast(pltpu.pack_elementwise([lo, hi], packed_dtype=BF16), U32)


def _riffle(x):
    return jnp.concatenate([_join(x[r:r + 16], x[r + 16:r + 32]) for r in range(0, x.shape[0], 32)],
                           axis=0)


def _lhs7(a11, a12, a21, a22):
    return [a11 + a22, a21 + a22, a11, a22, a11 + a12, a21 - a11, a12 - a22]


def _rhs7(b11, b12, b21, b22):
    return [b11 + b22, b11, b12 - b22, b21 - b11, b22, b11 + b12, b21 + b22]


def _steps():
    add = functools.partial(jax.tree.map, jnp.add)
    sub = functools.partial(jax.tree.map, jnp.subtract)
    m2 = yield 2
    m3 = yield 3
    m4 = yield 4
    c12 = add(m2, m4)
    t11 = sub(m3, m4)
    m1 = yield 1
    c21 = add(m1, m3)
    t22 = sub(m2, m1)
    m0 = yield 0
    t11 = add(t11, m0)
    t22 = add(t22, m0)
    c11 = add(t11, (yield 6))
    yield c11, c12, c21, add(t22, (yield 5))


def _combine(mm):
    g = _steps()
    k = next(g)
    for _ in range(7):
        k = g.send(mm(k))
    return k


ORDER = (2, 3, 4, 1, 0, 6, 5)


def _zero(i, m):
    return i >> (8 + m)


def _merge(vals):
    return _fold([v[r:r + 8, c:c + 128] for v in vals for r in range(0, v.shape[0], 8)
                  for c in range(0, v.shape[1], 128)], jnp.bitwise_or)


def _gate(never, g):
    def gate(x):
        t = jnp.tile(pltpu.bitcast(g, x.dtype), (x.shape[0] // 8, x.shape[1] // 128))
        return jnp.where(never, t, x)
    return gate


def _tie(never, x, deps):
    if not deps:
        return x
    top = jnp.where(never, _merge(deps), x[:8, :128])
    if x.shape[1] > 128:
        top = jnp.concatenate([top, x[:8, 128:]], axis=1)
    return jnp.concatenate([top, x[8:]], axis=0)


class _Sched:
    def __init__(self, never, plan, jobs):
        self.never, self.plan, self.jobs, self.pending = never, plan, jobs, {}

    def mm(self, site, a, b, dims=NN, width=128, step=32):
        deps = [d() if callable(d) else d for d in self.pending.pop(site, ())]
        a = a() if callable(a) else a
        tie = functools.partial(_tie, self.never, deps=deps)
        a, b = (_bf(tie(a)), _bf(b)) if a.dtype == U32 else (a, _bf(tie(b)))
        out = jax.lax.dot_general(a, b, dims, preferred_element_type=F32)
        per = out.shape[0] // step
        last = {}
        for k, (name, until) in enumerate(self.plan.get(site, ())):
            if name is not None:
                r, c = step * (k % per), min(width * (k // per), out.shape[1] - 128)
                vals, tag, stored = self.jobs[name].pop(0)(
                    _gate(self.never, out[r:r + 8, c:c + 128]))
                self.pending.setdefault(until, []).extend(vals)
                last[(name, tag, until)] = stored
        for (_, _, until), stored in last.items():
            if stored is not None:
                self.pending[until].append(stored)
        return out

    def finish(self):
        self.pending.pop(None, None)
        assert not any(self.jobs.values()) and not any(self.pending.values())


def _ops49(fn, blocks, m):
    return fn(*[fn(*[blocks[q][e] for q in range(4)])[m] for e in range(4)])


def _words49(fn, words, m):
    halves = [[_split(w) for w in q] for q in words]
    lo = _ops49(fn, [[h[0] for h in q] for q in halves], m)
    hi = _ops49(fn, [[h[1] for h in q] for q in halves], m)
    return [_join(a, b) for a, b in zip(lo, hi)]


def _fold(xs, op):
    acc = xs[0]
    for x in xs[1:]:
        acc = op(acc, x)
    return acc


def _tree(xs, op):
    while len(xs) > 1:
        xs = [op(a, b) for a, b in zip(xs[::2], xs[1::2])]
    return xs[0]


def _lane_chunks(x):
    return [x[:, j * 128:(j + 1) * 128] for j in range(x.shape[1] // 128)]


def _kernel(x_hbm, c_hbm, wq_hbm, wuk_hbm, wuv_hbm, wo_hbm, wqkv_hbm, wob_hbm, gw_hbm,
            out_hbm,
            xs_u, x_r, c_r, w_r, wv_r, wob_r, wkv_r, wq_r, wo_r,
            wperm, xq, cq, wv49, wob49, wo49, wkv, wq49, ups, sc_s, qn,
            qk_b, vb, lg_s, pr_s, o_s, ob49, ctx, ca0, ca1, g_s, out_s, gw_ref,
            sem_x, sem_p, sem_a):
    x_u = x_hbm.bitcast(U32)
    c_u = c_hbm.bitcast(U32)
    wo_u = wo_hbm.bitcast(U32)
    wq_u = wq_hbm.bitcast(U32)
    wuk_u = wuk_hbm.bitcast(U32)
    wuv_u = wuv_hbm.bitcast(U32)
    wob_u = wob_hbm.bitcast(U32)
    part = functools.partial

    def blk(j, n):
        return pl.ds(pl.multiple_of(j * n, n), n)

    def strip(j):
        return blk(j, 128)

    def cp_x(t, sem):
        k = (t + 1) >> 1
        return pltpu.make_async_copy(x_u.at[blk(t & 1, S // 4), strip(jnp.minimum(k, 7))],
                                     xs_u.at[jnp.minimum(k, 8), blk(t & 1, S // 4), :], sem)

    def cp_w(t, sem):
        u = t - 2 * (t >> 4)
        u = u - 2 * (u >> 4)
        return pltpu.make_async_copy(wqkv_hbm.at[u >> 3, strip((u >> 1) & 3), blk(u & 1, M)],
                                     w_r.at[u & 1], sem)

    def cp_wob(t, sem):
        b = (t + 1) >> 1
        c = jnp.minimum(b, 7)
        return tuple(pltpu.make_async_copy(
            wob_u.at[:, c & 1, 4 * (2 * (t & 1) + j) + (c & 2) + (c >> 2), :],
            wob_r.at[b & 1, 2 * (t & 1) + j], sem) for j in range(2))

    def group(t, sem1=None):
        sem = sem_x.at[t & 1]
        u = t - 2 * (t >> 4)
        return (
            cp_x(t, sem if sem1 is None else sem1),
            cp_w(t + 1, sem),
            pltpu.make_async_copy(x_u.at[blk(u, HQ), :], x_r.at[u & 1], sem),
            pltpu.make_async_copy(c_u.at[blk(u, HQ), :], c_r.at[u & 1], sem),
        ) + cp_wob(t, sem) + tuple(
            pltpu.make_async_copy(wqkv_hbm.at[e >> 1, blk(16 * (e & 1) + u, 16), pl.ds(2 * M, M)],
                                  wv_r.at[u & 1, e], sem) for e in range(4))

    def piece(t):
        late = t >> 4
        pq = (t >> 3) + late
        pk = (t >> 3) & 1
        u = (t & 15) + 2 * late
        sem = sem_a.at[3 + late]
        return (
            pltpu.make_async_copy(wo_u.at[blk(u, 16), pl.ds(0, M // 2)],
                                  wo_r.at[late, blk(u, 16), :], sem),
            pltpu.make_async_copy(wq_u.at[strip(t & 7), pq, :], wq_r.at[pq, strip(t & 7), :], sem),
            pltpu.make_async_copy(wq_u.at[blk(u, 64), 2, :], wq_r.at[2 + late, blk(u, 64), :], sem),
            pltpu.make_async_copy(wuk_u.at[blk(t & 7, 64), pk, :],
                                  wkv_r.at[1 - pk + late, blk(8 + (t & 7), 64), :], sem),
            pltpu.make_async_copy(wuv_u.at[blk(t & 7, 64), pk, :],
                                  wkv_r.at[1 - pk + late, blk(t & 7, 64), :], sem),
        )

    def cp_wq(p, sem):
        return pltpu.make_async_copy(wq_u.at[:, jnp.minimum(p, NP - 1), :], wq_r.at[p & 3], sem)

    def cp_p(g):
        slot = g & 1
        p = jnp.minimum(g + 1, NP - 1)
        o = jnp.minimum(g, NP - 1)
        sem = sem_p.at[slot]
        return (
            pltpu.make_async_copy(wo_u.at[blk(o >> 1, 2 * DA), blk(o & 1, M // 2)],
                                  wo_r.at[slot], sem),
            pltpu.make_async_copy(wuk_u.at[:, p, :], wkv_r.at[slot, pl.ds(DC, DC), :], sem),
            pltpu.make_async_copy(wuv_u.at[:, p, :], wkv_r.at[slot, pl.ds(0, DC), :], sem),
            cp_wq(g + 2, sem),
        )

    def cp_gw():
        return pltpu.make_async_copy(gw_hbm, gw_ref, sem_a.at[0])

    def cp_out(i, late):
        def cp(rows, cols):
            return pltpu.make_async_copy(out_s.at[rows, cols], out_hbm.at[rows, cols], sem_a.at[1])

        low = [cp(blk(2 * i + 1, TO // 2), pl.ds(512 * cc + 256 * late, 256)) for cc in range(2)]
        return low if late else [cp(blk(2 * i, TO // 2), pl.ds(0, M))] + low

    cp_w(0, sem_a.at[1]).start()
    group0, group1 = group(0, sem_a.at[2]), group(1)
    group0 = (group0[0], cp_x(-1, sem_x.at[0])) + group0[1:] + cp_wob(-1, sem_x.at[0])
    for d in group0 + group1[:1] + group1[2:]:
        d.start()

    for cc in range(8):
        qk_b[8 + cc, pl.ds(0, PAD), :] = jnp.zeros((PAD, 128), F32)
        vb[cc, pl.ds(TQ, PAD), :] = jnp.zeros((PAD, 128), F32)

    def stage_first(t, lo=0, hi=8):
        w = _permute8(_lane_chunks(pltpu.bitcast(w_r[t & 1], U32)))
        for cc in range(lo, hi):
            wperm[cc] = w[cc]

    def p1_step(t, peel, extra=None):
        if not peel:
            for d in group(t):
                d.wait()

        def act_sums(src, dst, ns, m, sr, r, gate):
            cw = [[gate(src[(t & 1) + _zero(t, m), pl.ds(32 * (q >> 1) + 16 * (e >> 1) + 8 * r, 8),
                            pl.ds(((2 * (q & 1) + (e & 1)) * ns + sr) * 128, 128)])
                   for e in range(4)] for q in range(4)]
            for n, w in enumerate(_words49(_lhs7, cw, m)):
                dst[7 * m + n, t, pl.ds(16 * sr + 8 * r, 8), :] = w
            return [], 0, lambda: dst[7 * m + _zero(t, 0), t, pl.ds(16 * sr + 8 * r, 8), :]

        wv = []

        def load_wv():
            wv.extend(_permute8(_lane_chunks(jnp.concatenate(
                [pltpu.bitcast(wv_r[t & 1, e], U32) for e in range(4)], axis=0))))

        def w_sums(src, dst, m, cc, gate):
            ww = [[gate(src(m, 2 * (q >> 1) + (e >> 1), 2 * (2 * (q & 1) + (e & 1)) + cc))
                   for e in range(4)] for q in range(4)]
            for n, w in enumerate(_words49(_rhs7, ww, m)):
                dst[7 * m + n, cc, blk(t, 8), :] = w
            return [], 0, lambda: dst[7 * m + _zero(t, 0), cc, blk(t, 8), :]

        def v_src(m, rq, ch):
            return wv[ch][8 * rq:8 * rq + 8]

        def o_src(m, rq, ch):
            return wob_r[((t >> 1) & 1) + _zero(t, m), rq, blk(t & 1, 8), pl.ds(128 * ch, 128)]

        segs, step = (P0S, P0T) if peel else (P1S, 32)
        sched = _Sched(t > 99, _plan1(segs, P0W * peel, step, P0N if peel else P1N,
                                     XS if extra else 0), dict(
            extra or {},
            x=[part(act_sums, x_r, xq, 2, m, sr, r)
               for m in range(7) for sr in range(2) for r in range(2)],
            c=[part(act_sums, c_r, cq, 1, m, 0, r) for m in range(7) for r in range(2)],
            v=[part(w_sums, v_src, wv49, m, cc) for m in range(7) for cc in range(2)],
            o=[part(w_sums, o_src, wob49, m, cc) for m in range(7) for cc in range(2)]))

        first = t < 2
        for k, (half, r0, n) in enumerate(segs):
            if k == P0W * peel:
                if peel:
                    for d in group0[1:]:
                        d.wait()
                    group1[1].start()
                load_wv()
            w = jnp.concatenate([wperm[4 * half + cc] for cc in range(4)], axis=1)
            r = sched.mm(k, xs_u[t >> 1, pl.ds(r0 // 2, n // 2), :], w, step=step)
            if k == len(segs) - 1 and not extra:
                sched.finish()
                stage_first(t + 1)
                d = group(t + 2)
                e = piece(t + 2)
                d = d[2:6] + e[:1] + d[6:] + d[:2] + e[1:]
                for d in d + (piece(0) + piece(1) + (cp_gw(),) if peel else ()):
                    d.start()
            for cc in range(4):
                sl = (8 * (t & 1) + 4 * half + cc, pl.ds(PAD + r0, n), slice(None))
                new = r[:, cc * 128:(cc + 1) * 128]
                qk_b[sl] = new if peel else jnp.where(first, 0.0, qk_b[sl]) + new
        return t

    zero = jnp.max(vb[0, pl.ds(TQ, 8), :]).astype(jnp.int32)
    cp_w(0, sem_a.at[1]).wait()
    stage_first(0, 0, 4)
    group0[0].wait()
    stage_first(0, 4, 8)
    p1_step(zero, True)
    last = jax.lax.fori_loop(1, 15, lambda t, c: p1_step(t, False), 0)
    for t in range(16):
        for d in piece(t):
            d.wait()

    row = jax.lax.broadcasted_iota(jnp.int32, (HQ, TQ), 0)
    col = jax.lax.broadcasted_iota(jnp.int32, (HQ, TQ), 1)
    col = (col & ~31) | ((col & 1) << 4) | ((col & 31) >> 1)
    rowi = jax.lax.broadcasted_iota(jnp.int32, (RB, 128), 0)
    odd = (jax.lax.broadcasted_iota(jnp.int32, (RB, 128), 1) & 1) == 1
    QSCALE = DA ** -0.5 * LOG2E

    def pair_rows(src, slot, r0, n, gate):
        return [_split(gate(src[slot, pl.ds(r0 + par, n // 2, stride=2), :])) for par in range(2)]

    def staging(g, z, never):
        ns = DC // SCR

        def scales(n1, k, gate):
            res = []
            for h in range(2):
                if k < ns:
                    w = gate(wkv_r[g & 1, pl.ds(n1 * DC + k * SCR, SCR), :])
                    w = pltpu.bitcast(w, jnp.int32) & (0x7F80 << (16 * h))
                else:
                    w = gate(sc_s[2 * n1 + h, pl.ds(0, 8 * ns), :])
                e = _tree([w[r:r + 8] for r in range(0, w.shape[0], 8)], jnp.maximum)
                if k == ns:
                    e = pltpu.bitcast(e << (16 - 16 * h), F32)
                    e = jnp.max(e, axis=0, keepdims=True)
                    e = jnp.clip(pltpu.bitcast(e, jnp.int32), 1 << 23, 253 << 23)
                    e = jnp.broadcast_to(e, (8, 128))
                    sc_s[2 * n1 + h, pl.ds(8 * ns + 8, 8), :] = (254 << 23) - e
                sc_s[2 * n1 + h, pl.ds(8 * k, 8), :] = e
                res.append(pltpu.bitcast(e, U32))
            return res, 0, lambda: pltpu.bitcast(sc_s[2 * n1, blk(k + _zero(z, 0), 8), :], U32)

        def rhs49(dst, tiles, scale, m, r, extra=()):
            res = [_ops49(_rhs7,
                          [[scale(tiles[2 * (q >> 1) + (e >> 1)][q & 1][par][e & 1],
                                  2 * (q & 1) + (e & 1)) for e in range(4)] for q in range(4)],
                          m) for par in range(2)]
            for k, (lo, hi) in enumerate(zip(*res)):
                w = _join(lo, hi)
                if k < len(extra):
                    w = jnp.where(never, extra[k], w)
                dst[7 * m + k, pl.ds(8 * r, 8), :] = w

        def kv(m, r, gate):
            if m == 0 and r == 0:
                for k in range(4):
                    ups[k] = pltpu.bitcast(gate(sc_s[k, pl.ds(8 * ns, 8), :]), F32)
            down = [pltpu.bitcast(sc_s[k + _zero(z, m), pl.ds(8 * ns + 8, 8), :], F32)
                    for k in range(4)]
            tiles = [[pair_rows(wkv_r, (g & 1) + _zero(z, m), n1 * DC + kt * 128 + 16 * r, 16, gate)
                      for n1 in range(2)] for kt in range(4)]
            rhs49(wkv, tiles, lambda w, k: w * down[k], m, r)
            return [], 0, lambda: wkv[7 * m, blk(r + _zero(z, 0), 8), :]

        def qw(m, r, gate):
            tiles = [[pair_rows(wq_r, ((g + 1 + n1) & 3) + _zero(z, m), kt * 256 + 16 * r, 16, gate)
                      for n1 in range(2)] for kt in range(4)]
            rhs49(wq49, tiles, lambda w, k: w, m, r, sc.pop(0)(gate)[0] if sc else ())
            return [], 0, lambda: wq49[7 * m, blk(r + _zero(z, 0), 8), :]

        sc = [part(scales, n1, k) for k in range(ns + 1) for n1 in range(2)]
        return dict(sc=sc,
                    kv=[part(kv, m, r) for m in range(7) for r in range(8)],
                    qw=[part(qw, m, r) for m in range(7) for r in range(16)])

    sched = _Sched(last > 99, _planx(), staging(-1, last, last > 99))
    p1_step(last + 1, False, sched.jobs)
    w0 = pair_rows(wq_r, 0, 0, M, lambda x: x)
    w0 = [_join(w0[0][h], w0[1][h]) for h in range(2)]
    for g in range(4):
        for e in range(2):
            for h in range(2):
                q = [sched.mm(8 * g + 4 * e + 2 * h + k, jnp.concatenate(
                    [xs_u[4 * k + u, pl.ds((4 * g + 2 + e) * HQ, HQ), :] for u in range(4)], axis=1),
                    w0[h][256 * k:256 * k + 256], step=16) for k in range(2)]
                qn[h, g, e] = _pack((q[0] + q[1]) * QSCALE)
    sched.finish()
    for d in group(16) + piece(16) + (cp_gw(),):
        d.wait()
    for d in cp_p(1):
        d.start()
    plan2 = _plan2()

    def p2_body(p, carry):
        @pl.when(p > 0)
        def _():
            for d in cp_p(p):
                d.wait()

        causal = col <= row + HQ
        never = p > NP
        jobs = staging(p, p, never)
        sched = _Sched(never, plan2, jobs)
        mm = sched.mm

        r0 = pl.multiple_of(p * TQ, TQ)

        prods = {}

        def project(kind, j, n, lhs, rhs):
            got = prods.setdefault((kind, j), {})
            for m in ORDER[len(got):len(got) + n]:
                g = _steps()
                k = next(g)
                for e in range(7):
                    k = g.send(mm((kind, j, 7 * len(got) + e), part(lhs, 7 * m + k), rhs(7 * m + k)))
                    if e < 6 or len(got) < 6:
                        yield
                got[m] = k
            if len(got) < 7:
                return None
            c = _combine(lambda m: got[m])
            return [[c[(rg & 2) + (cg >> 1)][2 * (rg & 1) + (cg & 1)] for rg in range(4)]
                    for cg in range(4)]

        def pair(ref, rows):
            return lambda k: jnp.concatenate([ref[k, sr, rows, :] for sr in range(2)], axis=1)

        def x_rows(b, n):
            return lambda k: jnp.concatenate([jnp.concatenate(
                [xq[k, b + j, pl.ds(16 * sr, 16), :] for sr in range(2)], axis=1)
                for j in range(n)], axis=0)

        def proj_b(kind, n, lhs, w, dst, off):
            c = yield from project(kind, 0, n, lhs, pair(w, slice(None)))
            for cg in range(4 * (c is not None)):
                for rg in range(4):
                    if kind == "bo" and 4 * cg + rg == DS:
                        for d in cp_p(p + 2):
                            d.start()
                    for cc in range(2):
                        dst[2 * cg + cc, pl.ds(off + (PAD + rg * QQ), QQ), :] = (
                            c[cg][rg][:, cc * 128:(cc + 1) * 128])

        def proj_bv():
            for cc in range(8):
                vb[cc, pl.ds(0, PAD), :] = vb[cc, pl.ds(TQ, PAD), :]
            return proj_b("bv", 7, x_rows(p, 1), wv49, vb, 0)

        def proj_bo(n):
            list(proj_b("bo", n, pair(ob49, slice(None)), wob49, qk_b, r0))

        def local_qk(rb, k, gate):
            rz = pl.multiple_of((p + _zero(p, k)) * TQ, TQ)
            q = [qk_b[cc, pl.ds(rz + (PAD + rb * RB), RB), :] for cc in range(8)]
            q[0] = gate(q[0])
            for w in range(LG * k, LG * k + LG):
                t = _fold([q[cc] * qk_b[8 + cc, pl.ds(r0 + (PAD + rb * RB - DIL * w), RB), :]
                           for cc in range(8)], jnp.add)
                t = t + pltpu.roll(t, 64, 1)
                t = t + jnp.where(odd, pltpu.roll(t, 1, 1), pltpu.roll(t, 127, 1))
                t = t * (DB ** -0.5 * LOG2E)
                if rb == 0 and w:
                    t = jnp.where(rowi + r0 >= DIL * w, t, NEG)
                lg_s[w, pl.ds(rb * RB, RB), :] = t
            return [], 1, lambda: pltpu.bitcast(lg_s[w, blk(2 * rb + _zero(p, 0), 8), :], U32)

        def local_sm(rb, e, gate):
            rows = pl.ds(rb * RB + SMR * e, SMR)
            lg = [gate(lg_s[w, rows, :]) for w in range(WIN)]
            m = _tree(lg, jnp.maximum)
            ps = [jnp.exp2(t - m) for t in lg]
            l = _tree(ps, jnp.add)
            r = pl.reciprocal(l, approx=True)
            r = r * (2.0 - l * r)
            for w in range(WIN):
                pr_s[w, rows, :] = ps[w] * r
            return [], 2, lambda: pltpu.bitcast(pr_s[0, blk(2 * rb + e + _zero(p, 0), 8), :], U32)

        def local_pv(rb, k, gate):
            rows = pl.ds(rb * RB, RB)
            ps = [pr_s[w + _zero(p, k), rows, :] for w in range(WIN)]
            ps[0] = gate(ps[0])
            o = [_fold([ps[w] * vb[cc, pl.ds(PAD + rb * RB - DIL * w, RB), :] for w in range(WIN)],
                       jnp.add) for cc in (k, k + 4)]
            for e in range(2):
                o_s[k + 4 * e, rows, :] = o[e]
            return [], 0, lambda: pltpu.bitcast(o_s[k, blk(2 * rb + _zero(p, 0), 8), :], U32)

        def o_sums(m, cc, r, gate):
            res = [_ops49(_lhs7, [[gate(o_s[
                2 * (2 * (q & 1) + (e & 1)) + cc + _zero(p, m),
                pl.ds(QQ * (2 * (q >> 1) + (e >> 1)) + 16 * r + par, 8, stride=2), :])
                for e in range(4)] for q in range(4)], m) for par in range(2)]
            for n, (lo, hi) in enumerate(zip(*res)):
                ob49[7 * m + n, cc, pl.ds(8 * r, 8), :] = _join(lo, hi)
            return [], 0, lambda: ob49[7 * m, cc, blk(r + _zero(p, 0), 8), :]

        jobs["os"] = [part(o_sums, m, cc, r) for r in range(2) for cc in range(2) for m in range(7)]
        order = list(range(0, 8, 2)) + list(range(1, 8, 2))
        jobs["lo"] = []
        for k in range(len(order) + SML):
            for f, d, n in ((local_sm, SML, RB // SMR), (local_qk, 0, 8 // LG)):
                if 0 <= k - d < len(order):
                    jobs["lo"] += [part(f, order[k - d], e) for e in range(n)]
        jobs["lv"] = [part(local_pv, rb, e) for rb in order for e in range(4)]

        def out_weights(m, r, gate):
            ww = [[gate(wo_r[(p & 1) + _zero(p, m),
                             pl.ds((2 * (q >> 1) + (e >> 1)) * HQ + 8 * r, 8),
                             pl.ds((2 * (q & 1) + (e & 1)) * 128, 128)])
                   for e in range(4)] for q in range(4)]
            rows = blk(8 * (p >> 1) + r, 8)
            extra = jobs["sc"].pop(0)(gate)[0] if jobs["sc"] else []
            for n, w in enumerate(_words49(_rhs7, ww, m)):
                if n < len(extra):
                    w = jnp.where(never, extra[n], w)
                wo49[7 * m + n, p & 1, rows, :] = w
            return [], 0, lambda: wo49[7 * m + _zero(p, 0), p & 1, rows, :]

        jobs["wo"] = [part(out_weights, m, r) for m in range(7) for r in range(8)]

        ks, vs, qs = {}, {}, {}
        done = {}

        def blocks(c, scale, pack):
            c = [[pack(t * scale(cg)) for t in c[cg]] for cg in range(4)]
            return [[jnp.concatenate([t[16 * e:16 * e + 16] for t in c[cg]], axis=0)
                     for e in range(2)] for cg in range(4)]

        def proj_kv(j, n):
            c = yield from project("kv", j, n, lambda k: jnp.concatenate(
                [cq[k, 2 * j], cq[k, 2 * j + 1]], axis=0), lambda k: wkv[k])
            if c is not None:
                c = blocks(c, lambda cg: ups[cg][:1], _riffle)
                for cg in range(4):
                    for e in range(2):
                        (vs, ks)[cg >> 1][(cg & 1, 2 * j + e)] = c[cg][e]

        def proj_q(g, n):
            c = yield from project("q", g, n, x_rows(4 * g + 2 * (p & 1), 2), lambda k: wq49[k])
            if c is not None:
                c = blocks(c, lambda cg: QSCALE, _pack)
                for h in range(2):
                    for e in range(2):
                        old = qn[h, g, e]
                        for b in range(2):
                            qs[(h, 4 * g + 2 * b + e)] = jnp.where((p & 1) == b, c[h][e], old)
                        qn[h, g, e] = c[2 + h][e]

        def halves(d, h, js):
            return jnp.concatenate([d[(h, j >> 1)][QQ * (j & 1):QQ * (j & 1) + QQ] for j in js],
                                   axis=0)

        def late(x, y, op):
            return jnp.concatenate([x[:HQ], op(x[HQ:], y)], axis=0)

        def unit(h, i):
            return halves(qs, h, (2 * (i & ~1) + (i & 1), 2 * (i | 1) + (i & 1)))

        def first(i):
            t = jnp.concatenate([mm(("kq", h, i), halves(ks, h, (0,)), unit(h, i), NT)
                                 for h in range(2)], axis=0).T
            keep = [col < HQ, col >= HQ]
            top = [col <= row, causal & keep[1]] if i == 0 else keep
            return [jnp.concatenate([jnp.where(a, t[:HQ], NEG), jnp.where(b, t[HQ:], NEG)], axis=0)
                    for a, b in zip(top, keep)]

        def qk(h, i, dep):
            off = 1 - (i & 1)
            q = unit(h, i)
            if dep is not None:
                q = jnp.where(never, done[(h, dep)], q)
            ch = []
            if i:
                ch = _lane_chunks(mm(("qk", h, i), q, halves(ks, h, range(off, off + 2 * i)),
                                     NT, 512))
                ch[-1] = jnp.concatenate([jnp.where(causal, ch[-1][:HQ], NEG), ch[-1][HQ:]],
                                         axis=0)
            ex = mm(("qx", h, i), q[QQ:], halves(ks, h, (off + 2 * i, off + 2 * i + 1)), NT)
            return ch, jnp.where(causal, ex, NEG)

        def softmax_pv(h, i, ch, ex):
            off = 1 - (i & 1)
            m = jnp.max(late(_fold(ch, jnp.maximum), ex, jnp.maximum), axis=1, keepdims=True)
            pe = jnp.exp2(ex - m[HQ:])
            ps = [jnp.exp2(c - m) for c in ch]
            lp = late(ps[0], pe, jnp.add)
            for j in range(1, len(ch)):
                lp = lp + ps[j]
                if TIE and (j % TIE == TIE - 1 or j == len(ch) - 1):
                    ps[j] = jnp.where(never, lp, ps[j])
            pb = jnp.concatenate(ps, axis=1).astype(BF16)
            vv = [halves(vs, h, range(off, off + 2 * i))] if i else []
            v0 = [halves(vs, e, (0,)) for e in range(2 * off)]
            vv = jnp.concatenate(v0 + vv, axis=0)
            o = mm(("pv", h, i), pb, vv)
            o = late(o, mm(("px", h, i), pe.astype(BF16),
                           halves(vs, h, (off + 2 * i, off + 2 * i + 1))), jnp.add)
            if i >= LDEP:
                lp = jnp.where(never, o, lp)
            l = jnp.sum(lp, axis=1, keepdims=True)
            r = pl.reciprocal(l, approx=True)
            r = r * (2.0 - l * r)
            cn = _pack(o * r)
            done[(h, i)] = cn
            if FA <= i < NQ - 1:
                if i + 3 < NQ:
                    site = ("kv", (i + 1) // 2 + 1, KVS * ((i + 1) & 1) + (F0, FD)[h])
                else:
                    site = ("bo", 0, 7 * (i + 3 - NQ) * BOP[0] + 8 * h)
                sched.pending.setdefault(site, []).append(cn)
            for e in range(2):
                ctx[2 * p + h, pl.ds(((i & ~1) + e) * HQ + QQ * (i & 1), QQ), :] = (
                    cn[QQ * e:QQ * e + QQ])

        head = dict(bv=proj_bv(), kv=proj_kv(0, 7), q=proj_q(0, 7))
        for site in _head():
            next(head[site[0]], None)
        lead = {}
        for i in range(NQ):
            dep = i - DEP if DEP <= i < FA + DEP else None
            for k in range(i, i + VL + 1):
                if k < NQ and not k & 1 and k not in lead and (0, k) in qs:
                    lead[k] = first(k)
            sx = [qk(h, i, dep) for h in range(2)]
            if i + 2 < NQ:
                list(proj_kv(i // 2 + 1, 7 if i & 1 else KVS // 7))
                if i < 6:
                    list(proj_q(i // 2 + 1, 7 if i & 1 else QS // 7))
            else:
                proj_bo(BOP[i + 2 - NQ])
            for h in range(2):
                c0 = [lead[i][h]] if i in lead else []
                softmax_pv(h, i, c0 + sx[h][0], sx[h][1])
        proj_bo(BOP[2])
        sched.finish()
        return carry

    jax.lax.fori_loop(0, NP, p2_body, 0)

    gw = gw_ref[...].astype(F32)
    plan3 = _plan3()
    cab = (ca0, ca1)

    def p3_body(i, carry):
        r0 = pl.multiple_of(i * TO, TO)
        h0 = pl.multiple_of(i * (TO // 2), TO // 2)
        never = i > S

        def ctx_words(m, u, r, n):
            return [[ctx[4 * u + 2 * (q & 1) + (e & 1),
                         pl.ds(h0 + _zero(i, m) * 8 + ((2 * (q >> 1) + (e >> 1)) * QQ + r), n), :]
                     for e in range(4)] for q in range(4)]

        def operands(k, u, r, gate):
            m = ORDER[k]
            cw = [[gate(w) for w in q] for q in ctx_words(m, u, r, 8)]
            for n, w in enumerate(_words49(_lhs7, cw, m)):
                if not (m in (2, 3) and n in (2, 3)):
                    cab[k & 1][n, pl.ds(r, 8), pl.ds(u * 128, 128)] = w
            return [], 0, lambda: cab[k & 1][_zero(i, 0), pl.ds(r, 8), pl.ds(u * 128, 128)]

        def gate_rows(r, gate):
            gs = _fold([_bf(gate(xs_u[j, pl.ds(h0 + r, 8), :])).astype(F32) * gw[j:j + 1]
                        for j in range(8)], jnp.add)
            g = jax.nn.sigmoid(jnp.sum(gs, axis=1, keepdims=True))
            g_s[pl.ds(2 * r, 16), :] = jnp.broadcast_to(g, (16, 128))
            return [], 0, lambda: pltpu.bitcast(g_s[blk(r // 4 + _zero(i, 0), 8), :], U32)

        pr = {}

        def mix(q, e, cc, gate):
            off = (2 * (q >> 1) + (e >> 1)) * HQ
            ch = 4 * cc + 2 * (q & 1) + (e & 1)
            a = _combine(lambda m: pr.get(m, pr[2])[e][:, cc * 128:(cc + 1) * 128])[q]
            g = gate(g_s[pl.ds(off, HQ), :])
            b = qk_b[ch, pl.ds(r0 + (PAD + off), HQ), :]
            out_s[pl.ds(r0 + off, HQ), pl.ds(ch * 128, 128)] = (g * a + (1.0 - g) * b).astype(BF16)
            return [], 0, lambda: pltpu.bitcast(
                out_s[blk(i * (TO // 16) + off // 16 + _zero(i, 0), 16), pl.ds(ch * 128, 128)], U32)

        sched = _Sched(never, plan3, dict(
            a=[part(operands, k, u, r) for k in range(1, 7) for u in range(HA // 4)
               for r in range(0, QQ, 8)],
            g=[part(gate_rows, r) for r in range(0, TO // 2, 8)],
            m=[part(mix, q, e, cc) for q in (1, 2, 0) for e in range(4) for cc in range(2)]))
        first = [[_words49(_lhs7, ctx_words(ORDER[0], u, 0, QQ), ORDER[0])[n]
                  for u in range(HA // 4)] for n in range(7)]

        def inner(m, n):
            k = ORDER.index(m)
            res = []
            for e in range(2):
                us = range(4 * e, 4 * e + 4)
                if m in (2, 3) and n in (2, 3):
                    lhs = jnp.concatenate([ctx_words(m, u, 0, QQ)[3 * (m - 2)][3 * (n - 2)]
                                           for u in us], axis=1)
                elif k == 0:
                    lhs = jnp.concatenate([first[n][u] for u in us], axis=1)
                else:
                    lhs = lambda: cab[k & 1][n, :, pl.ds(e * 512, 512)]
                rhs = jnp.concatenate([wo49[7 * m + n, cc, pl.ds(e * 256, 256), :]
                                       for cc in range(2)], axis=1)
                res.append(sched.mm((k, 2 * ORDER.index(n) + e), lhs, rhs))
                if (k, 2 * ORDER.index(n) + e) == (6, P3D):
                    for d in cp_out(i, 0):
                        d.start()
            return res[0] + res[1]

        for m in ORDER:
            pr[m] = _combine(lambda n: inner(m, n))
        sched.finish()
        for e in (1, 2, 0, 3):
            for cc in range(2):
                mix(3, e, cc, lambda x: x)
        for d in cp_out(i, 1):
            d.start()
        return carry

    jax.lax.fori_loop(0, S // TO, p3_body, 0)
    for d in cp_p(NP) + cp_p(NP + 1):
        d.wait()
    for i in range(S // TO):
        for d in cp_out(i, 0) + cp_out(i, 1):
            d.wait()


@jax.jit
def pallas_gated_mix__compressed_kv_cla__sliding_local_dilated__prompt_kernel(
    A_x: jax.Array,
    A_c_kv: jax.Array,
    A_w_q: jax.Array,
    A_w_uk: jax.Array,
    A_w_uv: jax.Array,
    A_w_o: jax.Array,
    B_x: jax.Array,
    B_wqkv: jax.Array,
    B_wo: jax.Array,
    gate_w: jax.Array,
):
    del B_x
    any_spec = pl.BlockSpec(memory_space=pl.ANY)
    out = pl.pallas_call(
        _kernel,
        in_specs=[any_spec] * 9,
        out_specs=any_spec,
        out_shape=jax.ShapeDtypeStruct((S, M), BF16),
        scratch_shapes=[
            pltpu.VMEM((9, S // 2, 128), U32),
            pltpu.VMEM((2, HQ, M), U32),
            pltpu.VMEM((2, HQ, DC), U32),
            pltpu.VMEM((2, 128, M), BF16),
            pltpu.VMEM((2, 4, 16, M), BF16),
            pltpu.VMEM((2, 4, 16, M), U32),
            pltpu.VMEM((3, 2 * DC, 128), U32),
            pltpu.VMEM((4, M, 128), U32),
            pltpu.VMEM((2, 2 * DA, M // 2), U32),
            pltpu.VMEM((8, 64, 128), U32),
            pltpu.VMEM((49, NQ, 32, 128), U32),
            pltpu.VMEM((49, NQ, 16, 128), U32),
            pltpu.VMEM((49, 2, M // 8, 128), U32),
            pltpu.VMEM((49, 2, M // 8, 128), U32),
            pltpu.VMEM((49, 2, NP * QQ, 128), U32),
            pltpu.VMEM((49, HQ, 128), U32),
            pltpu.VMEM((49, TQ, 128), U32),
            pltpu.VMEM((4, 8, 128), F32),
            pltpu.VMEM((4, DC // SCR * 8 + 16, 128), jnp.int32),
            pltpu.VMEM((2, 4, 2, HQ, 128), U32),
            pltpu.VMEM((16, S + PAD, 128), F32),
            pltpu.VMEM((8, TQ + PAD, 128), F32),
            pltpu.VMEM((WIN, TQ, 128), F32),
            pltpu.VMEM((WIN, TQ, 128), F32),
            pltpu.VMEM((8, TQ, 128), F32),
            pltpu.VMEM((49, 2, 16, 128), U32),
            pltpu.VMEM((HA, S // 2, 128), U32),
            pltpu.VMEM((7, QQ, M), U32),
            pltpu.VMEM((7, QQ, M), U32),
            pltpu.VMEM((TO, 128), F32),
            pltpu.VMEM((S, M), BF16),
            pltpu.VMEM((8, 128), BF16),
            pltpu.SemaphoreType.DMA((2,)),
            pltpu.SemaphoreType.DMA((2,)),
            pltpu.SemaphoreType.DMA((5,)),
        ],
        compiler_params=pltpu.CompilerParams(vmem_limit_bytes=120 * 1024 * 1024,
                                             disable_bounds_checks=True),
    )(
        A_x.reshape(S, M),
        A_c_kv.reshape(S, DC),
        A_w_q,
        A_w_uk,
        A_w_uv,
        A_w_o.reshape(HA * DA, M),
        B_wqkv.reshape(2, M // 2, 3 * M),
        B_wo.reshape(HB // 2, 2, DB, M),
        gate_w.reshape(8, 128),
    )
    return out.reshape(1, S, M)
```
